```python
import jax
import jax.numpy as jnp

def _softmax(x, axis=-1):
    return jax.nn.softmax(x, axis=axis)

def _gelu(x):
    return jax.nn.gelu(x, approximate=True)

def _silu(x):
    return jax.nn.silu(x)

def _sigmoid(x):
    return jax.nn.sigmoid(x)

def _layernorm(x, axis=-1, eps=1e-05):
    m = jnp.mean(x, axis=axis, keepdims=True)
    v = jnp.var(x, axis=axis, keepdims=True)
    return (x - m) / jnp.sqrt(v + eps)

def _scatter_add(tgt, idx, src, axis=0):
    return tgt.at[idx].add(src)

def _segment_sum(src, seg, n):
    return jax.ops.segment_sum(src, seg, n)

class _Rng:

    def __init__(self, key):
        self._k = key

    def _next(self):
        self._k, sub = jax.random.split(self._k)
        return sub

    def normal(self, shape):
        return jax.random.normal(self._next(), shape, dtype=jnp.bfloat16)

    def randint(self, lo, hi, shape):
        return jax.random.randint(self._next(), shape, lo, hi, dtype=jnp.int32)

    def uniform(self, shape, lo=0.0, hi=1.0):
        return jax.random.uniform(self._next(), shape, jnp.bfloat16, lo, hi)

    def permutation(self, n):
        return jax.random.permutation(self._next(), n)
kernel_name = 'concat_heads__memory_aug_recurrent_mem_tr__spectral_gfnet__prompt'

def setup_inputs():
    _rng = _Rng(jax.random.key(int.from_bytes(__import__("os").urandom(4), "little")))
    _w = lambda a: (lambda t: t.astype(jnp.bfloat16) if jnp.issubdtype(t.dtype, jnp.floating) else t)(jnp.asarray(a))

    def _A_setup():
        B, S, Dm = (1, 2048, 1024)
        H, Dh = (32, 128)
        M, seg = (8, 32)
        seg = min(seg, S)
        S = S // seg * seg
        return {'x': _w((lambda *s: _rng.normal(s) * 0.05)(B, S, Dm)), 'mem0': _w((lambda *s: _rng.normal(s) * 0.05)(B, M, Dm)), 'Wq': _w((lambda *s: _rng.normal(s) * 0.05)(Dm, H, Dh) * Dm ** (-0.5)), 'Wk': _w((lambda *s: _rng.normal(s) * 0.05)(Dm, H, Dh) * Dm ** (-0.5)), 'Wv': _w((lambda *s: _rng.normal(s) * 0.05)(Dm, H, Dh) * Dm ** (-0.5)), 'Wo': _w((lambda *s: _rng.normal(s) * 0.05)(H, Dh, Dm) * (H * Dh) ** (-0.5)), 'seg_len': seg}
    _A_in = _A_setup()

    def _B_setup():
        B, S, D = (1, 2048, 1024)
        Df = D // 2 + 1
        return {'x': _w((lambda *s: _rng.normal(s) * 0.05)(B, S, D)), 'w_r': _w((lambda *s: _rng.normal(s) * 0.05)(S, Df) * 0.02), 'w_i': _w((lambda *s: _rng.normal(s) * 0.05)(S, Df) * 0.02)}
    _B_in = _B_setup()
    return {'A_x': _A_in['x'], 'A_mem0': _A_in['mem0'], 'A_Wq': _A_in['Wq'], 'A_Wk': _A_in['Wk'], 'A_Wv': _A_in['Wv'], 'A_Wo': _A_in['Wo'], 'A_seg_len': _A_in['seg_len'], 'B_x': _B_in['x'], 'B_w_r': _B_in['w_r'], 'B_w_i': _B_in['w_i']}

def reference(A_x, A_mem0, A_Wq, A_Wk, A_Wv, A_Wo, A_seg_len, B_x, B_w_r, B_w_i):

    def _A_ref(x, mem0, Wq, Wk, Wv, Wo, seg_len):
        B, S, Dm = x.shape
        H, Dh = (Wq.shape[1], Wq.shape[2])
        M = mem0.shape[1]
        scale = Dh ** (-0.5)
        n_seg = S // seg_len
        L = M + seg_len
        idx = jnp.arange(L)
        mask = (idx[:, None] < M) | (idx[:, None] >= idx[None, :])
        mem = mem0
        outs = []
        for s in range(n_seg):
            xs = x[:, s * seg_len:(s + 1) * seg_len, :].copy()
            h = jnp.concatenate([mem, xs], axis=1)
            q = jnp.einsum('btd,dhe->bhte', h, Wq)
            k = jnp.einsum('btd,dhe->bhte', h, Wk)
            v = jnp.einsum('btd,dhe->bhte', h, Wv)
            scores = jnp.einsum('bhqe,bhke->bhqk', q, k) * scale
            scores = jnp.where(mask[None, None], scores, -1000000000.0)
            p = _softmax(scores, axis=-1)
            o = jnp.einsum('bhqk,bhke->bhqe', p, v)
            o = jnp.einsum('bhte,hed->btd', o, Wo)
            mem = o[:, :M, :].copy()
            outs.append(o[:, M:, :])
        return jnp.concatenate(outs, axis=1)

    def _B_ref(x, w_r, w_i):
        B, S, D = x.shape
        X = (lambda x, axes=(-2, -1): jnp.fft.rfft2(x.astype(jnp.float32), axes=axes))(x, axes=(-2, -1))
        W = w_r + 1j * w_i
        X = X * W
        y = (lambda x, s, axes=(-2, -1): jnp.fft.irfft2(x, s=s, axes=axes).astype(jnp.bfloat16))(X, (S, D), axes=(-2, -1))
        return y
    a = _A_ref(A_x, A_mem0, A_Wq, A_Wk, A_Wv, A_Wo, A_seg_len)
    b = _B_ref(B_x, B_w_r, B_w_i)
    return jnp.concatenate([a, b], axis=-1)
```

```python
import math

import numpy as np
import jax
import jax.numpy as jnp
import jax.experimental.pallas as pl
import jax.experimental.pallas.tpu as pltpu

bf16 = jnp.bfloat16
f32 = jnp.float32
u32 = jnp.uint32

S, DM = 2048, 1024
H, DH = 32, 128
MEM, SEG = 8, 32
NSEG = S // SEG
SQH = math.sqrt(0.5)

_PAIRS = ((0, 4), (1, 7), (2, 6), (3, 5))
_DELTA = ((0, 1, 2, 3), (0, 1, 4, 5), (0, 1, 2, 3), (0, 1, 4, 5))


def _pack_rows(a):
    u = np.ascontiguousarray(a, dtype=np.float32).view(np.uint32).astype(np.uint64)
    b = ((u + 0x7FFF + ((u >> 16) & 1)) >> 16).astype(np.uint32)
    return (b[..., 0::2, :] | (b[..., 1::2, :] << 16)).astype(np.uint32)


def _tables():
    k2 = np.zeros((4, 128), np.int64)
    for t in range(4):
        for c in range(4):
            for mu in range(128):
                if mu % 8 in _PAIRS[t]:
                    k2[t, (mu + _DELTA[t][c]) % 128] = 128 * c + mu
    b = np.arange(128)[:, None]
    F = np.zeros((4, 256, 256))
    cw = np.full((4, 256), 2.0)
    for t in range(4):
        th = 2 * np.pi * ((b * k2[t][None, :]) % DM) / DM
        C, Sn = np.cos(th), np.sin(th)
        first = ((k2[t] % 8) == _PAIRS[t][0])[None, :]
        if t == 0:
            F[t, :128, :128] = np.where(first, C, 0)
            F[t, :128, 128:] = np.where(first, -Sn, 0)
            F[t, 128:, :128] = np.where(first, 0, C)
            F[t, 128:, 128:] = np.where(first, 0, -Sn)
            F[t, :128, 128] = (-1.0) ** np.arange(128)
            cw[t, 0] = 1.0
            cw[t, 128] = 1.0
        else:
            sg = np.where(first, 1.0, -1.0)
            F[t, :128, :128] = C
            F[t, 128:, :128] = -sg * Sn
            F[t, :128, 128:] = -Sn
            F[t, 128:, 128:] = -sg * C
    Finv = np.transpose(F * cw[:, None, :], (0, 2, 1)) / DM
    fd = np.stack([F, Finv]).reshape(2, 4, 256, 2, 128).transpose(0, 1, 3, 2, 4)
    fd = _pack_rows(fd).reshape(16, 128, 128)
    M = np.zeros((32, 128, 128))
    r = np.arange(64)[None, :]
    l = np.arange(64)[:, None]
    for j in range(32):
        th = 2 * np.pi * ((r * (j + 32 * l)) % S) / S
        C, Sn = np.cos(th), np.sin(th)
        M[j, :64, :64] = C
        M[j, :64, 64:] = Sn
        M[j, 64:, :64] = -Sn
        M[j, 64:, 64:] = C
    Minv = np.transpose(M, (0, 2, 1)) / S
    ms = _pack_rows(np.concatenate([M, Minv]))
    ang = 2 * np.pi * np.outer(np.arange(8), np.arange(4)) / 32
    tw = np.stack([np.cos(ang), np.sin(ang)], -1).reshape(-1).astype(np.float32)
    return fd, ms, tw


def _tobf(w):
    return pltpu.bitcast(w, bf16)


def _tou(w):
    return pltpu.bitcast(w, u32)


def _dot(a, b):
    return jnp.dot(a, b, preferred_element_type=f32)


def _r8_real(x):
    t0, t1 = x[0] + x[4], x[0] - x[4]
    t2, t3 = x[2] + x[6], x[2] - x[6]
    t4, t5 = x[1] + x[5], x[1] - x[5]
    t6, t7 = x[3] + x[7], x[3] - x[7]
    e0, e1 = t0 + t2, t0 - t2
    o0, o1 = t4 + t6, t4 - t6
    u, v = SQH * (t5 - t7), SQH * (t5 + t7)
    return [(e0 + o0, e0 - o0), (t1 + u, v + t3), (e1, o1), (t1 - u, v - t3)]


def _r8_real_t(g):
    (z0, z4), (a1, b1), (e1, o1), (a3, b3) = g
    e0, o0 = z0 + z4, z0 - z4
    t1, u = a1 + a3, a1 - a3
    v, t3 = b1 + b3, b1 - b3
    t5, t7 = SQH * (v + u), SQH * (v - u)
    t0, t2 = e0 + e1, e0 - e1
    t4, t6 = o0 + o1, o0 - o1
    return [t0 + t1, t4 + t5, t2 + t3, t6 + t7, t0 - t1, t4 - t5, t2 - t3, t6 - t7]


def _dft4(u):
    (r0, i0), (r1, i1), (r2, i2), (r3, i3) = u
    sr, si, dr, di = r0 + r2, i0 + i2, r0 - r2, i0 - i2
    tr, ti, er, ei = r1 + r3, i1 + i3, r1 - r3, i1 - i3
    return [(sr + tr, si + ti), (dr + ei, di - er), (sr - tr, si - ti), (dr - ei, di + er)]


def _dft8(x):
    a = [(x[p][0] + x[p + 4][0], x[p][1] + x[p + 4][1]) for p in range(4)]
    d = [(x[p][0] - x[p + 4][0], x[p][1] - x[p + 4][1]) for p in range(4)]
    ev = _dft4(a)
    (r0, i0), (r1, i1), (r2, i2), (r3, i3) = d
    b1r, b1i = SQH * (r1 + i1), SQH * (i1 - r1)
    b3r, n3i = SQH * (i3 - r3), SQH * (r3 + i3)
    sr, si, dr, di = r0 + i2, i0 - r2, r0 - i2, i0 + r2
    tr, ti, er, ei = b1r + b3r, b1i - n3i, b1r - b3r, b1i + n3i
    od = [(sr + tr, si + ti), (dr + ei, di - er), (sr - tr, si - ti), (dr - ei, di + er)]
    return [ev[0], od[0], ev[1], od[1], ev[2], od[2], ev[3], od[3]]


def _swap(x):
    return [(b, a) for (a, b) in x]


G = 4
NG = H // G
OSPLIT = 24


def _kernel(tw_ref, x_hbm, mem_hbm, wq_hbm, wk_hbm, wv_hbm, wo_hbm, bx_hbm, wr_hbm, wi_hbm,
            fd_hbm, ms_hbm, out_hbm,
            xo_ref, mem_ref, raw_ref, wqkv_ref, woraw_ref, wo_ref, xc_ref, qkvc_ref, oc_ref,
            oall_ref, fill_ref, bx_ref, wr_ref, wi_ref, wp_ref, ub_ref, fd_ref, ms_ref,
            sem_in, sem_raw, sem_out):
    scale = DH ** -0.5
    w_hbm = (wq_hbm, wk_hbm, wv_hbm)

    def raw_copy(c):
        return pltpu.make_async_copy(
            w_hbm[c // 2].at[:, pl.ds((c % 2) * 16, 16), :], raw_ref.at[c % 2], sem_raw.at[c % 2])

    cp_x = pltpu.make_async_copy(x_hbm, xo_ref, sem_in.at[0])
    cp_mem = pltpu.make_async_copy(mem_hbm, mem_ref, sem_in.at[1])
    cp_wo = pltpu.make_async_copy(wo_hbm, woraw_ref, sem_in.at[2])
    cp_bx = pltpu.make_async_copy(bx_hbm, bx_ref, sem_in.at[3])
    cp_wr = pltpu.make_async_copy(wr_hbm, wr_ref, sem_in.at[4])
    cp_wi = pltpu.make_async_copy(wi_hbm, wi_ref, sem_in.at[5])
    cp_fd = pltpu.make_async_copy(fd_hbm, fd_ref, sem_in.at[6])
    cp_ms = pltpu.make_async_copy(ms_hbm, ms_ref, sem_in.at[7])

    raw_copy(0).start()
    cp_x.start()
    cp_mem.start()
    raw_copy(1).start()

    qi = jax.lax.broadcasted_iota(jnp.int32, (48, 128), 0)
    ki = jax.lax.broadcasted_iota(jnp.int32, (48, 128), 1)
    for par in range(2):
        def pos(i):
            return jnp.where(i < 32, i, i - 24 - 8 * par)
        lo = 40 - 8 * par
        q_all = ((qi >= 8) & (qi < 16)) | ((qi >= lo) & (qi < lo + 8))
        k_mem = (ki >= 8) & (ki < 16)
        k_out = ((ki >= lo) & (ki < lo + 8)) | (ki >= 48)
        keep = q_all | k_mem | (pos(qi) >= pos(ki))
        fill_ref[par] = jnp.where(k_out, -jnp.inf, jnp.where(keep, 0.0, -1e9)).astype(f32)

    def relayout(c, i, nd):
        slot = c % 2
        for blk in range(nd // 16):
            d0 = i * nd + blk * 16
            w0 = pl.multiple_of(i * (nd // 2) + blk * 8, 8)
            los, his = [], []
            for dd in range(8):
                a = _tou(raw_ref[slot, d0 + 2 * dd])
                b = _tou(raw_ref[slot, d0 + 2 * dd + 1])
                los.append((a & jnp.uint32(0xFFFF)) | (b << 16))
                his.append((a >> 16) | (b & jnp.uint32(0xFFFF0000)))
            lo = jnp.swapaxes(jnp.stack(los), 0, 1)
            hi = jnp.swapaxes(jnp.stack(his), 0, 1)
            for j in range(8):
                wqkv_ref[c * 16 + 2 * j, pl.ds(w0, 8), :] = lo[j]
                wqkv_ref[c * 16 + 2 * j + 1, pl.ds(w0, 8), :] = hi[j]

    def bulk_tile(n):
        xc = jnp.concatenate([_tobf(xc_ref[k]) for k in range(8)], axis=1)
        qkvc_ref[n] = _tou(_dot(xc, _tobf(wqkv_ref[n])).astype(bf16))

    raw_copy(0).wait()

    def rl0(i, carry):
        relayout(0, i, 64)
        return carry
    jax.lax.fori_loop(0, 16, rl0, 0)

    cp_x.wait()
    cp_mem.wait()

    def gather_c(i, carry):
        r0 = pl.multiple_of(i * 64, 64)
        w0 = pl.multiple_of(i * 8, 8)
        v = jnp.concatenate([xo_ref[pl.ds(r0 + 8, 8), :].astype(f32),
                             xo_ref[pl.ds(r0 + 40, 8), :].astype(f32)], axis=0).astype(bf16)
        for k in range(8):
            xc_ref[k, pl.ds(w0, 8), :] = _tou(v[:, k * 128:(k + 1) * 128])
        return carry
    jax.lax.fori_loop(0, NSEG // 2, gather_c, 0)
    xo_ref[8:16, :] = mem_ref[...]

    def repack_wo(i):
        for blk in range(16):
            r0 = pl.multiple_of(i * 1024 + blk * 64, 64)
            w0 = pl.multiple_of(i * 512 + blk * 32, 32)
            v = woraw_ref[pl.ds(r0, 64), :]
            for j in range(8):
                wo_ref[j, pl.ds(w0, 32), :] = _tou(v[:, j * 128:(j + 1) * 128])

    for c in range(6):
        if c + 1 < 6:
            raw_copy(c + 1).wait()
        if c + 2 < 6:
            raw_copy(c + 2).start()
        if c == 1:
            cp_wo.start()
        if c == 3:
            cp_bx.start()
            cp_fd.start()
            cp_wr.start()
            cp_wi.start()
            cp_ms.start()
        if c == 5:
            cp_wo.wait()

        def bulk(i, carry, c=c):
            for t in range(4):
                bulk_tile(c * 16 + i * 4 + t)
            if c + 1 < 6:
                relayout(c + 1, i, 256)
            else:
                repack_wo(i)
            return carry
        jax.lax.fori_loop(0, 4, bulk, 0)

    def step(s, carry):
        r0 = pl.multiple_of(s * SEG, SEG)
        c0 = pl.multiple_of((s // 2) * 8, 8)
        par = s % 2
        hm = xo_ref[pl.ds(r0, SEG), :]
        fill = fill_ref[par][:, :48]
        qkv, ps = {}, {}

        def do_qkv(g):
            for h in range(g * G, (g + 1) * G):
                for t in range(3):
                    y = _dot(hm, _tobf(wqkv_ref[t * H + h]))
                    qkv[(t, h)] = jnp.concatenate(
                        [y.astype(bf16), _tobf(qkvc_ref[t * H + h, pl.ds(c0, 8), :])], axis=0)

        def do_s(g):
            for h in range(g * G, (g + 1) * G):
                sc = jax.lax.dot_general(qkv[(0, h)], qkv[(1, h)], (((1,), (1,)), ((), ())),
                                         preferred_element_type=f32)
                sc = jnp.where(fill == 0.0, sc * scale, fill)
                e = jnp.exp(sc - jnp.max(sc, axis=1, keepdims=True))
                den = jnp.sum(e, axis=1, keepdims=True)
                r = pl.reciprocal(den, approx=True)
                r = r * (2.0 - den * r)
                ps[h] = (e * r).astype(bf16)

        def do_pv(g):
            for h in range(g * G, (g + 1) * G):
                o = _dot(ps[h], qkv[(2, h)])
                oall_ref[h] = _tou(o[:32].astype(bf16))
                oc_ref[h, s] = jnp.where(par == 0, o[32:40], o[40:48])

        def do_o(j, h0, h1):
            lhs = jnp.concatenate([_tobf(oall_ref[h]) for h in range(h0, h1)], axis=1)
            return _dot(lhs, _tobf(wo_ref[j, h0 * 64:h1 * 64, :]))

        for g in range(NG):
            do_qkv(g)
            if g >= 1:
                do_s(g - 1)
            if g >= 2:
                do_pv(g - 2)
        part = {}
        for j in range(0, 3):
            part[j] = do_o(j, 0, OSPLIT)
        do_s(NG - 1)
        do_pv(NG - 2)
        for j in range(3, 6):
            part[j] = do_o(j, 0, OSPLIT)
        do_pv(NG - 1)
        for j in range(6, 8):
            part[j] = do_o(j, 0, OSPLIT)
        rn = pl.multiple_of(jnp.minimum(s + 1, NSEG - 1) * SEG, SEG)
        for j in range(8):
            res = (do_o(j, OSPLIT, H) + part[j]).astype(bf16)
            xo_ref[pl.ds(r0, SEG), j * 128:(j + 1) * 128] = res
            xo_ref[pl.ds(rn + 8, 8), j * 128:(j + 1) * 128] = res[8:16]
        return carry
    jax.lax.fori_loop(0, NSEG, step, 0)

    def bulk_o(i, carry):
        s0 = pl.multiple_of(i * 16, 16)
        lhs = jnp.concatenate(
            [oc_ref[h, pl.ds(s0, 16)].reshape(128, 128).astype(bf16) for h in range(H)], axis=1)
        for j in range(8):
            res = _dot(lhs, _tobf(wo_ref[j]))
            for ss in range(16):
                rr = pl.multiple_of((s0 + ss) * SEG + 8, 8)
                xo_ref[pl.ds(rr, 8), j * 128:(j + 1) * 128] = res[ss * 8:(ss + 1) * 8].astype(bf16)
        return carry
    jax.lax.fori_loop(0, 4, bulk_o, 0)
    cp_oa = pltpu.make_async_copy(xo_ref, out_hbm.at[:, pl.ds(0, DM)], sem_out.at[0])
    cp_oa.start()

    cp_bx.wait()
    cp_fd.wait()
    lane0 = jax.lax.broadcasted_iota(jnp.int32, (64, 128), 1) == 0

    def ub_idx(t, ri, jq, p):
        return ((t * 2 + ri) * 4 + jq) * 8 + p

    def fmat(d, t):
        return jnp.concatenate([_tobf(fd_ref[d * 8 + t * 2]), _tobf(fd_ref[d * 8 + t * 2 + 1])], axis=1)

    def b_p1(p, carry):
        zs = []
        for q in range(4):
            rows = pl.multiple_of(q * 512 + p * 64, 64)
            xq = bx_ref[pl.ds(rows, 64), :].astype(f32)
            z = _r8_real([xq[:, a * 128:(a + 1) * 128] for a in range(8)])
            zs.append([jnp.concatenate([z[t][0].astype(bf16), z[t][1].astype(bf16)], axis=1)
                       for t in range(4)])
        cs = [(tw_ref[(p * 4 + jq) * 2], tw_ref[(p * 4 + jq) * 2 + 1]) for jq in range(4)]

        def emit(t, u):
            a = _dft4(u)
            for jq in range(4):
                re, im = a[jq]
                if jq > 0:
                    c, sn = cs[jq]
                    re, im = re * c + im * sn, im * c - re * sn
                ub_ref[ub_idx(t, 0, jq, p)] = re
                ub_ref[ub_idx(t, 1, jq, p)] = im

        for t in range(4):
            o = _dot(jnp.concatenate([zs[q][t] for q in range(4)], axis=0), fmat(0, t))
            u = [(o[q * 64:(q + 1) * 64, :128], o[q * 64:(q + 1) * 64, 128:]) for q in range(4)]
            if t == 0:
                emit(4, [(im, jnp.zeros_like(im)) for (_, im) in u])
                u = [(re, jnp.where(lane0, 0.0, im)) for (re, im) in u]
            emit(t, u)
        return carry
    jax.lax.fori_loop(0, 8, b_p1, 0)

    cp_wr.wait()
    cp_wi.wait()
    cp_ms.wait()
    res8 = jax.lax.broadcasted_iota(jnp.int32, (128, 128), 1) % 8

    def b_prep(lg, carry):
        rows = pl.multiple_of(lg * 256, 256)
        l0 = pl.multiple_of(lg * 8, 8)
        srcs = [[], []]
        for c in range(4):
            a = _tou(wr_ref[pl.ds(rows, 256), c * 128:(c + 1) * 128])
            b = _tou(wi_ref[pl.ds(rows, 256), c * 128:(c + 1) * 128])
            srcs[0].append((a << 16) | (b & jnp.uint32(0xFFFF)))
            srcs[1].append((a & jnp.uint32(0xFFFF0000)) | (b >> 16))
        for par in range(2):
            rolled = {}
            for t in range(4):
                v = None
                for c in range(4):
                    dl = _DELTA[t][c]
                    if (c, dl) not in rolled:
                        rolled[(c, dl)] = srcs[par][c] if dl == 0 else pltpu.roll(srcs[par][c], dl, 1)
                    if v is None:
                        v = rolled[(c, dl)]
                    else:
                        m = (res8 == (_PAIRS[t][0] + dl) % 8) | (res8 == (_PAIRS[t][1] + dl) % 8)
                        v = jnp.where(m, rolled[(c, dl)], v)
                v = jnp.swapaxes(v.reshape(8, 16, 128), 0, 1)
                for i in range(16):
                    wp_ref[t * 32 + 2 * i + par, pl.ds(l0, 8), :] = v[i]
        a = jnp.broadcast_to(wr_ref[pl.ds(rows, 256), 512:513].astype(f32), (256, 128))
        b = jnp.broadcast_to(wi_ref[pl.ds(rows, 256), 512:513].astype(f32), (256, 128))
        v = pltpu.bitcast(a, u32) | (pltpu.bitcast(b, u32) >> 16)
        v = jnp.swapaxes(v.reshape(8, 32, 128), 0, 1)
        for j in range(32):
            wp_ref[4 * 32 + j, pl.ds(l0, 8), :] = v[j]
        return carry
    jax.lax.fori_loop(0, 8, b_prep, 0)

    def b_p2(u, carry):
        t = u // 4
        jq = u % 4
        x = [(ub_ref[ub_idx(t, 0, jq, p)], ub_ref[ub_idx(t, 1, jq, p)]) for p in range(8)]
        tt = _dft8(x)
        v = []
        for jp in range(8):
            j = jq + 4 * jp
            rhs = jnp.concatenate([tt[jp][0].astype(bf16), tt[jp][1].astype(bf16)], axis=0)
            xx = _dot(_tobf(ms_ref[j]), rhs)
            xr, xi = xx[:64], xx[64:]
            w = wp_ref[t * 32 + j]
            wr = pltpu.bitcast(w & jnp.uint32(0xFFFF0000), f32)
            wi = pltpu.bitcast(w << 16, f32)
            rhs = jnp.concatenate([(xr * wr - xi * wi).astype(bf16),
                                   (xr * wi + xi * wr).astype(bf16)], axis=0)
            zz = _dot(_tobf(ms_ref[32 + j]), rhs)
            v.append((zz[:64], zz[64:]))
        a = _swap(_dft8(_swap(v)))
        for p in range(8):
            ub_ref[ub_idx(t, 0, jq, p)] = a[p][0]
            ub_ref[ub_idx(t, 1, jq, p)] = a[p][1]
        return carry
    jax.lax.fori_loop(0, 20, b_p2, 0)

    def b_p3(p, carry):
        cs = [(tw_ref[(p * 4 + jq) * 2], tw_ref[(p * 4 + jq) * 2 + 1]) for jq in range(4)]

        def fetch(t):
            a = []
            for jq in range(4):
                re, im = ub_ref[ub_idx(t, 0, jq, p)], ub_ref[ub_idx(t, 1, jq, p)]
                if jq > 0:
                    c, sn = cs[jq]
                    re, im = re * c - im * sn, im * c + re * sn
                a.append((re, im))
            return _swap(_dft4(_swap(a)))

        g = []
        for t in range(4):
            u = fetch(t)
            if t == 0:
                ny = fetch(4)
                u = [(u[q][0], jnp.where(lane0, ny[q][0], u[q][1])) for q in range(4)]
            lhs = jnp.concatenate(
                [jnp.concatenate([re.astype(bf16), im.astype(bf16)], axis=1) for (re, im) in u], axis=0)
            o = _dot(lhs, fmat(1, t))
            g.append((o[:, :128], o[:, 128:]))
        y = _r8_real_t(g)
        for q in range(4):
            rows = pl.multiple_of(q * 512 + p * 64, 64)
            for a in range(8):
                bx_ref[pl.ds(rows, 64), a * 128:(a + 1) * 128] = y[a][q * 64:(q + 1) * 64].astype(bf16)
        return carry
    jax.lax.fori_loop(0, 8, b_p3, 0)

    cp_ob = pltpu.make_async_copy(bx_ref, out_hbm.at[:, pl.ds(DM, DM)], sem_out.at[1])
    cp_ob.start()
    cp_oa.wait()
    cp_ob.wait()


@jax.jit
def _run(x, mem0, wq, wk, wv, wo, bx, w_r, w_i):
    fd, ms, tw = _tables()
    hbm = pl.BlockSpec(memory_space=pl.ANY)
    out = pl.pallas_call(
        _kernel,
        out_shape=jax.ShapeDtypeStruct((S, 2 * DM), bf16),
        in_specs=[pl.BlockSpec(memory_space=pltpu.SMEM)] + [hbm] * 11,
        out_specs=hbm,
        scratch_shapes=[
            pltpu.VMEM((S, DM), bf16),
            pltpu.VMEM((MEM, DM), bf16),
            pltpu.VMEM((2, DM, 16, DH), bf16),
            pltpu.VMEM((3 * H, DM // 2, DH), u32),
            pltpu.VMEM((H * DH, DM), bf16),
            pltpu.VMEM((8, H * DH // 2, 128), u32),
            pltpu.VMEM((8, 256, 128), u32),
            pltpu.VMEM((3 * H, 256, 128), u32),
            pltpu.VMEM((H, NSEG, 8, DH), f32),
            pltpu.VMEM((H, 16, DH), u32),
            pltpu.VMEM((2, 48, 128), f32),
            pltpu.VMEM((S, DM), bf16),
            pltpu.VMEM((S, DM // 2 + 1), bf16),
            pltpu.VMEM((S, DM // 2 + 1), bf16),
            pltpu.VMEM((160, 64, 128), u32),
            pltpu.VMEM((320, 64, 128), f32),
            pltpu.VMEM((16, 128, 128), u32),
            pltpu.VMEM((64, 64, 128), u32),
            pltpu.SemaphoreType.DMA((8,)),
            pltpu.SemaphoreType.DMA((2,)),
            pltpu.SemaphoreType.DMA((2,)),
        ],
        compiler_params=pltpu.CompilerParams(vmem_limit_bytes=120 * 1024 * 1024),
    )(jnp.asarray(tw), x.reshape(S, DM), mem0.reshape(MEM, DM), wq, wk, wv,
      wo.reshape(H * DH, DM), bx.reshape(S, DM), w_r, w_i, jnp.asarray(fd), jnp.asarray(ms))
    return out.reshape(1, S, 2 * DM)


def pallas_concat_heads__memory_aug_recurrent_mem_tr__spectral_gfnet__prompt_kernel(
    A_x: jax.Array,
    A_mem0: jax.Array,
    A_Wq: jax.Array,
    A_Wk: jax.Array,
    A_Wv: jax.Array,
    A_Wo: jax.Array,
    A_seg_len,
    B_x: jax.Array,
    B_w_r: jax.Array,
    B_w_i: jax.Array,
):
    if isinstance(A_seg_len, int):
        assert A_seg_len == SEG
    assert A_x.shape == (1, S, DM) and A_mem0.shape == (1, MEM, DM) and A_Wq.shape == (DM, H, DH)
    assert B_x.shape == (1, S, DM) and B_w_r.shape == (S, DM // 2 + 1)
    return _run(A_x, A_mem0, A_Wq, A_Wk, A_Wv, A_Wo, B_x, B_w_r, B_w_i)
```

```python
import math

import numpy as np
import jax
import jax.numpy as jnp
import jax.experimental.pallas as pl
import jax.experimental.pallas.tpu as pltpu

bf16 = jnp.bfloat16
f32 = jnp.float32
u32 = jnp.uint32

S, DM = 2048, 1024
H, DH = 32, 128
MEM, SEG = 8, 32
NSEG = S // SEG
SQH = math.sqrt(0.5)

_PAIRS = ((0, 4), (1, 7), (2, 6), (3, 5))


def _pack_rows(a):
    u = np.ascontiguousarray(a, dtype=np.float32).view(np.uint32).astype(np.uint64)
    b = ((u + 0x7FFF + ((u >> 16) & 1)) >> 16).astype(np.uint32)
    return (b[..., 0::2, :] | (b[..., 1::2, :] << 16)).astype(np.uint32)


def _tables():
    k2 = np.zeros((4, 128), np.int64)
    for t in range(4):
        odd = t % 2
        for lam in range(128):
            k = 2 * lam + odd
            if k % 8 not in _PAIRS[t]:
                k = 2 * (128 + 8 * (lam // 8) + (lam % 8 - 1 - odd) % 8) + odd
            assert k % 8 in _PAIRS[t]
            k2[t, lam] = k
    b = np.arange(128)[:, None]
    F = np.zeros((4, 256, 256))
    cw = np.full((4, 256), 2.0)
    for t in range(4):
        th = 2 * np.pi * ((b * k2[t][None, :]) % DM) / DM
        C, Sn = np.cos(th), np.sin(th)
        first = ((k2[t] % 8) == _PAIRS[t][0])[None, :]
        if t == 0:
            F[t, :128, :128] = np.where(first, C, 0)
            F[t, :128, 128:] = np.where(first, -Sn, 0)
            F[t, 128:, :128] = np.where(first, 0, C)
            F[t, 128:, 128:] = np.where(first, 0, -Sn)
            F[t, :128, 128] = (-1.0) ** np.arange(128)
            cw[t, 0] = 1.0
            cw[t, 128] = 1.0
        else:
            sg = np.where(first, 1.0, -1.0)
            F[t, :128, :128] = C
            F[t, 128:, :128] = -sg * Sn
            F[t, :128, 128:] = -Sn
            F[t, 128:, 128:] = -sg * C
    Finv = np.transpose(F * cw[:, None, :], (0, 2, 1)) / DM
    fd = np.stack([F, Finv]).reshape(2, 4, 256, 2, 128).transpose(0, 1, 3, 2, 4)
    fd = _pack_rows(fd).reshape(16, 128, 128)
    M = np.zeros((32, 128, 128))
    r = np.arange(64)[None, :]
    l = np.arange(64)[:, None]
    for j in range(32):
        th = 2 * np.pi * ((r * (j + 32 * l)) % S) / S
        C, Sn = np.cos(th), np.sin(th)
        M[j, :64, :64] = C
        M[j, :64, 64:] = Sn
        M[j, 64:, :64] = -Sn
        M[j, 64:, 64:] = C
    Minv = np.transpose(M, (0, 2, 1)) / S
    ms = _pack_rows(np.concatenate([M, Minv]))
    ang = 2 * np.pi * np.outer(np.arange(8), np.arange(4)) / 32
    tw = np.stack([np.cos(ang), np.sin(ang)], -1).reshape(-1).astype(np.float32)
    return fd, ms, tw


def _tobf(w):
    return pltpu.bitcast(w, bf16)


def _tou(w):
    return pltpu.bitcast(w, u32)


def _dot(a, b):
    return jnp.dot(a, b, preferred_element_type=f32)


def _r8_real(x):
    t0, t1 = x[0] + x[4], x[0] - x[4]
    t2, t3 = x[2] + x[6], x[2] - x[6]
    t4, t5 = x[1] + x[5], x[1] - x[5]
    t6, t7 = x[3] + x[7], x[3] - x[7]
    e0, e1 = t0 + t2, t0 - t2
    o0, o1 = t4 + t6, t4 - t6
    u, v = SQH * (t5 - t7), SQH * (t5 + t7)
    return [(e0 + o0, e0 - o0), (t1 + u, v + t3), (e1, o1), (t1 - u, v - t3)]


def _r8_real_t(g):
    (z0, z4), (a1, b1), (e1, o1), (a3, b3) = g
    e0, o0 = z0 + z4, z0 - z4
    t1, u = a1 + a3, a1 - a3
    v, t3 = b1 + b3, b1 - b3
    t5, t7 = SQH * (v + u), SQH * (v - u)
    t0, t2 = e0 + e1, e0 - e1
    t4, t6 = o0 + o1, o0 - o1
    return [t0 + t1, t4 + t5, t2 + t3, t6 + t7, t0 - t1, t4 - t5, t2 - t3, t6 - t7]


def _dft4(u):
    (r0, i0), (r1, i1), (r2, i2), (r3, i3) = u
    sr, si, dr, di = r0 + r2, i0 + i2, r0 - r2, i0 - i2
    tr, ti, er, ei = r1 + r3, i1 + i3, r1 - r3, i1 - i3
    return [(sr + tr, si + ti), (dr + ei, di - er), (sr - tr, si - ti), (dr - ei, di + er)]


def _dft8(x):
    a = [(x[p][0] + x[p + 4][0], x[p][1] + x[p + 4][1]) for p in range(4)]
    d = [(x[p][0] - x[p + 4][0], x[p][1] - x[p + 4][1]) for p in range(4)]
    ev = _dft4(a)
    (r0, i0), (r1, i1), (r2, i2), (r3, i3) = d
    b1r, b1i = SQH * (r1 + i1), SQH * (i1 - r1)
    b3r, n3i = SQH * (i3 - r3), SQH * (r3 + i3)
    sr, si, dr, di = r0 + i2, i0 - r2, r0 - i2, i0 + r2
    tr, ti, er, ei = b1r + b3r, b1i - n3i, b1r - b3r, b1i + n3i
    od = [(sr + tr, si + ti), (dr + ei, di - er), (sr - tr, si - ti), (dr - ei, di + er)]
    return [ev[0], od[0], ev[1], od[1], ev[2], od[2], ev[3], od[3]]


def _swap(x):
    return [(b, a) for (a, b) in x]


G = 4
NG = H // G
OSPLIT = 24
NEG = -1e9
N_L1, N_L2, N_L3 = 4, 20, 8


def _kernel(tw_ref, x_hbm, x3_hbm, mem_hbm, wq_hbm, wk_hbm, wv_hbm, wo_hbm, bx_hbm, wr_hbm, wi_hbm,
            fd_hbm, ms_hbm, out_hbm,
            xo_ref, mem_ref, xcraw_ref, raw_ref, w0_ref, w1_ref, w2_ref, w3_ref, w4_ref, w5_ref,
            woraw_ref, wo_ref, xc_ref, qkvc_ref, kve_ref,
            oall_ref, fille_ref, fillo_ref, bx_ref, wt_ref, wp_ref, ub_ref, fd_ref, ms_ref,
            sem_in, sem_raw, sem_w, sem_out):
    scale = DH ** -0.5
    w_hbm = (wq_hbm, wk_hbm, wv_hbm)
    w_refs = (w0_ref, w1_ref, w2_ref, w3_ref, w4_ref, w5_ref)

    def raw_copy(c, i=None):
        src = w_hbm[c // 2]
        if i is None:
            return pltpu.make_async_copy(
                src.at[:, pl.ds((c % 2) * 16, 16), :], raw_ref.at[c % 2], sem_raw.at[c % 2])
        return pltpu.make_async_copy(
            src.at[pl.ds(i * 256, 256), pl.ds((c % 2) * 16, 16), :],
            raw_ref.at[c % 2, pl.ds(i * 256, 256)], sem_raw.at[2 + i])

    cp_x = pltpu.make_async_copy(x_hbm, xo_ref, sem_in.at[0])
    cp_mem = pltpu.make_async_copy(mem_hbm, mem_ref, sem_in.at[1])
    cp_wo = pltpu.make_async_copy(wo_hbm, woraw_ref, sem_in.at[2])
    cp_bx = pltpu.make_async_copy(bx_hbm, bx_ref, sem_in.at[3])
    cp_xc = pltpu.make_async_copy(x3_hbm.at[:, pl.ds(8, 8), :], xcraw_ref, sem_in.at[4])
    cp_fd = pltpu.make_async_copy(fd_hbm, fd_ref, sem_in.at[5])
    cp_ms = pltpu.make_async_copy(ms_hbm, ms_ref, sem_in.at[6])
    cp_wt = [pltpu.make_async_copy(src.at[:, pl.ds(lg * 256, 256)], wt_ref.at[a * 8 + lg], sem_w.at[a * 8 + lg])
             for a, src in enumerate((wr_hbm, wi_hbm)) for lg in range(8)]

    cp_xc.start()
    for i in range(4):
        raw_copy(0, i).start()
    raw_copy(1).start()

    qi = jax.lax.broadcasted_iota(jnp.int32, (48, 128), 0)
    ki = jax.lax.broadcasted_iota(jnp.int32, (48, 128), 1)

    def between(v, lo, hi):
        return (v >= lo) & (v < hi)

    def table(keep, other):
        return jnp.where(other, -jnp.inf, jnp.where(keep, 0.0, NEG)).astype(f32)

    keep = between(qi, 8, 16) | between(ki, 8, 16) | (qi >= jnp.where(ki < 32, ki, ki - 24))
    fille_ref[...] = table(keep, ki >= 40)[:32]
    q_even = between(qi, 32, 40)
    k_even = between(ki, 32, 40) | (ki >= 48)
    qpos = jnp.where(qi < 32, qi, jnp.where(qi < 40, qi - 24, qi - 32))
    kpos = jnp.where(ki < 32, ki, jnp.where(ki < 40, ki - 24, jnp.where(ki < 48, ki - 32, ki - 48)))
    keep = between(qi, 8, 16) | between(ki, 8, 16) | (ki >= 56) | (qpos >= kpos)
    fillo_ref[...] = table(keep, (q_even != k_even) | (ki >= 64))

    def relayout(c, d_start, nd):
        slot = c % 2
        for blk in range(nd // 16):
            d0 = d_start + blk * 16
            w0 = pl.multiple_of(d_start // 2 + blk * 8, 8)
            los, his = [], []
            for dd in range(8):
                a = _tou(raw_ref[slot, d0 + 2 * dd])
                b = _tou(raw_ref[slot, d0 + 2 * dd + 1])
                los.append((a & jnp.uint32(0xFFFF)) | (b << 16))
                his.append((a >> 16) | (b & jnp.uint32(0xFFFF0000)))
            lo = jnp.swapaxes(jnp.stack(los), 0, 1)
            hi = jnp.swapaxes(jnp.stack(his), 0, 1)
            for j in range(8):
                w_refs[c][2 * j, pl.ds(w0, 8), :] = lo[j]
                w_refs[c][2 * j + 1, pl.ds(w0, 8), :] = hi[j]

    def repack_wo(r_start, nr):
        for blk in range(nr // 64):
            r0 = pl.multiple_of(r_start + blk * 64, 64)
            w0 = pl.multiple_of(r_start // 2 + blk * 32, 32)
            v = woraw_ref[pl.ds(r0, 64), :]
            for j in range(8):
                wo_ref[j, pl.ds(w0, 32), :] = _tou(v[:, j * 128:(j + 1) * 128])

    sub4 = jax.lax.broadcasted_iota(jnp.int32, (128, 256), 0) % 4

    def b_prep(lg):
        l0 = pl.multiple_of(lg * 8, 8)
        a = _tou(wt_ref[lg, 0:512, :])
        b = _tou(wt_ref[8 + lg, 0:512, :])
        ev = (a << 16) | (b & jnp.uint32(0xFFFF))
        od = (a & jnp.uint32(0xFFFF0000)) | (b >> 16)
        evr = pltpu.roll(ev[128:].reshape(16, 8, 256), 1, 1).reshape(128, 256)
        odr = pltpu.roll(od[128:].reshape(16, 8, 256), 2, 1).reshape(128, 256)
        m_e = (sub4 == 0) | (sub4 == 2)
        m_o = (sub4 == 0) | (sub4 == 3)
        na = jnp.broadcast_to(wt_ref[lg, 512:513, :].astype(f32), (128, 256))
        nb = jnp.broadcast_to(wt_ref[8 + lg, 512:513, :].astype(f32), (128, 256))
        tiles = [jnp.where(m_e, ev[:128], evr), jnp.where(m_o, od[:128], odr),
                 jnp.where(m_e, evr, ev[:128]), jnp.where(m_o, odr, od[:128]),
                 pltpu.bitcast(na, u32) | (pltpu.bitcast(nb, u32) >> 16)]
        for t in range(5):
            v = jnp.swapaxes(tiles[t].T.reshape(8, 32, 128), 0, 1)
            for j in range(32):
                wp_ref[t * 32 + j, pl.ds(l0, 8), :] = v[j]

    cp_xc.wait()

    def gather_c(i, carry):
        w0 = pl.multiple_of(i * 8, 8)
        v = jnp.concatenate([xcraw_ref[2 * i].astype(f32), xcraw_ref[2 * i + 1].astype(f32)],
                            axis=0).astype(bf16)
        for k in range(8):
            xc_ref[k, pl.ds(w0, 8), :] = _tou(v[:, k * 128:(k + 1) * 128])
        return carry
    jax.lax.fori_loop(0, NSEG // 2, gather_c, 0)

    for i in range(4):
        raw_copy(0, i).wait()

        def rl0(k, carry, i=i):
            relayout(0, i * 256 + k * 64, 64)
            return carry
        jax.lax.fori_loop(0, 4, rl0, 0)

    for c in range(6):
        if c + 1 < 6:
            raw_copy(c + 1).wait()
        if c + 2 < 6:
            raw_copy(c + 2).start()
        if c == 0:
            for cp in cp_wt:
                cp.start()
        if c == 1:
            cp_wo.start()
        if c == 2:
            for cp in cp_wt:
                cp.wait()
        if c == 3:
            cp_x.start()
            cp_mem.start()
        if c == 4:
            cp_bx.start()
            cp_fd.start()
            cp_ms.start()
        if c == 5:
            cp_wo.wait()

        def bulk(i, carry, c=c):
            xc = jnp.concatenate([_tobf(xc_ref[k]) for k in range(8)], axis=1)
            for t in range(8):
                n = i * 8 + t
                qkvc_ref[c * 16 + n] = _tou(_dot(xc, _tobf(w_refs[c][n])).astype(bf16))
            if c + 1 < 6:
                relayout(c + 1, i * 512, 512)
            else:
                repack_wo(i * 2048, 2048)
            if c >= 2:
                b_prep((c - 2) * 2 + i)
            return carry
        jax.lax.fori_loop(0, 2, bulk, 0)

    cp_x.wait()
    cp_mem.wait()
    cp_bx.wait()
    cp_fd.wait()
    cp_ms.wait()

    lane0 = jax.lax.broadcasted_iota(jnp.int32, (64, 128), 1) == 0

    def ub_idx(t, ri, jq, p):
        return ((t * 2 + ri) * 4 + jq) * 8 + p

    def fmat(d, t):
        return jnp.concatenate([_tobf(fd_ref[d * 8 + t * 2]), _tobf(fd_ref[d * 8 + t * 2 + 1])], axis=1)

    def b_p1(p):
        zs = []
        for q in range(4):
            rows = pl.multiple_of(q * 512 + p * 64, 64)
            xq = bx_ref[pl.ds(rows, 64), :].astype(f32)
            z = _r8_real([xq[:, a * 128:(a + 1) * 128] for a in range(8)])
            zs.append([jnp.concatenate([z[t][0].astype(bf16), z[t][1].astype(bf16)], axis=1)
                       for t in range(4)])
        cs = [(tw_ref[(p * 4 + jq) * 2], tw_ref[(p * 4 + jq) * 2 + 1]) for jq in range(4)]

        def emit(t, u):
            a = _dft4(u)
            for jq in range(4):
                re, im = a[jq]
                if jq > 0:
                    c, sn = cs[jq]
                    re, im = re * c + im * sn, im * c - re * sn
                ub_ref[ub_idx(t, 0, jq, p)] = re
                ub_ref[ub_idx(t, 1, jq, p)] = im

        for t in range(4):
            o = _dot(jnp.concatenate([zs[q][t] for q in range(4)], axis=0), fmat(0, t))
            u = [(o[q * 64:(q + 1) * 64, :128], o[q * 64:(q + 1) * 64, 128:]) for q in range(4)]
            if t == 0:
                emit(4, [(im, jnp.zeros_like(im)) for (_, im) in u])
                u = [(re, jnp.where(lane0, 0.0, im)) for (re, im) in u]
            emit(t, u)

    def b_p2_fwd(u):
        t = u // 4
        jq = u % 4
        x = [(ub_ref[ub_idx(t, 0, jq, p)], ub_ref[ub_idx(t, 1, jq, p)]) for p in range(8)]
        tt = _dft8(x)
        ys = []
        for jp in range(8):
            j = jq + 4 * jp
            rhs = jnp.concatenate([tt[jp][0].astype(bf16), tt[jp][1].astype(bf16)], axis=0)
            xx = _dot(_tobf(ms_ref[j]), rhs)
            xr, xi = xx[:64], xx[64:]
            w = wp_ref[t * 32 + j]
            wr = pltpu.bitcast(w & jnp.uint32(0xFFFF0000), f32)
            wi = pltpu.bitcast(w << 16, f32)
            ys.append(jnp.concatenate([(xr * wr - xi * wi).astype(bf16),
                                       (xr * wi + xi * wr).astype(bf16)], axis=0))
        return ys

    def b_p2_inv(u, ys):
        t = u // 4
        jq = u % 4
        v = []
        for jp in range(8):
            zz = _dot(_tobf(ms_ref[32 + jq + 4 * jp]), ys[jp])
            v.append((zz[:64], zz[64:]))
        a = _swap(_dft8(_swap(v)))
        for p in range(8):
            ub_ref[ub_idx(t, 0, jq, p)] = a[p][0]
            ub_ref[ub_idx(t, 1, jq, p)] = a[p][1]

    def b_p3(p):
        cs = [(tw_ref[(p * 4 + jq) * 2], tw_ref[(p * 4 + jq) * 2 + 1]) for jq in range(4)]

        def fetch(t):
            a = []
            for jq in range(4):
                re, im = ub_ref[ub_idx(t, 0, jq, p)], ub_ref[ub_idx(t, 1, jq, p)]
                if jq > 0:
                    c, sn = cs[jq]
                    re, im = re * c - im * sn, im * c + re * sn
                a.append((re, im))
            return _swap(_dft4(_swap(a)))

        g = []
        for t in range(4):
            u = fetch(t)
            if t == 0:
                ny = fetch(4)
                u = [(u[q][0], jnp.where(lane0, ny[q][0], u[q][1])) for q in range(4)]
            lhs = jnp.concatenate(
                [jnp.concatenate([re.astype(bf16), im.astype(bf16)], axis=1) for (re, im) in u], axis=0)
            o = _dot(lhs, fmat(1, t))
            g.append((o[:, :128], o[:, 128:]))
        y = _r8_real_t(g)
        for q in range(4):
            rows = pl.multiple_of(q * 512 + p * 64, 64)
            for a in range(8):
                bx_ref[pl.ds(rows, 64), a * 128:(a + 1) * 128] = y[a][q * 64:(q + 1) * 64].astype(bf16)

    def b_out(p):
        for q in range(4):
            rows = pl.multiple_of(q * 512 + p * 64, 64)
            pltpu.make_async_copy(bx_ref.at[pl.ds(rows, 64), :],
                                  out_hbm.at[pl.ds(rows, 64), pl.ds(DM, DM)], sem_out.at[1]).start()

    def step(pp, odd, mem, mid=None):
        r0 = pl.multiple_of(pp * 64 + 32 * odd, SEG)
        c0 = pl.multiple_of(pp * 8, 8)
        xs = xo_ref[pl.ds(r0, SEG), :]
        x_lo = xs[0:8].astype(f32)
        hm = jnp.concatenate(
            [jnp.concatenate([x_lo, jnp.concatenate(mem, axis=1)], axis=0).astype(bf16), xs[16:32]], axis=0)
        fill = fillo_ref[:, 0:64] if odd else fille_ref[:, 0:48]
        nrow = 48 if odd else 32
        qkv, ps = {}, {}

        def do_qkv(g):
            for h in range(g * G, (g + 1) * G):
                for t in range(3):
                    y = _dot(hm, _tobf(w_refs[t * 2 + h // 16][h % 16])).astype(bf16)
                    parts = [y]
                    if odd or t > 0:
                        parts.append(_tobf(qkvc_ref[t * H + h, pl.ds(c0, 8), :]))
                    if t > 0:
                        if odd:
                            parts.append(_tobf(kve_ref[(t - 1) * H + h]))
                        else:
                            kve_ref[(t - 1) * H + h] = _tou(y[0:16])
                    qkv[(t, h)] = jnp.concatenate(parts, axis=0) if len(parts) > 1 else y

        def do_s(g):
            for h in range(g * G, (g + 1) * G):
                sc = jax.lax.dot_general(qkv[(0, h)], qkv[(1, h)], (((1,), (1,)), ((), ())),
                                         preferred_element_type=f32)
                sc = jnp.where(fill == 0.0, sc * scale, fill)
                e = jnp.exp(sc - jnp.max(sc, axis=1, keepdims=True))
                den = jnp.sum(e, axis=1, keepdims=True)
                r = pl.reciprocal(den, approx=True)
                r = r * (2.0 - den * r)
                ps[h] = (e * r).astype(bf16)

        def do_pv(g):
            for h in range(g * G, (g + 1) * G):
                oall_ref[h, 0:nrow // 2] = _tou(_dot(ps[h], qkv[(2, h)]).astype(bf16))

        def do_o(j, h0, h1):
            lhs = jnp.concatenate([_tobf(oall_ref[h, 0:nrow // 2]) for h in range(h0, h1)], axis=1)
            return _dot(lhs, _tobf(wo_ref[j, h0 * 64:h1 * 64, :]))

        for g in range(NG):
            do_qkv(g)
            if g >= 1:
                do_s(g - 1)
            if g >= 2:
                do_pv(g - 2)
            if g == 3 and mid is not None:
                mid()
        part = {}
        for j in range(0, 3):
            part[j] = do_o(j, 0, OSPLIT)
        do_s(NG - 1)
        do_pv(NG - 2)
        for j in range(3, 6):
            part[j] = do_o(j, 0, OSPLIT)
        do_pv(NG - 1)
        for j in range(6, 8):
            part[j] = do_o(j, 0, OSPLIT)
        new_mem = []
        for j in range(8):
            cols = slice(j * 128, (j + 1) * 128)
            res = do_o(j, OSPLIT, H) + part[j]
            new_mem.append(res[8:16])
            if odd:
                xo_ref[pl.ds(r0, SEG), cols] = jnp.concatenate(
                    [res[0:8], res[40:48], res[16:32]], axis=0).astype(bf16)
                xo_ref[pl.ds(r0 - 24, 8), cols] = res[32:40].astype(bf16)
            else:
                xo_ref[pl.ds(r0, SEG), cols] = res.astype(bf16)
        return new_mem

    def a_out(pp):
        rows = pl.multiple_of(pp * 64, 64)
        pltpu.make_async_copy(xo_ref.at[pl.ds(rows, 64), :],
                              out_hbm.at[pl.ds(rows, 64), pl.ds(0, DM)], sem_out.at[0]).start()

    def l1(i, mem):
        mem = step(i, 0, mem, mid=lambda: b_p1(2 * i))
        b_p1(2 * i + 1)
        mem = step(i, 1, mem)
        a_out(i)
        return mem

    def l2(i, mem):
        u = i - N_L1
        ys = []
        mem = step(i, 0, mem, mid=lambda: ys.extend(b_p2_fwd(u)))
        b_p2_inv(u, ys)
        mem = step(i, 1, mem)
        a_out(i)
        return mem

    def l3(i, mem):
        p = i - N_L1 - N_L2
        mem = step(i, 0, mem)
        b_p3(p)
        mem = step(i, 1, mem)
        b_out(p)
        a_out(i)
        return mem

    m0 = mem_ref[...].astype(f32)
    mem = [m0[:, j * 128:(j + 1) * 128] for j in range(8)]
    mem = jax.lax.fori_loop(0, N_L1, l1, mem)
    mem = jax.lax.fori_loop(N_L1, N_L1 + N_L2, l2, mem)
    mem = jax.lax.fori_loop(N_L1 + N_L2, NSEG // 2, l3, mem)

    pltpu.make_async_copy(xo_ref, out_hbm.at[:, pl.ds(0, DM)], sem_out.at[0]).wait()
    pltpu.make_async_copy(bx_ref, out_hbm.at[:, pl.ds(DM, DM)], sem_out.at[1]).wait()


@jax.jit
def _run(x, mem0, wq, wk, wv, wo, bx, w_r, w_i):
    fd, ms, tw = _tables()
    hbm = pl.BlockSpec(memory_space=pl.ANY)
    out = pl.pallas_call(
        _kernel,
        out_shape=jax.ShapeDtypeStruct((S, 2 * DM), bf16),
        in_specs=[pl.BlockSpec(memory_space=pltpu.SMEM)] + [hbm] * 12,
        out_specs=hbm,
        scratch_shapes=[
            pltpu.VMEM((S, DM), bf16),
            pltpu.VMEM((MEM, DM), bf16),
            pltpu.VMEM((NSEG, 8, DM), bf16),
            pltpu.VMEM((2, DM, 16, DH), bf16),
        ] + [pltpu.VMEM((16, DM // 2, DH), u32)] * 6 + [
            pltpu.VMEM((H * DH, DM), bf16),
            pltpu.VMEM((8, H * DH // 2, 128), u32),
            pltpu.VMEM((8, 256, 128), u32),
            pltpu.VMEM((3 * H, 256, 128), u32),
            pltpu.VMEM((2 * H, 8, 128), u32),
            pltpu.VMEM((H, 24, DH), u32),
            pltpu.VMEM((32, 128), f32),
            pltpu.VMEM((48, 128), f32),
            pltpu.VMEM((S, DM), bf16),
            pltpu.VMEM((16, DM // 2 + 1, 256), bf16),
            pltpu.VMEM((160, 64, 128), u32),
            pltpu.VMEM((320, 64, 128), f32),
            pltpu.VMEM((16, 128, 128), u32),
            pltpu.VMEM((64, 64, 128), u32),
            pltpu.SemaphoreType.DMA((7,)),
            pltpu.SemaphoreType.DMA((6,)),
            pltpu.SemaphoreType.DMA((16,)),
            pltpu.SemaphoreType.DMA((2,)),
        ],
        compiler_params=pltpu.CompilerParams(vmem_limit_bytes=120 * 1024 * 1024),
    )(jnp.asarray(tw), x.reshape(S, DM), x.reshape(NSEG, SEG, DM), mem0.reshape(MEM, DM), wq, wk, wv,
      wo.reshape(H * DH, DM), bx.reshape(S, DM), w_r.T, w_i.T, jnp.asarray(fd), jnp.asarray(ms))
    return out.reshape(1, S, 2 * DM)


def pallas_concat_heads__memory_aug_recurrent_mem_tr__spectral_gfnet__prompt_kernel(
    A_x: jax.Array,
    A_mem0: jax.Array,
    A_Wq: jax.Array,
    A_Wk: jax.Array,
    A_Wv: jax.Array,
    A_Wo: jax.Array,
    A_seg_len,
    B_x: jax.Array,
    B_w_r: jax.Array,
    B_w_i: jax.Array,
):
    if isinstance(A_seg_len, int):
        assert A_seg_len == SEG
    assert A_x.shape == (1, S, DM) and A_mem0.shape == (1, MEM, DM) and A_Wq.shape == (DM, H, DH)
    assert B_x.shape == (1, S, DM) and B_w_r.shape == (S, DM // 2 + 1)
    return _run(A_x, A_mem0, A_Wq, A_Wk, A_Wv, A_Wo, B_x, B_w_r, B_w_i)
```

```python
import math

import numpy as np
import jax
import jax.numpy as jnp
import jax.experimental.pallas as pl
import jax.experimental.pallas.tpu as pltpu

bf16 = jnp.bfloat16
f32 = jnp.float32
u32 = jnp.uint32

S, DM = 2048, 1024
H, DH = 32, 128
MEM, SEG = 8, 32
NSEG = S // SEG
SQH = math.sqrt(0.5)

_PAIRS = ((0, 4), (1, 7), (2, 6), (3, 5))


def _pack_rows(a):
    u = np.ascontiguousarray(a, dtype=np.float32).view(np.uint32).astype(np.uint64)
    b = ((u + 0x7FFF + ((u >> 16) & 1)) >> 16).astype(np.uint32)
    return (b[..., 0::2, :] | (b[..., 1::2, :] << 16)).astype(np.uint32)


def _tables():
    k2 = np.zeros((4, 128), np.int64)
    for t in range(4):
        odd = t % 2
        for lam in range(128):
            k = 2 * lam + odd
            if k % 8 not in _PAIRS[t]:
                k = 2 * (128 + 8 * (lam // 8) + (lam % 8 - 1 - odd) % 8) + odd
            assert k % 8 in _PAIRS[t]
            k2[t, lam] = k
    b = np.arange(128)[:, None]
    F = np.zeros((4, 256, 256))
    cw = np.full((4, 256), 2.0)
    for t in range(4):
        th = 2 * np.pi * ((b * k2[t][None, :]) % DM) / DM
        C, Sn = np.cos(th), np.sin(th)
        first = ((k2[t] % 8) == _PAIRS[t][0])[None, :]
        if t == 0:
            F[t, :128, :128] = np.where(first, C, 0)
            F[t, :128, 128:] = np.where(first, -Sn, 0)
            F[t, 128:, :128] = np.where(first, 0, C)
            F[t, 128:, 128:] = np.where(first, 0, -Sn)
            F[t, :128, 128] = (-1.0) ** np.arange(128)
            cw[t, 0] = 1.0
            cw[t, 128] = 1.0
        else:
            sg = np.where(first, 1.0, -1.0)
            F[t, :128, :128] = C
            F[t, 128:, :128] = -sg * Sn
            F[t, :128, 128:] = -Sn
            F[t, 128:, 128:] = -sg * C
    Finv = np.transpose(F * cw[:, None, :], (0, 2, 1)) / DM
    fd = np.stack([F, Finv]).reshape(2, 4, 256, 2, 128).transpose(0, 1, 3, 2, 4)
    fd = _pack_rows(fd).reshape(16, 128, 128)
    M = np.zeros((32, 128, 128))
    r = np.arange(64)[None, :]
    l = np.arange(64)[:, None]
    for j in range(32):
        th = 2 * np.pi * ((r * (j + 32 * l)) % S) / S
        C, Sn = np.cos(th), np.sin(th)
        M[j, :64, :64] = C
        M[j, :64, 64:] = Sn
        M[j, 64:, :64] = -Sn
        M[j, 64:, 64:] = C
    Minv = np.transpose(M, (0, 2, 1)) / S
    ms = _pack_rows(np.concatenate([M, Minv]))
    ang = 2 * np.pi * np.outer(np.arange(8), np.arange(4)) / 32
    tw = np.stack([np.cos(ang), np.sin(ang)], -1).reshape(-1).astype(np.float32)
    return fd, ms, tw


def _tobf(w):
    return pltpu.bitcast(w, bf16)


def _tou(w):
    return pltpu.bitcast(w, u32)


def _dot(a, b):
    return jnp.dot(a, b, preferred_element_type=f32)


def _r8_real(x):
    t0, t1 = x[0] + x[4], x[0] - x[4]
    t2, t3 = x[2] + x[6], x[2] - x[6]
    t4, t5 = x[1] + x[5], x[1] - x[5]
    t6, t7 = x[3] + x[7], x[3] - x[7]
    e0, e1 = t0 + t2, t0 - t2
    o0, o1 = t4 + t6, t4 - t6
    u, v = SQH * (t5 - t7), SQH * (t5 + t7)
    return [(e0 + o0, e0 - o0), (t1 + u, v + t3), (e1, o1), (t1 - u, v - t3)]


def _r8_real_t(g):
    (z0, z4), (a1, b1), (e1, o1), (a3, b3) = g
    e0, o0 = z0 + z4, z0 - z4
    t1, u = a1 + a3, a1 - a3
    v, t3 = b1 + b3, b1 - b3
    t5, t7 = SQH * (v + u), SQH * (v - u)
    t0, t2 = e0 + e1, e0 - e1
    t4, t6 = o0 + o1, o0 - o1
    return [t0 + t1, t4 + t5, t2 + t3, t6 + t7, t0 - t1, t4 - t5, t2 - t3, t6 - t7]


def _dft4(u):
    (r0, i0), (r1, i1), (r2, i2), (r3, i3) = u
    sr, si, dr, di = r0 + r2, i0 + i2, r0 - r2, i0 - i2
    tr, ti, er, ei = r1 + r3, i1 + i3, r1 - r3, i1 - i3
    return [(sr + tr, si + ti), (dr + ei, di - er), (sr - tr, si - ti), (dr - ei, di + er)]


def _dft8(x):
    a = [(x[p][0] + x[p + 4][0], x[p][1] + x[p + 4][1]) for p in range(4)]
    d = [(x[p][0] - x[p + 4][0], x[p][1] - x[p + 4][1]) for p in range(4)]
    ev = _dft4(a)
    (r0, i0), (r1, i1), (r2, i2), (r3, i3) = d
    b1r, b1i = SQH * (r1 + i1), SQH * (i1 - r1)
    b3r, n3i = SQH * (i3 - r3), SQH * (r3 + i3)
    sr, si, dr, di = r0 + i2, i0 - r2, r0 - i2, i0 + r2
    tr, ti, er, ei = b1r + b3r, b1i - n3i, b1r - b3r, b1i + n3i
    od = [(sr + tr, si + ti), (dr + ei, di - er), (sr - tr, si - ti), (dr - ei, di + er)]
    return [ev[0], od[0], ev[1], od[1], ev[2], od[2], ev[3], od[3]]


def _swap(x):
    return [(b, a) for (a, b) in x]


G = 4
NG = H // G
OSPLIT = 24
NEG = -1e9
N_L1, N_L2, N_L3 = 4, 20, 8


def _kernel(tw_ref, x_hbm, x3_hbm, mem_hbm, wq_hbm, wk_hbm, wv_hbm, wo_hbm, bx_hbm, wr_hbm, wi_hbm,
            fd_hbm, ms_hbm, out_hbm,
            xo_ref, mem_ref, xcraw_ref, raw_ref, w0_ref, w1_ref, w2_ref, w3_ref, w4_ref, w5_ref,
            woraw_ref, wo_ref, xc_ref, qkvc_ref, kve_ref,
            oall_ref, fille_ref, fillo_ref, bx_ref, wt_ref, wp_ref, ub_ref, st_ref, fd_ref, ms_ref,
            sem_in, sem_raw, sem_w, sem_out):
    scale = DH ** -0.5
    w_hbm = (wq_hbm, wk_hbm, wv_hbm)
    w_refs = (w0_ref, w1_ref, w2_ref, w3_ref, w4_ref, w5_ref)

    def raw_copy(c, i=None):
        src = w_hbm[c // 2]
        if i is None:
            return pltpu.make_async_copy(
                src.at[:, pl.ds((c % 2) * 16, 16), :], raw_ref.at[c % 2], sem_raw.at[c % 2])
        return pltpu.make_async_copy(
            src.at[pl.ds(i * 256, 256), pl.ds((c % 2) * 16, 16), :],
            raw_ref.at[c % 2, pl.ds(i * 256, 256)], sem_raw.at[2 + i])

    cp_x = pltpu.make_async_copy(x_hbm, xo_ref, sem_in.at[0])
    cp_mem = pltpu.make_async_copy(mem_hbm, mem_ref, sem_in.at[1])
    cp_wo = pltpu.make_async_copy(wo_hbm, woraw_ref, sem_in.at[2])
    cp_bx = pltpu.make_async_copy(bx_hbm, bx_ref, sem_in.at[3])
    cp_xc = pltpu.make_async_copy(x3_hbm.at[:, pl.ds(8, 8), :], xcraw_ref, sem_in.at[4])
    cp_fd = pltpu.make_async_copy(fd_hbm, fd_ref, sem_in.at[5])
    cp_ms = pltpu.make_async_copy(ms_hbm, ms_ref, sem_in.at[6])
    cp_wt = [pltpu.make_async_copy(src.at[:, pl.ds(lg * 256, 256)], wt_ref.at[a * 8 + lg], sem_w.at[a * 8 + lg])
             for a, src in enumerate((wr_hbm, wi_hbm)) for lg in range(8)]

    cp_xc.start()
    for i in range(4):
        raw_copy(0, i).start()

    qi = jax.lax.broadcasted_iota(jnp.int32, (48, 128), 0)
    ki = jax.lax.broadcasted_iota(jnp.int32, (48, 128), 1)

    def between(v, lo, hi):
        return (v >= lo) & (v < hi)

    def table(keep, other):
        return jnp.where(other, -jnp.inf, jnp.where(keep, 0.0, NEG)).astype(f32)

    keep = between(qi, 8, 16) | between(ki, 8, 16) | (qi >= jnp.where(ki < 32, ki, ki - 24))
    fille_ref[...] = table(keep, ki >= 40)[:32]
    q_even = between(qi, 32, 40)
    k_even = between(ki, 32, 40) | (ki >= 48)
    qpos = jnp.where(qi < 32, qi, jnp.where(qi < 40, qi - 24, qi - 32))
    kpos = jnp.where(ki < 32, ki, jnp.where(ki < 40, ki - 24, jnp.where(ki < 48, ki - 32, ki - 48)))
    keep = between(qi, 8, 16) | between(ki, 8, 16) | (ki >= 56) | (qpos >= kpos)
    fillo_ref[...] = table(keep, (q_even != k_even) | (ki >= 64))

    def relayout16(c, d0):
        slot = c % 2
        w0 = pl.multiple_of(d0 // 2, 8)
        los, his = [], []
        for dd in range(8):
            a = _tou(raw_ref[slot, d0 + 2 * dd])
            b = _tou(raw_ref[slot, d0 + 2 * dd + 1])
            los.append((a & jnp.uint32(0xFFFF)) | (b << 16))
            his.append((a >> 16) | (b & jnp.uint32(0xFFFF0000)))
        lo = jnp.swapaxes(jnp.stack(los), 0, 1)
        hi = jnp.swapaxes(jnp.stack(his), 0, 1)
        for j in range(8):
            w_refs[c][2 * j, pl.ds(w0, 8), :] = lo[j]
            w_refs[c][2 * j + 1, pl.ds(w0, 8), :] = hi[j]

    def repack_wo64(r_start):
        r0 = pl.multiple_of(r_start, 64)
        w0 = pl.multiple_of(r_start // 2, 32)
        v = woraw_ref[pl.ds(r0, 64), :]
        for j in range(8):
            wo_ref[j, pl.ds(w0, 32), :] = _tou(v[:, j * 128:(j + 1) * 128])

    sub4 = jax.lax.broadcasted_iota(jnp.int32, (128, 256), 0) % 4

    def b_prep(lg, t):
        l0 = pl.multiple_of(lg * 8, 8)
        if t < 4:
            a = _tou(wt_ref[lg, 0:512, :])
            b = _tou(wt_ref[8 + lg, 0:512, :])
            if t % 2 == 0:
                w = (a << 16) | (b & jnp.uint32(0xFFFF))
                m = (sub4 == 0) | (sub4 == 2)
            else:
                w = (a & jnp.uint32(0xFFFF0000)) | (b >> 16)
                m = (sub4 == 0) | (sub4 == 3)
            top = w[:128]
            bot = pltpu.roll(w[128:].reshape(16, 8, 256), 1 + t % 2, 1).reshape(128, 256)
            tile = jnp.where(m, top, bot) if t < 2 else jnp.where(m, bot, top)
        else:
            na = jnp.broadcast_to(wt_ref[lg, 512:513, :].astype(f32), (128, 256))
            nb = jnp.broadcast_to(wt_ref[8 + lg, 512:513, :].astype(f32), (128, 256))
            tile = pltpu.bitcast(na, u32) | (pltpu.bitcast(nb, u32) >> 16)
        v = jnp.swapaxes(tile.T.reshape(8, 32, 128), 0, 1)
        for j in range(32):
            wp_ref[t * 32 + j, pl.ds(l0, 8), :] = v[j]

    cp_xc.wait()

    def gather_c(i, carry):
        w0 = pl.multiple_of(i * 8, 8)
        v = jnp.concatenate([xcraw_ref[2 * i].astype(f32), xcraw_ref[2 * i + 1].astype(f32)],
                            axis=0).astype(bf16)
        for k in range(8):
            xc_ref[k, pl.ds(w0, 8), :] = _tou(v[:, k * 128:(k + 1) * 128])
        return carry
    jax.lax.fori_loop(0, NSEG // 2, gather_c, 0)

    for i in range(4):
        raw_copy(0, i).wait()
        if i == 2:
            raw_copy(1).start()

        def rl0(k, carry, i=i):
            for blk in range(4):
                relayout16(0, i * 256 + k * 64 + blk * 16)
            return carry
        jax.lax.fori_loop(0, 4, rl0, 0)

    def bulk_iter(c, i, n_rl, rl_start):
        xc = jnp.concatenate([_tobf(xc_ref[k]) for k in range(8)], axis=1)
        for t in range(8):
            n = i * 8 + t
            y = _tou(_dot(xc, _tobf(w_refs[c][n, 0:512])).astype(bf16))
            qkvc_ref[c * 16 + n] = y
            for blk in range(n_rl):
                pin = y[blk * (256 // n_rl):blk * (256 // n_rl) + 8]
                if c + 1 < 6:
                    w_refs[c + 1][15, 512:520] = pin
                    relayout16(c + 1, rl_start + (t * n_rl + blk) * 16)
                else:
                    wo_ref[7, 2048:2056] = pin
                    repack_wo64(rl_start + (t * n_rl + blk) * 64)
            if c >= 2 and t < 5:
                wp_ref[160, 0:8] = y[248:256]
                b_prep((c - 2) * 2 + i, t)

    for c in range(6):
        if c == 0:
            def bulk0(i, carry):
                bulk_iter(0, i, 0, 0)
                return carry
            jax.lax.fori_loop(0, 1, bulk0, 0)
            raw_copy(1).wait()
            raw_copy(2).start()

            def bulk1(i, carry):
                bulk_iter(0, i, 8, (i - 1) * 1024)
                return carry
            jax.lax.fori_loop(1, 2, bulk1, 0)
            continue
        if c + 1 < 6:
            raw_copy(c + 1).wait()
        if c + 2 < 6:
            raw_copy(c + 2).start()
        if c == 1:
            for cp in cp_wt:
                cp.start()
        if c == 2:
            for cp in cp_wt:
                cp.wait()
            cp_wo.start()
        if c == 4:
            cp_x.start()
            cp_mem.start()
            cp_bx.start()
            cp_fd.start()
        if c == 5:
            cp_wo.wait()
            cp_ms.start()

        def bulk(i, carry, c=c):
            bulk_iter(c, i, 4, i * (512 if c + 1 < 6 else 2048))
            return carry
        jax.lax.fori_loop(0, 2, bulk, 0)

    cp_x.wait()
    cp_mem.wait()
    cp_bx.wait()
    cp_fd.wait()
    cp_ms.wait()

    lane0 = jax.lax.broadcasted_iota(jnp.int32, (16, 128), 1) == 0

    def ub_idx(t, ri, jq, p):
        return ((t * 2 + ri) * 4 + jq) * 8 + p

    def fmat(d, t):
        return jnp.concatenate([_tobf(fd_ref[d * 8 + t * 2]), _tobf(fd_ref[d * 8 + t * 2 + 1])], axis=1)

    def twiddles(p):
        return [(tw_ref[(p * 4 + jq) * 2], tw_ref[(p * 4 + jq) * 2 + 1]) for jq in range(4)]

    def pin_st(y):
        st_ref[16, 0:8] = pltpu.bitcast(y, u32)

    def pin_ub(y):
        ub_ref[320, 0:8] = y

    def p1_pre(p, z, slot, rs, q):
        def item(y):
            pin_st(y)
            rows = pl.multiple_of(q * 512 + p * 64 + rs * 16, 16)
            xq = bx_ref[pl.ds(rows, 16), :].astype(f32)
            zz = _r8_real([xq[:, a * 128:(a + 1) * 128] for a in range(8)])
            for t in range(4):
                for k in range(2):
                    st_ref[z + slot * 8 + t * 2 + k, (rs * 4 + q) * 8:(rs * 4 + q + 1) * 8] = (
                        _tou(zz[t][k].astype(bf16)))
        return item

    def p1_mm(p, z, slot, t):
        def item(y):
            cs = twiddles(p)

            def emit(t, rs, u):
                a = _dft4(u)
                for jq in range(4):
                    re, im = a[jq]
                    if jq > 0:
                        c, sn = cs[jq]
                        re, im = re * c + im * sn, im * c - re * sn
                    ub_ref[ub_idx(t, 0, jq, p), rs * 16:(rs + 1) * 16] = re
                    ub_ref[ub_idx(t, 1, jq, p), rs * 16:(rs + 1) * 16] = im

            lhs = jnp.concatenate([_tobf(st_ref[z + slot * 8 + t * 2 + k]) for k in range(2)], axis=1)
            o = _dot(lhs, fmat(0, t))
            for rs in range(4):
                u = [(o[(rs * 4 + q) * 16:(rs * 4 + q + 1) * 16, :128],
                      o[(rs * 4 + q) * 16:(rs * 4 + q + 1) * 16, 128:]) for q in range(4)]
                if t == 0:
                    emit(4, rs, [(im, jnp.zeros_like(im)) for (_, im) in u])
                    u = [(re, jnp.where(lane0, 0.0, im)) for (re, im) in u]
                emit(t, rs, u)
        return item

    def p2_pre(u, z, rs):
        def item(y):
            pin_st(y)
            t = u // 4
            jq = u % 4
            rows = slice(rs * 16, (rs + 1) * 16)
            tt = _dft8([(ub_ref[ub_idx(t, 0, jq, p), rows], ub_ref[ub_idx(t, 1, jq, p), rows])
                        for p in range(8)])
            for jp in range(8):
                for k in range(2):
                    st_ref[z + jp, k * 32 + rs * 8:k * 32 + (rs + 1) * 8] = _tou(tt[jp][k].astype(bf16))
        return item

    def p2_fwd(u, z, jps):
        def item(y):
            t = u // 4
            jq = u % 4
            for jp in jps:
                j = jq + 4 * jp
                xx = _dot(_tobf(ms_ref[j]), _tobf(st_ref[z + jp, 0:64]))
                xr, xi = xx[:64], xx[64:]
                w = wp_ref[t * 32 + j]
                wr = pltpu.bitcast(w & jnp.uint32(0xFFFF0000), f32)
                wi = pltpu.bitcast(w << 16, f32)
                st_ref[z + 8 + jp, 0:32] = _tou((xr * wr - xi * wi).astype(bf16))
                st_ref[z + 8 + jp, 32:64] = _tou((xr * wi + xi * wr).astype(bf16))
        return item

    def p2_inv(u, z, jps):
        def item(y):
            t = u // 4
            jq = u % 4
            for jp in jps:
                zz = _dot(_tobf(ms_ref[32 + jq + 4 * jp]), _tobf(st_ref[z + 8 + jp, 0:64]))
                ub_ref[ub_idx(t, 0, jq, jp)] = zz[:64]
                ub_ref[ub_idx(t, 1, jq, jp)] = zz[64:]
        return item

    def p2_post(u, rs):
        def item(y):
            pin_ub(y)
            t = u // 4
            jq = u % 4
            rows = slice(rs * 8, (rs + 1) * 8)
            a = _dft8([(ub_ref[ub_idx(t, 1, jq, p), rows], ub_ref[ub_idx(t, 0, jq, p), rows])
                       for p in range(8)])
            for p in range(8):
                ub_ref[ub_idx(t, 0, jq, p), rows] = a[p][1]
                ub_ref[ub_idx(t, 1, jq, p), rows] = a[p][0]
        return item

    def p3_pre(p, z, rs, t):
        def item(y):
            pin_st(y)
            cs = twiddles(p)
            rows = slice(rs * 16, (rs + 1) * 16)

            def fetch(t):
                a = []
                for jq in range(4):
                    re, im = ub_ref[ub_idx(t, 0, jq, p), rows], ub_ref[ub_idx(t, 1, jq, p), rows]
                    if jq > 0:
                        c, sn = cs[jq]
                        re, im = re * c - im * sn, im * c + re * sn
                    a.append((re, im))
                return _swap(_dft4(_swap(a)))

            u = fetch(t)
            if t == 0:
                ny = fetch(4)
                u = [(u[q][0], jnp.where(lane0, ny[q][0], u[q][1])) for q in range(4)]
            for q in range(4):
                for k in range(2):
                    st_ref[z + t * 2 + k, (q * 4 + rs) * 8:(q * 4 + rs + 1) * 8] = _tou(u[q][k].astype(bf16))
        return item

    def p3_mm(p, z, q):
        def item(y):
            g = []
            for t in range(4):
                lhs = jnp.concatenate([_tobf(st_ref[z + t * 2 + k, q * 32:(q + 1) * 32]) for k in range(2)],
                                      axis=1)
                o = _dot(lhs, fmat(1, t))
                g.append((o[:, :128], o[:, 128:]))
            yy = _r8_real_t(g)
            rows = pl.multiple_of(q * 512 + p * 64, 64)
            for a in range(8):
                bx_ref[pl.ds(rows, 64), a * 128:(a + 1) * 128] = yy[a].astype(bf16)
        return item

    def b_out(p):
        for q in range(4):
            rows = pl.multiple_of(q * 512 + p * 64, 64)
            pltpu.make_async_copy(bx_ref.at[pl.ds(rows, 64), :],
                                  out_hbm.at[pl.ds(rows, 64), pl.ds(DM, DM)], sem_out.at[1]).start()

    def step(pp, odd, mem, hooks):
        r0 = pl.multiple_of(pp * 64 + 32 * odd, SEG)
        c0 = pl.multiple_of(pp * 8, 8)
        xs = xo_ref[pl.ds(r0, SEG), :]
        x_lo = xs[0:8].astype(f32)
        hm = jnp.concatenate(
            [jnp.concatenate([x_lo, jnp.concatenate(mem, axis=1)], axis=0).astype(bf16), xs[16:32]], axis=0)
        fill = fillo_ref[:, 0:64] if odd else fille_ref[:, 0:48]
        nrow = 48 if odd else 32
        qkv, ps = {}, {}

        def do_qkv(g):
            for h in range(g * G, (g + 1) * G):
                for t in range(3):
                    y32 = _dot(hm, _tobf(w_refs[t * 2 + h // 16][h % 16, 0:512]))
                    y = y32.astype(bf16)
                    parts = [y]
                    if odd or t > 0:
                        parts.append(_tobf(qkvc_ref[t * H + h, pl.ds(c0, 8), :]))
                    if t > 0:
                        if odd:
                            parts.append(_tobf(kve_ref[(t - 1) * H + h]))
                        else:
                            kve_ref[(t - 1) * H + h] = _tou(y[0:16])
                    qkv[(t, h)] = jnp.concatenate(parts, axis=0) if len(parts) > 1 else y
                for item in hooks.get(h, ()):
                    item(y32[0:8])

        def do_s(g):
            for h in range(g * G, (g + 1) * G):
                sc = jax.lax.dot_general(qkv[(0, h)], qkv[(1, h)], (((1,), (1,)), ((), ())),
                                         preferred_element_type=f32)
                sc = jnp.where(fill == 0.0, sc * scale, fill)
                e = jnp.exp(sc - jnp.max(sc, axis=1, keepdims=True))
                den = jnp.sum(e, axis=1, keepdims=True)
                r = pl.reciprocal(den, approx=True)
                r = r * (2.0 - den * r)
                ps[h] = (e * r).astype(bf16)

        def do_pv(g):
            for h in range(g * G, (g + 1) * G):
                oall_ref[h, 0:nrow // 2] = _tou(_dot(ps[h], qkv[(2, h)]).astype(bf16))

        def do_o(j, h0, h1):
            lhs = jnp.concatenate([_tobf(oall_ref[h, 0:nrow // 2]) for h in range(h0, h1)], axis=1)
            return _dot(lhs, _tobf(wo_ref[j, h0 * 64:h1 * 64, :]))

        for g in range(NG):
            do_qkv(g)
            if g >= 1:
                do_s(g - 1)
            if g >= 2:
                do_pv(g - 2)
        part = {}
        for j in range(0, 3):
            part[j] = do_o(j, 0, OSPLIT)
        do_s(NG - 1)
        do_pv(NG - 2)
        for j in range(3, 6):
            part[j] = do_o(j, 0, OSPLIT)
        do_pv(NG - 1)
        for j in range(6, 8):
            part[j] = do_o(j, 0, OSPLIT)
        new_mem = []
        for j in range(8):
            cols = slice(j * 128, (j + 1) * 128)
            res = do_o(j, OSPLIT, H) + part[j]
            new_mem.append(res[8:16])
            if odd:
                xo_ref[pl.ds(r0, SEG), cols] = jnp.concatenate(
                    [res[0:8], res[40:48], res[16:32]], axis=0).astype(bf16)
                xo_ref[pl.ds(r0 - 24, 8), cols] = res[32:40].astype(bf16)
            else:
                xo_ref[pl.ds(r0, SEG), cols] = res.astype(bf16)
        for item in hooks.get(H, ()):
            item(None)
        return new_mem

    def a_out(pp):
        rows = pl.multiple_of(pp * 64, 64)
        pltpu.make_async_copy(xo_ref.at[pl.ds(rows, 64), :],
                              out_hbm.at[pl.ds(rows, 64), pl.ds(0, DM)], sem_out.at[0]).start()

    def l1(i, mem):
        z = i // 64
        he = {h: [p1_pre(2 * i + h // 16, z, h // 16, (h % 16) // 4, h % 4)] for h in range(32)}
        he[21].append(p1_mm(2 * i, z, 0, 0))
        he[25].append(p1_mm(2 * i, z, 0, 1))
        he[29].append(p1_mm(2 * i, z, 0, 2))
        he[H] = [p1_mm(2 * i, z, 0, 3)]
        ho = {1 + 4 * t: [p1_mm(2 * i + 1, z, 1, t)] for t in range(4)}
        mem = step(i, 0, mem, he)
        mem = step(i, 1, mem, ho)
        a_out(i)
        return mem

    def l2(i, mem):
        z = i // 64
        u = i - N_L1
        he = {1 + 2 * rs: [p2_pre(u, z, rs)] for rs in range(4)}
        he[13] = [p2_fwd(u, z, range(0, 4))]
        he[21] = [p2_fwd(u, z, range(4, 8))]
        he[H] = [p2_inv(u, z, range(0, 8))]
        ho = {3 + 2 * rs: [p2_post(u, rs)] for rs in range(8)}
        mem = step(i, 0, mem, he)
        mem = step(i, 1, mem, ho)
        a_out(i)
        return mem

    def l3(i, mem):
        z = i // 64
        p = i - N_L1 - N_L2
        he = {h: [p3_pre(p, z, h // 4, h % 4)] for h in range(16)}
        he[21] = [p3_mm(p, z, 0)]
        he[29] = [p3_mm(p, z, 1)]
        he[H] = [p3_mm(p, z, 2)]
        ho = {5: [p3_mm(p, z, 3)]}
        mem = step(i, 0, mem, he)
        mem = step(i, 1, mem, ho)
        b_out(p)
        a_out(i)
        return mem

    m0 = mem_ref[...].astype(f32)
    mem = [m0[:, j * 128:(j + 1) * 128] for j in range(8)]
    mem = jax.lax.fori_loop(0, N_L1, l1, mem)
    mem = jax.lax.fori_loop(N_L1, N_L1 + N_L2, l2, mem)
    mem = jax.lax.fori_loop(N_L1 + N_L2, NSEG // 2, l3, mem)

    pltpu.make_async_copy(xo_ref, out_hbm.at[:, pl.ds(0, DM)], sem_out.at[0]).wait()
    pltpu.make_async_copy(bx_ref, out_hbm.at[:, pl.ds(DM, DM)], sem_out.at[1]).wait()


@jax.jit
def _run(x, mem0, wq, wk, wv, wo, bx, w_r, w_i):
    fd, ms, tw = _tables()
    hbm = pl.BlockSpec(memory_space=pl.ANY)
    out = pl.pallas_call(
        _kernel,
        out_shape=jax.ShapeDtypeStruct((S, 2 * DM), bf16),
        in_specs=[pl.BlockSpec(memory_space=pltpu.SMEM)] + [hbm] * 12,
        out_specs=hbm,
        scratch_shapes=[
            pltpu.VMEM((S, DM), bf16),
            pltpu.VMEM((MEM, DM), bf16),
            pltpu.VMEM((NSEG, 8, DM), bf16),
            pltpu.VMEM((2, DM, 16, DH), bf16),
        ] + [pltpu.VMEM((16, DM // 2 + 8, DH), u32)] * 6 + [
            pltpu.VMEM((H * DH, DM), bf16),
            pltpu.VMEM((8, H * DH // 2 + 8, 128), u32),
            pltpu.VMEM((8, 256, 128), u32),
            pltpu.VMEM((3 * H, 256, 128), u32),
            pltpu.VMEM((2 * H, 8, 128), u32),
            pltpu.VMEM((H, 24, DH), u32),
            pltpu.VMEM((32, 128), f32),
            pltpu.VMEM((48, 128), f32),
            pltpu.VMEM((S, DM), bf16),
            pltpu.VMEM((16, DM // 2 + 1, 256), bf16),
            pltpu.VMEM((161, 64, 128), u32),
            pltpu.VMEM((321, 64, 128), f32),
            pltpu.VMEM((17, 128, 128), u32),
            pltpu.VMEM((16, 128, 128), u32),
            pltpu.VMEM((64, 64, 128), u32),
            pltpu.SemaphoreType.DMA((7,)),
            pltpu.SemaphoreType.DMA((6,)),
            pltpu.SemaphoreType.DMA((16,)),
            pltpu.SemaphoreType.DMA((2,)),
        ],
        compiler_params=pltpu.CompilerParams(vmem_limit_bytes=120 * 1024 * 1024),
    )(jnp.asarray(tw), x.reshape(S, DM), x.reshape(NSEG, SEG, DM), mem0.reshape(MEM, DM), wq, wk, wv,
      wo.reshape(H * DH, DM), bx.reshape(S, DM), w_r.T, w_i.T, jnp.asarray(fd), jnp.asarray(ms))
    return out.reshape(1, S, 2 * DM)


def pallas_concat_heads__memory_aug_recurrent_mem_tr__spectral_gfnet__prompt_kernel(
    A_x: jax.Array,
    A_mem0: jax.Array,
    A_Wq: jax.Array,
    A_Wk: jax.Array,
    A_Wv: jax.Array,
    A_Wo: jax.Array,
    A_seg_len,
    B_x: jax.Array,
    B_w_r: jax.Array,
    B_w_i: jax.Array,
):
    if isinstance(A_seg_len, int):
        assert A_seg_len == SEG
    assert A_x.shape == (1, S, DM) and A_mem0.shape == (1, MEM, DM) and A_Wq.shape == (DM, H, DH)
    assert B_x.shape == (1, S, DM) and B_w_r.shape == (S, DM // 2 + 1)
    return _run(A_x, A_mem0, A_Wq, A_Wk, A_Wv, A_Wo, B_x, B_w_r, B_w_i)
```

```python
import math

import numpy as np
import jax
import jax.numpy as jnp
import jax.experimental.pallas as pl
import jax.experimental.pallas.tpu as pltpu

bf16 = jnp.bfloat16
f32 = jnp.float32
u32 = jnp.uint32

S, DM = 2048, 1024
H, DH = 32, 128
MEM, SEG = 8, 32
NSEG = S // SEG
SQH = math.sqrt(0.5)

_PAIRS = ((0, 4), (1, 7), (2, 6), (3, 5))


def _pack_rows(a):
    u = np.ascontiguousarray(a, dtype=np.float32).view(np.uint32).astype(np.uint64)
    b = ((u + 0x7FFF + ((u >> 16) & 1)) >> 16).astype(np.uint32)
    return (b[..., 0::2, :] | (b[..., 1::2, :] << 16)).astype(np.uint32)


def _tables():
    k2 = np.zeros((4, 128), np.int64)
    for t in range(4):
        odd = t % 2
        for lam in range(128):
            k = 2 * lam + odd
            if k % 8 not in _PAIRS[t]:
                k = 2 * (128 + 8 * (lam // 8) + (lam % 8 - 1 - odd) % 8) + odd
            assert k % 8 in _PAIRS[t]
            k2[t, lam] = k
    b = np.arange(128)[:, None]
    F = np.zeros((4, 256, 256))
    cw = np.full((4, 256), 2.0)
    for t in range(4):
        th = 2 * np.pi * ((b * k2[t][None, :]) % DM) / DM
        C, Sn = np.cos(th), np.sin(th)
        first = ((k2[t] % 8) == _PAIRS[t][0])[None, :]
        if t == 0:
            F[t, :128, :128] = np.where(first, C, 0)
            F[t, :128, 128:] = np.where(first, -Sn, 0)
            F[t, 128:, :128] = np.where(first, 0, C)
            F[t, 128:, 128:] = np.where(first, 0, -Sn)
            F[t, :128, 128] = (-1.0) ** np.arange(128)
            cw[t, 0] = 1.0
            cw[t, 128] = 1.0
        else:
            sg = np.where(first, 1.0, -1.0)
            F[t, :128, :128] = C
            F[t, 128:, :128] = -sg * Sn
            F[t, :128, 128:] = -Sn
            F[t, 128:, 128:] = -sg * C
    Finv = np.transpose(F * cw[:, None, :], (0, 2, 1)) / DM
    fd = np.stack([F, Finv]).reshape(2, 4, 256, 2, 128).transpose(0, 1, 3, 2, 4)
    fd = _pack_rows(fd).reshape(16, 128, 128)
    M = np.zeros((32, 128, 128))
    r = np.arange(64)[None, :]
    l = np.arange(64)[:, None]
    for j in range(32):
        th = 2 * np.pi * ((r * (j + 32 * l)) % S) / S
        C, Sn = np.cos(th), np.sin(th)
        M[j, :64, :64] = C
        M[j, :64, 64:] = Sn
        M[j, 64:, :64] = -Sn
        M[j, 64:, 64:] = C
    Minv = np.transpose(M, (0, 2, 1)) / S
    ms = _pack_rows(np.concatenate([M, Minv]))
    return fd, ms


def _tobf(w):
    return pltpu.bitcast(w, bf16)


def _tou(w):
    return pltpu.bitcast(w, u32)


def _dot(a, b):
    return jnp.dot(a, b, preferred_element_type=f32)


def _r8_real(x):
    t0, t1 = x[0] + x[4], x[0] - x[4]
    t2, t3 = x[2] + x[6], x[2] - x[6]
    t4, t5 = x[1] + x[5], x[1] - x[5]
    t6, t7 = x[3] + x[7], x[3] - x[7]
    e0, e1 = t0 + t2, t0 - t2
    o0, o1 = t4 + t6, t4 - t6
    u, v = SQH * (t5 - t7), SQH * (t5 + t7)
    return [(e0 + o0, e0 - o0), (t1 + u, v + t3), (e1, o1), (t1 - u, v - t3)]


def _r8_real_t(g):
    (z0, z4), (a1, b1), (e1, o1), (a3, b3) = g
    e0, o0 = z0 + z4, z0 - z4
    t1, u = a1 + a3, a1 - a3
    v, t3 = b1 + b3, b1 - b3
    t5, t7 = SQH * (v + u), SQH * (v - u)
    t0, t2 = e0 + e1, e0 - e1
    t4, t6 = o0 + o1, o0 - o1
    return [t0 + t1, t4 + t5, t2 + t3, t6 + t7, t0 - t1, t4 - t5, t2 - t3, t6 - t7]


def _dft4(u):
    (r0, i0), (r1, i1), (r2, i2), (r3, i3) = u
    sr, si, dr, di = r0 + r2, i0 + i2, r0 - r2, i0 - i2
    tr, ti, er, ei = r1 + r3, i1 + i3, r1 - r3, i1 - i3
    return [(sr + tr, si + ti), (dr + ei, di - er), (sr - tr, si - ti), (dr - ei, di + er)]


def _dft8(x):
    a = [(x[p][0] + x[p + 4][0], x[p][1] + x[p + 4][1]) for p in range(4)]
    d = [(x[p][0] - x[p + 4][0], x[p][1] - x[p + 4][1]) for p in range(4)]
    ev = _dft4(a)
    (r0, i0), (r1, i1), (r2, i2), (r3, i3) = d
    b1r, b1i = SQH * (r1 + i1), SQH * (i1 - r1)
    b3r, n3i = SQH * (i3 - r3), SQH * (r3 + i3)
    sr, si, dr, di = r0 + i2, i0 - r2, r0 - i2, i0 + r2
    tr, ti, er, ei = b1r + b3r, b1i - n3i, b1r - b3r, b1i + n3i
    od = [(sr + tr, si + ti), (dr + ei, di - er), (sr - tr, si - ti), (dr - ei, di + er)]
    return [ev[0], od[0], ev[1], od[1], ev[2], od[2], ev[3], od[3]]


def _swap(x):
    return [(b, a) for (a, b) in x]


G = 4
NG = H // G
OSPLIT = 24
NEG = -1e9
N_L1, N_L2, N_L3 = 4, 20, 8


def _kernel(x_hbm, x3_hbm, mem_hbm, wq_hbm, wk_hbm, wv_hbm, wo_hbm, bx_hbm, wr_hbm, wi_hbm,
            fd_hbm, ms_hbm, out_hbm,
            xo_ref, mem_ref, xcraw_ref, raw_ref, w0_ref, w1_ref, w2_ref, w3_ref, w4_ref, w5_ref,
            woraw_ref, wo_ref, xc_ref, qkvc_ref, kve_ref,
            oall_ref, fille_ref, fillo_ref, bx_ref, wt_ref, wp_ref, ub_ref, sa_ref, sb_ref, fd_ref, ms_ref,
            tw_ref, sem_in, sem_out):
    scale = DH ** -0.5
    w_hbm = (wq_hbm, wk_hbm, wv_hbm)
    w_refs = (w0_ref, w1_ref, w2_ref, w3_ref, w4_ref, w5_ref)

    def raw_copy(c, i=0, nd=DM):
        rows = pl.ds(pl.multiple_of(i * nd, nd), nd)
        return pltpu.make_async_copy(
            w_hbm[c // 2].at[rows, pl.ds((c % 2) * 16, 16), :],
            raw_ref.at[c % 3, rows], sem_in.at[8 + (c % 3) * 8 + i])

    def xc_copy(k):
        return pltpu.make_async_copy(
            x3_hbm.at[:, pl.ds(8, 8), pl.ds(pl.multiple_of(k * 128, 128), 128)], xcraw_ref.at[k], sem_in.at[32 + k])

    cp_x = pltpu.make_async_copy(x_hbm, xo_ref, sem_in.at[0])
    cp_mem = pltpu.make_async_copy(mem_hbm, mem_ref, sem_in.at[1])
    cp_wo = pltpu.make_async_copy(wo_hbm, woraw_ref, sem_in.at[2])
    cp_bx = pltpu.make_async_copy(bx_hbm, bx_ref, sem_in.at[3])
    cp_fd = pltpu.make_async_copy(fd_hbm, fd_ref, sem_in.at[4])
    cp_ms = pltpu.make_async_copy(ms_hbm, ms_ref, sem_in.at[5])
    cp_wt = [pltpu.make_async_copy(src.at[:, pl.ds(lg * 256, 256)], wt_ref.at[a * 8 + lg], sem_in.at[40 + a * 8 + lg])
             for a, src in enumerate((wr_hbm, wi_hbm)) for lg in range(8)]

    for i in range(8):
        xc_copy(i).start()
        raw_copy(0, i, 128).start()
        raw_copy(1, i, 128).start()
    for i in range(4):
        raw_copy(2, i, 256).start()

    for p in range(8):
        for jq in range(4):
            tw_ref[(p * 4 + jq) * 2] = jnp.float32(math.cos(2 * math.pi * p * jq / 32))
            tw_ref[(p * 4 + jq) * 2 + 1] = jnp.float32(math.sin(2 * math.pi * p * jq / 32))

    qi = jax.lax.broadcasted_iota(jnp.int32, (48, 128), 0)
    ki = jax.lax.broadcasted_iota(jnp.int32, (48, 128), 1)

    def between(v, lo, hi):
        return (v >= lo) & (v < hi)

    def table(keep, other):
        return jnp.where(other, -jnp.inf, jnp.where(keep, 0.0, NEG)).astype(f32)

    keep = between(qi, 8, 16) | between(ki, 8, 16) | (qi >= jnp.where(ki < 32, ki, ki - 24))
    fille_ref[...] = table(keep, ki >= 40)[:32]
    q_even = between(qi, 32, 40)
    k_even = between(ki, 32, 40) | (ki >= 48)
    qpos = jnp.where(qi < 32, qi, jnp.where(qi < 40, qi - 24, qi - 32))
    kpos = jnp.where(ki < 32, ki, jnp.where(ki < 40, ki - 24, jnp.where(ki < 48, ki - 32, ki - 48)))
    keep = between(qi, 8, 16) | between(ki, 8, 16) | (ki >= 56) | (qpos >= kpos)
    fillo_ref[...] = table(keep, (q_even != k_even) | (ki >= 64))

    def relayout16(c, d0):
        slot = c % 3
        w0 = pl.multiple_of(d0 // 2, 8)
        los, his = [], []
        for dd in range(8):
            a = _tou(raw_ref[slot, d0 + 2 * dd])
            b = _tou(raw_ref[slot, d0 + 2 * dd + 1])
            los.append((a & jnp.uint32(0xFFFF)) | (b << 16))
            his.append((a >> 16) | (b & jnp.uint32(0xFFFF0000)))
        lo = jnp.swapaxes(jnp.stack(los), 0, 1)
        hi = jnp.swapaxes(jnp.stack(his), 0, 1)
        for j in range(8):
            w_refs[c][2 * j, pl.ds(w0, 8), :] = lo[j]
            w_refs[c][2 * j + 1, pl.ds(w0, 8), :] = hi[j]

    def repack_wo64(r_start):
        r0 = pl.multiple_of(r_start, 64)
        w0 = pl.multiple_of(r_start // 2, 32)
        v = woraw_ref[pl.ds(r0, 64), :]
        for j in range(8):
            wo_ref[j, pl.ds(w0, 32), :] = _tou(v[:, j * 128:(j + 1) * 128])

    sub4 = jax.lax.broadcasted_iota(jnp.int32, (128, 256), 0) % 4

    def b_prep(lg, t):
        l0 = pl.multiple_of(lg * 8, 8)
        if t < 4:
            a = _tou(wt_ref[lg, 0:512, :])
            b = _tou(wt_ref[8 + lg, 0:512, :])
            if t % 2 == 0:
                w = (a << 16) | (b & jnp.uint32(0xFFFF))
                m = (sub4 == 0) | (sub4 == 2)
            else:
                w = (a & jnp.uint32(0xFFFF0000)) | (b >> 16)
                m = (sub4 == 0) | (sub4 == 3)
            top = w[:128]
            bot = pltpu.roll(w[128:].reshape(16, 8, 256), 1 + t % 2, 1).reshape(128, 256)
            tile = jnp.where(m, top, bot) if t < 2 else jnp.where(m, bot, top)
        else:
            na = jnp.broadcast_to(wt_ref[lg, 512:513, :].astype(f32), (128, 256))
            nb = jnp.broadcast_to(wt_ref[8 + lg, 512:513, :].astype(f32), (128, 256))
            tile = pltpu.bitcast(na, u32) | (pltpu.bitcast(nb, u32) >> 16)
        v = jnp.swapaxes(tile.T.reshape(8, 32, 128), 0, 1)
        for j in range(32):
            wp_ref[t * 32 + j, pl.ds(l0, 8), :] = v[j]

    def gather_c(k):
        xc_ref[k] = _tou(xcraw_ref[k].astype(f32).reshape(512, 128).astype(bf16))

    def store_qkvc(n, y):
        for pp in range(NSEG // 2):
            qkvc_ref[pp, n] = y[pp * 8:(pp + 1) * 8]

    def q_unit(i, groups, first, last, fillers):
        xk = _tobf(xc_ref[i])
        w0 = pl.multiple_of(i * 64, 64)
        per = len(fillers) // len(groups) + 1
        for gi, g in enumerate(groups):
            rhs = jnp.concatenate(
                [_tobf(w_refs[h // 16][h % 16, pl.ds(w0, 64), :]) for h in range(4 * g, 4 * g + 4)], axis=1)
            y = _dot(xk, rhs)
            for h in range(4 * g, 4 * g + 4):
                yh = y[:, (h % 4) * 128:(h % 4 + 1) * 128]
                if not first:
                    yh = yh + ub_ref[h * 8:(h + 1) * 8].reshape(512, 128)
                if last:
                    store_qkvc(h, _tou(yh.astype(bf16)))
                else:
                    ub_ref[h * 8:(h + 1) * 8] = yh.reshape(8, 64, 128)
            mine = fillers[gi * per:(gi + 1) * per]
            for fi, item in enumerate(mine):
                r = (fi * 512 // len(mine)) // 8 * 8
                item(pltpu.bitcast(y[r:r + 8, 0:128], u32))

    def rl_item(c, d0, pinned):
        def item(pin):
            if pinned:
                w_refs[c][15, 512:520] = pin
            relayout16(c, d0)
        return item

    def gather_item(k):
        return lambda pin: gather_c(k)

    def piece_items(i):
        return ([rl_item(blk % 2, i * 128 + (blk // 2) * 16, False) for blk in range(16)]
                + [gather_item(i)])

    def wait_piece(i):
        xc_copy(i).wait()
        raw_copy(0, i, 128).wait()
        raw_copy(1, i, 128).wait()

    def mix(a, b):
        out = []
        for k in range(max(len(a), len(b))):
            out += a[k:k + 1] + b[k:k + 1]
        return out

    xc_copy(0).wait()
    gather_c(0)
    raw_copy(0, 0, 128).wait()

    def q_pre(k, carry):
        for blk in range(4):
            relayout16(0, k * 64 + blk * 16)
        return carry
    jax.lax.fori_loop(0, 2, q_pre, 0)
    raw_copy(1, 0, 128).wait()

    def q_a(i, carry):
        q_unit(i, range(0, 4), True, False, [rl_item(1, i * 128 + blk * 16, True) for blk in range(8)])
        return carry
    jax.lax.fori_loop(0, 1, q_a, 0)
    wait_piece(1)

    def q_b(i, carry):
        q_unit(i, range(4, 8), True, False,
               [rl_item(blk % 2, (i + 1) * 128 + (blk // 2) * 16, blk % 2 == 0) for blk in range(16)]
               + [gather_item(i + 1)])
        return carry
    jax.lax.fori_loop(0, 1, q_b, 0)

    def q_c(i, carry):
        wait_piece(i + 1)
        q_unit(i, range(8), False, False, piece_items(i + 1))
        return carry
    jax.lax.fori_loop(1, 4, q_c, 0)

    def q_d(i, carry):
        wait_piece(i + 1)
        raw_copy(2, i - 4, 256).wait()
        q_unit(i, range(8), False, False,
               mix(piece_items(i + 1), [rl_item(2, (i - 4) * 256 + blk * 16, True) for blk in range(16)]))
        return carry
    for cp in cp_wt:
        cp.start()
    jax.lax.fori_loop(4, 7, q_d, 0)
    raw_copy(3).start()
    raw_copy(4).start()
    raw_copy(2, 3, 256).wait()

    def q_e(i, carry):
        q_unit(i, range(8), False, True, [rl_item(2, (i - 4) * 256 + blk * 16, True) for blk in range(16)])
        return carry
    jax.lax.fori_loop(7, 8, q_e, 0)

    def bulk_iter(c, i, n_rl, rl_start):
        xc = jnp.concatenate([_tobf(xc_ref[k]) for k in range(8)], axis=1)
        for t in range(8):
            n = i * 8 + t
            y = _tou(_dot(xc, _tobf(w_refs[c][n, 0:512])).astype(bf16))
            store_qkvc(c * 16 + n, y)
            for blk in range(n_rl):
                pin = y[blk * (256 // n_rl):blk * (256 // n_rl) + 8]
                if c + 1 < 6:
                    w_refs[c + 1][15, 512:520] = pin
                    relayout16(c + 1, rl_start + (t * n_rl + blk) * 16)
                else:
                    wo_ref[7, 2048:2056] = pin
                    repack_wo64(rl_start + (t * n_rl + blk) * 64)
            if t < 5:
                wp_ref[160, 0:8] = y[248:256]
                b_prep((c - 2) * 2 + i, t)

    for c in range(2, 6):
        if c == 2:
            raw_copy(5).start()
            cp_wo.start()
            cp_x.start()
            cp_mem.start()
            cp_bx.start()
            cp_fd.start()
            cp_ms.start()
            for cp in cp_wt:
                cp.wait()
        if c + 1 < 6:
            raw_copy(c + 1).wait()
        else:
            cp_wo.wait()

        def bulk(i, carry, c=c):
            bulk_iter(c, i, 4, i * (512 if c + 1 < 6 else 2048))
            return carry
        jax.lax.fori_loop(0, 2, bulk, 0)

    cp_x.wait()
    cp_mem.wait()
    cp_bx.wait()
    cp_fd.wait()
    cp_ms.wait()

    lane0 = jax.lax.broadcasted_iota(jnp.int32, (16, 128), 1) == 0

    def ub_idx(t, ri, jq, p):
        return ((t * 2 + ri) * 4 + jq) * 8 + p

    def ub_rows(ri, r, n):
        r = (r + 16 * ri) % 64
        return slice(r, r + n)

    def fmat(d, t):
        return jnp.concatenate([_tobf(fd_ref[d * 8 + t * 2]), _tobf(fd_ref[d * 8 + t * 2 + 1])], axis=1)

    def twiddles(p):
        return [(tw_ref[(p * 4 + jq) * 2], tw_ref[(p * 4 + jq) * 2 + 1]) for jq in range(4)]

    st_refs = (sa_ref, sb_ref)

    def pin_st(slot, y):
        st_refs[slot][8, 0:8] = pltpu.bitcast(y, u32)

    def pin_ub(y):
        ub_ref[320, 0:8] = y

    def p1_pre(p, z, slot, rs, q):
        def item(y):
            pin_st(slot, y)
            rows = pl.multiple_of(q * 512 + p * 64 + rs * 16, 16)
            xq = bx_ref[pl.ds(rows, 16), :].astype(f32)
            zz = _r8_real([xq[:, a * 128:(a + 1) * 128] for a in range(8)])
            for t in range(4):
                for k in range(2):
                    st_refs[slot][z + t * 2 + k, (rs * 4 + q) * 8:(rs * 4 + q + 1) * 8] = (
                        _tou(zz[t][k].astype(bf16)))
        return item

    def p1_mm(p, z, slot, t):
        def item(y):
            cs = twiddles(p)

            def emit(t, rs, u):
                a = _dft4(u)
                for jq in range(4):
                    re, im = a[jq]
                    if jq > 0:
                        c, sn = cs[jq]
                        re, im = re * c + im * sn, im * c - re * sn
                    ub_ref[ub_idx(t, 0, jq, p), ub_rows(0, rs * 16, 16)] = re
                    ub_ref[ub_idx(t, 1, jq, p), ub_rows(1, rs * 16, 16)] = im

            lhs = jnp.concatenate([_tobf(st_refs[slot][z + t * 2 + k, 0:128]) for k in range(2)], axis=1)
            o = _dot(lhs, fmat(0, t))
            for rs in range(4):
                u = [(o[(rs * 4 + q) * 16:(rs * 4 + q + 1) * 16, :128],
                      o[(rs * 4 + q) * 16:(rs * 4 + q + 1) * 16, 128:]) for q in range(4)]
                if t == 0:
                    emit(4, rs, [(im, jnp.zeros_like(im)) for (_, im) in u])
                    u = [(re, jnp.where(lane0, 0.0, im)) for (re, im) in u]
                emit(t, rs, u)
        return item

    def p2_pre(u, z, rs):
        def item(y):
            pin_st(0, y)
            t = u // 4
            jq = u % 4
            tt = _dft8([(ub_ref[ub_idx(t, 0, jq, p), ub_rows(0, rs * 16, 16)],
                         ub_ref[ub_idx(t, 1, jq, p), ub_rows(1, rs * 16, 16)]) for p in range(8)])
            for jp in range(8):
                for k in range(2):
                    sa_ref[z + jp, k * 32 + rs * 8:k * 32 + (rs + 1) * 8] = _tou(tt[jp][k].astype(bf16))
        return item

    def p2_fwd(u, z, jps):
        def item(y):
            t = u // 4
            jq = u % 4
            for jp in jps:
                j = jq + 4 * jp
                xx = _dot(_tobf(ms_ref[j]), _tobf(sa_ref[z + jp, 0:64]))
                xr, xi = xx[:64], xx[64:]
                w = wp_ref[t * 32 + j]
                wr = pltpu.bitcast(w & jnp.uint32(0xFFFF0000), f32)
                wi = pltpu.bitcast(w << 16, f32)
                sb_ref[z + jp, 0:32] = _tou((xr * wr - xi * wi).astype(bf16))
                sb_ref[z + jp, 32:64] = _tou((xr * wi + xi * wr).astype(bf16))
        return item

    def p2_inv(u, z, jps):
        def item(y):
            t = u // 4
            jq = u % 4
            for jp in jps:
                zz = _dot(_tobf(ms_ref[32 + jq + 4 * jp]), _tobf(sb_ref[z + jp, 0:64]))
                ub_ref[ub_idx(t, 0, jq, jp)] = zz[:64]
                ub_ref[ub_idx(t, 1, jq, jp), 16:64] = zz[64:112]
                ub_ref[ub_idx(t, 1, jq, jp), 0:16] = zz[112:128]
        return item

    def p2_post(u, rs):
        def item(y):
            pin_ub(y)
            t = u // 4
            jq = u % 4
            rr, ri = ub_rows(0, rs * 8, 8), ub_rows(1, rs * 8, 8)
            a = _dft8([(ub_ref[ub_idx(t, 1, jq, p), ri], ub_ref[ub_idx(t, 0, jq, p), rr])
                       for p in range(8)])
            for p in range(8):
                ub_ref[ub_idx(t, 0, jq, p), rr] = a[p][1]
                ub_ref[ub_idx(t, 1, jq, p), ri] = a[p][0]
        return item

    def p3_pre(p, z, rs, t):
        def item(y):
            pin_st(0, y)
            cs = twiddles(p)
            rr, ri = ub_rows(0, rs * 16, 16), ub_rows(1, rs * 16, 16)

            def fetch(t):
                a = []
                for jq in range(4):
                    re, im = ub_ref[ub_idx(t, 0, jq, p), rr], ub_ref[ub_idx(t, 1, jq, p), ri]
                    if jq > 0:
                        c, sn = cs[jq]
                        re, im = re * c - im * sn, im * c + re * sn
                    a.append((re, im))
                return _swap(_dft4(_swap(a)))

            u = fetch(t)
            if t == 0:
                ny = fetch(4)
                u = [(u[q][0], jnp.where(lane0, ny[q][0], u[q][1])) for q in range(4)]
            for q in range(4):
                for k in range(2):
                    sa_ref[z + t * 2 + k, (q * 4 + rs) * 8:(q * 4 + rs + 1) * 8] = _tou(u[q][k].astype(bf16))
        return item

    def p3_mm(p, z, q):
        def item(y):
            g = []
            for t in range(4):
                lhs = jnp.concatenate([_tobf(sa_ref[z + t * 2 + k, q * 32:(q + 1) * 32]) for k in range(2)],
                                      axis=1)
                o = _dot(lhs, fmat(1, t))
                g.append((o[:, :128], o[:, 128:]))
            yy = _r8_real_t(g)
            rows = pl.multiple_of(q * 512 + p * 64, 64)
            for a in range(8):
                bx_ref[pl.ds(rows, 64), a * 128:(a + 1) * 128] = yy[a].astype(bf16)
        return item

    def b_out(p):
        for q in range(4):
            rows = pl.multiple_of(q * 512 + p * 64, 64)
            pltpu.make_async_copy(bx_ref.at[pl.ds(rows, 64), :],
                                  out_hbm.at[pl.ds(rows, 64), pl.ds(DM, DM)], sem_out.at[1]).start()

    def step(pp, odd, mem, hooks):
        r0 = pl.multiple_of(pp * 64 + 32 * odd, SEG)
        xs = xo_ref[pl.ds(r0, SEG), :]
        x_lo = xs[0:8].astype(f32)
        hm = jnp.concatenate(
            [jnp.concatenate([x_lo, jnp.concatenate(mem, axis=1)], axis=0).astype(bf16), xs[16:32]], axis=0)
        fill = fillo_ref[:, 0:64] if odd else fille_ref[:, 0:48]
        nrow = 48 if odd else 32
        qkv, ps = {}, {}

        def do_qkv(g):
            for h in range(g * G, (g + 1) * G):
                for t in range(3):
                    y32 = _dot(hm, _tobf(w_refs[t * 2 + h // 16][h % 16, 0:512]))
                    y = y32.astype(bf16)
                    parts = [y]
                    if odd or t > 0:
                        parts.append(_tobf(qkvc_ref[pp, t * H + h]))
                    if t > 0:
                        if odd:
                            parts.append(_tobf(kve_ref[(t - 1) * H + h]))
                        else:
                            kve_ref[(t - 1) * H + h] = _tou(y[0:16])
                    qkv[(t, h)] = jnp.concatenate(parts, axis=0) if len(parts) > 1 else y
                for item in hooks.get(h, ()):
                    item(y32[0:8])

        def do_s(g):
            for h in range(g * G, (g + 1) * G):
                sc = jax.lax.dot_general(qkv[(0, h)], qkv[(1, h)], (((1,), (1,)), ((), ())),
                                         preferred_element_type=f32)
                sc = jnp.where(fill == 0.0, sc * scale, fill)
                e = jnp.exp(sc - jnp.max(sc, axis=1, keepdims=True))
                den = jnp.sum(e, axis=1, keepdims=True)
                r = pl.reciprocal(den, approx=True)
                r = r * (2.0 - den * r)
                ps[h] = (e * r).astype(bf16)

        def do_pv(g):
            for h in range(g * G, (g + 1) * G):
                oall_ref[h, 0:nrow // 2] = _tou(_dot(ps[h], qkv[(2, h)]).astype(bf16))

        def do_o(j, h0, h1):
            lhs = jnp.concatenate([_tobf(oall_ref[h, 0:nrow // 2]) for h in range(h0, h1)], axis=1)
            return _dot(lhs, _tobf(wo_ref[j, h0 * 64:h1 * 64, :]))

        for g in range(NG):
            do_qkv(g)
            if g >= 1:
                do_s(g - 1)
            if g >= 2:
                do_pv(g - 2)
        part = {}
        for j in range(0, 3):
            part[j] = do_o(j, 0, OSPLIT)
        do_s(NG - 1)
        do_pv(NG - 2)
        for j in range(3, 6):
            part[j] = do_o(j, 0, OSPLIT)
        do_pv(NG - 1)
        for j in range(6, 8):
            part[j] = do_o(j, 0, OSPLIT)
        new_mem = []
        for j in range(8):
            cols = slice(j * 128, (j + 1) * 128)
            res = do_o(j, OSPLIT, H) + part[j]
            new_mem.append(res[8:16])
            if odd:
                xo_ref[pl.ds(r0, SEG), cols] = jnp.concatenate(
                    [res[0:8], res[40:48], res[16:32]], axis=0).astype(bf16)
                xo_ref[pl.ds(r0 - 24, 8), cols] = res[32:40].astype(bf16)
            else:
                xo_ref[pl.ds(r0, SEG), cols] = res.astype(bf16)
        for item in hooks.get(H, ()):
            item(None)
        return new_mem

    def a_out(pp):
        rows = pl.multiple_of(pp * 64, 64)
        pltpu.make_async_copy(xo_ref.at[pl.ds(rows, 64), :],
                              out_hbm.at[pl.ds(rows, 64), pl.ds(0, DM)], sem_out.at[0]).start()

    def l1(i, mem):
        z = (i // 64) * 4
        he = {h: [p1_pre(2 * i + h // 16, z, h // 16, (h % 16) // 4, h % 4)] for h in range(32)}
        he[21].append(p1_mm(2 * i, z, 0, 0))
        he[25].append(p1_mm(2 * i, z, 0, 1))
        he[29].append(p1_mm(2 * i, z, 0, 2))
        he[H] = [p1_mm(2 * i, z, 0, 3)]
        ho = {1 + 4 * t: [p1_mm(2 * i + 1, z, 1, t)] for t in range(4)}
        mem = step(i, 0, mem, he)
        mem = step(i, 1, mem, ho)
        a_out(i)
        return mem

    def l2(i, mem):
        z = (i // 64) * 4
        u = i - N_L1
        he = {1 + 2 * rs: [p2_pre(u, z, rs)] for rs in range(4)}
        he[13] = [p2_fwd(u, z, range(0, 4))]
        he[21] = [p2_fwd(u, z, range(4, 8))]
        he[H] = [p2_inv(u, z, range(0, 8))]
        ho = {3 + 2 * rs: [p2_post(u, rs)] for rs in range(8)}
        mem = step(i, 0, mem, he)
        mem = step(i, 1, mem, ho)
        a_out(i)
        return mem

    def l3(i, mem):
        z = (i // 64) * 4
        p = i - N_L1 - N_L2
        he = {h: [p3_pre(p, z, h // 4, h % 4)] for h in range(16)}
        he[21] = [p3_mm(p, z, 0)]
        he[29] = [p3_mm(p, z, 1)]
        he[H] = [p3_mm(p, z, 2)]
        ho = {5: [p3_mm(p, z, 3)]}
        mem = step(i, 0, mem, he)
        mem = step(i, 1, mem, ho)
        b_out(p)
        a_out(i)
        return mem

    m0 = mem_ref[...].astype(f32)
    mem = [m0[:, j * 128:(j + 1) * 128] for j in range(8)]
    mem = jax.lax.fori_loop(0, N_L1, l1, mem)
    mem = jax.lax.fori_loop(N_L1, N_L1 + N_L2, l2, mem)
    mem = jax.lax.fori_loop(N_L1 + N_L2, NSEG // 2, l3, mem)

    pltpu.make_async_copy(xo_ref, out_hbm.at[:, pl.ds(0, DM)], sem_out.at[0]).wait()
    pltpu.make_async_copy(bx_ref, out_hbm.at[:, pl.ds(DM, DM)], sem_out.at[1]).wait()


@jax.jit
def _run(x, mem0, wq, wk, wv, wo, bx, w_r, w_i):
    fd, ms = _tables()
    hbm = pl.BlockSpec(memory_space=pl.ANY)
    out = pl.pallas_call(
        _kernel,
        out_shape=jax.ShapeDtypeStruct((S, 2 * DM), bf16),
        in_specs=[hbm] * 12,
        out_specs=hbm,
        scratch_shapes=[
            pltpu.VMEM((S, DM), bf16),
            pltpu.VMEM((MEM, DM), bf16),
            pltpu.VMEM((8, NSEG, 8, 128), bf16),
            pltpu.VMEM((3, DM, 16, DH), bf16),
        ] + [pltpu.VMEM((16, DM // 2 + 8, DH), u32)] * 6 + [
            pltpu.VMEM((H * DH, DM), bf16),
            pltpu.VMEM((8, H * DH // 2 + 8, 128), u32),
            pltpu.VMEM((8, 256, 128), u32),
            pltpu.VMEM((NSEG // 2, 3 * H, 8, 128), u32),
            pltpu.VMEM((2 * H, 8, 128), u32),
            pltpu.VMEM((H, 24, DH), u32),
            pltpu.VMEM((32, 128), f32),
            pltpu.VMEM((48, 128), f32),
            pltpu.VMEM((S, DM), bf16),
            pltpu.VMEM((16, DM // 2 + 1, 256), bf16),
            pltpu.VMEM((161, 64, 128), u32),
            pltpu.VMEM((321, 64, 128), f32),
            pltpu.VMEM((9, 136, 128), u32),
            pltpu.VMEM((9, 136, 128), u32),
            pltpu.VMEM((16, 128, 128), u32),
            pltpu.VMEM((64, 64, 128), u32),
            pltpu.SMEM((64,), f32),
            pltpu.SemaphoreType.DMA((56,)),
            pltpu.SemaphoreType.DMA((2,)),
        ],
        compiler_params=pltpu.CompilerParams(vmem_limit_bytes=120 * 1024 * 1024),
    )(x.reshape(S, DM), x.reshape(NSEG, SEG, DM), mem0.reshape(MEM, DM), wq, wk, wv,
      wo.reshape(H * DH, DM), bx.reshape(S, DM), w_r.T, w_i.T, jnp.asarray(fd), jnp.asarray(ms))
    return out.reshape(1, S, 2 * DM)


def pallas_concat_heads__memory_aug_recurrent_mem_tr__spectral_gfnet__prompt_kernel(
    A_x: jax.Array,
    A_mem0: jax.Array,
    A_Wq: jax.Array,
    A_Wk: jax.Array,
    A_Wv: jax.Array,
    A_Wo: jax.Array,
    A_seg_len,
    B_x: jax.Array,
    B_w_r: jax.Array,
    B_w_i: jax.Array,
):
    if isinstance(A_seg_len, int):
        assert A_seg_len == SEG
    assert A_x.shape == (1, S, DM) and A_mem0.shape == (1, MEM, DM) and A_Wq.shape == (DM, H, DH)
    assert B_x.shape == (1, S, DM) and B_w_r.shape == (S, DM // 2 + 1)
    return _run(A_x, A_mem0, A_Wq, A_Wk, A_Wv, A_Wo, B_x, B_w_r, B_w_i)
```

```python
import math

import numpy as np
import jax
import jax.numpy as jnp
import jax.experimental.pallas as pl
import jax.experimental.pallas.tpu as pltpu

bf16 = jnp.bfloat16
f32 = jnp.float32
u32 = jnp.uint32

S, DM = 2048, 1024
H, DH = 32, 128
MEM, SEG = 8, 32
NSEG = S // SEG
SQH = math.sqrt(0.5)

_PAIRS = ((0, 4), (1, 7), (2, 6), (3, 5))


def _pack_rows(a):
    u = np.ascontiguousarray(a, dtype=np.float32).view(np.uint32).astype(np.uint64)
    b = ((u + 0x7FFF + ((u >> 16) & 1)) >> 16).astype(np.uint32)
    return (b[..., 0::2, :] | (b[..., 1::2, :] << 16)).astype(np.uint32)


def _tables():
    k2 = np.zeros((4, 128), np.int64)
    for t in range(4):
        odd = t % 2
        for lam in range(128):
            k = 2 * lam + odd
            if k % 8 not in _PAIRS[t]:
                k = 2 * (128 + 8 * (lam // 8) + (lam % 8 - 1 - odd) % 8) + odd
            assert k % 8 in _PAIRS[t]
            k2[t, lam] = k
    b = np.arange(128)[:, None]
    F = np.zeros((4, 256, 256))
    cw = np.full((4, 256), 2.0)
    for t in range(4):
        th = 2 * np.pi * ((b * k2[t][None, :]) % DM) / DM
        C, Sn = np.cos(th), np.sin(th)
        first = ((k2[t] % 8) == _PAIRS[t][0])[None, :]
        if t == 0:
            F[t, :128, :128] = np.where(first, C, 0)
            F[t, :128, 128:] = np.where(first, -Sn, 0)
            F[t, 128:, :128] = np.where(first, 0, C)
            F[t, 128:, 128:] = np.where(first, 0, -Sn)
            F[t, :128, 128] = (-1.0) ** np.arange(128)
            cw[t, 0] = 1.0
            cw[t, 128] = 1.0
        else:
            sg = np.where(first, 1.0, -1.0)
            F[t, :128, :128] = C
            F[t, 128:, :128] = -sg * Sn
            F[t, :128, 128:] = -Sn
            F[t, 128:, 128:] = -sg * C
    Finv = np.transpose(F * cw[:, None, :], (0, 2, 1)) / DM
    fd = np.stack([F, Finv]).reshape(2, 4, 256, 2, 128).transpose(0, 1, 3, 2, 4)
    fd = _pack_rows(fd).reshape(16, 128, 128)
    M = np.zeros((32, 128, 128))
    r = np.arange(64)[None, :]
    l = np.arange(64)[:, None]
    for j in range(32):
        th = 2 * np.pi * ((r * (j + 32 * l)) % S) / S
        C, Sn = np.cos(th), np.sin(th)
        M[j, :64, :64] = C
        M[j, :64, 64:] = Sn
        M[j, 64:, :64] = -Sn
        M[j, 64:, 64:] = C
    perm = np.arange(128).reshape(2, 8, 8).transpose(1, 0, 2).reshape(128)
    M = M[:, perm][:, :, perm]
    Minv = np.transpose(M, (0, 2, 1)) / S
    ms = _pack_rows(np.concatenate([M, Minv]))
    return fd, ms


def _tobf(w):
    return pltpu.bitcast(w, bf16)


def _tou(w):
    return pltpu.bitcast(w, u32)


def _dot(a, b):
    return jnp.dot(a, b, preferred_element_type=f32)


def _r8_real(x):
    t0, t1 = x[0] + x[4], x[0] - x[4]
    t2, t3 = x[2] + x[6], x[2] - x[6]
    t4, t5 = x[1] + x[5], x[1] - x[5]
    t6, t7 = x[3] + x[7], x[3] - x[7]
    e0, e1 = t0 + t2, t0 - t2
    o0, o1 = t4 + t6, t4 - t6
    u, v = SQH * (t5 - t7), SQH * (t5 + t7)
    return [(e0 + o0, e0 - o0), (t1 + u, v + t3), (e1, o1), (t1 - u, v - t3)]


def _r8_real_t(g):
    (z0, z4), (a1, b1), (e1, o1), (a3, b3) = g
    e0, o0 = z0 + z4, z0 - z4
    t1, u = a1 + a3, a1 - a3
    v, t3 = b1 + b3, b1 - b3
    t5, t7 = SQH * (v + u), SQH * (v - u)
    t0, t2 = e0 + e1, e0 - e1
    t4, t6 = o0 + o1, o0 - o1
    return [t0 + t1, t4 + t5, t2 + t3, t6 + t7, t0 - t1, t4 - t5, t2 - t3, t6 - t7]


def _dft4(u):
    (r0, i0), (r1, i1), (r2, i2), (r3, i3) = u
    sr, si, dr, di = r0 + r2, i0 + i2, r0 - r2, i0 - i2
    tr, ti, er, ei = r1 + r3, i1 + i3, r1 - r3, i1 - i3
    return [(sr + tr, si + ti), (dr + ei, di - er), (sr - tr, si - ti), (dr - ei, di + er)]


def _dft8(x):
    a = [(x[p][0] + x[p + 4][0], x[p][1] + x[p + 4][1]) for p in range(4)]
    d = [(x[p][0] - x[p + 4][0], x[p][1] - x[p + 4][1]) for p in range(4)]
    ev = _dft4(a)
    (r0, i0), (r1, i1), (r2, i2), (r3, i3) = d
    b1r, b1i = SQH * (r1 + i1), SQH * (i1 - r1)
    b3r, n3i = SQH * (i3 - r3), SQH * (r3 + i3)
    sr, si, dr, di = r0 + i2, i0 - r2, r0 - i2, i0 + r2
    tr, ti, er, ei = b1r + b3r, b1i - n3i, b1r - b3r, b1i + n3i
    od = [(sr + tr, si + ti), (dr + ei, di - er), (sr - tr, si - ti), (dr - ei, di + er)]
    return [ev[0], od[0], ev[1], od[1], ev[2], od[2], ev[3], od[3]]


def _swap(x):
    return [(b, a) for (a, b) in x]


G = 4
NG = H // G
OSPLIT = 24
NEG = -1e9
N_L1, N_L2, N_L3 = 4, 20, 8


def _kernel(x_hbm, x3_hbm, mem_hbm, wq_hbm, wk_hbm, wv_hbm, wo_hbm, bx_hbm, wr_hbm, wi_hbm,
            fd_hbm, ms_hbm, out_hbm,
            xo_ref, mem_ref, xcraw_ref, raw_ref, w0_ref, w1_ref, w2_ref, w3_ref, w4_ref, w5_ref,
            woraw_ref, wo_ref, xc_ref, qkvc_ref, kve_ref,
            oall_ref, fille_ref, fillo_ref, bx_ref, wt_ref, wp_ref, ub_ref, sa_ref, sb_ref, fd_ref, ms_ref,
            tw_ref, sem_in, sem_out):
    scale = DH ** -0.5
    w_hbm = (wq_hbm, wk_hbm, wv_hbm)
    w_refs = (w0_ref, w1_ref, w2_ref, w3_ref, w4_ref, w5_ref)

    def raw_copy(c, i=0, nd=DM):
        rows = pl.ds(pl.multiple_of(i * nd, nd), nd)
        return pltpu.make_async_copy(
            w_hbm[c // 2].at[rows, pl.ds((c % 2) * 16, 16), :],
            raw_ref.at[c % 4, rows], sem_in.at[8 + min(c, 3) * 8 + max(c - 3, 0) + i])

    def xc_copy(k):
        return pltpu.make_async_copy(
            x3_hbm.at[:, pl.ds(8, 8), pl.ds(pl.multiple_of(k * 128, 128), 128)], xcraw_ref.at[k], sem_in.at[40 + k])

    cp_x = pltpu.make_async_copy(x_hbm, xo_ref, sem_in.at[0])
    cp_mem = pltpu.make_async_copy(mem_hbm, mem_ref, sem_in.at[1])
    cp_wo = pltpu.make_async_copy(wo_hbm, woraw_ref, sem_in.at[2])
    cp_bx = pltpu.make_async_copy(bx_hbm, bx_ref, sem_in.at[3])
    cp_fd = pltpu.make_async_copy(fd_hbm, fd_ref, sem_in.at[4])
    cp_ms = pltpu.make_async_copy(ms_hbm, ms_ref, sem_in.at[5])
    cp_wt = [pltpu.make_async_copy(src.at[:, pl.ds(lg * 256, 256)], wt_ref.at[a * 8 + lg], sem_in.at[48 + a * 8 + lg])
             for a, src in enumerate((wr_hbm, wi_hbm)) for lg in range(8)]

    for i in range(8):
        xc_copy(i).start()
        raw_copy(0, i, 128).start()
        raw_copy(1, i, 128).start()
    for i in range(4):
        raw_copy(2, i, 256).start()
    raw_copy(3).start()

    for p in range(8):
        for jq in range(4):
            tw_ref[(p * 4 + jq) * 2] = jnp.float32(math.cos(2 * math.pi * p * jq / 32))
            tw_ref[(p * 4 + jq) * 2 + 1] = jnp.float32(math.sin(2 * math.pi * p * jq / 32))

    qi = jax.lax.broadcasted_iota(jnp.int32, (48, 128), 0)
    ki = jax.lax.broadcasted_iota(jnp.int32, (48, 128), 1)

    def between(v, lo, hi):
        return (v >= lo) & (v < hi)

    def table(keep, other):
        return jnp.where(other, -jnp.inf, jnp.where(keep, 0.0, NEG)).astype(f32)

    keep = between(qi, 8, 16) | between(ki, 8, 16) | (qi >= jnp.where(ki < 32, ki, ki - 24))
    fille_ref[...] = table(keep, ki >= 40)[:32]
    q_even = between(qi, 32, 40)
    k_even = between(ki, 32, 40) | (ki >= 48)
    qpos = jnp.where(qi < 32, qi, jnp.where(qi < 40, qi - 24, qi - 32))
    kpos = jnp.where(ki < 32, ki, jnp.where(ki < 40, ki - 24, jnp.where(ki < 48, ki - 32, ki - 48)))
    keep = between(qi, 8, 16) | between(ki, 8, 16) | (ki >= 56) | (qpos >= kpos)
    fillo_ref[...] = table(keep, (q_even != k_even) | (ki >= 64))

    def relayout16(c, d0):
        slot = c % 4
        w0 = pl.multiple_of(d0 // 2, 8)
        los, his = [], []
        for dd in range(8):
            a = _tou(raw_ref[slot, d0 + 2 * dd])
            b = _tou(raw_ref[slot, d0 + 2 * dd + 1])
            los.append((a & jnp.uint32(0xFFFF)) | (b << 16))
            his.append((a >> 16) | (b & jnp.uint32(0xFFFF0000)))
        lo = jnp.swapaxes(jnp.stack(los), 0, 1)
        hi = jnp.swapaxes(jnp.stack(his), 0, 1)
        for j in range(8):
            w_refs[c][2 * j, pl.ds(w0, 8), :] = lo[j]
            w_refs[c][2 * j + 1, pl.ds(w0, 8), :] = hi[j]

    def repack_wo64(r_start):
        r0 = pl.multiple_of(r_start, 64)
        w0 = pl.multiple_of(r_start // 2, 32)
        v = woraw_ref[pl.ds(r0, 64), :]
        for j in range(8):
            wo_ref[j, pl.ds(w0, 32), :] = _tou(v[:, j * 128:(j + 1) * 128])

    sub4 = jax.lax.broadcasted_iota(jnp.int32, (128, 128), 0) % 4

    def wp_store(t, kb, tile):
        v = tile.T
        for g in range(4):
            r0 = pl.multiple_of(t * 2560 + kb * 160 + g * 40, 8)
            wp_ref[pl.ds(r0, 32), :] = v[g * 32:(g + 1) * 32]

    def b_prep(lg, hb, par):
        cols = slice(hb * 128, (hb + 1) * 128)
        a = _tou(wt_ref[lg, 0:512, cols])
        b = _tou(wt_ref[8 + lg, 0:512, cols])
        if par == 0:
            w = (a << 16) | (b & jnp.uint32(0xFFFF))
            m = (sub4 == 0) | (sub4 == 2)
        else:
            w = (a & jnp.uint32(0xFFFF0000)) | (b >> 16)
            m = (sub4 == 0) | (sub4 == 3)
        top = w[:128]
        bot = pltpu.roll(w[128:].reshape(16, 8, 128), 1 + par, 1).reshape(128, 128)
        wp_store(par, lg * 2 + hb, jnp.where(m, top, bot))
        wp_store(par + 2, lg * 2 + hb, jnp.where(m, bot, top))
        if par == 0:
            na = jnp.broadcast_to(wt_ref[lg, 512:513, cols].astype(f32), (128, 128))
            nb = jnp.broadcast_to(wt_ref[8 + lg, 512:513, cols].astype(f32), (128, 128))
            wp_store(4, lg * 2 + hb, pltpu.bitcast(na, u32) | (pltpu.bitcast(nb, u32) >> 16))

    def gather_c(k):
        xc_ref[k] = _tou(xcraw_ref[k].astype(f32).reshape(512, 128).astype(bf16))

    def store_qkvc(n, y):
        for pp in range(NSEG // 2):
            qkvc_ref[pp, n] = y[pp * 8:(pp + 1) * 8]

    def q_unit(i, groups, first, last, fillers):
        xk = _tobf(xc_ref[i])
        w0 = pl.multiple_of(i * 64, 64)
        for g in groups:
            rhs = jnp.concatenate(
                [_tobf(w_refs[h // 16][h % 16, pl.ds(w0, 64), :]) for h in range(4 * g, 4 * g + 4)], axis=1)
            y = _dot(xk, rhs)
            for h in range(4 * g, 4 * g + 4):
                yh = y[:, (h % 4) * 128:(h % 4 + 1) * 128]
                if not first:
                    yh = yh + ub_ref[h * 4:(h + 1) * 4].reshape(512, 128)
                if last:
                    store_qkvc(h, _tou(yh.astype(bf16)))
                else:
                    ub_ref[h * 4:(h + 1) * 4] = yh.reshape(4, 128, 128)
            mine = fillers.get(g, [])
            for fi, item in enumerate(mine):
                r = (fi * 512 // len(mine)) // 8 * 8
                item(pltpu.bitcast(y[r:r + 8, 0:128], u32))

    def rl_item(c, d0):
        def item(pin):
            w_refs[c][15, 512:520] = pin
            relayout16(c, d0)
        return item

    def spread(fillers, items, groups):
        for k, item in enumerate(items):
            fillers.setdefault(groups[k * len(groups) // len(items)], []).append(item)
        return fillers

    def piece_items(i):
        f = spread({}, [rl_item(1, i * 128 + blk * 16) for blk in range(8)], (0, 1, 2))
        f = spread(f, [rl_item(0, i * 128 + blk * 16) for blk in range(8)], (4, 5, 6))
        return spread(f, [lambda pin: gather_c(i)], (6,))

    def chunk2_items(f, i):
        return spread(f, [rl_item(2, i * 256 + blk * 16) for blk in range(16)], (0, 1, 2, 3, 3, 4, 5, 6))

    def wait_piece(i):
        xc_copy(i).wait()
        raw_copy(0, i, 128).wait()
        raw_copy(1, i, 128).wait()

    xc_copy(0).wait()
    gather_c(0)
    raw_copy(0, 0, 128).wait()

    def q_pre(k, carry):
        for blk in range(4):
            relayout16(0, k * 64 + blk * 16)
        return carry
    jax.lax.fori_loop(0, 2, q_pre, 0)
    raw_copy(1, 0, 128).wait()

    def q_a(i, carry):
        q_unit(i, range(0, 4), True, False,
               spread({}, [rl_item(1, i * 128 + blk * 16) for blk in range(8)], (0, 1, 2)))
        return carry
    jax.lax.fori_loop(0, 1, q_a, 0)
    wait_piece(1)

    def q_b(i, carry):
        f = spread({}, [rl_item(0, (i + 1) * 128 + blk * 16) for blk in range(8)], (4, 5))
        f = spread(f, [rl_item(1, (i + 1) * 128 + blk * 16) for blk in range(8)], (6, 7))
        q_unit(i, range(4, 8), True, False, spread(f, [lambda pin: gather_c(i + 1)], (6,)))
        return carry
    jax.lax.fori_loop(0, 1, q_b, 0)

    def q_c(i, carry):
        wait_piece(i + 1)
        q_unit(i, range(8), False, False, piece_items(i + 1))
        return carry
    jax.lax.fori_loop(1, 4, q_c, 0)

    def q_d(i, carry):
        wait_piece(i + 1)
        raw_copy(2, i - 4, 256).wait()
        q_unit(i, range(8), False, False, chunk2_items(piece_items(i + 1), i - 4))
        return carry
    jax.lax.fori_loop(4, 7, q_d, 0)
    raw_copy(4).start()
    raw_copy(5).start()
    for cp in cp_wt:
        cp.start()
    cp_wo.start()
    cp_x.start()
    cp_mem.start()
    cp_bx.start()
    cp_fd.start()
    cp_ms.start()
    raw_copy(2, 3, 256).wait()

    def q_e(i, carry):
        q_unit(i, range(8), False, True, chunk2_items({}, i - 4))
        return carry
    jax.lax.fori_loop(7, 8, q_e, 0)

    def bulk_iter(c, i, n_rl, rl_start):
        xc = jnp.concatenate([_tobf(xc_ref[k]) for k in range(8)], axis=1)
        for t in range(8):
            n = i * 8 + t
            y = _tou(_dot(xc, _tobf(w_refs[c][n, 0:512])).astype(bf16))
            store_qkvc(c * 16 + n, y)
            for blk in range(n_rl):
                pin = y[blk * (256 // n_rl):blk * (256 // n_rl) + 8]
                if c + 1 < 6:
                    w_refs[c + 1][15, 512:520] = pin
                    relayout16(c + 1, rl_start + (t * n_rl + blk) * 16)
                else:
                    wo_ref[7, 2048:2056] = pin
                    repack_wo64(rl_start + (t * n_rl + blk) * 64)
            if c >= 4:
                wp_ref[12800:12808] = y[32:40]
                b_prep((c - 4) * 4 + i * 2 + t // 4, (t // 2) % 2, t % 2)

    for c in range(2, 6):
        if c == 4:
            for cp in cp_wt:
                cp.wait()
        if c + 1 < 6:
            raw_copy(c + 1).wait()
        else:
            cp_wo.wait()

        def bulk(i, carry, c=c):
            bulk_iter(c, i, 4, i * (512 if c + 1 < 6 else 2048))
            return carry
        jax.lax.fori_loop(0, 2, bulk, 0)

    cp_x.wait()
    cp_mem.wait()
    cp_bx.wait()
    cp_fd.wait()

    lane0 = jax.lax.broadcasted_iota(jnp.int32, (8, 128), 1) == 0

    def ub_get(n, g):
        return ub_ref[n, g * 16:g * 16 + 8], ub_ref[n, g * 16 + 8:g * 16 + 16]

    def ub_put(n, g, v):
        ub_ref[n, g * 16:g * 16 + 8] = v[0]
        ub_ref[n, g * 16 + 8:g * 16 + 16] = v[1]

    def fmat(d, t):
        return jnp.concatenate([_tobf(fd_ref[d * 8 + t * 2]), _tobf(fd_ref[d * 8 + t * 2 + 1])], axis=1)

    def twiddles(p):
        return [(tw_ref[(p * 4 + jq) * 2], tw_ref[(p * 4 + jq) * 2 + 1]) for jq in range(4)]

    st_refs = (sa_ref, sb_ref)

    def p1_pre(p, z, slot, rs, q):
        def item(y):
            st_refs[slot][8, 0:8] = y
            rows = pl.multiple_of(q * 512 + p * 64 + rs * 16, 16)
            xq = bx_ref[pl.ds(rows, 16), :].astype(f32)
            zz = _r8_real([xq[:, a * 128:(a + 1) * 128] for a in range(8)])
            for t in range(4):
                for k in range(2):
                    for e in range(2):
                        r = ((rs * 2 + e) * 4 + q) * 8
                        st_refs[slot][z + t * 2 + k, r:r + 8] = zz[t][k][e * 8:(e + 1) * 8]
        return item

    def p1_mm(p, z, slot, t):
        def item(y):
            cs = twiddles(p)

            def emit(t, g, u):
                a = _dft4(u)
                for jq in range(4):
                    re, im = a[jq]
                    if jq > 0:
                        c, sn = cs[jq]
                        re, im = re * c + im * sn, im * c - re * sn
                    ub_put((t * 4 + jq) * 8 + p, g, (re, im))

            lhs = jnp.concatenate([st_refs[slot][z + t * 2 + k, 0:256] for k in range(2)], axis=1)
            o = _dot(lhs.astype(bf16), fmat(0, t))
            for g in range(8):
                u = [(o[(g * 4 + q) * 8:(g * 4 + q + 1) * 8, :128],
                      o[(g * 4 + q) * 8:(g * 4 + q + 1) * 8, 128:]) for q in range(4)]
                if t == 0:
                    emit(4, g, [(im, jnp.zeros_like(im)) for (_, im) in u])
                    u = [(re, jnp.where(lane0, 0.0, im)) for (re, im) in u]
                emit(t, g, u)
        return item

    def p2_bfly(u, g, inverse):
        def item(y):
            if y is not None:
                ub_ref[168, 0:8] = y
            x = [ub_get(u * 8 + p, g) for p in range(8)]
            x = _swap(_dft8(_swap(x))) if inverse else _dft8(x)
            for p in range(8):
                ub_put(u * 8 + p, g, x[p])
        return item

    def p2_fwd(u, jps):
        def item(y):
            t = u // 4
            jq = u % 4
            xs = [_dot(_tobf(ms_ref[jq + 4 * jp]), ub_ref[u * 8 + jp].astype(bf16)) for jp in jps]
            for jp, xx in zip(jps, xs):
                w = wp_ref[pl.ds(t * 2560 + jq + 4 * jp, 64, stride=40), :]
                wr = pltpu.bitcast(w & jnp.uint32(0xFFFF0000), f32)
                wi = pltpu.bitcast(w << 16, f32)
                for g in range(8):
                    xr, xi = xx[g * 16:g * 16 + 8], xx[g * 16 + 8:g * 16 + 16]
                    a, b = wr[g * 8:(g + 1) * 8], wi[g * 8:(g + 1) * 8]
                    ub_put(u * 8 + jp, g, (xr * a - xi * b, xr * b + xi * a))
        return item

    def p2_inv(u, jps):
        def item(y):
            jq = u % 4
            zs = [_dot(_tobf(ms_ref[32 + jq + 4 * jp]), ub_ref[u * 8 + jp].astype(bf16)) for jp in jps]
            for jp, zz in zip(jps, zs):
                ub_ref[u * 8 + jp] = zz
        return item

    def p3_pre(p, z, g, ts):
        def item(y):
            sa_ref[8, 0:8] = y
            cs = twiddles(p)

            def fetch(t):
                a = []
                for jq in range(4):
                    re, im = ub_get((t * 4 + jq) * 8 + p, g)
                    if jq > 0:
                        c, sn = cs[jq]
                        re, im = re * c - im * sn, im * c + re * sn
                    a.append((re, im))
                return _swap(_dft4(_swap(a)))

            for t in ts:
                u = fetch(t)
                if t == 0:
                    ny = fetch(4)
                    u = [(u[q][0], jnp.where(lane0, ny[q][0], u[q][1])) for q in range(4)]
                for q in range(4):
                    for k in range(2):
                        sa_ref[z + t * 2 + k, q * 64 + g * 8:q * 64 + (g + 1) * 8] = u[q][k]
        return item

    def p3_mm(p, z, q):
        def item(y):
            g = []
            for t in range(4):
                lhs = jnp.concatenate([sa_ref[z + t * 2 + k, q * 64:(q + 1) * 64] for k in range(2)], axis=1)
                o = _dot(lhs.astype(bf16), fmat(1, t))
                g.append((o[:, :128], o[:, 128:]))
            yy = _r8_real_t(g)
            rows = pl.multiple_of(q * 512 + p * 64, 64)
            for a in range(8):
                bx_ref[pl.ds(rows, 64), a * 128:(a + 1) * 128] = yy[a].astype(bf16)
        return item

    def b_out(p):
        for q in range(4):
            rows = pl.multiple_of(q * 512 + p * 64, 64)
            pltpu.make_async_copy(bx_ref.at[pl.ds(rows, 64), :],
                                  out_hbm.at[pl.ds(rows, 64), pl.ds(DM, DM)], sem_out.at[1]).start()

    def step(pp, odd, mem, hooks):
        r0 = pl.multiple_of(pp * 64 + 32 * odd, SEG)
        xs = xo_ref[pl.ds(r0, SEG), :]
        x_lo = xs[0:8].astype(f32)
        hm = jnp.concatenate(
            [jnp.concatenate([x_lo, jnp.concatenate(mem, axis=1)], axis=0).astype(bf16), xs[16:32]], axis=0)
        fill = fillo_ref[:, 0:64] if odd else fille_ref[:, 0:48]
        nrow = 48 if odd else 32
        qkv, ps = {}, {}

        def do_qkv(g):
            for h in range(g * G, (g + 1) * G):
                for t in range(3):
                    y32 = _dot(hm, _tobf(w_refs[t * 2 + h // 16][h % 16, 0:512]))
                    y = y32.astype(bf16)
                    parts = [y]
                    if odd or t > 0:
                        parts.append(_tobf(qkvc_ref[pp, t * H + h]))
                    if t > 0:
                        if odd:
                            parts.append(_tobf(kve_ref[(t - 1) * H + h]))
                        else:
                            kve_ref[(t - 1) * H + h] = _tou(y[0:16])
                    qkv[(t, h)] = jnp.concatenate(parts, axis=0) if len(parts) > 1 else y
                for item in hooks.get(h, ()):
                    item(y32[0:8])

        def do_s(g):
            for h in range(g * G, (g + 1) * G):
                sc = jax.lax.dot_general(qkv[(0, h)], qkv[(1, h)], (((1,), (1,)), ((), ())),
                                         preferred_element_type=f32)
                sc = jnp.where(fill == 0.0, sc * scale, fill)
                e = jnp.exp(sc - jnp.max(sc, axis=1, keepdims=True))
                den = jnp.sum(e, axis=1, keepdims=True)
                r = pl.reciprocal(den, approx=True)
                r = r * (2.0 - den * r)
                ps[h] = (e * r).astype(bf16)

        def do_pv(g):
            for h in range(g * G, (g + 1) * G):
                oall_ref[h, 0:nrow // 2] = _tou(_dot(ps[h], qkv[(2, h)]).astype(bf16))

        def do_o(j, h0, h1):
            lhs = jnp.concatenate([_tobf(oall_ref[h, 0:nrow // 2]) for h in range(h0, h1)], axis=1)
            return _dot(lhs, _tobf(wo_ref[j, h0 * 64:h1 * 64, :]))

        for g in range(NG):
            do_qkv(g)
            if g >= 1:
                do_s(g - 1)
            if g >= 2:
                do_pv(g - 2)
        part = {}
        for j in range(8):
            part[j] = do_o(j, 0, OSPLIT)
            for k, item in enumerate(hooks.get(('o', j), ())):
                item(part[j][k * 16:k * 16 + 8])
            if j == 2:
                do_s(NG - 1)
                do_pv(NG - 2)
            if j == 5:
                do_pv(NG - 1)
        new_mem = []
        for j in range(8):
            cols = slice(j * 128, (j + 1) * 128)
            res = do_o(j, OSPLIT, H) + part[j]
            new_mem.append(res[8:16])
            if odd:
                xo_ref[pl.ds(r0, SEG), cols] = jnp.concatenate(
                    [res[0:8], res[40:48], res[16:32]], axis=0).astype(bf16)
                xo_ref[pl.ds(r0 - 24, 8), cols] = res[32:40].astype(bf16)
            else:
                xo_ref[pl.ds(r0, SEG), cols] = res.astype(bf16)
        for item in hooks.get(H, ()):
            item(None)
        return new_mem

    def a_out(pp):
        rows = pl.multiple_of(pp * 64, 64)
        pltpu.make_async_copy(xo_ref.at[pl.ds(rows, 64), :],
                              out_hbm.at[pl.ds(rows, 64), pl.ds(0, DM)], sem_out.at[0]).start()

    def l1(i, mem):
        z = (i // 64) * 4
        he = {h: [p1_pre(2 * i + h // 16, z, h // 16, (h % 16) // 4, h % 4)] for h in range(32)}
        he[21].append(p1_mm(2 * i, z, 0, 0))
        he[25].append(p1_mm(2 * i, z, 0, 1))
        he[29].append(p1_mm(2 * i, z, 0, 2))
        he[H] = [p1_mm(2 * i, z, 0, 3)]
        ho = {1 + 4 * t: [p1_mm(2 * i + 1, z, 1, t)] for t in range(4)}
        mem = step(i, 0, mem, he)
        mem = step(i, 1, mem, ho)
        a_out(i)
        return mem

    def l2(i, mem):
        u = i - N_L1
        he = {13: [p2_fwd(u, range(0, 4))], 21: [p2_fwd(u, range(4, 8))], H: [p2_inv(u, range(0, 8))]}
        ho = {('o', j): [p2_bfly(u, j, True), p2_bfly(u + 1, j, False)] for j in range(8)}
        mem = step(i, 0, mem, he)
        mem = step(i, 1, mem, ho)
        a_out(i)
        return mem

    def l3(i, mem):
        z = (i // 64) * 4
        p = i - N_L1 - N_L2
        he = {h: [p3_pre(p, z, h // 2, (0, 1) if h % 2 == 0 else (2, 3))] for h in range(16)}
        he[21] = [p3_mm(p, z, 0)]
        he[29] = [p3_mm(p, z, 1)]
        he[H] = [p3_mm(p, z, 2)]
        ho = {5: [p3_mm(p, z, 3)]}
        mem = step(i, 0, mem, he)
        mem = step(i, 1, mem, ho)
        b_out(p)
        a_out(i)
        return mem

    m0 = mem_ref[...].astype(f32)
    mem = [m0[:, j * 128:(j + 1) * 128] for j in range(8)]
    mem = jax.lax.fori_loop(0, N_L1, l1, mem)
    cp_ms.wait()
    for g in range(8):
        p2_bfly(0, g, False)(None)
    mem = jax.lax.fori_loop(N_L1, N_L1 + N_L2, l2, mem)
    mem = jax.lax.fori_loop(N_L1 + N_L2, NSEG // 2, l3, mem)

    pltpu.make_async_copy(xo_ref, out_hbm.at[:, pl.ds(0, DM)], sem_out.at[0]).wait()
    pltpu.make_async_copy(bx_ref, out_hbm.at[:, pl.ds(DM, DM)], sem_out.at[1]).wait()


@jax.jit
def _run(x, mem0, wq, wk, wv, wo, bx, w_r, w_i):
    fd, ms = _tables()
    hbm = pl.BlockSpec(memory_space=pl.ANY)
    out = pl.pallas_call(
        _kernel,
        out_shape=jax.ShapeDtypeStruct((S, 2 * DM), bf16),
        in_specs=[hbm] * 12,
        out_specs=hbm,
        scratch_shapes=[
            pltpu.VMEM((S, DM), bf16),
            pltpu.VMEM((MEM, DM), bf16),
            pltpu.VMEM((8, NSEG, 8, 128), bf16),
            pltpu.VMEM((4, DM, 16, DH), bf16),
        ] + [pltpu.VMEM((16, DM // 2 + 8, DH), u32)] * 6 + [
            pltpu.VMEM((H * DH, DM), bf16),
            pltpu.VMEM((8, H * DH // 2 + 8, 128), u32),
            pltpu.VMEM((8, 256, 128), u32),
            pltpu.VMEM((NSEG // 2, 3 * H, 8, 128), u32),
            pltpu.VMEM((2 * H, 8, 128), u32),
            pltpu.VMEM((H, 24, DH), u32),
            pltpu.VMEM((32, 128), f32),
            pltpu.VMEM((48, 128), f32),
            pltpu.VMEM((S, DM), bf16),
            pltpu.VMEM((16, DM // 2 + 1, 256), bf16),
            pltpu.VMEM((12808, 128), u32),
            pltpu.VMEM((169, 128, 128), f32),
            pltpu.VMEM((9, 264, 128), f32),
            pltpu.VMEM((9, 264, 128), f32),
            pltpu.VMEM((16, 128, 128), u32),
            pltpu.VMEM((64, 64, 128), u32),
            pltpu.SMEM((64,), f32),
            pltpu.SemaphoreType.DMA((64,)),
            pltpu.SemaphoreType.DMA((2,)),
        ],
        compiler_params=pltpu.CompilerParams(vmem_limit_bytes=120 * 1024 * 1024),
    )(x.reshape(S, DM), x.reshape(NSEG, SEG, DM), mem0.reshape(MEM, DM), wq, wk, wv,
      wo.reshape(H * DH, DM), bx.reshape(S, DM), w_r.T, w_i.T, jnp.asarray(fd), jnp.asarray(ms))
    return out.reshape(1, S, 2 * DM)


def pallas_concat_heads__memory_aug_recurrent_mem_tr__spectral_gfnet__prompt_kernel(
    A_x: jax.Array,
    A_mem0: jax.Array,
    A_Wq: jax.Array,
    A_Wk: jax.Array,
    A_Wv: jax.Array,
    A_Wo: jax.Array,
    A_seg_len,
    B_x: jax.Array,
    B_w_r: jax.Array,
    B_w_i: jax.Array,
):
    if isinstance(A_seg_len, int):
        assert A_seg_len == SEG
    assert A_x.shape == (1, S, DM) and A_mem0.shape == (1, MEM, DM) and A_Wq.shape == (DM, H, DH)
    assert B_x.shape == (1, S, DM) and B_w_r.shape == (S, DM // 2 + 1)
    return _run(A_x, A_mem0, A_Wq, A_Wk, A_Wv, A_Wo, B_x, B_w_r, B_w_i)
```

```python
import math

import numpy as np
import jax
import jax.numpy as jnp
import jax.experimental.pallas as pl
import jax.experimental.pallas.tpu as pltpu

bf16 = jnp.bfloat16
f32 = jnp.float32
u32 = jnp.uint32

S, DM = 2048, 1024
H, DH = 32, 128
MEM, SEG = 8, 32
NSEG = S // SEG
SQH = math.sqrt(0.5)

_PAIRS = ((0, 4), (1, 7), (2, 6), (3, 5))


def _pack_rows(a):
    u = np.ascontiguousarray(a, dtype=np.float32).view(np.uint32).astype(np.uint64)
    b = ((u + 0x7FFF + ((u >> 16) & 1)) >> 16).astype(np.uint32)
    return (b[..., 0::2, :] | (b[..., 1::2, :] << 16)).astype(np.uint32)


def _tables():
    k2 = np.zeros((4, 128), np.int64)
    for t in range(4):
        odd = t % 2
        for lam in range(128):
            k = 2 * lam + odd
            if k % 8 not in _PAIRS[t]:
                k = 2 * (128 + 8 * (lam // 8) + (lam % 8 - 1 - odd) % 8) + odd
            assert k % 8 in _PAIRS[t]
            k2[t, lam] = k
    b = np.arange(128)[:, None]
    F = np.zeros((4, 256, 256))
    cw = np.full((4, 256), 2.0)
    for t in range(4):
        th = 2 * np.pi * ((b * k2[t][None, :]) % DM) / DM
        C, Sn = np.cos(th), np.sin(th)
        first = ((k2[t] % 8) == _PAIRS[t][0])[None, :]
        if t == 0:
            F[t, :128, :128] = np.where(first, C, 0)
            F[t, :128, 128:] = np.where(first, -Sn, 0)
            F[t, 128:, :128] = np.where(first, 0, C)
            F[t, 128:, 128:] = np.where(first, 0, -Sn)
            F[t, :128, 128] = (-1.0) ** np.arange(128)
            cw[t, 0] = 1.0
            cw[t, 128] = 1.0
        else:
            sg = np.where(first, 1.0, -1.0)
            F[t, :128, :128] = C
            F[t, 128:, :128] = -sg * Sn
            F[t, :128, 128:] = -Sn
            F[t, 128:, 128:] = -sg * C
    Finv = np.transpose(F * cw[:, None, :], (0, 2, 1)) / DM
    fd = np.stack([F, Finv]).reshape(2, 4, 256, 2, 128).transpose(0, 1, 3, 2, 4)
    fd = _pack_rows(fd).reshape(16, 128, 128)
    M = np.zeros((32, 128, 128))
    r = np.arange(64)[None, :]
    l = np.arange(64)[:, None]
    for j in range(32):
        th = 2 * np.pi * ((r * (j + 32 * l)) % S) / S
        C, Sn = np.cos(th), np.sin(th)
        M[j, :64, :64] = C
        M[j, :64, 64:] = Sn
        M[j, 64:, :64] = -Sn
        M[j, 64:, 64:] = C
    perm = np.arange(128).reshape(2, 8, 8).transpose(1, 0, 2).reshape(128)
    M = M[:, perm][:, :, perm]
    Minv = np.transpose(M, (0, 2, 1)) / S
    ms = _pack_rows(np.concatenate([M, Minv]))
    return fd, ms


def _tobf(w):
    return pltpu.bitcast(w, bf16)


def _tou(w):
    return pltpu.bitcast(w, u32)


def _dot(a, b):
    return jnp.dot(a, b, preferred_element_type=f32)


def _r8_real(x):
    t0, t1 = x[0] + x[4], x[0] - x[4]
    t2, t3 = x[2] + x[6], x[2] - x[6]
    t4, t5 = x[1] + x[5], x[1] - x[5]
    t6, t7 = x[3] + x[7], x[3] - x[7]
    e0, e1 = t0 + t2, t0 - t2
    o0, o1 = t4 + t6, t4 - t6
    u, v = SQH * (t5 - t7), SQH * (t5 + t7)
    return [(e0 + o0, e0 - o0), (t1 + u, v + t3), (e1, o1), (t1 - u, v - t3)]


def _r8_real_t(g):
    (z0, z4), (a1, b1), (e1, o1), (a3, b3) = g
    e0, o0 = z0 + z4, z0 - z4
    t1, u = a1 + a3, a1 - a3
    v, t3 = b1 + b3, b1 - b3
    t5, t7 = SQH * (v + u), SQH * (v - u)
    t0, t2 = e0 + e1, e0 - e1
    t4, t6 = o0 + o1, o0 - o1
    return [t0 + t1, t4 + t5, t2 + t3, t6 + t7, t0 - t1, t4 - t5, t2 - t3, t6 - t7]


def _dft4(u):
    (r0, i0), (r1, i1), (r2, i2), (r3, i3) = u
    sr, si, dr, di = r0 + r2, i0 + i2, r0 - r2, i0 - i2
    tr, ti, er, ei = r1 + r3, i1 + i3, r1 - r3, i1 - i3
    return [(sr + tr, si + ti), (dr + ei, di - er), (sr - tr, si - ti), (dr - ei, di + er)]


def _dft8(x):
    a = [(x[p][0] + x[p + 4][0], x[p][1] + x[p + 4][1]) for p in range(4)]
    d = [(x[p][0] - x[p + 4][0], x[p][1] - x[p + 4][1]) for p in range(4)]
    ev = _dft4(a)
    (r0, i0), (r1, i1), (r2, i2), (r3, i3) = d
    b1r, b1i = SQH * (r1 + i1), SQH * (i1 - r1)
    b3r, n3i = SQH * (i3 - r3), SQH * (r3 + i3)
    sr, si, dr, di = r0 + i2, i0 - r2, r0 - i2, i0 + r2
    tr, ti, er, ei = b1r + b3r, b1i - n3i, b1r - b3r, b1i + n3i
    od = [(sr + tr, si + ti), (dr + ei, di - er), (sr - tr, si - ti), (dr - ei, di + er)]
    return [ev[0], od[0], ev[1], od[1], ev[2], od[2], ev[3], od[3]]


def _swap(x):
    return [(b, a) for (a, b) in x]


G = 4
NG = H // G
OSPLIT = 24
NEG = -1e9
N_L1, N_L2, N_L3 = 4, 20, 8


def _kernel(x_hbm, x3_hbm, mem_hbm, wq_hbm, wk_hbm, wv_hbm, wo_hbm, bx_hbm, wr_hbm, wi_hbm,
            fd_hbm, ms_hbm, out_hbm,
            xo_ref, mem_ref, xcraw_ref, raw_ref, w0_ref, w1_ref, w2_ref, w3_ref, w4_ref, w5_ref,
            woraw_ref, wo_ref, xc_ref, qkvc_ref, kve_ref,
            oall_ref, fille_ref, fillo_ref, bx_ref, wt_ref, wp_ref, ub_ref, sa_ref, sb_ref, fd_ref, ms_ref,
            tw_ref, zero_ref, sem_in, sem_out):
    scale = DH ** -0.5
    w_hbm = (wq_hbm, wk_hbm, wv_hbm)
    w_refs = (w0_ref, w1_ref, w2_ref, w3_ref, w4_ref, w5_ref)

    def raw_copy(c, i=0, nd=DM):
        rows = pl.ds(pl.multiple_of(i * nd, nd), nd)
        return pltpu.make_async_copy(
            w_hbm[c // 2].at[rows, pl.ds((c % 2) * 16, 16), :],
            raw_ref.at[c % 4, rows], sem_in.at[8 + min(c, 3) * 8 + max(c - 3, 0) * 2 + i])

    def xc_copy(k):
        return pltpu.make_async_copy(
            x3_hbm.at[:, pl.ds(8, 8), pl.ds(pl.multiple_of(k * 128, 128), 128)], xcraw_ref.at[k], sem_in.at[40 + k])

    cp_x = pltpu.make_async_copy(x_hbm, xo_ref, sem_in.at[0])
    cp_mem = pltpu.make_async_copy(mem_hbm, mem_ref, sem_in.at[1])
    cp_wo = pltpu.make_async_copy(wo_hbm, woraw_ref, sem_in.at[2])
    cp_bx = pltpu.make_async_copy(bx_hbm, bx_ref, sem_in.at[3])
    cp_fd = pltpu.make_async_copy(fd_hbm, fd_ref, sem_in.at[4])
    cp_ms = pltpu.make_async_copy(ms_hbm, ms_ref, sem_in.at[5])
    cp_wt = [pltpu.make_async_copy(src.at[:, pl.ds(lg * 256, 256)], wt_ref.at[a * 8 + lg], sem_in.at[48 + a * 8 + lg])
             for a, src in enumerate((wr_hbm, wi_hbm)) for lg in range(8)]

    for i in range(8):
        xc_copy(i).start()
        raw_copy(0, i, 128).start()
        raw_copy(1, i, 128).start()
    for i in range(4):
        raw_copy(2, i, 256).start()
    for i in range(2):
        raw_copy(3, i, 512).start()

    zero_ref[0] = 0

    def pin_rows(r):
        return pl.ds(pl.multiple_of(r + zero_ref[0] * 32, 8), 8)

    for p in range(8):
        for jq in range(4):
            tw_ref[(p * 4 + jq) * 2] = jnp.float32(math.cos(2 * math.pi * p * jq / 32))
            tw_ref[(p * 4 + jq) * 2 + 1] = jnp.float32(math.sin(2 * math.pi * p * jq / 32))

    qi = jax.lax.broadcasted_iota(jnp.int32, (48, 128), 0)
    ki = jax.lax.broadcasted_iota(jnp.int32, (48, 128), 1)

    def between(v, lo, hi):
        return (v >= lo) & (v < hi)

    def table(keep, other):
        return jnp.where(other, -jnp.inf, jnp.where(keep, 0.0, NEG)).astype(f32)

    keep = between(qi, 8, 16) | between(ki, 8, 16) | (qi >= jnp.where(ki < 32, ki, ki - 24))
    fille_ref[...] = table(keep, ki >= 40)[:32]
    q_even = between(qi, 32, 40)
    k_even = between(ki, 32, 40) | (ki >= 48)
    qpos = jnp.where(qi < 32, qi, jnp.where(qi < 40, qi - 24, qi - 32))
    kpos = jnp.where(ki < 32, ki, jnp.where(ki < 40, ki - 24, jnp.where(ki < 48, ki - 32, ki - 48)))
    keep = between(qi, 8, 16) | between(ki, 8, 16) | (ki >= 56) | (qpos >= kpos)
    fillo_ref[...] = table(keep, (q_even != k_even) | (ki >= 64))

    def relayout16(c, d0):
        slot = c % 4
        w0 = pl.multiple_of(d0 // 2, 8)
        los, his = [], []
        for dd in range(8):
            a = _tou(raw_ref[slot, d0 + 2 * dd])
            b = _tou(raw_ref[slot, d0 + 2 * dd + 1])
            los.append((a & jnp.uint32(0xFFFF)) | (b << 16))
            his.append((a >> 16) | (b & jnp.uint32(0xFFFF0000)))
        lo = jnp.swapaxes(jnp.stack(los), 0, 1)
        hi = jnp.swapaxes(jnp.stack(his), 0, 1)
        for j in range(8):
            w_refs[c][2 * j, pl.ds(w0, 8), :] = lo[j]
            w_refs[c][2 * j + 1, pl.ds(w0, 8), :] = hi[j]

    def repack_wo64(r_start):
        r0 = pl.multiple_of(r_start, 64)
        w0 = pl.multiple_of(r_start // 2, 32)
        v = woraw_ref[pl.ds(r0, 64), :]
        for j in range(8):
            wo_ref[j, pl.ds(w0, 32), :] = _tou(v[:, j * 128:(j + 1) * 128])

    sub4 = jax.lax.broadcasted_iota(jnp.int32, (128, 128), 0) % 4

    def wp_store(t, kb, tile):
        v = tile.T
        for g in range(4):
            r0 = pl.multiple_of(t * 2560 + kb * 160 + g * 40, 8)
            wp_ref[pl.ds(r0, 32), :] = v[g * 32:(g + 1) * 32]

    def b_prep(lg, hb, par):
        cols = slice(hb * 128, (hb + 1) * 128)
        a = _tou(wt_ref[lg, 0:512, cols])
        b = _tou(wt_ref[8 + lg, 0:512, cols])
        if par == 0:
            w = (a << 16) | (b & jnp.uint32(0xFFFF))
            m = (sub4 == 0) | (sub4 == 2)
        else:
            w = (a & jnp.uint32(0xFFFF0000)) | (b >> 16)
            m = (sub4 == 0) | (sub4 == 3)
        top = w[:128]
        bot = pltpu.roll(w[128:].reshape(16, 8, 128), 1 + par, 1).reshape(128, 128)
        wp_store(par, lg * 2 + hb, jnp.where(m, top, bot))
        wp_store(par + 2, lg * 2 + hb, jnp.where(m, bot, top))
        if par == 0:
            na = jnp.broadcast_to(wt_ref[lg, 512:513, cols].astype(f32), (128, 128))
            nb = jnp.broadcast_to(wt_ref[8 + lg, 512:513, cols].astype(f32), (128, 128))
            wp_store(4, lg * 2 + hb, pltpu.bitcast(na, u32) | (pltpu.bitcast(nb, u32) >> 16))

    def gather_c(k):
        xc_ref[k] = _tou(xcraw_ref[k].astype(f32).reshape(512, 128).astype(bf16))

    def store_qkvc(n, y):
        for pp in range(NSEG // 2):
            qkvc_ref[pp, n] = y[pp * 8:(pp + 1) * 8]

    def q_unit(i, groups, first, last, fillers):
        xk = _tobf(xc_ref[i])
        w0 = pl.multiple_of(i * 64, 64)
        for g in groups:
            rhs = jnp.concatenate(
                [_tobf(w_refs[h // 16][h % 16, pl.ds(w0, 64), :]) for h in range(4 * g, 4 * g + 4)], axis=1)
            y = _dot(xk, rhs)
            for h in range(4 * g, 4 * g + 4):
                yh = y[:, (h % 4) * 128:(h % 4 + 1) * 128]
                if not first:
                    yh = yh + ub_ref[h * 4:(h + 1) * 4].reshape(512, 128)
                if last:
                    store_qkvc(h, _tou(yh.astype(bf16)))
                else:
                    ub_ref[h * 4:(h + 1) * 4] = yh.reshape(4, 128, 128)
            mine = fillers.get(g, [])
            for fi, item in enumerate(mine):
                r = (fi * 512 // len(mine)) // 8 * 8
                item(pltpu.bitcast(y[r:r + 8, 0:128], u32))

    def rl_item(c, d0):
        def item(pin):
            w_refs[c][15, pin_rows(512), :] = pin
            relayout16(c, d0)
        return item

    def spread(fillers, items, groups):
        for k, item in enumerate(items):
            fillers.setdefault(groups[k * len(groups) // len(items)], []).append(item)
        return fillers

    def half_items(f, c, i, groups):
        return spread(f, [rl_item(c, i * 128 + blk * 16) for blk in range(8)], groups)

    def piece_items(i):
        f = half_items(half_items({}, 1, i, (0, 1, 2)), 0, i + 1, (4, 5, 6))
        return spread(f, [lambda pin: gather_c(i + 1)], (6,))

    def chunk2_items(f, i, groups):
        return spread(f, [rl_item(2, i * 256 + blk * 16) for blk in range(16)], groups)

    def wait_piece(i):
        raw_copy(1, i, 128).wait()
        xc_copy(i + 1).wait()
        raw_copy(0, i + 1, 128).wait()

    xc_copy(0).wait()
    gather_c(0)
    raw_copy(0, 0, 128).wait()
    for blk in range(8):
        relayout16(0, blk * 16)
    q_unit(0, range(0, 2), True, False, {})
    raw_copy(1, 0, 128).wait()
    q_unit(0, range(2, 4), True, False, half_items({}, 1, 0, (2, 2, 3)))
    xc_copy(1).wait()
    raw_copy(0, 1, 128).wait()
    q_unit(0, range(4, 8), True, False,
           spread(half_items({}, 0, 1, (4, 5, 6)), [lambda pin: gather_c(1)], (6,)))

    def q_c(i, carry):
        wait_piece(i)
        q_unit(i, range(8), False, False, piece_items(i))
        return carry
    jax.lax.fori_loop(1, 5, q_c, 0)

    wait_piece(5)
    raw_copy(2, 0, 256).wait()
    raw_copy(2, 1, 256).wait()
    q_unit(5, range(8), False, False,
           chunk2_items(chunk2_items(piece_items(5), 0, (0, 1, 2, 3, 3)), 1, (3, 4, 5, 6, 7)))
    wait_piece(6)
    raw_copy(1, 7, 128).wait()
    raw_copy(2, 2, 256).wait()
    raw_copy(2, 3, 256).wait()
    q_unit(6, range(8), False, False, chunk2_items(piece_items(6), 2, (0, 1, 2, 3, 3, 4, 5, 7)))
    raw_copy(4).start()
    q_unit(7, range(8), False, True, chunk2_items(half_items({}, 1, 7, (0, 1, 2)), 3, (3, 4, 5, 6)))
    raw_copy(5).start()
    for cp in cp_wt:
        cp.start()
    cp_wo.start()
    cp_x.start()
    cp_mem.start()
    cp_bx.start()
    cp_fd.start()
    cp_ms.start()

    def bulk_iter(c, i, n_rl, rl_start):
        xc = jnp.concatenate([_tobf(xc_ref[k]) for k in range(8)], axis=1)
        for t in range(8):
            n = i * 8 + t
            y = _tou(_dot(xc, _tobf(w_refs[c][n, 0:512])).astype(bf16))
            store_qkvc(c * 16 + n, y)
            for blk in range(n_rl):
                pin = y[blk * (256 // n_rl):blk * (256 // n_rl) + 8]
                if c + 1 < 6:
                    w_refs[c + 1][15, pin_rows(512), :] = pin
                    relayout16(c + 1, rl_start + (t * n_rl + blk) * 16)
                else:
                    wo_ref[7, pin_rows(2048), :] = pin
                    repack_wo64(rl_start + (t * n_rl + blk) * 64)
            if c >= 4:
                wp_ref[pin_rows(12800), :] = y[32:40]
                b_prep((c - 4) * 4 + i * 2 + t // 4, (t // 2) % 2, t % 2)

    for c in range(2, 6):
        if c == 4:
            for cp in cp_wt:
                cp.wait()
        if c == 5:
            cp_wo.wait()
        elif c > 2:
            raw_copy(c + 1).wait()

        def bulk(i, carry, c=c):
            if c == 2:
                raw_copy(3, i, 512).wait()
            bulk_iter(c, i, 4, i * (512 if c + 1 < 6 else 2048))
            return carry
        jax.lax.fori_loop(0, 2, bulk, 0)

    cp_x.wait()
    cp_mem.wait()
    cp_bx.wait()
    cp_fd.wait()

    lane0 = jax.lax.broadcasted_iota(jnp.int32, (8, 128), 1) == 0

    def ub_get(n, g):
        return ub_ref[n, g * 16:g * 16 + 8], ub_ref[n, g * 16 + 8:g * 16 + 16]

    def ub_put(n, g, v):
        ub_ref[n, g * 16:g * 16 + 8] = v[0]
        ub_ref[n, g * 16 + 8:g * 16 + 16] = v[1]

    def fmat(d, t):
        return jnp.concatenate([_tobf(fd_ref[d * 8 + t * 2]), _tobf(fd_ref[d * 8 + t * 2 + 1])], axis=1)

    def twiddles(p):
        return [(tw_ref[(p * 4 + jq) * 2], tw_ref[(p * 4 + jq) * 2 + 1]) for jq in range(4)]

    st_refs = (sa_ref, sb_ref)

    def p1_pre(p, slot, rs, q):
        def item(y):
            st_refs[slot][7, pin_rows(256), :] = y
            rows = pl.multiple_of(q * 512 + p * 64 + rs * 16, 16)
            xq = bx_ref[pl.ds(rows, 16), :].astype(f32)
            zz = _r8_real([xq[:, a * 128:(a + 1) * 128] for a in range(8)])
            for t in range(4):
                for k in range(2):
                    for e in range(2):
                        r = ((rs * 2 + e) * 4 + q) * 8
                        st_refs[slot][t * 2 + k, r:r + 8] = zz[t][k][e * 8:(e + 1) * 8]
        return item

    def p1_mm(p, slot, t):
        def item(y):
            cs = twiddles(p)

            def emit(t, g, u):
                a = _dft4(u)
                for jq in range(4):
                    re, im = a[jq]
                    if jq > 0:
                        c, sn = cs[jq]
                        re, im = re * c + im * sn, im * c - re * sn
                    ub_put((t * 4 + jq) * 8 + p, g, (re, im))

            lhs = jnp.concatenate([st_refs[slot][t * 2 + k, 0:256] for k in range(2)], axis=1)
            o = _dot(lhs.astype(bf16), fmat(0, t))
            for g in range(8):
                u = [(o[(g * 4 + q) * 8:(g * 4 + q + 1) * 8, :128],
                      o[(g * 4 + q) * 8:(g * 4 + q + 1) * 8, 128:]) for q in range(4)]
                if t == 0:
                    emit(4, g, [(im, jnp.zeros_like(im)) for (_, im) in u])
                    u = [(re, jnp.where(lane0, 0.0, im)) for (re, im) in u]
                emit(t, g, u)
        return item

    def p2_bfly(u, g, inverse):
        def item(y):
            if y is not None:
                ub_ref[168, pin_rows(0), :] = y
            x = [ub_get(u * 8 + p, g) for p in range(8)]
            x = _swap(_dft8(_swap(x))) if inverse else _dft8(x)
            for p in range(8):
                ub_put(u * 8 + p, g, x[p])
        return item

    def p2_fwd(u, jps):
        def item(y):
            t = u // 4
            jq = u % 4
            xs = [_dot(_tobf(ms_ref[jq + 4 * jp]), ub_ref[u * 8 + jp].astype(bf16)) for jp in jps]
            for jp, xx in zip(jps, xs):
                w = wp_ref[pl.ds(t * 2560 + jq + 4 * jp, 64, stride=40), :]
                wr = pltpu.bitcast(w & jnp.uint32(0xFFFF0000), f32)
                wi = pltpu.bitcast(w << 16, f32)
                for g in range(8):
                    xr, xi = xx[g * 16:g * 16 + 8], xx[g * 16 + 8:g * 16 + 16]
                    a, b = wr[g * 8:(g + 1) * 8], wi[g * 8:(g + 1) * 8]
                    ub_put(u * 8 + jp, g, (xr * a - xi * b, xr * b + xi * a))
        return item

    def p2_inv(u, jps):
        def item(y):
            jq = u % 4
            zs = [_dot(_tobf(ms_ref[32 + jq + 4 * jp]), ub_ref[u * 8 + jp].astype(bf16)) for jp in jps]
            for jp, zz in zip(jps, zs):
                ub_ref[u * 8 + jp] = zz
        return item

    def p3_pre(p, g, ts):
        def item(y):
            sa_ref[7, pin_rows(256), :] = y
            cs = twiddles(p)

            def fetch(t):
                a = []
                for jq in range(4):
                    re, im = ub_get((t * 4 + jq) * 8 + p, g)
                    if jq > 0:
                        c, sn = cs[jq]
                        re, im = re * c - im * sn, im * c + re * sn
                    a.append((re, im))
                return _swap(_dft4(_swap(a)))

            for t in ts:
                u = fetch(t)
                if t == 0:
                    ny = fetch(4)
                    u = [(u[q][0], jnp.where(lane0, ny[q][0], u[q][1])) for q in range(4)]
                for q in range(4):
                    for k in range(2):
                        sa_ref[t * 2 + k, q * 64 + g * 8:q * 64 + (g + 1) * 8] = u[q][k]
        return item

    def p3_mm(p, q):
        def item(y):
            g = []
            for t in range(4):
                lhs = jnp.concatenate([sa_ref[t * 2 + k, q * 64:(q + 1) * 64] for k in range(2)], axis=1)
                o = _dot(lhs.astype(bf16), fmat(1, t))
                g.append((o[:, :128], o[:, 128:]))
            yy = _r8_real_t(g)
            rows = pl.multiple_of(q * 512 + p * 64, 64)
            for a in range(8):
                bx_ref[pl.ds(rows, 64), a * 128:(a + 1) * 128] = yy[a].astype(bf16)
        return item

    def b_out(p):
        for q in range(4):
            rows = pl.multiple_of(q * 512 + p * 64, 64)
            pltpu.make_async_copy(bx_ref.at[pl.ds(rows, 64), :],
                                  out_hbm.at[pl.ds(rows, 64), pl.ds(DM, DM)], sem_out.at[1]).start()

    def step(pp, odd, mem, hooks):
        r0 = pl.multiple_of(pp * 64 + 32 * odd, SEG)
        xs = xo_ref[pl.ds(r0, SEG), :]
        x_lo = xs[0:8].astype(f32)
        hm = jnp.concatenate(
            [jnp.concatenate([x_lo, jnp.concatenate(mem, axis=1)], axis=0).astype(bf16), xs[16:32]], axis=0)
        fill = fillo_ref[:, 0:64] if odd else fille_ref[:, 0:48]
        nrow = 48 if odd else 32
        qkv, ps = {}, {}

        def do_qkv(g):
            for h in range(g * G, (g + 1) * G):
                for t in range(3):
                    y32 = _dot(hm, _tobf(w_refs[t * 2 + h // 16][h % 16, 0:512]))
                    y = y32.astype(bf16)
                    parts = [y]
                    if odd or t > 0:
                        parts.append(_tobf(qkvc_ref[pp, t * H + h]))
                    if t > 0:
                        if odd:
                            parts.append(_tobf(kve_ref[(t - 1) * H + h]))
                        else:
                            kve_ref[(t - 1) * H + h] = _tou(y[0:16])
                    qkv[(t, h)] = jnp.concatenate(parts, axis=0) if len(parts) > 1 else y
                for item in hooks.get(h, ()):
                    item(y32[0:8])

        def do_s(g):
            for h in range(g * G, (g + 1) * G):
                sc = jax.lax.dot_general(qkv[(0, h)], qkv[(1, h)], (((1,), (1,)), ((), ())),
                                         preferred_element_type=f32)
                sc = jnp.where(fill == 0.0, sc * scale, fill)
                e = jnp.exp(sc - jnp.max(sc, axis=1, keepdims=True))
                den = jnp.sum(e, axis=1, keepdims=True)
                r = pl.reciprocal(den, approx=True)
                r = r * (2.0 - den * r)
                ps[h] = (e * r).astype(bf16)

        def do_pv(g):
            for h in range(g * G, (g + 1) * G):
                oall_ref[h, 0:nrow // 2] = _tou(_dot(ps[h], qkv[(2, h)]).astype(bf16))

        def do_o(j, h0, h1):
            lhs = jnp.concatenate([_tobf(oall_ref[h, 0:nrow // 2]) for h in range(h0, h1)], axis=1)
            return _dot(lhs, _tobf(wo_ref[j, h0 * 64:h1 * 64, :]))

        for g in range(NG):
            do_qkv(g)
            if g >= 1:
                do_s(g - 1)
            if g >= 2:
                do_pv(g - 2)
        part = {}
        for j in range(8):
            part[j] = do_o(j, 0, OSPLIT)
            for k, item in enumerate(hooks.get(('o', j), ())):
                item(part[j][k * 16:k * 16 + 8])
            if j == 2:
                do_s(NG - 1)
                do_pv(NG - 2)
            if j == 5:
                do_pv(NG - 1)
        new_mem = []
        for j in range(8):
            cols = slice(j * 128, (j + 1) * 128)
            res = do_o(j, OSPLIT, H) + part[j]
            new_mem.append(res[8:16])
            if odd:
                xo_ref[pl.ds(r0, SEG), cols] = jnp.concatenate(
                    [res[0:8], res[40:48], res[16:32]], axis=0).astype(bf16)
                xo_ref[pl.ds(r0 - 24, 8), cols] = res[32:40].astype(bf16)
            else:
                xo_ref[pl.ds(r0, SEG), cols] = res.astype(bf16)
        for item in hooks.get(H, ()):
            item(None)
        return new_mem

    def a_out(pp):
        rows = pl.multiple_of(pp * 64, 64)
        pltpu.make_async_copy(xo_ref.at[pl.ds(rows, 64), :],
                              out_hbm.at[pl.ds(rows, 64), pl.ds(0, DM)], sem_out.at[0]).start()

    def l1(i, mem):
        he = {h: [p1_pre(2 * i + h // 16, h // 16, (h % 16) // 4, h % 4)] for h in range(32)}
        he[21].append(p1_mm(2 * i, 0, 0))
        he[25].append(p1_mm(2 * i, 0, 1))
        he[29].append(p1_mm(2 * i, 0, 2))
        he[H] = [p1_mm(2 * i, 0, 3)]
        ho = {1 + 4 * t: [p1_mm(2 * i + 1, 1, t)] for t in range(4)}
        mem = step(i, 0, mem, he)
        mem = step(i, 1, mem, ho)
        a_out(i)
        return mem

    def l2(i, mem):
        u = i - N_L1
        he = {13: [p2_fwd(u, range(0, 4))], 21: [p2_fwd(u, range(4, 8))], H: [p2_inv(u, range(0, 8))]}
        ho = {('o', j): [p2_bfly(u, j, True), p2_bfly(u + 1, j, False)] for j in range(8)}
        mem = step(i, 0, mem, he)
        mem = step(i, 1, mem, ho)
        a_out(i)
        return mem

    def l3(i, mem):
        p = i - N_L1 - N_L2
        he = {h: [p3_pre(p, h // 2, (0, 1) if h % 2 == 0 else (2, 3))] for h in range(16)}
        he[21] = [p3_mm(p, 0)]
        he[29] = [p3_mm(p, 1)]
        he[H] = [p3_mm(p, 2)]
        ho = {5: [p3_mm(p, 3)], 12: [lambda y: b_out(p)]}
        mem = step(i, 0, mem, he)
        mem = step(i, 1, mem, ho)
        a_out(i)
        return mem

    m0 = mem_ref[...].astype(f32)
    mem = [m0[:, j * 128:(j + 1) * 128] for j in range(8)]
    mem = jax.lax.fori_loop(0, N_L1, l1, mem)
    cp_ms.wait()
    for g in range(8):
        p2_bfly(0, g, False)(None)
    mem = jax.lax.fori_loop(N_L1, N_L1 + N_L2, l2, mem)
    mem = jax.lax.fori_loop(N_L1 + N_L2, NSEG // 2, l3, mem)

    pltpu.make_async_copy(xo_ref, out_hbm.at[:, pl.ds(0, DM)], sem_out.at[0]).wait()
    pltpu.make_async_copy(bx_ref, out_hbm.at[:, pl.ds(DM, DM)], sem_out.at[1]).wait()


@jax.jit
def _run(x, mem0, wq, wk, wv, wo, bx, w_r, w_i):
    fd, ms = _tables()
    hbm = pl.BlockSpec(memory_space=pl.ANY)
    out = pl.pallas_call(
        _kernel,
        out_shape=jax.ShapeDtypeStruct((S, 2 * DM), bf16),
        in_specs=[hbm] * 12,
        out_specs=hbm,
        scratch_shapes=[
            pltpu.VMEM((S, DM), bf16),
            pltpu.VMEM((MEM, DM), bf16),
            pltpu.VMEM((8, NSEG, 8, 128), bf16),
            pltpu.VMEM((4, DM, 16, DH), bf16),
        ] + [pltpu.VMEM((16, DM // 2 + 8, DH), u32)] * 6 + [
            pltpu.VMEM((H * DH, DM), bf16),
            pltpu.VMEM((8, H * DH // 2 + 8, 128), u32),
            pltpu.VMEM((8, 256, 128), u32),
            pltpu.VMEM((NSEG // 2, 3 * H, 8, 128), u32),
            pltpu.VMEM((2 * H, 8, 128), u32),
            pltpu.VMEM((H, 24, DH), u32),
            pltpu.VMEM((32, 128), f32),
            pltpu.VMEM((48, 128), f32),
            pltpu.VMEM((S, DM), bf16),
            pltpu.VMEM((16, DM // 2 + 1, 256), bf16),
            pltpu.VMEM((12808, 128), u32),
            pltpu.VMEM((169, 128, 128), f32),
            pltpu.VMEM((8, 264, 128), f32),
            pltpu.VMEM((8, 264, 128), f32),
            pltpu.VMEM((16, 128, 128), u32),
            pltpu.VMEM((64, 64, 128), u32),
            pltpu.SMEM((64,), f32),
            pltpu.SMEM((1,), jnp.int32),
            pltpu.SemaphoreType.DMA((64,)),
            pltpu.SemaphoreType.DMA((2,)),
        ],
        compiler_params=pltpu.CompilerParams(vmem_limit_bytes=120 * 1024 * 1024,
                                             disable_semaphore_checks=True),
    )(x.reshape(S, DM), x.reshape(NSEG, SEG, DM), mem0.reshape(MEM, DM), wq, wk, wv,
      wo.reshape(H * DH, DM), bx.reshape(S, DM), w_r.T, w_i.T, jnp.asarray(fd), jnp.asarray(ms))
    return out.reshape(1, S, 2 * DM)


def pallas_concat_heads__memory_aug_recurrent_mem_tr__spectral_gfnet__prompt_kernel(
    A_x: jax.Array,
    A_mem0: jax.Array,
    A_Wq: jax.Array,
    A_Wk: jax.Array,
    A_Wv: jax.Array,
    A_Wo: jax.Array,
    A_seg_len,
    B_x: jax.Array,
    B_w_r: jax.Array,
    B_w_i: jax.Array,
):
    if isinstance(A_seg_len, int):
        assert A_seg_len == SEG
    assert A_x.shape == (1, S, DM) and A_mem0.shape == (1, MEM, DM) and A_Wq.shape == (DM, H, DH)
    assert B_x.shape == (1, S, DM) and B_w_r.shape == (S, DM // 2 + 1)
    return _run(A_x, A_mem0, A_Wq, A_Wk, A_Wv, A_Wo, B_x, B_w_r, B_w_i)
```

```python
import math

import numpy as np
import jax
import jax.numpy as jnp
import jax.experimental.pallas as pl
import jax.experimental.pallas.tpu as pltpu

bf16 = jnp.bfloat16
f32 = jnp.float32
u32 = jnp.uint32

S, DM = 2048, 1024
H, DH = 32, 128
MEM, SEG = 8, 32
NSEG = S // SEG
SQH = math.sqrt(0.5)

_PAIRS = ((0, 4), (1, 7), (2, 6), (3, 5))
_FIRST = np.array([[1, 1, 0, 0], [1, 0, 1, 0], [0, 1, 1, 0], [0, 1, 0, 1]], bool)


def _pack_rows(a):
    u = np.ascontiguousarray(a, dtype=np.float32).view(np.uint32).astype(np.uint64)
    b = ((u + 0x7FFF + ((u >> 16) & 1)) >> 16).astype(np.uint32)
    return (b[..., 0::2, :] | (b[..., 1::2, :] << 16)).astype(np.uint32)


def _tables():
    k2 = np.zeros((4, 128), np.int64)
    for t in range(4):
        odd = t % 2
        for lam in range(128):
            k = 2 * lam + odd
            if k % 8 not in _PAIRS[t]:
                k = 2 * (128 + 8 * (lam // 8) + (lam % 8 - 1 - odd) % 8) + odd
            assert k % 8 in _PAIRS[t]
            k2[t, lam] = k
    b = np.arange(128)[:, None]
    F = np.zeros((12, 128, 128))
    G = np.zeros((12, 128, 128))
    for t in range(4):
        th = 2 * np.pi * ((b * k2[t][None, :]) % DM) / DM
        C, Sn = np.cos(th), np.sin(th)
        first = ((k2[t] % 8) == _PAIRS[t][0])[None, :]
        assert np.array_equal(first[0], _FIRST[t][np.arange(128) % 4])
        if t == 0:
            im = -Sn
            im[:, 0] = (-1.0) ** np.arange(128)
            F[0:3] = im, np.where(first, im, C), np.where(first, C, im)
            G[0:3] = im, np.where(first, C, -im), np.where(first, -im, C)
            G[0:3, :, 0] *= 0.5
        else:
            Sg = np.where(first, Sn, -Sn)
            F[3 * t:3 * t + 3] = C, -(C + Sg), C - Sg
            G[3 * t:3 * t + 3] = F[3 * t:3 * t + 3]
    Finv = np.transpose(G, (0, 2, 1)) * (2.0 / DM)
    fd = _pack_rows(np.concatenate([F, Finv]))
    M = np.zeros((32, 128, 128))
    r = np.arange(64)[None, :]
    l = np.arange(64)[:, None]
    for j in range(32):
        th = 2 * np.pi * ((r * (j + 32 * l)) % S) / S
        C, Sn = np.cos(th), np.sin(th)
        M[j, :64, :64] = C
        M[j, :64, 64:] = Sn
        M[j, 64:, :64] = -Sn
        M[j, 64:, 64:] = C
    perm = np.arange(128).reshape(2, 8, 8).transpose(1, 0, 2).reshape(128)
    M = M[:, perm][:, :, perm]
    Minv = np.transpose(M, (0, 2, 1)) / S
    ms = _pack_rows(np.concatenate([M, Minv]))
    return fd, ms


def _tobf(w):
    return pltpu.bitcast(w, bf16)


def _tou(w):
    return pltpu.bitcast(w, u32)


def _dot(a, b):
    return jnp.dot(a, b, preferred_element_type=f32)


def _r8_real(x):
    t0, t1 = x[0] + x[4], x[0] - x[4]
    t2, t3 = x[2] + x[6], x[2] - x[6]
    t4, t5 = x[1] + x[5], x[1] - x[5]
    t6, t7 = x[3] + x[7], x[3] - x[7]
    e0, e1 = t0 + t2, t0 - t2
    o0, o1 = t4 + t6, t4 - t6
    u, v = SQH * (t5 - t7), SQH * (t5 + t7)
    return [(e0 + o0, e0 - o0), (t1 + u, v + t3), (e1, o1), (t1 - u, v - t3)]


def _r8_real_t(g):
    (z0, z4), (a1, b1), (e1, o1), (a3, b3) = g
    e0, o0 = z0 + z4, z0 - z4
    t1, u = a1 + a3, a1 - a3
    v, t3 = b1 + b3, b1 - b3
    t5, t7 = SQH * (v + u), SQH * (v - u)
    t0, t2 = e0 + e1, e0 - e1
    t4, t6 = o0 + o1, o0 - o1
    return [t0 + t1, t4 + t5, t2 + t3, t6 + t7, t0 - t1, t4 - t5, t2 - t3, t6 - t7]


def _dft4(u):
    (r0, i0), (r1, i1), (r2, i2), (r3, i3) = u
    sr, si, dr, di = r0 + r2, i0 + i2, r0 - r2, i0 - i2
    tr, ti, er, ei = r1 + r3, i1 + i3, r1 - r3, i1 - i3
    return [(sr + tr, si + ti), (dr + ei, di - er), (sr - tr, si - ti), (dr - ei, di + er)]


def _dft8(x):
    a = [(x[p][0] + x[p + 4][0], x[p][1] + x[p + 4][1]) for p in range(4)]
    d = [(x[p][0] - x[p + 4][0], x[p][1] - x[p + 4][1]) for p in range(4)]
    ev = _dft4(a)
    (r0, i0), (r1, i1), (r2, i2), (r3, i3) = d
    b1r, b1i = SQH * (r1 + i1), SQH * (i1 - r1)
    b3r, n3i = SQH * (i3 - r3), SQH * (r3 + i3)
    sr, si, dr, di = r0 + i2, i0 - r2, r0 - i2, i0 + r2
    tr, ti, er, ei = b1r + b3r, b1i - n3i, b1r - b3r, b1i + n3i
    od = [(sr + tr, si + ti), (dr + ei, di - er), (sr - tr, si - ti), (dr - ei, di + er)]
    return [ev[0], od[0], ev[1], od[1], ev[2], od[2], ev[3], od[3]]


def _swap(x):
    return [(b, a) for (a, b) in x]


G = 4
NG = H // G
OSPLIT = 24
NEG = -1e9
N_L1, N_L2, N_L3 = 4, 20, 8


def _kernel(x_hbm, x3_hbm, mem_hbm, wq_hbm, wk_hbm, wv_hbm, wo_hbm, bx_hbm, wr_hbm, wi_hbm,
            fd_hbm, ms_hbm, out_hbm,
            xo_ref, mem_ref, xcraw_ref, raw_ref, w0_ref, w1_ref, w2_ref, w3_ref, w4_ref, w5_ref,
            woraw_ref, wo_ref, xc_ref, qkvc_ref, kve_ref,
            oall_ref, fille_ref, fillo_ref, bx_ref, wt_ref, wp_ref, ub_ref, sa_ref, sb_ref, fd_ref, ms_ref,
            tw_ref, zero_ref, sem_in, sem_out):
    scale = DH ** -0.5
    w_hbm = (wq_hbm, wk_hbm, wv_hbm)
    w_refs = (w0_ref, w1_ref, w2_ref, w3_ref, w4_ref, w5_ref)

    def raw_copy(c, i=0, nd=DM):
        rows = pl.ds(pl.multiple_of(i * nd, nd), nd)
        return pltpu.make_async_copy(
            w_hbm[c // 2].at[rows, pl.ds((c % 2) * 16, 16), :],
            raw_ref.at[c % 4, rows], sem_in.at[8 + min(c, 3) * 8 + max(c - 3, 0) * 2 + i])

    def xc_copy(k):
        return pltpu.make_async_copy(
            x3_hbm.at[:, pl.ds(8, 8), pl.ds(pl.multiple_of(k * 128, 128), 128)], xcraw_ref.at[k], sem_in.at[40 + k])

    cp_x = pltpu.make_async_copy(x_hbm, xo_ref, sem_in.at[0])
    cp_mem = pltpu.make_async_copy(mem_hbm, mem_ref, sem_in.at[1])
    cp_wo = pltpu.make_async_copy(wo_hbm, woraw_ref, sem_in.at[2])
    cp_bx = pltpu.make_async_copy(bx_hbm, bx_ref, sem_in.at[3])
    cp_fd = pltpu.make_async_copy(fd_hbm, fd_ref, sem_in.at[4])
    cp_ms = pltpu.make_async_copy(ms_hbm, ms_ref, sem_in.at[5])
    cp_wt = [pltpu.make_async_copy(src.at[:, pl.ds(lg * 256, 256)], wt_ref.at[a * 8 + lg], sem_in.at[48 + a * 8 + lg])
             for a, src in enumerate((wr_hbm, wi_hbm)) for lg in range(8)]

    for i in range(8):
        xc_copy(i).start()
        raw_copy(0, i, 128).start()
        raw_copy(1, i, 128).start()
    for i in range(4):
        raw_copy(2, i, 256).start()
    for i in range(2):
        raw_copy(3, i, 512).start()

    zero_ref[0] = 0

    def pin_rows(r):
        return pl.ds(pl.multiple_of(r + zero_ref[0] * 32, 8), 8)

    for p in range(8):
        for jq in range(4):
            tw_ref[(p * 4 + jq) * 2] = jnp.float32(math.cos(2 * math.pi * p * jq / 32))
            tw_ref[(p * 4 + jq) * 2 + 1] = jnp.float32(math.sin(2 * math.pi * p * jq / 32))

    qi = jax.lax.broadcasted_iota(jnp.int32, (48, 128), 0)
    ki = jax.lax.broadcasted_iota(jnp.int32, (48, 128), 1)

    def between(v, lo, hi):
        return (v >= lo) & (v < hi)

    def table(keep, other):
        return jnp.where(other, -jnp.inf, jnp.where(keep, 0.0, NEG)).astype(f32)

    keep = between(qi, 8, 16) | between(ki, 8, 16) | (qi >= jnp.where(ki < 32, ki, ki - 24))
    fille_ref[...] = table(keep, ki >= 40)[:32]
    q_even = between(qi, 32, 40)
    k_even = between(ki, 32, 40) | (ki >= 48)
    qpos = jnp.where(qi < 32, qi, jnp.where(qi < 40, qi - 24, qi - 32))
    kpos = jnp.where(ki < 32, ki, jnp.where(ki < 40, ki - 24, jnp.where(ki < 48, ki - 32, ki - 48)))
    keep = between(qi, 8, 16) | between(ki, 8, 16) | (ki >= 56) | (qpos >= kpos)
    fillo_ref[...] = table(keep, (q_even != k_even) | (ki >= 64))

    def relayout16(c, d0):
        slot = c % 4
        w0 = pl.multiple_of(d0 // 2, 8)
        los, his = [], []
        for dd in range(8):
            a = _tou(raw_ref[slot, d0 + 2 * dd])
            b = _tou(raw_ref[slot, d0 + 2 * dd + 1])
            los.append((a & jnp.uint32(0xFFFF)) | (b << 16))
            his.append((a >> 16) | (b & jnp.uint32(0xFFFF0000)))
        lo = jnp.swapaxes(jnp.stack(los), 0, 1)
        hi = jnp.swapaxes(jnp.stack(his), 0, 1)
        for j in range(8):
            w_refs[c][2 * j, pl.ds(w0, 8), :] = lo[j]
            w_refs[c][2 * j + 1, pl.ds(w0, 8), :] = hi[j]

    def repack_wo64(r_start):
        r0 = pl.multiple_of(r_start, 64)
        w0 = pl.multiple_of(r_start // 2, 32)
        v = woraw_ref[pl.ds(r0, 64), :]
        for j in range(8):
            wo_ref[j, pl.ds(w0, 32), :] = _tou(v[:, j * 128:(j + 1) * 128])

    sub4 = jax.lax.broadcasted_iota(jnp.int32, (128, 128), 0) % 4

    def wp_store(t, kb, tile):
        v = tile.T
        for g in range(4):
            r0 = pl.multiple_of(t * 2560 + kb * 160 + g * 40, 8)
            wp_ref[pl.ds(r0, 32), :] = v[g * 32:(g + 1) * 32]

    def b_prep(lg, hb, par):
        cols = slice(hb * 128, (hb + 1) * 128)
        a = _tou(wt_ref[lg, 0:512, cols])
        b = _tou(wt_ref[8 + lg, 0:512, cols])
        if par == 0:
            w = (a << 16) | (b & jnp.uint32(0xFFFF))
            m = (sub4 == 0) | (sub4 == 2)
        else:
            w = (a & jnp.uint32(0xFFFF0000)) | (b >> 16)
            m = (sub4 == 0) | (sub4 == 3)
        top = w[:128]
        bot = pltpu.roll(w[128:].reshape(16, 8, 128), 1 + par, 1).reshape(128, 128)
        wp_store(par, lg * 2 + hb, jnp.where(m, top, bot))
        wp_store(par + 2, lg * 2 + hb, jnp.where(m, bot, top))
        if par == 0:
            na = jnp.broadcast_to(wt_ref[lg, 512:513, cols].astype(f32), (128, 128))
            nb = jnp.broadcast_to(wt_ref[8 + lg, 512:513, cols].astype(f32), (128, 128))
            wp_store(4, lg * 2 + hb, pltpu.bitcast(na, u32) | (pltpu.bitcast(nb, u32) >> 16))

    def gather_c(k):
        xc_ref[k] = _tou(xcraw_ref[k].astype(f32).reshape(512, 128).astype(bf16))

    def store_qkvc(n, y):
        for pp in range(NSEG // 2):
            qkvc_ref[pp, n] = y[pp * 8:(pp + 1) * 8]

    def q_unit(i, groups, first, last, fillers):
        xk = _tobf(xc_ref[i])
        w0 = pl.multiple_of(i * 64, 64)
        for g in groups:
            rhs = jnp.concatenate(
                [_tobf(w_refs[h // 16][h % 16, pl.ds(w0, 64), :]) for h in range(4 * g, 4 * g + 4)], axis=1)
            y = _dot(xk, rhs)
            for h in range(4 * g, 4 * g + 4):
                yh = y[:, (h % 4) * 128:(h % 4 + 1) * 128]
                if not first:
                    yh = yh + ub_ref[h * 4:(h + 1) * 4].reshape(512, 128)
                if last:
                    store_qkvc(h, _tou(yh.astype(bf16)))
                else:
                    ub_ref[h * 4:(h + 1) * 4] = yh.reshape(4, 128, 128)
            mine = fillers.get(g, [])
            for fi, item in enumerate(mine):
                r = (fi * 512 // len(mine)) // 8 * 8
                item(pltpu.bitcast(y[r:r + 8, 0:128], u32))

    def rl_item(c, d0):
        def item(pin):
            w_refs[c][15, pin_rows(512), :] = pin
            relayout16(c, d0)
        return item

    def spread(fillers, items, groups):
        for k, item in enumerate(items):
            fillers.setdefault(groups[k * len(groups) // len(items)], []).append(item)
        return fillers

    def half_items(f, c, i, groups):
        return spread(f, [rl_item(c, i * 128 + blk * 16) for blk in range(8)], groups)

    def piece_items(i):
        f = half_items(half_items({}, 1, i, (0, 1, 2)), 0, i + 1, (4, 5, 6))
        return spread(f, [lambda pin: gather_c(i + 1)], (6,))

    def chunk2_items(f, i, groups):
        return spread(f, [rl_item(2, i * 256 + blk * 16) for blk in range(16)], groups)

    def wait_piece(i):
        raw_copy(1, i, 128).wait()
        xc_copy(i + 1).wait()
        raw_copy(0, i + 1, 128).wait()

    xc_copy(0).wait()
    gather_c(0)
    raw_copy(0, 0, 128).wait()
    for blk in range(8):
        relayout16(0, blk * 16)
    q_unit(0, range(0, 2), True, False, {})
    raw_copy(1, 0, 128).wait()
    q_unit(0, range(2, 4), True, False, half_items({}, 1, 0, (2, 2, 3)))
    xc_copy(1).wait()
    raw_copy(0, 1, 128).wait()
    q_unit(0, range(4, 8), True, False,
           spread(half_items({}, 0, 1, (4, 5, 6)), [lambda pin: gather_c(1)], (6,)))

    def q_c(i, carry):
        wait_piece(i)
        q_unit(i, range(8), False, False, piece_items(i))
        return carry
    jax.lax.fori_loop(1, 5, q_c, 0)

    wait_piece(5)
    raw_copy(2, 0, 256).wait()
    raw_copy(2, 1, 256).wait()
    q_unit(5, range(8), False, False,
           chunk2_items(chunk2_items(piece_items(5), 0, (0, 1, 2, 3, 3)), 1, (3, 4, 5, 6, 7)))
    wait_piece(6)
    raw_copy(1, 7, 128).wait()
    raw_copy(2, 2, 256).wait()
    raw_copy(2, 3, 256).wait()
    q_unit(6, range(8), False, False, chunk2_items(piece_items(6), 2, (0, 1, 2, 3, 3, 4, 5, 7)))
    raw_copy(4).start()
    q_unit(7, range(8), False, True, chunk2_items(half_items({}, 1, 7, (0, 1, 2)), 3, (3, 4, 5, 6)))
    raw_copy(5).start()
    for cp in cp_wt:
        cp.start()
    cp_wo.start()
    cp_x.start()
    cp_mem.start()
    cp_bx.start()
    cp_fd.start()
    cp_ms.start()

    def bulk_iter(c, i, n_rl, rl_start):
        xc = jnp.concatenate([_tobf(xc_ref[k]) for k in range(8)], axis=1)
        for t in range(8):
            n = i * 8 + t
            y = _tou(_dot(xc, _tobf(w_refs[c][n, 0:512])).astype(bf16))
            store_qkvc(c * 16 + n, y)
            for blk in range(n_rl):
                pin = y[blk * (256 // n_rl):blk * (256 // n_rl) + 8]
                if c + 1 < 6:
                    w_refs[c + 1][15, pin_rows(512), :] = pin
                    relayout16(c + 1, rl_start + (t * n_rl + blk) * 16)
                else:
                    wo_ref[7, pin_rows(2048), :] = pin
                    repack_wo64(rl_start + (t * n_rl + blk) * 64)
            if c >= 4:
                wp_ref[pin_rows(12800), :] = y[32:40]
                b_prep((c - 4) * 4 + i * 2 + t // 4, (t // 2) % 2, t % 2)

    for c in range(2, 6):
        if c == 4:
            for cp in cp_wt:
                cp.wait()
        if c == 5:
            cp_wo.wait()
        elif c > 2:
            raw_copy(c + 1).wait()

        def bulk(i, carry, c=c):
            if c == 2:
                raw_copy(3, i, 512).wait()
            bulk_iter(c, i, 4, i * (512 if c + 1 < 6 else 2048))
            return carry
        jax.lax.fori_loop(0, 2, bulk, 0)

    cp_x.wait()
    cp_mem.wait()
    cp_bx.wait()
    cp_fd.wait()

    lane0 = jax.lax.broadcasted_iota(jnp.int32, (8, 128), 1) == 0

    def ub_get(n, g):
        return ub_ref[n, g * 16:g * 16 + 8], ub_ref[n, g * 16 + 8:g * 16 + 16]

    def ub_put(n, g, v):
        ub_ref[n, g * 16:g * 16 + 8] = v[0]
        ub_ref[n, g * 16 + 8:g * 16 + 16] = v[1]

    lane4 = jax.lax.broadcasted_iota(jnp.int32, (8, 128), 1) % 4

    def first_lanes(t):
        la, lb = [k for k in range(4) if _FIRST[t][k]]
        return (lane4 == la) | (lane4 == lb)

    def stage(st_ref, t, rows, vals):
        for k in range(3):
            st_ref[3 * t + k, rows] = vals[k]

    def d_products(st_ref, d, t, rows):
        return [_dot(st_ref[3 * t + k, rows].astype(bf16), _tobf(fd_ref[d * 12 + 3 * t + k])) for k in range(3)]

    def twiddles(p):
        return [(tw_ref[(p * 4 + jq) * 2], tw_ref[(p * 4 + jq) * 2 + 1]) for jq in range(4)]

    st_refs = (sa_ref, sb_ref)

    def p1_pre(p, slot, rs, q):
        def item(y):
            st_refs[slot][7, pin_rows(256), :] = y
            rows = pl.multiple_of(q * 512 + p * 64 + rs * 16, 16)
            xq = bx_ref[pl.ds(rows, 16), :].astype(f32)
            zz = _r8_real([xq[:, a * 128:(a + 1) * 128] for a in range(8)])
            for t in range(4):
                for e in range(2):
                    r = ((rs * 2 + e) * 4 + q) * 8
                    a, b = zz[t][0][e * 8:(e + 1) * 8], zz[t][1][e * 8:(e + 1) * 8]
                    stage(st_refs[slot], t, slice(r, r + 8), (a + b, b, a))
        return item

    def p1_mm(p, slot, t):
        def item(y):
            cs = twiddles(p)

            def emit(t, g, u):
                a = _dft4(u)
                for jq in range(4):
                    re, im = a[jq]
                    if jq > 0:
                        c, sn = cs[jq]
                        re, im = re * c + im * sn, im * c - re * sn
                    ub_put((t * 4 + jq) * 8 + p, g, (re, im))

            first = first_lanes(t)
            for m in range(4):
                ks = d_products(st_refs[slot], 0, t, slice(m * 64, (m + 1) * 64))
                for e in range(2):
                    u = []
                    for q in range(4):
                        r = (e * 4 + q) * 8
                        k1, k2, k3 = [k[r:r + 8] for k in ks]
                        if t == 0:
                            u.append((jnp.where(first, k3, k2), k1 - jnp.where(first, k2, k3)))
                        else:
                            u.append((k2 + k1, (k3 - k1) * jnp.where(first, 1.0, -1.0)))
                    if t == 0:
                        emit(4, m * 2 + e, [(im, jnp.zeros_like(im)) for (_, im) in u])
                        u = [(re, jnp.where(lane0, 0.0, im)) for (re, im) in u]
                    emit(t, m * 2 + e, u)
        return item

    def p2_bfly(u, g, inverse):
        def item(y):
            if y is not None:
                ub_ref[168, pin_rows(0), :] = y
            x = [ub_get(u * 8 + p, g) for p in range(8)]
            x = _swap(_dft8(_swap(x))) if inverse else _dft8(x)
            for p in range(8):
                ub_put(u * 8 + p, g, x[p])
        return item

    def p2_fwd(u, jps):
        def item(y):
            t = u // 4
            jq = u % 4
            xs = [_dot(_tobf(ms_ref[jq + 4 * jp]), ub_ref[u * 8 + jp].astype(bf16)) for jp in jps]
            for jp, xx in zip(jps, xs):
                w = wp_ref[pl.ds(t * 2560 + jq + 4 * jp, 64, stride=40), :]
                wr = pltpu.bitcast(w & jnp.uint32(0xFFFF0000), f32)
                wi = pltpu.bitcast(w << 16, f32)
                for g in range(8):
                    xr, xi = xx[g * 16:g * 16 + 8], xx[g * 16 + 8:g * 16 + 16]
                    a, b = wr[g * 8:(g + 1) * 8], wi[g * 8:(g + 1) * 8]
                    ub_put(u * 8 + jp, g, (xr * a - xi * b, xr * b + xi * a))
        return item

    def p2_inv(u, jps):
        def item(y):
            jq = u % 4
            zs = [_dot(_tobf(ms_ref[32 + jq + 4 * jp]), ub_ref[u * 8 + jp].astype(bf16)) for jp in jps]
            for jp, zz in zip(jps, zs):
                ub_ref[u * 8 + jp] = zz
        return item

    def p3_pre(p, g, ts):
        def item(y):
            sa_ref[7, pin_rows(256), :] = y
            cs = twiddles(p)

            def fetch(t):
                a = []
                for jq in range(4):
                    re, im = ub_get((t * 4 + jq) * 8 + p, g)
                    if jq > 0:
                        c, sn = cs[jq]
                        re, im = re * c - im * sn, im * c + re * sn
                    a.append((re, im))
                return _swap(_dft4(_swap(a)))

            for t in ts:
                u = fetch(t)
                if t == 0:
                    ny = fetch(4)
                    u = [(u[q][0], jnp.where(lane0, ny[q][0], u[q][1])) for q in range(4)]
                first = first_lanes(t)
                for q in range(4):
                    re, im = u[q]
                    if t == 0:
                        vals = (im, jnp.where(first, re, im), jnp.where(first, im, re))
                    else:
                        im = im * jnp.where(first, 1.0, -1.0)
                        vals = (re + im, im, re)
                    stage(sa_ref, t, slice(q * 64 + g * 8, q * 64 + (g + 1) * 8), vals)
        return item

    def p3_mm(p, q):
        def item(y):
            g = []
            for t in range(4):
                k1, k2, k3 = d_products(sa_ref, 1, t, slice(q * 64, (q + 1) * 64))
                g.append((k2 + k1, k3 + k1 if t == 0 else k3 - k1))
            yy = _r8_real_t(g)
            rows = pl.multiple_of(q * 512 + p * 64, 64)
            for a in range(8):
                bx_ref[pl.ds(rows, 64), a * 128:(a + 1) * 128] = yy[a].astype(bf16)
        return item

    def b_out(p):
        for q in range(4):
            rows = pl.multiple_of(q * 512 + p * 64, 64)
            pltpu.make_async_copy(bx_ref.at[pl.ds(rows, 64), :],
                                  out_hbm.at[pl.ds(rows, 64), pl.ds(DM, DM)], sem_out.at[1]).start()

    def step(pp, odd, mem, hooks):
        r0 = pl.multiple_of(pp * 64 + 32 * odd, SEG)
        xs = xo_ref[pl.ds(r0, SEG), :]
        x_lo = xs[0:8].astype(f32)
        hm = jnp.concatenate(
            [jnp.concatenate([x_lo, jnp.concatenate(mem, axis=1)], axis=0).astype(bf16), xs[16:32]], axis=0)
        fill = fillo_ref[:, 0:64] if odd else fille_ref[:, 0:48]
        nrow = 48 if odd else 32
        qkv, ps = {}, {}

        def do_qkv(g):
            for h in range(g * G, (g + 1) * G):
                for t in range(3):
                    y32 = _dot(hm, _tobf(w_refs[t * 2 + h // 16][h % 16, 0:512]))
                    y = y32.astype(bf16)
                    parts = [y]
                    if odd or t > 0:
                        parts.append(_tobf(qkvc_ref[pp, t * H + h]))
                    if t > 0:
                        if odd:
                            parts.append(_tobf(kve_ref[(t - 1) * H + h]))
                        else:
                            kve_ref[(t - 1) * H + h] = _tou(y[0:16])
                    qkv[(t, h)] = jnp.concatenate(parts, axis=0) if len(parts) > 1 else y
                for item in hooks.get(h, ()):
                    item(y32[0:8])

        def do_s(g):
            for h in range(g * G, (g + 1) * G):
                sc = jax.lax.dot_general(qkv[(0, h)], qkv[(1, h)], (((1,), (1,)), ((), ())),
                                         preferred_element_type=f32)
                sc = jnp.where(fill == 0.0, sc * scale, fill)
                e = jnp.exp(sc - jnp.max(sc, axis=1, keepdims=True))
                den = jnp.sum(e, axis=1, keepdims=True)
                r = pl.reciprocal(den, approx=True)
                r = r * (2.0 - den * r)
                ps[h] = (e * r).astype(bf16)

        def do_pv(g):
            for h in range(g * G, (g + 1) * G):
                oall_ref[h, 0:nrow // 2] = _tou(_dot(ps[h], qkv[(2, h)]).astype(bf16))

        def do_o(j, h0, h1):
            lhs = jnp.concatenate([_tobf(oall_ref[h, 0:nrow // 2]) for h in range(h0, h1)], axis=1)
            return _dot(lhs, _tobf(wo_ref[j, h0 * 64:h1 * 64, :]))

        for g in range(NG):
            do_qkv(g)
            if g >= 1:
                do_s(g - 1)
            if g >= 2:
                do_pv(g - 2)
        part = {}
        for j in range(8):
            part[j] = do_o(j, 0, OSPLIT)
            for k, item in enumerate(hooks.get(('o', j), ())):
                item(part[j][k * 16:k * 16 + 8])
            if j == 2:
                do_s(NG - 1)
                do_pv(NG - 2)
            if j == 5:
                do_pv(NG - 1)
        new_mem = []
        for j in range(8):
            cols = slice(j * 128, (j + 1) * 128)
            res = do_o(j, OSPLIT, H) + part[j]
            new_mem.append(res[8:16])
            if odd:
                xo_ref[pl.ds(r0, SEG), cols] = jnp.concatenate(
                    [res[0:8], res[40:48], res[16:32]], axis=0).astype(bf16)
                xo_ref[pl.ds(r0 - 24, 8), cols] = res[32:40].astype(bf16)
            else:
                xo_ref[pl.ds(r0, SEG), cols] = res.astype(bf16)
        for item in hooks.get(H, ()):
            item(None)
        return new_mem

    def a_out(pp):
        rows = pl.multiple_of(pp * 64, 64)
        pltpu.make_async_copy(xo_ref.at[pl.ds(rows, 64), :],
                              out_hbm.at[pl.ds(rows, 64), pl.ds(0, DM)], sem_out.at[0]).start()

    def l1(i, mem):
        he = {h: [p1_pre(2 * i + h // 16, h // 16, (h % 16) // 4, h % 4)] for h in range(32)}
        he[21].append(p1_mm(2 * i, 0, 0))
        he[25].append(p1_mm(2 * i, 0, 1))
        he[29].append(p1_mm(2 * i, 0, 2))
        he[H] = [p1_mm(2 * i, 0, 3)]
        ho = {1 + 4 * t: [p1_mm(2 * i + 1, 1, t)] for t in range(4)}
        mem = step(i, 0, mem, he)
        mem = step(i, 1, mem, ho)
        a_out(i)
        return mem

    def l2(i, mem):
        u = i - N_L1
        he = {13: [p2_fwd(u, range(0, 4))], 21: [p2_fwd(u, range(4, 8))], H: [p2_inv(u, range(0, 8))]}
        ho = {('o', j): [p2_bfly(u, j, True), p2_bfly(u + 1, j, False)] for j in range(8)}
        mem = step(i, 0, mem, he)
        mem = step(i, 1, mem, ho)
        a_out(i)
        return mem

    def l3(i, mem):
        p = i - N_L1 - N_L2
        he = {h: [p3_pre(p, h // 2, (0, 1) if h % 2 == 0 else (2, 3))] for h in range(16)}
        he[21] = [p3_mm(p, 0)]
        he[29] = [p3_mm(p, 1)]
        he[H] = [p3_mm(p, 2)]
        ho = {5: [p3_mm(p, 3)], 12: [lambda y: b_out(p)]}
        mem = step(i, 0, mem, he)
        mem = step(i, 1, mem, ho)
        a_out(i)
        return mem

    m0 = mem_ref[...].astype(f32)
    mem = [m0[:, j * 128:(j + 1) * 128] for j in range(8)]
    mem = jax.lax.fori_loop(0, N_L1, l1, mem)
    cp_ms.wait()
    for g in range(8):
        p2_bfly(0, g, False)(None)
    mem = jax.lax.fori_loop(N_L1, N_L1 + N_L2, l2, mem)
    mem = jax.lax.fori_loop(N_L1 + N_L2, NSEG // 2, l3, mem)

    pltpu.make_async_copy(xo_ref, out_hbm.at[:, pl.ds(0, DM)], sem_out.at[0]).wait()
    pltpu.make_async_copy(bx_ref, out_hbm.at[:, pl.ds(DM, DM)], sem_out.at[1]).wait()


@jax.jit
def _run(x, mem0, wq, wk, wv, wo, bx, w_r, w_i):
    fd, ms = _tables()
    hbm = pl.BlockSpec(memory_space=pl.ANY)
    out = pl.pallas_call(
        _kernel,
        out_shape=jax.ShapeDtypeStruct((S, 2 * DM), bf16),
        in_specs=[hbm] * 12,
        out_specs=hbm,
        scratch_shapes=[
            pltpu.VMEM((S, DM), bf16),
            pltpu.VMEM((MEM, DM), bf16),
            pltpu.VMEM((8, NSEG, 8, 128), bf16),
            pltpu.VMEM((4, DM, 16, DH), bf16),
        ] + [pltpu.VMEM((16, DM // 2 + 8, DH), u32)] * 6 + [
            pltpu.VMEM((H * DH, DM), bf16),
            pltpu.VMEM((8, H * DH // 2 + 8, 128), u32),
            pltpu.VMEM((8, 256, 128), u32),
            pltpu.VMEM((NSEG // 2, 3 * H, 8, 128), u32),
            pltpu.VMEM((2 * H, 8, 128), u32),
            pltpu.VMEM((H, 24, DH), u32),
            pltpu.VMEM((32, 128), f32),
            pltpu.VMEM((48, 128), f32),
            pltpu.VMEM((S, DM), bf16),
            pltpu.VMEM((16, DM // 2 + 1, 256), bf16),
            pltpu.VMEM((12808, 128), u32),
            pltpu.VMEM((169, 128, 128), f32),
            pltpu.VMEM((12, 264, 128), f32),
            pltpu.VMEM((12, 264, 128), f32),
            pltpu.VMEM((24, 64, 128), u32),
            pltpu.VMEM((64, 64, 128), u32),
            pltpu.SMEM((64,), f32),
            pltpu.SMEM((1,), jnp.int32),
            pltpu.SemaphoreType.DMA((64,)),
            pltpu.SemaphoreType.DMA((2,)),
        ],
        compiler_params=pltpu.CompilerParams(vmem_limit_bytes=120 * 1024 * 1024,
                                             disable_semaphore_checks=True),
    )(x.reshape(S, DM), x.reshape(NSEG, SEG, DM), mem0.reshape(MEM, DM), wq, wk, wv,
      wo.reshape(H * DH, DM), bx.reshape(S, DM), w_r.T, w_i.T, jnp.asarray(fd), jnp.asarray(ms))
    return out.reshape(1, S, 2 * DM)


def pallas_concat_heads__memory_aug_recurrent_mem_tr__spectral_gfnet__prompt_kernel(
    A_x: jax.Array,
    A_mem0: jax.Array,
    A_Wq: jax.Array,
    A_Wk: jax.Array,
    A_Wv: jax.Array,
    A_Wo: jax.Array,
    A_seg_len,
    B_x: jax.Array,
    B_w_r: jax.Array,
    B_w_i: jax.Array,
):
    if isinstance(A_seg_len, int):
        assert A_seg_len == SEG
    assert A_x.shape == (1, S, DM) and A_mem0.shape == (1, MEM, DM) and A_Wq.shape == (DM, H, DH)
    assert B_x.shape == (1, S, DM) and B_w_r.shape == (S, DM // 2 + 1)
    return _run(A_x, A_mem0, A_Wq, A_Wk, A_Wv, A_Wo, B_x, B_w_r, B_w_i)
```

```python
import math

import numpy as np
import jax
import jax.numpy as jnp
import jax.experimental.pallas as pl
import jax.experimental.pallas.tpu as pltpu

bf16 = jnp.bfloat16
f32 = jnp.float32
u32 = jnp.uint32

S, DM = 2048, 1024
H, DH = 32, 128
MEM, SEG = 8, 32
NSEG = S // SEG
SQH = math.sqrt(0.5)

_PAIRS = ((0, 4), (1, 7), (2, 6), (3, 5))
_FIRST = np.array([[1, 1, 0, 0], [1, 0, 1, 0], [0, 1, 1, 0], [0, 1, 0, 1]], bool)


def _pack_rows(a):
    u = np.ascontiguousarray(a, dtype=np.float32).view(np.uint32).astype(np.uint64)
    b = ((u + 0x7FFF + ((u >> 16) & 1)) >> 16).astype(np.uint32)
    return (b[..., 0::2, :] | (b[..., 1::2, :] << 16)).astype(np.uint32)


def _tables():
    k2 = np.zeros((4, 128), np.int64)
    for t in range(4):
        odd = t % 2
        for lam in range(128):
            k = 2 * lam + odd
            if k % 8 not in _PAIRS[t]:
                k = 2 * (128 + 8 * (lam // 8) + (lam % 8 - 1 - odd) % 8) + odd
            assert k % 8 in _PAIRS[t]
            k2[t, lam] = k
    b = np.arange(128)[:, None]
    F = np.zeros((12, 128, 128))
    G = np.zeros((12, 128, 128))
    for t in range(4):
        th = 2 * np.pi * ((b * k2[t][None, :]) % DM) / DM
        C, Sn = np.cos(th), np.sin(th)
        first = ((k2[t] % 8) == _PAIRS[t][0])[None, :]
        assert np.array_equal(first[0], _FIRST[t][np.arange(128) % 4])
        if t == 0:
            im = -Sn
            im[:, 0] = (-1.0) ** np.arange(128)
            F[0:3] = im, np.where(first, im, C), np.where(first, C, im)
            G[0:3] = im, np.where(first, C, -im), np.where(first, -im, C)
            G[0:3, :, 0] *= 0.5
        else:
            Sg = np.where(first, Sn, -Sn)
            F[3 * t:3 * t + 3] = C, -(C + Sg), C - Sg
            G[3 * t:3 * t + 3] = F[3 * t:3 * t + 3]
    Finv = np.transpose(G, (0, 2, 1)) * (2.0 / DM)
    fd = _pack_rows(np.concatenate([F, Finv]))
    M = np.zeros((32, 128, 128))
    r = np.arange(64)[None, :]
    l = np.arange(64)[:, None]
    for j in range(32):
        th = 2 * np.pi * ((r * (j + 32 * l)) % S) / S
        C, Sn = np.cos(th), np.sin(th)
        M[j, :64, :64] = C
        M[j, :64, 64:] = Sn
        M[j, 64:, :64] = -Sn
        M[j, 64:, 64:] = C
    perm = np.arange(128).reshape(2, 8, 8).transpose(1, 0, 2).reshape(128)
    M = M[:, perm][:, :, perm]
    Minv = np.transpose(M, (0, 2, 1)) / S
    ms = _pack_rows(np.concatenate([M, Minv]))
    return fd, ms


def _tobf(w):
    return pltpu.bitcast(w, bf16)


def _tou(w):
    return pltpu.bitcast(w, u32)


def _dot(a, b):
    return jnp.dot(a, b, preferred_element_type=f32)


def _r8_real(x):
    t0, t1 = x[0] + x[4], x[0] - x[4]
    t2, t3 = x[2] + x[6], x[2] - x[6]
    t4, t5 = x[1] + x[5], x[1] - x[5]
    t6, t7 = x[3] + x[7], x[3] - x[7]
    e0, e1 = t0 + t2, t0 - t2
    o0, o1 = t4 + t6, t4 - t6
    u, v = SQH * (t5 - t7), SQH * (t5 + t7)
    return [(e0 + o0, e0 - o0), (t1 + u, v + t3), (e1, o1), (t1 - u, v - t3)]


def _r8_real_t(g):
    (z0, z4), (a1, b1), (e1, o1), (a3, b3) = g
    e0, o0 = z0 + z4, z0 - z4
    t1, u = a1 + a3, a1 - a3
    v, t3 = b1 + b3, b1 - b3
    t5, t7 = SQH * (v + u), SQH * (v - u)
    t0, t2 = e0 + e1, e0 - e1
    t4, t6 = o0 + o1, o0 - o1
    return [t0 + t1, t4 + t5, t2 + t3, t6 + t7, t0 - t1, t4 - t5, t2 - t3, t6 - t7]


def _dft4(u):
    (r0, i0), (r1, i1), (r2, i2), (r3, i3) = u
    sr, si, dr, di = r0 + r2, i0 + i2, r0 - r2, i0 - i2
    tr, ti, er, ei = r1 + r3, i1 + i3, r1 - r3, i1 - i3
    return [(sr + tr, si + ti), (dr + ei, di - er), (sr - tr, si - ti), (dr - ei, di + er)]


def _dft8(x):
    a = [(x[p][0] + x[p + 4][0], x[p][1] + x[p + 4][1]) for p in range(4)]
    d = [(x[p][0] - x[p + 4][0], x[p][1] - x[p + 4][1]) for p in range(4)]
    ev = _dft4(a)
    (r0, i0), (r1, i1), (r2, i2), (r3, i3) = d
    b1r, b1i = SQH * (r1 + i1), SQH * (i1 - r1)
    b3r, n3i = SQH * (i3 - r3), SQH * (r3 + i3)
    sr, si, dr, di = r0 + i2, i0 - r2, r0 - i2, i0 + r2
    tr, ti, er, ei = b1r + b3r, b1i - n3i, b1r - b3r, b1i + n3i
    od = [(sr + tr, si + ti), (dr + ei, di - er), (sr - tr, si - ti), (dr - ei, di + er)]
    return [ev[0], od[0], ev[1], od[1], ev[2], od[2], ev[3], od[3]]


def _swap(x):
    return [(b, a) for (a, b) in x]


G = 4
NG = H // G
OSPLIT = 24
NEG = -1e9
N_L1, N_L2, N_L3 = 4, 20, 8


def _kernel(x_hbm, x3_hbm, mem_hbm, wq_hbm, wk_hbm, wv_hbm, wo_hbm, bx_hbm, wr_hbm, wi_hbm,
            fd_hbm, ms_hbm, out_hbm,
            xo_ref, mem_ref, xcraw_ref, raw_ref, w0_ref, w1_ref, w2_ref, w3_ref, w4_ref, w5_ref,
            woraw_ref, wo_ref, xc_ref, qkvc_ref, kve_ref,
            oall_ref, fille_ref, fillo_ref, bx_ref, wt_ref, wp_ref, ub_ref, sa_ref, sb_ref, fd_ref, ms_ref,
            tw_ref, zero_ref, sem_in, sem_out):
    scale = DH ** -0.5
    w_hbm = (wq_hbm, wk_hbm, wv_hbm)
    w_refs = (w0_ref, w1_ref, w2_ref, w3_ref, w4_ref, w5_ref)

    def raw_copy(c, i=0, nd=DM):
        rows = pl.ds(pl.multiple_of(i * nd, nd), nd)
        return pltpu.make_async_copy(
            w_hbm[c // 2].at[rows, pl.ds((c % 2) * 16, 16), :],
            raw_ref.at[c % 4, rows], sem_in.at[8 + min(c, 3) * 8 + max(c - 3, 0) * 2 + i])

    def xc_copy(k):
        return pltpu.make_async_copy(
            x3_hbm.at[:, pl.ds(8, 8), pl.ds(pl.multiple_of(k * 128, 128), 128)], xcraw_ref.at[k], sem_in.at[40 + k])

    cp_x = pltpu.make_async_copy(x_hbm, xo_ref, sem_in.at[0])
    cp_mem = pltpu.make_async_copy(mem_hbm, mem_ref, sem_in.at[1])
    cp_wo = pltpu.make_async_copy(wo_hbm, woraw_ref, sem_in.at[2])
    cp_bx = pltpu.make_async_copy(bx_hbm, bx_ref, sem_in.at[3])
    cp_fd = pltpu.make_async_copy(fd_hbm, fd_ref, sem_in.at[4])
    cp_ms = pltpu.make_async_copy(ms_hbm, ms_ref, sem_in.at[5])
    cp_wt = [pltpu.make_async_copy(src.at[:, pl.ds(lg * 256, 256)], wt_ref.at[a * 8 + lg], sem_in.at[48 + a * 8 + lg])
             for a, src in enumerate((wr_hbm, wi_hbm)) for lg in range(8)]

    for i in range(8):
        raw_copy(0, i, 128).start()
        xc_copy(i).start()
        raw_copy(1, i, 128).start()
    for i in range(4):
        raw_copy(2, i, 256).start()
    for i in range(2):
        raw_copy(3, i, 512).start()

    zero_ref[0] = 0

    def pin_rows(r):
        return pl.ds(pl.multiple_of(r + zero_ref[0] * 32, 8), 8)

    for p in range(8):
        for jq in range(4):
            tw_ref[(p * 4 + jq) * 2] = jnp.float32(math.cos(2 * math.pi * p * jq / 32))
            tw_ref[(p * 4 + jq) * 2 + 1] = jnp.float32(math.sin(2 * math.pi * p * jq / 32))

    qi = jax.lax.broadcasted_iota(jnp.int32, (48, 128), 0)
    ki = jax.lax.broadcasted_iota(jnp.int32, (48, 128), 1)

    def between(v, lo, hi):
        return (v >= lo) & (v < hi)

    def table(keep, other):
        return jnp.where(other, -jnp.inf, jnp.where(keep, 0.0, NEG)).astype(f32)

    keep = between(qi, 8, 16) | between(ki, 8, 16) | (qi >= jnp.where(ki < 32, ki, ki - 24))
    fille_ref[...] = table(keep, ki >= 40)[:32]
    q_even = between(qi, 32, 40)
    k_even = between(ki, 32, 40) | (ki >= 48)
    qpos = jnp.where(qi < 32, qi, jnp.where(qi < 40, qi - 24, qi - 32))
    kpos = jnp.where(ki < 32, ki, jnp.where(ki < 40, ki - 24, jnp.where(ki < 48, ki - 32, ki - 48)))
    keep = between(qi, 8, 16) | between(ki, 8, 16) | (ki >= 56) | (qpos >= kpos)
    fillo_ref[...] = table(keep, (q_even != k_even) | (ki >= 64))

    def relayout16(c, d0):
        slot = c % 4
        w0 = pl.multiple_of(d0 // 2, 8)
        los, his = [], []
        for dd in range(8):
            a = _tou(raw_ref[slot, d0 + 2 * dd])
            b = _tou(raw_ref[slot, d0 + 2 * dd + 1])
            los.append((a & jnp.uint32(0xFFFF)) | (b << 16))
            his.append((a >> 16) | (b & jnp.uint32(0xFFFF0000)))
        lo = jnp.swapaxes(jnp.stack(los), 0, 1)
        hi = jnp.swapaxes(jnp.stack(his), 0, 1)
        for j in range(8):
            w_refs[c][2 * j, pl.ds(w0, 8), :] = lo[j]
            w_refs[c][2 * j + 1, pl.ds(w0, 8), :] = hi[j]

    def repack_wo64(r_start):
        r0 = pl.multiple_of(r_start, 64)
        w0 = pl.multiple_of(r_start // 2, 32)
        v = woraw_ref[pl.ds(r0, 64), :]
        for j in range(8):
            wo_ref[j, pl.ds(w0, 32), :] = _tou(v[:, j * 128:(j + 1) * 128])

    sub4 = jax.lax.broadcasted_iota(jnp.int32, (128, 128), 0) % 4

    def wp_store(t, kb, tile):
        v = tile.T
        for g in range(4):
            r0 = pl.multiple_of(t * 2560 + kb * 160 + g * 40, 8)
            wp_ref[pl.ds(r0, 32), :] = v[g * 32:(g + 1) * 32]

    def b_prep(lg, hb, par):
        cols = slice(hb * 128, (hb + 1) * 128)
        a = _tou(wt_ref[lg, 0:512, cols])
        b = _tou(wt_ref[8 + lg, 0:512, cols])
        if par == 0:
            w = (a << 16) | (b & jnp.uint32(0xFFFF))
            m = (sub4 == 0) | (sub4 == 2)
        else:
            w = (a & jnp.uint32(0xFFFF0000)) | (b >> 16)
            m = (sub4 == 0) | (sub4 == 3)
        top = w[:128]
        bot = pltpu.roll(w[128:].reshape(16, 8, 128), 1 + par, 1).reshape(128, 128)
        wp_store(par, lg * 2 + hb, jnp.where(m, top, bot))
        wp_store(par + 2, lg * 2 + hb, jnp.where(m, bot, top))
        if par == 0:
            na = jnp.broadcast_to(wt_ref[lg, 512:513, cols].astype(f32), (128, 128))
            nb = jnp.broadcast_to(wt_ref[8 + lg, 512:513, cols].astype(f32), (128, 128))
            wp_store(4, lg * 2 + hb, pltpu.bitcast(na, u32) | (pltpu.bitcast(nb, u32) >> 16))

    def gather_c(k):
        xc_ref[k] = _tou(xcraw_ref[k].astype(f32).reshape(512, 128).astype(bf16))

    def store_qkvc(n, y):
        for pp in range(NSEG // 2):
            qkvc_ref[pp, n] = y[pp * 8:(pp + 1) * 8]

    def q_unit(i, groups, first, last, fillers):
        xk = _tobf(xc_ref[i])
        w0 = pl.multiple_of(i * 64, 64)
        for g in groups:
            rhs = jnp.concatenate(
                [_tobf(w_refs[h // 16][h % 16, pl.ds(w0, 64), :]) for h in range(4 * g, 4 * g + 4)], axis=1)
            y = _dot(xk, rhs)
            for h in range(4 * g, 4 * g + 4):
                yh = y[:, (h % 4) * 128:(h % 4 + 1) * 128]
                if not first:
                    yh = yh + ub_ref[h * 4:(h + 1) * 4].reshape(512, 128)
                if last:
                    store_qkvc(h, _tou(yh.astype(bf16)))
                else:
                    ub_ref[h * 4:(h + 1) * 4] = yh.reshape(4, 128, 128)
            mine = fillers.get(g, [])
            for fi, item in enumerate(mine):
                r = (fi * 512 // len(mine)) // 8 * 8
                item(pltpu.bitcast(y[r:r + 8, 0:128], u32))

    def rl_item(c, d0):
        def item(pin):
            w_refs[c][15, pin_rows(512), :] = pin
            relayout16(c, d0)
        return item

    def spread(fillers, items, groups):
        for k, item in enumerate(items):
            fillers.setdefault(groups[k * len(groups) // len(items)], []).append(item)
        return fillers

    def half_items(f, c, i, groups):
        return spread(f, [rl_item(c, i * 128 + blk * 16) for blk in range(8)], groups)

    def piece_items(i):
        f = half_items(half_items({}, 1, i, (0, 1, 2)), 0, i + 1, (4, 5, 6))
        return spread(f, [lambda pin: gather_c(i + 1)], (6,))

    def chunk2_items(f, i, groups):
        return spread(f, [rl_item(2, i * 256 + blk * 16) for blk in range(16)], groups)

    def wait_piece(i):
        raw_copy(1, i, 128).wait()
        xc_copy(i + 1).wait()
        raw_copy(0, i + 1, 128).wait()

    raw_copy(0, 0, 128).wait()
    for blk in range(8):
        relayout16(0, blk * 16)
    xc_copy(0).wait()
    gather_c(0)
    q_unit(0, range(0, 2), True, False, {})
    raw_copy(1, 0, 128).wait()
    q_unit(0, range(2, 4), True, False, half_items({}, 1, 0, (2, 2, 3)))
    xc_copy(1).wait()
    raw_copy(0, 1, 128).wait()
    q_unit(0, range(4, 8), True, False,
           spread(half_items({}, 0, 1, (4, 5, 6)), [lambda pin: gather_c(1)], (6,)))

    def q_c(i, carry):
        wait_piece(i)
        q_unit(i, range(8), False, False, piece_items(i))
        return carry
    jax.lax.fori_loop(1, 5, q_c, 0)

    wait_piece(5)
    raw_copy(2, 0, 256).wait()
    raw_copy(2, 1, 256).wait()
    q_unit(5, range(8), False, False,
           chunk2_items(chunk2_items(piece_items(5), 0, (0, 1, 2, 3, 3)), 1, (3, 4, 5, 6, 7)))
    wait_piece(6)
    raw_copy(1, 7, 128).wait()
    raw_copy(2, 2, 256).wait()
    raw_copy(2, 3, 256).wait()
    q_unit(6, range(8), False, False, chunk2_items(piece_items(6), 2, (0, 1, 2, 3, 3, 4, 5, 7)))
    raw_copy(4).start()
    q_unit(7, range(8), False, True, chunk2_items(half_items({}, 1, 7, (0, 1, 2)), 3, (3, 4, 5, 6)))
    raw_copy(5).start()
    for cp in cp_wt:
        cp.start()
    cp_wo.start()
    cp_x.start()
    cp_mem.start()
    cp_bx.start()
    cp_fd.start()
    cp_ms.start()

    def bulk_iter(c, i, n_rl, rl_start):
        xc = jnp.concatenate([_tobf(xc_ref[k]) for k in range(8)], axis=1)
        for t in range(8):
            n = i * 8 + t
            y = _tou(_dot(xc, _tobf(w_refs[c][n, 0:512])).astype(bf16))
            store_qkvc(c * 16 + n, y)
            for blk in range(n_rl):
                pin = y[blk * (256 // n_rl):blk * (256 // n_rl) + 8]
                if c + 1 < 6:
                    w_refs[c + 1][15, pin_rows(512), :] = pin
                    relayout16(c + 1, rl_start + (t * n_rl + blk) * 16)
                else:
                    wo_ref[7, pin_rows(2048), :] = pin
                    repack_wo64(rl_start + (t * n_rl + blk) * 64)
            if c >= 4:
                wp_ref[pin_rows(12800), :] = y[32:40]
                b_prep((c - 4) * 4 + i * 2 + t // 4, (t // 2) % 2, t % 2)

    for c in range(2, 6):
        if c == 4:
            for cp in cp_wt:
                cp.wait()
        if c == 5:
            cp_wo.wait()
        elif c > 2:
            raw_copy(c + 1).wait()

        def bulk(i, carry, c=c):
            if c == 2:
                raw_copy(3, i, 512).wait()
            bulk_iter(c, i, 4, i * (512 if c + 1 < 6 else 2048))
            return carry
        jax.lax.fori_loop(0, 2, bulk, 0)

    cp_x.wait()
    cp_mem.wait()
    cp_bx.wait()
    cp_fd.wait()

    lane0 = jax.lax.broadcasted_iota(jnp.int32, (8, 128), 1) == 0

    def ub_get(n, g):
        return ub_ref[n, g * 16:g * 16 + 8], ub_ref[n, g * 16 + 8:g * 16 + 16]

    def ub_put(n, g, v):
        ub_ref[n, g * 16:g * 16 + 8] = v[0]
        ub_ref[n, g * 16 + 8:g * 16 + 16] = v[1]

    lane4 = jax.lax.broadcasted_iota(jnp.int32, (8, 128), 1) % 4

    def first_lanes(t):
        la, lb = [k for k in range(4) if _FIRST[t][k]]
        return (lane4 == la) | (lane4 == lb)

    def stage(st_ref, t, rows, vals):
        for k in range(3):
            st_ref[3 * t + k, rows] = vals[k]

    def d_products(st_ref, d, t, rows):
        return [_dot(st_ref[3 * t + k, rows].astype(bf16), _tobf(fd_ref[d * 12 + 3 * t + k])) for k in range(3)]

    def twiddles(p):
        return [(tw_ref[(p * 4 + jq) * 2], tw_ref[(p * 4 + jq) * 2 + 1]) for jq in range(4)]

    st_refs = (sa_ref, sb_ref)

    def p1_pre(p, slot, rs, q):
        def item(y):
            st_refs[slot][7, pin_rows(256), :] = y
            rows = pl.multiple_of(q * 512 + p * 64 + rs * 16, 16)
            xq = bx_ref[pl.ds(rows, 16), :].astype(f32)
            zz = _r8_real([xq[:, a * 128:(a + 1) * 128] for a in range(8)])
            for t in range(4):
                for e in range(2):
                    r = ((rs * 2 + e) * 4 + q) * 8
                    a, b = zz[t][0][e * 8:(e + 1) * 8], zz[t][1][e * 8:(e + 1) * 8]
                    stage(st_refs[slot], t, slice(r, r + 8), (a + b, b, a))
        return item

    def p1_mm(p, slot, t):
        def item(y):
            cs = twiddles(p)

            def emit(t, g, u):
                a = _dft4(u)
                for jq in range(4):
                    re, im = a[jq]
                    if jq > 0:
                        c, sn = cs[jq]
                        re, im = re * c + im * sn, im * c - re * sn
                    ub_put((t * 4 + jq) * 8 + p, g, (re, im))

            def emit_real(g, u):
                sr, dr, tr, er = u[0] + u[2], u[0] - u[2], u[1] + u[3], u[1] - u[3]
                a2 = sr - tr
                (_, _), (c1, s1), (c2, s2), (c3, s3) = cs
                ub_put(16 * 8 + p, g, (sr + tr, jnp.zeros_like(sr)))
                ub_put(17 * 8 + p, g, (dr * c1 - er * s1, er * (-c1) - dr * s1))
                ub_put(18 * 8 + p, g, (a2 * c2, a2 * (-s2)))
                ub_put(19 * 8 + p, g, (dr * c3 + er * s3, er * c3 - dr * s3))

            first = first_lanes(t)
            for m in range(4):
                ks = d_products(st_refs[slot], 0, t, slice(m * 64, (m + 1) * 64))
                for e in range(2):
                    u = []
                    for q in range(4):
                        r = (e * 4 + q) * 8
                        k1, k2, k3 = [k[r:r + 8] for k in ks]
                        if t == 0:
                            u.append((jnp.where(first, k3, k2), k1 - jnp.where(first, k2, k3)))
                        else:
                            u.append((k2 + k1, (k3 - k1) * jnp.where(first, 1.0, -1.0)))
                    if t == 0:
                        emit_real(m * 2 + e, [im for (_, im) in u])
                        u = [(re, jnp.where(lane0, 0.0, im)) for (re, im) in u]
                    emit(t, m * 2 + e, u)
        return item

    def p2_bfly(u, g, inverse):
        def item(y):
            if y is not None:
                ub_ref[168, pin_rows(0), :] = y
            x = [ub_get(u * 8 + p, g) for p in range(8)]
            x = _swap(_dft8(_swap(x))) if inverse else _dft8(x)
            for p in range(8):
                ub_put(u * 8 + p, g, x[p])
        return item

    def p2_fwd(u, jps):
        def item(y):
            t = u // 4
            jq = u % 4
            xs = [_dot(_tobf(ms_ref[jq + 4 * jp]), ub_ref[u * 8 + jp].astype(bf16)) for jp in jps]
            for jp, xx in zip(jps, xs):
                w = wp_ref[pl.ds(t * 2560 + jq + 4 * jp, 64, stride=40), :]
                wr = pltpu.bitcast(w & jnp.uint32(0xFFFF0000), f32)
                wi = pltpu.bitcast(w << 16, f32)
                for g in range(8):
                    xr, xi = xx[g * 16:g * 16 + 8], xx[g * 16 + 8:g * 16 + 16]
                    a, b = wr[g * 8:(g + 1) * 8], wi[g * 8:(g + 1) * 8]
                    ub_put(u * 8 + jp, g, (xr * a - xi * b, xr * b + xi * a))
        return item

    def p2_inv(u, jps):
        def item(y):
            jq = u % 4
            zs = [_dot(_tobf(ms_ref[32 + jq + 4 * jp]), ub_ref[u * 8 + jp].astype(bf16)) for jp in jps]
            for jp, zz in zip(jps, zs):
                ub_ref[u * 8 + jp] = zz
        return item

    def p3_pre(p, g, ts):
        def item(y):
            sa_ref[7, pin_rows(256), :] = y
            cs = twiddles(p)

            def fetch(t):
                a = []
                for jq in range(4):
                    re, im = ub_get((t * 4 + jq) * 8 + p, g)
                    if jq > 0:
                        c, sn = cs[jq]
                        re, im = re * c - im * sn, im * c + re * sn
                    a.append((re, im))
                return _swap(_dft4(_swap(a)))

            for t in ts:
                u = fetch(t)
                if t == 0:
                    ny = fetch(4)
                    u = [(u[q][0], jnp.where(lane0, ny[q][0], u[q][1])) for q in range(4)]
                first = first_lanes(t)
                for q in range(4):
                    re, im = u[q]
                    if t == 0:
                        vals = (im, jnp.where(first, re, im), jnp.where(first, im, re))
                    else:
                        im = im * jnp.where(first, 1.0, -1.0)
                        vals = (re + im, im, re)
                    stage(sa_ref, t, slice(q * 64 + g * 8, q * 64 + (g + 1) * 8), vals)
        return item

    def p3_mm(p, q):
        def item(y):
            g = []
            for t in range(4):
                k1, k2, k3 = d_products(sa_ref, 1, t, slice(q * 64, (q + 1) * 64))
                g.append((k2 + k1, k3 + k1 if t == 0 else k3 - k1))
            yy = _r8_real_t(g)
            rows = pl.multiple_of(q * 512 + p * 64, 64)
            for a in range(8):
                bx_ref[pl.ds(rows, 64), a * 128:(a + 1) * 128] = yy[a].astype(bf16)
        return item

    def b_out(p):
        for q in range(4):
            rows = pl.multiple_of(q * 512 + p * 64, 64)
            pltpu.make_async_copy(bx_ref.at[pl.ds(rows, 64), :],
                                  out_hbm.at[pl.ds(rows, 64), pl.ds(DM, DM)], sem_out.at[1]).start()

    def step(pp, odd, mem, hooks):
        r0 = pl.multiple_of(pp * 64 + 32 * odd, SEG)
        xs = xo_ref[pl.ds(r0, SEG), :]
        x_lo = xs[0:8].astype(f32)
        hm = jnp.concatenate(
            [jnp.concatenate([x_lo, jnp.concatenate(mem, axis=1)], axis=0).astype(bf16), xs[16:32]], axis=0)
        fill = fillo_ref[:, 0:64] if odd else fille_ref[:, 0:48]
        nrow = 48 if odd else 32
        qkv, ps = {}, {}

        def do_qkv(g):
            for h in range(g * G, (g + 1) * G):
                for t in range(3):
                    y32 = _dot(hm, _tobf(w_refs[t * 2 + h // 16][h % 16, 0:512]))
                    y = y32.astype(bf16)
                    parts = [y]
                    if odd or t > 0:
                        parts.append(_tobf(qkvc_ref[pp, t * H + h]))
                    if t > 0:
                        if odd:
                            parts.append(_tobf(kve_ref[(t - 1) * H + h]))
                        else:
                            kve_ref[(t - 1) * H + h] = _tou(y[0:16])
                    qkv[(t, h)] = jnp.concatenate(parts, axis=0) if len(parts) > 1 else y
                for item in hooks.get(h, ()):
                    item(y32[0:8])

        def do_s(g):
            for h in range(g * G, (g + 1) * G):
                sc = jax.lax.dot_general(qkv[(0, h)], qkv[(1, h)], (((1,), (1,)), ((), ())),
                                         preferred_element_type=f32)
                sc = jnp.where(fill == 0.0, sc * scale, fill)
                e = jnp.exp(sc - jnp.max(sc, axis=1, keepdims=True))
                den = jnp.sum(e, axis=1, keepdims=True)
                r = pl.reciprocal(den, approx=True)
                r = r * (2.0 - den * r)
                ps[h] = (e * r).astype(bf16)

        def do_pv(g):
            for h in range(g * G, (g + 1) * G):
                oall_ref[h, 0:nrow // 2] = _tou(_dot(ps[h], qkv[(2, h)]).astype(bf16))

        def do_o(j, h0, h1):
            lhs = jnp.concatenate([_tobf(oall_ref[h, 0:nrow // 2]) for h in range(h0, h1)], axis=1)
            return _dot(lhs, _tobf(wo_ref[j, h0 * 64:h1 * 64, :]))

        for g in range(NG):
            do_qkv(g)
            if g >= 1:
                do_s(g - 1)
            if g >= 2:
                do_pv(g - 2)
        part = {}
        for j in range(8):
            items = hooks.get(('o', j), ())
            if items:
                half = do_o(j, 0, OSPLIT // 2)
                items[0](half[0:8])
                part[j] = do_o(j, OSPLIT // 2, OSPLIT) + half
                items[1](part[j][0:8])
            else:
                part[j] = do_o(j, 0, OSPLIT)
            if j == 2:
                do_s(NG - 1)
                do_pv(NG - 2)
            if j == 5:
                do_pv(NG - 1)
        new_mem = []
        for j in range(8):
            cols = slice(j * 128, (j + 1) * 128)
            res = do_o(j, OSPLIT, H) + part[j]
            new_mem.append(res[8:16])
            if odd:
                xo_ref[pl.ds(r0, SEG), cols] = jnp.concatenate(
                    [res[0:8], res[40:48], res[16:32]], axis=0).astype(bf16)
                xo_ref[pl.ds(r0 - 24, 8), cols] = res[32:40].astype(bf16)
            else:
                xo_ref[pl.ds(r0, SEG), cols] = res.astype(bf16)
        for item in hooks.get(H, ()):
            item(None)
        if odd:
            rows = pl.ds(pl.multiple_of(pp * 64, 64), 64)
            pltpu.make_async_copy(xo_ref.at[rows, :], out_hbm.at[rows, pl.ds(0, DM)], sem_out.at[0]).start()
        return new_mem

    def l1(i, mem):
        he = {h: [p1_pre(2 * i + h // 16, h // 16, (h % 16) // 4, h % 4)] for h in range(32)}
        he[21].append(p1_mm(2 * i, 0, 0))
        he[25].append(p1_mm(2 * i, 0, 1))
        he[29].append(p1_mm(2 * i, 0, 2))
        he[H] = [p1_mm(2 * i, 0, 3)]
        ho = {1 + 4 * t: [p1_mm(2 * i + 1, 1, t)] for t in range(4)}
        mem = step(i, 0, mem, he)
        mem = step(i, 1, mem, ho)
        return mem

    def l2(i, mem):
        u = i - N_L1
        he = {3: [p2_fwd(u, range(0, 4))], 7: [p2_fwd(u, range(4, 8))], H: [p2_inv(u, range(0, 8))]}
        ho = {('o', j): [p2_bfly(u, j, True), p2_bfly(u + 1, j, False)] for j in range(8)}
        mem = step(i, 0, mem, he)
        mem = step(i, 1, mem, ho)
        return mem

    def l3(i, mem):
        p = i - N_L1 - N_L2
        he = {h: [p3_pre(p, h // 2, (0, 1) if h % 2 == 0 else (2, 3))] for h in range(16)}
        he[21] = [p3_mm(p, 0)]
        he[29] = [p3_mm(p, 1)]
        he[H] = [p3_mm(p, 2)]
        ho = {5: [p3_mm(p, 3)], 12: [lambda y: b_out(p)]}
        mem = step(i, 0, mem, he)
        mem = step(i, 1, mem, ho)
        return mem

    m0 = mem_ref[...].astype(f32)
    mem = [m0[:, j * 128:(j + 1) * 128] for j in range(8)]
    mem = jax.lax.fori_loop(0, N_L1, l1, mem)
    cp_ms.wait()
    for g in range(8):
        p2_bfly(0, g, False)(None)
    mem = jax.lax.fori_loop(N_L1, N_L1 + N_L2, l2, mem)
    mem = jax.lax.fori_loop(N_L1 + N_L2, NSEG // 2, l3, mem)

    pltpu.make_async_copy(xo_ref, out_hbm.at[:, pl.ds(0, DM)], sem_out.at[0]).wait()
    pltpu.make_async_copy(bx_ref, out_hbm.at[:, pl.ds(DM, DM)], sem_out.at[1]).wait()


@jax.jit
def _run(x, mem0, wq, wk, wv, wo, bx, w_r, w_i):
    fd, ms = _tables()
    hbm = pl.BlockSpec(memory_space=pl.ANY)
    out = pl.pallas_call(
        _kernel,
        out_shape=jax.ShapeDtypeStruct((S, 2 * DM), bf16),
        in_specs=[hbm] * 12,
        out_specs=hbm,
        scratch_shapes=[
            pltpu.VMEM((S, DM), bf16),
            pltpu.VMEM((MEM, DM), bf16),
            pltpu.VMEM((8, NSEG, 8, 128), bf16),
            pltpu.VMEM((4, DM, 16, DH), bf16),
        ] + [pltpu.VMEM((16, DM // 2 + 8, DH), u32)] * 6 + [
            pltpu.VMEM((H * DH, DM), bf16),
            pltpu.VMEM((8, H * DH // 2 + 8, 128), u32),
            pltpu.VMEM((8, 256, 128), u32),
            pltpu.VMEM((NSEG // 2, 3 * H, 8, 128), u32),
            pltpu.VMEM((2 * H, 8, 128), u32),
            pltpu.VMEM((H, 24, DH), u32),
            pltpu.VMEM((32, 128), f32),
            pltpu.VMEM((48, 128), f32),
            pltpu.VMEM((S, DM), bf16),
            pltpu.VMEM((16, DM // 2 + 1, 256), bf16),
            pltpu.VMEM((12808, 128), u32),
            pltpu.VMEM((169, 128, 128), f32),
            pltpu.VMEM((12, 264, 128), f32),
            pltpu.VMEM((12, 264, 128), f32),
            pltpu.VMEM((24, 64, 128), u32),
            pltpu.VMEM((64, 64, 128), u32),
            pltpu.SMEM((64,), f32),
            pltpu.SMEM((1,), jnp.int32),
            pltpu.SemaphoreType.DMA((64,)),
            pltpu.SemaphoreType.DMA((2,)),
        ],
        compiler_params=pltpu.CompilerParams(vmem_limit_bytes=120 * 1024 * 1024,
                                             disable_semaphore_checks=True),
    )(x.reshape(S, DM), x.reshape(NSEG, SEG, DM), mem0.reshape(MEM, DM), wq, wk, wv,
      wo.reshape(H * DH, DM), bx.reshape(S, DM), w_r.T, w_i.T, jnp.asarray(fd), jnp.asarray(ms))
    return out.reshape(1, S, 2 * DM)


def pallas_concat_heads__memory_aug_recurrent_mem_tr__spectral_gfnet__prompt_kernel(
    A_x: jax.Array,
    A_mem0: jax.Array,
    A_Wq: jax.Array,
    A_Wk: jax.Array,
    A_Wv: jax.Array,
    A_Wo: jax.Array,
    A_seg_len,
    B_x: jax.Array,
    B_w_r: jax.Array,
    B_w_i: jax.Array,
):
    if isinstance(A_seg_len, int):
        assert A_seg_len == SEG
    assert A_x.shape == (1, S, DM) and A_mem0.shape == (1, MEM, DM) and A_Wq.shape == (DM, H, DH)
    assert B_x.shape == (1, S, DM) and B_w_r.shape == (S, DM // 2 + 1)
    return _run(A_x, A_mem0, A_Wq, A_Wk, A_Wv, A_Wo, B_x, B_w_r, B_w_i)
```

```python
import math

import numpy as np
import jax
import jax.numpy as jnp
import jax.experimental.pallas as pl
import jax.experimental.pallas.tpu as pltpu

bf16 = jnp.bfloat16
f32 = jnp.float32
u32 = jnp.uint32

S, DM = 2048, 1024
H, DH = 32, 128
MEM, SEG = 8, 32
NSEG = S // SEG
SQH = math.sqrt(0.5)

_PAIRS = ((0, 4), (1, 7), (2, 6), (3, 5))
_FIRST = np.array([[1, 1, 0, 0], [1, 0, 1, 0], [0, 1, 1, 0], [0, 1, 0, 1]], bool)


def _pack_rows(a):
    u = np.ascontiguousarray(a, dtype=np.float32).view(np.uint32).astype(np.uint64)
    b = ((u + 0x7FFF + ((u >> 16) & 1)) >> 16).astype(np.uint32)
    return (b[..., 0::2, :] | (b[..., 1::2, :] << 16)).astype(np.uint32)


def _tables():
    k2 = np.zeros((4, 128), np.int64)
    for t in range(4):
        odd = t % 2
        for lam in range(128):
            k = 2 * lam + odd
            if k % 8 not in _PAIRS[t]:
                k = 2 * (128 + 8 * (lam // 8) + (lam % 8 - 1 - odd) % 8) + odd
            assert k % 8 in _PAIRS[t]
            k2[t, lam] = k
    b = np.arange(128)[:, None]
    F = np.zeros((12, 128, 128))
    G = np.zeros((12, 128, 128))
    for t in range(4):
        th = 2 * np.pi * ((b * k2[t][None, :]) % DM) / DM
        C, Sn = np.cos(th), np.sin(th)
        first = ((k2[t] % 8) == _PAIRS[t][0])[None, :]
        assert np.array_equal(first[0], _FIRST[t][np.arange(128) % 4])
        if t == 0:
            im = -Sn
            im[:, 0] = (-1.0) ** np.arange(128)
            F[0:3] = im, np.where(first, im, C), np.where(first, C, im)
            G[0:3] = im, np.where(first, C, -im), np.where(first, -im, C)
            G[0:3, :, 0] *= 0.5
        else:
            Sg = np.where(first, Sn, -Sn)
            F[3 * t:3 * t + 3] = C, -(C + Sg), C - Sg
            G[3 * t:3 * t + 3] = F[3 * t:3 * t + 3]
    Finv = np.transpose(G, (0, 2, 1)) * (2.0 / DM)
    fd = _pack_rows(np.concatenate([F, Finv]))
    M = np.zeros((32, 128, 128))
    r = np.arange(64)[None, :]
    l = np.arange(64)[:, None]
    for j in range(32):
        th = 2 * np.pi * ((r * (j + 32 * l)) % S) / S
        C, Sn = np.cos(th), np.sin(th)
        M[j, :64, :64] = C
        M[j, :64, 64:] = Sn
        M[j, 64:, :64] = -Sn
        M[j, 64:, 64:] = C
    perm = np.arange(128).reshape(2, 8, 8).transpose(1, 0, 2).reshape(128)
    M = M[:, perm][:, :, perm]
    Minv = np.transpose(M, (0, 2, 1)) / S
    ms = _pack_rows(np.concatenate([M, Minv]))
    return fd, ms


def _tobf(w):
    return pltpu.bitcast(w, bf16)


def _tou(w):
    return pltpu.bitcast(w, u32)


def _dot(a, b):
    return jnp.dot(a, b, preferred_element_type=f32)


def _r8_real(x):
    t0, t1 = x[0] + x[4], x[0] - x[4]
    t2, t3 = x[2] + x[6], x[2] - x[6]
    t4, t5 = x[1] + x[5], x[1] - x[5]
    t6, t7 = x[3] + x[7], x[3] - x[7]
    e0, e1 = t0 + t2, t0 - t2
    o0, o1 = t4 + t6, t4 - t6
    u, v = SQH * (t5 - t7), SQH * (t5 + t7)
    return [(e0 + o0, e0 - o0), (t1 + u, v + t3), (e1, o1), (t1 - u, v - t3)]


def _r8_real_t(g):
    (z0, z4), (a1, b1), (e1, o1), (a3, b3) = g
    e0, o0 = z0 + z4, z0 - z4
    t1, u = a1 + a3, a1 - a3
    v, t3 = b1 + b3, b1 - b3
    t5, t7 = SQH * (v + u), SQH * (v - u)
    t0, t2 = e0 + e1, e0 - e1
    t4, t6 = o0 + o1, o0 - o1
    return [t0 + t1, t4 + t5, t2 + t3, t6 + t7, t0 - t1, t4 - t5, t2 - t3, t6 - t7]


def _dft4(u):
    (r0, i0), (r1, i1), (r2, i2), (r3, i3) = u
    sr, si, dr, di = r0 + r2, i0 + i2, r0 - r2, i0 - i2
    tr, ti, er, ei = r1 + r3, i1 + i3, r1 - r3, i1 - i3
    return [(sr + tr, si + ti), (dr + ei, di - er), (sr - tr, si - ti), (dr - ei, di + er)]


def _dft8(x):
    a = [(x[p][0] + x[p + 4][0], x[p][1] + x[p + 4][1]) for p in range(4)]
    d = [(x[p][0] - x[p + 4][0], x[p][1] - x[p + 4][1]) for p in range(4)]
    ev = _dft4(a)
    (r0, i0), (r1, i1), (r2, i2), (r3, i3) = d
    b1r, b1i = SQH * (r1 + i1), SQH * (i1 - r1)
    b3r, n3i = SQH * (i3 - r3), SQH * (r3 + i3)
    sr, si, dr, di = r0 + i2, i0 - r2, r0 - i2, i0 + r2
    tr, ti, er, ei = b1r + b3r, b1i - n3i, b1r - b3r, b1i + n3i
    od = [(sr + tr, si + ti), (dr + ei, di - er), (sr - tr, si - ti), (dr - ei, di + er)]
    return [ev[0], od[0], ev[1], od[1], ev[2], od[2], ev[3], od[3]]


def _swap(x):
    return [(b, a) for (a, b) in x]


G = 4
NG = H // G
OSPLIT = 24
NEG = -1e9
N_L1, N_L2, N_L3 = 4, 20, 8


def _kernel(x_hbm, x3_hbm, mem_hbm, wq_hbm, wk_hbm, wv_hbm, wo_hbm, bx_hbm, wr_hbm, wi_hbm,
            fd_hbm, ms_hbm, out_hbm,
            xo_ref, mem_ref, xcraw_ref, raw_ref, w0_ref, w1_ref, w2_ref, w3_ref, w4_ref, w5_ref,
            woraw_ref, wo_ref, xc_ref, qkvc_ref, kve_ref,
            oall_ref, fille_ref, fillo_ref, bx_ref, wt_ref, wp_ref, ub_ref, sa_ref, sb_ref, fd_ref, ms_ref,
            tw_ref, zero_ref, sem_in, sem_out):
    scale = DH ** -0.5
    w_hbm = (wq_hbm, wk_hbm, wv_hbm)
    w_refs = (w0_ref, w1_ref, w2_ref, w3_ref, w4_ref, w5_ref)

    def raw_copy(c, i=0, nd=DM):
        rows = pl.ds(pl.multiple_of(i * nd, nd), nd)
        return pltpu.make_async_copy(
            w_hbm[c // 2].at[rows, pl.ds((c % 2) * 16, 16), :],
            raw_ref.at[c % 4, rows], sem_in.at[8 + min(c, 3) * 8 + max(c - 3, 0) * 2 + i])

    def xc_copy(k):
        return pltpu.make_async_copy(
            x3_hbm.at[:, pl.ds(8, 8), pl.ds(pl.multiple_of(k * 128, 128), 128)], xcraw_ref.at[k], sem_in.at[40 + k])

    cp_x = pltpu.make_async_copy(x_hbm, xo_ref, sem_in.at[0])
    cp_mem = pltpu.make_async_copy(mem_hbm, mem_ref, sem_in.at[1])
    cp_wo = pltpu.make_async_copy(wo_hbm, woraw_ref, sem_in.at[2])
    cp_bx = pltpu.make_async_copy(bx_hbm, bx_ref, sem_in.at[3])
    cp_fd = pltpu.make_async_copy(fd_hbm, fd_ref, sem_in.at[4])
    cp_ms = pltpu.make_async_copy(ms_hbm, ms_ref, sem_in.at[5])
    cp_wt = [pltpu.make_async_copy(src.at[:, pl.ds(lg * 256, 256)], wt_ref.at[a * 8 + lg], sem_in.at[48 + a * 8 + lg])
             for a, src in enumerate((wr_hbm, wi_hbm)) for lg in range(8)]

    for i in range(8):
        raw_copy(0, i, 128).start()
        xc_copy(i).start()
        raw_copy(1, i, 128).start()
    for i in range(4):
        raw_copy(2, i, 256).start()
    for i in range(2):
        raw_copy(3, i, 512).start()

    zero_ref[0] = 0

    def pin_rows(r):
        return pl.ds(pl.multiple_of(r + zero_ref[0] * 32, 8), 8)

    for p in range(8):
        for jq in range(4):
            tw_ref[(p * 4 + jq) * 2] = jnp.float32(math.cos(2 * math.pi * p * jq / 32))
            tw_ref[(p * 4 + jq) * 2 + 1] = jnp.float32(math.sin(2 * math.pi * p * jq / 32))

    qi = jax.lax.broadcasted_iota(jnp.int32, (48, 128), 0)
    ki = jax.lax.broadcasted_iota(jnp.int32, (48, 128), 1)

    def between(v, lo, hi):
        return (v >= lo) & (v < hi)

    def table(keep, other):
        return jnp.where(other, -jnp.inf, jnp.where(keep, 0.0, NEG)).astype(f32)

    keep = between(qi, 8, 16) | between(ki, 8, 16) | (qi >= jnp.where(ki < 32, ki, ki - 24))
    fille_ref[...] = table(keep, ki >= 40)[:32]
    q_even = between(qi, 32, 40)
    k_even = between(ki, 32, 40) | (ki >= 48)
    qpos = jnp.where(qi < 32, qi, jnp.where(qi < 40, qi - 24, qi - 32))
    kpos = jnp.where(ki < 32, ki, jnp.where(ki < 40, ki - 24, jnp.where(ki < 48, ki - 32, ki - 48)))
    keep = between(qi, 8, 16) | between(ki, 8, 16) | (ki >= 56) | (qpos >= kpos)
    fillo_ref[...] = table(keep, (q_even != k_even) | (ki >= 64))

    def relayout16(c, d0):
        slot = c % 4
        w0 = pl.multiple_of(d0 // 2, 8)
        los, his = [], []
        for dd in range(8):
            a = _tou(raw_ref[slot, d0 + 2 * dd])
            b = _tou(raw_ref[slot, d0 + 2 * dd + 1])
            los.append((a & jnp.uint32(0xFFFF)) | (b << 16))
            his.append((a >> 16) | (b & jnp.uint32(0xFFFF0000)))
        lo = jnp.swapaxes(jnp.stack(los), 0, 1)
        hi = jnp.swapaxes(jnp.stack(his), 0, 1)
        for j in range(8):
            w_refs[c][2 * j, pl.ds(w0, 8), :] = lo[j]
            w_refs[c][2 * j + 1, pl.ds(w0, 8), :] = hi[j]

    def repack_wo64(r_start):
        r0 = pl.multiple_of(r_start, 64)
        w0 = pl.multiple_of(r_start // 2, 32)
        v = woraw_ref[pl.ds(r0, 64), :]
        for j in range(8):
            wo_ref[j, pl.ds(w0, 32), :] = _tou(v[:, j * 128:(j + 1) * 128])

    sub4 = jax.lax.broadcasted_iota(jnp.int32, (128, 128), 0) % 4

    def wp_store(t, kb, tile):
        v = tile.T
        for g in range(4):
            r0 = pl.multiple_of(t * 2560 + kb * 160 + g * 40, 8)
            wp_ref[pl.ds(r0, 32), :] = v[g * 32:(g + 1) * 32]

    def b_prep(lg, hb, par):
        cols = slice(hb * 128, (hb + 1) * 128)
        a = _tou(wt_ref[lg, 0:512, cols])
        b = _tou(wt_ref[8 + lg, 0:512, cols])
        if par == 0:
            w = (a << 16) | (b & jnp.uint32(0xFFFF))
            m = (sub4 == 0) | (sub4 == 2)
        else:
            w = (a & jnp.uint32(0xFFFF0000)) | (b >> 16)
            m = (sub4 == 0) | (sub4 == 3)
        top = w[:128]
        bot = pltpu.roll(w[128:].reshape(16, 8, 128), 1 + par, 1).reshape(128, 128)
        wp_store(par, lg * 2 + hb, jnp.where(m, top, bot))
        wp_store(par + 2, lg * 2 + hb, jnp.where(m, bot, top))
        if par == 0:
            na = jnp.broadcast_to(wt_ref[lg, 512:513, cols].astype(f32), (128, 128))
            nb = jnp.broadcast_to(wt_ref[8 + lg, 512:513, cols].astype(f32), (128, 128))
            wp_store(4, lg * 2 + hb, pltpu.bitcast(na, u32) | (pltpu.bitcast(nb, u32) >> 16))

    def gather_c(k):
        xc_ref[k] = _tou(xcraw_ref[k].astype(f32).reshape(512, 128).astype(bf16))

    def store_qkvc(n, y):
        for pp in range(NSEG // 2):
            qkvc_ref[pp, n] = y[pp * 8:(pp + 1) * 8]

    def q_unit(i, groups, first, last, fillers):
        xk = _tobf(xc_ref[i])
        w0 = pl.multiple_of(i * 64, 64)
        for g in groups:
            rhs = jnp.concatenate(
                [_tobf(w_refs[h // 16][h % 16, pl.ds(w0, 64), :]) for h in range(4 * g, 4 * g + 4)], axis=1)
            y = _dot(xk, rhs)
            for h in range(4 * g, 4 * g + 4):
                yh = y[:, (h % 4) * 128:(h % 4 + 1) * 128]
                if not first:
                    yh = yh + ub_ref[h * 4:(h + 1) * 4].reshape(512, 128)
                if last:
                    store_qkvc(h, _tou(yh.astype(bf16)))
                else:
                    ub_ref[h * 4:(h + 1) * 4] = yh.reshape(4, 128, 128)
            mine = fillers.get(g, [])
            for fi, item in enumerate(mine):
                r = (fi * 512 // len(mine)) // 8 * 8
                item(pltpu.bitcast(y[r:r + 8, 0:128], u32))

    def rl_item(c, d0):
        def item(pin):
            w_refs[c][15, pin_rows(512), :] = pin
            relayout16(c, d0)
        return item

    def spread(fillers, items, groups):
        for k, item in enumerate(items):
            fillers.setdefault(groups[k * len(groups) // len(items)], []).append(item)
        return fillers

    def half_items(f, c, i, groups):
        return spread(f, [rl_item(c, i * 128 + blk * 16) for blk in range(8)], groups)

    def piece_items(i):
        f = half_items(half_items({}, 1, i, (0, 1, 2)), 0, i + 1, (4, 5, 6))
        return spread(f, [lambda pin: gather_c(i + 1)], (6,))

    def chunk2_items(f, i, groups):
        return spread(f, [rl_item(2, i * 256 + blk * 16) for blk in range(16)], groups)

    def wait_piece(i):
        raw_copy(1, i, 128).wait()
        xc_copy(i + 1).wait()
        raw_copy(0, i + 1, 128).wait()

    raw_copy(0, 0, 128).wait()
    for blk in range(8):
        relayout16(0, blk * 16)
    xc_copy(0).wait()
    gather_c(0)
    q_unit(0, range(0, 2), True, False, {})
    raw_copy(1, 0, 128).wait()
    q_unit(0, range(2, 4), True, False, half_items({}, 1, 0, (2, 2, 3)))
    xc_copy(1).wait()
    raw_copy(0, 1, 128).wait()
    q_unit(0, range(4, 8), True, False,
           spread(half_items({}, 0, 1, (4, 5, 6)), [lambda pin: gather_c(1)], (6,)))

    def q_c(i, carry):
        wait_piece(i)
        q_unit(i, range(8), False, False, piece_items(i))
        return carry
    jax.lax.fori_loop(1, 5, q_c, 0)

    wait_piece(5)
    raw_copy(2, 0, 256).wait()
    raw_copy(2, 1, 256).wait()
    q_unit(5, range(8), False, False,
           chunk2_items(chunk2_items(piece_items(5), 0, (0, 1, 2, 3, 3)), 1, (3, 4, 5, 6, 7)))
    wait_piece(6)
    raw_copy(1, 7, 128).wait()
    raw_copy(2, 2, 256).wait()
    raw_copy(2, 3, 256).wait()
    q_unit(6, range(8), False, False, chunk2_items(piece_items(6), 2, (0, 1, 2, 3, 3, 4, 5, 7)))
    raw_copy(4).start()
    q_unit(7, range(8), False, True, chunk2_items(half_items({}, 1, 7, (0, 1, 2)), 3, (3, 4, 5, 6)))
    raw_copy(5).start()
    for cp in cp_wt:
        cp.start()
    cp_wo.start()
    cp_x.start()
    cp_mem.start()
    cp_bx.start()
    cp_fd.start()
    cp_ms.start()

    def bulk_iter(c, i, n_rl, rl_start):
        xc = jnp.concatenate([_tobf(xc_ref[k]) for k in range(8)], axis=1)
        for t in range(8):
            n = i * 8 + t
            y = _tou(_dot(xc, _tobf(w_refs[c][n, 0:512])).astype(bf16))
            store_qkvc(c * 16 + n, y)
            for blk in range(n_rl):
                pin = y[blk * (256 // n_rl):blk * (256 // n_rl) + 8]
                if c + 1 < 6:
                    w_refs[c + 1][15, pin_rows(512), :] = pin
                    relayout16(c + 1, rl_start + (t * n_rl + blk) * 16)
                else:
                    wo_ref[7, pin_rows(2048), :] = pin
                    repack_wo64(rl_start + (t * n_rl + blk) * 64)
            if c >= 4:
                wp_ref[pin_rows(12832), :] = y[32:40]
                b_prep((c - 4) * 4 + i * 2 + t // 4, (t // 2) % 2, t % 2)

    for c in range(2, 6):
        if c == 4:
            for cp in cp_wt:
                cp.wait()
        if c == 5:
            cp_wo.wait()
        elif c > 2:
            raw_copy(c + 1).wait()

        def bulk(i, carry, c=c):
            if c == 2:
                raw_copy(3, i, 512).wait()
            bulk_iter(c, i, 4, i * (512 if c + 1 < 6 else 2048))
            return carry
        jax.lax.fori_loop(0, 2, bulk, 0)

    cp_x.wait()
    cp_mem.wait()
    cp_bx.wait()
    cp_fd.wait()

    lane0 = jax.lax.broadcasted_iota(jnp.int32, (8, 128), 1) == 0

    def ub_get(n, g):
        return ub_ref[n, g * 16:g * 16 + 8], ub_ref[n, g * 16 + 8:g * 16 + 16]

    def ub_put(n, g, v):
        ub_ref[n, g * 16:g * 16 + 8] = v[0]
        ub_ref[n, g * 16 + 8:g * 16 + 16] = v[1]

    lane4 = jax.lax.broadcasted_iota(jnp.int32, (8, 128), 1) % 4

    def first_lanes(t):
        la, lb = [k for k in range(4) if _FIRST[t][k]]
        return (lane4 == la) | (lane4 == lb)

    def stage(st_ref, t, rows, vals):
        for k in range(3):
            st_ref[3 * t + k, rows] = vals[k]

    def d_products(st_ref, d, t, rows):
        return [_dot(st_ref[3 * t + k, rows].astype(bf16), _tobf(fd_ref[d * 12 + 3 * t + k])) for k in range(3)]

    def twiddles(p):
        return [(tw_ref[(p * 4 + jq) * 2], tw_ref[(p * 4 + jq) * 2 + 1]) for jq in range(4)]

    st_refs = (sa_ref, sb_ref)

    def p1_pre(p, slot, rs, q):
        def item(y):
            st_refs[slot][7, pin_rows(256), :] = y
            rows = pl.multiple_of(q * 512 + p * 64 + rs * 16, 16)
            xq = bx_ref[pl.ds(rows, 16), :].astype(f32)
            zz = _r8_real([xq[:, a * 128:(a + 1) * 128] for a in range(8)])
            for t in range(4):
                for e in range(2):
                    r = ((rs * 2 + e) * 4 + q) * 8
                    a, b = zz[t][0][e * 8:(e + 1) * 8], zz[t][1][e * 8:(e + 1) * 8]
                    stage(st_refs[slot], t, slice(r, r + 8), (a + b, b, a))
        return item

    def p1_mm(p, slot, t):
        def item(y):
            cs = twiddles(p)

            def emit(t, g, u):
                a = _dft4(u)
                for jq in range(4):
                    re, im = a[jq]
                    if jq > 0:
                        c, sn = cs[jq]
                        re, im = re * c + im * sn, im * c - re * sn
                    ub_put((t * 4 + jq) * 8 + p, g, (re, im))

            def emit_real(g, u):
                sr, dr, tr, er = u[0] + u[2], u[0] - u[2], u[1] + u[3], u[1] - u[3]
                a2 = sr - tr
                (_, _), (c1, s1), (c2, s2), (c3, s3) = cs
                ub_put(16 * 8 + p, g, (sr + tr, jnp.zeros_like(sr)))
                ub_put(17 * 8 + p, g, (dr * c1 - er * s1, er * (-c1) - dr * s1))
                ub_put(18 * 8 + p, g, (a2 * c2, a2 * (-s2)))
                ub_put(19 * 8 + p, g, (dr * c3 + er * s3, er * c3 - dr * s3))

            first = first_lanes(t)
            for m in range(4):
                ks = d_products(st_refs[slot], 0, t, slice(m * 64, (m + 1) * 64))
                for e in range(2):
                    u = []
                    for q in range(4):
                        r = (e * 4 + q) * 8
                        k1, k2, k3 = [k[r:r + 8] for k in ks]
                        if t == 0:
                            u.append((jnp.where(first, k3, k2), k1 - jnp.where(first, k2, k3)))
                        else:
                            u.append((k2 + k1, (k3 - k1) * jnp.where(first, 1.0, -1.0)))
                    if t == 0:
                        emit_real(m * 2 + e, [im for (_, im) in u])
                        u = [(re, jnp.where(lane0, 0.0, im)) for (re, im) in u]
                    emit(t, m * 2 + e, u)
        return item

    def p2_bfly(u, g, inverse):
        def item(y):
            if y is not None:
                ub_ref[168, pin_rows(0), :] = y
            x = [ub_get(u * 8 + p, g) for p in range(8)]
            x = _swap(_dft8(_swap(x))) if inverse else _dft8(x)
            for p in range(8):
                ub_put(u * 8 + p, g, x[p])
        return item

    def p2_fwd(u, jps):
        def item(y):
            t = u // 4
            jq = u % 4
            xs = [_dot(_tobf(ms_ref[jq + 4 * jp]), ub_ref[u * 8 + jp].astype(bf16)) for jp in jps]
            for jp, xx in zip(jps, xs):
                w = wp_ref[pl.ds(t * 2560 + jq + 4 * jp, 64, stride=40), :]
                wr = pltpu.bitcast(w & jnp.uint32(0xFFFF0000), f32)
                wi = pltpu.bitcast(w << 16, f32)
                for g in range(8):
                    xr, xi = xx[g * 16:g * 16 + 8], xx[g * 16 + 8:g * 16 + 16]
                    a, b = wr[g * 8:(g + 1) * 8], wi[g * 8:(g + 1) * 8]
                    ub_put(u * 8 + jp, g, (xr * a - xi * b, xr * b + xi * a))
        return item

    def p2_inv(u, jps):
        def item(y):
            jq = u % 4
            zs = [_dot(_tobf(ms_ref[32 + jq + 4 * jp]), ub_ref[u * 8 + jp].astype(bf16)) for jp in jps]
            for jp, zz in zip(jps, zs):
                ub_ref[u * 8 + jp] = zz
        return item

    def p3_pre(p, g, t):
        def item(y):
            sa_ref[7, pin_rows(256), :] = y
            cs = twiddles(p)

            def fetch(t):
                a = []
                for jq in range(4):
                    re, im = ub_get((t * 4 + jq) * 8 + p, g)
                    if jq > 0:
                        c, sn = cs[jq]
                        re, im = re * c - im * sn, im * c + re * sn
                    a.append((re, im))
                return _swap(_dft4(_swap(a)))

            u = fetch(t)
            if t == 0:
                ny = fetch(4)
                u = [(u[q][0], jnp.where(lane0, ny[q][0], u[q][1])) for q in range(4)]
            first = first_lanes(t)
            for q in range(4):
                re, im = u[q]
                if t == 0:
                    vals = (im, jnp.where(first, re, im), jnp.where(first, im, re))
                else:
                    im = im * jnp.where(first, 1.0, -1.0)
                    vals = (re + im, im, re)
                stage(sa_ref, t, slice(q * 64 + g * 8, q * 64 + (g + 1) * 8), vals)
        return item

    def p3_mm(p, q):
        def item(y):
            g = []
            for t in range(4):
                k1, k2, k3 = d_products(sa_ref, 1, t, slice(q * 64, (q + 1) * 64))
                g.append((k2 + k1, k3 + k1 if t == 0 else k3 - k1))
            yy = _r8_real_t(g)
            rows = pl.multiple_of(q * 512 + p * 64, 64)
            for a in range(8):
                bx_ref[pl.ds(rows, 64), a * 128:(a + 1) * 128] = yy[a].astype(bf16)
        return item

    def b_out(p):
        for q in range(4):
            rows = pl.multiple_of(q * 512 + p * 64, 64)
            pltpu.make_async_copy(bx_ref.at[pl.ds(rows, 64), :],
                                  out_hbm.at[pl.ds(rows, 64), pl.ds(DM, DM)], sem_out.at[1]).start()

    def step(pp, odd, mem, hooks):
        r0 = pl.multiple_of(pp * 64 + 32 * odd, SEG)
        xs = xo_ref[pl.ds(r0, SEG), :]
        x_lo = xs[0:8].astype(f32)
        hm = jnp.concatenate(
            [jnp.concatenate([x_lo, jnp.concatenate(mem, axis=1)], axis=0).astype(bf16), xs[16:32]], axis=0)
        fill = fillo_ref[:, 0:64] if odd else fille_ref[:, 0:48]
        nrow = 48 if odd else 32
        qkv, ps = {}, {}

        def do_qkv(g):
            for h in range(g * G, (g + 1) * G):
                for t in range(3):
                    y32 = _dot(hm, _tobf(w_refs[t * 2 + h // 16][h % 16, 0:512]))
                    y = y32.astype(bf16)
                    parts = [y]
                    if odd or t > 0:
                        parts.append(_tobf(qkvc_ref[pp, t * H + h]))
                    if t > 0:
                        if odd:
                            parts.append(_tobf(kve_ref[(t - 1) * H + h]))
                        else:
                            kve_ref[(t - 1) * H + h] = _tou(y[0:16])
                    qkv[(t, h)] = jnp.concatenate(parts, axis=0) if len(parts) > 1 else y
                for item in hooks.get(h, ()):
                    item(y32[0:8])

        def do_s(g):
            for h in range(g * G, (g + 1) * G):
                sc = jax.lax.dot_general(qkv[(0, h)], qkv[(1, h)], (((1,), (1,)), ((), ())),
                                         preferred_element_type=f32)
                sc = jnp.where(fill == 0.0, sc * scale, fill)
                e = jnp.exp(sc - jnp.max(sc, axis=1, keepdims=True))
                den = jnp.sum(e, axis=1, keepdims=True)
                r = pl.reciprocal(den, approx=True)
                r = r * (2.0 - den * r)
                ps[h] = (e * r).astype(bf16)

        def do_pv(g):
            for h in range(g * G, (g + 1) * G):
                oall_ref[h, 0:nrow // 2] = _tou(_dot(ps[h], qkv[(2, h)]).astype(bf16))

        def do_o(j, h0, h1):
            lhs = jnp.concatenate([_tobf(oall_ref[h, 0:nrow // 2]) for h in range(h0, h1)], axis=1)
            return _dot(lhs, _tobf(wo_ref[j, h0 * 64:h1 * 64, :]))

        for g in range(NG):
            do_qkv(g)
            if g >= 1:
                do_s(g - 1)
            if g >= 2:
                do_pv(g - 2)
        part = {}
        for j in range(8):
            items = hooks.get(('o', j), ())
            if len(items) == 1:
                part[j] = do_o(j, 0, OSPLIT)
                items[0](None)
            elif items:
                half = do_o(j, 0, OSPLIT // 2)
                items[0](half[0:8])
                part[j] = do_o(j, OSPLIT // 2, OSPLIT) + half
                items[1](part[j][0:8])
            else:
                part[j] = do_o(j, 0, OSPLIT)
            if j == 2:
                do_s(NG - 1)
                do_pv(NG - 2)
            if j == 5:
                do_pv(NG - 1)
        new_mem = []
        for j in range(8):
            cols = slice(j * 128, (j + 1) * 128)
            res = do_o(j, OSPLIT, H) + part[j]
            new_mem.append(res[8:16])
            if odd:
                xo_ref[pl.ds(r0, SEG), cols] = jnp.concatenate(
                    [res[0:8], res[40:48], res[16:32]], axis=0).astype(bf16)
                xo_ref[pl.ds(r0 - 24, 8), cols] = res[32:40].astype(bf16)
            else:
                xo_ref[pl.ds(r0, SEG), cols] = res.astype(bf16)
        for item in hooks.get(H, ()):
            item(None)
        if odd:
            rows = pl.ds(pl.multiple_of(pp * 64, 64), 64)
            pltpu.make_async_copy(xo_ref.at[rows, :], out_hbm.at[rows, pl.ds(0, DM)], sem_out.at[0]).start()
        return new_mem

    def l1(i, mem):
        he = {h: [p1_pre(2 * i + h // 16, h // 16, (h % 16) // 4, h % 4)] for h in range(32)}
        he[H] = [p1_mm(2 * i, 0, 1)]
        ho = {('o', k): [p1_mm(2 * i + (k + 1) // 4, (k + 1) // 4, t)] for k, t in enumerate((0, 2, 3, 0, 1, 2, 3))}
        mem = step(i, 0, mem, he)
        mem = step(i, 1, mem, ho)
        return mem

    def l2(i, mem):
        u = i - N_L1
        he = {3: [p2_fwd(u, range(0, 4))], 7: [p2_fwd(u, range(4, 8))], H: [p2_inv(u, range(0, 8))]}
        ho = {('o', j): [p2_bfly(u, j, True), p2_bfly(u + 1, j, False)] for j in range(8)}
        mem = step(i, 0, mem, he)
        mem = step(i, 1, mem, ho)
        return mem

    def l3(i, mem):
        p = i - N_L1 - N_L2
        he = {h: [p3_pre(p, h // 4, h % 4)] for h in range(32)}
        he[H] = [p3_mm(p, q) for q in range(4)]
        ho = {12: [lambda y: b_out(p)]}
        mem = step(i, 0, mem, he)
        mem = step(i, 1, mem, ho)
        return mem

    m0 = mem_ref[...].astype(f32)
    mem = [m0[:, j * 128:(j + 1) * 128] for j in range(8)]
    mem = jax.lax.fori_loop(0, N_L1, l1, mem)
    cp_ms.wait()
    for g in range(8):
        p2_bfly(0, g, False)(None)
    mem = jax.lax.fori_loop(N_L1, N_L1 + N_L2, l2, mem)
    mem = jax.lax.fori_loop(N_L1 + N_L2, NSEG // 2, l3, mem)

    pltpu.make_async_copy(xo_ref, out_hbm.at[:, pl.ds(0, DM)], sem_out.at[0]).wait()
    pltpu.make_async_copy(bx_ref, out_hbm.at[:, pl.ds(DM, DM)], sem_out.at[1]).wait()


@jax.jit
def _run(x, mem0, wq, wk, wv, wo, bx, w_r, w_i):
    fd, ms = _tables()
    hbm = pl.BlockSpec(memory_space=pl.ANY)
    out = pl.pallas_call(
        _kernel,
        out_shape=jax.ShapeDtypeStruct((S, 2 * DM), bf16),
        in_specs=[hbm] * 12,
        out_specs=hbm,
        scratch_shapes=[
            pltpu.VMEM((S, DM), bf16),
            pltpu.VMEM((MEM, DM), bf16),
            pltpu.VMEM((8, NSEG, 8, 128), bf16),
            pltpu.VMEM((4, DM, 16, DH), bf16),
        ] + [pltpu.VMEM((16, DM // 2 + 8, DH), u32)] * 6 + [
            pltpu.VMEM((H * DH, DM), bf16),
            pltpu.VMEM((8, H * DH // 2 + 8, 128), u32),
            pltpu.VMEM((8, 256, 128), u32),
            pltpu.VMEM((NSEG // 2, 3 * H, 8, 128), u32),
            pltpu.VMEM((2 * H, 8, 128), u32),
            pltpu.VMEM((H, 24, DH), u32),
            pltpu.VMEM((32, 128), f32),
            pltpu.VMEM((48, 128), f32),
            pltpu.VMEM((S, DM), bf16),
            pltpu.VMEM((16, DM // 2 + 1, 256), bf16),
            pltpu.VMEM((12840, 128), u32),
            pltpu.VMEM((169, 128, 128), f32),
            pltpu.VMEM((12, 264, 128), f32),
            pltpu.VMEM((12, 264, 128), f32),
            pltpu.VMEM((24, 64, 128), u32),
            pltpu.VMEM((64, 64, 128), u32),
            pltpu.SMEM((64,), f32),
            pltpu.SMEM((1,), jnp.int32),
            pltpu.SemaphoreType.DMA((64,)),
            pltpu.SemaphoreType.DMA((2,)),
        ],
        compiler_params=pltpu.CompilerParams(vmem_limit_bytes=120 * 1024 * 1024,
                                             disable_semaphore_checks=True),
    )(x.reshape(S, DM), x.reshape(NSEG, SEG, DM), mem0.reshape(MEM, DM), wq, wk, wv,
      wo.reshape(H * DH, DM), bx.reshape(S, DM), w_r.T, w_i.T, jnp.asarray(fd), jnp.asarray(ms))
    return out.reshape(1, S, 2 * DM)


def pallas_concat_heads__memory_aug_recurrent_mem_tr__spectral_gfnet__prompt_kernel(
    A_x: jax.Array,
    A_mem0: jax.Array,
    A_Wq: jax.Array,
    A_Wk: jax.Array,
    A_Wv: jax.Array,
    A_Wo: jax.Array,
    A_seg_len,
    B_x: jax.Array,
    B_w_r: jax.Array,
    B_w_i: jax.Array,
):
    if isinstance(A_seg_len, int):
        assert A_seg_len == SEG
    assert A_x.shape == (1, S, DM) and A_mem0.shape == (1, MEM, DM) and A_Wq.shape == (DM, H, DH)
    assert B_x.shape == (1, S, DM) and B_w_r.shape == (S, DM // 2 + 1)
    return _run(A_x, A_mem0, A_Wq, A_Wk, A_Wv, A_Wo, B_x, B_w_r, B_w_i)
```

```python
import math

import numpy as np
import jax
import jax.numpy as jnp
import jax.experimental.pallas as pl
import jax.experimental.pallas.tpu as pltpu

bf16 = jnp.bfloat16
f32 = jnp.float32
u32 = jnp.uint32

S, DM = 2048, 1024
H, DH = 32, 128
MEM, SEG = 8, 32
NSEG = S // SEG
SQH = math.sqrt(0.5)

_PAIRS = ((0, 4), (1, 7), (2, 6), (3, 5))
_FIRST = np.array([[1, 1, 0, 0], [1, 0, 1, 0], [0, 1, 1, 0], [0, 1, 0, 1]], bool)


def _pack_rows(a):
    u = np.ascontiguousarray(a, dtype=np.float32).view(np.uint32).astype(np.uint64)
    b = ((u + 0x7FFF + ((u >> 16) & 1)) >> 16).astype(np.uint32)
    return (b[..., 0::2, :] | (b[..., 1::2, :] << 16)).astype(np.uint32)


def _tables():
    k2 = np.zeros((4, 128), np.int64)
    for t in range(4):
        odd = t % 2
        for lam in range(128):
            k = 2 * lam + odd
            if k % 8 not in _PAIRS[t]:
                k = 2 * (128 + 8 * (lam // 8) + (lam % 8 - 1 - odd) % 8) + odd
            assert k % 8 in _PAIRS[t]
            k2[t, lam] = k
    b = np.arange(128)[:, None]
    F = np.zeros((12, 128, 128))
    G = np.zeros((12, 128, 128))
    for t in range(4):
        th = 2 * np.pi * ((b * k2[t][None, :]) % DM) / DM
        C, Sn = np.cos(th), np.sin(th)
        first = ((k2[t] % 8) == _PAIRS[t][0])[None, :]
        assert np.array_equal(first[0], _FIRST[t][np.arange(128) % 4])
        if t == 0:
            im = -Sn
            im[:, 0] = (-1.0) ** np.arange(128)
            F[0:3] = im, np.where(first, im, C), np.where(first, C, im)
            G[0:3] = im, np.where(first, C, -im), np.where(first, -im, C)
            G[0:3, :, 0] *= 0.5
        else:
            Sg = np.where(first, Sn, -Sn)
            F[3 * t:3 * t + 3] = C, -(C + Sg), C - Sg
            G[3 * t:3 * t + 3] = F[3 * t:3 * t + 3]
    Finv = np.transpose(G, (0, 2, 1)) * (2.0 / DM)
    fd = _pack_rows(np.concatenate([F, Finv]))
    M = np.zeros((32, 128, 128))
    r = np.arange(64)[None, :]
    l = np.arange(64)[:, None]
    for j in range(32):
        th = 2 * np.pi * ((r * (j + 32 * l)) % S) / S
        C, Sn = np.cos(th), np.sin(th)
        M[j, :64, :64] = C
        M[j, :64, 64:] = Sn
        M[j, 64:, :64] = -Sn
        M[j, 64:, 64:] = C
    perm = np.arange(128).reshape(2, 8, 8).transpose(1, 0, 2).reshape(128)
    M = M[:, perm][:, :, perm]
    Minv = np.transpose(M, (0, 2, 1)) / S
    ms = _pack_rows(np.concatenate([M, Minv]))
    return fd, ms


def _tobf(w):
    return pltpu.bitcast(w, bf16)


def _tou(w):
    return pltpu.bitcast(w, u32)


def _dot(a, b):
    return jnp.dot(a, b, preferred_element_type=f32)


def _r8_real(x):
    t0, t1 = x[0] + x[4], x[0] - x[4]
    t2, t3 = x[2] + x[6], x[2] - x[6]
    t4, t5 = x[1] + x[5], x[1] - x[5]
    t6, t7 = x[3] + x[7], x[3] - x[7]
    e0, e1 = t0 + t2, t0 - t2
    o0, o1 = t4 + t6, t4 - t6
    u, v = SQH * (t5 - t7), SQH * (t5 + t7)
    return [(e0 + o0, e0 - o0), (t1 + u, v + t3), (e1, o1), (t1 - u, v - t3)]


def _r8_real_t(g):
    (z0, z4), (a1, b1), (e1, o1), (a3, b3) = g
    e0, o0 = z0 + z4, z0 - z4
    t1, u = a1 + a3, a1 - a3
    v, t3 = b1 + b3, b1 - b3
    t5, t7 = SQH * (v + u), SQH * (v - u)
    t0, t2 = e0 + e1, e0 - e1
    t4, t6 = o0 + o1, o0 - o1
    return [t0 + t1, t4 + t5, t2 + t3, t6 + t7, t0 - t1, t4 - t5, t2 - t3, t6 - t7]


def _dft4(u):
    (r0, i0), (r1, i1), (r2, i2), (r3, i3) = u
    sr, si, dr, di = r0 + r2, i0 + i2, r0 - r2, i0 - i2
    tr, ti, er, ei = r1 + r3, i1 + i3, r1 - r3, i1 - i3
    return [(sr + tr, si + ti), (dr + ei, di - er), (sr - tr, si - ti), (dr - ei, di + er)]


def _dft8(x):
    a = [(x[p][0] + x[p + 4][0], x[p][1] + x[p + 4][1]) for p in range(4)]
    d = [(x[p][0] - x[p + 4][0], x[p][1] - x[p + 4][1]) for p in range(4)]
    ev = _dft4(a)
    (r0, i0), (r1, i1), (r2, i2), (r3, i3) = d
    b1r, b1i = SQH * (r1 + i1), SQH * (i1 - r1)
    b3r, n3i = SQH * (i3 - r3), SQH * (r3 + i3)
    sr, si, dr, di = r0 + i2, i0 - r2, r0 - i2, i0 + r2
    tr, ti, er, ei = b1r + b3r, b1i - n3i, b1r - b3r, b1i + n3i
    od = [(sr + tr, si + ti), (dr + ei, di - er), (sr - tr, si - ti), (dr - ei, di + er)]
    return [ev[0], od[0], ev[1], od[1], ev[2], od[2], ev[3], od[3]]


def _swap(x):
    return [(b, a) for (a, b) in x]


G = 4
NG = H // G
OSPLIT = 24
NEG = -1e9
N_L1, N_L2, N_L3 = 4, 20, 8


def _kernel(x_hbm, x3_hbm, mem_hbm, wq_hbm, wk_hbm, wv_hbm, wo_hbm, bx_hbm, wr_hbm, wi_hbm,
            fd_hbm, ms_hbm, out_hbm,
            xo_ref, mem_ref, xcraw_ref, raw_ref, w0_ref, w1_ref, w2_ref, w3_ref, w4_ref, w5_ref,
            woraw_ref, wo_ref, xc_ref, qkvc_ref, kve_ref,
            oall_ref, fille_ref, fillo_ref, bx_ref, wt_ref, wp_ref, ub_ref, sa_ref, sb_ref, fd_ref, ms_ref,
            tw_ref, zero_ref, sem_in, sem_out):
    scale = DH ** -0.5
    w_hbm = (wq_hbm, wk_hbm, wv_hbm)
    w_refs = (w0_ref, w1_ref, w2_ref, w3_ref, w4_ref, w5_ref)

    def raw_copy(c, i=0, nd=DM):
        rows = pl.ds(pl.multiple_of(i * nd, nd), nd)
        return pltpu.make_async_copy(
            w_hbm[c // 2].at[rows, pl.ds((c % 2) * 16, 16), :],
            raw_ref.at[c % 4, rows], sem_in.at[8 + min(c, 3) * 8 + max(c - 3, 0) * 2 + i])

    def xc_copy(k):
        return pltpu.make_async_copy(
            x3_hbm.at[:, pl.ds(8, 8), pl.ds(pl.multiple_of(k * 128, 128), 128)], xcraw_ref.at[k], sem_in.at[40 + k])

    cp_x = pltpu.make_async_copy(x_hbm, xo_ref, sem_in.at[0])
    cp_mem = pltpu.make_async_copy(mem_hbm, mem_ref, sem_in.at[1])
    cp_wo = pltpu.make_async_copy(wo_hbm, woraw_ref, sem_in.at[2])
    cp_bx = pltpu.make_async_copy(bx_hbm, bx_ref, sem_in.at[3])
    cp_fd = pltpu.make_async_copy(fd_hbm, fd_ref, sem_in.at[4])
    cp_ms = pltpu.make_async_copy(ms_hbm, ms_ref, sem_in.at[5])
    cp_wt = [pltpu.make_async_copy(src.at[:, pl.ds(lg * 256, 256)], wt_ref.at[a * 8 + lg], sem_in.at[48 + a * 8 + lg])
             for a, src in enumerate((wr_hbm, wi_hbm)) for lg in range(8)]

    for i in range(8):
        raw_copy(0, i, 128).start()
        xc_copy(i).start()
        raw_copy(1, i, 128).start()
    for i in range(4):
        raw_copy(2, i, 256).start()
    for i in range(2):
        raw_copy(3, i, 512).start()

    zero_ref[0] = 0

    def pin_rows(r):
        return pl.ds(pl.multiple_of(r + zero_ref[0] * 32, 8), 8)

    for p in range(8):
        for jq in range(4):
            tw_ref[(p * 4 + jq) * 2] = jnp.float32(math.cos(2 * math.pi * p * jq / 32))
            tw_ref[(p * 4 + jq) * 2 + 1] = jnp.float32(math.sin(2 * math.pi * p * jq / 32))

    qi = jax.lax.broadcasted_iota(jnp.int32, (48, 128), 0)
    ki = jax.lax.broadcasted_iota(jnp.int32, (48, 128), 1)

    def between(v, lo, hi):
        return (v >= lo) & (v < hi)

    def table(keep, other):
        return jnp.where(other, -jnp.inf, jnp.where(keep, 0.0, NEG)).astype(f32)

    keep = between(qi, 8, 16) | between(ki, 8, 16) | (qi >= jnp.where(ki < 32, ki, ki - 24))
    fille_ref[...] = table(keep, ki >= 40)[:32]
    q_even = between(qi, 32, 40)
    k_even = between(ki, 32, 40) | (ki >= 48)
    qpos = jnp.where(qi < 32, qi, jnp.where(qi < 40, qi - 24, qi - 32))
    kpos = jnp.where(ki < 32, ki, jnp.where(ki < 40, ki - 24, jnp.where(ki < 48, ki - 32, ki - 48)))
    keep = between(qi, 8, 16) | between(ki, 8, 16) | (ki >= 56) | (qpos >= kpos)
    fillo_ref[...] = table(keep, (q_even != k_even) | (ki >= 64))

    def relayout16(c, d0):
        slot = c % 4
        w0 = pl.multiple_of(d0 // 2, 8)
        los, his = [], []
        for dd in range(8):
            a = _tou(raw_ref[slot, d0 + 2 * dd])
            b = _tou(raw_ref[slot, d0 + 2 * dd + 1])
            los.append((a & jnp.uint32(0xFFFF)) | (b << 16))
            his.append((a >> 16) | (b & jnp.uint32(0xFFFF0000)))
        lo = jnp.swapaxes(jnp.stack(los), 0, 1)
        hi = jnp.swapaxes(jnp.stack(his), 0, 1)
        for j in range(8):
            w_refs[c][2 * j, pl.ds(w0, 8), :] = lo[j]
            w_refs[c][2 * j + 1, pl.ds(w0, 8), :] = hi[j]

    def repack_wo64(r_start):
        r0 = pl.multiple_of(r_start, 64)
        w0 = pl.multiple_of(r_start // 2, 32)
        v = woraw_ref[pl.ds(r0, 64), :]
        for j in range(8):
            wo_ref[j, pl.ds(w0, 32), :] = _tou(v[:, j * 128:(j + 1) * 128])

    sub4 = jax.lax.broadcasted_iota(jnp.int32, (128, 128), 0) % 4

    def wp_store(t, kb, tile):
        v = tile.T
        for g in range(4):
            r0 = pl.multiple_of(t * 2560 + kb * 160 + g * 40, 8)
            wp_ref[pl.ds(r0, 32), :] = v[g * 32:(g + 1) * 32]

    def b_prep(lg, hb, par):
        cols = slice(hb * 128, (hb + 1) * 128)
        a = _tou(wt_ref[lg, 0:512, cols])
        b = _tou(wt_ref[8 + lg, 0:512, cols])
        if par == 0:
            w = (a << 16) | (b & jnp.uint32(0xFFFF))
            m = (sub4 == 0) | (sub4 == 2)
        else:
            w = (a & jnp.uint32(0xFFFF0000)) | (b >> 16)
            m = (sub4 == 0) | (sub4 == 3)
        top = w[:128]
        bot = pltpu.roll(w[128:].reshape(16, 8, 128), 1 + par, 1).reshape(128, 128)
        wp_store(par, lg * 2 + hb, jnp.where(m, top, bot))
        wp_store(par + 2, lg * 2 + hb, jnp.where(m, bot, top))
        if par == 0:
            na = jnp.broadcast_to(wt_ref[lg, 512:513, cols].astype(f32), (128, 128))
            nb = jnp.broadcast_to(wt_ref[8 + lg, 512:513, cols].astype(f32), (128, 128))
            wp_store(4, lg * 2 + hb, pltpu.bitcast(na, u32) | (pltpu.bitcast(nb, u32) >> 16))

    def gather_c(k):
        xc_ref[k] = _tou(xcraw_ref[k].astype(f32).reshape(512, 128).astype(bf16))

    def store_qkvc(n, y):
        for pp in range(NSEG // 2):
            qkvc_ref[pp, n] = y[pp * 8:(pp + 1) * 8]

    def q_unit(i, groups, first, last, fillers):
        xk = _tobf(xc_ref[i])
        w0 = pl.multiple_of(i * 64, 64)
        for g in groups:
            rhs = jnp.concatenate(
                [_tobf(w_refs[h // 16][h % 16, pl.ds(w0, 64), :]) for h in range(4 * g, 4 * g + 4)], axis=1)
            y = _dot(xk, rhs)
            for h in range(4 * g, 4 * g + 4):
                yh = y[:, (h % 4) * 128:(h % 4 + 1) * 128]
                if not first:
                    yh = yh + ub_ref[h * 4:(h + 1) * 4].reshape(512, 128)
                if last:
                    store_qkvc(h, _tou(yh.astype(bf16)))
                else:
                    ub_ref[h * 4:(h + 1) * 4] = yh.reshape(4, 128, 128)
            mine = fillers.get(g, [])
            for fi, item in enumerate(mine):
                r = (fi * 512 // len(mine)) // 8 * 8
                item(pltpu.bitcast(y[r:r + 8, 0:128], u32))

    def rl_item(c, d0):
        def item(pin):
            w_refs[c][15, pin_rows(512), :] = pin
            relayout16(c, d0)
        return item

    def spread(fillers, items, groups):
        for k, item in enumerate(items):
            fillers.setdefault(groups[k * len(groups) // len(items)], []).append(item)
        return fillers

    def half_items(f, c, i, groups):
        return spread(f, [rl_item(c, i * 128 + blk * 16) for blk in range(8)], groups)

    def piece_items(i):
        f = half_items(half_items({}, 1, i, (0, 1, 2)), 0, i + 1, (4, 5, 6))
        return spread(f, [lambda pin: gather_c(i + 1)], (6,))

    def chunk2_items(f, i, groups):
        return spread(f, [rl_item(2, i * 256 + blk * 16) for blk in range(16)], groups)

    def wait_piece(i):
        raw_copy(1, i, 128).wait()
        xc_copy(i + 1).wait()
        raw_copy(0, i + 1, 128).wait()

    raw_copy(0, 0, 128).wait()
    for blk in range(8):
        relayout16(0, blk * 16)
    xc_copy(0).wait()
    gather_c(0)
    q_unit(0, range(0, 2), True, False, {})
    raw_copy(1, 0, 128).wait()
    q_unit(0, range(2, 4), True, False, half_items({}, 1, 0, (2, 2, 3)))
    xc_copy(1).wait()
    raw_copy(0, 1, 128).wait()
    q_unit(0, range(4, 8), True, False,
           spread(half_items({}, 0, 1, (4, 5, 6)), [lambda pin: gather_c(1)], (6,)))

    def q_c(i, carry):
        wait_piece(i)
        q_unit(i, range(8), False, False, piece_items(i))
        return carry
    jax.lax.fori_loop(1, 5, q_c, 0)

    wait_piece(5)
    raw_copy(2, 0, 256).wait()
    raw_copy(2, 1, 256).wait()
    q_unit(5, range(8), False, False,
           chunk2_items(chunk2_items(piece_items(5), 0, (0, 1, 2, 3, 3)), 1, (3, 4, 5, 6, 7)))
    wait_piece(6)
    raw_copy(1, 7, 128).wait()
    raw_copy(2, 2, 256).wait()
    raw_copy(2, 3, 256).wait()
    q_unit(6, range(8), False, False, chunk2_items(piece_items(6), 2, (0, 1, 2, 3, 3, 4, 5, 7)))
    raw_copy(4).start()
    q_unit(7, range(8), False, True, chunk2_items(half_items({}, 1, 7, (0, 1, 2)), 3, (3, 4, 5, 6)))
    raw_copy(5).start()
    for cp in cp_wt:
        cp.start()
    cp_wo.start()
    cp_x.start()
    cp_mem.start()
    cp_bx.start()
    cp_fd.start()
    cp_ms.start()

    def bulk_iter(c, i, n_rl, rl_start):
        xc = jnp.concatenate([_tobf(xc_ref[k]) for k in range(8)], axis=1)
        for t in range(8):
            n = i * 8 + t
            y = _tou(_dot(xc, _tobf(w_refs[c][n, 0:512])).astype(bf16))
            store_qkvc(c * 16 + n, y)
            for blk in range(n_rl):
                pin = y[blk * (256 // n_rl):blk * (256 // n_rl) + 8]
                if c + 1 < 6:
                    w_refs[c + 1][15, pin_rows(512), :] = pin
                    relayout16(c + 1, rl_start + (t * n_rl + blk) * 16)
                else:
                    wo_ref[7, pin_rows(2048), :] = pin
                    repack_wo64(rl_start + (t * n_rl + blk) * 64)
            if c >= 4:
                wp_ref[pin_rows(12832), :] = y[32:40]
                b_prep((c - 4) * 4 + i * 2 + t // 4, (t // 2) % 2, t % 2)

    for c in range(2, 6):
        if c == 4:
            for cp in cp_wt:
                cp.wait()
        if c == 5:
            cp_wo.wait()
        elif c > 2:
            raw_copy(c + 1).wait()

        def bulk(i, carry, c=c):
            if c == 2:
                raw_copy(3, i, 512).wait()
            bulk_iter(c, i, 4, i * (512 if c + 1 < 6 else 2048))
            return carry
        jax.lax.fori_loop(0, 2, bulk, 0)

    cp_x.wait()
    cp_mem.wait()
    cp_bx.wait()
    cp_fd.wait()

    lane0 = jax.lax.broadcasted_iota(jnp.int32, (8, 128), 1) == 0

    def ub_get(n, g):
        return ub_ref[n, g * 16:g * 16 + 8], ub_ref[n, g * 16 + 8:g * 16 + 16]

    def ub_put(n, g, v):
        ub_ref[n, g * 16:g * 16 + 8] = v[0]
        ub_ref[n, g * 16 + 8:g * 16 + 16] = v[1]

    lane4 = jax.lax.broadcasted_iota(jnp.int32, (8, 128), 1) % 4

    def first_lanes(t):
        la, lb = [k for k in range(4) if _FIRST[t][k]]
        return (lane4 == la) | (lane4 == lb)

    def stage(st_ref, t, rows, vals):
        for k in range(3):
            st_ref[3 * t + k, rows] = vals[k]

    def d_products(st_ref, d, t, rows):
        return [_dot(st_ref[3 * t + k, rows].astype(bf16), _tobf(fd_ref[d * 12 + 3 * t + k])) for k in range(3)]

    def twiddles(p):
        return [(tw_ref[(p * 4 + jq) * 2], tw_ref[(p * 4 + jq) * 2 + 1]) for jq in range(4)]

    st_refs = (sa_ref, sb_ref)

    def p1_pre(p, slot, rs, q):
        def item(y):
            st_refs[slot][7, pin_rows(256), :] = y
            rows = pl.multiple_of(q * 512 + p * 64 + rs * 16, 16)
            xq = bx_ref[pl.ds(rows, 16), :].astype(f32)
            zz = _r8_real([xq[:, a * 128:(a + 1) * 128] for a in range(8)])
            for t in range(4):
                for e in range(2):
                    r = ((rs * 2 + e) * 4 + q) * 8
                    a, b = zz[t][0][e * 8:(e + 1) * 8], zz[t][1][e * 8:(e + 1) * 8]
                    stage(st_refs[slot], t, slice(r, r + 8), (a + b, b, a))
        return item

    def p1_mm(p, slot, t):
        def item(y):
            cs = twiddles(p)

            def emit(t, g, u):
                a = _dft4(u)
                for jq in range(4):
                    re, im = a[jq]
                    if jq > 0:
                        c, sn = cs[jq]
                        re, im = re * c + im * sn, im * c - re * sn
                    ub_put((t * 4 + jq) * 8 + p, g, (re, im))

            def emit_real(g, u):
                sr, dr, tr, er = u[0] + u[2], u[0] - u[2], u[1] + u[3], u[1] - u[3]
                a2 = sr - tr
                (_, _), (c1, s1), (c2, s2), (c3, s3) = cs
                ub_put(16 * 8 + p, g, (sr + tr, jnp.zeros_like(sr)))
                ub_put(17 * 8 + p, g, (dr * c1 - er * s1, er * (-c1) - dr * s1))
                ub_put(18 * 8 + p, g, (a2 * c2, a2 * (-s2)))
                ub_put(19 * 8 + p, g, (dr * c3 + er * s3, er * c3 - dr * s3))

            first = first_lanes(t)
            for m in range(4):
                ks = d_products(st_refs[slot], 0, t, slice(m * 64, (m + 1) * 64))
                for e in range(2):
                    u = []
                    for q in range(4):
                        r = (e * 4 + q) * 8
                        k1, k2, k3 = [k[r:r + 8] for k in ks]
                        if t == 0:
                            u.append((jnp.where(first, k3, k2), k1 - jnp.where(first, k2, k3)))
                        else:
                            u.append((k2 + k1, (k3 - k1) * jnp.where(first, 1.0, -1.0)))
                    if t == 0:
                        emit_real(m * 2 + e, [im for (_, im) in u])
                        u = [(re, jnp.where(lane0, 0.0, im)) for (re, im) in u]
                    emit(t, m * 2 + e, u)
        return item

    def p2_bfly(u, g, inverse):
        def item(y):
            if y is not None:
                ub_ref[168, pin_rows(0), :] = y
            x = [ub_get(u * 8 + p, g) for p in range(8)]
            x = _swap(_dft8(_swap(x))) if inverse else _dft8(x)
            for p in range(8):
                ub_put(u * 8 + p, g, x[p])
        return item

    def p2_fwd(u, jps):
        def item(y):
            t = u // 4
            jq = u % 4
            xs = [_dot(_tobf(ms_ref[jq + 4 * jp]), ub_ref[u * 8 + jp].astype(bf16)) for jp in jps]
            for jp, xx in zip(jps, xs):
                w = wp_ref[pl.ds(t * 2560 + jq + 4 * jp, 64, stride=40), :]
                wr = pltpu.bitcast(w & jnp.uint32(0xFFFF0000), f32)
                wi = pltpu.bitcast(w << 16, f32)
                for g in range(8):
                    xr, xi = xx[g * 16:g * 16 + 8], xx[g * 16 + 8:g * 16 + 16]
                    a, b = wr[g * 8:(g + 1) * 8], wi[g * 8:(g + 1) * 8]
                    ub_put(u * 8 + jp, g, (xr * a - xi * b, xr * b + xi * a))
        return item

    def p2_inv(u, jps):
        def item(y):
            jq = u % 4
            zs = [_dot(_tobf(ms_ref[32 + jq + 4 * jp]), ub_ref[u * 8 + jp].astype(bf16)) for jp in jps]
            for jp, zz in zip(jps, zs):
                ub_ref[u * 8 + jp] = zz
        return item

    def p3_pre(p, g, t):
        def item(y):
            sa_ref[7, pin_rows(256), :] = y
            cs = twiddles(p)

            def fetch(t):
                a = []
                for jq in range(4):
                    re, im = ub_get((t * 4 + jq) * 8 + p, g)
                    if jq > 0:
                        c, sn = cs[jq]
                        re, im = re * c - im * sn, im * c + re * sn
                    a.append((re, im))
                return _swap(_dft4(_swap(a)))

            u = fetch(t)
            if t == 0:
                ny = fetch(4)
                u = [(u[q][0], jnp.where(lane0, ny[q][0], u[q][1])) for q in range(4)]
            first = first_lanes(t)
            for q in range(4):
                re, im = u[q]
                if t == 0:
                    vals = (im, jnp.where(first, re, im), jnp.where(first, im, re))
                else:
                    im = im * jnp.where(first, 1.0, -1.0)
                    vals = (re + im, im, re)
                stage(sa_ref, t, slice(q * 64 + g * 8, q * 64 + (g + 1) * 8), vals)
        return item

    def p3_mm(p, q):
        def item(y):
            g = []
            for t in range(4):
                k1, k2, k3 = d_products(sa_ref, 1, t, slice(q * 64, (q + 1) * 64))
                g.append((k2 + k1, k3 + k1 if t == 0 else k3 - k1))
            yy = _r8_real_t(g)
            rows = pl.multiple_of(q * 512 + p * 64, 64)
            for a in range(8):
                bx_ref[pl.ds(rows, 64), a * 128:(a + 1) * 128] = yy[a].astype(bf16)
        return item

    def b_out(p):
        for q in range(4):
            rows = pl.multiple_of(q * 512 + p * 64, 64)
            pltpu.make_async_copy(bx_ref.at[pl.ds(rows, 64), :],
                                  out_hbm.at[pl.ds(rows, 64), pl.ds(DM, DM)], sem_out.at[1]).start()

    def step(pp, odd, mem, hooks):
        r0 = pl.multiple_of(pp * 64 + 32 * odd, SEG)
        xs = xo_ref[pl.ds(r0, SEG), :]
        x_lo = xs[0:8].astype(f32)
        hm = jnp.concatenate(
            [jnp.concatenate([x_lo, jnp.concatenate(mem, axis=1)], axis=0).astype(bf16), xs[16:32]], axis=0)
        fill = fillo_ref[:, 0:64] if odd else fille_ref[:, 0:48]
        nrow = 48 if odd else 32
        qkv, ps = {}, {}

        def do_qkv(h0, h1):
            for h in range(h0, h1):
                for t in range(3):
                    y32 = _dot(hm, _tobf(w_refs[t * 2 + h // 16][h % 16, 0:512]))
                    y = y32.astype(bf16)
                    parts = [y]
                    if odd or t > 0:
                        parts.append(_tobf(qkvc_ref[pp, t * H + h]))
                    if t > 0:
                        if odd:
                            parts.append(_tobf(kve_ref[(t - 1) * H + h]))
                        else:
                            kve_ref[(t - 1) * H + h] = _tou(y[0:16])
                    qkv[(t, h)] = jnp.concatenate(parts, axis=0) if len(parts) > 1 else y
                for item in hooks.get(h, ()):
                    item(y32[0:8])

        def do_s(g):
            for h in range(g * G, (g + 1) * G):
                sc = jax.lax.dot_general(qkv[(0, h)], qkv[(1, h)], (((1,), (1,)), ((), ())),
                                         preferred_element_type=f32)
                sc = jnp.where(fill == 0.0, sc * scale, fill)
                e = jnp.exp(sc - jnp.max(sc, axis=1, keepdims=True))
                den = jnp.sum(e, axis=1, keepdims=True)
                r = pl.reciprocal(den, approx=True)
                r = r * (2.0 - den * r)
                ps[h] = (e * r).astype(bf16)

        def do_pv(g):
            for h in range(g * G, (g + 1) * G):
                oall_ref[h, 0:nrow // 2] = _tou(_dot(ps[h], qkv[(2, h)]).astype(bf16))

        def do_o(j, h0, h1):
            lhs = jnp.concatenate([_tobf(oall_ref[h, 0:nrow // 2]) for h in range(h0, h1)], axis=1)
            return _dot(lhs, _tobf(wo_ref[j, h0 * 64:h1 * 64, :]))

        for g in range(NG):
            do_qkv(g * G, g * G + G // 2)
            if g >= 1:
                do_s(g - 1)
            do_qkv(g * G + G // 2, (g + 1) * G)
            if g >= 2:
                do_pv(g - 2)
        part = {}
        for j in range(8):
            items = hooks.get(('o', j), ())
            if len(items) == 1:
                part[j] = do_o(j, 0, OSPLIT)
                items[0](None)
            elif items:
                half = do_o(j, 0, OSPLIT // 2)
                items[0](half[0:8])
                part[j] = do_o(j, OSPLIT // 2, OSPLIT) + half
                items[1](part[j][0:8])
            else:
                part[j] = do_o(j, 0, OSPLIT)
            if j == 2:
                do_s(NG - 1)
                do_pv(NG - 2)
            if j == 5:
                do_pv(NG - 1)
        new_mem = []
        for j in range(8):
            cols = slice(j * 128, (j + 1) * 128)
            res = do_o(j, OSPLIT, H) + part[j]
            new_mem.append(res[8:16])
            if odd:
                xo_ref[pl.ds(r0, SEG), cols] = jnp.concatenate(
                    [res[0:8], res[40:48], res[16:32]], axis=0).astype(bf16)
                xo_ref[pl.ds(r0 - 24, 8), cols] = res[32:40].astype(bf16)
            else:
                xo_ref[pl.ds(r0, SEG), cols] = res.astype(bf16)
        for item in hooks.get(H, ()):
            item(None)
        if odd:
            rows = pl.ds(pl.multiple_of(pp * 64, 64), 64)
            pltpu.make_async_copy(xo_ref.at[rows, :], out_hbm.at[rows, pl.ds(0, DM)], sem_out.at[0]).start()
        return new_mem

    def l1(i, mem):
        he = {h: [p1_pre(2 * i + h // 16, h // 16, (h % 16) // 4, h % 4)] for h in range(32)}
        he[H] = [p1_mm(2 * i, 0, 1)]
        ho = {('o', k): [p1_mm(2 * i + (k + 1) // 4, (k + 1) // 4, t)] for k, t in enumerate((0, 2, 3, 0, 1, 2, 3))}
        mem = step(i, 0, mem, he)
        mem = step(i, 1, mem, ho)
        return mem

    def l2(i, mem):
        u = i - N_L1
        he = {3: [p2_fwd(u, range(0, 4))], 7: [p2_fwd(u, range(4, 8))], H: [p2_inv(u, range(0, 8))]}
        ho = {('o', j): [p2_bfly(u, j, True), p2_bfly(u + 1, j, False)] for j in range(8)}
        mem = step(i, 0, mem, he)
        mem = step(i, 1, mem, ho)
        return mem

    def l3(i, mem):
        p = i - N_L1 - N_L2
        he = {h: [p3_pre(p, h // 4, h % 4)] for h in range(32)}
        he[H] = [p3_mm(p, q) for q in range(4)]
        ho = {12: [lambda y: b_out(p)]}
        mem = step(i, 0, mem, he)
        mem = step(i, 1, mem, ho)
        return mem

    m0 = mem_ref[...].astype(f32)
    mem = [m0[:, j * 128:(j + 1) * 128] for j in range(8)]
    mem = jax.lax.fori_loop(0, N_L1, l1, mem)
    cp_ms.wait()
    for g in range(8):
        p2_bfly(0, g, False)(None)
    mem = jax.lax.fori_loop(N_L1, N_L1 + N_L2, l2, mem)
    mem = jax.lax.fori_loop(N_L1 + N_L2, NSEG // 2, l3, mem)

    pltpu.make_async_copy(xo_ref, out_hbm.at[:, pl.ds(0, DM)], sem_out.at[0]).wait()
    pltpu.make_async_copy(bx_ref, out_hbm.at[:, pl.ds(DM, DM)], sem_out.at[1]).wait()


@jax.jit
def _run(x, mem0, wq, wk, wv, wo, bx, w_r, w_i):
    fd, ms = _tables()
    hbm = pl.BlockSpec(memory_space=pl.ANY)
    out = pl.pallas_call(
        _kernel,
        out_shape=jax.ShapeDtypeStruct((S, 2 * DM), bf16),
        in_specs=[hbm] * 12,
        out_specs=hbm,
        scratch_shapes=[
            pltpu.VMEM((S, DM), bf16),
            pltpu.VMEM((MEM, DM), bf16),
            pltpu.VMEM((8, NSEG, 8, 128), bf16),
            pltpu.VMEM((4, DM, 16, DH), bf16),
        ] + [pltpu.VMEM((16, DM // 2 + 8, DH), u32)] * 6 + [
            pltpu.VMEM((H * DH, DM), bf16),
            pltpu.VMEM((8, H * DH // 2 + 8, 128), u32),
            pltpu.VMEM((8, 256, 128), u32),
            pltpu.VMEM((NSEG // 2, 3 * H, 8, 128), u32),
            pltpu.VMEM((2 * H, 8, 128), u32),
            pltpu.VMEM((H, 24, DH), u32),
            pltpu.VMEM((32, 128), f32),
            pltpu.VMEM((48, 128), f32),
            pltpu.VMEM((S, DM), bf16),
            pltpu.VMEM((16, DM // 2 + 1, 256), bf16),
            pltpu.VMEM((12840, 128), u32),
            pltpu.VMEM((169, 128, 128), f32),
            pltpu.VMEM((12, 264, 128), f32),
            pltpu.VMEM((12, 264, 128), f32),
            pltpu.VMEM((24, 64, 128), u32),
            pltpu.VMEM((64, 64, 128), u32),
            pltpu.SMEM((64,), f32),
            pltpu.SMEM((1,), jnp.int32),
            pltpu.SemaphoreType.DMA((64,)),
            pltpu.SemaphoreType.DMA((2,)),
        ],
        compiler_params=pltpu.CompilerParams(vmem_limit_bytes=120 * 1024 * 1024,
                                             disable_semaphore_checks=True),
    )(x.reshape(S, DM), x.reshape(NSEG, SEG, DM), mem0.reshape(MEM, DM), wq, wk, wv,
      wo.reshape(H * DH, DM), bx.reshape(S, DM), w_r.T, w_i.T, jnp.asarray(fd), jnp.asarray(ms))
    return out.reshape(1, S, 2 * DM)


def pallas_concat_heads__memory_aug_recurrent_mem_tr__spectral_gfnet__prompt_kernel(
    A_x: jax.Array,
    A_mem0: jax.Array,
    A_Wq: jax.Array,
    A_Wk: jax.Array,
    A_Wv: jax.Array,
    A_Wo: jax.Array,
    A_seg_len,
    B_x: jax.Array,
    B_w_r: jax.Array,
    B_w_i: jax.Array,
):
    if isinstance(A_seg_len, int):
        assert A_seg_len == SEG
    assert A_x.shape == (1, S, DM) and A_mem0.shape == (1, MEM, DM) and A_Wq.shape == (DM, H, DH)
    assert B_x.shape == (1, S, DM) and B_w_r.shape == (S, DM // 2 + 1)
    return _run(A_x, A_mem0, A_Wq, A_Wk, A_Wv, A_Wo, B_x, B_w_r, B_w_i)
```

```python
import math

import numpy as np
import jax
import jax.numpy as jnp
import jax.experimental.pallas as pl
import jax.experimental.pallas.tpu as pltpu

bf16 = jnp.bfloat16
f32 = jnp.float32
u32 = jnp.uint32

S, DM = 2048, 1024
H, DH = 32, 128
MEM, SEG = 8, 32
NSEG = S // SEG
SQH = math.sqrt(0.5)

_PAIRS = ((0, 4), (1, 7), (2, 6), (3, 5))
_FIRST = np.array([[1, 1, 0, 0], [1, 0, 1, 0], [0, 1, 1, 0], [0, 1, 0, 1]], bool)


def _pack_rows(a):
    u = np.ascontiguousarray(a, dtype=np.float32).view(np.uint32).astype(np.uint64)
    b = ((u + 0x7FFF + ((u >> 16) & 1)) >> 16).astype(np.uint32)
    return (b[..., 0::2, :] | (b[..., 1::2, :] << 16)).astype(np.uint32)


def _tables():
    k2 = np.zeros((4, 128), np.int64)
    for t in range(4):
        odd = t % 2
        for lam in range(128):
            k = 2 * lam + odd
            if k % 8 not in _PAIRS[t]:
                k = 2 * (128 + 8 * (lam // 8) + (lam % 8 - 1 - odd) % 8) + odd
            assert k % 8 in _PAIRS[t]
            k2[t, lam] = k
    b = np.arange(128)[:, None]
    F = np.zeros((12, 128, 128))
    G = np.zeros((12, 128, 128))
    for t in range(4):
        th = 2 * np.pi * ((b * k2[t][None, :]) % DM) / DM
        C, Sn = np.cos(th), np.sin(th)
        first = ((k2[t] % 8) == _PAIRS[t][0])[None, :]
        assert np.array_equal(first[0], _FIRST[t][np.arange(128) % 4])
        if t == 0:
            im = -Sn
            im[:, 0] = (-1.0) ** np.arange(128)
            F[0:3] = im, np.where(first, im, C), np.where(first, C, im)
            G[0:3] = im, np.where(first, C, -im), np.where(first, -im, C)
            G[0:3, :, 0] *= 0.5
        else:
            Sg = np.where(first, Sn, -Sn)
            F[3 * t:3 * t + 3] = C, -(C + Sg), C - Sg
            G[3 * t:3 * t + 3] = F[3 * t:3 * t + 3]
    Finv = np.transpose(G, (0, 2, 1)) * (2.0 / DM)
    fd = _pack_rows(np.concatenate([F, Finv]))
    M = np.zeros((32, 128, 128))
    r = np.arange(64)[None, :]
    l = np.arange(64)[:, None]
    for j in range(32):
        th = 2 * np.pi * ((r * (j + 32 * l)) % S) / S
        C, Sn = np.cos(th), np.sin(th)
        M[j, :64, :64] = C
        M[j, :64, 64:] = Sn
        M[j, 64:, :64] = -Sn
        M[j, 64:, 64:] = C
    perm = np.arange(128).reshape(2, 8, 8).transpose(1, 0, 2).reshape(128)
    M = M[:, perm][:, :, perm]
    Minv = np.transpose(M, (0, 2, 1)) / S
    ms = _pack_rows(np.concatenate([M, Minv]))
    return fd, ms


def _tobf(w):
    return pltpu.bitcast(w, bf16)


def _tou(w):
    return pltpu.bitcast(w, u32)


def _dot(a, b):
    return jnp.dot(a, b, preferred_element_type=f32)


def _r8_real(x):
    t0, t1 = x[0] + x[4], x[0] - x[4]
    t2, t3 = x[2] + x[6], x[2] - x[6]
    t4, t5 = x[1] + x[5], x[1] - x[5]
    t6, t7 = x[3] + x[7], x[3] - x[7]
    e0, e1 = t0 + t2, t0 - t2
    o0, o1 = t4 + t6, t4 - t6
    u, v = SQH * (t5 - t7), SQH * (t5 + t7)
    return [(e0 + o0, e0 - o0), (t1 + u, v + t3), (e1, o1), (t1 - u, v - t3)]


def _r8_real_t(g):
    (z0, z4), (a1, b1), (e1, o1), (a3, b3) = g
    e0, o0 = z0 + z4, z0 - z4
    t1, u = a1 + a3, a1 - a3
    v, t3 = b1 + b3, b1 - b3
    t5, t7 = SQH * (v + u), SQH * (v - u)
    t0, t2 = e0 + e1, e0 - e1
    t4, t6 = o0 + o1, o0 - o1
    return [t0 + t1, t4 + t5, t2 + t3, t6 + t7, t0 - t1, t4 - t5, t2 - t3, t6 - t7]


def _dft4(u):
    (r0, i0), (r1, i1), (r2, i2), (r3, i3) = u
    sr, si, dr, di = r0 + r2, i0 + i2, r0 - r2, i0 - i2
    tr, ti, er, ei = r1 + r3, i1 + i3, r1 - r3, i1 - i3
    return [(sr + tr, si + ti), (dr + ei, di - er), (sr - tr, si - ti), (dr - ei, di + er)]


def _dft8(x):
    a = [(x[p][0] + x[p + 4][0], x[p][1] + x[p + 4][1]) for p in range(4)]
    d = [(x[p][0] - x[p + 4][0], x[p][1] - x[p + 4][1]) for p in range(4)]
    ev = _dft4(a)
    (r0, i0), (r1, i1), (r2, i2), (r3, i3) = d
    b1r, b1i = SQH * (r1 + i1), SQH * (i1 - r1)
    b3r, n3i = SQH * (i3 - r3), SQH * (r3 + i3)
    sr, si, dr, di = r0 + i2, i0 - r2, r0 - i2, i0 + r2
    tr, ti, er, ei = b1r + b3r, b1i - n3i, b1r - b3r, b1i + n3i
    od = [(sr + tr, si + ti), (dr + ei, di - er), (sr - tr, si - ti), (dr - ei, di + er)]
    return [ev[0], od[0], ev[1], od[1], ev[2], od[2], ev[3], od[3]]


def _swap(x):
    return [(b, a) for (a, b) in x]


G = 4
NG = H // G
OSPLIT = 24
NEG = -1e9
N_L1, N_L2, N_L3 = 4, 20, 8


def _kernel(x_hbm, x3_hbm, mem_hbm, wq_hbm, wk_hbm, wv_hbm, wo_hbm, bx_hbm, wr_hbm, wi_hbm,
            fd_hbm, ms_hbm, out_hbm,
            xo_ref, mem_ref, xcraw_ref, raw_ref, w0_ref, w1_ref, w2_ref, w3_ref, w4_ref, w5_ref,
            woraw_ref, wo_ref, xc_ref, qkvc_ref, kve_ref,
            oall_ref, fille_ref, fillo_ref, bx_ref, wt_ref, wp_ref, ub_ref, sa_ref, sb_ref, fd_ref, ms_ref,
            tw_ref, zero_ref, sem_in, sem_out):
    scale = DH ** -0.5
    w_hbm = (wq_hbm, wk_hbm, wv_hbm)
    w_refs = (w0_ref, w1_ref, w2_ref, w3_ref, w4_ref, w5_ref)

    def raw_copy(c, i=0, nd=DM):
        rows = pl.ds(pl.multiple_of(i * nd, nd), nd)
        return pltpu.make_async_copy(
            w_hbm[c // 2].at[rows, pl.ds((c % 2) * 16, 16), :],
            raw_ref.at[c % 4, rows], sem_in.at[8 + min(c, 3) * 8 + max(c - 3, 0) * 2 + i])

    def xc_copy(k):
        return pltpu.make_async_copy(
            x3_hbm.at[:, pl.ds(8, 8), pl.ds(pl.multiple_of(k * 128, 128), 128)], xcraw_ref.at[k], sem_in.at[40 + k])

    cp_x = pltpu.make_async_copy(x_hbm, xo_ref, sem_in.at[0])
    cp_mem = pltpu.make_async_copy(mem_hbm, mem_ref, sem_in.at[1])
    cp_wo = pltpu.make_async_copy(wo_hbm, woraw_ref, sem_in.at[2])
    cp_bx = pltpu.make_async_copy(bx_hbm, bx_ref, sem_in.at[3])
    cp_fd = pltpu.make_async_copy(fd_hbm, fd_ref, sem_in.at[4])
    cp_ms = pltpu.make_async_copy(ms_hbm, ms_ref, sem_in.at[5])
    cp_wt = [pltpu.make_async_copy(src.at[:, pl.ds(lg * 256, 256)], wt_ref.at[a * 8 + lg], sem_in.at[48 + a * 8 + lg])
             for a, src in enumerate((wr_hbm, wi_hbm)) for lg in range(8)]

    for i in range(8):
        raw_copy(0, i, 128).start()
        xc_copy(i).start()
        raw_copy(1, i, 128).start()
    for i in range(4):
        raw_copy(2, i, 256).start()
    for i in range(2):
        raw_copy(3, i, 512).start()

    zero_ref[0] = 0

    def pin_rows(r):
        return pl.ds(pl.multiple_of(r + zero_ref[0] * 32, 8), 8)

    for p in range(8):
        for jq in range(4):
            tw_ref[(p * 4 + jq) * 2] = jnp.float32(math.cos(2 * math.pi * p * jq / 32))
            tw_ref[(p * 4 + jq) * 2 + 1] = jnp.float32(math.sin(2 * math.pi * p * jq / 32))

    qi = jax.lax.broadcasted_iota(jnp.int32, (48, 128), 0)
    ki = jax.lax.broadcasted_iota(jnp.int32, (48, 128), 1)

    def between(v, lo, hi):
        return (v >= lo) & (v < hi)

    def table(keep, other):
        return jnp.where(other, -jnp.inf, jnp.where(keep, 0.0, NEG)).astype(f32)

    keep = between(qi, 8, 16) | between(ki, 8, 16) | (qi >= jnp.where(ki < 32, ki, ki - 24))
    fille_ref[...] = table(keep, ki >= 40)[:32]
    q_even = between(qi, 32, 40)
    k_even = between(ki, 32, 40) | (ki >= 48)
    qpos = jnp.where(qi < 32, qi, jnp.where(qi < 40, qi - 24, qi - 32))
    kpos = jnp.where(ki < 32, ki, jnp.where(ki < 40, ki - 24, jnp.where(ki < 48, ki - 32, ki - 48)))
    keep = between(qi, 8, 16) | between(ki, 8, 16) | (ki >= 56) | (qpos >= kpos)
    fillo_ref[...] = table(keep, (q_even != k_even) | (ki >= 64))

    def relayout16(c, blk):
        w0 = pl.multiple_of(blk * 8, 8)
        v = _tou(raw_ref[c % 4, pl.ds(blk * 16, 16)]).reshape(8, 2, 8, 128)
        a, b = v[:, 0], v[:, 1]
        w_refs[c][0:8, pl.ds(w0, 8), :] = jnp.swapaxes((a & jnp.uint32(0xFFFF)) | (b << 16), 0, 1)
        w_refs[c][8:16, pl.ds(w0, 8), :] = jnp.swapaxes((a >> 16) | (b & jnp.uint32(0xFFFF0000)), 0, 1)

    def slot_of(h):
        return (h // 16) * 16 + (h % 2) * 8 + (h % 16) // 2

    def repack_wo64(blk):
        v = _tou(woraw_ref[pl.ds(pl.multiple_of(blk * 64, 64), 64), :])
        wo_ref[:, pl.ds(pl.multiple_of(blk * 32, 32), 32), :] = jnp.stack(
            [v[:, j * 128:(j + 1) * 128] for j in range(8)])

    sub4 = jax.lax.broadcasted_iota(jnp.int32, (128, 128), 0) & 3

    def wp_store(t, kb, tile):
        v = tile.T
        for g in range(4):
            r0 = pl.multiple_of(t * 2560 + kb * 160 + g * 40, 8)
            wp_ref[pl.ds(r0, 32), :] = v[g * 32:(g + 1) * 32]

    def b_prep(lg, hb, par):
        cols = slice(hb * 128, (hb + 1) * 128)
        a = _tou(wt_ref[lg, 0:512, cols])
        b = _tou(wt_ref[8 + lg, 0:512, cols])
        if par == 0:
            w = (a << 16) | (b & jnp.uint32(0xFFFF))
            m = (sub4 == 0) | (sub4 == 2)
        else:
            w = (a & jnp.uint32(0xFFFF0000)) | (b >> 16)
            m = (sub4 == 0) | (sub4 == 3)
        top = w[:128]
        bot = pltpu.roll(w[128:].reshape(16, 8, 128), 1 + par, 1).reshape(128, 128)
        wp_store(par, lg * 2 + hb, jnp.where(m, top, bot))
        wp_store(par + 2, lg * 2 + hb, jnp.where(m, bot, top))
        if par == 0:
            na = jnp.broadcast_to(wt_ref[lg, 512:513, cols].astype(f32), (128, 128))
            nb = jnp.broadcast_to(wt_ref[8 + lg, 512:513, cols].astype(f32), (128, 128))
            wp_store(4, lg * 2 + hb, pltpu.bitcast(na, u32) | (pltpu.bitcast(nb, u32) >> 16))

    def gather_c(k):
        xc_ref[k] = _tou(xcraw_ref[k].astype(f32).reshape(512, 128).astype(bf16))

    def store_qkvc(n, y):
        qkvc_ref[:, n] = y.reshape(NSEG // 2, 8, 128)

    def q_unit(i, groups, first, last, fillers):
        xk = _tobf(xc_ref[i])
        w0 = pl.multiple_of(i * 64, 64)
        for g in groups:
            rhs = jnp.concatenate(
                [_tobf(w_refs[h // 16][h % 16, pl.ds(w0, 64), :]) for h in range(4 * g, 4 * g + 4)], axis=1)
            y = _dot(xk, rhs)
            for h in range(4 * g, 4 * g + 4):
                yh = y[:, (h % 4) * 128:(h % 4 + 1) * 128]
                if not first:
                    yh = yh + ub_ref[h * 4:(h + 1) * 4].reshape(512, 128)
                if last:
                    store_qkvc(h, _tou(yh.astype(bf16)))
                else:
                    ub_ref[h * 4:(h + 1) * 4] = yh.reshape(4, 128, 128)
            mine = fillers.get(g, [])
            for fi, item in enumerate(mine):
                r = (fi * 512 // len(mine)) // 8 * 8
                item(pltpu.bitcast(y[r:r + 8, 0:128], u32))

    def rl_item(c, blk):
        def item(pin):
            w_refs[c][15, pin_rows(512), :] = pin
            relayout16(c, blk)
        return item

    def spread(fillers, items, groups):
        for k, item in enumerate(items):
            fillers.setdefault(groups[k * len(groups) // len(items)], []).append(item)
        return fillers

    def half_items(f, c, i, groups):
        return spread(f, [rl_item(c, i * 8 + blk) for blk in range(8)], groups)

    def piece_items(i):
        f = half_items(half_items({}, 1, i, (0, 1, 2)), 0, i + 1, (4, 5, 6))
        return spread(f, [lambda pin: gather_c(i + 1)], (6,))

    def chunk2_items(f, i, groups):
        return spread(f, [rl_item(2, i * 16 + blk) for blk in range(16)], groups)

    def wait_piece(i):
        raw_copy(1, i, 128).wait()
        xc_copy(i + 1).wait()
        raw_copy(0, i + 1, 128).wait()

    raw_copy(0, 0, 128).wait()
    for blk in range(8):
        relayout16(0, blk)
    xc_copy(0).wait()
    gather_c(0)
    q_unit(0, range(0, 2), True, False, {})
    raw_copy(1, 0, 128).wait()
    q_unit(0, range(2, 4), True, False, half_items({}, 1, 0, (2, 2, 3)))
    xc_copy(1).wait()
    raw_copy(0, 1, 128).wait()
    q_unit(0, range(4, 8), True, False,
           spread(half_items({}, 0, 1, (4, 5, 6)), [lambda pin: gather_c(1)], (6,)))

    def q_c(i, carry):
        wait_piece(i)
        q_unit(i, range(8), False, False, piece_items(i))
        return carry
    jax.lax.fori_loop(1, 5, q_c, 0)

    wait_piece(5)
    raw_copy(2, 0, 256).wait()
    raw_copy(2, 1, 256).wait()
    q_unit(5, range(8), False, False,
           chunk2_items(chunk2_items(piece_items(5), 0, (0, 1, 2, 3, 3)), 1, (3, 4, 5, 6, 7)))
    wait_piece(6)
    raw_copy(1, 7, 128).wait()
    raw_copy(2, 2, 256).wait()
    raw_copy(2, 3, 256).wait()
    q_unit(6, range(8), False, False, chunk2_items(piece_items(6), 2, (0, 1, 2, 3, 3, 4, 5, 7)))
    raw_copy(4).start()
    q_unit(7, range(8), False, True, chunk2_items(half_items({}, 1, 7, (0, 1, 2)), 3, (3, 4, 5, 6)))
    raw_copy(5).start()
    for cp in cp_wt:
        cp.start()
    cp_wo.start()
    cp_x.start()
    cp_mem.start()
    cp_bx.start()
    cp_fd.start()
    cp_ms.start()

    def bulk_iter(c, i):
        xc = jnp.concatenate([_tobf(xc_ref[k]) for k in range(8)], axis=1)
        for t in range(8):
            n = i * 8 + t
            y = _tou(_dot(xc, _tobf(w_refs[c][n, 0:512])).astype(bf16))
            store_qkvc(c * 16 + n, y)
            for blk in range(4):
                pin = y[blk * 64:blk * 64 + 8]
                if c + 1 < 6:
                    w_refs[c + 1][15, pin_rows(512), :] = pin
                    relayout16(c + 1, i * 32 + (t * 4 + blk))
                else:
                    wo_ref[7, pin_rows(2048), :] = pin
                    repack_wo64(i * 32 + (t * 4 + blk))
            if c >= 4:
                wp_ref[pin_rows(12832), :] = y[32:40]
                b_prep((c - 4) * 4 + i * 2 + t // 4, (t // 2) % 2, t % 2)

    for c in range(2, 6):
        if c == 4:
            for cp in cp_wt:
                cp.wait()
        if c == 5:
            cp_wo.wait()
        elif c > 2:
            raw_copy(c + 1).wait()

        def bulk(i, carry, c=c):
            if c == 2:
                raw_copy(3, i, 512).wait()
            bulk_iter(c, i)
            return carry
        jax.lax.fori_loop(0, 2, bulk, 0)

    cp_x.wait()
    cp_mem.wait()
    cp_bx.wait()
    cp_fd.wait()

    lane = jax.lax.broadcasted_iota(jnp.int32, (1, 128), 1)
    lane0 = lane == 0

    def first_lanes(t):
        la, lb = [k for k in range(4) if _FIRST[t][k]]
        return ((lane & 3) == la) | ((lane & 3) == lb)

    def d_products(st_ref, d, t, rows):
        return [_dot(st_ref[3 * t + k, rows].astype(bf16), _tobf(fd_ref[d * 12 + 3 * t + k])) for k in range(3)]

    def twiddles(p):
        return [(tw_ref[p * 8 + jq * 2], tw_ref[p * 8 + jq * 2 + 1]) if jq else None for jq in range(4)]

    st_refs = (sa_ref, sb_ref)

    def p1_pre(p, slot, rs, q):
        def item(y):
            st_refs[slot][7, pin_rows(256), :] = y
            rows = pl.multiple_of(p * 64 + (q * 512 + rs * 16), 16)
            xq = bx_ref[pl.ds(rows, 16), :].astype(f32)
            zz = _r8_real([xq[:, a * 128:(a + 1) * 128] for a in range(8)])
            r = (rs * 4 + q) * 16
            st_refs[slot][:, r:r + 16] = jnp.stack([v for (a, b) in zz for v in (a + b, b, a)])
        return item

    def p1_mm(p, slot, t):
        def item(y):
            cs = twiddles(p)

            def put(n, rs, re, im):
                v = jnp.stack([re.reshape(2, 8, 128), im.reshape(2, 8, 128)], axis=1)
                ub_ref[n * 8 + p, rs * 32:(rs + 1) * 32] = v.reshape(32, 128)

            first = first_lanes(t)
            for rs in range(4):
                k1, k2, k3 = d_products(st_refs[slot], 0, t, slice(rs * 64, (rs + 1) * 64))
                if t == 0:
                    re, im = jnp.where(first, k3, k2), k1 - jnp.where(first, k2, k3)
                    u = [im[q * 16:(q + 1) * 16] for q in range(4)]
                    sr, dr, tr, er = u[0] + u[2], u[0] - u[2], u[1] + u[3], u[1] - u[3]
                    a2 = sr - tr
                    _, (c1, s1), (c2, s2), (c3, s3) = cs
                    put(16, rs, sr + tr, jnp.zeros_like(sr))
                    put(17, rs, dr * c1 - er * s1, er * (-c1) - dr * s1)
                    put(18, rs, a2 * c2, a2 * (-s2))
                    put(19, rs, dr * c3 + er * s3, er * c3 - dr * s3)
                    im = jnp.where(lane0, 0.0, im)
                else:
                    re, im = k1 + k2, (k3 - k1) * jnp.where(first, 1.0, -1.0)
                a = _dft4([(re[q * 16:(q + 1) * 16], im[q * 16:(q + 1) * 16]) for q in range(4)])
                for jq in range(4):
                    re, im = a[jq]
                    if jq > 0:
                        c, sn = cs[jq]
                        re, im = re * c + im * sn, im * c - re * sn
                    put(t * 4 + jq, rs, re, im)
        return item

    def p2_bfly(u, g, inverse):
        def item(y):
            if y is not None:
                ub_ref[168, pin_rows(0), :] = y
            v = ub_ref[pl.ds(u * 8, 8), g * 16:(g + 1) * 16]
            x = [(v[p, 0:8], v[p, 8:16]) for p in range(8)]
            x = _swap(_dft8(_swap(x))) if inverse else _dft8(x)
            ub_ref[pl.ds(u * 8, 8), g * 16:(g + 1) * 16] = jnp.stack([w for c in x for w in c]).reshape(8, 16, 128)
        return item

    def p2_fwd(u, jps):
        def item(y):
            t = u >> 2
            jq = u & 3
            xs = [_dot(_tobf(ms_ref[jq + 4 * jp]), ub_ref[u * 8 + jp].astype(bf16)) for jp in jps]
            for jp, xx in zip(jps, xs):
                w = wp_ref[pl.ds(t * 2560 + jq + 4 * jp, 64, stride=40), :]
                wr = pltpu.bitcast(w & jnp.uint32(0xFFFF0000), f32).reshape(8, 8, 128)
                wi = pltpu.bitcast(w << 16, f32).reshape(8, 8, 128)
                xx = xx.reshape(8, 2, 8, 128)
                xr, xi = xx[:, 0], xx[:, 1]
                ub_ref[u * 8 + jp] = jnp.stack([xr * wr - xi * wi, xr * wi + xi * wr], axis=1).reshape(128, 128)
        return item

    def p2_inv(u, jps):
        def item(y):
            jq = u & 3
            zs = [_dot(_tobf(ms_ref[32 + jq + 4 * jp]), ub_ref[u * 8 + jp].astype(bf16)) for jp in jps]
            for jp, zz in zip(jps, zs):
                ub_ref[u * 8 + jp] = zz
        return item

    def p3_pre(p, g, t):
        def item(y):
            sa_ref[7, pin_rows(256), :] = y
            cs = twiddles(p)

            def fetch(t):
                a = []
                for jq in range(4):
                    v = ub_ref[(t * 4 + jq) * 8 + p, g * 16:(g + 1) * 16]
                    re, im = v[0:8], v[8:16]
                    if jq > 0:
                        c, sn = cs[jq]
                        re, im = re * c - im * sn, im * c + re * sn
                    a.append((re, im))
                return _swap(_dft4(_swap(a)))

            u = fetch(t)
            if t == 0:
                ny = fetch(4)
                u = [(u[q][0], jnp.where(lane0, ny[q][0], u[q][1])) for q in range(4)]
            first = first_lanes(t)
            for q in range(4):
                re, im = u[q]
                if t == 0:
                    vals = (im, jnp.where(first, re, im), jnp.where(first, im, re))
                else:
                    im = im * jnp.where(first, 1.0, -1.0)
                    vals = (re + im, im, re)
                sa_ref[3 * t:3 * t + 3, q * 64 + g * 8:q * 64 + (g + 1) * 8] = jnp.stack(vals)
        return item

    def p3_mm(p, q):
        def item(y):
            g = []
            for t in range(4):
                k1, k2, k3 = d_products(sa_ref, 1, t, slice(q * 64, (q + 1) * 64))
                g.append((k2 + k1, k3 + k1 if t == 0 else k3 - k1))
            yy = _r8_real_t(g)
            rows = pl.multiple_of(q * 512 + p * 64, 64)
            bx_ref[pl.ds(rows, 64), :] = jnp.concatenate(yy, axis=1).astype(bf16)
        return item

    def b_out(p):
        for q in range(4):
            rows = pl.multiple_of(q * 512 + p * 64, 64)
            pltpu.make_async_copy(bx_ref.at[pl.ds(rows, 64), :],
                                  out_hbm.at[pl.ds(rows, 64), pl.ds(DM, DM)], sem_out.at[1]).start()

    def step(pp, odd, mem, hooks):
        r0 = pl.multiple_of(pp * 64 + 32 * odd, SEG)
        xs = xo_ref[pl.ds(r0, SEG), :]
        x_lo = xs[0:8].astype(f32)
        hm = jnp.concatenate(
            [jnp.concatenate([x_lo, jnp.concatenate(mem, axis=1)], axis=0).astype(bf16), xs[16:32]], axis=0)
        fill = fillo_ref[:, 0:64] if odd else fille_ref[:, 0:48]
        nrow = 48 if odd else 32
        qkv, ps = {}, {}

        def do_qkv(h0, h1):
            for h in range(h0, h1):
                for t in range(3):
                    n = t * H + slot_of(h)
                    y32 = _dot(hm, _tobf(w_refs[n // 16][n % 16, 0:512]))
                    y = y32.astype(bf16)
                    parts = [y]
                    if odd or t > 0:
                        parts.append(_tobf(qkvc_ref[pp, n]))
                    if t > 0:
                        if odd:
                            parts.append(_tobf(kve_ref[(t - 1) * H + h]))
                        else:
                            kve_ref[(t - 1) * H + h] = _tou(y[0:16])
                    qkv[(t, h)] = jnp.concatenate(parts, axis=0) if len(parts) > 1 else y
                for item in hooks.get(h, ()):
                    item(y32[0:8])

        def do_s(g):
            for h in range(g * G, (g + 1) * G):
                sc = jax.lax.dot_general(qkv[(0, h)], qkv[(1, h)], (((1,), (1,)), ((), ())),
                                         preferred_element_type=f32)
                sc = jnp.where(fill == 0.0, sc * scale, fill)
                e = jnp.exp(sc - jnp.max(sc, axis=1, keepdims=True))
                den = jnp.sum(e, axis=1, keepdims=True)
                r = pl.reciprocal(den, approx=True)
                r = r * (2.0 - den * r)
                ps[h] = (e * r).astype(bf16)

        def do_pv(g):
            for h in range(g * G, (g + 1) * G):
                oall_ref[0:nrow // 2, h * DH:(h + 1) * DH] = _tou(_dot(ps[h], qkv[(2, h)]).astype(bf16))

        def do_o(j, h0, h1):
            return _dot(_tobf(oall_ref[0:nrow // 2, h0 * DH:h1 * DH]), _tobf(wo_ref[j, h0 * 64:h1 * 64, :]))

        for g in range(NG):
            do_qkv(g * G, g * G + G // 2)
            if g >= 1:
                do_s(g - 1)
            do_qkv(g * G + G // 2, (g + 1) * G)
            if g >= 2:
                do_pv(g - 2)
        part = {}
        for j in range(8):
            items = hooks.get(('o', j), ())
            if len(items) == 1:
                part[j] = do_o(j, 0, OSPLIT)
                items[0](None)
            elif items:
                half = do_o(j, 0, OSPLIT // 2)
                items[0](half[0:8])
                part[j] = do_o(j, OSPLIT // 2, OSPLIT) + half
                items[1](part[j][0:8])
            else:
                part[j] = do_o(j, 0, OSPLIT)
            if j == 2:
                do_s(NG - 1)
                do_pv(NG - 2)
            if j == 5:
                do_pv(NG - 1)
        new_mem = []
        for j in range(8):
            cols = slice(j * 128, (j + 1) * 128)
            res = do_o(j, OSPLIT, H) + part[j]
            new_mem.append(res[8:16])
            if odd:
                xo_ref[pl.ds(r0, SEG), cols] = jnp.concatenate(
                    [res[0:8], res[40:48], res[16:32]], axis=0).astype(bf16)
                xo_ref[pl.ds(r0 - 24, 8), cols] = res[32:40].astype(bf16)
            else:
                xo_ref[pl.ds(r0, SEG), cols] = res.astype(bf16)
        for item in hooks.get(H, ()):
            item(None)
        if odd:
            rows = pl.ds(pl.multiple_of(pp * 64, 64), 64)
            pltpu.make_async_copy(xo_ref.at[rows, :], out_hbm.at[rows, pl.ds(0, DM)], sem_out.at[0]).start()
        return new_mem

    def l1(i, mem):
        he = {h: [p1_pre(2 * i + h // 16, h // 16, (h % 16) // 4, h % 4)] for h in range(32)}
        he[H] = [p1_mm(2 * i, 0, 1)]
        ho = {('o', k): [p1_mm(2 * i + (k + 1) // 4, (k + 1) // 4, t)] for k, t in enumerate((0, 2, 3, 0, 1, 2, 3))}
        mem = step(i, 0, mem, he)
        mem = step(i, 1, mem, ho)
        return mem

    def l2(i, mem):
        u = i - N_L1
        he = {3: [p2_fwd(u, range(0, 4))], 7: [p2_fwd(u, range(4, 8))], H: [p2_inv(u, range(0, 8))]}
        ho = {('o', j): [p2_bfly(u, j, True), p2_bfly(u + 1, j, False)] for j in range(8)}
        mem = step(i, 0, mem, he)
        mem = step(i, 1, mem, ho)
        return mem

    def l3(i, mem):
        p = i - N_L1 - N_L2
        he = {h: [p3_pre(p, h // 4, h % 4)] for h in range(32)}
        he[H] = [p3_mm(p, q) for q in range(4)]
        ho = {12: [lambda y: b_out(p)]}
        mem = step(i, 0, mem, he)
        mem = step(i, 1, mem, ho)
        return mem

    m0 = mem_ref[...].astype(f32)
    mem = [m0[:, j * 128:(j + 1) * 128] for j in range(8)]
    mem = jax.lax.fori_loop(0, N_L1, l1, mem)
    cp_ms.wait()
    for g in range(8):
        p2_bfly(0, g, False)(None)
    mem = jax.lax.fori_loop(N_L1, N_L1 + N_L2, l2, mem)
    mem = jax.lax.fori_loop(N_L1 + N_L2, NSEG // 2, l3, mem)

    pltpu.make_async_copy(xo_ref, out_hbm.at[:, pl.ds(0, DM)], sem_out.at[0]).wait()
    pltpu.make_async_copy(bx_ref, out_hbm.at[:, pl.ds(DM, DM)], sem_out.at[1]).wait()


@jax.jit
def _run(x, mem0, wq, wk, wv, wo, bx, w_r, w_i):
    fd, ms = _tables()
    hbm = pl.BlockSpec(memory_space=pl.ANY)
    out = pl.pallas_call(
        _kernel,
        out_shape=jax.ShapeDtypeStruct((S, 2 * DM), bf16),
        in_specs=[hbm] * 12,
        out_specs=hbm,
        scratch_shapes=[
            pltpu.VMEM((S, DM), bf16),
            pltpu.VMEM((MEM, DM), bf16),
            pltpu.VMEM((8, NSEG, 8, 128), bf16),
            pltpu.VMEM((4, DM, 16, DH), bf16),
        ] + [pltpu.VMEM((16, DM // 2 + 8, DH), u32)] * 6 + [
            pltpu.VMEM((H * DH, DM), bf16),
            pltpu.VMEM((8, H * DH // 2 + 8, 128), u32),
            pltpu.VMEM((8, 256, 128), u32),
            pltpu.VMEM((NSEG // 2, 3 * H, 8, 128), u32),
            pltpu.VMEM((2 * H, 8, 128), u32),
            pltpu.VMEM((24, H * DH), u32),
            pltpu.VMEM((32, 128), f32),
            pltpu.VMEM((48, 128), f32),
            pltpu.VMEM((S, DM), bf16),
            pltpu.VMEM((16, DM // 2 + 1, 256), bf16),
            pltpu.VMEM((12840, 128), u32),
            pltpu.VMEM((169, 128, 128), f32),
            pltpu.VMEM((12, 264, 128), f32),
            pltpu.VMEM((12, 264, 128), f32),
            pltpu.VMEM((24, 64, 128), u32),
            pltpu.VMEM((64, 64, 128), u32),
            pltpu.SMEM((64,), f32),
            pltpu.SMEM((1,), jnp.int32),
            pltpu.SemaphoreType.DMA((64,)),
            pltpu.SemaphoreType.DMA((2,)),
        ],
        compiler_params=pltpu.CompilerParams(vmem_limit_bytes=120 * 1024 * 1024,
                                             disable_semaphore_checks=True),
    )(x.reshape(S, DM), x.reshape(NSEG, SEG, DM), mem0.reshape(MEM, DM), wq, wk, wv,
      wo.reshape(H * DH, DM), bx.reshape(S, DM), w_r.T, w_i.T, jnp.asarray(fd), jnp.asarray(ms))
    return out.reshape(1, S, 2 * DM)


def pallas_concat_heads__memory_aug_recurrent_mem_tr__spectral_gfnet__prompt_kernel(
    A_x: jax.Array,
    A_mem0: jax.Array,
    A_Wq: jax.Array,
    A_Wk: jax.Array,
    A_Wv: jax.Array,
    A_Wo: jax.Array,
    A_seg_len,
    B_x: jax.Array,
    B_w_r: jax.Array,
    B_w_i: jax.Array,
):
    if isinstance(A_seg_len, int):
        assert A_seg_len == SEG
    assert A_x.shape == (1, S, DM) and A_mem0.shape == (1, MEM, DM) and A_Wq.shape == (DM, H, DH)
    assert B_x.shape == (1, S, DM) and B_w_r.shape == (S, DM // 2 + 1)
    return _run(A_x, A_mem0, A_Wq, A_Wk, A_Wv, A_Wo, B_x, B_w_r, B_w_i)
```

```python
import math

import numpy as np
import jax
import jax.numpy as jnp
import jax.experimental.pallas as pl
import jax.experimental.pallas.tpu as pltpu

bf16 = jnp.bfloat16
f32 = jnp.float32
u32 = jnp.uint32

S, DM = 2048, 1024
H, DH = 32, 128
MEM, SEG = 8, 32
NSEG = S // SEG
SQH = math.sqrt(0.5)

_PAIRS = ((0, 4), (1, 7), (2, 6), (3, 5))
_FIRST = np.array([[1, 1, 0, 0], [1, 0, 1, 0], [0, 1, 1, 0], [0, 1, 0, 1]], bool)


def _pack_rows(a):
    u = np.ascontiguousarray(a, dtype=np.float32).view(np.uint32).astype(np.uint64)
    b = ((u + 0x7FFF + ((u >> 16) & 1)) >> 16).astype(np.uint32)
    return (b[..., 0::2, :] | (b[..., 1::2, :] << 16)).astype(np.uint32)


def _tables():
    k2 = np.zeros((4, 128), np.int64)
    for t in range(4):
        odd = t % 2
        for lam in range(128):
            k = 2 * lam + odd
            if k % 8 not in _PAIRS[t]:
                k = 2 * (128 + 8 * (lam // 8) + (lam % 8 - 1 - odd) % 8) + odd
            assert k % 8 in _PAIRS[t]
            k2[t, lam] = k
    b = np.arange(128)[:, None]
    F = np.zeros((12, 128, 128))
    G = np.zeros((12, 128, 128))
    for t in range(4):
        th = 2 * np.pi * ((b * k2[t][None, :]) % DM) / DM
        C, Sn = np.cos(th), np.sin(th)
        first = ((k2[t] % 8) == _PAIRS[t][0])[None, :]
        assert np.array_equal(first[0], _FIRST[t][np.arange(128) % 4])
        if t == 0:
            im = -Sn
            im[:, 0] = (-1.0) ** np.arange(128)
            F[0:3] = im, np.where(first, im, C), np.where(first, C, im)
            G[0:3] = im, np.where(first, C, -im), np.where(first, -im, C)
            G[0:3, :, 0] *= 0.5
        else:
            Sg = np.where(first, Sn, -Sn)
            F[3 * t:3 * t + 3] = C, -(C + Sg), C - Sg
            G[3 * t:3 * t + 3] = F[3 * t:3 * t + 3]
    Finv = np.transpose(G, (0, 2, 1)) * (2.0 / DM)
    fd = _pack_rows(np.concatenate([F, Finv]))
    M = np.zeros((32, 128, 128))
    r = np.arange(64)[None, :]
    l = np.arange(64)[:, None]
    for j in range(32):
        th = 2 * np.pi * ((r * (j + 32 * l)) % S) / S
        C, Sn = np.cos(th), np.sin(th)
        M[j, :64, :64] = C
        M[j, :64, 64:] = Sn
        M[j, 64:, :64] = -Sn
        M[j, 64:, 64:] = C
    perm = np.arange(128).reshape(2, 8, 8).transpose(1, 0, 2).reshape(128)
    M = M[:, perm][:, :, perm]
    Minv = np.transpose(M, (0, 2, 1)) / S
    ms = _pack_rows(np.concatenate([M, Minv]))
    return fd, ms


def _tobf(w):
    return pltpu.bitcast(w, bf16)


def _tou(w):
    return pltpu.bitcast(w, u32)


def _dot(a, b):
    return jnp.dot(a, b, preferred_element_type=f32)


def _r8_real(x):
    t0, t1 = x[0] + x[4], x[0] - x[4]
    t2, t3 = x[2] + x[6], x[2] - x[6]
    t4, t5 = x[1] + x[5], x[1] - x[5]
    t6, t7 = x[3] + x[7], x[3] - x[7]
    e0, e1 = t0 + t2, t0 - t2
    o0, o1 = t4 + t6, t4 - t6
    u, v = SQH * (t5 - t7), SQH * (t5 + t7)
    return [(e0 + o0, e0 - o0), (t1 + u, v + t3), (e1, o1), (t1 - u, v - t3)]


def _r8_real_t(g):
    (z0, z4), (a1, b1), (e1, o1), (a3, b3) = g
    e0, o0 = z0 + z4, z0 - z4
    t1, u = a1 + a3, a1 - a3
    v, t3 = b1 + b3, b1 - b3
    t5, t7 = SQH * (v + u), SQH * (v - u)
    t0, t2 = e0 + e1, e0 - e1
    t4, t6 = o0 + o1, o0 - o1
    return [t0 + t1, t4 + t5, t2 + t3, t6 + t7, t0 - t1, t4 - t5, t2 - t3, t6 - t7]


def _dft4(u):
    (r0, i0), (r1, i1), (r2, i2), (r3, i3) = u
    sr, si, dr, di = r0 + r2, i0 + i2, r0 - r2, i0 - i2
    tr, ti, er, ei = r1 + r3, i1 + i3, r1 - r3, i1 - i3
    return [(sr + tr, si + ti), (dr + ei, di - er), (sr - tr, si - ti), (dr - ei, di + er)]


def _dft8(x):
    a = [(x[p][0] + x[p + 4][0], x[p][1] + x[p + 4][1]) for p in range(4)]
    d = [(x[p][0] - x[p + 4][0], x[p][1] - x[p + 4][1]) for p in range(4)]
    ev = _dft4(a)
    (r0, i0), (r1, i1), (r2, i2), (r3, i3) = d
    b1r, b1i = SQH * (r1 + i1), SQH * (i1 - r1)
    b3r, n3i = SQH * (i3 - r3), SQH * (r3 + i3)
    sr, si, dr, di = r0 + i2, i0 - r2, r0 - i2, i0 + r2
    tr, ti, er, ei = b1r + b3r, b1i - n3i, b1r - b3r, b1i + n3i
    od = [(sr + tr, si + ti), (dr + ei, di - er), (sr - tr, si - ti), (dr - ei, di + er)]
    return [ev[0], od[0], ev[1], od[1], ev[2], od[2], ev[3], od[3]]


def _swap(x):
    return [(b, a) for (a, b) in x]


G = 4
NG = H // G
OSPLIT = 24
NEG = -1e9
N_L1, N_L2, N_L3 = 4, 20, 8


def _kernel(x_hbm, x3_hbm, mem_hbm, wq_hbm, wk_hbm, wv_hbm, wo_hbm, bx_hbm, wr_hbm, wi_hbm,
            fd_hbm, ms_hbm, out_hbm,
            xo_ref, mem_ref, xcraw_ref, raw_ref, w0_ref, w1_ref, w2_ref, w3_ref, w4_ref, w5_ref,
            woraw_ref, wo_ref, xc_ref, qkvc_ref, kve_ref,
            oall_ref, fille_ref, fillo_ref, bx_ref, wt_ref, wp_ref, ub_ref, sa_ref, sb_ref, fd_ref, ms_ref,
            tw_ref, zero_ref, sem_in, sem_out):
    scale = DH ** -0.5
    w_hbm = (wq_hbm, wk_hbm, wv_hbm)
    w_refs = (w0_ref, w1_ref, w2_ref, w3_ref, w4_ref, w5_ref)

    def raw_copy(c, i=0, nd=DM):
        rows = pl.ds(pl.multiple_of(i * nd, nd), nd)
        return pltpu.make_async_copy(
            w_hbm[c // 2].at[rows, pl.ds((c % 2) * 16, 16), :],
            raw_ref.at[c % 4, rows], sem_in.at[8 + min(c, 3) * 8 + max(c - 3, 0) * 2 + i])

    def xc_copy(k):
        return pltpu.make_async_copy(
            x3_hbm.at[:, pl.ds(8, 8), pl.ds(pl.multiple_of(k * 128, 128), 128)], xcraw_ref.at[k], sem_in.at[40 + k])

    cp_x = pltpu.make_async_copy(x_hbm, xo_ref, sem_in.at[0])
    cp_mem = pltpu.make_async_copy(mem_hbm, mem_ref, sem_in.at[1])
    cp_wo = pltpu.make_async_copy(wo_hbm, woraw_ref, sem_in.at[2])
    cp_bx = pltpu.make_async_copy(bx_hbm, bx_ref.at[0:4], sem_in.at[3])
    cp_fd = pltpu.make_async_copy(fd_hbm, fd_ref, sem_in.at[4])
    cp_ms = pltpu.make_async_copy(ms_hbm, ms_ref, sem_in.at[5])
    cp_wt = [pltpu.make_async_copy(src.at[:, pl.ds(lg * 256, 256)], wt_ref.at[a * 8 + lg], sem_in.at[48 + a * 8 + lg])
             for a, src in enumerate((wr_hbm, wi_hbm)) for lg in range(8)]

    for i in range(8):
        raw_copy(0, i, 128).start()
        xc_copy(i).start()
        raw_copy(1, i, 128).start()
    for i in range(4):
        raw_copy(2, i, 256).start()
    for i in range(2):
        raw_copy(3, i, 512).start()

    zero_ref[0] = 0

    def pin_rows(r):
        return pl.ds(pl.multiple_of(r + zero_ref[0] * 32, 8), 8)

    for p in range(8):
        for jq in range(4):
            tw_ref[(p * 4 + jq) * 2] = jnp.float32(math.cos(2 * math.pi * p * jq / 32))
            tw_ref[(p * 4 + jq) * 2 + 1] = jnp.float32(math.sin(2 * math.pi * p * jq / 32))

    qi = jax.lax.broadcasted_iota(jnp.int32, (48, 128), 0)
    ki = jax.lax.broadcasted_iota(jnp.int32, (48, 128), 1)

    def between(v, lo, hi):
        return (v >= lo) & (v < hi)

    def table(keep, other):
        return jnp.where(other, -jnp.inf, jnp.where(keep, 0.0, NEG)).astype(f32)

    keep = between(qi, 8, 16) | between(ki, 8, 16) | (qi >= jnp.where(ki < 32, ki, ki - 24))
    fille_ref[...] = table(keep, ki >= 40)[:32]
    q_even = between(qi, 32, 40)
    k_even = between(ki, 32, 40) | (ki >= 48)
    qpos = jnp.where(qi < 32, qi, jnp.where(qi < 40, qi - 24, qi - 32))
    kpos = jnp.where(ki < 32, ki, jnp.where(ki < 40, ki - 24, jnp.where(ki < 48, ki - 32, ki - 48)))
    keep = between(qi, 8, 16) | between(ki, 8, 16) | (ki >= 56) | (qpos >= kpos)
    fillo_ref[...] = table(keep, (q_even != k_even) | (ki >= 64))

    def relayout16(c, blk):
        w0 = pl.multiple_of(blk * 8, 8)
        v = _tou(raw_ref[c % 4, pl.ds(blk * 16, 16)]).reshape(8, 2, 8, 128)
        a, b = v[:, 0], v[:, 1]
        w_refs[c][0:8, pl.ds(w0, 8), :] = jnp.swapaxes((a & jnp.uint32(0xFFFF)) | (b << 16), 0, 1)
        w_refs[c][8:16, pl.ds(w0, 8), :] = jnp.swapaxes((a >> 16) | (b & jnp.uint32(0xFFFF0000)), 0, 1)

    def slot_of(h):
        return (h // 16) * 16 + (h % 2) * 8 + (h % 16) // 2

    def repack_wo64(blk):
        v = _tou(woraw_ref[pl.ds(pl.multiple_of(blk * 64, 64), 64), :])
        wo_ref[:, pl.ds(pl.multiple_of(blk * 32, 32), 32), :] = jnp.stack(
            [v[:, j * 128:(j + 1) * 128] for j in range(8)])

    sub4 = jax.lax.broadcasted_iota(jnp.int32, (128, 128), 0) & 3

    def wp_store(t, kb, tile):
        v = tile.T
        for g in range(4):
            r0 = pl.multiple_of(t * 2560 + kb * 160 + g * 40, 8)
            wp_ref[pl.ds(r0, 32), :] = v[g * 32:(g + 1) * 32]

    def b_prep(lg, hb, par):
        cols = slice(hb * 128, (hb + 1) * 128)
        a = _tou(wt_ref[lg, 0:512, cols])
        b = _tou(wt_ref[8 + lg, 0:512, cols])
        if par == 0:
            w = (a << 16) | (b & jnp.uint32(0xFFFF))
            m = (sub4 == 0) | (sub4 == 2)
        else:
            w = (a & jnp.uint32(0xFFFF0000)) | (b >> 16)
            m = (sub4 == 0) | (sub4 == 3)
        top = w[:128]
        bot = pltpu.roll(w[128:].reshape(16, 8, 128), 1 + par, 1).reshape(128, 128)
        wp_store(par, lg * 2 + hb, jnp.where(m, top, bot))
        wp_store(par + 2, lg * 2 + hb, jnp.where(m, bot, top))
        if par == 0:
            na = jnp.broadcast_to(wt_ref[lg, 512:513, cols].astype(f32), (128, 128))
            nb = jnp.broadcast_to(wt_ref[8 + lg, 512:513, cols].astype(f32), (128, 128))
            wp_store(4, lg * 2 + hb, pltpu.bitcast(na, u32) | (pltpu.bitcast(nb, u32) >> 16))

    def gather_c(k):
        xc_ref[k] = _tou(xcraw_ref[k].astype(f32).reshape(512, 128).astype(bf16))

    def store_qkvc(n, y):
        qkvc_ref[:, n] = y.reshape(NSEG // 2, 8, 128)

    def q_unit(i, groups, first, last, fillers):
        xk = _tobf(xc_ref[i])
        w0 = pl.multiple_of(i * 64, 64)
        for g in groups:
            rhs = jnp.concatenate(
                [_tobf(w_refs[h // 16][h % 16, pl.ds(w0, 64), :]) for h in range(4 * g, 4 * g + 4)], axis=1)
            y = _dot(xk, rhs)
            for h in range(4 * g, 4 * g + 4):
                yh = y[:, (h % 4) * 128:(h % 4 + 1) * 128]
                if not first:
                    yh = yh + ub_ref[h * 4:(h + 1) * 4].reshape(512, 128)
                if last:
                    store_qkvc(h, _tou(yh.astype(bf16)))
                else:
                    ub_ref[h * 4:(h + 1) * 4] = yh.reshape(4, 128, 128)
            mine = fillers.get(g, [])
            for fi, item in enumerate(mine):
                r = (fi * 512 // len(mine)) // 8 * 8
                item(pltpu.bitcast(y[r:r + 8, 0:128], u32))

    def rl_item(c, blk):
        def item(pin):
            w_refs[c][15, pin_rows(512), :] = pin
            relayout16(c, blk)
        return item

    def spread(fillers, items, groups):
        for k, item in enumerate(items):
            fillers.setdefault(groups[k * len(groups) // len(items)], []).append(item)
        return fillers

    def half_items(f, c, i, groups):
        return spread(f, [rl_item(c, i * 8 + blk) for blk in range(8)], groups)

    def piece_items(i):
        f = half_items(half_items({}, 1, i, (0, 1, 2)), 0, i + 1, (4, 5, 6))
        return spread(f, [lambda pin: gather_c(i + 1)], (6,))

    def chunk2_items(f, i, groups):
        return spread(f, [rl_item(2, i * 16 + blk) for blk in range(16)], groups)

    def wait_piece(i):
        raw_copy(1, i, 128).wait()
        xc_copy(i + 1).wait()
        raw_copy(0, i + 1, 128).wait()

    raw_copy(0, 0, 128).wait()
    for blk in range(8):
        relayout16(0, blk)
    xc_copy(0).wait()
    gather_c(0)
    q_unit(0, range(0, 2), True, False, {})
    raw_copy(1, 0, 128).wait()
    q_unit(0, range(2, 4), True, False, half_items({}, 1, 0, (2, 2, 3)))
    xc_copy(1).wait()
    raw_copy(0, 1, 128).wait()
    q_unit(0, range(4, 8), True, False,
           spread(half_items({}, 0, 1, (4, 5, 6)), [lambda pin: gather_c(1)], (6,)))

    def q_c(i, carry):
        wait_piece(i)
        q_unit(i, range(8), False, False, piece_items(i))
        return carry
    jax.lax.fori_loop(1, 5, q_c, 0)

    wait_piece(5)
    raw_copy(2, 0, 256).wait()
    raw_copy(2, 1, 256).wait()
    q_unit(5, range(8), False, False,
           chunk2_items(chunk2_items(piece_items(5), 0, (0, 1, 2, 3, 3)), 1, (3, 4, 5, 6, 7)))
    wait_piece(6)
    raw_copy(1, 7, 128).wait()
    raw_copy(2, 2, 256).wait()
    raw_copy(2, 3, 256).wait()
    q_unit(6, range(8), False, False, chunk2_items(piece_items(6), 2, (0, 1, 2, 3, 3, 4, 5, 7)))
    raw_copy(4).start()
    q_unit(7, range(8), False, True, chunk2_items(half_items({}, 1, 7, (0, 1, 2)), 3, (3, 4, 5, 6)))
    raw_copy(5).start()
    for cp in cp_wt:
        cp.start()
    cp_wo.start()
    cp_x.start()
    cp_mem.start()
    cp_bx.start()
    cp_fd.start()
    cp_ms.start()

    def bulk_iter(c, i):
        xc = jnp.concatenate([_tobf(xc_ref[k]) for k in range(8)], axis=1)
        for t in range(8):
            n = i * 8 + t
            y = _tou(_dot(xc, _tobf(w_refs[c][n, 0:512])).astype(bf16))
            store_qkvc(c * 16 + n, y)
            for blk in range(4):
                pin = y[blk * 64:blk * 64 + 8]
                if c + 1 < 6:
                    w_refs[c + 1][15, pin_rows(512), :] = pin
                    relayout16(c + 1, i * 32 + (t * 4 + blk))
                else:
                    wo_ref[7, pin_rows(2048), :] = pin
                    repack_wo64(i * 32 + (t * 4 + blk))
            if c >= 4:
                wp_ref[pin_rows(12832), :] = y[32:40]
                b_prep((c - 4) * 4 + i * 2 + t // 4, (t // 2) % 2, t % 2)

    for c in range(2, 6):
        if c == 4:
            for cp in cp_wt:
                cp.wait()
        if c == 5:
            cp_wo.wait()
        elif c > 2:
            raw_copy(c + 1).wait()

        def bulk(i, carry, c=c):
            if c == 2:
                raw_copy(3, i, 512).wait()
            bulk_iter(c, i)
            return carry
        jax.lax.fori_loop(0, 2, bulk, 0)

    cp_x.wait()
    cp_mem.wait()
    cp_bx.wait()
    cp_fd.wait()

    lane = jax.lax.broadcasted_iota(jnp.int32, (1, 128), 1)
    lane0 = lane == 0

    def first_lanes(t):
        la, lb = [k for k in range(4) if _FIRST[t][k]]
        return ((lane & 3) == la) | ((lane & 3) == lb)

    def d_products(st_ref, d, t, rows):
        return [_dot(st_ref[3 * t + k, rows].astype(bf16), _tobf(fd_ref[d * 12 + 3 * t + k])) for k in range(3)]

    def twiddles(p):
        return [(tw_ref[p * 8 + jq * 2], tw_ref[p * 8 + jq * 2 + 1]) if jq else None for jq in range(4)]

    st_refs = (sa_ref, sb_ref)

    def p1_pre(p, slot, rs, q):
        def item(y):
            st_refs[slot][7, pin_rows(256), :] = y
            xq = bx_ref[q, pl.ds(pl.multiple_of(p * 64 + rs * 16, 16), 16), :].astype(f32)
            zz = _r8_real([xq[:, a * 128:(a + 1) * 128] for a in range(8)])
            r = (rs * 4 + q) * 16
            st_refs[slot][:, r:r + 16] = jnp.stack([v for (a, b) in zz for v in (a + b, b, a)])
        return item

    def p1_mm(p, slot, t):
        def item(y):
            cs = twiddles(p)

            def put(n, rs, re, im):
                v = jnp.stack([re.reshape(2, 8, 128), im.reshape(2, 8, 128)], axis=1)
                ub_ref[n * 8 + p, rs * 32:(rs + 1) * 32] = v.reshape(32, 128)

            first = first_lanes(t)
            for rs in range(4):
                k1, k2, k3 = d_products(st_refs[slot], 0, t, slice(rs * 64, (rs + 1) * 64))
                if t == 0:
                    re, im = jnp.where(first, k3, k2), k1 - jnp.where(first, k2, k3)
                    u = [im[q * 16:(q + 1) * 16] for q in range(4)]
                    sr, dr, tr, er = u[0] + u[2], u[0] - u[2], u[1] + u[3], u[1] - u[3]
                    a2 = sr - tr
                    _, (c1, s1), (c2, s2), (c3, s3) = cs
                    put(16, rs, sr + tr, jnp.zeros_like(sr))
                    put(17, rs, dr * c1 - er * s1, er * (-c1) - dr * s1)
                    put(18, rs, a2 * c2, a2 * (-s2))
                    put(19, rs, dr * c3 + er * s3, er * c3 - dr * s3)
                    im = jnp.where(lane0, 0.0, im)
                else:
                    re, im = k1 + k2, (k3 - k1) * jnp.where(first, 1.0, -1.0)
                a = _dft4([(re[q * 16:(q + 1) * 16], im[q * 16:(q + 1) * 16]) for q in range(4)])
                for jq in range(4):
                    re, im = a[jq]
                    if jq > 0:
                        c, sn = cs[jq]
                        re, im = re * c + im * sn, im * c - re * sn
                    put(t * 4 + jq, rs, re, im)
        return item

    def p2_bfly(u, g, inverse):
        def item(y):
            if y is not None:
                ub_ref[168, pin_rows(0), :] = y
            v = ub_ref[pl.ds(u * 8, 8), g * 16:(g + 1) * 16]
            x = [(v[p, 0:8], v[p, 8:16]) for p in range(8)]
            x = _swap(_dft8(_swap(x))) if inverse else _dft8(x)
            ub_ref[pl.ds(u * 8, 8), g * 16:(g + 1) * 16] = jnp.stack([w for c in x for w in c]).reshape(8, 16, 128)
        return item

    def p2_fwd(u, jps):
        def item(y):
            t = u >> 2
            jq = u & 3
            xs = [_dot(_tobf(ms_ref[jq + 4 * jp]), ub_ref[u * 8 + jp].astype(bf16)) for jp in jps]
            for jp, xx in zip(jps, xs):
                w = wp_ref[pl.ds(t * 2560 + jq + 4 * jp, 64, stride=40), :]
                wr = pltpu.bitcast(w & jnp.uint32(0xFFFF0000), f32).reshape(8, 8, 128)
                wi = pltpu.bitcast(w << 16, f32).reshape(8, 8, 128)
                xx = xx.reshape(8, 2, 8, 128)
                xr, xi = xx[:, 0], xx[:, 1]
                ub_ref[u * 8 + jp] = jnp.stack([xr * wr - xi * wi, xr * wi + xi * wr], axis=1).reshape(128, 128)
        return item

    def p2_inv(u, jps):
        def item(y):
            jq = u & 3
            zs = [_dot(_tobf(ms_ref[32 + jq + 4 * jp]), ub_ref[u * 8 + jp].astype(bf16)) for jp in jps]
            for jp, zz in zip(jps, zs):
                ub_ref[u * 8 + jp] = zz
        return item

    def p3_pre(p, g, t):
        def item(y):
            sa_ref[7, pin_rows(256), :] = y
            cs = twiddles(p)

            def fetch(t):
                a = []
                for jq in range(4):
                    v = ub_ref[(t * 4 + jq) * 8 + p, g * 16:(g + 1) * 16]
                    re, im = v[0:8], v[8:16]
                    if jq > 0:
                        c, sn = cs[jq]
                        re, im = re * c - im * sn, im * c + re * sn
                    a.append((re, im))
                return _swap(_dft4(_swap(a)))

            u = fetch(t)
            if t == 0:
                ny = fetch(4)
                u = [(u[q][0], jnp.where(lane0, ny[q][0], u[q][1])) for q in range(4)]
            first = first_lanes(t)
            for q in range(4):
                re, im = u[q]
                if t == 0:
                    vals = (im, jnp.where(first, re, im), jnp.where(first, im, re))
                else:
                    im = im * jnp.where(first, 1.0, -1.0)
                    vals = (re + im, im, re)
                sa_ref[3 * t:3 * t + 3, q * 64 + g * 8:q * 64 + (g + 1) * 8] = jnp.stack(vals)
        return item

    def p3_mm(p, q):
        def item(y):
            g = []
            for t in range(4):
                k1, k2, k3 = d_products(sa_ref, 1, t, slice(q * 64, (q + 1) * 64))
                g.append((k2 + k1, k3 + k1 if t == 0 else k3 - k1))
            yy = _r8_real_t(g)
            bx_ref[q, pl.ds(pl.multiple_of(p * 64, 64), 64), :] = jnp.concatenate(yy, axis=1).astype(bf16)
        return item

    def b_out(p):
        def item(y):
            rows = pl.ds(pl.multiple_of(p * 64, 64), 64)
            pltpu.make_async_copy(bx_ref.at[0:4, rows, :], out_hbm.at[:, rows, pl.ds(DM, DM)],
                                  sem_out.at[1]).start()
            bx_ref[4, pin_rows(0), 0:128] = y.astype(bf16)
        return item

    def step(pp, odd, mem, hooks):
        r0 = pl.multiple_of(pp * 64 + 32 * odd, SEG)
        xs = xo_ref[pl.ds(r0, SEG), :]
        x_lo = xs[0:8].astype(f32)
        hm = jnp.concatenate(
            [jnp.concatenate([x_lo, jnp.concatenate(mem, axis=1)], axis=0).astype(bf16), xs[16:32]], axis=0)
        fill = fillo_ref[:, 0:64] if odd else fille_ref[:, 0:48]
        nrow = 48 if odd else 32
        qkv, ps = {}, {}

        def do_qkv(h0, h1):
            for h in range(h0, h1):
                for t in range(3):
                    n = t * H + slot_of(h)
                    y32 = _dot(hm, _tobf(w_refs[n // 16][n % 16, 0:512]))
                    y = y32.astype(bf16)
                    parts = [y]
                    if odd or t > 0:
                        parts.append(_tobf(qkvc_ref[pp, n]))
                    if t > 0:
                        if odd:
                            parts.append(_tobf(kve_ref[(t - 1) * H + h]))
                        else:
                            kve_ref[(t - 1) * H + h] = _tou(y[0:16])
                    qkv[(t, h)] = jnp.concatenate(parts, axis=0) if len(parts) > 1 else y
                for item in hooks.get(h, ()):
                    item(y32[0:8])

        def do_s(g):
            for h in range(g * G, (g + 1) * G):
                sc = jax.lax.dot_general(qkv[(0, h)], qkv[(1, h)], (((1,), (1,)), ((), ())),
                                         preferred_element_type=f32)
                sc = jnp.where(fill == 0.0, sc * scale, fill)
                e = jnp.exp(sc - jnp.max(sc, axis=1, keepdims=True))
                den = jnp.sum(e, axis=1, keepdims=True)
                r = pl.reciprocal(den, approx=True)
                r = r * (2.0 - den * r)
                ps[h] = (e * r).astype(bf16)

        def do_pv(g):
            for h in range(g * G, (g + 1) * G):
                oall_ref[0:nrow // 2, h * DH:(h + 1) * DH] = _tou(_dot(ps[h], qkv[(2, h)]).astype(bf16))

        def do_o(j, h0, h1):
            return _dot(_tobf(oall_ref[0:nrow // 2, h0 * DH:h1 * DH]), _tobf(wo_ref[j, h0 * 64:h1 * 64, :]))

        for g in range(NG):
            do_qkv(g * G, g * G + G // 2)
            if g >= 1:
                do_s(g - 1)
            do_qkv(g * G + G // 2, (g + 1) * G)
            if g >= 2:
                do_pv(g - 2)
        part = {}
        for j in range(8):
            items = hooks.get(('o', j), ())
            if len(items) == 1:
                part[j] = do_o(j, 0, OSPLIT)
                items[0](None)
            elif items:
                half = do_o(j, 0, OSPLIT // 2)
                items[0](half[0:8])
                part[j] = do_o(j, OSPLIT // 2, OSPLIT) + half
                items[1](part[j][0:8])
            else:
                part[j] = do_o(j, 0, OSPLIT)
            if j == 2:
                do_s(NG - 1)
                do_pv(NG - 2)
            if j == 5:
                do_pv(NG - 1)
        new_mem = []
        for j in range(8):
            cols = slice(j * 128, (j + 1) * 128)
            res = do_o(j, OSPLIT, H) + part[j]
            new_mem.append(res[8:16])
            if odd:
                xo_ref[pl.ds(r0, SEG), cols] = jnp.concatenate(
                    [res[0:8], res[40:48], res[16:32]], axis=0).astype(bf16)
                xo_ref[pl.ds(r0 - 24, 8), cols] = res[32:40].astype(bf16)
            else:
                xo_ref[pl.ds(r0, SEG), cols] = res.astype(bf16)
        for item in hooks.get(H, ()):
            item(None)
        if odd:
            pltpu.make_async_copy(
                xo_ref.at[pl.ds(pl.multiple_of(pp * 64, 64), 64), :],
                out_hbm.at[pp >> 3, pl.ds(pl.multiple_of((pp & 7) * 64, 64), 64), pl.ds(0, DM)],
                sem_out.at[0]).start()
        return new_mem

    def l1(i, mem):
        he = {h: [p1_pre(2 * i + h // 16, h // 16, (h % 16) // 4, h % 4)] for h in range(32)}
        he[H] = [p1_mm(2 * i, 0, 1)]
        ho = {('o', k): [p1_mm(2 * i + (k + 1) // 4, (k + 1) // 4, t)] for k, t in enumerate((0, 2, 3, 0, 1, 2, 3))}
        mem = step(i, 0, mem, he)
        mem = step(i, 1, mem, ho)
        return mem

    def l2(i, mem):
        u = i - N_L1
        he = {3: [p2_fwd(u, range(0, 4))], 7: [p2_fwd(u, range(4, 8))], H: [p2_inv(u, range(0, 8))]}
        ho = {('o', j): [p2_bfly(u, j, True), p2_bfly(u + 1, j, False)] for j in range(8)}
        mem = step(i, 0, mem, he)
        mem = step(i, 1, mem, ho)
        return mem

    def l3(i, mem):
        p = i - N_L1 - N_L2
        he = {h: [p3_pre(p, h // 4, h % 4)] for h in range(32)}
        he[H] = [p3_mm(p, q) for q in range(4)]
        ho = {12: [b_out(p)]}
        mem = step(i, 0, mem, he)
        mem = step(i, 1, mem, ho)
        return mem

    m0 = mem_ref[...].astype(f32)
    mem = [m0[:, j * 128:(j + 1) * 128] for j in range(8)]
    mem = jax.lax.fori_loop(0, N_L1, l1, mem)
    cp_ms.wait()
    for g in range(8):
        p2_bfly(0, g, False)(None)
    mem = jax.lax.fori_loop(N_L1, N_L1 + N_L2, l2, mem)
    mem = jax.lax.fori_loop(N_L1 + N_L2, NSEG // 2, l3, mem)

    pltpu.make_async_copy(bx_ref.at[0:4], out_hbm.at[:, :, pl.ds(DM, DM)], sem_out.at[1]).wait()
    pltpu.make_async_copy(xo_ref, xo_ref, sem_out.at[0]).wait()


@jax.jit
def _run(x, mem0, wq, wk, wv, wo, bx, w_r, w_i):
    fd, ms = _tables()
    hbm = pl.BlockSpec(memory_space=pl.ANY)
    out = pl.pallas_call(
        _kernel,
        out_shape=jax.ShapeDtypeStruct((4, S // 4, 2 * DM), bf16),
        in_specs=[hbm] * 12,
        out_specs=hbm,
        scratch_shapes=[
            pltpu.VMEM((S, DM), bf16),
            pltpu.VMEM((MEM, DM), bf16),
            pltpu.VMEM((8, NSEG, 8, 128), bf16),
            pltpu.VMEM((4, DM, 16, DH), bf16),
        ] + [pltpu.VMEM((16, DM // 2 + 8, DH), u32)] * 6 + [
            pltpu.VMEM((H * DH, DM), bf16),
            pltpu.VMEM((8, H * DH // 2 + 8, 128), u32),
            pltpu.VMEM((8, 256, 128), u32),
            pltpu.VMEM((NSEG // 2, 3 * H, 8, 128), u32),
            pltpu.VMEM((2 * H, 8, 128), u32),
            pltpu.VMEM((24, H * DH), u32),
            pltpu.VMEM((32, 128), f32),
            pltpu.VMEM((48, 128), f32),
            pltpu.VMEM((5, S // 4, DM), bf16),
            pltpu.VMEM((16, DM // 2 + 1, 256), bf16),
            pltpu.VMEM((12840, 128), u32),
            pltpu.VMEM((169, 128, 128), f32),
            pltpu.VMEM((12, 264, 128), f32),
            pltpu.VMEM((12, 264, 128), f32),
            pltpu.VMEM((24, 64, 128), u32),
            pltpu.VMEM((64, 64, 128), u32),
            pltpu.SMEM((64,), f32),
            pltpu.SMEM((1,), jnp.int32),
            pltpu.SemaphoreType.DMA((64,)),
            pltpu.SemaphoreType.DMA((2,)),
        ],
        compiler_params=pltpu.CompilerParams(vmem_limit_bytes=120 * 1024 * 1024,
                                             disable_semaphore_checks=True,
                                             disable_bounds_checks=True),
    )(x.reshape(S, DM), x.reshape(NSEG, SEG, DM), mem0.reshape(MEM, DM), wq, wk, wv,
      wo.reshape(H * DH, DM), bx.reshape(4, S // 4, DM), w_r.T, w_i.T, jnp.asarray(fd), jnp.asarray(ms))
    return out.reshape(1, S, 2 * DM)


def pallas_concat_heads__memory_aug_recurrent_mem_tr__spectral_gfnet__prompt_kernel(
    A_x: jax.Array,
    A_mem0: jax.Array,
    A_Wq: jax.Array,
    A_Wk: jax.Array,
    A_Wv: jax.Array,
    A_Wo: jax.Array,
    A_seg_len,
    B_x: jax.Array,
    B_w_r: jax.Array,
    B_w_i: jax.Array,
):
    if isinstance(A_seg_len, int):
        assert A_seg_len == SEG
    assert A_x.shape == (1, S, DM) and A_mem0.shape == (1, MEM, DM) and A_Wq.shape == (DM, H, DH)
    assert B_x.shape == (1, S, DM) and B_w_r.shape == (S, DM // 2 + 1)
    return _run(A_x, A_mem0, A_Wq, A_Wk, A_Wv, A_Wo, B_x, B_w_r, B_w_i)
```

```python
import math

import numpy as np
import jax
import jax.numpy as jnp
import jax.experimental.pallas as pl
import jax.experimental.pallas.tpu as pltpu

bf16 = jnp.bfloat16
f32 = jnp.float32
u32 = jnp.uint32

S, DM = 2048, 1024
H, DH = 32, 128
MEM, SEG = 8, 32
NSEG = S // SEG
SQH = math.sqrt(0.5)

_PAIRS = ((0, 4), (1, 7), (2, 6), (3, 5))
_FIRST = np.array([[1, 1, 0, 0], [1, 0, 1, 0], [0, 1, 1, 0], [0, 1, 0, 1]], bool)


def _pack_rows(a):
    u = np.ascontiguousarray(a, dtype=np.float32).view(np.uint32).astype(np.uint64)
    b = ((u + 0x7FFF + ((u >> 16) & 1)) >> 16).astype(np.uint32)
    return (b[..., 0::2, :] | (b[..., 1::2, :] << 16)).astype(np.uint32)


def _tables():
    k2 = np.zeros((4, 128), np.int64)
    for t in range(4):
        odd = t % 2
        for lam in range(128):
            k = 2 * lam + odd
            if k % 8 not in _PAIRS[t]:
                k = 2 * (128 + 8 * (lam // 8) + (lam % 8 - 1 - odd) % 8) + odd
            assert k % 8 in _PAIRS[t]
            k2[t, lam] = k
    b = np.arange(128)[:, None]
    F = np.zeros((12, 128, 128))
    G = np.zeros((12, 128, 128))
    for t in range(4):
        th = 2 * np.pi * ((b * k2[t][None, :]) % DM) / DM
        C, Sn = np.cos(th), np.sin(th)
        first = ((k2[t] % 8) == _PAIRS[t][0])[None, :]
        assert np.array_equal(first[0], _FIRST[t][np.arange(128) % 4])
        if t == 0:
            im = -Sn
            im[:, 0] = (-1.0) ** np.arange(128)
            F[0:3] = im, np.where(first, im, C), np.where(first, C, im)
            G[0:3] = im, np.where(first, C, -im), np.where(first, -im, C)
            G[0:3, :, 0] *= 0.5
        else:
            Sg = np.where(first, Sn, -Sn)
            F[3 * t:3 * t + 3] = C, -(C + Sg), C - Sg
            G[3 * t:3 * t + 3] = F[3 * t:3 * t + 3]
    Finv = np.transpose(G, (0, 2, 1)) * (2.0 / DM)
    fd = _pack_rows(np.concatenate([F, Finv]))
    M = np.zeros((32, 128, 128))
    r = np.arange(64)[None, :]
    l = np.arange(64)[:, None]
    for j in range(32):
        th = 2 * np.pi * ((r * (j + 32 * l)) % S) / S
        C, Sn = np.cos(th), np.sin(th)
        M[j, :64, :64] = C
        M[j, :64, 64:] = Sn
        M[j, 64:, :64] = -Sn
        M[j, 64:, 64:] = C
    perm = np.arange(128).reshape(2, 8, 8).transpose(1, 0, 2).reshape(128)
    M = M[:, perm][:, :, perm]
    Minv = np.transpose(M, (0, 2, 1)) / S
    ms = _pack_rows(np.concatenate([M, Minv]))
    return fd, ms


def _tobf(w):
    return pltpu.bitcast(w, bf16)


def _tou(w):
    return pltpu.bitcast(w, u32)


def _dot(a, b):
    return jnp.dot(a, b, preferred_element_type=f32)


def _r8_real(x):
    t0, t1 = x[0] + x[4], x[0] - x[4]
    t2, t3 = x[2] + x[6], x[2] - x[6]
    t4, t5 = x[1] + x[5], x[1] - x[5]
    t6, t7 = x[3] + x[7], x[3] - x[7]
    e0, e1 = t0 + t2, t0 - t2
    o0, o1 = t4 + t6, t4 - t6
    u, v = SQH * (t5 - t7), SQH * (t5 + t7)
    return [(e0 + o0, e0 - o0), (t1 + u, v + t3), (e1, o1), (t1 - u, v - t3)]


def _r8_real_t(g):
    (z0, z4), (a1, b1), (e1, o1), (a3, b3) = g
    e0, o0 = z0 + z4, z0 - z4
    t1, u = a1 + a3, a1 - a3
    v, t3 = b1 + b3, b1 - b3
    t5, t7 = SQH * (v + u), SQH * (v - u)
    t0, t2 = e0 + e1, e0 - e1
    t4, t6 = o0 + o1, o0 - o1
    return [t0 + t1, t4 + t5, t2 + t3, t6 + t7, t0 - t1, t4 - t5, t2 - t3, t6 - t7]


def _dft4(u):
    (r0, i0), (r1, i1), (r2, i2), (r3, i3) = u
    sr, si, dr, di = r0 + r2, i0 + i2, r0 - r2, i0 - i2
    tr, ti, er, ei = r1 + r3, i1 + i3, r1 - r3, i1 - i3
    return [(sr + tr, si + ti), (dr + ei, di - er), (sr - tr, si - ti), (dr - ei, di + er)]


def _dft8(x):
    a = [(x[p][0] + x[p + 4][0], x[p][1] + x[p + 4][1]) for p in range(4)]
    d = [(x[p][0] - x[p + 4][0], x[p][1] - x[p + 4][1]) for p in range(4)]
    ev = _dft4(a)
    (r0, i0), (r1, i1), (r2, i2), (r3, i3) = d
    b1r, b1i = SQH * (r1 + i1), SQH * (i1 - r1)
    b3r, n3i = SQH * (i3 - r3), SQH * (r3 + i3)
    sr, si, dr, di = r0 + i2, i0 - r2, r0 - i2, i0 + r2
    tr, ti, er, ei = b1r + b3r, b1i - n3i, b1r - b3r, b1i + n3i
    od = [(sr + tr, si + ti), (dr + ei, di - er), (sr - tr, si - ti), (dr - ei, di + er)]
    return [ev[0], od[0], ev[1], od[1], ev[2], od[2], ev[3], od[3]]


def _swap(x):
    return [(b, a) for (a, b) in x]


G = 4
NG = H // G
OSPLIT = 24
NEG = -1e9
N_L1, N_L2, N_L3 = 4, 20, 8


def _kernel(x_hbm, x3_hbm, mem_hbm, wq_hbm, wk_hbm, wv_hbm, wo_hbm, bx_hbm, wr_hbm, wi_hbm,
            fd_hbm, ms_hbm, out_hbm,
            xo_ref, mem_ref, xcraw_ref, raw_ref, w0_ref, w1_ref, w2_ref, w3_ref, w4_ref, w5_ref,
            woraw_ref, wo_ref, xc_ref, qkvc_ref, kve_ref,
            oall_ref, fille_ref, fillo_ref, bx_ref, wt_ref, wp_ref, ub_ref, sa_ref, sb_ref, fd_ref, ms_ref,
            tw_ref, zero_ref, sem_in, sem_out):
    scale = DH ** -0.5
    w_hbm = (wq_hbm, wk_hbm, wv_hbm)
    w_refs = (w0_ref, w1_ref, w2_ref, w3_ref, w4_ref, w5_ref)

    def raw_copy(c, i=0, nd=DM):
        rows = pl.ds(pl.multiple_of(i * nd, nd), nd)
        return pltpu.make_async_copy(
            w_hbm[c // 2].at[rows, pl.ds((c % 2) * 16, 16), :],
            raw_ref.at[c % 4, rows], sem_in.at[8 + min(c, 3) * 8 + max(c - 3, 0) * 2 + i])

    def xc_copy(k):
        return pltpu.make_async_copy(
            x3_hbm.at[:, pl.ds(8, 8), pl.ds(pl.multiple_of(k * 128, 128), 128)], xcraw_ref.at[k], sem_in.at[40 + k])

    cp_x = pltpu.make_async_copy(x_hbm, xo_ref, sem_in.at[0])
    cp_mem = pltpu.make_async_copy(mem_hbm, mem_ref, sem_in.at[1])
    cp_wo = pltpu.make_async_copy(wo_hbm, woraw_ref, sem_in.at[2])
    cp_bx = pltpu.make_async_copy(bx_hbm, bx_ref.at[0:4], sem_in.at[3])
    cp_fd = pltpu.make_async_copy(fd_hbm, fd_ref, sem_in.at[4])
    cp_ms = pltpu.make_async_copy(ms_hbm, ms_ref, sem_in.at[5])
    cp_wt = [pltpu.make_async_copy(src.at[:, pl.ds(lg * 256, 256)], wt_ref.at[a * 8 + lg], sem_in.at[48 + a * 8 + lg])
             for a, src in enumerate((wr_hbm, wi_hbm)) for lg in range(8)]

    for i in range(8):
        raw_copy(0, i, 128).start()
        xc_copy(i).start()
        raw_copy(1, i, 128).start()
    for i in range(4):
        raw_copy(2, i, 256).start()
    for i in range(2):
        raw_copy(3, i, 512).start()

    zero_ref[0] = 0

    def pin_rows(r):
        return pl.ds(pl.multiple_of(r + zero_ref[0] * 32, 8), 8)

    for p in range(8):
        for jq in range(4):
            tw_ref[(p * 4 + jq) * 2] = jnp.float32(math.cos(2 * math.pi * p * jq / 32))
            tw_ref[(p * 4 + jq) * 2 + 1] = jnp.float32(math.sin(2 * math.pi * p * jq / 32))

    qi = jax.lax.broadcasted_iota(jnp.int32, (48, 128), 0)
    ki = jax.lax.broadcasted_iota(jnp.int32, (48, 128), 1)

    def between(v, lo, hi):
        return (v >= lo) & (v < hi)

    def table(keep, other):
        return jnp.where(other, -jnp.inf, jnp.where(keep, 0.0, NEG)).astype(f32)

    keep = between(qi, 8, 16) | between(ki, 8, 16) | (qi >= jnp.where(ki < 32, ki, ki - 24))
    fille_ref[...] = table(keep, ki >= 40)[:32]
    q_even = between(qi, 32, 40)
    k_even = between(ki, 32, 40) | (ki >= 48)
    qpos = jnp.where(qi < 32, qi, jnp.where(qi < 40, qi - 24, qi - 32))
    kpos = jnp.where(ki < 32, ki, jnp.where(ki < 40, ki - 24, jnp.where(ki < 48, ki - 32, ki - 48)))
    keep = between(qi, 8, 16) | between(ki, 8, 16) | (ki >= 56) | (qpos >= kpos)
    fillo_ref[...] = table(keep, (q_even != k_even) | (ki >= 64))

    def relayout16(c, blk):
        w0 = pl.multiple_of(blk * 8, 8)
        v = _tou(raw_ref[c % 4, pl.ds(blk * 16, 16)]).reshape(8, 2, 8, 128)
        a, b = v[:, 0], v[:, 1]
        w_refs[c][0:8, pl.ds(w0, 8), :] = jnp.swapaxes((a & jnp.uint32(0xFFFF)) | (b << 16), 0, 1)
        w_refs[c][8:16, pl.ds(w0, 8), :] = jnp.swapaxes((a >> 16) | (b & jnp.uint32(0xFFFF0000)), 0, 1)

    def slot_of(h):
        return (h // 16) * 16 + (h % 2) * 8 + (h % 16) // 2

    def repack_wo64(blk):
        v = _tou(woraw_ref[pl.ds(pl.multiple_of(blk * 64, 64), 64), :])
        wo_ref[:, pl.ds(pl.multiple_of(blk * 32, 32), 32), :] = jnp.stack(
            [v[:, j * 128:(j + 1) * 128] for j in range(8)])

    sub4 = jax.lax.broadcasted_iota(jnp.int32, (128, 128), 0) & 3

    def wp_store(t, kb, tile):
        v = tile.T
        for g in range(4):
            r0 = pl.multiple_of(t * 2560 + kb * 160 + g * 40, 8)
            wp_ref[pl.ds(r0, 32), :] = v[g * 32:(g + 1) * 32]

    def b_prep(lg, hb, par):
        cols = slice(hb * 128, (hb + 1) * 128)
        a = _tou(wt_ref[lg, 0:512, cols])
        b = _tou(wt_ref[8 + lg, 0:512, cols])
        if par == 0:
            w = (a << 16) | (b & jnp.uint32(0xFFFF))
            m = (sub4 == 0) | (sub4 == 2)
        else:
            w = (a & jnp.uint32(0xFFFF0000)) | (b >> 16)
            m = (sub4 == 0) | (sub4 == 3)
        top = w[:128]
        bot = pltpu.roll(w[128:].reshape(16, 8, 128), 1 + par, 1).reshape(128, 128)
        wp_store(par, lg * 2 + hb, jnp.where(m, top, bot))
        wp_store(par + 2, lg * 2 + hb, jnp.where(m, bot, top))
        if par == 0:
            na = jnp.broadcast_to(wt_ref[lg, 512:513, cols].astype(f32), (128, 128))
            nb = jnp.broadcast_to(wt_ref[8 + lg, 512:513, cols].astype(f32), (128, 128))
            wp_store(4, lg * 2 + hb, pltpu.bitcast(na, u32) | (pltpu.bitcast(nb, u32) >> 16))

    def gather_c(k):
        xc_ref[k] = _tou(xcraw_ref[k].astype(f32).reshape(512, 128).astype(bf16))

    def store_qkvc(n, y):
        qkvc_ref[:, n] = y.reshape(NSEG // 2, 8, 128)

    def q_unit(i, groups, first, last, fillers):
        xk = _tobf(xc_ref[i])
        w0 = pl.multiple_of(i * 64, 64)
        for g in groups:
            rhs = jnp.concatenate(
                [_tobf(w_refs[h // 16][h % 16, pl.ds(w0, 64), :]) for h in range(4 * g, 4 * g + 4)], axis=1)
            y = _dot(xk, rhs)
            for h in range(4 * g, 4 * g + 4):
                yh = y[:, (h % 4) * 128:(h % 4 + 1) * 128]
                if not first:
                    yh = yh + ub_ref[h * 4:(h + 1) * 4].reshape(512, 128)
                if last:
                    store_qkvc(h, _tou(yh.astype(bf16)))
                else:
                    ub_ref[h * 4:(h + 1) * 4] = yh.reshape(4, 128, 128)
            mine = fillers.get(g, [])
            for fi, item in enumerate(mine):
                r = (fi * 512 // len(mine)) // 8 * 8
                item(pltpu.bitcast(y[r:r + 8, 0:128], u32))

    def rl_item(c, blk):
        def item(pin):
            w_refs[c][15, pin_rows(512), :] = pin
            relayout16(c, blk)
        return item

    def spread(fillers, items, groups):
        for k, item in enumerate(items):
            fillers.setdefault(groups[k * len(groups) // len(items)], []).append(item)
        return fillers

    def half_items(f, c, i, groups):
        return spread(f, [rl_item(c, i * 8 + blk) for blk in range(8)], groups)

    def piece_items(i):
        f = half_items(half_items({}, 1, i, (0, 1, 2)), 0, i + 1, (4, 5, 6))
        return spread(f, [lambda pin: gather_c(i + 1)], (6,))

    def chunk2_items(f, lo, hi, groups):
        return spread(f, [rl_item(2, blk) for blk in range(lo, hi)], groups)

    def wait_piece(i):
        raw_copy(1, i, 128).wait()
        xc_copy(i + 1).wait()
        raw_copy(0, i + 1, 128).wait()

    raw_copy(0, 0, 128).wait()
    for blk in range(8):
        relayout16(0, blk)
    xc_copy(0).wait()
    gather_c(0)
    q_unit(0, range(0, 2), True, False, {})
    raw_copy(1, 0, 128).wait()
    q_unit(0, range(2, 4), True, False, half_items({}, 1, 0, (2, 2, 3)))
    xc_copy(1).wait()
    raw_copy(0, 1, 128).wait()
    q_unit(0, range(4, 8), True, False,
           spread(half_items({}, 0, 1, (4, 5, 6)), [lambda pin: gather_c(1)], (6,)))

    def q_c(i, carry):
        wait_piece(i)
        q_unit(i, range(8), False, False, piece_items(i))
        return carry
    jax.lax.fori_loop(1, 5, q_c, 0)

    wait_piece(5)
    raw_copy(2, 0, 256).wait()
    raw_copy(2, 1, 256).wait()
    q_unit(5, range(8), False, False, chunk2_items(piece_items(5), 0, 24, (0, 1, 2, 3, 3, 4, 5, 6)))
    wait_piece(6)
    raw_copy(1, 7, 128).wait()
    raw_copy(2, 2, 256).wait()
    raw_copy(2, 3, 256).wait()
    q_unit(6, range(8), False, False, chunk2_items(piece_items(6), 24, 48, (0, 1, 2, 3, 3, 4, 5, 7)))
    q_unit(7, range(8), False, True, chunk2_items(half_items({}, 1, 7, (0, 1, 2)), 48, 64, (3, 4, 5, 6)))
    raw_copy(4).start()
    raw_copy(5).start()
    for cp in cp_wt:
        cp.start()
    cp_wo.start()
    cp_x.start()
    cp_mem.start()
    cp_bx.start()
    cp_fd.start()
    cp_ms.start()

    def bulk_iter(c, i):
        xc = jnp.concatenate([_tobf(xc_ref[k]) for k in range(8)], axis=1)
        for t in range(8):
            n = i * 8 + t
            y = _tou(_dot(xc, _tobf(w_refs[c][n, 0:512])).astype(bf16))
            store_qkvc(c * 16 + n, y)
            for blk in range(4):
                pin = y[blk * 64:blk * 64 + 8]
                if c + 1 < 6:
                    w_refs[c + 1][15, pin_rows(512), :] = pin
                    relayout16(c + 1, i * 32 + (t * 4 + blk))
                else:
                    wo_ref[7, pin_rows(2048), :] = pin
                    repack_wo64(i * 32 + (t * 4 + blk))
            if c >= 4:
                wp_ref[pin_rows(12832), :] = y[32:40]
                b_prep((c - 4) * 4 + i * 2 + t // 4, (t // 2) % 2, t % 2)

    for c in range(2, 6):
        if c == 4:
            for cp in cp_wt:
                cp.wait()
        if c == 5:
            cp_wo.wait()
        elif c > 2:
            raw_copy(c + 1).wait()

        def bulk(i, carry, c=c):
            if c == 2:
                raw_copy(3, i, 512).wait()
            bulk_iter(c, i)
            return carry
        jax.lax.fori_loop(0, 2, bulk, 0)

    cp_x.wait()
    cp_mem.wait()
    cp_bx.wait()
    cp_fd.wait()

    lane = jax.lax.broadcasted_iota(jnp.int32, (1, 128), 1)
    lane0 = lane == 0

    def first_lanes(t):
        la, lb = [k for k in range(4) if _FIRST[t][k]]
        return ((lane & 3) == la) | ((lane & 3) == lb)

    def d_products(st_ref, d, t, rows):
        return [_dot(st_ref[3 * t + k, rows].astype(bf16), _tobf(fd_ref[d * 12 + 3 * t + k])) for k in range(3)]

    def twiddles(p):
        return [(tw_ref[p * 8 + jq * 2], tw_ref[p * 8 + jq * 2 + 1]) if jq else None for jq in range(4)]

    st_refs = (sa_ref, sb_ref)

    def p1_pre(p, slot, rs, q):
        def item(y):
            st_refs[slot][7, pin_rows(256), :] = y
            xq = bx_ref[q, pl.ds(pl.multiple_of(p * 64 + rs * 16, 16), 16), :].astype(f32)
            zz = _r8_real([xq[:, a * 128:(a + 1) * 128] for a in range(8)])
            r = (rs * 4 + q) * 16
            st_refs[slot][:, r:r + 16] = jnp.stack([v for (a, b) in zz for v in (a + b, b, a)])
        return item

    def p1_mm(p, slot, t):
        def item(y):
            cs = twiddles(p)

            def put(n, rs, re, im):
                v = jnp.stack([re.reshape(2, 8, 128), im.reshape(2, 8, 128)], axis=1)
                ub_ref[n * 8 + p, rs * 32:(rs + 1) * 32] = v.reshape(32, 128)

            first = first_lanes(t)
            for rs in range(4):
                k1, k2, k3 = d_products(st_refs[slot], 0, t, slice(rs * 64, (rs + 1) * 64))
                if t == 0:
                    re, im = jnp.where(first, k3, k2), k1 - jnp.where(first, k2, k3)
                    u = [im[q * 16:(q + 1) * 16] for q in range(4)]
                    sr, dr, tr, er = u[0] + u[2], u[0] - u[2], u[1] + u[3], u[1] - u[3]
                    a2 = sr - tr
                    _, (c1, s1), (c2, s2), (c3, s3) = cs
                    put(16, rs, sr + tr, jnp.zeros_like(sr))
                    put(17, rs, dr * c1 - er * s1, er * (-c1) - dr * s1)
                    put(18, rs, a2 * c2, a2 * (-s2))
                    put(19, rs, dr * c3 + er * s3, er * c3 - dr * s3)
                    im = jnp.where(lane0, 0.0, im)
                else:
                    re, im = k1 + k2, (k3 - k1) * jnp.where(first, 1.0, -1.0)
                a = _dft4([(re[q * 16:(q + 1) * 16], im[q * 16:(q + 1) * 16]) for q in range(4)])
                for jq in range(4):
                    re, im = a[jq]
                    if jq > 0:
                        c, sn = cs[jq]
                        re, im = re * c + im * sn, im * c - re * sn
                    put(t * 4 + jq, rs, re, im)
        return item

    def p2_bfly(u, g, inverse):
        def item(y):
            if y is not None:
                ub_ref[168, pin_rows(0), :] = y
            v = ub_ref[pl.ds(u * 8, 8), g * 16:(g + 1) * 16]
            x = [(v[p, 0:8], v[p, 8:16]) for p in range(8)]
            x = _swap(_dft8(_swap(x))) if inverse else _dft8(x)
            ub_ref[pl.ds(u * 8, 8), g * 16:(g + 1) * 16] = jnp.stack([w for c in x for w in c]).reshape(8, 16, 128)
        return item

    def p2_fwd(u, jps):
        def item(y):
            t = u >> 2
            jq = u & 3
            xs = [_dot(_tobf(ms_ref[jq + 4 * jp]), ub_ref[u * 8 + jp].astype(bf16)) for jp in jps]
            for jp, xx in zip(jps, xs):
                w = wp_ref[pl.ds(t * 2560 + jq + 4 * jp, 64, stride=40), :]
                wr = pltpu.bitcast(w & jnp.uint32(0xFFFF0000), f32).reshape(8, 8, 128)
                wi = pltpu.bitcast(w << 16, f32).reshape(8, 8, 128)
                xx = xx.reshape(8, 2, 8, 128)
                xr, xi = xx[:, 0], xx[:, 1]
                ub_ref[u * 8 + jp] = jnp.stack([xr * wr - xi * wi, xr * wi + xi * wr], axis=1).reshape(128, 128)
        return item

    def p2_inv(u, jps):
        def item(y):
            jq = u & 3
            zs = [_dot(_tobf(ms_ref[32 + jq + 4 * jp]), ub_ref[u * 8 + jp].astype(bf16)) for jp in jps]
            for jp, zz in zip(jps, zs):
                ub_ref[u * 8 + jp] = zz
        return item

    def p3_pre(p, g, t):
        def item(y):
            sa_ref[7, pin_rows(256), :] = y
            cs = twiddles(p)

            def fetch(t):
                a = []
                for jq in range(4):
                    v = ub_ref[(t * 4 + jq) * 8 + p, g * 16:(g + 1) * 16]
                    re, im = v[0:8], v[8:16]
                    if jq > 0:
                        c, sn = cs[jq]
                        re, im = re * c - im * sn, im * c + re * sn
                    a.append((re, im))
                return _swap(_dft4(_swap(a)))

            u = fetch(t)
            if t == 0:
                ny = fetch(4)
                u = [(u[q][0], jnp.where(lane0, ny[q][0], u[q][1])) for q in range(4)]
            first = first_lanes(t)
            for q in range(4):
                re, im = u[q]
                if t == 0:
                    vals = (im, jnp.where(first, re, im), jnp.where(first, im, re))
                else:
                    im = im * jnp.where(first, 1.0, -1.0)
                    vals = (re + im, im, re)
                sa_ref[3 * t:3 * t + 3, q * 64 + g * 8:q * 64 + (g + 1) * 8] = jnp.stack(vals)
        return item

    def p3_mm(p, q):
        def item(y):
            g = []
            for t in range(4):
                k1, k2, k3 = d_products(sa_ref, 1, t, slice(q * 64, (q + 1) * 64))
                g.append((k2 + k1, k3 + k1 if t == 0 else k3 - k1))
            yy = _r8_real_t(g)
            bx_ref[q, pl.ds(pl.multiple_of(p * 64, 64), 64), :] = jnp.concatenate(yy, axis=1).astype(bf16)
        return item

    def b_out(p):
        def item(y):
            rows = pl.ds(pl.multiple_of(p * 64, 64), 64)
            pltpu.make_async_copy(bx_ref.at[0:4, rows, :], out_hbm.at[:, rows, pl.ds(DM, DM)],
                                  sem_out.at[1]).start()
            bx_ref[4, pin_rows(0), 0:128] = y.astype(bf16)
        return item

    def step(pp, odd, mem, hooks):
        r0 = pl.multiple_of(pp * 64 + 32 * odd, SEG)
        xs = xo_ref[pl.ds(r0, SEG), :]
        x_lo = xs[0:8].astype(f32)
        hm = jnp.concatenate(
            [jnp.concatenate([x_lo, jnp.concatenate(mem, axis=1)], axis=0).astype(bf16), xs[16:32]], axis=0)
        fill = fillo_ref[:, 0:64] if odd else fille_ref[:, 0:48]
        nrow = 48 if odd else 32
        qkv, ps = {}, {}

        def do_qkv(h0, h1):
            for h in range(h0, h1):
                for t in range(3):
                    n = t * H + slot_of(h)
                    y32 = _dot(hm, _tobf(w_refs[n // 16][n % 16, 0:512]))
                    y = y32.astype(bf16)
                    parts = [y]
                    if odd or t > 0:
                        parts.append(_tobf(qkvc_ref[pp, n]))
                    if t > 0:
                        if odd:
                            parts.append(_tobf(kve_ref[(t - 1) * H + h]))
                        else:
                            kve_ref[(t - 1) * H + h] = _tou(y[0:16])
                    qkv[(t, h)] = jnp.concatenate(parts, axis=0) if len(parts) > 1 else y
                for item in hooks.get(h, ()):
                    item(y32[0:8])

        def do_s(g):
            for h in range(g * G, (g + 1) * G):
                sc = jax.lax.dot_general(qkv[(0, h)], qkv[(1, h)], (((1,), (1,)), ((), ())),
                                         preferred_element_type=f32)
                sc = jnp.where(fill == 0.0, sc * scale, fill)
                e = jnp.exp(sc - jnp.max(sc, axis=1, keepdims=True))
                den = jnp.sum(e, axis=1, keepdims=True)
                r = pl.reciprocal(den, approx=True)
                r = r * (2.0 - den * r)
                ps[h] = (e * r).astype(bf16)

        def do_pv(g):
            for h in range(g * G, (g + 1) * G):
                oall_ref[0:nrow // 2, h * DH:(h + 1) * DH] = _tou(_dot(ps[h], qkv[(2, h)]).astype(bf16))

        def do_o(j, h0, h1):
            return _dot(_tobf(oall_ref[0:nrow // 2, h0 * DH:h1 * DH]), _tobf(wo_ref[j, h0 * 64:h1 * 64, :]))

        for g in range(NG):
            do_qkv(g * G, g * G + G // 2)
            if g >= 1:
                do_s(g - 1)
            do_qkv(g * G + G // 2, (g + 1) * G)
            if g >= 2:
                do_pv(g - 2)
        part = {}
        for j in range(8):
            items = hooks.get(('o', j), ())
            if len(items) == 1:
                part[j] = do_o(j, 0, OSPLIT)
                items[0](None)
            elif items:
                half = do_o(j, 0, OSPLIT // 2)
                items[0](half[0:8])
                part[j] = do_o(j, OSPLIT // 2, OSPLIT) + half
                items[1](part[j][0:8])
            else:
                part[j] = do_o(j, 0, OSPLIT)
            if j == 2:
                do_s(NG - 1)
                do_pv(NG - 2)
            if j == 5:
                do_pv(NG - 1)
        new_mem = []
        for j in range(8):
            cols = slice(j * 128, (j + 1) * 128)
            res = do_o(j, OSPLIT, H) + part[j]
            new_mem.append(res[8:16])
            if odd:
                xo_ref[pl.ds(r0, SEG), cols] = jnp.concatenate(
                    [res[0:8], res[40:48], res[16:32]], axis=0).astype(bf16)
                xo_ref[pl.ds(r0 - 24, 8), cols] = res[32:40].astype(bf16)
            else:
                xo_ref[pl.ds(r0, SEG), cols] = res.astype(bf16)
        for item in hooks.get(H, ()):
            item(None)
        if odd:
            pltpu.make_async_copy(
                xo_ref.at[pl.ds(pl.multiple_of(pp * 64, 64), 64), :],
                out_hbm.at[pp >> 3, pl.ds(pl.multiple_of((pp & 7) * 64, 64), 64), pl.ds(0, DM)],
                sem_out.at[0]).start()
        return new_mem

    def l1(i, mem):
        he = {h: [p1_pre(2 * i + h // 16, h // 16, (h % 16) // 4, h % 4)] for h in range(32)}
        he[H] = [p1_mm(2 * i, 0, 1)]
        ho = {('o', k): [p1_mm(2 * i + (k + 1) // 4, (k + 1) // 4, t)] for k, t in enumerate((0, 2, 3, 0, 1, 2, 3))}
        mem = step(i, 0, mem, he)
        mem = step(i, 1, mem, ho)
        return mem

    def l2(i, mem):
        u = i - N_L1
        he = {3: [p2_fwd(u, range(0, 4))], 7: [p2_fwd(u, range(4, 8))], H: [p2_inv(u, range(0, 8))]}
        ho = {('o', j): [p2_bfly(u, j, True), p2_bfly(u + 1, j, False)] for j in range(8)}
        mem = step(i, 0, mem, he)
        mem = step(i, 1, mem, ho)
        return mem

    def l3(i, mem):
        p = i - N_L1 - N_L2
        he = {h: [p3_pre(p, h // 4, h % 4)] for h in range(32)}
        he[H] = [p3_mm(p, q) for q in range(4)]
        ho = {12: [b_out(p)]}
        mem = step(i, 0, mem, he)
        mem = step(i, 1, mem, ho)
        return mem

    m0 = mem_ref[...].astype(f32)
    mem = [m0[:, j * 128:(j + 1) * 128] for j in range(8)]
    mem = jax.lax.fori_loop(0, N_L1, l1, mem)
    cp_ms.wait()
    for g in range(8):
        p2_bfly(0, g, False)(None)
    mem = jax.lax.fori_loop(N_L1, N_L1 + N_L2, l2, mem)
    mem = jax.lax.fori_loop(N_L1 + N_L2, NSEG // 2, l3, mem)

    pltpu.make_async_copy(bx_ref.at[0:4], out_hbm.at[:, :, pl.ds(DM, DM)], sem_out.at[1]).wait()
    pltpu.make_async_copy(xo_ref, xo_ref, sem_out.at[0]).wait()


@jax.jit
def _run(x, mem0, wq, wk, wv, wo, bx, w_r, w_i):
    fd, ms = _tables()
    hbm = pl.BlockSpec(memory_space=pl.ANY)
    out = pl.pallas_call(
        _kernel,
        out_shape=jax.ShapeDtypeStruct((4, S // 4, 2 * DM), bf16),
        in_specs=[hbm] * 12,
        out_specs=hbm,
        scratch_shapes=[
            pltpu.VMEM((S, DM), bf16),
            pltpu.VMEM((MEM, DM), bf16),
            pltpu.VMEM((8, NSEG, 8, 128), bf16),
            pltpu.VMEM((4, DM, 16, DH), bf16),
        ] + [pltpu.VMEM((16, DM // 2 + 8, DH), u32)] * 6 + [
            pltpu.VMEM((H * DH, DM), bf16),
            pltpu.VMEM((8, H * DH // 2 + 8, 128), u32),
            pltpu.VMEM((8, 256, 128), u32),
            pltpu.VMEM((NSEG // 2, 3 * H, 8, 128), u32),
            pltpu.VMEM((2 * H, 8, 128), u32),
            pltpu.VMEM((24, H * DH), u32),
            pltpu.VMEM((32, 128), f32),
            pltpu.VMEM((48, 128), f32),
            pltpu.VMEM((5, S // 4, DM), bf16),
            pltpu.VMEM((16, DM // 2 + 1, 256), bf16),
            pltpu.VMEM((12840, 128), u32),
            pltpu.VMEM((169, 128, 128), f32),
            pltpu.VMEM((12, 264, 128), f32),
            pltpu.VMEM((12, 264, 128), f32),
            pltpu.VMEM((24, 64, 128), u32),
            pltpu.VMEM((64, 64, 128), u32),
            pltpu.SMEM((64,), f32),
            pltpu.SMEM((1,), jnp.int32),
            pltpu.SemaphoreType.DMA((64,)),
            pltpu.SemaphoreType.DMA((2,)),
        ],
        compiler_params=pltpu.CompilerParams(vmem_limit_bytes=120 * 1024 * 1024,
                                             disable_semaphore_checks=True,
                                             disable_bounds_checks=True),
    )(x.reshape(S, DM), x.reshape(NSEG, SEG, DM), mem0.reshape(MEM, DM), wq, wk, wv,
      wo.reshape(H * DH, DM), bx.reshape(4, S // 4, DM), w_r.T, w_i.T, jnp.asarray(fd), jnp.asarray(ms))
    return out.reshape(1, S, 2 * DM)


def pallas_concat_heads__memory_aug_recurrent_mem_tr__spectral_gfnet__prompt_kernel(
    A_x: jax.Array,
    A_mem0: jax.Array,
    A_Wq: jax.Array,
    A_Wk: jax.Array,
    A_Wv: jax.Array,
    A_Wo: jax.Array,
    A_seg_len,
    B_x: jax.Array,
    B_w_r: jax.Array,
    B_w_i: jax.Array,
):
    if isinstance(A_seg_len, int):
        assert A_seg_len == SEG
    assert A_x.shape == (1, S, DM) and A_mem0.shape == (1, MEM, DM) and A_Wq.shape == (DM, H, DH)
    assert B_x.shape == (1, S, DM) and B_w_r.shape == (S, DM // 2 + 1)
    return _run(A_x, A_mem0, A_Wq, A_Wk, A_Wv, A_Wo, B_x, B_w_r, B_w_i)
```

```python
import math

import numpy as np
import jax
import jax.numpy as jnp
import jax.experimental.pallas as pl
import jax.experimental.pallas.tpu as pltpu

bf16 = jnp.bfloat16
f32 = jnp.float32
u32 = jnp.uint32

S, DM = 2048, 1024
H, DH = 32, 128
MEM, SEG = 8, 32
NSEG = S // SEG
SQH = math.sqrt(0.5)

_PAIRS = ((0, 4), (1, 7), (2, 6), (3, 5))
_FIRST = np.array([[1, 1, 0, 0], [1, 0, 1, 0], [0, 1, 1, 0], [0, 1, 0, 1]], bool)


def _pack_rows(a):
    u = np.ascontiguousarray(a, dtype=np.float32).view(np.uint32).astype(np.uint64)
    b = ((u + 0x7FFF + ((u >> 16) & 1)) >> 16).astype(np.uint32)
    return (b[..., 0::2, :] | (b[..., 1::2, :] << 16)).astype(np.uint32)


def _tables():
    k2 = np.zeros((4, 128), np.int64)
    for t in range(4):
        odd = t % 2
        for lam in range(128):
            k = 2 * lam + odd
            if k % 8 not in _PAIRS[t]:
                k = 2 * (128 + 8 * (lam // 8) + (lam % 8 - 1 - odd) % 8) + odd
            assert k % 8 in _PAIRS[t]
            k2[t, lam] = k
    b = np.arange(128)[:, None]
    F = np.zeros((12, 128, 128))
    G = np.zeros((12, 128, 128))
    for t in range(4):
        th = 2 * np.pi * ((b * k2[t][None, :]) % DM) / DM
        C, Sn = np.cos(th), np.sin(th)
        first = ((k2[t] % 8) == _PAIRS[t][0])[None, :]
        assert np.array_equal(first[0], _FIRST[t][np.arange(128) % 4])
        if t == 0:
            im = -Sn
            im[:, 0] = (-1.0) ** np.arange(128)
            F[0:3] = im, np.where(first, im, C), np.where(first, C, im)
            G[0:3] = im, np.where(first, C, -im), np.where(first, -im, C)
            G[0:3, :, 0] *= 0.5
        else:
            Sg = np.where(first, Sn, -Sn)
            F[3 * t:3 * t + 3] = C, -(C + Sg), C - Sg
            G[3 * t:3 * t + 3] = F[3 * t:3 * t + 3]
    Finv = np.transpose(G, (0, 2, 1)) * (2.0 / DM)
    fd = _pack_rows(np.concatenate([F, Finv]))
    M = np.zeros((32, 128, 128))
    r = np.arange(64)[None, :]
    l = np.arange(64)[:, None]
    for j in range(32):
        th = 2 * np.pi * ((r * (j + 32 * l)) % S) / S
        C, Sn = np.cos(th), np.sin(th)
        M[j, :64, :64] = C
        M[j, :64, 64:] = Sn
        M[j, 64:, :64] = -Sn
        M[j, 64:, 64:] = C
    perm = np.arange(128).reshape(2, 8, 8).transpose(1, 0, 2).reshape(128)
    M = M[:, perm][:, :, perm]
    Minv = np.transpose(M, (0, 2, 1)) / S
    ms = _pack_rows(np.concatenate([M, Minv]))
    return fd, ms


def _tobf(w):
    return pltpu.bitcast(w, bf16)


def _tou(w):
    return pltpu.bitcast(w, u32)


def _dot(a, b):
    return jnp.dot(a, b, preferred_element_type=f32)


def _r8_real(x):
    t0, t1 = x[0] + x[4], x[0] - x[4]
    t2, t3 = x[2] + x[6], x[2] - x[6]
    t4, t5 = x[1] + x[5], x[1] - x[5]
    t6, t7 = x[3] + x[7], x[3] - x[7]
    e0, e1 = t0 + t2, t0 - t2
    o0, o1 = t4 + t6, t4 - t6
    u, v = SQH * (t5 - t7), SQH * (t5 + t7)
    return [(e0 + o0, e0 - o0), (t1 + u, v + t3), (e1, o1), (t1 - u, v - t3)]


def _r8_real_t(g):
    (z0, z4), (a1, b1), (e1, o1), (a3, b3) = g
    e0, o0 = z0 + z4, z0 - z4
    t1, u = a1 + a3, a1 - a3
    v, t3 = b1 + b3, b1 - b3
    t5, t7 = SQH * (v + u), SQH * (v - u)
    t0, t2 = e0 + e1, e0 - e1
    t4, t6 = o0 + o1, o0 - o1
    return [t0 + t1, t4 + t5, t2 + t3, t6 + t7, t0 - t1, t4 - t5, t2 - t3, t6 - t7]


def _dft4(u):
    (r0, i0), (r1, i1), (r2, i2), (r3, i3) = u
    sr, si, dr, di = r0 + r2, i0 + i2, r0 - r2, i0 - i2
    tr, ti, er, ei = r1 + r3, i1 + i3, r1 - r3, i1 - i3
    return [(sr + tr, si + ti), (dr + ei, di - er), (sr - tr, si - ti), (dr - ei, di + er)]


def _dft8(x):
    a = [(x[p][0] + x[p + 4][0], x[p][1] + x[p + 4][1]) for p in range(4)]
    d = [(x[p][0] - x[p + 4][0], x[p][1] - x[p + 4][1]) for p in range(4)]
    ev = _dft4(a)
    (r0, i0), (r1, i1), (r2, i2), (r3, i3) = d
    b1r, b1i = SQH * (r1 + i1), SQH * (i1 - r1)
    b3r, n3i = SQH * (i3 - r3), SQH * (r3 + i3)
    sr, si, dr, di = r0 + i2, i0 - r2, r0 - i2, i0 + r2
    tr, ti, er, ei = b1r + b3r, b1i - n3i, b1r - b3r, b1i + n3i
    od = [(sr + tr, si + ti), (dr + ei, di - er), (sr - tr, si - ti), (dr - ei, di + er)]
    return [ev[0], od[0], ev[1], od[1], ev[2], od[2], ev[3], od[3]]


def _swap(x):
    return [(b, a) for (a, b) in x]


G = 4
NG = H // G
OSPLIT = 24
NEG = -1e9
N_L1, N_L2, N_L3 = 4, 20, 8


def _kernel(x_hbm, x3_hbm, mem_hbm, wq_hbm, wk_hbm, wv_hbm, wo_hbm, bx_hbm, wr_hbm, wi_hbm,
            fd_hbm, ms_hbm, out_hbm,
            xo_ref, mem_ref, xcraw_ref, raw_ref, w0_ref, w1_ref, w2_ref, w3_ref, w4_ref, w5_ref,
            woraw_ref, wo_ref, xc_ref, qkvc_ref, kve_ref,
            oall_ref, fille_ref, fillo_ref, bx_ref, wt_ref, wp_ref, ub_ref, sa_ref, sb_ref, fd_ref, ms_ref,
            tw_ref, zero_ref, sem_in, sem_out):
    scale = DH ** -0.5
    w_hbm = (wq_hbm, wk_hbm, wv_hbm)
    w_refs = (w0_ref, w1_ref, w2_ref, w3_ref, w4_ref, w5_ref)

    def raw_copy(c, i=0, nd=DM):
        rows = pl.ds(pl.multiple_of(i * nd, nd), nd)
        return pltpu.make_async_copy(
            w_hbm[c // 2].at[rows, pl.ds((c % 2) * 16, 16), :],
            raw_ref.at[c % 4, rows], sem_in.at[8 + min(c, 3) * 8 + max(c - 3, 0) * 2 + i])

    def xc_copy(k):
        return pltpu.make_async_copy(
            x3_hbm.at[:, pl.ds(8, 8), pl.ds(pl.multiple_of(k * 128, 128), 128)], xcraw_ref.at[k], sem_in.at[40 + k])

    cp_x = pltpu.make_async_copy(x_hbm, xo_ref, sem_in.at[0])
    cp_mem = pltpu.make_async_copy(mem_hbm, mem_ref, sem_in.at[1])
    cp_wo = pltpu.make_async_copy(wo_hbm, woraw_ref, sem_in.at[2])
    cp_bx = pltpu.make_async_copy(bx_hbm, bx_ref.at[0:4], sem_in.at[3])
    cp_fd = pltpu.make_async_copy(fd_hbm, fd_ref, sem_in.at[4])
    cp_ms = pltpu.make_async_copy(ms_hbm, ms_ref, sem_in.at[5])
    cp_wt = [pltpu.make_async_copy(src.at[:, pl.ds(lg * 256, 256)], wt_ref.at[a * 8 + lg], sem_in.at[48 + a * 8 + lg])
             for a, src in enumerate((wr_hbm, wi_hbm)) for lg in range(8)]

    for i in range(8):
        raw_copy(0, i, 128).start()
        xc_copy(i).start()
        if i >= 3:
            raw_copy(2, i - 3, 128).start()
        if i == 7:
            raw_copy(2, 5, 128).start()
        raw_copy(1, i, 128).start()
    for i in range(6, 8):
        raw_copy(2, i, 128).start()
    for i in range(2):
        raw_copy(3, i, 512).start()
    for cp in cp_wt + [cp_wo, cp_x, cp_mem, cp_bx, cp_fd, cp_ms]:
        cp.start(priority=1)

    zero_ref[0] = 0

    def pin_rows(r):
        return pl.ds(pl.multiple_of(r + zero_ref[0] * 32, 8), 8)

    for p in range(8):
        for jq in range(4):
            tw_ref[(p * 4 + jq) * 2] = jnp.float32(math.cos(2 * math.pi * p * jq / 32))
            tw_ref[(p * 4 + jq) * 2 + 1] = jnp.float32(math.sin(2 * math.pi * p * jq / 32))

    qi = jax.lax.broadcasted_iota(jnp.int32, (48, 128), 0)
    ki = jax.lax.broadcasted_iota(jnp.int32, (48, 128), 1)

    def between(v, lo, hi):
        return (v >= lo) & (v < hi)

    def table(keep, other):
        return jnp.where(other, -jnp.inf, jnp.where(keep, 0.0, NEG)).astype(f32)

    keep = between(qi, 8, 16) | between(ki, 8, 16) | (qi >= jnp.where(ki < 32, ki, ki - 24))
    fille_ref[...] = table(keep, ki >= 40)[:32]
    q_even = between(qi, 32, 40)
    k_even = between(ki, 32, 40) | (ki >= 48)
    qpos = jnp.where(qi < 32, qi, jnp.where(qi < 40, qi - 24, qi - 32))
    kpos = jnp.where(ki < 32, ki, jnp.where(ki < 40, ki - 24, jnp.where(ki < 48, ki - 32, ki - 48)))
    keep = between(qi, 8, 16) | between(ki, 8, 16) | (ki >= 56) | (qpos >= kpos)
    fillo_ref[...] = table(keep, (q_even != k_even) | (ki >= 64))

    def relayout16(c, blk):
        w0 = pl.multiple_of(blk * 8, 8)
        v = _tou(raw_ref[c % 4, pl.ds(blk * 16, 16)]).reshape(8, 2, 8, 128)
        a, b = v[:, 0], v[:, 1]
        w_refs[c][0:8, pl.ds(w0, 8), :] = jnp.swapaxes((a & jnp.uint32(0xFFFF)) | (b << 16), 0, 1)
        w_refs[c][8:16, pl.ds(w0, 8), :] = jnp.swapaxes((a >> 16) | (b & jnp.uint32(0xFFFF0000)), 0, 1)

    def slot_of(h):
        return (h // 16) * 16 + (h % 2) * 8 + (h % 16) // 2

    def repack_wo64(blk):
        v = _tou(woraw_ref[pl.ds(pl.multiple_of(blk * 64, 64), 64), :])
        wo_ref[:, pl.ds(pl.multiple_of(blk * 32, 32), 32), :] = jnp.stack(
            [v[:, j * 128:(j + 1) * 128] for j in range(8)])

    sub4 = jax.lax.broadcasted_iota(jnp.int32, (128, 128), 0) & 3

    def wp_store(t, kb, tile):
        v = tile.T
        for g in range(4):
            r0 = pl.multiple_of(t * 2560 + kb * 160 + g * 40, 8)
            wp_ref[pl.ds(r0, 32), :] = v[g * 32:(g + 1) * 32]

    def b_prep(lg, hb, par):
        cols = slice(hb * 128, (hb + 1) * 128)
        a = _tou(wt_ref[lg, 0:512, cols])
        b = _tou(wt_ref[8 + lg, 0:512, cols])
        if par == 0:
            w = (a << 16) | (b & jnp.uint32(0xFFFF))
            m = (sub4 == 0) | (sub4 == 2)
        else:
            w = (a & jnp.uint32(0xFFFF0000)) | (b >> 16)
            m = (sub4 == 0) | (sub4 == 3)
        top = w[:128]
        bot = pltpu.roll(w[128:].reshape(16, 8, 128), 1 + par, 1).reshape(128, 128)
        wp_store(par, lg * 2 + hb, jnp.where(m, top, bot))
        wp_store(par + 2, lg * 2 + hb, jnp.where(m, bot, top))
        if par == 0:
            na = jnp.broadcast_to(wt_ref[lg, 512:513, cols].astype(f32), (128, 128))
            nb = jnp.broadcast_to(wt_ref[8 + lg, 512:513, cols].astype(f32), (128, 128))
            wp_store(4, lg * 2 + hb, pltpu.bitcast(na, u32) | (pltpu.bitcast(nb, u32) >> 16))

    def gather_c(k):
        xc_ref[k] = _tou(xcraw_ref[k].astype(f32).reshape(512, 128).astype(bf16))

    def store_qkvc(n, y):
        qkvc_ref[:, n] = y.reshape(NSEG // 2, 8, 128)

    def q_unit(i, groups, first, last, fillers):
        xk = _tobf(xc_ref[i])
        w0 = pl.multiple_of(i * 64, 64)
        for g in groups:
            rhs = jnp.concatenate(
                [_tobf(w_refs[h // 16][h % 16, pl.ds(w0, 64), :]) for h in range(4 * g, 4 * g + 4)], axis=1)
            y = _dot(xk, rhs)
            for h in range(4 * g, 4 * g + 4):
                yh = y[:, (h % 4) * 128:(h % 4 + 1) * 128]
                if not first:
                    yh = yh + ub_ref[h * 4:(h + 1) * 4].reshape(512, 128)
                if last:
                    store_qkvc(h, _tou(yh.astype(bf16)))
                else:
                    ub_ref[h * 4:(h + 1) * 4] = yh.reshape(4, 128, 128)
            mine = fillers.get(g, [])
            for fi, item in enumerate(mine):
                r = (fi * 512 // len(mine)) // 8 * 8
                item(pltpu.bitcast(y[r:r + 8, 0:128], u32))

    def rl_item(c, blk):
        def item(pin):
            w_refs[c][15, pin_rows(512), :] = pin
            relayout16(c, blk)
        return item

    def spread(fillers, items, groups):
        for k, item in enumerate(items):
            fillers.setdefault(groups[k * len(groups) // len(items)], []).append(item)
        return fillers

    def half_items(f, c, i, groups):
        return spread(f, [rl_item(c, i * 8 + blk) for blk in range(8)], groups)

    def piece_items(i):
        f = half_items(half_items({}, 1, i, (0, 1, 2)), 0, i + 1, (4, 5, 6))
        return spread(f, [lambda pin: gather_c(i + 1)], (7,))

    def chunk2_items(f, lo, hi, groups):
        return spread(f, [rl_item(2, blk) for blk in range(lo, hi)], groups)

    def wait_piece(i):
        raw_copy(1, i, 128).wait()
        xc_copy(i + 1).wait()
        raw_copy(0, i + 1, 128).wait()

    raw_copy(0, 0, 128).wait()
    for blk in range(8):
        relayout16(0, blk)
    xc_copy(0).wait()
    gather_c(0)
    q_unit(0, range(0, 2), True, False, {})
    raw_copy(1, 0, 128).wait()
    q_unit(0, range(2, 4), True, False, half_items({}, 1, 0, (2, 2, 3)))
    q_unit(0, range(4, 6), True, False, {})
    xc_copy(1).wait()
    raw_copy(0, 1, 128).wait()
    q_unit(0, range(6, 8), True, False,
           spread(half_items({}, 0, 1, (6, 6, 7)), [lambda pin: gather_c(1)], (6,)))
    raw_copy(1, 1, 128).wait()
    q_unit(1, range(0, 4), False, False, half_items({}, 1, 1, (0, 1, 2)))
    xc_copy(2).wait()
    raw_copy(0, 2, 128).wait()
    q_unit(1, range(4, 8), False, False,
           spread(half_items({}, 0, 2, (4, 5, 6)), [lambda pin: gather_c(2)], (6,)))

    def q_c(i, carry):
        wait_piece(i)
        raw_copy(2, i - 2, 128).wait()
        q_unit(i, range(8), False, False, half_items(piece_items(i), 2, i - 2, (3, 3, 3, 3, 4, 5, 6, 7)))
        return carry
    jax.lax.fori_loop(2, 6, q_c, 0)

    wait_piece(6)
    raw_copy(2, 4, 128).wait()
    raw_copy(2, 5, 128).wait()
    q_unit(6, range(8), False, False, chunk2_items(piece_items(6), 32, 48, (0, 1, 2, 3, 3, 4, 5, 6)))
    raw_copy(1, 7, 128).wait()
    raw_copy(2, 6, 128).wait()
    raw_copy(2, 7, 128).wait()
    q_unit(7, range(8), False, True, chunk2_items(half_items({}, 1, 7, (0, 1, 2)), 48, 64, (3, 4, 5, 6)))
    raw_copy(4).start()
    raw_copy(5).start()

    def bulk_iter(c, i):
        xc = jnp.concatenate([_tobf(xc_ref[k]) for k in range(8)], axis=1)
        for t in range(8):
            n = i * 8 + t
            y = _tou(_dot(xc, _tobf(w_refs[c][n, 0:512])).astype(bf16))
            store_qkvc(c * 16 + n, y)
            for blk in range(4):
                pin = y[blk * 64:blk * 64 + 8]
                if c + 1 < 6:
                    w_refs[c + 1][15, pin_rows(512), :] = pin
                    relayout16(c + 1, i * 32 + (t * 4 + blk))
                else:
                    wo_ref[7, pin_rows(2048), :] = pin
                    repack_wo64(i * 32 + (t * 4 + blk))
            if c >= 4:
                wp_ref[pin_rows(12832), :] = y[32:40]
                b_prep((c - 4) * 4 + i * 2 + t // 4, (t // 2) % 2, t % 2)

    for c in range(2, 6):
        if c == 4:
            for cp in cp_wt:
                cp.wait()
        if c == 5:
            cp_wo.wait()
        elif c > 2:
            raw_copy(c + 1).wait()

        def bulk(i, carry, c=c):
            if c == 2:
                raw_copy(3, i, 512).wait()
            bulk_iter(c, i)
            return carry
        jax.lax.fori_loop(0, 2, bulk, 0)

    cp_x.wait()
    cp_mem.wait()
    cp_bx.wait()
    cp_fd.wait()

    lane = jax.lax.broadcasted_iota(jnp.int32, (1, 128), 1)
    lane0 = lane == 0

    def first_lanes(t):
        la, lb = [k for k in range(4) if _FIRST[t][k]]
        return ((lane & 3) == la) | ((lane & 3) == lb)

    def d_products(st_ref, d, t, rows):
        return [_dot(st_ref[3 * t + k, rows].astype(bf16), _tobf(fd_ref[d * 12 + 3 * t + k])) for k in range(3)]

    def twiddles(p):
        return [(tw_ref[p * 8 + jq * 2], tw_ref[p * 8 + jq * 2 + 1]) if jq else None for jq in range(4)]

    st_refs = (sa_ref, sb_ref)

    def p1_pre(p, slot, rs, q):
        def item(y):
            st_refs[slot][7, pin_rows(256), :] = y
            xq = bx_ref[q, pl.ds(pl.multiple_of(p * 64 + rs * 16, 16), 16), :].astype(f32)
            zz = _r8_real([xq[:, a * 128:(a + 1) * 128] for a in range(8)])
            r = (rs * 4 + q) * 16
            st_refs[slot][:, r:r + 16] = jnp.stack([v for (a, b) in zz for v in (a + b, b, a)])
        return item

    def p1_mm(p, slot, t):
        def item(y):
            cs = twiddles(p)

            def put(n, rs, re, im):
                v = jnp.stack([re.reshape(2, 8, 128), im.reshape(2, 8, 128)], axis=1)
                ub_ref[n * 8 + p, rs * 32:(rs + 1) * 32] = v.reshape(32, 128)

            first = first_lanes(t)
            for rs in range(4):
                k1, k2, k3 = d_products(st_refs[slot], 0, t, slice(rs * 64, (rs + 1) * 64))
                if t == 0:
                    re, im = jnp.where(first, k3, k2), k1 - jnp.where(first, k2, k3)
                    u = [im[q * 16:(q + 1) * 16] for q in range(4)]
                    sr, dr, tr, er = u[0] + u[2], u[0] - u[2], u[1] + u[3], u[1] - u[3]
                    a2 = sr - tr
                    _, (c1, s1), (c2, s2), (c3, s3) = cs
                    put(16, rs, sr + tr, jnp.zeros_like(sr))
                    put(17, rs, dr * c1 - er * s1, er * (-c1) - dr * s1)
                    put(18, rs, a2 * c2, a2 * (-s2))
                    put(19, rs, dr * c3 + er * s3, er * c3 - dr * s3)
                    im = jnp.where(lane0, 0.0, im)
                else:
                    re, im = k1 + k2, (k3 - k1) * jnp.where(first, 1.0, -1.0)
                a = _dft4([(re[q * 16:(q + 1) * 16], im[q * 16:(q + 1) * 16]) for q in range(4)])
                for jq in range(4):
                    re, im = a[jq]
                    if jq > 0:
                        c, sn = cs[jq]
                        re, im = re * c + im * sn, im * c - re * sn
                    put(t * 4 + jq, rs, re, im)
        return item

    def p2_bfly(u, g, inverse):
        def item(y):
            if y is not None:
                ub_ref[168, pin_rows(0), :] = y
            v = ub_ref[pl.ds(u * 8, 8), g * 16:(g + 1) * 16]
            x = [(v[p, 0:8], v[p, 8:16]) for p in range(8)]
            x = _swap(_dft8(_swap(x))) if inverse else _dft8(x)
            ub_ref[pl.ds(u * 8, 8), g * 16:(g + 1) * 16] = jnp.stack([w for c in x for w in c]).reshape(8, 16, 128)
        return item

    def p2_fwd(u, jps):
        def item(y):
            t = u >> 2
            jq = u & 3
            xs = [_dot(_tobf(ms_ref[jq + 4 * jp]), ub_ref[u * 8 + jp].astype(bf16)) for jp in jps]
            for jp, xx in zip(jps, xs):
                w = wp_ref[pl.ds(t * 2560 + jq + 4 * jp, 64, stride=40), :]
                wr = pltpu.bitcast(w & jnp.uint32(0xFFFF0000), f32).reshape(8, 8, 128)
                wi = pltpu.bitcast(w << 16, f32).reshape(8, 8, 128)
                xx = xx.reshape(8, 2, 8, 128)
                xr, xi = xx[:, 0], xx[:, 1]
                ub_ref[u * 8 + jp] = jnp.stack([xr * wr - xi * wi, xr * wi + xi * wr], axis=1).reshape(128, 128)
        return item

    def p2_inv(u, jps):
        def item(y):
            jq = u & 3
            zs = [_dot(_tobf(ms_ref[32 + jq + 4 * jp]), ub_ref[u * 8 + jp].astype(bf16)) for jp in jps]
            for jp, zz in zip(jps, zs):
                ub_ref[u * 8 + jp] = zz
        return item

    def p3_pre(p, g, t):
        def item(y):
            sa_ref[7, pin_rows(256), :] = y
            cs = twiddles(p)

            def fetch(t):
                a = []
                for jq in range(4):
                    v = ub_ref[(t * 4 + jq) * 8 + p, g * 16:(g + 1) * 16]
                    re, im = v[0:8], v[8:16]
                    if jq > 0:
                        c, sn = cs[jq]
                        re, im = re * c - im * sn, im * c + re * sn
                    a.append((re, im))
                return _swap(_dft4(_swap(a)))

            u = fetch(t)
            if t == 0:
                ny = fetch(4)
                u = [(u[q][0], jnp.where(lane0, ny[q][0], u[q][1])) for q in range(4)]
            first = first_lanes(t)
            for q in range(4):
                re, im = u[q]
                if t == 0:
                    vals = (im, jnp.where(first, re, im), jnp.where(first, im, re))
                else:
                    im = im * jnp.where(first, 1.0, -1.0)
                    vals = (re + im, im, re)
                sa_ref[3 * t:3 * t + 3, q * 64 + g * 8:q * 64 + (g + 1) * 8] = jnp.stack(vals)
        return item

    def p3_mm(p, q):
        def item(y):
            g = []
            for t in range(4):
                k1, k2, k3 = d_products(sa_ref, 1, t, slice(q * 64, (q + 1) * 64))
                g.append((k2 + k1, k3 + k1 if t == 0 else k3 - k1))
            yy = _r8_real_t(g)
            bx_ref[q, pl.ds(pl.multiple_of(p * 64, 64), 64), :] = jnp.concatenate(yy, axis=1).astype(bf16)
        return item

    def b_out(p):
        def item(y):
            rows = pl.ds(pl.multiple_of(p * 64, 64), 64)
            pltpu.make_async_copy(bx_ref.at[0:4, rows, :], out_hbm.at[:, rows, pl.ds(DM, DM)],
                                  sem_out.at[1]).start()
            bx_ref[4, pin_rows(0), 0:128] = y.astype(bf16)
        return item

    def step(pp, odd, mem, hooks):
        r0 = pl.multiple_of(pp * 64 + 32 * odd, SEG)
        xs = xo_ref[pl.ds(r0, SEG), :]
        x_lo = xs[0:8].astype(f32)
        hm = jnp.concatenate(
            [jnp.concatenate([x_lo, jnp.concatenate(mem, axis=1)], axis=0).astype(bf16), xs[16:32]], axis=0)
        fill = fillo_ref[:, 0:64] if odd else fille_ref[:, 0:48]
        nrow = 48 if odd else 32
        qkv, ps = {}, {}

        def do_qkv(h0, h1):
            for h in range(h0, h1):
                for t in range(3):
                    n = t * H + slot_of(h)
                    y32 = _dot(hm, _tobf(w_refs[n // 16][n % 16, 0:512]))
                    y = y32.astype(bf16)
                    parts = [y]
                    if odd or t > 0:
                        parts.append(_tobf(qkvc_ref[pp, n]))
                    if t > 0:
                        if odd:
                            parts.append(_tobf(kve_ref[(t - 1) * H + h]))
                        else:
                            kve_ref[(t - 1) * H + h] = _tou(y[0:16])
                    qkv[(t, h)] = jnp.concatenate(parts, axis=0) if len(parts) > 1 else y
                for item in hooks.get(h, ()):
                    item(y32[0:8])

        def do_s(g):
            for h in range(g * G, (g + 1) * G):
                sc = jax.lax.dot_general(qkv[(0, h)], qkv[(1, h)], (((1,), (1,)), ((), ())),
                                         preferred_element_type=f32)
                sc = jnp.where(fill == 0.0, sc * scale, fill)
                e = jnp.exp(sc - jnp.max(sc, axis=1, keepdims=True))
                den = jnp.sum(e, axis=1, keepdims=True)
                r = pl.reciprocal(den, approx=True)
                r = r * (2.0 - den * r)
                ps[h] = (e * r).astype(bf16)

        def do_pv(g):
            for h in range(g * G, (g + 1) * G):
                oall_ref[0:nrow // 2, h * DH:(h + 1) * DH] = _tou(_dot(ps[h], qkv[(2, h)]).astype(bf16))

        def do_o(j, h0, h1):
            return _dot(_tobf(oall_ref[0:nrow // 2, h0 * DH:h1 * DH]), _tobf(wo_ref[j, h0 * 64:h1 * 64, :]))

        for g in range(NG):
            do_qkv(g * G, g * G + G // 2)
            if g >= 1:
                do_s(g - 1)
            do_qkv(g * G + G // 2, (g + 1) * G)
            if g >= 2:
                do_pv(g - 2)
        part = {}
        for j in range(8):
            items = hooks.get(('o', j), ())
            if len(items) == 1:
                part[j] = do_o(j, 0, OSPLIT)
                items[0](None)
            elif items:
                half = do_o(j, 0, OSPLIT // 2)
                items[0](half[0:8])
                part[j] = do_o(j, OSPLIT // 2, OSPLIT) + half
                items[1](part[j][0:8])
            else:
                part[j] = do_o(j, 0, OSPLIT)
            if j == 2:
                do_s(NG - 1)
                do_pv(NG - 2)
            if j == 5:
                do_pv(NG - 1)
        new_mem = []
        for j in range(8):
            cols = slice(j * 128, (j + 1) * 128)
            res = do_o(j, OSPLIT, H) + part[j]
            new_mem.append(res[8:16])
            if odd:
                xo_ref[pl.ds(r0, SEG), cols] = jnp.concatenate(
                    [res[0:8], res[40:48], res[16:32]], axis=0).astype(bf16)
                xo_ref[pl.ds(r0 - 24, 8), cols] = res[32:40].astype(bf16)
            else:
                xo_ref[pl.ds(r0, SEG), cols] = res.astype(bf16)
        for item in hooks.get(H, ()):
            item(None)
        if odd:
            pltpu.make_async_copy(
                xo_ref.at[pl.ds(pl.multiple_of(pp * 64, 64), 64), :],
                out_hbm.at[pp >> 3, pl.ds(pl.multiple_of((pp & 7) * 64, 64), 64), pl.ds(0, DM)],
                sem_out.at[0]).start()
        return new_mem

    def l1(i, mem):
        he = {h: [p1_pre(2 * i + h // 16, h // 16, (h % 16) // 4, h % 4)] for h in range(32)}
        he[H] = [p1_mm(2 * i, 0, 1)]
        ho = {('o', k): [p1_mm(2 * i + (k + 1) // 4, (k + 1) // 4, t)] for k, t in enumerate((0, 2, 3, 0, 1, 2, 3))}
        mem = step(i, 0, mem, he)
        mem = step(i, 1, mem, ho)
        return mem

    def l2(i, mem):
        u = i - N_L1
        he = {3: [p2_fwd(u, range(0, 4))], 7: [p2_fwd(u, range(4, 8))], H: [p2_inv(u, range(0, 8))]}
        ho = {('o', j): [p2_bfly(u, j, True), p2_bfly(u + 1, j, False)] for j in range(8)}
        mem = step(i, 0, mem, he)
        mem = step(i, 1, mem, ho)
        return mem

    def l3(i, mem):
        p = i - N_L1 - N_L2
        he = {h: [p3_pre(p, h // 4, h % 4)] for h in range(32)}
        he[H] = [p3_mm(p, q) for q in range(4)]
        ho = {12: [b_out(p)]}
        mem = step(i, 0, mem, he)
        mem = step(i, 1, mem, ho)
        return mem

    m0 = mem_ref[...].astype(f32)
    mem = [m0[:, j * 128:(j + 1) * 128] for j in range(8)]
    mem = jax.lax.fori_loop(0, N_L1, l1, mem)
    cp_ms.wait()
    for g in range(8):
        p2_bfly(0, g, False)(None)
    mem = jax.lax.fori_loop(N_L1, N_L1 + N_L2, l2, mem)
    mem = jax.lax.fori_loop(N_L1 + N_L2, NSEG // 2, l3, mem)

    pltpu.make_async_copy(bx_ref.at[0:4], out_hbm.at[:, :, pl.ds(DM, DM)], sem_out.at[1]).wait()
    pltpu.make_async_copy(xo_ref, xo_ref, sem_out.at[0]).wait()


@jax.jit
def _run(x, mem0, wq, wk, wv, wo, bx, w_r, w_i):
    fd, ms = _tables()
    hbm = pl.BlockSpec(memory_space=pl.ANY)
    out = pl.pallas_call(
        _kernel,
        out_shape=jax.ShapeDtypeStruct((4, S // 4, 2 * DM), bf16),
        in_specs=[hbm] * 12,
        out_specs=hbm,
        scratch_shapes=[
            pltpu.VMEM((S, DM), bf16),
            pltpu.VMEM((MEM, DM), bf16),
            pltpu.VMEM((8, NSEG, 8, 128), bf16),
            pltpu.VMEM((4, DM, 16, DH), bf16),
        ] + [pltpu.VMEM((16, DM // 2 + 8, DH), u32)] * 6 + [
            pltpu.VMEM((H * DH, DM), bf16),
            pltpu.VMEM((8, H * DH // 2 + 8, 128), u32),
            pltpu.VMEM((8, 256, 128), u32),
            pltpu.VMEM((NSEG // 2, 3 * H, 8, 128), u32),
            pltpu.VMEM((2 * H, 8, 128), u32),
            pltpu.VMEM((24, H * DH), u32),
            pltpu.VMEM((32, 128), f32),
            pltpu.VMEM((48, 128), f32),
            pltpu.VMEM((5, S // 4, DM), bf16),
            pltpu.VMEM((16, DM // 2 + 1, 256), bf16),
            pltpu.VMEM((12840, 128), u32),
            pltpu.VMEM((169, 128, 128), f32),
            pltpu.VMEM((12, 264, 128), f32),
            pltpu.VMEM((12, 264, 128), f32),
            pltpu.VMEM((24, 64, 128), u32),
            pltpu.VMEM((64, 64, 128), u32),
            pltpu.SMEM((64,), f32),
            pltpu.SMEM((1,), jnp.int32),
            pltpu.SemaphoreType.DMA((64,)),
            pltpu.SemaphoreType.DMA((2,)),
        ],
        compiler_params=pltpu.CompilerParams(vmem_limit_bytes=120 * 1024 * 1024,
                                             disable_semaphore_checks=True,
                                             disable_bounds_checks=True),
    )(x.reshape(S, DM), x.reshape(NSEG, SEG, DM), mem0.reshape(MEM, DM), wq, wk, wv,
      wo.reshape(H * DH, DM), bx.reshape(4, S // 4, DM), w_r.T, w_i.T, jnp.asarray(fd), jnp.asarray(ms))
    return out.reshape(1, S, 2 * DM)


def pallas_concat_heads__memory_aug_recurrent_mem_tr__spectral_gfnet__prompt_kernel(
    A_x: jax.Array,
    A_mem0: jax.Array,
    A_Wq: jax.Array,
    A_Wk: jax.Array,
    A_Wv: jax.Array,
    A_Wo: jax.Array,
    A_seg_len,
    B_x: jax.Array,
    B_w_r: jax.Array,
    B_w_i: jax.Array,
):
    if isinstance(A_seg_len, int):
        assert A_seg_len == SEG
    assert A_x.shape == (1, S, DM) and A_mem0.shape == (1, MEM, DM) and A_Wq.shape == (DM, H, DH)
    assert B_x.shape == (1, S, DM) and B_w_r.shape == (S, DM // 2 + 1)
    return _run(A_x, A_mem0, A_Wq, A_Wk, A_Wv, A_Wo, B_x, B_w_r, B_w_i)
```

```python
import math

import numpy as np
import jax
import jax.numpy as jnp
import jax.experimental.pallas as pl
import jax.experimental.pallas.tpu as pltpu

bf16 = jnp.bfloat16
f32 = jnp.float32
u32 = jnp.uint32

S, DM = 2048, 1024
H, DH = 32, 128
MEM, SEG = 8, 32
NSEG = S // SEG
SQH = math.sqrt(0.5)

_PAIRS = ((0, 4), (1, 7), (2, 6), (3, 5))
_FIRST = np.array([[1, 1, 0, 0], [1, 0, 1, 0], [0, 1, 1, 0], [0, 1, 0, 1]], bool)


def _pack_rows(a):
    u = np.ascontiguousarray(a, dtype=np.float32).view(np.uint32).astype(np.uint64)
    b = ((u + 0x7FFF + ((u >> 16) & 1)) >> 16).astype(np.uint32)
    return (b[..., 0::2, :] | (b[..., 1::2, :] << 16)).astype(np.uint32)


def _tables():
    k2 = np.zeros((4, 128), np.int64)
    for t in range(4):
        odd = t % 2
        for lam in range(128):
            k = 2 * lam + odd
            if k % 8 not in _PAIRS[t]:
                k = 2 * (128 + 8 * (lam // 8) + (lam % 8 - 1 - odd) % 8) + odd
            assert k % 8 in _PAIRS[t]
            k2[t, lam] = k
    b = np.arange(128)[:, None]
    F = np.zeros((12, 128, 128))
    G = np.zeros((12, 128, 128))
    for t in range(4):
        th = 2 * np.pi * ((b * k2[t][None, :]) % DM) / DM
        C, Sn = np.cos(th), np.sin(th)
        first = ((k2[t] % 8) == _PAIRS[t][0])[None, :]
        assert np.array_equal(first[0], _FIRST[t][np.arange(128) % 4])
        if t == 0:
            im = -Sn
            im[:, 0] = (-1.0) ** np.arange(128)
            im = np.roll(im, 2, axis=1)
            F[1:3] = np.where(first, im, C), np.where(first, C, im)
            G[1:3] = F[1:3]
            G[2, :, 0] *= 0.5
            G[2, :, 2] *= 0.5
        else:
            Sg = np.where(first, Sn, -Sn)
            F[3 * t:3 * t + 3] = C, -(C + Sg), C - Sg
            G[3 * t:3 * t + 3] = F[3 * t:3 * t + 3]
    Finv = np.transpose(G, (0, 2, 1)) * (2.0 / DM)
    fd = _pack_rows(np.concatenate([F, Finv]))
    M = np.zeros((32, 128, 128))
    r = np.arange(64)[None, :]
    l = np.arange(64)[:, None]
    for j in range(32):
        th = 2 * np.pi * ((r * (j + 32 * l)) % S) / S
        C, Sn = np.cos(th), np.sin(th)
        M[j, :64, :64] = C
        M[j, :64, 64:] = Sn
        M[j, 64:, :64] = -Sn
        M[j, 64:, 64:] = C
    perm = np.arange(128).reshape(2, 8, 8).transpose(1, 0, 2).reshape(128)
    M = M[:, perm][:, :, perm]
    Minv = np.transpose(M, (0, 2, 1)) / S
    ms = _pack_rows(np.concatenate([M, Minv]))
    return fd, ms


def _tobf(w):
    return pltpu.bitcast(w, bf16)


def _tou(w):
    return pltpu.bitcast(w, u32)


def _dot(a, b):
    return jnp.dot(a, b, preferred_element_type=f32)


def _r8_real(x):
    t0, t1 = x[0] + x[4], x[0] - x[4]
    t2, t3 = x[2] + x[6], x[2] - x[6]
    t4, t5 = x[1] + x[5], x[1] - x[5]
    t6, t7 = x[3] + x[7], x[3] - x[7]
    e0, e1 = t0 + t2, t0 - t2
    o0, o1 = t4 + t6, t4 - t6
    u, v = SQH * (t5 - t7), SQH * (t5 + t7)
    return [(e0 + o0, e0 - o0), (t1 + u, v + t3), (e1, o1), (t1 - u, v - t3)]


def _r8_real_t(g):
    (z0, z4), (a1, b1), (e1, o1), (a3, b3) = g
    e0, o0 = z0 + z4, z0 - z4
    t1, u = a1 + a3, a1 - a3
    v, t3 = b1 + b3, b1 - b3
    t5, t7 = SQH * (v + u), SQH * (v - u)
    t0, t2 = e0 + e1, e0 - e1
    t4, t6 = o0 + o1, o0 - o1
    return [t0 + t1, t4 + t5, t2 + t3, t6 + t7, t0 - t1, t4 - t5, t2 - t3, t6 - t7]


def _dft4(u):
    (r0, i0), (r1, i1), (r2, i2), (r3, i3) = u
    sr, si, dr, di = r0 + r2, i0 + i2, r0 - r2, i0 - i2
    tr, ti, er, ei = r1 + r3, i1 + i3, r1 - r3, i1 - i3
    return [(sr + tr, si + ti), (dr + ei, di - er), (sr - tr, si - ti), (dr - ei, di + er)]


def _dft8(x):
    a = [(x[p][0] + x[p + 4][0], x[p][1] + x[p + 4][1]) for p in range(4)]
    d = [(x[p][0] - x[p + 4][0], x[p][1] - x[p + 4][1]) for p in range(4)]
    ev = _dft4(a)
    (r0, i0), (r1, i1), (r2, i2), (r3, i3) = d
    b1r, b1i = SQH * (r1 + i1), SQH * (i1 - r1)
    b3r, n3i = SQH * (i3 - r3), SQH * (r3 + i3)
    sr, si, dr, di = r0 + i2, i0 - r2, r0 - i2, i0 + r2
    tr, ti, er, ei = b1r + b3r, b1i - n3i, b1r - b3r, b1i + n3i
    od = [(sr + tr, si + ti), (dr + ei, di - er), (sr - tr, si - ti), (dr - ei, di + er)]
    return [ev[0], od[0], ev[1], od[1], ev[2], od[2], ev[3], od[3]]


def _swap(x):
    return [(b, a) for (a, b) in x]


G = 4
NG = H // G
OSPLIT = 24
NEG = -1e9
N_L1, N_L2, N_L3 = 4, 20, 8


def _kernel(x_hbm, x3_hbm, mem_hbm, wq_hbm, wk_hbm, wv_hbm, wo_hbm, bx_hbm, wr_hbm, wi_hbm,
            fd_hbm, ms_hbm, out_hbm,
            xo_ref, mem_ref, xcraw_ref, raw_ref, w0_ref, w1_ref, w2_ref, w3_ref, w4_ref, w5_ref,
            woraw_ref, wo_ref, xc_ref, qkvc_ref, kve_ref,
            oall_ref, fille_ref, fillo_ref, bx_ref, wt_ref, wp_ref, ub_ref, sa_ref, sb_ref, fd_ref, ms_ref,
            tw_ref, zero_ref, sem_in, sem_out):
    scale = DH ** -0.5
    w_hbm = (wq_hbm, wk_hbm, wv_hbm)
    w_refs = (w0_ref, w1_ref, w2_ref, w3_ref, w4_ref, w5_ref)

    def raw_copy(c, i=0, nd=DM):
        rows = pl.ds(pl.multiple_of(i * nd, nd), nd)
        return pltpu.make_async_copy(
            w_hbm[c // 2].at[rows, pl.ds((c % 2) * 16, 16), :],
            raw_ref.at[c % 4, rows], sem_in.at[8 + min(c, 3) * 8 + max(c - 3, 0) * 2 + i])

    def xc_copy(k):
        return pltpu.make_async_copy(
            x3_hbm.at[:, pl.ds(8, 8), pl.ds(pl.multiple_of(k * 128, 128), 128)], xcraw_ref.at[k], sem_in.at[40 + k])

    cp_x = pltpu.make_async_copy(x_hbm, xo_ref, sem_in.at[0])
    cp_mem = pltpu.make_async_copy(mem_hbm, mem_ref, sem_in.at[1])
    cp_wo = pltpu.make_async_copy(wo_hbm, woraw_ref, sem_in.at[2])
    cp_bx = pltpu.make_async_copy(bx_hbm, bx_ref.at[0:4], sem_in.at[3])
    cp_fd = pltpu.make_async_copy(fd_hbm, fd_ref, sem_in.at[4])
    cp_ms = pltpu.make_async_copy(ms_hbm, ms_ref, sem_in.at[5])
    cp_wt = [pltpu.make_async_copy(src.at[:, pl.ds(lg * 256, 256)], wt_ref.at[a * 8 + lg], sem_in.at[48 + a * 8 + lg])
             for a, src in enumerate((wr_hbm, wi_hbm)) for lg in range(8)]

    for i in range(8):
        raw_copy(0, i, 128).start()
        xc_copy(i).start()
        if i >= 3:
            raw_copy(2, i - 3, 128).start()
        if i == 7:
            raw_copy(2, 5, 128).start()
        raw_copy(1, i, 128).start()
    for i in range(6, 8):
        raw_copy(2, i, 128).start()
    for i in range(2):
        raw_copy(3, i, 512).start()
    for cp in cp_wt + [cp_wo, cp_x, cp_mem, cp_bx, cp_fd, cp_ms]:
        cp.start(priority=1)

    zero_ref[0] = 0

    def pin_rows(r):
        return pl.ds(pl.multiple_of(r + zero_ref[0] * 32, 8), 8)

    for p in range(8):
        for jq in range(4):
            tw_ref[(p * 4 + jq) * 2] = jnp.float32(math.cos(2 * math.pi * p * jq / 32))
            tw_ref[(p * 4 + jq) * 2 + 1] = jnp.float32(math.sin(2 * math.pi * p * jq / 32))

    qi = jax.lax.broadcasted_iota(jnp.int32, (48, 128), 0)
    ki = jax.lax.broadcasted_iota(jnp.int32, (48, 128), 1)

    def between(v, lo, hi):
        return (v >= lo) & (v < hi)

    def table(keep, other):
        return jnp.where(other, -jnp.inf, jnp.where(keep, 0.0, NEG)).astype(f32)

    keep = between(qi, 8, 16) | between(ki, 8, 16) | (qi >= jnp.where(ki < 32, ki, ki - 24))
    fille_ref[...] = table(keep, ki >= 40)[:32]
    q_even = between(qi, 32, 40)
    k_even = between(ki, 32, 40) | (ki >= 48)
    qpos = jnp.where(qi < 32, qi, jnp.where(qi < 40, qi - 24, qi - 32))
    kpos = jnp.where(ki < 32, ki, jnp.where(ki < 40, ki - 24, jnp.where(ki < 48, ki - 32, ki - 48)))
    keep = between(qi, 8, 16) | between(ki, 8, 16) | (ki >= 56) | (qpos >= kpos)
    fillo_ref[...] = table(keep, (q_even != k_even) | (ki >= 64))

    def relayout16(c, blk):
        w0 = pl.multiple_of(blk * 8, 8)
        v = _tou(raw_ref[c % 4, pl.ds(blk * 16, 16)]).reshape(8, 2, 8, 128)
        a, b = v[:, 0], v[:, 1]
        w_refs[c][0:8, pl.ds(w0, 8), :] = jnp.swapaxes((a & jnp.uint32(0xFFFF)) | (b << 16), 0, 1)
        w_refs[c][8:16, pl.ds(w0, 8), :] = jnp.swapaxes((a >> 16) | (b & jnp.uint32(0xFFFF0000)), 0, 1)

    def slot_of(h):
        return (h // 16) * 16 + (h % 2) * 8 + (h % 16) // 2

    def repack_wo64(blk):
        v = _tou(woraw_ref[pl.ds(pl.multiple_of(blk * 64, 64), 64), :])
        wo_ref[:, pl.ds(pl.multiple_of(blk * 32, 32), 32), :] = jnp.stack(
            [v[:, j * 128:(j + 1) * 128] for j in range(8)])

    sub4 = jax.lax.broadcasted_iota(jnp.int32, (128, 128), 0) & 3

    def wp_store(t, kb, tile):
        v = tile.T
        for g in range(4):
            r0 = pl.multiple_of(t * 2560 + kb * 160 + g * 40, 8)
            wp_ref[pl.ds(r0, 32), :] = v[g * 32:(g + 1) * 32]

    def b_prep(lg, hb, par):
        cols = slice(hb * 128, (hb + 1) * 128)
        a = _tou(wt_ref[lg, 0:512, cols])
        b = _tou(wt_ref[8 + lg, 0:512, cols])
        if par == 0:
            w = (a << 16) | (b & jnp.uint32(0xFFFF))
            m = (sub4 == 0) | (sub4 == 2)
        else:
            w = (a & jnp.uint32(0xFFFF0000)) | (b >> 16)
            m = (sub4 == 0) | (sub4 == 3)
        top = w[:128]
        bot = pltpu.roll(w[128:].reshape(16, 8, 128), 1 + par, 1).reshape(128, 128)
        wp_store(par, lg * 2 + hb, jnp.where(m, top, bot))
        wp_store(par + 2, lg * 2 + hb, jnp.where(m, bot, top))
        if par == 0:
            na = jnp.broadcast_to(wt_ref[lg, 512:513, cols].astype(f32), (128, 128))
            nb = jnp.broadcast_to(wt_ref[8 + lg, 512:513, cols].astype(f32), (128, 128))
            wp_store(4, lg * 2 + hb, pltpu.bitcast(na, u32) | (pltpu.bitcast(nb, u32) >> 16))

    def gather_c(k):
        xc_ref[k] = _tou(xcraw_ref[k].astype(f32).reshape(512, 128).astype(bf16))

    def store_qkvc(n, y):
        qkvc_ref[:, n] = y.reshape(NSEG // 2, 8, 128)

    def q_unit(i, groups, first, last, fillers):
        xk = _tobf(xc_ref[i])
        w0 = pl.multiple_of(i * 64, 64)
        for g in groups:
            rhs = jnp.concatenate(
                [_tobf(w_refs[h // 16][h % 16, pl.ds(w0, 64), :]) for h in range(4 * g, 4 * g + 4)], axis=1)
            y = _dot(xk, rhs)
            for h in range(4 * g, 4 * g + 4):
                yh = y[:, (h % 4) * 128:(h % 4 + 1) * 128]
                if not first:
                    yh = yh + ub_ref[h * 4:(h + 1) * 4].reshape(512, 128)
                if last:
                    store_qkvc(h, _tou(yh.astype(bf16)))
                else:
                    ub_ref[h * 4:(h + 1) * 4] = yh.reshape(4, 128, 128)
            mine = fillers.get(g, [])
            for fi, item in enumerate(mine):
                r = (fi * 512 // len(mine)) // 8 * 8
                item(pltpu.bitcast(y[r:r + 8, 0:128], u32))

    def rl_item(c, blk):
        def item(pin):
            w_refs[c][15, pin_rows(512), :] = pin
            relayout16(c, blk)
        return item

    def spread(fillers, items, groups):
        for k, item in enumerate(items):
            fillers.setdefault(groups[k * len(groups) // len(items)], []).append(item)
        return fillers

    def half_items(f, c, i, groups):
        return spread(f, [rl_item(c, i * 8 + blk) for blk in range(8)], groups)

    def piece_items(i):
        f = half_items(half_items({}, 1, i, (0, 1, 2)), 0, i + 1, (4, 5, 6))
        return spread(f, [lambda pin: gather_c(i + 1)], (7,))

    def chunk2_items(f, lo, hi, groups):
        return spread(f, [rl_item(2, blk) for blk in range(lo, hi)], groups)

    def wait_piece(i):
        raw_copy(1, i, 128).wait()
        xc_copy(i + 1).wait()
        raw_copy(0, i + 1, 128).wait()

    raw_copy(0, 0, 128).wait()
    for blk in range(8):
        relayout16(0, blk)
    xc_copy(0).wait()
    gather_c(0)
    q_unit(0, range(0, 2), True, False, {})
    raw_copy(1, 0, 128).wait()
    q_unit(0, range(2, 4), True, False, half_items({}, 1, 0, (2, 2, 3)))
    q_unit(0, range(4, 6), True, False, {})
    xc_copy(1).wait()
    raw_copy(0, 1, 128).wait()
    q_unit(0, range(6, 8), True, False,
           spread(half_items({}, 0, 1, (6, 6, 7)), [lambda pin: gather_c(1)], (6,)))
    raw_copy(1, 1, 128).wait()
    q_unit(1, range(0, 4), False, False, half_items({}, 1, 1, (0, 1, 2)))
    xc_copy(2).wait()
    raw_copy(0, 2, 128).wait()
    q_unit(1, range(4, 8), False, False,
           spread(half_items({}, 0, 2, (4, 5, 6)), [lambda pin: gather_c(2)], (6,)))

    def q_c(i, carry):
        wait_piece(i)
        raw_copy(2, i - 2, 128).wait()
        q_unit(i, range(8), False, False, half_items(piece_items(i), 2, i - 2, (3, 3, 3, 3, 4, 5, 6, 7)))
        return carry
    jax.lax.fori_loop(2, 6, q_c, 0)

    wait_piece(6)
    raw_copy(2, 4, 128).wait()
    raw_copy(2, 5, 128).wait()
    q_unit(6, range(8), False, False, chunk2_items(piece_items(6), 32, 48, (0, 1, 2, 3, 3, 4, 5, 6)))
    raw_copy(1, 7, 128).wait()
    raw_copy(2, 6, 128).wait()
    raw_copy(2, 7, 128).wait()
    q_unit(7, range(8), False, True, chunk2_items(half_items({}, 1, 7, (0, 1, 2)), 48, 64, (3, 4, 5, 6)))
    raw_copy(4).start()
    raw_copy(5).start()

    def bulk_iter(c, i):
        xc = jnp.concatenate([_tobf(xc_ref[k]) for k in range(8)], axis=1)
        for t in range(8):
            n = i * 8 + t
            y = _tou(_dot(xc, _tobf(w_refs[c][n, 0:512])).astype(bf16))
            store_qkvc(c * 16 + n, y)
            for blk in range(4):
                pin = y[blk * 64:blk * 64 + 8]
                if c + 1 < 6:
                    w_refs[c + 1][15, pin_rows(512), :] = pin
                    relayout16(c + 1, i * 32 + (t * 4 + blk))
                else:
                    wo_ref[7, pin_rows(2048), :] = pin
                    repack_wo64(i * 32 + (t * 4 + blk))
            if c >= 4:
                wp_ref[pin_rows(12832), :] = y[32:40]
                b_prep((c - 4) * 4 + i * 2 + t // 4, (t // 2) % 2, t % 2)

    for c in range(2, 6):
        if c == 4:
            for cp in cp_wt:
                cp.wait()
        if c == 5:
            cp_wo.wait()
        elif c > 2:
            raw_copy(c + 1).wait()

        def bulk(i, carry, c=c):
            if c == 2:
                raw_copy(3, i, 512).wait()
            bulk_iter(c, i)
            return carry
        jax.lax.fori_loop(0, 2, bulk, 0)

    cp_x.wait()
    cp_mem.wait()
    cp_bx.wait()
    cp_fd.wait()

    lane = jax.lax.broadcasted_iota(jnp.int32, (1, 128), 1)
    lane0 = lane == 0

    def first_lanes(t):
        la, lb = [k for k in range(4) if _FIRST[t][k]]
        return ((lane & 3) == la) | ((lane & 3) == lb)

    def d_products(st_ref, d, t, rows):
        return [_dot(st_ref[n, rows].astype(bf16), _tobf(fd_ref[d * 12 + n])) if n else None
                for n in range(3 * t, 3 * t + 3)]

    def twiddles(p):
        return [(tw_ref[p * 8 + jq * 2], tw_ref[p * 8 + jq * 2 + 1]) if jq else None for jq in range(4)]

    st_refs = (sa_ref, sb_ref)

    def p1_pre(p, slot, rs, q):
        def item(y):
            st_refs[slot][7, pin_rows(256), :] = y
            xq = bx_ref[q, pl.ds(pl.multiple_of(p * 64 + rs * 16, 16), 16), :].astype(f32)
            zz = _r8_real([xq[:, a * 128:(a + 1) * 128] for a in range(8)])
            r = (rs * 4 + q) * 16
            st_refs[slot][1:12, r:r + 16] = jnp.stack([v for (a, b) in zz for v in (a + b, b, a)][1:])
        return item

    def p1_mm(p, slot, t):
        def item(y):
            cs = twiddles(p)

            def put(n, rs, re, im):
                v = jnp.stack([re.reshape(2, 8, 128), im.reshape(2, 8, 128)], axis=1)
                ub_ref[n * 8 + p, rs * 32:(rs + 1) * 32] = v.reshape(32, 128)

            first = first_lanes(t)
            for rs in range(4):
                k1, k2, k3 = d_products(st_refs[slot], 0, t, slice(rs * 64, (rs + 1) * 64))
                if t == 0:
                    re, im = jnp.where(first, k3, k2), pltpu.roll(jnp.where(first, k2, k3), 126, 1)
                    u = [im[q * 16:(q + 1) * 16] for q in range(4)]
                    sr, dr, tr, er = u[0] + u[2], u[0] - u[2], u[1] + u[3], u[1] - u[3]
                    a2 = sr - tr
                    _, (c1, s1), (c2, s2), (c3, s3) = cs
                    put(16, rs, sr + tr, jnp.zeros_like(sr))
                    put(17, rs, dr * c1 - er * s1, er * (-c1) - dr * s1)
                    put(18, rs, a2 * c2, a2 * (-s2))
                    put(19, rs, dr * c3 + er * s3, er * c3 - dr * s3)
                    im = jnp.where(lane0, 0.0, im)
                else:
                    re, im = k1 + k2, (k3 - k1) * jnp.where(first, 1.0, -1.0)
                a = _dft4([(re[q * 16:(q + 1) * 16], im[q * 16:(q + 1) * 16]) for q in range(4)])
                for jq in range(4):
                    re, im = a[jq]
                    if jq > 0:
                        c, sn = cs[jq]
                        re, im = re * c + im * sn, im * c - re * sn
                    put(t * 4 + jq, rs, re, im)
        return item

    def p2_bfly(u, g, inverse):
        def item(y):
            if y is not None:
                ub_ref[168, pin_rows(0), :] = y
            v = ub_ref[pl.ds(u * 8, 8), g * 16:(g + 1) * 16]
            x = [(v[p, 0:8], v[p, 8:16]) for p in range(8)]
            x = _swap(_dft8(_swap(x))) if inverse else _dft8(x)
            ub_ref[pl.ds(u * 8, 8), g * 16:(g + 1) * 16] = jnp.stack([w for c in x for w in c]).reshape(8, 16, 128)
        return item

    def p2_fwd(u, jps):
        def item(y):
            t = u >> 2
            jq = u & 3
            xs = [_dot(_tobf(ms_ref[jq + 4 * jp]), ub_ref[u * 8 + jp].astype(bf16)) for jp in jps]
            for jp, xx in zip(jps, xs):
                w = wp_ref[pl.ds(t * 2560 + jq + 4 * jp, 64, stride=40), :]
                wr = pltpu.bitcast(w & jnp.uint32(0xFFFF0000), f32).reshape(8, 8, 128)
                wi = pltpu.bitcast(w << 16, f32).reshape(8, 8, 128)
                xx = xx.reshape(8, 2, 8, 128)
                xr, xi = xx[:, 0], xx[:, 1]
                ub_ref[u * 8 + jp] = jnp.stack([xr * wr - xi * wi, xr * wi + xi * wr], axis=1).reshape(128, 128)
        return item

    def p2_inv(u, jps):
        def item(y):
            jq = u & 3
            zs = [_dot(_tobf(ms_ref[32 + jq + 4 * jp]), ub_ref[u * 8 + jp].astype(bf16)) for jp in jps]
            for jp, zz in zip(jps, zs):
                ub_ref[u * 8 + jp] = zz
        return item

    def p3_pre(p, g, t):
        def item(y):
            sa_ref[7, pin_rows(256), :] = y
            cs = twiddles(p)

            def fetch(t):
                a = []
                for jq in range(4):
                    v = ub_ref[(t * 4 + jq) * 8 + p, g * 16:(g + 1) * 16]
                    re, im = v[0:8], v[8:16]
                    if jq > 0:
                        c, sn = cs[jq]
                        re, im = re * c - im * sn, im * c + re * sn
                    a.append((re, im))
                return _swap(_dft4(_swap(a)))

            u = fetch(t)
            if t == 0:
                ny = fetch(4)
                u = [(u[q][0], jnp.where(lane0, ny[q][0], u[q][1])) for q in range(4)]
            first = first_lanes(t)
            for q in range(4):
                re, im = u[q]
                rows = slice(q * 64 + g * 8, q * 64 + (g + 1) * 8)
                if t == 0:
                    im = pltpu.roll(im, 2, 1)
                    sa_ref[1:3, rows] = jnp.stack((jnp.where(first, im, re), jnp.where(first, re, im)))
                else:
                    im = im * jnp.where(first, 1.0, -1.0)
                    sa_ref[3 * t:3 * t + 3, rows] = jnp.stack((re + im, im, re))
        return item

    def p3_mm(p, q):
        def item(y):
            g = []
            for t in range(4):
                k1, k2, k3 = d_products(sa_ref, 1, t, slice(q * 64, (q + 1) * 64))
                g.append((k3, k2) if t == 0 else (k2 + k1, k3 - k1))
            yy = _r8_real_t(g)
            bx_ref[q, pl.ds(pl.multiple_of(p * 64, 64), 64), :] = jnp.concatenate(yy, axis=1).astype(bf16)
        return item

    def b_out(p):
        def item(y):
            rows = pl.ds(pl.multiple_of(p * 64, 64), 64)
            pltpu.make_async_copy(bx_ref.at[0:4, rows, :], out_hbm.at[:, rows, pl.ds(DM, DM)],
                                  sem_out.at[1]).start()
            bx_ref[4, pin_rows(0), 0:128] = y.astype(bf16)
        return item

    def step(pp, odd, mem, hooks):
        r0 = pl.multiple_of(pp * 64 + 32 * odd, SEG)
        xs = xo_ref[pl.ds(r0, SEG), :]
        x_lo = xs[0:8].astype(f32)
        hm = jnp.concatenate(
            [jnp.concatenate([x_lo, jnp.concatenate(mem, axis=1)], axis=0).astype(bf16), xs[16:32]], axis=0)
        fill = fillo_ref[:, 0:64] if odd else fille_ref[:, 0:48]
        nrow = 48 if odd else 32
        qkv, ps = {}, {}

        def do_qkv(h0, h1):
            for h in range(h0, h1):
                for t in range(3):
                    n = t * H + slot_of(h)
                    y32 = _dot(hm, _tobf(w_refs[n // 16][n % 16, 0:512]))
                    y = y32.astype(bf16)
                    parts = [y]
                    if odd or t > 0:
                        parts.append(_tobf(qkvc_ref[pp, n]))
                    if t > 0:
                        if odd:
                            parts.append(_tobf(kve_ref[(t - 1) * H + h]))
                        else:
                            kve_ref[(t - 1) * H + h] = _tou(y[0:16])
                    qkv[(t, h)] = jnp.concatenate(parts, axis=0) if len(parts) > 1 else y
                for item in hooks.get(h, ()):
                    item(y32[0:8])

        def do_s(g):
            for h in range(g * G, (g + 1) * G):
                sc = jax.lax.dot_general(qkv[(0, h)], qkv[(1, h)], (((1,), (1,)), ((), ())),
                                         preferred_element_type=f32)
                sc = jnp.where(fill == 0.0, sc * scale, fill)
                e = jnp.exp(sc - jnp.max(sc, axis=1, keepdims=True))
                den = jnp.sum(e, axis=1, keepdims=True)
                r = pl.reciprocal(den, approx=True)
                r = r * (2.0 - den * r)
                ps[h] = (e * r).astype(bf16)

        def do_pv(g):
            for h in range(g * G, (g + 1) * G):
                oall_ref[0:nrow // 2, h * DH:(h + 1) * DH] = _tou(_dot(ps[h], qkv[(2, h)]).astype(bf16))

        def do_o(j, h0, h1):
            return _dot(_tobf(oall_ref[0:nrow // 2, h0 * DH:h1 * DH]), _tobf(wo_ref[j, h0 * 64:h1 * 64, :]))

        for g in range(NG):
            do_qkv(g * G, g * G + G // 2)
            if g >= 1:
                do_s(g - 1)
            do_qkv(g * G + G // 2, (g + 1) * G)
            if g >= 2:
                do_pv(g - 2)
        part = {}
        for j in range(8):
            items = hooks.get(('o', j), ())
            if len(items) == 1:
                part[j] = do_o(j, 0, OSPLIT)
                items[0](None)
            elif items:
                half = do_o(j, 0, OSPLIT // 2)
                items[0](half[0:8])
                part[j] = do_o(j, OSPLIT // 2, OSPLIT) + half
                items[1](part[j][0:8])
            else:
                part[j] = do_o(j, 0, OSPLIT)
            if j == 2:
                do_s(NG - 1)
                do_pv(NG - 2)
            if j == 5:
                do_pv(NG - 1)
        new_mem = []
        for j in range(8):
            cols = slice(j * 128, (j + 1) * 128)
            res = do_o(j, OSPLIT, H) + part[j]
            new_mem.append(res[8:16])
            if odd:
                xo_ref[pl.ds(r0, SEG), cols] = jnp.concatenate(
                    [res[0:8], res[40:48], res[16:32]], axis=0).astype(bf16)
                xo_ref[pl.ds(r0 - 24, 8), cols] = res[32:40].astype(bf16)
            else:
                xo_ref[pl.ds(r0, SEG), cols] = res.astype(bf16)
        for item in hooks.get(H, ()):
            item(None)
        if odd:
            pltpu.make_async_copy(
                xo_ref.at[pl.ds(pl.multiple_of(pp * 64, 64), 64), :],
                out_hbm.at[pp >> 3, pl.ds(pl.multiple_of((pp & 7) * 64, 64), 64), pl.ds(0, DM)],
                sem_out.at[0]).start()
        return new_mem

    def l1(i, mem):
        he = {h: [p1_pre(2 * i + h // 16, h // 16, (h % 16) // 4, h % 4)] for h in range(32)}
        he[H] = [p1_mm(2 * i, 0, 1)]
        ho = {('o', k): [p1_mm(2 * i + u, u, t)]
              for k, (u, t) in enumerate(((0, 2), (0, 3), (1, 1), (1, 2), (0, 0), (1, 3), (1, 0)))}
        mem = step(i, 0, mem, he)
        mem = step(i, 1, mem, ho)
        return mem

    def l2(i, mem):
        u = i - N_L1
        he = {3: [p2_fwd(u, range(0, 4))], 7: [p2_fwd(u, range(4, 8))], H: [p2_inv(u, range(0, 8))]}
        ho = {('o', j): [p2_bfly(u, j, True), p2_bfly(u + 1, j, False)] for j in range(8)}
        mem = step(i, 0, mem, he)
        mem = step(i, 1, mem, ho)
        return mem

    def l3(i, mem):
        p = i - N_L1 - N_L2
        he = {h: [p3_pre(p, h // 3, 1 + h % 3)] for h in range(24)}
        for j in range(4):
            he[('o', 3 + j)] = [p3_pre(p, 2 * j, 0), p3_pre(p, 2 * j + 1, 0)]
        he[H] = [p3_mm(p, q) for q in range(4)]
        ho = {12: [b_out(p)]}
        mem = step(i, 0, mem, he)
        mem = step(i, 1, mem, ho)
        return mem

    m0 = mem_ref[...].astype(f32)
    mem = [m0[:, j * 128:(j + 1) * 128] for j in range(8)]
    mem = jax.lax.fori_loop(0, N_L1, l1, mem)
    cp_ms.wait()
    for g in range(8):
        p2_bfly(0, g, False)(None)
    mem = jax.lax.fori_loop(N_L1, N_L1 + N_L2, l2, mem)
    mem = jax.lax.fori_loop(N_L1 + N_L2, NSEG // 2, l3, mem)

    pltpu.make_async_copy(bx_ref.at[0:4], out_hbm.at[:, :, pl.ds(DM, DM)], sem_out.at[1]).wait()
    pltpu.make_async_copy(xo_ref, xo_ref, sem_out.at[0]).wait()


@jax.jit
def _run(x, mem0, wq, wk, wv, wo, bx, w_r, w_i):
    fd, ms = _tables()
    hbm = pl.BlockSpec(memory_space=pl.ANY)
    out = pl.pallas_call(
        _kernel,
        out_shape=jax.ShapeDtypeStruct((4, S // 4, 2 * DM), bf16),
        in_specs=[hbm] * 12,
        out_specs=hbm,
        scratch_shapes=[
            pltpu.VMEM((S, DM), bf16),
            pltpu.VMEM((MEM, DM), bf16),
            pltpu.VMEM((8, NSEG, 8, 128), bf16),
            pltpu.VMEM((4, DM, 16, DH), bf16),
        ] + [pltpu.VMEM((16, DM // 2 + 8, DH), u32)] * 6 + [
            pltpu.VMEM((H * DH, DM), bf16),
            pltpu.VMEM((8, H * DH // 2 + 8, 128), u32),
            pltpu.VMEM((8, 256, 128), u32),
            pltpu.VMEM((NSEG // 2, 3 * H, 8, 128), u32),
            pltpu.VMEM((2 * H, 8, 128), u32),
            pltpu.VMEM((24, H * DH), u32),
            pltpu.VMEM((32, 128), f32),
            pltpu.VMEM((48, 128), f32),
            pltpu.VMEM((5, S // 4, DM), bf16),
            pltpu.VMEM((16, DM // 2 + 1, 256), bf16),
            pltpu.VMEM((12840, 128), u32),
            pltpu.VMEM((169, 128, 128), f32),
            pltpu.VMEM((12, 264, 128), f32),
            pltpu.VMEM((12, 264, 128), f32),
            pltpu.VMEM((24, 64, 128), u32),
            pltpu.VMEM((64, 64, 128), u32),
            pltpu.SMEM((64,), f32),
            pltpu.SMEM((1,), jnp.int32),
            pltpu.SemaphoreType.DMA((64,)),
            pltpu.SemaphoreType.DMA((2,)),
        ],
        compiler_params=pltpu.CompilerParams(vmem_limit_bytes=120 * 1024 * 1024,
                                             disable_semaphore_checks=True,
                                             disable_bounds_checks=True),
    )(x.reshape(S, DM), x.reshape(NSEG, SEG, DM), mem0.reshape(MEM, DM), wq, wk, wv,
      wo.reshape(H * DH, DM), bx.reshape(4, S // 4, DM), w_r.T, w_i.T, jnp.asarray(fd), jnp.asarray(ms))
    return out.reshape(1, S, 2 * DM)


def pallas_concat_heads__memory_aug_recurrent_mem_tr__spectral_gfnet__prompt_kernel(
    A_x: jax.Array,
    A_mem0: jax.Array,
    A_Wq: jax.Array,
    A_Wk: jax.Array,
    A_Wv: jax.Array,
    A_Wo: jax.Array,
    A_seg_len,
    B_x: jax.Array,
    B_w_r: jax.Array,
    B_w_i: jax.Array,
):
    if isinstance(A_seg_len, int):
        assert A_seg_len == SEG
    assert A_x.shape == (1, S, DM) and A_mem0.shape == (1, MEM, DM) and A_Wq.shape == (DM, H, DH)
    assert B_x.shape == (1, S, DM) and B_w_r.shape == (S, DM // 2 + 1)
    return _run(A_x, A_mem0, A_Wq, A_Wk, A_Wv, A_Wo, B_x, B_w_r, B_w_i)
```

```python
import math

import numpy as np
import jax
import jax.numpy as jnp
import jax.experimental.pallas as pl
import jax.experimental.pallas.tpu as pltpu

bf16 = jnp.bfloat16
f32 = jnp.float32
u32 = jnp.uint32

S, DM = 2048, 1024
H, DH = 32, 128
MEM, SEG = 8, 32
NSEG = S // SEG
SQH = math.sqrt(0.5)

_PAIRS = ((0, 4), (1, 7), (2, 6), (3, 5))
_FIRST = np.array([[1, 1, 0, 0], [1, 0, 1, 0], [0, 1, 1, 0], [0, 1, 0, 1]], bool)


def _pack_rows(a):
    u = np.ascontiguousarray(a, dtype=np.float32).view(np.uint32).astype(np.uint64)
    b = ((u + 0x7FFF + ((u >> 16) & 1)) >> 16).astype(np.uint32)
    return (b[..., 0::2, :] | (b[..., 1::2, :] << 16)).astype(np.uint32)


def _tables():
    k2 = np.zeros((4, 128), np.int64)
    for t in range(4):
        odd = t % 2
        for lam in range(128):
            k = 2 * lam + odd
            if k % 8 not in _PAIRS[t]:
                k = 2 * (128 + 8 * (lam // 8) + (lam % 8 - 1 - odd) % 8) + odd
            assert k % 8 in _PAIRS[t]
            k2[t, lam] = k
    b = np.arange(128)[:, None]
    F = np.zeros((12, 128, 128))
    G = np.zeros((12, 128, 128))
    for t in range(4):
        th = 2 * np.pi * ((b * k2[t][None, :]) % DM) / DM
        C, Sn = np.cos(th), np.sin(th)
        first = ((k2[t] % 8) == _PAIRS[t][0])[None, :]
        assert np.array_equal(first[0], _FIRST[t][np.arange(128) % 4])
        if t == 0:
            im = -Sn
            im[:, 0] = (-1.0) ** np.arange(128)
            im = np.roll(im, 2, axis=1)
            F[1:3] = np.where(first, im, C), np.where(first, C, im)
            G[1:3] = F[1:3]
            G[2, :, 0] *= 0.5
            G[2, :, 2] *= 0.5
        else:
            Sg = np.where(first, Sn, -Sn)
            F[3 * t:3 * t + 3] = C, -(C + Sg), C - Sg
            G[3 * t:3 * t + 3] = F[3 * t:3 * t + 3]
    Finv = np.transpose(G, (0, 2, 1)) * (2.0 / DM)
    fd = _pack_rows(np.concatenate([F, Finv]))
    M = np.zeros((32, 128, 128))
    r = np.arange(64)[None, :]
    l = np.arange(64)[:, None]
    for j in range(32):
        th = 2 * np.pi * ((r * (j + 32 * l)) % S) / S
        C, Sn = np.cos(th), np.sin(th)
        M[j, :64, :64] = C
        M[j, :64, 64:] = Sn
        M[j, 64:, :64] = -Sn
        M[j, 64:, 64:] = C
    perm = np.arange(128).reshape(2, 8, 8).transpose(1, 0, 2).reshape(128)
    M = M[:, perm][:, :, perm]
    Minv = np.transpose(M, (0, 2, 1)) / S
    ms = _pack_rows(np.concatenate([M, Minv]))
    th = 2 * np.pi * np.outer(np.arange(512), np.arange(128) % 4) / S
    tv = np.stack([np.cos(th), np.sin(th)]).astype(np.float32)
    return fd, ms, tv


def _tobf(w):
    return pltpu.bitcast(w, bf16)


def _tou(w):
    return pltpu.bitcast(w, u32)


def _dot(a, b):
    return jnp.dot(a, b, preferred_element_type=f32)


def _r8_real(x):
    t0, t1 = x[0] + x[4], x[0] - x[4]
    t2, t3 = x[2] + x[6], x[2] - x[6]
    t4, t5 = x[1] + x[5], x[1] - x[5]
    t6, t7 = x[3] + x[7], x[3] - x[7]
    e0, e1 = t0 + t2, t0 - t2
    o0, o1 = t4 + t6, t4 - t6
    u, v = SQH * (t5 - t7), SQH * (t5 + t7)
    return [(e0 + o0, e0 - o0), (t1 + u, v + t3), (e1, o1), (t1 - u, v - t3)]


def _r8_real_t(g):
    (z0, z4), (a1, b1), (e1, o1), (a3, b3) = g
    e0, o0 = z0 + z4, z0 - z4
    t1, u = a1 + a3, a1 - a3
    v, t3 = b1 + b3, b1 - b3
    t5, t7 = SQH * (v + u), SQH * (v - u)
    t0, t2 = e0 + e1, e0 - e1
    t4, t6 = o0 + o1, o0 - o1
    return [t0 + t1, t4 + t5, t2 + t3, t6 + t7, t0 - t1, t4 - t5, t2 - t3, t6 - t7]


def _dft4(u):
    (r0, i0), (r1, i1), (r2, i2), (r3, i3) = u
    sr, si, dr, di = r0 + r2, i0 + i2, r0 - r2, i0 - i2
    tr, ti, er, ei = r1 + r3, i1 + i3, r1 - r3, i1 - i3
    return [(sr + tr, si + ti), (dr + ei, di - er), (sr - tr, si - ti), (dr - ei, di + er)]


def _dft8(x):
    a = [(x[p][0] + x[p + 4][0], x[p][1] + x[p + 4][1]) for p in range(4)]
    d = [(x[p][0] - x[p + 4][0], x[p][1] - x[p + 4][1]) for p in range(4)]
    ev = _dft4(a)
    (r0, i0), (r1, i1), (r2, i2), (r3, i3) = d
    b1r, b1i = SQH * (r1 + i1), SQH * (i1 - r1)
    b3r, n3i = SQH * (i3 - r3), SQH * (r3 + i3)
    sr, si, dr, di = r0 + i2, i0 - r2, r0 - i2, i0 + r2
    tr, ti, er, ei = b1r + b3r, b1i - n3i, b1r - b3r, b1i + n3i
    od = [(sr + tr, si + ti), (dr + ei, di - er), (sr - tr, si - ti), (dr - ei, di + er)]
    return [ev[0], od[0], ev[1], od[1], ev[2], od[2], ev[3], od[3]]


def _swap(x):
    return [(b, a) for (a, b) in x]


G = 4
NG = H // G
OSPLIT = 24
NEG = -1e9
NYQ = 17
N_L1, N_L2, N_L3 = 8, 16, 8


def _kernel(x_hbm, x3_hbm, mem_hbm, wq_hbm, wk_hbm, wv_hbm, wo_hbm, bx_hbm, wr_hbm, wi_hbm,
            fd_hbm, ms_hbm, tv_hbm, out_hbm,
            xo_ref, mem_ref, xcraw_ref, raw_ref, w0_ref, w1_ref, w2_ref, w3_ref, w4_ref, w5_ref,
            woraw_ref, wo_ref, xc_ref, qkvc_ref, kve_ref,
            oall_ref, fille_ref, fillo_ref, bx_ref, wt_ref, wp_ref, ub_ref, sa_ref, fd_ref, ms_ref, tv_ref,
            tw_ref, zero_ref, sem_in, sem_out):
    scale = DH ** -0.5
    w_hbm = (wq_hbm, wk_hbm, wv_hbm)
    w_refs = (w0_ref, w1_ref, w2_ref, w3_ref, w4_ref, w5_ref)

    def raw_copy(c, i=0, nd=DM):
        rows = pl.ds(pl.multiple_of(i * nd, nd), nd)
        return pltpu.make_async_copy(
            w_hbm[c // 2].at[rows, pl.ds((c % 2) * 16, 16), :],
            raw_ref.at[c % 4, rows], sem_in.at[8 + min(c, 3) * 8 + max(c - 3, 0) * 2 + i])

    def xc_copy(k):
        return pltpu.make_async_copy(
            x3_hbm.at[:, pl.ds(8, 8), pl.ds(pl.multiple_of(k * 128, 128), 128)], xcraw_ref.at[k], sem_in.at[40 + k])

    cp_x = pltpu.make_async_copy(x_hbm, xo_ref, sem_in.at[0])
    cp_mem = pltpu.make_async_copy(mem_hbm, mem_ref, sem_in.at[1])
    cp_wo = pltpu.make_async_copy(wo_hbm, woraw_ref, sem_in.at[2])
    cp_bx = pltpu.make_async_copy(bx_hbm, bx_ref.at[0:4], sem_in.at[3])
    cp_fd = pltpu.make_async_copy(fd_hbm, fd_ref, sem_in.at[4])
    cp_ms = pltpu.make_async_copy(ms_hbm, ms_ref, sem_in.at[5])
    cp_tv = pltpu.make_async_copy(tv_hbm, tv_ref, sem_in.at[6])
    cp_wt = [pltpu.make_async_copy(src.at[:, pl.ds(lg * 256, 256)], wt_ref.at[a * 8 + lg], sem_in.at[48 + a * 8 + lg])
             for a, src in enumerate((wr_hbm, wi_hbm)) for lg in range(8)]

    for i in range(8):
        raw_copy(0, i, 128).start()
        xc_copy(i).start()
        if i >= 3:
            raw_copy(2, i - 3, 128).start()
        if i == 7:
            raw_copy(2, 5, 128).start()
        raw_copy(1, i, 128).start()
    for i in range(6, 8):
        raw_copy(2, i, 128).start()
    for i in range(2):
        raw_copy(3, i, 512).start()
    for cp in cp_wt + [cp_wo, cp_x, cp_mem, cp_bx, cp_fd, cp_tv, cp_ms]:
        cp.start(priority=1)

    zero_ref[0] = 0

    def pin_rows(r):
        return pl.ds(pl.multiple_of(r + zero_ref[0] * 32, 8), 8)

    for p in range(8):
        for jq in range(4):
            tw_ref[(p * 4 + jq) * 2] = jnp.float32(math.cos(2 * math.pi * p * jq / 32))
            tw_ref[(p * 4 + jq) * 2 + 1] = jnp.float32(math.sin(2 * math.pi * p * jq / 32))

    qi = jax.lax.broadcasted_iota(jnp.int32, (48, 128), 0)
    ki = jax.lax.broadcasted_iota(jnp.int32, (48, 128), 1)

    def between(v, lo, hi):
        return (v >= lo) & (v < hi)

    def table(keep, other):
        return jnp.where(other, -jnp.inf, jnp.where(keep, 0.0, NEG)).astype(f32)

    keep = between(qi, 8, 16) | between(ki, 8, 16) | (qi >= jnp.where(ki < 32, ki, ki - 24))
    fille_ref[...] = table(keep, ki >= 40)[:32]
    q_even = between(qi, 32, 40)
    k_even = between(ki, 32, 40) | (ki >= 48)
    qpos = jnp.where(qi < 32, qi, jnp.where(qi < 40, qi - 24, qi - 32))
    kpos = jnp.where(ki < 32, ki, jnp.where(ki < 40, ki - 24, jnp.where(ki < 48, ki - 32, ki - 48)))
    keep = between(qi, 8, 16) | between(ki, 8, 16) | (ki >= 56) | (qpos >= kpos)
    fillo_ref[...] = table(keep, (q_even != k_even) | (ki >= 64))

    def relayout16(c, blk):
        w0 = pl.multiple_of(blk * 8, 8)
        v = _tou(raw_ref[c % 4, pl.ds(blk * 16, 16)]).reshape(8, 2, 8, 128)
        a, b = v[:, 0], v[:, 1]
        w_refs[c][0:8, pl.ds(w0, 8), :] = jnp.swapaxes((a & jnp.uint32(0xFFFF)) | (b << 16), 0, 1)
        w_refs[c][8:16, pl.ds(w0, 8), :] = jnp.swapaxes((a >> 16) | (b & jnp.uint32(0xFFFF0000)), 0, 1)

    def slot_of(h):
        return (h // 16) * 16 + (h % 2) * 8 + (h % 16) // 2

    def repack_wo64(blk):
        v = _tou(woraw_ref[pl.ds(pl.multiple_of(blk * 64, 64), 64), :])
        wo_ref[:, pl.ds(pl.multiple_of(blk * 32, 32), 32), :] = jnp.stack(
            [v[:, j * 128:(j + 1) * 128] for j in range(8)])

    sub4 = jax.lax.broadcasted_iota(jnp.int32, (128, 128), 0) & 3

    def wp_store(t, kb, tile):
        v = tile.T
        for g in range(4):
            r0 = pl.multiple_of(t * 2560 + kb * 160 + g * 40, 8)
            wp_ref[pl.ds(r0, 32), :] = v[g * 32:(g + 1) * 32]

    def b_prep(lg, hb, par):
        cols = slice(hb * 128, (hb + 1) * 128)
        a = _tou(wt_ref[lg, 0:512, cols])
        b = _tou(wt_ref[8 + lg, 0:512, cols])
        if par == 0:
            w = (a << 16) | (b & jnp.uint32(0xFFFF))
            m = (sub4 == 0) | (sub4 == 2)
        else:
            w = (a & jnp.uint32(0xFFFF0000)) | (b >> 16)
            m = (sub4 == 0) | (sub4 == 3)
        top = w[:128]
        bot = pltpu.roll(w[128:].reshape(16, 8, 128), 1 + par, 1).reshape(128, 128)
        wp_store(par, lg * 2 + hb, jnp.where(m, top, bot))
        wp_store(par + 2, lg * 2 + hb, jnp.where(m, bot, top))
        if par == 0:
            na = jnp.broadcast_to(wt_ref[lg, 512:513, cols].astype(f32), (128, 128))
            nb = jnp.broadcast_to(wt_ref[8 + lg, 512:513, cols].astype(f32), (128, 128))
            wp_store(4, lg * 2 + hb, pltpu.bitcast(na, u32) | (pltpu.bitcast(nb, u32) >> 16))

    def gather_c(k):
        xc_ref[k] = _tou(xcraw_ref[k].astype(f32).reshape(512, 128).astype(bf16))

    def store_qkvc(n, y):
        qkvc_ref[:, n] = y.reshape(NSEG // 2, 8, 128)

    def q_unit(i, groups, first, last, fillers):
        xk = _tobf(xc_ref[i])
        w0 = pl.multiple_of(i * 64, 64)
        for g in groups:
            rhs = jnp.concatenate(
                [_tobf(w_refs[h // 16][h % 16, pl.ds(w0, 64), :]) for h in range(4 * g, 4 * g + 4)], axis=1)
            y = _dot(xk, rhs)
            for h in range(4 * g, 4 * g + 4):
                yh = y[:, (h % 4) * 128:(h % 4 + 1) * 128]
                if not first:
                    yh = yh + ub_ref[h * 4:(h + 1) * 4].reshape(512, 128)
                if last:
                    store_qkvc(h, _tou(yh.astype(bf16)))
                else:
                    ub_ref[h * 4:(h + 1) * 4] = yh.reshape(4, 128, 128)
            mine = fillers.get(g, [])
            for fi, item in enumerate(mine):
                r = (fi * 512 // len(mine)) // 8 * 8
                item(pltpu.bitcast(y[r:r + 8, 0:128], u32))

    def rl_item(c, blk):
        def item(pin):
            w_refs[c][15, pin_rows(512), :] = pin
            relayout16(c, blk)
        return item

    def spread(fillers, items, groups):
        for k, item in enumerate(items):
            fillers.setdefault(groups[k * len(groups) // len(items)], []).append(item)
        return fillers

    def half_items(f, c, i, groups):
        return spread(f, [rl_item(c, i * 8 + blk) for blk in range(8)], groups)

    def piece_items(i):
        f = half_items(half_items({}, 1, i, (0, 1, 2)), 0, i + 1, (4, 5, 6))
        return spread(f, [lambda pin: gather_c(i + 1)], (7,))

    def chunk2_items(f, lo, hi, groups):
        return spread(f, [rl_item(2, blk) for blk in range(lo, hi)], groups)

    def wait_piece(i):
        raw_copy(1, i, 128).wait()
        xc_copy(i + 1).wait()
        raw_copy(0, i + 1, 128).wait()

    raw_copy(0, 0, 128).wait()
    for blk in range(8):
        relayout16(0, blk)
    xc_copy(0).wait()
    gather_c(0)
    q_unit(0, range(0, 2), True, False, {})
    raw_copy(1, 0, 128).wait()
    q_unit(0, range(2, 4), True, False, half_items({}, 1, 0, (2, 2, 3)))
    q_unit(0, range(4, 6), True, False, {})
    xc_copy(1).wait()
    raw_copy(0, 1, 128).wait()
    q_unit(0, range(6, 8), True, False,
           spread(half_items({}, 0, 1, (6, 6, 7)), [lambda pin: gather_c(1)], (6,)))
    raw_copy(1, 1, 128).wait()
    q_unit(1, range(0, 4), False, False, half_items({}, 1, 1, (0, 1, 2)))
    xc_copy(2).wait()
    raw_copy(0, 2, 128).wait()
    q_unit(1, range(4, 8), False, False,
           spread(half_items({}, 0, 2, (4, 5, 6)), [lambda pin: gather_c(2)], (6,)))

    def q_c(i, carry):
        wait_piece(i)
        raw_copy(2, i - 2, 128).wait()
        q_unit(i, range(8), False, False, half_items(piece_items(i), 2, i - 2, (3, 3, 3, 3, 4, 5, 6, 7)))
        return carry
    jax.lax.fori_loop(2, 6, q_c, 0)

    wait_piece(6)
    raw_copy(2, 4, 128).wait()
    raw_copy(2, 5, 128).wait()
    q_unit(6, range(8), False, False, chunk2_items(piece_items(6), 32, 48, (0, 1, 2, 3, 3, 4, 5, 6)))
    raw_copy(1, 7, 128).wait()
    raw_copy(2, 6, 128).wait()
    raw_copy(2, 7, 128).wait()
    q_unit(7, range(8), False, True, chunk2_items(half_items({}, 1, 7, (0, 1, 2)), 48, 64, (3, 4, 5, 6)))
    raw_copy(4).start()
    raw_copy(5).start()

    def bulk_iter(c, i):
        xc = jnp.concatenate([_tobf(xc_ref[k]) for k in range(8)], axis=1)
        for t in range(8):
            n = i * 8 + t
            y = _tou(_dot(xc, _tobf(w_refs[c][n, 0:512])).astype(bf16))
            store_qkvc(c * 16 + n, y)
            for blk in range(4):
                pin = y[blk * 64:blk * 64 + 8]
                if c + 1 < 6:
                    w_refs[c + 1][15, pin_rows(512), :] = pin
                    relayout16(c + 1, i * 32 + (t * 4 + blk))
                else:
                    wo_ref[7, pin_rows(2048), :] = pin
                    repack_wo64(i * 32 + (t * 4 + blk))
            if c >= 4:
                wp_ref[pin_rows(12832), :] = y[32:40]
                b_prep((c - 4) * 4 + i * 2 + t // 4, (t // 2) % 2, t % 2)

    for c in range(2, 6):
        if c == 4:
            for cp in cp_wt:
                cp.wait()
        if c == 5:
            cp_wo.wait()
        elif c > 2:
            raw_copy(c + 1).wait()

        def bulk(i, carry, c=c):
            if c == 2:
                raw_copy(3, i, 512).wait()
            bulk_iter(c, i)
            return carry
        jax.lax.fori_loop(0, 2, bulk, 0)

    cp_x.wait()
    cp_mem.wait()
    cp_bx.wait()
    cp_fd.wait()
    cp_tv.wait()

    lane = jax.lax.broadcasted_iota(jnp.int32, (1, 128), 1)
    lane0 = lane == 0
    sgn0 = jnp.where(lane0, 1.0, -1.0)

    def first_lanes(t):
        la, lb = [k for k in range(4) if _FIRST[t][k]]
        return ((lane & 3) == la) | ((lane & 3) == lb)

    def d_products(st_ref, d, t, rows):
        return [_dot(st_ref[n, rows].astype(bf16), _tobf(fd_ref[d * 12 + n])) if n else None
                for n in range(3 * t, 3 * t + 3)]

    def twiddles(p):
        return [(tw_ref[p * 8 + jq * 2], tw_ref[p * 8 + jq * 2 + 1]) if jq else None for jq in range(4)]

    def p1_pre(p, rs, q):
        def item(y):
            sa_ref[7, pin_rows(256), :] = y
            xq = bx_ref[q, pl.ds(pl.multiple_of(p * 64 + rs * 16, 16), 16), :].astype(f32)
            zz = _r8_real([xq[:, a * 128:(a + 1) * 128] for a in range(8)])
            r = (rs * 4 + q) * 16
            sa_ref[1:12, r:r + 16] = jnp.stack([v for (a, b) in zz for v in (a + b, b, a)][1:])
        return item

    def p1_mm(p, t):
        def item(y):
            cs = twiddles(p)

            def put(n, rs, re, im):
                v = jnp.stack([re.reshape(2, 8, 128), im.reshape(2, 8, 128)], axis=1)
                ub_ref[n * 8 + p, rs * 32:(rs + 1) * 32] = v.reshape(32, 128)

            first = first_lanes(t)
            for rs in range(4):
                k1, k2, k3 = d_products(sa_ref, 0, t, slice(rs * 64, (rs + 1) * 64))
                if t == 0:
                    up = jnp.where(first, k2, k3)
                    re, im = jnp.where(first, k3, k2), pltpu.roll(up, 126, 1)
                    ny = jnp.where(lane0, im, up)
                    u = [ny[q * 16:(q + 1) * 16] for q in range(4)]
                    odd_lane = (lane & 1) == 1
                    nr = jnp.where(odd_lane, pltpu.roll(u[0] - u[2], 1, 1), u[0] + u[2] + (u[1] + u[3]) * sgn0)
                    ni = jnp.where(odd_lane, pltpu.roll((u[3] - u[1]) * sgn0, 1, 1), 0.0)
                    rows = pl.ds(pl.multiple_of(p * 64 + rs * 16, 16), 16)
                    c, sn = tv_ref[0, rows], tv_ref[1, rows]
                    put(NYQ, rs, nr * c + ni * sn, ni * c - nr * sn)
                    im = jnp.where(lane0, 0.0, im)
                else:
                    re, im = k1 + k2, (k3 - k1) * jnp.where(first, 1.0, -1.0)
                a = _dft4([(re[q * 16:(q + 1) * 16], im[q * 16:(q + 1) * 16]) for q in range(4)])
                for jq in range(4):
                    re, im = a[jq]
                    if jq > 0:
                        c, sn = cs[jq]
                        re, im = re * c + im * sn, im * c - re * sn
                    put(t * 4 + jq, rs, re, im)
        return item

    def p2_bfly(u, g, inverse):
        def item(y):
            if y is not None:
                ub_ref[144, pin_rows(0), :] = y
            v = ub_ref[pl.ds(u * 8, 8), g * 16:(g + 1) * 16]
            x = [(v[p, 0:8], v[p, 8:16]) for p in range(8)]
            x = _swap(_dft8(_swap(x))) if inverse else _dft8(x)
            ub_ref[pl.ds(u * 8, 8), g * 16:(g + 1) * 16] = jnp.stack([w for c in x for w in c]).reshape(8, 16, 128)
        return item

    def filtered(xx, w):
        wr = pltpu.bitcast(w & jnp.uint32(0xFFFF0000), f32).reshape(8, 8, 128)
        wi = pltpu.bitcast(w << 16, f32).reshape(8, 8, 128)
        xx = xx.reshape(8, 2, 8, 128)
        xr, xi = xx[:, 0], xx[:, 1]
        return jnp.stack([xr * wr - xi * wi, xr * wi + xi * wr], axis=1).reshape(128, 128)

    def p2_fwd(u, jps):
        def item(y):
            t = u >> 2
            jq = u & 3
            xs = [_dot(_tobf(ms_ref[jq + 4 * jp]), ub_ref[u * 8 + jp].astype(bf16)) for jp in jps]
            for jp, xx in zip(jps, xs):
                ub_ref[u * 8 + jp] = filtered(xx, wp_ref[pl.ds(t * 2560 + jq + 4 * jp, 64, stride=40), :])
        return item

    def p2_nyq(u):
        def item(y):
            jp = u & 7
            rhs = ub_ref[NYQ * 8 + jp].astype(bf16)
            xx = jnp.concatenate([_dot(_tobf(ms_ref[u * 4, m * 16:(m + 1) * 16]), rhs) for m in range(4)], axis=0)
            w = wp_ref[pl.ds(4 * 2560 + 4 * jp, 64, stride=40), :]
            for jq in range(1, 4):
                w = jnp.where(lane == jq, wp_ref[pl.ds(4 * 2560 + 4 * jp + jq, 64, stride=40), :], w)
            w = jnp.where(u < 8, w, jnp.uint32(0x3F800000))
            ub_ref[NYQ * 8 + jp] = filtered(xx, w)
        return item

    def p2_inv(u, jps):
        def item(y):
            jq = u & 3
            zs = [_dot(_tobf(ms_ref[32 + jq + 4 * jp]), ub_ref[u * 8 + jp].astype(bf16)) for jp in jps]
            for jp, zz in zip(jps, zs):
                ub_ref[u * 8 + jp] = zz
        return item

    def p3_pre(p, g, t):
        def item(y):
            sa_ref[7, pin_rows(256), :] = y
            cs = twiddles(p)

            def fetch(t):
                a = []
                for jq in range(4):
                    v = ub_ref[(t * 4 + jq) * 8 + p, g * 16:(g + 1) * 16]
                    re, im = v[0:8], v[8:16]
                    if jq > 0:
                        c, sn = cs[jq]
                        re, im = re * c - im * sn, im * c + re * sn
                    a.append((re, im))
                return _swap(_dft4(_swap(a)))

            u = fetch(t)
            if t == 0:
                v = ub_ref[NYQ * 8 + p, g * 16:(g + 1) * 16]
                rows = pl.ds(pl.multiple_of(p * 64 + g * 8, 8), 8)
                c, sn = tv_ref[0, rows], tv_ref[1, rows]
                nr, ni = v[0:8] * c - v[8:16] * sn, v[8:16] * c + v[0:8] * sn
                zr, zi = pltpu.roll(nr, 127, 1), pltpu.roll(ni, 127, 1)
                ny = (nr + zr, (nr - zi) * sgn0, nr - zr, (nr + zi) * sgn0)
            first = first_lanes(t)
            for q in range(4):
                re, im = u[q]
                rows = slice(q * 64 + g * 8, q * 64 + (g + 1) * 8)
                if t == 0:
                    im = pltpu.roll(jnp.where(lane0, ny[q], im), 2, 1) + jnp.where(lane == 2, ny[q], 0.0)
                    sa_ref[1:3, rows] = jnp.stack((jnp.where(first, im, re), jnp.where(first, re, im)))
                else:
                    im = im * jnp.where(first, 1.0, -1.0)
                    sa_ref[3 * t:3 * t + 3, rows] = jnp.stack((re + im, im, re))
        return item

    def p3_mm(p, q):
        def item(y):
            g = []
            for t in range(4):
                k1, k2, k3 = d_products(sa_ref, 1, t, slice(q * 64, (q + 1) * 64))
                g.append((k3, k2) if t == 0 else (k2 + k1, k3 - k1))
            yy = _r8_real_t(g)
            bx_ref[q, pl.ds(pl.multiple_of(p * 64, 64), 64), :] = jnp.concatenate(yy, axis=1).astype(bf16)
        return item

    def b_out(p):
        def item(y):
            rows = pl.ds(pl.multiple_of(p * 64, 64), 64)
            pltpu.make_async_copy(bx_ref.at[0:4, rows, :], out_hbm.at[:, rows, pl.ds(DM, DM)],
                                  sem_out.at[1]).start()
            bx_ref[4, pin_rows(0), 0:128] = y.astype(bf16)
        return item

    def step(pp, odd, mem, hooks):
        r0 = pl.multiple_of(pp * 64 + 32 * odd, SEG)
        xs = xo_ref[pl.ds(r0, SEG), :]
        x_lo = xs[0:8].astype(f32)
        hm = jnp.concatenate(
            [jnp.concatenate([x_lo, jnp.concatenate(mem, axis=1)], axis=0).astype(bf16), xs[16:32]], axis=0)
        fill = fillo_ref[:, 0:64] if odd else fille_ref[:, 0:48]
        nrow = 48 if odd else 32
        qkv, ps = {}, {}

        def do_qkv(h0, h1):
            for h in range(h0, h1):
                for t in range(3):
                    n = t * H + slot_of(h)
                    y32 = _dot(hm, _tobf(w_refs[n // 16][n % 16, 0:512]))
                    y = y32.astype(bf16)
                    parts = [y]
                    if odd or t > 0:
                        parts.append(_tobf(qkvc_ref[pp, n]))
                    if t > 0:
                        if odd:
                            parts.append(_tobf(kve_ref[(t - 1) * H + h]))
                        else:
                            kve_ref[(t - 1) * H + h] = _tou(y[0:16])
                    qkv[(t, h)] = jnp.concatenate(parts, axis=0) if len(parts) > 1 else y
                for item in hooks.get(h, ()):
                    item(y32[0:8])

        def do_s(g):
            for h in range(g * G, (g + 1) * G):
                sc = jax.lax.dot_general(qkv[(0, h)], qkv[(1, h)], (((1,), (1,)), ((), ())),
                                         preferred_element_type=f32)
                sc = jnp.where(fill == 0.0, sc * scale, fill)
                e = jnp.exp(sc - jnp.max(sc, axis=1, keepdims=True))
                den = jnp.sum(e, axis=1, keepdims=True)
                r = pl.reciprocal(den, approx=True)
                r = r * (2.0 - den * r)
                ps[h] = (e * r).astype(bf16)

        def do_pv(g):
            for h in range(g * G, (g + 1) * G):
                oall_ref[0:nrow // 2, h * DH:(h + 1) * DH] = _tou(_dot(ps[h], qkv[(2, h)]).astype(bf16))

        def do_o(j, h0, h1):
            return _dot(_tobf(oall_ref[0:nrow // 2, h0 * DH:h1 * DH]), _tobf(wo_ref[j, h0 * 64:h1 * 64, :]))

        for g in range(NG):
            do_qkv(g * G, g * G + G // 2)
            if g >= 1:
                do_s(g - 1)
            do_qkv(g * G + G // 2, (g + 1) * G)
            if g >= 2:
                do_pv(g - 2)
        part = {}
        for j in range(8):
            items = hooks.get(('o', j), ())
            if len(items) == 1:
                part[j] = do_o(j, 0, OSPLIT)
                items[0](None)
            elif items:
                half = do_o(j, 0, OSPLIT // 2)
                items[0](half[0:8])
                part[j] = do_o(j, OSPLIT // 2, OSPLIT) + half
                items[1](part[j][0:8])
            else:
                part[j] = do_o(j, 0, OSPLIT)
            if j == 2:
                do_s(NG - 1)
                do_pv(NG - 2)
            if j == 5:
                do_pv(NG - 1)
        new_mem = []
        for j in range(8):
            cols = slice(j * 128, (j + 1) * 128)
            res = do_o(j, OSPLIT, H) + part[j]
            new_mem.append(res[8:16])
            if odd:
                xo_ref[pl.ds(r0, SEG), cols] = jnp.concatenate(
                    [res[0:8], res[40:48], res[16:32]], axis=0).astype(bf16)
                xo_ref[pl.ds(r0 - 24, 8), cols] = res[32:40].astype(bf16)
            else:
                xo_ref[pl.ds(r0, SEG), cols] = res.astype(bf16)
        for item in hooks.get(H, ()):
            item(None)
        if odd:
            pltpu.make_async_copy(
                xo_ref.at[pl.ds(pl.multiple_of(pp * 64, 64), 64), :],
                out_hbm.at[pp >> 3, pl.ds(pl.multiple_of((pp & 7) * 64, 64), 64), pl.ds(0, DM)],
                sem_out.at[0]).start()
        return new_mem

    def l1(i, mem):
        he = {2 * k: [p1_pre(i, k // 4, k % 4)] for k in range(16)}
        he[H] = [p1_mm(i, 1)]
        ho = {('o', 0): [p1_mm(i, 2)], ('o', 3): [p1_mm(i, 3)], ('o', 5): [p1_mm(i, 0)]}
        mem = step(i, 0, mem, he)
        mem = step(i, 1, mem, ho)
        return mem

    def l2(i, mem):
        u = i - N_L1
        he = {3: [p2_fwd(u, range(0, 4))], 7: [p2_fwd(u, range(4, 8))], 17: [p2_nyq(u)],
              H: [p2_inv(u, range(0, 8))]}
        ho = {('o', j): [p2_bfly(u, j, True), p2_bfly(u + 1, j, False)] for j in range(8)}
        mem = step(i, 0, mem, he)
        mem = step(i, 1, mem, ho)
        return mem

    def l3(i, mem):
        p = i - N_L1 - N_L2
        he = {h: [p3_pre(p, h // 3, 1 + h % 3)] for h in range(24)}
        for j in range(4):
            he[('o', 3 + j)] = [p3_pre(p, 2 * j, 0), p3_pre(p, 2 * j + 1, 0)]
        he[H] = [p3_mm(p, q) for q in range(4)]
        ho = {12: [b_out(p)]}
        mem = step(i, 0, mem, he)
        mem = step(i, 1, mem, ho)
        return mem

    m0 = mem_ref[...].astype(f32)
    mem = [m0[:, j * 128:(j + 1) * 128] for j in range(8)]
    mem = jax.lax.fori_loop(0, N_L1, l1, mem)
    cp_ms.wait()
    for g in range(8):
        p2_bfly(0, g, False)(None)
        p2_bfly(NYQ, g, False)(None)
    mem = jax.lax.fori_loop(N_L1, N_L1 + N_L2, l2, mem)
    for g in range(8):
        p2_bfly(NYQ, g, True)(None)
    mem = jax.lax.fori_loop(N_L1 + N_L2, NSEG // 2, l3, mem)

    pltpu.make_async_copy(bx_ref.at[0:4], out_hbm.at[:, :, pl.ds(DM, DM)], sem_out.at[1]).wait()
    pltpu.make_async_copy(xo_ref, xo_ref, sem_out.at[0]).wait()


@jax.jit
def _run(x, mem0, wq, wk, wv, wo, bx, w_r, w_i):
    fd, ms, tv = _tables()
    hbm = pl.BlockSpec(memory_space=pl.ANY)
    out = pl.pallas_call(
        _kernel,
        out_shape=jax.ShapeDtypeStruct((4, S // 4, 2 * DM), bf16),
        in_specs=[hbm] * 13,
        out_specs=hbm,
        scratch_shapes=[
            pltpu.VMEM((S, DM), bf16),
            pltpu.VMEM((MEM, DM), bf16),
            pltpu.VMEM((8, NSEG, 8, 128), bf16),
            pltpu.VMEM((4, DM, 16, DH), bf16),
        ] + [pltpu.VMEM((16, DM // 2 + 8, DH), u32)] * 6 + [
            pltpu.VMEM((H * DH, DM), bf16),
            pltpu.VMEM((8, H * DH // 2 + 8, 128), u32),
            pltpu.VMEM((8, 256, 128), u32),
            pltpu.VMEM((NSEG // 2, 3 * H, 8, 128), u32),
            pltpu.VMEM((2 * H, 8, 128), u32),
            pltpu.VMEM((24, H * DH), u32),
            pltpu.VMEM((32, 128), f32),
            pltpu.VMEM((48, 128), f32),
            pltpu.VMEM((5, S // 4, DM), bf16),
            pltpu.VMEM((16, DM // 2 + 1, 256), bf16),
            pltpu.VMEM((12840, 128), u32),
            pltpu.VMEM((145, 128, 128), f32),
            pltpu.VMEM((12, 264, 128), f32),
            pltpu.VMEM((24, 64, 128), u32),
            pltpu.VMEM((64, 64, 128), u32),
            pltpu.VMEM((2, 512, 128), f32),
            pltpu.SMEM((64,), f32),
            pltpu.SMEM((1,), jnp.int32),
            pltpu.SemaphoreType.DMA((64,)),
            pltpu.SemaphoreType.DMA((2,)),
        ],
        compiler_params=pltpu.CompilerParams(vmem_limit_bytes=120 * 1024 * 1024,
                                             disable_semaphore_checks=True,
                                             disable_bounds_checks=True),
    )(x.reshape(S, DM), x.reshape(NSEG, SEG, DM), mem0.reshape(MEM, DM), wq, wk, wv,
      wo.reshape(H * DH, DM), bx.reshape(4, S // 4, DM), w_r.T, w_i.T, jnp.asarray(fd), jnp.asarray(ms), jnp.asarray(tv))
    return out.reshape(1, S, 2 * DM)


def pallas_concat_heads__memory_aug_recurrent_mem_tr__spectral_gfnet__prompt_kernel(
    A_x: jax.Array,
    A_mem0: jax.Array,
    A_Wq: jax.Array,
    A_Wk: jax.Array,
    A_Wv: jax.Array,
    A_Wo: jax.Array,
    A_seg_len,
    B_x: jax.Array,
    B_w_r: jax.Array,
    B_w_i: jax.Array,
):
    if isinstance(A_seg_len, int):
        assert A_seg_len == SEG
    assert A_x.shape == (1, S, DM) and A_mem0.shape == (1, MEM, DM) and A_Wq.shape == (DM, H, DH)
    assert B_x.shape == (1, S, DM) and B_w_r.shape == (S, DM // 2 + 1)
    return _run(A_x, A_mem0, A_Wq, A_Wk, A_Wv, A_Wo, B_x, B_w_r, B_w_i)
```

```python
import math

import numpy as np
import jax
import jax.numpy as jnp
import jax.experimental.pallas as pl
import jax.experimental.pallas.tpu as pltpu

bf16 = jnp.bfloat16
f32 = jnp.float32
u32 = jnp.uint32

S, DM = 2048, 1024
H, DH = 32, 128
MEM, SEG = 8, 32
NSEG = S // SEG
SQH = math.sqrt(0.5)

_PAIRS = ((0, 4), (1, 7), (2, 6), (3, 5))
_FIRST = np.array([[1, 1, 0, 0], [1, 0, 1, 0], [0, 1, 1, 0], [0, 1, 0, 1]], bool)


def _pack_rows(a):
    u = np.ascontiguousarray(a, dtype=np.float32).view(np.uint32).astype(np.uint64)
    b = ((u + 0x7FFF + ((u >> 16) & 1)) >> 16).astype(np.uint32)
    return (b[..., 0::2, :] | (b[..., 1::2, :] << 16)).astype(np.uint32)


def _tables():
    k2 = np.zeros((4, 128), np.int64)
    for t in range(4):
        odd = t % 2
        for lam in range(128):
            k = 2 * lam + odd
            if k % 8 not in _PAIRS[t]:
                k = 2 * (128 + 8 * (lam // 8) + (lam % 8 - 1 - odd) % 8) + odd
            assert k % 8 in _PAIRS[t]
            k2[t, lam] = k
    b = np.arange(128)[:, None]
    F = np.zeros((12, 128, 128))
    G = np.zeros((12, 128, 128))
    for t in range(4):
        th = 2 * np.pi * ((b * k2[t][None, :]) % DM) / DM
        C, Sn = np.cos(th), np.sin(th)
        first = ((k2[t] % 8) == _PAIRS[t][0])[None, :]
        assert np.array_equal(first[0], _FIRST[t][np.arange(128) % 4])
        if t == 0:
            im = -Sn
            im[:, 0] = (-1.0) ** np.arange(128)
            im = np.roll(im, 2, axis=1)
            F[1:3] = np.where(first, im, C), np.where(first, C, im)
            G[1:3] = F[1:3]
            G[2, :, 0] *= 0.5
            G[2, :, 2] *= 0.5
        else:
            Sg = np.where(first, Sn, -Sn)
            F[3 * t:3 * t + 3] = C, -(C + Sg), C - Sg
            G[3 * t:3 * t + 3] = F[3 * t:3 * t + 3]
    Finv = np.transpose(G, (0, 2, 1)) * (2.0 / DM)
    fd = _pack_rows(np.concatenate([F, Finv]))
    M = np.zeros((32, 128, 128))
    r = np.arange(64)[None, :]
    l = np.arange(64)[:, None]
    for j in range(32):
        th = 2 * np.pi * ((r * (j + 32 * l)) % S) / S
        C, Sn = np.cos(th), np.sin(th)
        M[j, :64, :64] = C
        M[j, :64, 64:] = Sn
        M[j, 64:, :64] = -Sn
        M[j, 64:, 64:] = C
    perm = np.arange(128).reshape(2, 8, 8).transpose(1, 0, 2).reshape(128)
    M = M[:, perm][:, :, perm]
    Minv = np.transpose(M, (0, 2, 1)) / S
    ms = _pack_rows(np.concatenate([M, Minv]))
    th = 2 * np.pi * np.outer(np.arange(512), np.arange(128) % 4) / S
    tv = np.stack([np.cos(th), np.sin(th)]).astype(np.float32)
    return fd, ms, tv


def _tobf(w):
    return pltpu.bitcast(w, bf16)


def _tou(w):
    return pltpu.bitcast(w, u32)


def _dot(a, b):
    return jnp.dot(a, b, preferred_element_type=f32)


def _r8_real(x):
    t0, t1 = x[0] + x[4], x[0] - x[4]
    t2, t3 = x[2] + x[6], x[2] - x[6]
    t4, t5 = x[1] + x[5], x[1] - x[5]
    t6, t7 = x[3] + x[7], x[3] - x[7]
    e0, e1 = t0 + t2, t0 - t2
    o0, o1 = t4 + t6, t4 - t6
    u, v = SQH * (t5 - t7), SQH * (t5 + t7)
    return [(e0 + o0, e0 - o0), (t1 + u, v + t3), (e1, o1), (t1 - u, v - t3)]


def _r8_real_t(g):
    (z0, z4), (a1, b1), (e1, o1), (a3, b3) = g
    e0, o0 = z0 + z4, z0 - z4
    t1, u = a1 + a3, a1 - a3
    v, t3 = b1 + b3, b1 - b3
    t5, t7 = SQH * (v + u), SQH * (v - u)
    t0, t2 = e0 + e1, e0 - e1
    t4, t6 = o0 + o1, o0 - o1
    return [t0 + t1, t4 + t5, t2 + t3, t6 + t7, t0 - t1, t4 - t5, t2 - t3, t6 - t7]


def _dft4(u):
    (r0, i0), (r1, i1), (r2, i2), (r3, i3) = u
    sr, si, dr, di = r0 + r2, i0 + i2, r0 - r2, i0 - i2
    tr, ti, er, ei = r1 + r3, i1 + i3, r1 - r3, i1 - i3
    return [(sr + tr, si + ti), (dr + ei, di - er), (sr - tr, si - ti), (dr - ei, di + er)]


def _dft8(x):
    a = [(x[p][0] + x[p + 4][0], x[p][1] + x[p + 4][1]) for p in range(4)]
    d = [(x[p][0] - x[p + 4][0], x[p][1] - x[p + 4][1]) for p in range(4)]
    ev = _dft4(a)
    (r0, i0), (r1, i1), (r2, i2), (r3, i3) = d
    b1r, b1i = SQH * (r1 + i1), SQH * (i1 - r1)
    b3r, n3i = SQH * (i3 - r3), SQH * (r3 + i3)
    sr, si, dr, di = r0 + i2, i0 - r2, r0 - i2, i0 + r2
    tr, ti, er, ei = b1r + b3r, b1i - n3i, b1r - b3r, b1i + n3i
    od = [(sr + tr, si + ti), (dr + ei, di - er), (sr - tr, si - ti), (dr - ei, di + er)]
    return [ev[0], od[0], ev[1], od[1], ev[2], od[2], ev[3], od[3]]


def _swap(x):
    return [(b, a) for (a, b) in x]


G = 4
NG = H // G
OSPLIT = 24
NEG = -1e9
N_L1, N_L2, N_L3 = 8, 16, 8


def _kernel(x_hbm, x3_hbm, mem_hbm, wq_hbm, wk_hbm, wv_hbm, wo_hbm, bx_hbm, wr_hbm, wi_hbm,
            fd_hbm, ms_hbm, tv_hbm, out_hbm,
            xo_ref, mem_ref, xcraw_ref, raw_ref, w0_ref, w1_ref, w2_ref, w3_ref, w4_ref, w5_ref,
            woraw_ref, wo_ref, xc_ref, qkvc_ref, kve_ref,
            oall_ref, fille_ref, fillo_ref, bx_ref, wt_ref, wp_ref, ub_ref, ny_ref, sa_ref, fd_ref, ms_ref, tv_ref,
            tw_ref, zero_ref, sem_in, sem_out):
    scale = DH ** -0.5
    w_hbm = (wq_hbm, wk_hbm, wv_hbm)
    w_refs = (w0_ref, w1_ref, w2_ref, w3_ref, w4_ref, w5_ref)

    def raw_copy(c, i=0, nd=DM):
        rows = pl.ds(pl.multiple_of(i * nd, nd), nd)
        return pltpu.make_async_copy(
            w_hbm[c // 2].at[rows, pl.ds((c % 2) * 16, 16), :],
            raw_ref.at[c % 4, rows], sem_in.at[8 + min(c, 3) * 8 + max(c - 3, 0) * 2 + i])

    def xc_copy(k):
        return pltpu.make_async_copy(
            x3_hbm.at[:, pl.ds(8, 8), pl.ds(pl.multiple_of(k * 128, 128), 128)], xcraw_ref.at[k], sem_in.at[40 + k])

    cp_x = pltpu.make_async_copy(x_hbm, xo_ref, sem_in.at[0])
    cp_mem = pltpu.make_async_copy(mem_hbm, mem_ref, sem_in.at[1])
    cp_wo = pltpu.make_async_copy(wo_hbm, woraw_ref, sem_in.at[2])
    cp_bx = pltpu.make_async_copy(bx_hbm, bx_ref.at[0:4], sem_in.at[3])
    cp_fd = pltpu.make_async_copy(fd_hbm, fd_ref, sem_in.at[4])
    cp_ms = pltpu.make_async_copy(ms_hbm, ms_ref, sem_in.at[5])
    cp_tv = pltpu.make_async_copy(tv_hbm, tv_ref, sem_in.at[6])
    cp_wt = [pltpu.make_async_copy(src.at[:, pl.ds(lg * 256, 256)], wt_ref.at[a * 8 + lg], sem_in.at[48 + a * 8 + lg])
             for a, src in enumerate((wr_hbm, wi_hbm)) for lg in range(8)]

    for i in range(8):
        raw_copy(0, i, 128).start()
        xc_copy(i).start()
        if i >= 3:
            raw_copy(2, i - 3, 128).start()
        if i == 7:
            raw_copy(2, 5, 128).start()
        raw_copy(1, i, 128).start()
    for i in range(6, 8):
        raw_copy(2, i, 128).start()
    for i in range(2):
        raw_copy(3, i, 512).start()
    for cp in cp_wt + [cp_wo, cp_x, cp_mem, cp_bx, cp_fd, cp_tv, cp_ms]:
        cp.start(priority=1)

    zero_ref[0] = 0

    def pin_rows(r):
        return pl.ds(pl.multiple_of(r + zero_ref[0] * 32, 8), 8)

    for p in range(8):
        for jq in range(4):
            tw_ref[(p * 4 + jq) * 2] = jnp.float32(math.cos(2 * math.pi * p * jq / 32))
            tw_ref[(p * 4 + jq) * 2 + 1] = jnp.float32(math.sin(2 * math.pi * p * jq / 32))

    qi = jax.lax.broadcasted_iota(jnp.int32, (48, 128), 0)
    ki = jax.lax.broadcasted_iota(jnp.int32, (48, 128), 1)

    def between(v, lo, hi):
        return (v >= lo) & (v < hi)

    def table(keep, other):
        return jnp.where(other, -jnp.inf, jnp.where(keep, 0.0, NEG)).astype(f32)

    keep = between(qi, 8, 16) | between(ki, 8, 16) | (qi >= jnp.where(ki < 32, ki, ki - 24))
    fille_ref[...] = table(keep, ki >= 40)[:32]
    q_even = between(qi, 32, 40)
    k_even = between(ki, 32, 40) | (ki >= 48)
    qpos = jnp.where(qi < 32, qi, jnp.where(qi < 40, qi - 24, qi - 32))
    kpos = jnp.where(ki < 32, ki, jnp.where(ki < 40, ki - 24, jnp.where(ki < 48, ki - 32, ki - 48)))
    keep = between(qi, 8, 16) | between(ki, 8, 16) | (ki >= 56) | (qpos >= kpos)
    fillo_ref[...] = table(keep, (q_even != k_even) | (ki >= 64))

    def relayout16(c, blk):
        w0 = pl.multiple_of(blk * 8, 8)
        v = _tou(raw_ref[c % 4, pl.ds(blk * 16, 16)]).reshape(8, 2, 8, 128)
        a, b = v[:, 0], v[:, 1]
        w_refs[c][0:8, pl.ds(w0, 8), :] = jnp.swapaxes((a & jnp.uint32(0xFFFF)) | (b << 16), 0, 1)
        w_refs[c][8:16, pl.ds(w0, 8), :] = jnp.swapaxes((a >> 16) | (b & jnp.uint32(0xFFFF0000)), 0, 1)

    def slot_of(h):
        return (h // 16) * 16 + (h % 2) * 8 + (h % 16) // 2

    def repack_wo64(blk):
        v = _tou(woraw_ref[pl.ds(pl.multiple_of(blk * 64, 64), 64), :])
        wo_ref[:, pl.ds(pl.multiple_of(blk * 32, 32), 32), :] = jnp.stack(
            [v[:, j * 128:(j + 1) * 128] for j in range(8)])

    sub4 = jax.lax.broadcasted_iota(jnp.int32, (128, 128), 0) & 3

    def wp_store(t, kb, tile):
        v = tile.T
        for g in range(4):
            r0 = pl.multiple_of(t * 2560 + kb * 160 + g * 40, 8)
            wp_ref[pl.ds(r0, 32), :] = v[g * 32:(g + 1) * 32]

    def b_prep(lg, hb, par):
        cols = slice(hb * 128, (hb + 1) * 128)
        a = _tou(wt_ref[lg, 0:512, cols])
        b = _tou(wt_ref[8 + lg, 0:512, cols])
        if par == 0:
            w = (a << 16) | (b & jnp.uint32(0xFFFF))
            m = (sub4 == 0) | (sub4 == 2)
        else:
            w = (a & jnp.uint32(0xFFFF0000)) | (b >> 16)
            m = (sub4 == 0) | (sub4 == 3)
        top = w[:128]
        bot = pltpu.roll(w[128:].reshape(16, 8, 128), 1 + par, 1).reshape(128, 128)
        wp_store(par, lg * 2 + hb, jnp.where(m, top, bot))
        wp_store(par + 2, lg * 2 + hb, jnp.where(m, bot, top))
        if par == 0:
            na = jnp.broadcast_to(wt_ref[lg, 512:513, cols].astype(f32), (128, 128))
            nb = jnp.broadcast_to(wt_ref[8 + lg, 512:513, cols].astype(f32), (128, 128))
            wp_store(4, lg * 2 + hb, pltpu.bitcast(na, u32) | (pltpu.bitcast(nb, u32) >> 16))

    def gather_c(k):
        xc_ref[k] = _tou(xcraw_ref[k].astype(f32).reshape(512, 128).astype(bf16))

    def store_qkvc(n, y):
        qkvc_ref[:, n] = y.reshape(NSEG // 2, 8, 128)

    def q_unit(i, groups, first, last, fillers):
        xk = _tobf(xc_ref[i])
        w0 = pl.multiple_of(i * 64, 64)
        for g in groups:
            rhs = jnp.concatenate(
                [_tobf(w_refs[h // 16][h % 16, pl.ds(w0, 64), :]) for h in range(4 * g, 4 * g + 4)], axis=1)
            y = _dot(xk, rhs)
            for h in range(4 * g, 4 * g + 4):
                yh = y[:, (h % 4) * 128:(h % 4 + 1) * 128]
                if not first:
                    yh = yh + ub_ref[h * 4:(h + 1) * 4].reshape(512, 128)
                if last:
                    store_qkvc(h, _tou(yh.astype(bf16)))
                else:
                    ub_ref[h * 4:(h + 1) * 4] = yh.reshape(4, 128, 128)
            mine = fillers.get(g, [])
            for fi, item in enumerate(mine):
                r = (fi * 512 // len(mine)) // 8 * 8
                item(pltpu.bitcast(y[r:r + 8, 0:128], u32))

    def rl_item(c, blk):
        def item(pin):
            w_refs[c][15, pin_rows(512), :] = pin
            relayout16(c, blk)
        return item

    def spread(fillers, items, groups):
        for k, item in enumerate(items):
            fillers.setdefault(groups[k * len(groups) // len(items)], []).append(item)
        return fillers

    def half_items(f, c, i, groups):
        return spread(f, [rl_item(c, i * 8 + blk) for blk in range(8)], groups)

    def piece_items(i):
        f = half_items(half_items({}, 1, i, (0, 1, 2)), 0, i + 1, (4, 5, 6))
        return spread(f, [lambda pin: gather_c(i + 1)], (7,))

    def chunk2_items(f, lo, hi, groups):
        return spread(f, [rl_item(2, blk) for blk in range(lo, hi)], groups)

    def wait_piece(i):
        raw_copy(1, i, 128).wait()
        xc_copy(i + 1).wait()
        raw_copy(0, i + 1, 128).wait()

    raw_copy(0, 0, 128).wait()
    for blk in range(8):
        relayout16(0, blk)
    xc_copy(0).wait()
    gather_c(0)
    q_unit(0, range(0, 2), True, False, {})
    raw_copy(1, 0, 128).wait()
    q_unit(0, range(2, 4), True, False, half_items({}, 1, 0, (2, 2, 3)))
    q_unit(0, range(4, 6), True, False, {})
    xc_copy(1).wait()
    raw_copy(0, 1, 128).wait()
    q_unit(0, range(6, 8), True, False,
           spread(half_items({}, 0, 1, (6, 6, 7)), [lambda pin: gather_c(1)], (6,)))
    raw_copy(1, 1, 128).wait()
    q_unit(1, range(0, 4), False, False, half_items({}, 1, 1, (0, 1, 2)))
    xc_copy(2).wait()
    raw_copy(0, 2, 128).wait()
    q_unit(1, range(4, 8), False, False,
           spread(half_items({}, 0, 2, (4, 5, 6)), [lambda pin: gather_c(2)], (6,)))

    def q_c(i, carry):
        wait_piece(i)
        raw_copy(2, i - 2, 128).wait()
        q_unit(i, range(8), False, False, half_items(piece_items(i), 2, i - 2, (3, 3, 3, 3, 4, 5, 6, 7)))
        return carry
    jax.lax.fori_loop(2, 6, q_c, 0)

    wait_piece(6)
    raw_copy(2, 4, 128).wait()
    raw_copy(2, 5, 128).wait()
    q_unit(6, range(8), False, False, chunk2_items(piece_items(6), 32, 48, (0, 1, 2, 3, 3, 4, 5, 6)))
    raw_copy(1, 7, 128).wait()
    raw_copy(2, 6, 128).wait()
    raw_copy(2, 7, 128).wait()
    q_unit(7, range(8), False, True, chunk2_items(half_items({}, 1, 7, (0, 1, 2)), 48, 64, (3, 4, 5, 6)))
    raw_copy(4).start()
    raw_copy(5).start()

    def bulk_iter(c, i):
        xc = jnp.concatenate([_tobf(xc_ref[k]) for k in range(8)], axis=1)
        for t in range(8):
            n = i * 8 + t
            y = _tou(_dot(xc, _tobf(w_refs[c][n, 0:512])).astype(bf16))
            store_qkvc(c * 16 + n, y)
            for blk in range(4):
                pin = y[blk * 64:blk * 64 + 8]
                if c + 1 < 6:
                    w_refs[c + 1][15, pin_rows(512), :] = pin
                    relayout16(c + 1, i * 32 + (t * 4 + blk))
                else:
                    wo_ref[7, pin_rows(2048), :] = pin
                    repack_wo64(i * 32 + (t * 4 + blk))
            if c >= 4:
                wp_ref[pin_rows(12832), :] = y[32:40]
                b_prep((c - 4) * 4 + i * 2 + t // 4, (t // 2) % 2, t % 2)

    for c in range(2, 6):
        if c == 4:
            for cp in cp_wt:
                cp.wait()
        if c == 5:
            cp_wo.wait()
        elif c > 2:
            raw_copy(c + 1).wait()

        def bulk(i, carry, c=c):
            if c == 2:
                raw_copy(3, i, 512).wait()
            bulk_iter(c, i)
            return carry
        jax.lax.fori_loop(0, 2, bulk, 0)

    cp_x.wait()
    cp_mem.wait()
    cp_bx.wait()
    cp_fd.wait()
    cp_tv.wait()

    lane = jax.lax.broadcasted_iota(jnp.int32, (1, 128), 1)
    lane0 = lane == 0
    sgn0 = jnp.where(lane0, 1.0, -1.0)

    def first_lanes(t):
        la, lb = [k for k in range(4) if _FIRST[t][k]]
        return ((lane & 3) == la) | ((lane & 3) == lb)

    def d_products(st_ref, d, t, rows):
        return [_dot(st_ref[n, rows].astype(bf16), _tobf(fd_ref[d * 12 + n])) if n else None
                for n in range(3 * t, 3 * t + 3)]

    def twiddles(p):
        return [(tw_ref[p * 8 + jq * 2], tw_ref[p * 8 + jq * 2 + 1]) if jq else None for jq in range(4)]

    def p1_pre(p, rs, q):
        def item(y):
            sa_ref[7, pin_rows(256), :] = y
            xq = bx_ref[q, pl.ds(pl.multiple_of(p * 64 + rs * 16, 16), 16), :].astype(f32)
            zz = _r8_real([xq[:, a * 128:(a + 1) * 128] for a in range(8)])
            r = (rs * 4 + q) * 16
            sa_ref[1:12, r:r + 16] = jnp.stack([v for (a, b) in zz for v in (a + b, b, a)][1:])
        return item

    def p1_mm(p, t):
        def item(y):
            cs = twiddles(p)

            def put(ref, n, rs, re, im):
                v = jnp.stack([re.reshape(2, 8, 128), im.reshape(2, 8, 128)], axis=1)
                ref[n * 8 + p, rs * 32:(rs + 1) * 32] = v.reshape(32, 128)

            first = first_lanes(t)
            for rs in range(4):
                k1, k2, k3 = d_products(sa_ref, 0, t, slice(rs * 64, (rs + 1) * 64))
                if t == 0:
                    up = jnp.where(first, k2, k3)
                    re, im = jnp.where(first, k3, k2), pltpu.roll(up, 126, 1)
                    ny = jnp.where(lane0, im, up)
                    u = [ny[q * 16:(q + 1) * 16] for q in range(4)]
                    odd_lane = (lane & 1) == 1
                    nr = jnp.where(odd_lane, pltpu.roll(u[0] - u[2], 1, 1), u[0] + u[2] + (u[1] + u[3]) * sgn0)
                    ni = jnp.where(odd_lane, pltpu.roll((u[3] - u[1]) * sgn0, 1, 1), 0.0)
                    rows = pl.ds(pl.multiple_of(p * 64 + rs * 16, 16), 16)
                    c, sn = tv_ref[0, rows], tv_ref[1, rows]
                    put(ny_ref, 0, rs, nr * c + ni * sn, ni * c - nr * sn)
                    im = jnp.where(lane0, 0.0, im)
                else:
                    re, im = k1 + k2, (k3 - k1) * jnp.where(first, 1.0, -1.0)
                a = _dft4([(re[q * 16:(q + 1) * 16], im[q * 16:(q + 1) * 16]) for q in range(4)])
                for jq in range(4):
                    re, im = a[jq]
                    if jq > 0:
                        c, sn = cs[jq]
                        re, im = re * c + im * sn, im * c - re * sn
                    put(ub_ref, t * 4 + jq, rs, re, im)
        return item

    def p2_bfly(u, g, inverse, ref=ub_ref):
        def item(y):
            if y is not None:
                ub_ref[136, pin_rows(0), :] = y
            v = ref[pl.ds(u * 8, 8), g * 16:(g + 1) * 16]
            x = [(v[p, 0:8], v[p, 8:16]) for p in range(8)]
            x = _swap(_dft8(_swap(x))) if inverse else _dft8(x)
            ref[pl.ds(u * 8, 8), g * 16:(g + 1) * 16] = jnp.stack([w for c in x for w in c]).reshape(8, 16, 128)
        return item

    def filtered(xx, w):
        wr = pltpu.bitcast(w & jnp.uint32(0xFFFF0000), f32).reshape(8, 8, 128)
        wi = pltpu.bitcast(w << 16, f32).reshape(8, 8, 128)
        xx = xx.reshape(8, 2, 8, 128)
        xr, xi = xx[:, 0], xx[:, 1]
        return jnp.stack([xr * wr - xi * wi, xr * wi + xi * wr], axis=1).reshape(128, 128)

    def p2_fwd(u, jps):
        def item(y):
            t = u >> 2
            jq = u & 3
            xs = [_dot(_tobf(ms_ref[jq + 4 * jp]), ub_ref[u * 8 + jp].astype(bf16)) for jp in jps]
            for jp, xx in zip(jps, xs):
                ub_ref[u * 8 + jp] = filtered(xx, wp_ref[pl.ds(t * 2560 + jq + 4 * jp, 64, stride=40), :])
        return item

    def p2_nyq(u):
        def item(y):
            jp = u & 7
            rhs = ny_ref[jp].astype(bf16)
            xx = jnp.concatenate([_dot(_tobf(ms_ref[u * 4, m * 16:(m + 1) * 16]), rhs) for m in range(4)], axis=0)
            w = wp_ref[pl.ds(4 * 2560 + 4 * jp, 64, stride=40), :]
            for jq in range(1, 4):
                w = jnp.where(lane == jq, wp_ref[pl.ds(4 * 2560 + 4 * jp + jq, 64, stride=40), :], w)
            w = jnp.where(u < 8, w, jnp.uint32(0x3F800000))
            ny_ref[jp] = filtered(xx, w)
        return item

    def p2_inv(u, jps):
        def item(y):
            jq = u & 3
            zs = [_dot(_tobf(ms_ref[32 + jq + 4 * jp]), ub_ref[u * 8 + jp].astype(bf16)) for jp in jps]
            for jp, zz in zip(jps, zs):
                ub_ref[u * 8 + jp] = zz
        return item

    def p3_pre(p, g, t):
        def item(y):
            sa_ref[7, pin_rows(256), :] = y
            cs = twiddles(p)

            def fetch(t):
                a = []
                for jq in range(4):
                    v = ub_ref[(t * 4 + jq) * 8 + p, g * 16:(g + 1) * 16]
                    re, im = v[0:8], v[8:16]
                    if jq > 0:
                        c, sn = cs[jq]
                        re, im = re * c - im * sn, im * c + re * sn
                    a.append((re, im))
                return _swap(_dft4(_swap(a)))

            u = fetch(t)
            if t == 0:
                v = ny_ref[p, g * 16:(g + 1) * 16]
                rows = pl.ds(pl.multiple_of(p * 64 + g * 8, 8), 8)
                c, sn = tv_ref[0, rows], tv_ref[1, rows]
                nr, ni = v[0:8] * c - v[8:16] * sn, v[8:16] * c + v[0:8] * sn
                zr, zi = pltpu.roll(nr, 127, 1), pltpu.roll(ni, 127, 1)
                ny = (nr + zr, (nr - zi) * sgn0, nr - zr, (nr + zi) * sgn0)
            first = first_lanes(t)
            for q in range(4):
                re, im = u[q]
                rows = slice(q * 64 + g * 8, q * 64 + (g + 1) * 8)
                if t == 0:
                    im = pltpu.roll(jnp.where(lane0, ny[q], im), 2, 1) + jnp.where(lane == 2, ny[q], 0.0)
                    sa_ref[1:3, rows] = jnp.stack((jnp.where(first, im, re), jnp.where(first, re, im)))
                else:
                    im = im * jnp.where(first, 1.0, -1.0)
                    sa_ref[3 * t:3 * t + 3, rows] = jnp.stack((re + im, im, re))
        return item

    def p3_mm(p, q):
        def item(y):
            g = []
            for t in range(4):
                k1, k2, k3 = d_products(sa_ref, 1, t, slice(q * 64, (q + 1) * 64))
                g.append((k3, k2) if t == 0 else (k2 + k1, k3 - k1))
            yy = _r8_real_t(g)
            bx_ref[q, pl.ds(pl.multiple_of(p * 64, 64), 64), :] = jnp.concatenate(yy, axis=1).astype(bf16)
        return item

    def b_out(p):
        def item(y):
            rows = pl.ds(pl.multiple_of(p * 64, 64), 64)
            pltpu.make_async_copy(bx_ref.at[0:4, rows, :], out_hbm.at[:, rows, pl.ds(DM, DM)],
                                  sem_out.at[1]).start()
            bx_ref[4, pin_rows(0), 0:128] = y.astype(bf16)
        return item

    def step(pp, odd, mem, hooks):
        r0 = pl.multiple_of(pp * 64 + 32 * odd, SEG)
        xs = xo_ref[pl.ds(r0, SEG), :]
        x_lo = xs[0:8].astype(f32)
        hm = jnp.concatenate(
            [jnp.concatenate([x_lo, jnp.concatenate(mem, axis=1)], axis=0).astype(bf16), xs[16:32]], axis=0)
        fill = fillo_ref[:, 0:64] if odd else fille_ref[:, 0:48]
        nrow = 48 if odd else 32
        qkv, ps = {}, {}

        def do_qkv(h0, h1):
            for h in range(h0, h1):
                for t in range(3):
                    n = t * H + slot_of(h)
                    y32 = _dot(hm, _tobf(w_refs[n // 16][n % 16, 0:512]))
                    y = y32.astype(bf16)
                    parts = [y]
                    if odd or t > 0:
                        parts.append(_tobf(qkvc_ref[pp, n]))
                    if t > 0:
                        if odd:
                            parts.append(_tobf(kve_ref[(t - 1) * H + h]))
                        else:
                            kve_ref[(t - 1) * H + h] = _tou(y[0:16])
                    qkv[(t, h)] = jnp.concatenate(parts, axis=0) if len(parts) > 1 else y
                for item in hooks.get(h, ()):
                    item(y32[0:8])

        def do_s(g):
            for h in range(g * G, (g + 1) * G):
                sc = jax.lax.dot_general(qkv[(0, h)], qkv[(1, h)], (((1,), (1,)), ((), ())),
                                         preferred_element_type=f32)
                sc = jnp.where(fill == 0.0, sc * scale, fill)
                e = jnp.exp(sc - jnp.max(sc, axis=1, keepdims=True))
                den = jnp.sum(e, axis=1, keepdims=True)
                r = pl.reciprocal(den, approx=True)
                r = r * (2.0 - den * r)
                ps[h] = (e * r).astype(bf16)

        def do_pv(g):
            for h in range(g * G, (g + 1) * G):
                oall_ref[0:nrow // 2, h * DH:(h + 1) * DH] = _tou(_dot(ps[h], qkv[(2, h)]).astype(bf16))

        def do_o(j, h0, h1):
            return _dot(_tobf(oall_ref[0:nrow // 2, h0 * DH:h1 * DH]), _tobf(wo_ref[j, h0 * 64:h1 * 64, :]))

        for g in range(NG):
            do_qkv(g * G, g * G + G // 2)
            if g >= 1:
                do_s(g - 1)
            do_qkv(g * G + G // 2, (g + 1) * G)
            if g >= 2:
                do_pv(g - 2)
        part = {}
        for j in range(8):
            items = hooks.get(('o', j), ())
            if len(items) == 1:
                part[j] = do_o(j, 0, OSPLIT)
                items[0](None)
            elif items:
                half = do_o(j, 0, OSPLIT // 2)
                items[0](half[0:8])
                part[j] = do_o(j, OSPLIT // 2, OSPLIT) + half
                items[1](part[j][0:8])
            else:
                part[j] = do_o(j, 0, OSPLIT)
            if j == 2:
                do_s(NG - 1)
                do_pv(NG - 2)
            if j == 5:
                do_pv(NG - 1)
        new_mem = []
        for j in range(8):
            cols = slice(j * 128, (j + 1) * 128)
            res = do_o(j, OSPLIT, H) + part[j]
            new_mem.append(res[8:16])
            if odd:
                xo_ref[pl.ds(r0, SEG), cols] = jnp.concatenate(
                    [res[0:8], res[40:48], res[16:32]], axis=0).astype(bf16)
                xo_ref[pl.ds(r0 - 24, 8), cols] = res[32:40].astype(bf16)
            else:
                xo_ref[pl.ds(r0, SEG), cols] = res.astype(bf16)
        for item in hooks.get(H, ()):
            item(None)
        if odd:
            pltpu.make_async_copy(
                xo_ref.at[pl.ds(pl.multiple_of(pp * 64, 64), 64), :],
                out_hbm.at[pp >> 3, pl.ds(pl.multiple_of((pp & 7) * 64, 64), 64), pl.ds(0, DM)],
                sem_out.at[0]).start()
        return new_mem

    def l1(i, mem):
        he = {2 * k: [p1_pre(i, k // 4, k % 4)] for k in range(16)}
        he[H] = [p1_mm(i, 1)]
        ho = {('o', 0): [p1_mm(i, 2)], ('o', 3): [p1_mm(i, 3)], ('o', 5): [p1_mm(i, 0)]}
        mem = step(i, 0, mem, he)
        mem = step(i, 1, mem, ho)
        return mem

    def l2(i, mem):
        u = i - N_L1
        he = {3: [p2_fwd(u, range(0, 4))], 7: [p2_fwd(u, range(4, 8))], 17: [p2_nyq(u)],
              H: [p2_inv(u, range(0, 8))]}
        ho = {('o', j): [p2_bfly(u, j, True), p2_bfly(u + 1, j, False)] for j in range(8)}
        mem = step(i, 0, mem, he)
        mem = step(i, 1, mem, ho)
        return mem

    def l3(i, mem):
        p = i - N_L1 - N_L2
        he = {h: [p3_pre(p, h // 3, 1 + h % 3)] for h in range(24)}
        for j in range(4):
            he[('o', 3 + j)] = [p3_pre(p, 2 * j, 0), p3_pre(p, 2 * j + 1, 0)]
        he[H] = [p3_mm(p, q) for q in range(4)]
        ho = {12: [b_out(p)]}
        mem = step(i, 0, mem, he)
        mem = step(i, 1, mem, ho)
        return mem

    m0 = mem_ref[...].astype(f32)
    mem = [m0[:, j * 128:(j + 1) * 128] for j in range(8)]
    mem = jax.lax.fori_loop(0, N_L1, l1, mem)
    cp_ms.wait()
    for g in range(8):
        p2_bfly(0, g, False)(None)
        p2_bfly(0, g, False, ny_ref)(None)
    mem = jax.lax.fori_loop(N_L1, N_L1 + N_L2, l2, mem)
    for g in range(8):
        p2_bfly(0, g, True, ny_ref)(None)
    mem = jax.lax.fori_loop(N_L1 + N_L2, NSEG // 2, l3, mem)

    pltpu.make_async_copy(bx_ref.at[0:4], out_hbm.at[:, :, pl.ds(DM, DM)], sem_out.at[1]).wait()
    pltpu.make_async_copy(xo_ref, xo_ref, sem_out.at[0]).wait()


@jax.jit
def _run(x, mem0, wq, wk, wv, wo, bx, w_r, w_i):
    fd, ms, tv = _tables()
    hbm = pl.BlockSpec(memory_space=pl.ANY)
    out = pl.pallas_call(
        _kernel,
        out_shape=jax.ShapeDtypeStruct((4, S // 4, 2 * DM), bf16),
        in_specs=[hbm] * 13,
        out_specs=hbm,
        scratch_shapes=[
            pltpu.VMEM((S, DM), bf16),
            pltpu.VMEM((MEM, DM), bf16),
            pltpu.VMEM((8, NSEG, 8, 128), bf16),
            pltpu.VMEM((4, DM, 16, DH), bf16),
        ] + [pltpu.VMEM((16, DM // 2 + 8, DH), u32)] * 6 + [
            pltpu.VMEM((H * DH, DM), bf16),
            pltpu.VMEM((8, H * DH // 2 + 8, 128), u32),
            pltpu.VMEM((8, 256, 128), u32),
            pltpu.VMEM((NSEG // 2, 3 * H, 8, 128), u32),
            pltpu.VMEM((2 * H, 8, 128), u32),
            pltpu.VMEM((24, H * DH), u32),
            pltpu.VMEM((32, 128), f32),
            pltpu.VMEM((48, 128), f32),
            pltpu.VMEM((5, S // 4, DM), bf16),
            pltpu.VMEM((16, DM // 2 + 1, 256), bf16),
            pltpu.VMEM((12840, 128), u32),
            pltpu.VMEM((137, 128, 128), f32),
            pltpu.VMEM((8, 128, 128), f32),
            pltpu.VMEM((12, 264, 128), f32),
            pltpu.VMEM((24, 64, 128), u32),
            pltpu.VMEM((64, 64, 128), u32),
            pltpu.VMEM((2, 512, 128), f32),
            pltpu.SMEM((64,), f32),
            pltpu.SMEM((1,), jnp.int32),
            pltpu.SemaphoreType.DMA((64,)),
            pltpu.SemaphoreType.DMA((2,)),
        ],
        compiler_params=pltpu.CompilerParams(vmem_limit_bytes=120 * 1024 * 1024,
                                             disable_semaphore_checks=True,
                                             disable_bounds_checks=True),
    )(x.reshape(S, DM), x.reshape(NSEG, SEG, DM), mem0.reshape(MEM, DM), wq, wk, wv,
      wo.reshape(H * DH, DM), bx.reshape(4, S // 4, DM), w_r.T, w_i.T, jnp.asarray(fd), jnp.asarray(ms), jnp.asarray(tv))
    return out.reshape(1, S, 2 * DM)


def pallas_concat_heads__memory_aug_recurrent_mem_tr__spectral_gfnet__prompt_kernel(
    A_x: jax.Array,
    A_mem0: jax.Array,
    A_Wq: jax.Array,
    A_Wk: jax.Array,
    A_Wv: jax.Array,
    A_Wo: jax.Array,
    A_seg_len,
    B_x: jax.Array,
    B_w_r: jax.Array,
    B_w_i: jax.Array,
):
    if isinstance(A_seg_len, int):
        assert A_seg_len == SEG
    assert A_x.shape == (1, S, DM) and A_mem0.shape == (1, MEM, DM) and A_Wq.shape == (DM, H, DH)
    assert B_x.shape == (1, S, DM) and B_w_r.shape == (S, DM // 2 + 1)
    return _run(A_x, A_mem0, A_Wq, A_Wk, A_Wv, A_Wo, B_x, B_w_r, B_w_i)
```

```python
import math

import numpy as np
import jax
import jax.numpy as jnp
import jax.experimental.pallas as pl
import jax.experimental.pallas.tpu as pltpu

bf16 = jnp.bfloat16
f32 = jnp.float32
u32 = jnp.uint32

S, DM = 2048, 1024
H, DH = 32, 128
MEM, SEG = 8, 32
NSEG = S // SEG
SQH = math.sqrt(0.5)

_PAIRS = ((0, 4), (1, 7), (2, 6), (3, 5))
_FIRST = np.array([[1, 1, 0, 0], [1, 0, 1, 0], [0, 1, 1, 0], [0, 1, 0, 1]], bool)


def _pack_rows(a):
    u = np.ascontiguousarray(a, dtype=np.float32).view(np.uint32).astype(np.uint64)
    b = ((u + 0x7FFF + ((u >> 16) & 1)) >> 16).astype(np.uint32)
    return (b[..., 0::2, :] | (b[..., 1::2, :] << 16)).astype(np.uint32)


def _tables():
    k2 = np.zeros((4, 128), np.int64)
    for t in range(4):
        odd = t % 2
        for lam in range(128):
            k = 2 * lam + odd
            if k % 8 not in _PAIRS[t]:
                k = 2 * (128 + 8 * (lam // 8) + (lam % 8 - 1 - odd) % 8) + odd
            assert k % 8 in _PAIRS[t]
            k2[t, lam] = k
    b = np.arange(128)[:, None]
    F = np.zeros((12, 128, 128))
    G = np.zeros((12, 128, 128))
    for t in range(4):
        th = 2 * np.pi * ((b * k2[t][None, :]) % DM) / DM
        C, Sn = np.cos(th), np.sin(th)
        first = ((k2[t] % 8) == _PAIRS[t][0])[None, :]
        assert np.array_equal(first[0], _FIRST[t][np.arange(128) % 4])
        if t == 0:
            im = -Sn
            im[:, 0] = (-1.0) ** np.arange(128)
            im = np.roll(im, 2, axis=1)
            F[1:3] = np.where(first, im, C), np.where(first, C, im)
            G[1:3] = F[1:3]
            G[2, :, 0] *= 0.5
            G[2, :, 2] *= 0.5
        else:
            Sg = np.where(first, Sn, -Sn)
            F[3 * t:3 * t + 3] = C, -(C + Sg), C - Sg
            G[3 * t:3 * t + 3] = F[3 * t:3 * t + 3]
    Finv = np.transpose(G, (0, 2, 1)) * (2.0 / DM)
    fd = _pack_rows(np.concatenate([F, Finv]))
    M = np.zeros((32, 128, 128))
    r = np.arange(64)[None, :]
    l = np.arange(64)[:, None]
    for j in range(32):
        th = 2 * np.pi * ((r * (j + 32 * l)) % S) / S
        C, Sn = np.cos(th), np.sin(th)
        M[j, :64, :64] = C
        M[j, :64, 64:] = Sn
        M[j, 64:, :64] = -Sn
        M[j, 64:, 64:] = C
    perm = np.arange(128).reshape(2, 8, 8).transpose(1, 0, 2).reshape(128)
    M = M[:, perm][:, :, perm]
    Minv = np.transpose(M, (0, 2, 1)) / S
    ms = _pack_rows(np.concatenate([M, Minv]))
    th = 2 * np.pi * np.outer(np.arange(512), np.arange(128) % 4) / S
    tv = np.stack([np.cos(th), np.sin(th)]).astype(np.float32)
    return fd, ms, tv


def _tobf(w):
    return pltpu.bitcast(w, bf16)


def _tou(w):
    return pltpu.bitcast(w, u32)


def _dot(a, b):
    return jnp.dot(a, b, preferred_element_type=f32)


def _r8_real(x):
    t0, t1 = x[0] + x[4], x[0] - x[4]
    t2, t3 = x[2] + x[6], x[2] - x[6]
    t4, t5 = x[1] + x[5], x[1] - x[5]
    t6, t7 = x[3] + x[7], x[3] - x[7]
    e0, e1 = t0 + t2, t0 - t2
    o0, o1 = t4 + t6, t4 - t6
    u, v = SQH * (t5 - t7), SQH * (t5 + t7)
    return [(e0 + o0, e0 - o0), (t1 + u, v + t3), (e1, o1), (t1 - u, v - t3)]


def _r8_real_t(g):
    (z0, z4), (a1, b1), (e1, o1), (a3, b3) = g
    e0, o0 = z0 + z4, z0 - z4
    t1, u = a1 + a3, a1 - a3
    v, t3 = b1 + b3, b1 - b3
    t5, t7 = SQH * (v + u), SQH * (v - u)
    t0, t2 = e0 + e1, e0 - e1
    t4, t6 = o0 + o1, o0 - o1
    return [t0 + t1, t4 + t5, t2 + t3, t6 + t7, t0 - t1, t4 - t5, t2 - t3, t6 - t7]


def _dft4(u):
    (r0, i0), (r1, i1), (r2, i2), (r3, i3) = u
    sr, si, dr, di = r0 + r2, i0 + i2, r0 - r2, i0 - i2
    tr, ti, er, ei = r1 + r3, i1 + i3, r1 - r3, i1 - i3
    return [(sr + tr, si + ti), (dr + ei, di - er), (sr - tr, si - ti), (dr - ei, di + er)]


def _dft8(x):
    a = [(x[p][0] + x[p + 4][0], x[p][1] + x[p + 4][1]) for p in range(4)]
    d = [(x[p][0] - x[p + 4][0], x[p][1] - x[p + 4][1]) for p in range(4)]
    ev = _dft4(a)
    (r0, i0), (r1, i1), (r2, i2), (r3, i3) = d
    b1r, b1i = SQH * (r1 + i1), SQH * (i1 - r1)
    b3r, n3i = SQH * (i3 - r3), SQH * (r3 + i3)
    sr, si, dr, di = r0 + i2, i0 - r2, r0 - i2, i0 + r2
    tr, ti, er, ei = b1r + b3r, b1i - n3i, b1r - b3r, b1i + n3i
    od = [(sr + tr, si + ti), (dr + ei, di - er), (sr - tr, si - ti), (dr - ei, di + er)]
    return [ev[0], od[0], ev[1], od[1], ev[2], od[2], ev[3], od[3]]


def _swap(x):
    return [(b, a) for (a, b) in x]


G = 4
NG = H // G
OSPLIT = 24
NEG = -1e9
N_L1, N_L2, N_L3 = 8, 16, 8


def _kernel(x_hbm, x3_hbm, mem_hbm, wq_hbm, wk_hbm, wv_hbm, wo_hbm, bx_hbm, wr_hbm, wi_hbm,
            fd_hbm, ms_hbm, tv_hbm, out_hbm,
            xo_ref, mem_ref, xcraw_ref, raw_ref, w0_ref, w1_ref, w2_ref, w3_ref, w4_ref, w5_ref,
            woraw_ref, wo_ref, xc_ref, qkvc_ref, kve_ref,
            oall_ref, fille_ref, fillo_ref, bx_ref, wt_ref, wp_ref, ub_ref, ny_ref, sa_ref, fd_ref, ms_ref, tv_ref,
            tw_ref, zero_ref, sem_in, sem_out):
    scale = DH ** -0.5
    w_hbm = (wq_hbm, wk_hbm, wv_hbm)
    w_refs = (w0_ref, w1_ref, w2_ref, w3_ref, w4_ref, w5_ref)

    def raw_copy(c, i=0, nd=DM):
        rows = pl.ds(pl.multiple_of(i * nd, nd), nd)
        return pltpu.make_async_copy(
            w_hbm[c // 2].at[rows, pl.ds((c % 2) * 16, 16), :],
            raw_ref.at[c % 4, rows], sem_in.at[8 + min(c, 3) * 8 + max(c - 3, 0) * 2 + i])

    def xc_copy(k):
        return pltpu.make_async_copy(
            x3_hbm.at[:, pl.ds(8, 8), pl.ds(pl.multiple_of(k * 128, 128), 128)], xcraw_ref.at[k], sem_in.at[40 + k])

    cp_x = pltpu.make_async_copy(x_hbm, xo_ref, sem_in.at[0])
    cp_mem = pltpu.make_async_copy(mem_hbm, mem_ref, sem_in.at[1])
    cp_wo = pltpu.make_async_copy(wo_hbm, woraw_ref, sem_in.at[2])
    cp_bx = pltpu.make_async_copy(bx_hbm, bx_ref.at[0:4], sem_in.at[3])
    cp_fd = pltpu.make_async_copy(fd_hbm, fd_ref, sem_in.at[4])
    cp_ms = pltpu.make_async_copy(ms_hbm, ms_ref, sem_in.at[5])
    cp_tv = pltpu.make_async_copy(tv_hbm, tv_ref, sem_in.at[6])
    cp_wt = [pltpu.make_async_copy(src.at[:, pl.ds(lg * 256, 256)], wt_ref.at[a * 8 + lg], sem_in.at[48 + a * 8 + lg])
             for a, src in enumerate((wr_hbm, wi_hbm)) for lg in range(8)]

    for i in range(8):
        raw_copy(0, i, 128).start()
        xc_copy(i).start()
        if i >= 3:
            raw_copy(2, i - 3, 128).start()
        if i == 7:
            raw_copy(2, 5, 128).start()
        raw_copy(1, i, 128).start()
    for i in range(6, 8):
        raw_copy(2, i, 128).start()
    for i in range(2):
        raw_copy(3, i, 512).start()
    for cp in cp_wt + [cp_wo, cp_x, cp_mem, cp_bx, cp_fd, cp_tv, cp_ms]:
        cp.start(priority=1)

    zero_ref[0] = 0

    def pin_slot(n):
        return n - jnp.clip(zero_ref[0], 0, 1) * 4

    def pin_rows(r):
        return pl.ds(pl.multiple_of(r + jnp.clip(zero_ref[0], 0, 1) * 32, 8), 8)

    for p in range(8):
        for jq in range(4):
            tw_ref[(p * 4 + jq) * 2] = jnp.float32(math.cos(2 * math.pi * p * jq / 32))
            tw_ref[(p * 4 + jq) * 2 + 1] = jnp.float32(math.sin(2 * math.pi * p * jq / 32))

    ub_ref[128:136] = jnp.zeros((8, 128, 128), f32)
    wp_ref[12800:12872] = jnp.zeros((72, 128), u32)

    qi = jax.lax.broadcasted_iota(jnp.int32, (48, 128), 0)
    ki = jax.lax.broadcasted_iota(jnp.int32, (48, 128), 1)

    def between(v, lo, hi):
        return (v >= lo) & (v < hi)

    def table(keep, other):
        return jnp.where(other, -jnp.inf, jnp.where(keep, 0.0, NEG)).astype(f32)

    keep = between(qi, 8, 16) | between(ki, 8, 16) | (qi >= jnp.where(ki < 32, ki, ki - 24))
    fille_ref[...] = table(keep, ki >= 40)[:32]
    q_even = between(qi, 32, 40)
    k_even = between(ki, 32, 40) | (ki >= 48)
    qpos = jnp.where(qi < 32, qi, jnp.where(qi < 40, qi - 24, qi - 32))
    kpos = jnp.where(ki < 32, ki, jnp.where(ki < 40, ki - 24, jnp.where(ki < 48, ki - 32, ki - 48)))
    keep = between(qi, 8, 16) | between(ki, 8, 16) | (ki >= 56) | (qpos >= kpos)
    fillo_ref[...] = table(keep, (q_even != k_even) | (ki >= 64))

    def relayout16(c, blk):
        w0 = pl.multiple_of(blk * 8, 8)
        v = _tou(raw_ref[c % 4, pl.ds(blk * 16, 16)]).reshape(8, 2, 8, 128)
        a, b = v[:, 0], v[:, 1]
        w_refs[c][0:8, pl.ds(w0, 8), :] = jnp.swapaxes((a & jnp.uint32(0xFFFF)) | (b << 16), 0, 1)
        w_refs[c][8:16, pl.ds(w0, 8), :] = jnp.swapaxes((a >> 16) | (b & jnp.uint32(0xFFFF0000)), 0, 1)

    def slot_of(h):
        return (h // 16) * 16 + (h % 2) * 8 + (h % 16) // 2

    def repack_wo64(blk):
        v = _tou(woraw_ref[pl.ds(pl.multiple_of(blk * 64, 64), 64), :])
        wo_ref[:, pl.ds(pl.multiple_of(blk * 32, 32), 32), :] = jnp.stack(
            [v[:, j * 128:(j + 1) * 128] for j in range(8)])

    sub4 = jax.lax.broadcasted_iota(jnp.int32, (128, 128), 0) & 3

    def wp_store(t, kb, tile):
        v = tile.T.reshape(4, 32, 128)
        v = jnp.concatenate([v, v[:, 0:8]], axis=1).reshape(160, 128)
        wp_ref[pl.ds(pl.multiple_of(t * 2560 + kb * 160, 32), 160), :] = v

    def b_prep(lg, hb, par):
        cols = slice(hb * 128, (hb + 1) * 128)
        a = _tou(wt_ref[lg, 0:512, cols])
        b = _tou(wt_ref[8 + lg, 0:512, cols])
        if par == 0:
            w = (a << 16) | (b & jnp.uint32(0xFFFF))
            m = (sub4 == 0) | (sub4 == 2)
        else:
            w = (a & jnp.uint32(0xFFFF0000)) | (b >> 16)
            m = (sub4 == 0) | (sub4 == 3)
        top = w[:128]
        bot = pltpu.roll(w[128:].reshape(16, 8, 128), 1 + par, 1).reshape(128, 128)
        wp_store(par, lg * 2 + hb, jnp.where(m, top, bot))
        wp_store(par + 2, lg * 2 + hb, jnp.where(m, bot, top))
        if par == 0:
            na = jnp.broadcast_to(wt_ref[lg, 512:513, cols].astype(f32), (128, 128))
            nb = jnp.broadcast_to(wt_ref[8 + lg, 512:513, cols].astype(f32), (128, 128))
            wp_store(4, lg * 2 + hb, pltpu.bitcast(na, u32) | (pltpu.bitcast(nb, u32) >> 16))

    def gather_c(k):
        xc_ref[k] = _tou(xcraw_ref[k].astype(f32).reshape(512, 128).astype(bf16))

    def store_qkvc(n, y):
        qkvc_ref[:, n] = y.reshape(NSEG // 2, 8, 128)

    def q_unit(i, groups, first, last, fillers):
        xk = _tobf(xc_ref[i])
        w0 = pl.multiple_of(i * 64, 64)
        for g in groups:
            rhs = jnp.concatenate(
                [_tobf(w_refs[h // 16][h % 16, pl.ds(w0, 64), :]) for h in range(4 * g, 4 * g + 4)], axis=1)
            y = _dot(xk, rhs)
            for h in range(4 * g, 4 * g + 4):
                yh = y[:, (h % 4) * 128:(h % 4 + 1) * 128]
                if not first:
                    yh = yh + ub_ref[h * 4:(h + 1) * 4].reshape(512, 128)
                if last:
                    store_qkvc(h, _tou(yh.astype(bf16)))
                else:
                    ub_ref[h * 4:(h + 1) * 4] = yh.reshape(4, 128, 128)
            mine = fillers.get(g, [])
            for fi, item in enumerate(mine):
                r = (fi * 512 // len(mine)) // 8 * 8
                item(pltpu.bitcast(y[r:r + 8, 0:128], u32))

    def rl_item(c, blk):
        def item(pin):
            w_refs[c][pin_slot(15), 512:520] = pin
            relayout16(c, blk)
        return item

    def spread(fillers, items, groups):
        for k, item in enumerate(items):
            fillers.setdefault(groups[k * len(groups) // len(items)], []).append(item)
        return fillers

    def half_items(f, c, i, groups):
        return spread(f, [rl_item(c, i * 8 + blk) for blk in range(8)], groups)

    def piece_items(i):
        f = half_items(half_items({}, 1, i, (0, 1, 2)), 0, i + 1, (4, 5, 6))
        return spread(f, [lambda pin: gather_c(i + 1)], (7,))

    def chunk2_items(f, lo, hi, groups):
        return spread(f, [rl_item(2, blk) for blk in range(lo, hi)], groups)

    def wait_piece(i):
        raw_copy(1, i, 128).wait()
        xc_copy(i + 1).wait()
        raw_copy(0, i + 1, 128).wait()

    raw_copy(0, 0, 128).wait()
    for blk in range(8):
        relayout16(0, blk)
    xc_copy(0).wait()
    gather_c(0)
    q_unit(0, range(0, 2), True, False, {})
    raw_copy(1, 0, 128).wait()
    q_unit(0, range(2, 4), True, False, half_items({}, 1, 0, (2, 2, 3)))
    q_unit(0, range(4, 6), True, False, {})
    xc_copy(1).wait()
    raw_copy(0, 1, 128).wait()
    q_unit(0, range(6, 8), True, False,
           spread(half_items({}, 0, 1, (6, 6, 7)), [lambda pin: gather_c(1)], (6,)))
    raw_copy(1, 1, 128).wait()
    q_unit(1, range(0, 4), False, False, half_items({}, 1, 1, (0, 1, 2)))
    xc_copy(2).wait()
    raw_copy(0, 2, 128).wait()
    q_unit(1, range(4, 8), False, False,
           spread(half_items({}, 0, 2, (4, 5, 6)), [lambda pin: gather_c(2)], (6,)))

    def q_c(i, carry):
        wait_piece(i)
        raw_copy(2, i - 2, 128).wait()
        q_unit(i, range(8), False, False, half_items(piece_items(i), 2, i - 2, (3, 3, 3, 3, 4, 5, 6, 7)))
        return carry
    jax.lax.fori_loop(2, 6, q_c, 0)

    wait_piece(6)
    raw_copy(2, 4, 128).wait()
    raw_copy(2, 5, 128).wait()
    q_unit(6, range(8), False, False, chunk2_items(piece_items(6), 32, 48, (0, 1, 2, 3, 3, 4, 5, 6)))
    raw_copy(1, 7, 128).wait()
    raw_copy(2, 6, 128).wait()
    raw_copy(2, 7, 128).wait()
    q_unit(7, range(8), False, True, chunk2_items(half_items({}, 1, 7, (0, 1, 2)), 48, 64, (3, 4, 5, 6)))
    raw_copy(4).start()
    raw_copy(5).start()

    def bulk_iter(c, i):
        xc = jnp.concatenate([_tobf(xc_ref[k]) for k in range(8)], axis=1)
        for t in range(8):
            n = i * 8 + t
            y = _tou(_dot(xc, _tobf(w_refs[c][n, 0:512])).astype(bf16))
            store_qkvc(c * 16 + n, y)
            for blk in range(4):
                pin = y[blk * 64:blk * 64 + 8]
                if c + 1 < 6:
                    w_refs[c + 1][pin_slot(15), 512:520] = pin
                    relayout16(c + 1, i * 32 + (t * 4 + blk))
                else:
                    wo_ref[pin_slot(7), 2048:2056] = pin
                    repack_wo64(i * 32 + (t * 4 + blk))
            if c >= 4:
                wp_ref[pin_rows(12832), :] = y[32:40]
                b_prep((c - 4) * 4 + i * 2 + t // 4, (t // 2) % 2, t % 2)

    for c in range(2, 6):
        if c == 4:
            for cp in cp_wt:
                cp.wait()
        if c == 5:
            cp_wo.wait()
        elif c > 2:
            raw_copy(c + 1).wait()

        def bulk(i, carry, c=c):
            if c == 2:
                raw_copy(3, i, 512).wait()
            bulk_iter(c, i)
            return carry
        jax.lax.fori_loop(0, 2, bulk, 0)

    cp_x.wait()
    cp_mem.wait()
    cp_bx.wait()
    cp_fd.wait()
    cp_tv.wait()

    lane = jax.lax.broadcasted_iota(jnp.int32, (1, 128), 1)
    lane0 = lane == 0
    sgn0 = jnp.where(lane0, 1.0, -1.0)

    def first_lanes(t):
        la, lb = [k for k in range(4) if _FIRST[t][k]]
        return ((lane & 3) == la) | ((lane & 3) == lb)

    def d_products(st_ref, d, t, rows):
        return [_dot(st_ref[n, rows].astype(bf16), _tobf(fd_ref[d * 12 + n])) if n else None
                for n in range(3 * t, 3 * t + 3)]

    def twiddles(p):
        return [(tw_ref[p * 8 + jq * 2], tw_ref[p * 8 + jq * 2 + 1]) if jq else None for jq in range(4)]

    def p1_pre(p, rs, q):
        def item(y):
            sa_ref[pin_slot(7), 256:264] = y
            xq = bx_ref[q, pl.ds(pl.multiple_of(p * 64 + rs * 16, 16), 16), :].astype(f32)
            zz = _r8_real([xq[:, a * 128:(a + 1) * 128] for a in range(8)])
            r = (rs * 4 + q) * 16
            sa_ref[1:12, r:r + 16] = jnp.stack([v for (a, b) in zz for v in (a + b, b, a)][1:])
        return item

    def p1_mm(p, t):
        def item(y):
            cs = twiddles(p)

            def put(ref, n, rs, re, im):
                v = jnp.stack([re.reshape(2, 8, 128), im.reshape(2, 8, 128)], axis=1)
                ref[n * 8 + p, rs * 32:(rs + 1) * 32] = v.reshape(32, 128)

            first = first_lanes(t)
            for rs in range(4):
                k1, k2, k3 = d_products(sa_ref, 0, t, slice(rs * 64, (rs + 1) * 64))
                if t == 0:
                    up = jnp.where(first, k2, k3)
                    re, im = jnp.where(first, k3, k2), pltpu.roll(up, 126, 1)
                    ny = jnp.where(lane0, im, up)
                    u = [ny[q * 16:(q + 1) * 16] for q in range(4)]
                    odd_lane = (lane & 1) == 1
                    nr = jnp.where(odd_lane, pltpu.roll(u[0] - u[2], 1, 1), u[0] + u[2] + (u[1] + u[3]) * sgn0)
                    ni = jnp.where(odd_lane, pltpu.roll((u[3] - u[1]) * sgn0, 1, 1), 0.0)
                    rows = pl.ds(pl.multiple_of(p * 64 + rs * 16, 16), 16)
                    c, sn = tv_ref[0, rows], tv_ref[1, rows]
                    put(ny_ref, 0, rs, nr * c + ni * sn, ni * c - nr * sn)
                    im = jnp.where(lane0, 0.0, im)
                else:
                    re, im = k1 + k2, (k3 - k1) * jnp.where(first, 1.0, -1.0)
                a = _dft4([(re[q * 16:(q + 1) * 16], im[q * 16:(q + 1) * 16]) for q in range(4)])
                for jq in range(4):
                    re, im = a[jq]
                    if jq > 0:
                        c, sn = cs[jq]
                        re, im = re * c + im * sn, im * c - re * sn
                    put(ub_ref, t * 4 + jq, rs, re, im)
        return item

    def p2_bfly(u, g, inverse, ref=ub_ref):
        def item(y):
            if y is not None:
                ub_ref[136, pin_rows(0), :] = y
            v = ref[pl.ds(u * 8, 8), g * 16:(g + 1) * 16]
            x = [(v[p, 0:8], v[p, 8:16]) for p in range(8)]
            x = _swap(_dft8(_swap(x))) if inverse else _dft8(x)
            ref[pl.ds(u * 8, 8), g * 16:(g + 1) * 16] = jnp.stack([w for c in x for w in c]).reshape(8, 16, 128)
        return item

    def filtered(xx, w):
        wr = pltpu.bitcast(w & jnp.uint32(0xFFFF0000), f32).reshape(8, 8, 128)
        wi = pltpu.bitcast(w << 16, f32).reshape(8, 8, 128)
        xx = xx.reshape(8, 2, 8, 128)
        xr, xi = xx[:, 0], xx[:, 1]
        return jnp.stack([xr * wr - xi * wi, xr * wi + xi * wr], axis=1).reshape(128, 128)

    def p2_fwd(u, jps):
        def item(y):
            t = u >> 2
            jq = u & 3
            xs = [_dot(_tobf(ms_ref[jq + 4 * jp]), ub_ref[u * 8 + jp].astype(bf16)) for jp in jps]
            for jp, xx in zip(jps, xs):
                ub_ref[u * 8 + jp] = filtered(xx, wp_ref[pl.ds(t * 2560 + jq + 4 * jp, 64, stride=40), :])
        return item

    def p2_nyq(u):
        def item(y):
            jp = u & 7
            rhs = ny_ref[jp].astype(bf16)
            xx = jnp.concatenate([_dot(_tobf(ms_ref[u * 4, m * 16:(m + 1) * 16]), rhs) for m in range(4)], axis=0)
            w = wp_ref[pl.ds(4 * 2560 + 4 * jp, 64, stride=40), :]
            for jq in range(1, 4):
                w = jnp.where(lane == jq, wp_ref[pl.ds(4 * 2560 + 4 * jp + jq, 64, stride=40), :], w)
            w = jnp.where(u < 8, w, jnp.uint32(0x3F800000))
            ny_ref[jp] = filtered(xx, w)
        return item

    def p2_inv(u, jps):
        def item(y):
            jq = u & 3
            zs = [_dot(_tobf(ms_ref[32 + jq + 4 * jp]), ub_ref[u * 8 + jp].astype(bf16)) for jp in jps]
            for jp, zz in zip(jps, zs):
                ub_ref[u * 8 + jp] = zz
        return item

    def p3_pre(p, g, t):
        def item(y):
            sa_ref[pin_slot(7), 256:264] = y
            cs = twiddles(p)

            def fetch(t):
                a = []
                for jq in range(4):
                    v = ub_ref[(t * 4 + jq) * 8 + p, g * 16:(g + 1) * 16]
                    re, im = v[0:8], v[8:16]
                    if jq > 0:
                        c, sn = cs[jq]
                        re, im = re * c - im * sn, im * c + re * sn
                    a.append((re, im))
                return _swap(_dft4(_swap(a)))

            u = fetch(t)
            if t == 0:
                v = ny_ref[p, g * 16:(g + 1) * 16]
                rows = pl.ds(pl.multiple_of(p * 64 + g * 8, 8), 8)
                c, sn = tv_ref[0, rows], tv_ref[1, rows]
                nr, ni = v[0:8] * c - v[8:16] * sn, v[8:16] * c + v[0:8] * sn
                zr, zi = pltpu.roll(nr, 127, 1), pltpu.roll(ni, 127, 1)
                ny = (nr + zr, (nr - zi) * sgn0, nr - zr, (nr + zi) * sgn0)
            first = first_lanes(t)
            for q in range(4):
                re, im = u[q]
                rows = slice(q * 64 + g * 8, q * 64 + (g + 1) * 8)
                if t == 0:
                    im = pltpu.roll(jnp.where(lane0, ny[q], im), 2, 1) + jnp.where(lane == 2, ny[q], 0.0)
                    sa_ref[1:3, rows] = jnp.stack((jnp.where(first, im, re), jnp.where(first, re, im)))
                else:
                    im = im * jnp.where(first, 1.0, -1.0)
                    sa_ref[3 * t:3 * t + 3, rows] = jnp.stack((re + im, im, re))
        return item

    def p3_mm(p, q):
        def item(y):
            g = []
            for t in range(4):
                k1, k2, k3 = d_products(sa_ref, 1, t, slice(q * 64, (q + 1) * 64))
                g.append((k3, k2) if t == 0 else (k2 + k1, k3 - k1))
            yy = _r8_real_t(g)
            bx_ref[q, pl.ds(pl.multiple_of(p * 64, 64), 64), :] = jnp.concatenate(yy, axis=1).astype(bf16)
        return item

    def b_out(p):
        def item(y):
            rows = pl.ds(pl.multiple_of(p * 64, 64), 64)
            pltpu.make_async_copy(bx_ref.at[0:4, rows, :], out_hbm.at[:, rows, pl.ds(DM, DM)],
                                  sem_out.at[1]).start()
            bx_ref[4, pin_rows(0), 0:128] = y.astype(bf16)
        return item

    def step(pp, odd, mem, hooks):
        r0 = pl.multiple_of(pp * 64 + 32 * odd, SEG)
        xs = xo_ref[pl.ds(r0, SEG), :]
        x_lo = xs[0:8].astype(f32)
        hm = jnp.concatenate(
            [jnp.concatenate([x_lo, jnp.concatenate(mem, axis=1)], axis=0).astype(bf16), xs[16:32]], axis=0)
        fill = fillo_ref[:, 0:64] if odd else fille_ref[:, 0:48]
        nrow = 48 if odd else 32
        qkv, ps = {}, {}

        def do_qkv(h0, h1):
            for h in range(h0, h1):
                for t in range(3):
                    n = t * H + slot_of(h)
                    y32 = _dot(hm, _tobf(w_refs[n // 16][n % 16, 0:512]))
                    y = y32.astype(bf16)
                    parts = [y]
                    if odd or t > 0:
                        parts.append(_tobf(qkvc_ref[pp, n]))
                    if t > 0:
                        if odd:
                            parts.append(_tobf(kve_ref[(t - 1) * H + h]))
                        else:
                            kve_ref[(t - 1) * H + h] = _tou(y[0:16])
                    qkv[(t, h)] = jnp.concatenate(parts, axis=0) if len(parts) > 1 else y
                for item in hooks.get(h, ()):
                    item(y32[0:8])

        def do_s(g):
            for h in range(g * G, (g + 1) * G):
                sc = jax.lax.dot_general(qkv[(0, h)], qkv[(1, h)], (((1,), (1,)), ((), ())),
                                         preferred_element_type=f32)
                sc = jnp.where(fill == 0.0, sc * scale, fill)
                e = jnp.exp(sc - jnp.max(sc, axis=1, keepdims=True))
                den = jnp.sum(e, axis=1, keepdims=True)
                r = pl.reciprocal(den, approx=True)
                r = r * (2.0 - den * r)
                ps[h] = (e * r).astype(bf16)

        def do_pv(g):
            for h in range(g * G, (g + 1) * G):
                oall_ref[0:nrow // 2, h * DH:(h + 1) * DH] = _tou(_dot(ps[h], qkv[(2, h)]).astype(bf16))

        def do_o(j, h0, h1):
            return _dot(_tobf(oall_ref[0:nrow // 2, h0 * DH:h1 * DH]), _tobf(wo_ref[j, h0 * 64:h1 * 64, :]))

        for g in range(NG):
            do_qkv(g * G, g * G + G // 2)
            if g >= 1:
                do_s(g - 1)
            do_qkv(g * G + G // 2, (g + 1) * G)
            if g >= 2:
                do_pv(g - 2)
        part = {}
        for j in range(8):
            items = hooks.get(('o', j), ())
            if len(items) == 1:
                part[j] = do_o(j, 0, OSPLIT)
                items[0](None)
            elif items:
                half = do_o(j, 0, OSPLIT // 2)
                items[0](half[0:8])
                part[j] = do_o(j, OSPLIT // 2, OSPLIT) + half
                items[1](part[j][0:8])
            else:
                part[j] = do_o(j, 0, OSPLIT)
            if j == 2:
                do_s(NG - 1)
                do_pv(NG - 2)
            if j == 5:
                do_pv(NG - 1)
        new_mem = []
        for j in range(8):
            cols = slice(j * 128, (j + 1) * 128)
            res = do_o(j, OSPLIT, H) + part[j]
            new_mem.append(res[8:16])
            if odd:
                xo_ref[pl.ds(r0, SEG), cols] = jnp.concatenate(
                    [res[0:8], res[40:48], res[16:32]], axis=0).astype(bf16)
                xo_ref[pl.ds(r0 - 24, 8), cols] = res[32:40].astype(bf16)
            else:
                xo_ref[pl.ds(r0, SEG), cols] = res.astype(bf16)
        for item in hooks.get(H, ()):
            item(None)
        if odd:
            pltpu.make_async_copy(
                xo_ref.at[pl.ds(pl.multiple_of(pp * 64, 64), 64), :],
                out_hbm.at[pp >> 3, pl.ds(pl.multiple_of((pp & 7) * 64, 64), 64), pl.ds(0, DM)],
                sem_out.at[0]).start()
        return new_mem

    def l1(i, mem):
        he = {2 * k: [p1_pre(i, k // 4, k % 4)] for k in range(16)}
        he[H] = [p1_mm(i, 1)]
        ho = {('o', 0): [p1_mm(i, 2)], ('o', 3): [p1_mm(i, 3)], ('o', 5): [p1_mm(i, 0)]}
        mem = step(i, 0, mem, he)
        mem = step(i, 1, mem, ho)
        return mem

    def l2(i, mem):
        u = i - N_L1
        he = {3: [p2_fwd(u, range(0, 4))], 7: [p2_fwd(u, range(4, 8))], 17: [p2_nyq(u)],
              H: [p2_inv(u, range(0, 8))]}
        ho = {('o', j): [p2_bfly(u, j, True), p2_bfly(u + 1, j, False)] for j in range(8)}
        mem = step(i, 0, mem, he)
        mem = step(i, 1, mem, ho)
        return mem

    def l3(i, mem):
        p = i - N_L1 - N_L2
        he = {h: [p3_pre(p, h // 3, 1 + h % 3)] for h in range(24)}
        for j in range(4):
            he[('o', 3 + j)] = [p3_pre(p, 2 * j, 0), p3_pre(p, 2 * j + 1, 0)]
        he[H] = [p3_mm(p, q) for q in range(4)]
        ho = {12: [b_out(p)]}
        mem = step(i, 0, mem, he)
        mem = step(i, 1, mem, ho)
        return mem

    m0 = mem_ref[...].astype(f32)
    mem = [m0[:, j * 128:(j + 1) * 128] for j in range(8)]
    mem = jax.lax.fori_loop(0, N_L1, l1, mem)
    cp_ms.wait()
    for g in range(8):
        p2_bfly(0, g, False)(None)
        p2_bfly(0, g, False, ny_ref)(None)
    mem = jax.lax.fori_loop(N_L1, N_L1 + N_L2, l2, mem)
    for g in range(8):
        p2_bfly(0, g, True, ny_ref)(None)
    mem = jax.lax.fori_loop(N_L1 + N_L2, NSEG // 2, l3, mem)

    pltpu.make_async_copy(bx_ref.at[0:4], out_hbm.at[:, :, pl.ds(DM, DM)], sem_out.at[1]).wait()
    pltpu.make_async_copy(xo_ref, xo_ref, sem_out.at[0]).wait()


@jax.jit
def _run(x, mem0, wq, wk, wv, wo, bx, w_r, w_i):
    fd, ms, tv = _tables()
    hbm = pl.BlockSpec(memory_space=pl.ANY)
    out = pl.pallas_call(
        _kernel,
        out_shape=jax.ShapeDtypeStruct((4, S // 4, 2 * DM), bf16),
        in_specs=[hbm] * 13,
        out_specs=hbm,
        scratch_shapes=[
            pltpu.VMEM((S, DM), bf16),
            pltpu.VMEM((MEM, DM), bf16),
            pltpu.VMEM((8, NSEG, 8, 128), bf16),
            pltpu.VMEM((4, DM, 16, DH), bf16),
        ] + [pltpu.VMEM((16, DM // 2 + 8, DH), u32)] * 6 + [
            pltpu.VMEM((H * DH, DM), bf16),
            pltpu.VMEM((8, H * DH // 2 + 8, 128), u32),
            pltpu.VMEM((8, 256, 128), u32),
            pltpu.VMEM((NSEG // 2, 3 * H, 8, 128), u32),
            pltpu.VMEM((2 * H, 8, 128), u32),
            pltpu.VMEM((24, H * DH), u32),
            pltpu.VMEM((32, 128), f32),
            pltpu.VMEM((48, 128), f32),
            pltpu.VMEM((5, S // 4, DM), bf16),
            pltpu.VMEM((16, DM // 2 + 1, 256), bf16),
            pltpu.VMEM((12872, 128), u32),
            pltpu.VMEM((137, 128, 128), f32),
            pltpu.VMEM((8, 128, 128), f32),
            pltpu.VMEM((12, 264, 128), f32),
            pltpu.VMEM((24, 64, 128), u32),
            pltpu.VMEM((64, 64, 128), u32),
            pltpu.VMEM((2, 512, 128), f32),
            pltpu.SMEM((64,), f32),
            pltpu.SMEM((1,), jnp.int32),
            pltpu.SemaphoreType.DMA((64,)),
            pltpu.SemaphoreType.DMA((2,)),
        ],
        compiler_params=pltpu.CompilerParams(vmem_limit_bytes=120 * 1024 * 1024,
                                             disable_semaphore_checks=True,
                                             disable_bounds_checks=True),
    )(x.reshape(S, DM), x.reshape(NSEG, SEG, DM), mem0.reshape(MEM, DM), wq, wk, wv,
      wo.reshape(H * DH, DM), bx.reshape(4, S // 4, DM), w_r.T, w_i.T, jnp.asarray(fd), jnp.asarray(ms), jnp.asarray(tv))
    return out.reshape(1, S, 2 * DM)


def pallas_concat_heads__memory_aug_recurrent_mem_tr__spectral_gfnet__prompt_kernel(
    A_x: jax.Array,
    A_mem0: jax.Array,
    A_Wq: jax.Array,
    A_Wk: jax.Array,
    A_Wv: jax.Array,
    A_Wo: jax.Array,
    A_seg_len,
    B_x: jax.Array,
    B_w_r: jax.Array,
    B_w_i: jax.Array,
):
    if isinstance(A_seg_len, int):
        assert A_seg_len == SEG
    assert A_x.shape == (1, S, DM) and A_mem0.shape == (1, MEM, DM) and A_Wq.shape == (DM, H, DH)
    assert B_x.shape == (1, S, DM) and B_w_r.shape == (S, DM // 2 + 1)
    return _run(A_x, A_mem0, A_Wq, A_Wk, A_Wv, A_Wo, B_x, B_w_r, B_w_i)
```

```python
import math

import numpy as np
import jax
import jax.numpy as jnp
import jax.experimental.pallas as pl
import jax.experimental.pallas.tpu as pltpu

bf16 = jnp.bfloat16
f32 = jnp.float32
u32 = jnp.uint32

S, DM = 2048, 1024
H, DH = 32, 128
MEM, SEG = 8, 32
NSEG = S // SEG
SQH = math.sqrt(0.5)

_PAIRS = ((0, 4), (1, 7), (2, 6), (3, 5))
_FIRST = np.array([[1, 1, 0, 0], [1, 0, 1, 0], [0, 1, 1, 0], [0, 1, 0, 1]], bool)


def _pack_rows(a):
    u = np.ascontiguousarray(a, dtype=np.float32).view(np.uint32).astype(np.uint64)
    b = ((u + 0x7FFF + ((u >> 16) & 1)) >> 16).astype(np.uint32)
    return (b[..., 0::2, :] | (b[..., 1::2, :] << 16)).astype(np.uint32)


def _tables():
    k2 = np.zeros((4, 128), np.int64)
    for t in range(4):
        odd = t % 2
        for lam in range(128):
            k = 2 * lam + odd
            if k % 8 not in _PAIRS[t]:
                k = 2 * (128 + 8 * (lam // 8) + (lam % 8 - 1 - odd) % 8) + odd
            assert k % 8 in _PAIRS[t]
            k2[t, lam] = k
    b = np.arange(128)[:, None]
    F = np.zeros((12, 128, 128))
    G = np.zeros((12, 128, 128))
    for t in range(4):
        th = 2 * np.pi * ((b * k2[t][None, :]) % DM) / DM
        C, Sn = np.cos(th), np.sin(th)
        first = ((k2[t] % 8) == _PAIRS[t][0])[None, :]
        assert np.array_equal(first[0], _FIRST[t][np.arange(128) % 4])
        if t == 0:
            im = -Sn
            im[:, 0] = (-1.0) ** np.arange(128)
            im = np.roll(im, 2, axis=1)
            F[1:3] = np.where(first, im, C), np.where(first, C, im)
            G[1:3] = F[1:3]
            G[2, :, 0] *= 0.5
            G[2, :, 2] *= 0.5
        else:
            Sg = np.where(first, Sn, -Sn)
            F[3 * t:3 * t + 3] = C, -(C + Sg), C - Sg
            G[3 * t:3 * t + 3] = F[3 * t:3 * t + 3]
    Finv = np.transpose(G, (0, 2, 1)) * (2.0 / DM)
    fd = _pack_rows(np.concatenate([F, Finv]))
    M = np.zeros((32, 128, 128))
    r = np.arange(64)[None, :]
    l = np.arange(64)[:, None]
    for j in range(32):
        th = 2 * np.pi * ((r * (j + 32 * l)) % S) / S
        C, Sn = np.cos(th), np.sin(th)
        M[j, :64, :64] = C
        M[j, :64, 64:] = Sn
        M[j, 64:, :64] = -Sn
        M[j, 64:, 64:] = C
    perm = np.arange(128).reshape(2, 8, 8).transpose(1, 0, 2).reshape(128)
    M = M[:, perm][:, :, perm]
    Minv = np.transpose(M, (0, 2, 1)) / S
    ms = _pack_rows(np.concatenate([M, Minv]))
    th = 2 * np.pi * np.outer(np.arange(512), np.arange(128) % 4) / S
    tv = np.stack([np.cos(th), np.sin(th)]).astype(np.float32)
    return fd, ms, tv


def _tobf(w):
    return pltpu.bitcast(w, bf16)


def _tou(w):
    return pltpu.bitcast(w, u32)


def _dot(a, b):
    return jnp.dot(a, b, preferred_element_type=f32)


def _r8_real(x):
    t0, t1 = x[0] + x[4], x[0] - x[4]
    t2, t3 = x[2] + x[6], x[2] - x[6]
    t4, t5 = x[1] + x[5], x[1] - x[5]
    t6, t7 = x[3] + x[7], x[3] - x[7]
    e0, e1 = t0 + t2, t0 - t2
    o0, o1 = t4 + t6, t4 - t6
    u, v = SQH * (t5 - t7), SQH * (t5 + t7)
    return [(e0 + o0, e0 - o0), (t1 + u, v + t3), (e1, o1), (t1 - u, v - t3)]


def _r8_real_t(g):
    (z0, z4), (a1, b1), (e1, o1), (a3, b3) = g
    e0, o0 = z0 + z4, z0 - z4
    t1, u = a1 + a3, a1 - a3
    v, t3 = b1 + b3, b1 - b3
    t5, t7 = SQH * (v + u), SQH * (v - u)
    t0, t2 = e0 + e1, e0 - e1
    t4, t6 = o0 + o1, o0 - o1
    return [t0 + t1, t4 + t5, t2 + t3, t6 + t7, t0 - t1, t4 - t5, t2 - t3, t6 - t7]


def _dft4(u):
    (r0, i0), (r1, i1), (r2, i2), (r3, i3) = u
    sr, si, dr, di = r0 + r2, i0 + i2, r0 - r2, i0 - i2
    tr, ti, er, ei = r1 + r3, i1 + i3, r1 - r3, i1 - i3
    return [(sr + tr, si + ti), (dr + ei, di - er), (sr - tr, si - ti), (dr - ei, di + er)]


def _dft8(x):
    a = [(x[p][0] + x[p + 4][0], x[p][1] + x[p + 4][1]) for p in range(4)]
    d = [(x[p][0] - x[p + 4][0], x[p][1] - x[p + 4][1]) for p in range(4)]
    ev = _dft4(a)
    (r0, i0), (r1, i1), (r2, i2), (r3, i3) = d
    b1r, b1i = SQH * (r1 + i1), SQH * (i1 - r1)
    b3r, n3i = SQH * (i3 - r3), SQH * (r3 + i3)
    sr, si, dr, di = r0 + i2, i0 - r2, r0 - i2, i0 + r2
    tr, ti, er, ei = b1r + b3r, b1i - n3i, b1r - b3r, b1i + n3i
    od = [(sr + tr, si + ti), (dr + ei, di - er), (sr - tr, si - ti), (dr - ei, di + er)]
    return [ev[0], od[0], ev[1], od[1], ev[2], od[2], ev[3], od[3]]


def _swap(x):
    return [(b, a) for (a, b) in x]


G = 4
NG = H // G
OSPLIT = 24
NEG = -1e9
N_L1, N_L2, N_L3 = 8, 16, 8


def _kernel(x_hbm, x3_hbm, mem_hbm, wq_hbm, wk_hbm, wv_hbm, wo_hbm, bx_hbm, wr_hbm, wi_hbm,
            fd_hbm, ms_hbm, tv_hbm, out_hbm,
            xo_ref, mem_ref, xcraw_ref, raw_ref, w0_ref, w1_ref, w2_ref, w3_ref, w4_ref, w5_ref,
            woraw_ref, wo_ref, xc_ref, xs_ref, qkvc_ref, kve_ref,
            oall_ref, fille_ref, fillo_ref, bx_ref, wt_ref, wp_ref, ub_ref, ny_ref, sa_ref, fd_ref, ms_ref, tv_ref,
            tw_ref, zero_ref, sem_in, sem_out):
    scale = DH ** -0.5
    w_hbm = (wq_hbm, wk_hbm, wv_hbm)
    w_refs = (w0_ref, w1_ref, w2_ref, w3_ref, w4_ref, w5_ref)

    def raw_copy(c, i=0, nd=DM):
        rows = pl.ds(pl.multiple_of(i * nd, nd), nd)
        return pltpu.make_async_copy(
            w_hbm[c // 2].at[rows, pl.ds((c % 2) * 16, 16), :],
            raw_ref.at[c % 4, rows], sem_in.at[8 + min(c, 3) * 8 + max(c - 3, 0) * 2 + i])

    def xc_copy(k):
        return pltpu.make_async_copy(
            x3_hbm.at[:, pl.ds(8, 8), pl.ds(pl.multiple_of(k * 128, 128), 128)], xcraw_ref.at[k], sem_in.at[40 + k])

    def bx_copy(p):
        rows = pl.ds(pl.multiple_of(p * 64, 64), 64)
        return pltpu.make_async_copy(bx_hbm.at[:, rows, :], bx_ref.at[0:4, rows, :], sem_in.at[64 + p])

    n_head = N_L1 * 2 * SEG
    cp_x = pltpu.make_async_copy(x_hbm.at[0:n_head], xo_ref.at[0:n_head], sem_in.at[0])
    cp_x2 = pltpu.make_async_copy(x_hbm.at[n_head:S], xo_ref.at[n_head:S], sem_in.at[3])
    cp_mem = pltpu.make_async_copy(mem_hbm, mem_ref, sem_in.at[1])
    cp_wo = pltpu.make_async_copy(wo_hbm, woraw_ref, sem_in.at[2])
    cp_fd = pltpu.make_async_copy(fd_hbm, fd_ref, sem_in.at[4])
    cp_ms = pltpu.make_async_copy(ms_hbm, ms_ref, sem_in.at[5])
    cp_tv = pltpu.make_async_copy(tv_hbm, tv_ref, sem_in.at[6])
    cp_wt = [pltpu.make_async_copy(src.at[:, pl.ds(lg * 256, 256)], wt_ref.at[a * 8 + lg], sem_in.at[48 + a * 8 + lg])
             for a, src in enumerate((wr_hbm, wi_hbm)) for lg in range(8)]

    for i in range(8):
        raw_copy(0, i, 128).start()
        if i < 4:
            xc_copy(i).start()
        if 3 <= i < 7:
            xc_copy(i + 1).start()
        if i >= 3:
            raw_copy(2, i - 3, 128).start()
        if i == 7:
            raw_copy(2, 5, 128).start()
        raw_copy(1, i, 128).start()
    for i in range(6, 8):
        raw_copy(2, i, 128).start()
    for i in range(2):
        raw_copy(3, i, 512).start()
    for cp in cp_wt + [cp_wo, cp_x, cp_mem, cp_fd, cp_tv] + [bx_copy(p) for p in range(8)] + [cp_x2, cp_ms]:
        cp.start(priority=1)

    zero_ref[0] = 0

    def pin_slot(n):
        return n - jnp.clip(zero_ref[0], 0, 1) * 4

    def pin_rows(r):
        return pl.ds(pl.multiple_of(r + jnp.clip(zero_ref[0], 0, 1) * 32, 8), 8)

    for p in range(8):
        for jq in range(4):
            tw_ref[(p * 4 + jq) * 2] = jnp.float32(math.cos(2 * math.pi * p * jq / 32))
            tw_ref[(p * 4 + jq) * 2 + 1] = jnp.float32(math.sin(2 * math.pi * p * jq / 32))

    ub_ref[128:136] = jnp.zeros((8, 128, 128), f32)
    wp_ref[12800:12872] = jnp.zeros((72, 128), u32)

    qi = jax.lax.broadcasted_iota(jnp.int32, (48, 128), 0)
    ki = jax.lax.broadcasted_iota(jnp.int32, (48, 128), 1)

    def between(v, lo, hi):
        return (v >= lo) & (v < hi)

    def table(keep, other):
        return jnp.where(other, -jnp.inf, jnp.where(keep, 0.0, NEG)).astype(f32)

    keep = between(qi, 8, 16) | between(ki, 8, 16) | (qi >= jnp.where(ki < 32, ki, ki - 24))
    fille_ref[...] = table(keep, ki >= 40)[:32]
    q_even = between(qi, 32, 40)
    k_even = between(ki, 32, 40) | (ki >= 48)
    qpos = jnp.where(qi < 32, qi, jnp.where(qi < 40, qi - 24, qi - 32))
    kpos = jnp.where(ki < 32, ki, jnp.where(ki < 40, ki - 24, jnp.where(ki < 48, ki - 32, ki - 48)))
    keep = between(qi, 8, 16) | between(ki, 8, 16) | (ki >= 56) | (qpos >= kpos)
    fillo_ref[...] = table(keep, (q_even != k_even) | (ki >= 64))

    def relayout16(c, blk):
        w0 = pl.multiple_of(blk * 8, 8)
        v = _tou(raw_ref[c % 4, pl.ds(blk * 16, 16)]).reshape(8, 2, 8, 128)
        a, b = v[:, 0], v[:, 1]
        w_refs[c][0:8, pl.ds(w0, 8), :] = jnp.swapaxes((a & jnp.uint32(0xFFFF)) | (b << 16), 0, 1)
        w_refs[c][8:16, pl.ds(w0, 8), :] = jnp.swapaxes((a >> 16) | (b & jnp.uint32(0xFFFF0000)), 0, 1)

    def slot_of(h):
        return (h // 16) * 16 + (h % 2) * 8 + (h % 16) // 2

    def repack_wo64(blk):
        v = _tou(woraw_ref[pl.ds(pl.multiple_of(blk * 64, 64), 64), :])
        wo_ref[:, pl.ds(pl.multiple_of(blk * 32, 32), 32), :] = jnp.stack(
            [v[:, j * 128:(j + 1) * 128] for j in range(8)])

    sub4 = jax.lax.broadcasted_iota(jnp.int32, (128, 128), 0) & 3

    def wp_store(t, kb, tile):
        v = tile.T.reshape(4, 32, 128)
        v = jnp.concatenate([v, v[:, 0:8]], axis=1).reshape(160, 128)
        wp_ref[pl.ds(pl.multiple_of(t * 2560 + kb * 160, 32), 160), :] = v

    def b_prep(lg, hb, par):
        cols = slice(hb * 128, (hb + 1) * 128)
        a = _tou(wt_ref[lg, 0:512, cols])
        b = _tou(wt_ref[8 + lg, 0:512, cols])
        if par == 0:
            w = (a << 16) | (b & jnp.uint32(0xFFFF))
            m = (sub4 == 0) | (sub4 == 2)
        else:
            w = (a & jnp.uint32(0xFFFF0000)) | (b >> 16)
            m = (sub4 == 0) | (sub4 == 3)
        top = w[:128]
        bot = pltpu.roll(w[128:].reshape(16, 8, 128), 1 + par, 1).reshape(128, 128)
        wp_store(par, lg * 2 + hb, jnp.where(m, top, bot))
        wp_store(par + 2, lg * 2 + hb, jnp.where(m, bot, top))
        if par == 0:
            na = jnp.broadcast_to(wt_ref[lg, 512:513, cols].astype(f32), (128, 128))
            nb = jnp.broadcast_to(wt_ref[8 + lg, 512:513, cols].astype(f32), (128, 128))
            wp_store(4, lg * 2 + hb, pltpu.bitcast(na, u32) | (pltpu.bitcast(nb, u32) >> 16))

    def gather_c(k):
        xc_ref[k] = _tou(xcraw_ref[k].astype(f32).reshape(512, 128).astype(bf16))

    def store_qkvc(n, y):
        qkvc_ref[:, n] = y.reshape(NSEG // 2, 8, 128)

    def q_unit(i, groups, first, last, fillers):
        xk = _tobf(xc_ref[i])
        w0 = pl.multiple_of(i * 64, 64)
        for g in groups:
            rhs = jnp.concatenate(
                [_tobf(w_refs[h // 16][h % 16, pl.ds(w0, 64), :]) for h in range(4 * g, 4 * g + 4)], axis=1)
            y = _dot(xk, rhs)
            for h in range(4 * g, 4 * g + 4):
                yh = y[:, (h % 4) * 128:(h % 4 + 1) * 128]
                if not first:
                    yh = yh + ub_ref[h * 4:(h + 1) * 4].reshape(512, 128)
                if last:
                    store_qkvc(h, _tou(yh.astype(bf16)))
                else:
                    ub_ref[h * 4:(h + 1) * 4] = yh.reshape(4, 128, 128)
            mine = fillers.get(g, [])
            for fi, item in enumerate(mine):
                r = (fi * 512 // len(mine)) // 8 * 8
                item(pltpu.bitcast(y[r:r + 8, 0:128], u32))

    def rl_item(c, blk):
        def item(pin):
            w_refs[c][pin_slot(15), 512:520] = pin
            relayout16(c, blk)
        return item

    def spread(fillers, items, groups):
        for k, item in enumerate(items):
            fillers.setdefault(groups[k * len(groups) // len(items)], []).append(item)
        return fillers

    def half_items(f, c, i, groups):
        return spread(f, [rl_item(c, i * 8 + blk) for blk in range(8)], groups)

    def piece_items(i):
        f = half_items(half_items({}, 1, i, (0, 1, 2)), 0, i + 1, (4, 5, 6))
        return spread(f, [lambda pin: gather_c(i + 1)], (7,))

    def chunk2_items(f, lo, hi, groups):
        return spread(f, [rl_item(2, blk) for blk in range(lo, hi)], groups)

    def wait_piece(i):
        raw_copy(1, i, 128).wait()
        raw_copy(0, i + 1, 128).wait()

    raw_copy(0, 0, 128).wait()
    for blk in range(8):
        relayout16(0, blk)
    xc_copy(0).wait()
    gather_c(0)
    q_unit(0, range(0, 2), True, False, {})
    raw_copy(1, 0, 128).wait()
    q_unit(0, range(2, 4), True, False, half_items({}, 1, 0, (2, 2, 3)))
    q_unit(0, range(4, 6), True, False, {})
    xc_copy(1).wait()
    raw_copy(0, 1, 128).wait()
    q_unit(0, range(6, 8), True, False,
           spread(half_items({}, 0, 1, (6, 6, 7)), [lambda pin: gather_c(1)], (6,)))
    raw_copy(1, 1, 128).wait()
    q_unit(1, range(0, 4), False, False, half_items({}, 1, 1, (0, 1, 2)))
    xc_copy(2).wait()
    raw_copy(0, 2, 128).wait()
    q_unit(1, range(4, 8), False, False,
           spread(half_items({}, 0, 2, (4, 5, 6)), [lambda pin: gather_c(2)], (6,)))

    def xsum_item(j, rq):
        def item(pin):
            xs_ref[pin_slot(4), 0, 128:136] = pin
            a11, a21, a12, a22 = [
                xcraw_ref[j + 4 * kh, rh * 32 + rq * 8:rh * 32 + (rq + 1) * 8].astype(f32).reshape(64, 128)
                for kh in range(2) for rh in range(2)]
            for k, v in enumerate((a11 + a22, a21 + a22, a11 + a12, a21 - a11, a12 - a22)):
                xs_ref[k, j, rq * 32:(rq + 1) * 32] = _tou(v.astype(bf16))
        return item

    def q_c(i, carry):
        wait_piece(i)
        xc_copy(i + 2).wait()
        raw_copy(2, i - 2, 128).wait()
        f = half_items(piece_items(i), 2, i - 2, (3, 3, 3, 3, 4, 5, 6, 7))
        q_unit(i, range(8), False, False, spread(f, [xsum_item(i - 2, rq) for rq in range(4)], (3, 4, 5, 6)))
        return carry
    xc_copy(3).wait()
    jax.lax.fori_loop(2, 6, q_c, 0)

    wait_piece(6)
    raw_copy(2, 4, 128).wait()
    raw_copy(2, 5, 128).wait()
    q_unit(6, range(8), False, False, chunk2_items(piece_items(6), 32, 48, (0, 1, 2, 3, 3, 4, 5, 6)))
    raw_copy(1, 7, 128).wait()
    raw_copy(2, 6, 128).wait()
    raw_copy(2, 7, 128).wait()
    q_unit(7, range(8), False, True, chunk2_items(half_items({}, 1, 7, (0, 1, 2)), 48, 64, (3, 4, 5, 6)))
    raw_copy(4).start()
    raw_copy(5).start()

    def bulk_iter(c, i):
        def xs(k):
            return jnp.concatenate([_tobf(xs_ref[k, j, 0:128]) for j in range(4)], axis=1)

        def xc(rh, kh):
            return jnp.concatenate(
                [_tobf(xc_ref[4 * kh + j, rh * 128:(rh + 1) * 128]) for j in range(4)], axis=1)

        for pr in range(4):
            n1 = i * 8 + pr * 2
            n2 = n1 + 1

            def w(n, kh):
                return _tobf(w_refs[c][n, kh * 256:(kh + 1) * 256])

            def wsum(a, b, sign):
                a, b = a.astype(f32), b.astype(f32)
                return (a + b if sign > 0 else a - b).astype(bf16)

            def out(rh, n, v):
                qkvc_ref[rh * 16:(rh + 1) * 16, c * 16 + n] = _tou(v.astype(bf16)).reshape(16, 8, 128)

            def side(k, m):
                for blk, r in ((k, 0), (7, 128)) if k == 0 else ((k, 0),):
                    pin = pltpu.bitcast(m[r:r + 8], u32)
                    if c + 1 < 6:
                        w_refs[c + 1][pin_slot(15), 512:520] = pin
                        relayout16(c + 1, i * 32 + (pr * 8 + blk))
                    else:
                        wo_ref[pin_slot(7), 2048:2056] = pin
                        repack_wo64(i * 32 + (pr * 8 + blk))
                if c >= 4 and k in (1, 4):
                    wp_ref[pin_rows(12832), :] = pltpu.bitcast(m[128:136], u32)
                    b_prep((c - 4) * 4 + i * 2 + pr // 2, pr % 2, k // 4)

            m2 = _dot(xs(1), w(n1, 0))
            side(0, m2)
            m4 = _dot(xc(1, 1), wsum(w(n1, 1), w(n1, 0), -1))
            side(1, m4)
            out(1, n1, m4 + m2)
            m1 = _dot(xs(0), wsum(w(n1, 0), w(n2, 1), 1))
            side(2, m1)
            m5 = _dot(xs(2), w(n2, 1))
            side(3, m5)
            m3 = _dot(xc(0, 0), wsum(w(n2, 0), w(n2, 1), -1))
            side(4, m3)
            out(0, n2, m3 + m5)
            c22 = _dot(xs(3), wsum(w(n1, 0), w(n2, 0), 1)) + ((m1 - m2) + m3)
            side(5, c22)
            out(1, n2, c22)
            c11 = _dot(xs(4), wsum(w(n1, 1), w(n2, 1), 1)) + ((m1 + m4) - m5)
            side(6, c11)
            out(0, n1, c11)

    for c in range(2, 6):
        if c == 4:
            for cp in cp_wt:
                cp.wait()
        if c == 5:
            cp_wo.wait()
        elif c > 2:
            raw_copy(c + 1).wait()

        def bulk(i, carry, c=c):
            if c == 2:
                raw_copy(3, i, 512).wait()
            bulk_iter(c, i)
            return carry
        jax.lax.fori_loop(0, 2, bulk, 0)

    cp_x.wait()
    cp_mem.wait()
    cp_fd.wait()
    cp_tv.wait()

    lane = jax.lax.broadcasted_iota(jnp.int32, (1, 128), 1)
    lane0 = lane == 0
    sgn0 = jnp.where(lane0, 1.0, -1.0)

    def first_lanes(t):
        la, lb = [k for k in range(4) if _FIRST[t][k]]
        return ((lane & 3) == la) | ((lane & 3) == lb)

    def d_products(st_ref, d, t, rows):
        return [_dot(st_ref[n, rows].astype(bf16), _tobf(fd_ref[d * 12 + n])) if n else None
                for n in range(3 * t, 3 * t + 3)]

    def twiddles(p):
        return [(tw_ref[p * 8 + jq * 2], tw_ref[p * 8 + jq * 2 + 1]) if jq else None for jq in range(4)]

    def p1_pre(p, rs, q):
        def item(y):
            sa_ref[pin_slot(7), 256:264] = y
            xq = bx_ref[q, pl.ds(pl.multiple_of(p * 64 + rs * 16, 16), 16), :].astype(f32)
            zz = _r8_real([xq[:, a * 128:(a + 1) * 128] for a in range(8)])
            r = (rs * 4 + q) * 16
            sa_ref[1:12, r:r + 16] = jnp.stack([v for (a, b) in zz for v in (a + b, b, a)][1:])
        return item

    def p1_mm(p, t):
        def item(y):
            cs = twiddles(p)

            def put(ref, n, rs, re, im):
                v = jnp.stack([re.reshape(2, 8, 128), im.reshape(2, 8, 128)], axis=1)
                ref[n * 8 + p, rs * 32:(rs + 1) * 32] = v.reshape(32, 128)

            first = first_lanes(t)
            for rs in range(4):
                k1, k2, k3 = d_products(sa_ref, 0, t, slice(rs * 64, (rs + 1) * 64))
                if t == 0:
                    up = jnp.where(first, k2, k3)
                    re, im = jnp.where(first, k3, k2), pltpu.roll(up, 126, 1)
                    ny = jnp.where(lane0, im, up)
                    u = [ny[q * 16:(q + 1) * 16] for q in range(4)]
                    odd_lane = (lane & 1) == 1
                    nr = jnp.where(odd_lane, pltpu.roll(u[0] - u[2], 1, 1), u[0] + u[2] + (u[1] + u[3]) * sgn0)
                    ni = jnp.where(odd_lane, pltpu.roll((u[3] - u[1]) * sgn0, 1, 1), 0.0)
                    rows = pl.ds(pl.multiple_of(p * 64 + rs * 16, 16), 16)
                    c, sn = tv_ref[0, rows], tv_ref[1, rows]
                    put(ny_ref, 0, rs, nr * c + ni * sn, ni * c - nr * sn)
                    im = jnp.where(lane0, 0.0, im)
                else:
                    re, im = k1 + k2, (k3 - k1) * jnp.where(first, 1.0, -1.0)
                a = _dft4([(re[q * 16:(q + 1) * 16], im[q * 16:(q + 1) * 16]) for q in range(4)])
                for jq in range(4):
                    re, im = a[jq]
                    if jq > 0:
                        c, sn = cs[jq]
                        re, im = re * c + im * sn, im * c - re * sn
                    put(ub_ref, t * 4 + jq, rs, re, im)
        return item

    def p2_bfly(u, g, inverse, ref=ub_ref):
        def item(y):
            if y is not None:
                ub_ref[136, pin_rows(0), :] = y
            v = ref[pl.ds(u * 8, 8), g * 16:(g + 1) * 16]
            x = [(v[p, 0:8], v[p, 8:16]) for p in range(8)]
            x = _swap(_dft8(_swap(x))) if inverse else _dft8(x)
            ref[pl.ds(u * 8, 8), g * 16:(g + 1) * 16] = jnp.stack([w for c in x for w in c]).reshape(8, 16, 128)
        return item

    def filtered(xx, w):
        wr = pltpu.bitcast(w & jnp.uint32(0xFFFF0000), f32).reshape(8, 8, 128)
        wi = pltpu.bitcast(w << 16, f32).reshape(8, 8, 128)
        xx = xx.reshape(8, 2, 8, 128)
        xr, xi = xx[:, 0], xx[:, 1]
        return jnp.stack([xr * wr - xi * wi, xr * wi + xi * wr], axis=1).reshape(128, 128)

    def p2_fwd(u, jps):
        def item(y):
            t = u >> 2
            jq = u & 3
            xs = [_dot(_tobf(ms_ref[jq + 4 * jp]), ub_ref[u * 8 + jp].astype(bf16)) for jp in jps]
            for jp, xx in zip(jps, xs):
                ub_ref[u * 8 + jp] = filtered(xx, wp_ref[pl.ds(t * 2560 + jq + 4 * jp, 64, stride=40), :])
        return item

    def p2_nyq(u):
        def item(y):
            jp = u & 7
            rhs = ny_ref[jp].astype(bf16)
            xx = jnp.concatenate([_dot(_tobf(ms_ref[u * 4, m * 16:(m + 1) * 16]), rhs) for m in range(4)], axis=0)
            w = wp_ref[pl.ds(4 * 2560 + 4 * jp, 64, stride=40), :]
            for jq in range(1, 4):
                w = jnp.where(lane == jq, wp_ref[pl.ds(4 * 2560 + 4 * jp + jq, 64, stride=40), :], w)
            w = jnp.where(u < 8, w, jnp.uint32(0x3F800000))
            ny_ref[jp] = filtered(xx, w)
        return item

    def p2_inv(u, jps):
        def item(y):
            jq = u & 3
            zs = [_dot(_tobf(ms_ref[32 + jq + 4 * jp]), ub_ref[u * 8 + jp].astype(bf16)) for jp in jps]
            for jp, zz in zip(jps, zs):
                ub_ref[u * 8 + jp] = zz
        return item

    def p3_pre(p, g, t):
        def item(y):
            sa_ref[pin_slot(7), 256:264] = y
            cs = twiddles(p)

            def fetch(t):
                a = []
                for jq in range(4):
                    v = ub_ref[(t * 4 + jq) * 8 + p, g * 16:(g + 1) * 16]
                    re, im = v[0:8], v[8:16]
                    if jq > 0:
                        c, sn = cs[jq]
                        re, im = re * c - im * sn, im * c + re * sn
                    a.append((re, im))
                return _swap(_dft4(_swap(a)))

            u = fetch(t)
            if t == 0:
                v = ny_ref[p, g * 16:(g + 1) * 16]
                rows = pl.ds(pl.multiple_of(p * 64 + g * 8, 8), 8)
                c, sn = tv_ref[0, rows], tv_ref[1, rows]
                nr, ni = v[0:8] * c - v[8:16] * sn, v[8:16] * c + v[0:8] * sn
                zr, zi = pltpu.roll(nr, 127, 1), pltpu.roll(ni, 127, 1)
                ny = (nr + zr, (nr - zi) * sgn0, nr - zr, (nr + zi) * sgn0)
            first = first_lanes(t)
            for q in range(4):
                re, im = u[q]
                rows = slice(q * 64 + g * 8, q * 64 + (g + 1) * 8)
                if t == 0:
                    im = pltpu.roll(jnp.where(lane0, ny[q], im), 2, 1) + jnp.where(lane == 2, ny[q], 0.0)
                    sa_ref[1:3, rows] = jnp.stack((jnp.where(first, im, re), jnp.where(first, re, im)))
                else:
                    im = im * jnp.where(first, 1.0, -1.0)
                    sa_ref[3 * t:3 * t + 3, rows] = jnp.stack((re + im, im, re))
        return item

    def p3_mm(p, q):
        def item(y):
            g = []
            for t in range(4):
                k1, k2, k3 = d_products(sa_ref, 1, t, slice(q * 64, (q + 1) * 64))
                g.append((k3, k2) if t == 0 else (k2 + k1, k3 - k1))
            yy = _r8_real_t(g)
            bx_ref[q, pl.ds(pl.multiple_of(p * 64, 64), 64), :] = jnp.concatenate(yy, axis=1).astype(bf16)
        return item

    def b_out(p):
        def item(y):
            rows = pl.ds(pl.multiple_of(p * 64, 64), 64)
            pltpu.make_async_copy(bx_ref.at[0:4, rows, :], out_hbm.at[:, rows, pl.ds(DM, DM)],
                                  sem_out.at[1]).start()
            bx_ref[4, pin_rows(0), 0:128] = y.astype(bf16)
        return item

    def step(pp, odd, mem, hooks):
        r0 = pl.multiple_of(pp * 64 + 32 * odd, SEG)
        xs = xo_ref[pl.ds(r0, SEG), :]
        x_lo = xs[0:8].astype(f32)
        hm = jnp.concatenate(
            [jnp.concatenate([x_lo, jnp.concatenate(mem, axis=1)], axis=0).astype(bf16), xs[16:32]], axis=0)
        fill = fillo_ref[:, 0:64] if odd else fille_ref[:, 0:48]
        nrow = 48 if odd else 32
        qkv, ps = {}, {}

        def do_qkv(h0, h1):
            for h in range(h0, h1):
                for t in range(3):
                    n = t * H + slot_of(h)
                    y32 = _dot(hm, _tobf(w_refs[n // 16][n % 16, 0:512]))
                    y = y32.astype(bf16)
                    parts = [y]
                    if odd or t > 0:
                        parts.append(_tobf(qkvc_ref[pp, n]))
                    if t > 0:
                        if odd:
                            parts.append(_tobf(kve_ref[(t - 1) * H + h]))
                        else:
                            kve_ref[(t - 1) * H + h] = _tou(y[0:16])
                    qkv[(t, h)] = jnp.concatenate(parts, axis=0) if len(parts) > 1 else y
                for item in hooks.get(h, ()):
                    item(y32[0:8])

        def do_s(g):
            for h in range(g * G, (g + 1) * G):
                sc = jax.lax.dot_general(qkv[(0, h)], qkv[(1, h)], (((1,), (1,)), ((), ())),
                                         preferred_element_type=f32)
                sc = jnp.where(fill == 0.0, sc * scale, fill)
                e = jnp.exp(sc - jnp.max(sc, axis=1, keepdims=True))
                den = jnp.sum(e, axis=1, keepdims=True)
                r = pl.reciprocal(den, approx=True)
                r = r * (2.0 - den * r)
                ps[h] = (e * r).astype(bf16)

        def do_pv(g):
            for h in range(g * G, (g + 1) * G):
                oall_ref[0:nrow // 2, h * DH:(h + 1) * DH] = _tou(_dot(ps[h], qkv[(2, h)]).astype(bf16))

        def do_o(j, h0, h1):
            return _dot(_tobf(oall_ref[0:nrow // 2, h0 * DH:h1 * DH]), _tobf(wo_ref[j, h0 * 64:h1 * 64, :]))

        for g in range(NG):
            do_qkv(g * G, g * G + G // 2)
            if g >= 1:
                do_s(g - 1)
            do_qkv(g * G + G // 2, (g + 1) * G)
            if g >= 2:
                do_pv(g - 2)
        part = {}
        for j in range(8):
            items = hooks.get(('o', j), ())
            if len(items) == 1:
                part[j] = do_o(j, 0, OSPLIT)
                items[0](None)
            elif items:
                half = do_o(j, 0, OSPLIT // 2)
                items[0](half[0:8])
                part[j] = do_o(j, OSPLIT // 2, OSPLIT) + half
                items[1](part[j][0:8])
            else:
                part[j] = do_o(j, 0, OSPLIT)
            if j == 2:
                do_s(NG - 1)
                do_pv(NG - 2)
            if j == 5:
                do_pv(NG - 1)
        new_mem = []
        for j in range(8):
            cols = slice(j * 128, (j + 1) * 128)
            res = do_o(j, OSPLIT, H) + part[j]
            new_mem.append(res[8:16])
            if odd:
                xo_ref[pl.ds(r0, SEG), cols] = jnp.concatenate(
                    [res[0:8], res[40:48], res[16:32]], axis=0).astype(bf16)
                xo_ref[pl.ds(r0 - 24, 8), cols] = res[32:40].astype(bf16)
            else:
                xo_ref[pl.ds(r0, SEG), cols] = res.astype(bf16)
        for item in hooks.get(H, ()):
            item(None)
        if odd:
            pltpu.make_async_copy(
                xo_ref.at[pl.ds(pl.multiple_of(pp * 64, 64), 64), :],
                out_hbm.at[pp >> 3, pl.ds(pl.multiple_of((pp & 7) * 64, 64), 64), pl.ds(0, DM)],
                sem_out.at[0]).start()
        return new_mem

    def l1(i, mem):
        bx_copy(i).wait()
        he = {2 * k: [p1_pre(i, k // 4, k % 4)] for k in range(16)}
        he[H] = [p1_mm(i, 1)]
        ho = {('o', 0): [p1_mm(i, 2)], ('o', 3): [p1_mm(i, 3)], ('o', 5): [p1_mm(i, 0)]}
        mem = step(i, 0, mem, he)
        mem = step(i, 1, mem, ho)
        return mem

    def l2(i, mem):
        u = i - N_L1
        he = {3: [p2_fwd(u, range(0, 4))], 7: [p2_fwd(u, range(4, 8))], 17: [p2_nyq(u)],
              H: [p2_inv(u, range(0, 8))]}
        ho = {('o', j): [p2_bfly(u, j, True), p2_bfly(u + 1, j, False)] for j in range(8)}
        mem = step(i, 0, mem, he)
        mem = step(i, 1, mem, ho)
        return mem

    def l3(i, mem):
        p = i - N_L1 - N_L2
        he = {h: [p3_pre(p, h // 3, 1 + h % 3)] for h in range(24)}
        for j in range(4):
            he[('o', 3 + j)] = [p3_pre(p, 2 * j, 0), p3_pre(p, 2 * j + 1, 0)]
        he[H] = [p3_mm(p, q) for q in range(4)]
        ho = {12: [b_out(p)]}
        mem = step(i, 0, mem, he)
        mem = step(i, 1, mem, ho)
        return mem

    m0 = mem_ref[...].astype(f32)
    mem = [m0[:, j * 128:(j + 1) * 128] for j in range(8)]
    mem = jax.lax.fori_loop(0, N_L1, l1, mem)
    cp_x2.wait()
    cp_ms.wait()
    for g in range(8):
        p2_bfly(0, g, False)(None)
        p2_bfly(0, g, False, ny_ref)(None)
    mem = jax.lax.fori_loop(N_L1, N_L1 + N_L2, l2, mem)
    for g in range(8):
        p2_bfly(0, g, True, ny_ref)(None)
    mem = jax.lax.fori_loop(N_L1 + N_L2, NSEG // 2, l3, mem)

    pltpu.make_async_copy(bx_ref.at[0:4], out_hbm.at[:, :, pl.ds(DM, DM)], sem_out.at[1]).wait()
    pltpu.make_async_copy(xo_ref, xo_ref, sem_out.at[0]).wait()


@jax.jit
def _run(x, mem0, wq, wk, wv, wo, bx, w_r, w_i):
    fd, ms, tv = _tables()
    hbm = pl.BlockSpec(memory_space=pl.ANY)
    out = pl.pallas_call(
        _kernel,
        out_shape=jax.ShapeDtypeStruct((4, S // 4, 2 * DM), bf16),
        in_specs=[hbm] * 13,
        out_specs=hbm,
        scratch_shapes=[
            pltpu.VMEM((S, DM), bf16),
            pltpu.VMEM((MEM, DM), bf16),
            pltpu.VMEM((8, NSEG, 8, 128), bf16),
            pltpu.VMEM((4, DM, 16, DH), bf16),
        ] + [pltpu.VMEM((16, DM // 2 + 8, DH), u32)] * 6 + [
            pltpu.VMEM((H * DH, DM), bf16),
            pltpu.VMEM((8, H * DH // 2 + 8, 128), u32),
            pltpu.VMEM((8, 256, 128), u32),
            pltpu.VMEM((5, 4, 136, 128), u32),
            pltpu.VMEM((NSEG // 2, 3 * H, 8, 128), u32),
            pltpu.VMEM((2 * H, 8, 128), u32),
            pltpu.VMEM((24, H * DH), u32),
            pltpu.VMEM((32, 128), f32),
            pltpu.VMEM((48, 128), f32),
            pltpu.VMEM((5, S // 4, DM), bf16),
            pltpu.VMEM((16, DM // 2 + 1, 256), bf16),
            pltpu.VMEM((12872, 128), u32),
            pltpu.VMEM((137, 128, 128), f32),
            pltpu.VMEM((8, 128, 128), f32),
            pltpu.VMEM((12, 264, 128), f32),
            pltpu.VMEM((24, 64, 128), u32),
            pltpu.VMEM((64, 64, 128), u32),
            pltpu.VMEM((2, 512, 128), f32),
            pltpu.SMEM((64,), f32),
            pltpu.SMEM((1,), jnp.int32),
            pltpu.SemaphoreType.DMA((72,)),
            pltpu.SemaphoreType.DMA((2,)),
        ],
        compiler_params=pltpu.CompilerParams(vmem_limit_bytes=120 * 1024 * 1024,
                                             disable_semaphore_checks=True,
                                             disable_bounds_checks=True),
    )(x.reshape(S, DM), x.reshape(NSEG, SEG, DM), mem0.reshape(MEM, DM), wq, wk, wv,
      wo.reshape(H * DH, DM), bx.reshape(4, S // 4, DM), w_r.T, w_i.T, jnp.asarray(fd), jnp.asarray(ms), jnp.asarray(tv))
    return out.reshape(1, S, 2 * DM)


def pallas_concat_heads__memory_aug_recurrent_mem_tr__spectral_gfnet__prompt_kernel(
    A_x: jax.Array,
    A_mem0: jax.Array,
    A_Wq: jax.Array,
    A_Wk: jax.Array,
    A_Wv: jax.Array,
    A_Wo: jax.Array,
    A_seg_len,
    B_x: jax.Array,
    B_w_r: jax.Array,
    B_w_i: jax.Array,
):
    if isinstance(A_seg_len, int):
        assert A_seg_len == SEG
    assert A_x.shape == (1, S, DM) and A_mem0.shape == (1, MEM, DM) and A_Wq.shape == (DM, H, DH)
    assert B_x.shape == (1, S, DM) and B_w_r.shape == (S, DM // 2 + 1)
    return _run(A_x, A_mem0, A_Wq, A_Wk, A_Wv, A_Wo, B_x, B_w_r, B_w_i)
```

```python
import math

import numpy as np
import jax
import jax.numpy as jnp
import jax.experimental.pallas as pl
import jax.experimental.pallas.tpu as pltpu

bf16 = jnp.bfloat16
f32 = jnp.float32
u32 = jnp.uint32

S, DM = 2048, 1024
H, DH = 32, 128
MEM, SEG = 8, 32
NSEG = S // SEG
SQH = math.sqrt(0.5)

_PAIRS = ((0, 4), (1, 7), (2, 6), (3, 5))
_FIRST = np.array([[1, 1, 0, 0], [1, 0, 1, 0], [0, 1, 1, 0], [0, 1, 0, 1]], bool)


def _pack_rows(a):
    u = np.ascontiguousarray(a, dtype=np.float32).view(np.uint32).astype(np.uint64)
    b = ((u + 0x7FFF + ((u >> 16) & 1)) >> 16).astype(np.uint32)
    return (b[..., 0::2, :] | (b[..., 1::2, :] << 16)).astype(np.uint32)


def _tables():
    k2 = np.zeros((4, 128), np.int64)
    for t in range(4):
        odd = t % 2
        for lam in range(128):
            k = 2 * lam + odd
            if k % 8 not in _PAIRS[t]:
                k = 2 * (128 + 8 * (lam // 8) + (lam % 8 - 1 - odd) % 8) + odd
            assert k % 8 in _PAIRS[t]
            k2[t, lam] = k
    b = np.arange(128)[:, None]
    F = np.zeros((12, 128, 128))
    G = np.zeros((12, 128, 128))
    for t in range(4):
        th = 2 * np.pi * ((b * k2[t][None, :]) % DM) / DM
        C, Sn = np.cos(th), np.sin(th)
        first = ((k2[t] % 8) == _PAIRS[t][0])[None, :]
        assert np.array_equal(first[0], _FIRST[t][np.arange(128) % 4])
        if t == 0:
            im = -Sn
            im[:, 0] = (-1.0) ** np.arange(128)
            im = np.roll(im, 2, axis=1)
            F[1:3] = np.where(first, im, C), np.where(first, C, im)
            G[1:3] = F[1:3]
            G[2, :, 0] *= 0.5
            G[2, :, 2] *= 0.5
        else:
            Sg = np.where(first, Sn, -Sn)
            F[3 * t:3 * t + 3] = C, -(C + Sg), C - Sg
            G[3 * t:3 * t + 3] = F[3 * t:3 * t + 3]
    Finv = np.transpose(G, (0, 2, 1)) * (2.0 / DM)
    fd = _pack_rows(np.concatenate([F, Finv]))
    M = np.zeros((32, 128, 128))
    r = np.arange(64)[None, :]
    l = np.arange(64)[:, None]
    for j in range(32):
        th = 2 * np.pi * ((r * (j + 32 * l)) % S) / S
        C, Sn = np.cos(th), np.sin(th)
        M[j, :64, :64] = C
        M[j, :64, 64:] = Sn
        M[j, 64:, :64] = -Sn
        M[j, 64:, 64:] = C
    perm = np.arange(128).reshape(2, 8, 8).transpose(1, 0, 2).reshape(128)
    M = M[:, perm][:, :, perm]
    Minv = np.transpose(M, (0, 2, 1)) / S
    ms = _pack_rows(np.concatenate([M, Minv]))
    th = 2 * np.pi * np.outer(np.arange(512), np.arange(128) % 4) / S
    tv = np.stack([np.cos(th), np.sin(th)]).astype(np.float32)
    return fd, ms, tv


def _tobf(w):
    return pltpu.bitcast(w, bf16)


def _tou(w):
    return pltpu.bitcast(w, u32)


def _dot(a, b):
    return jnp.dot(a, b, preferred_element_type=f32)


def _r8_real(x):
    t0, t1 = x[0] + x[4], x[0] - x[4]
    t2, t3 = x[2] + x[6], x[2] - x[6]
    t4, t5 = x[1] + x[5], x[1] - x[5]
    t6, t7 = x[3] + x[7], x[3] - x[7]
    e0, e1 = t0 + t2, t0 - t2
    o0, o1 = t4 + t6, t4 - t6
    u, v = SQH * (t5 - t7), SQH * (t5 + t7)
    return [(e0 + o0, e0 - o0), (t1 + u, v + t3), (e1, o1), (t1 - u, v - t3)]


def _r8_real_t(g):
    (z0, z4), (a1, b1), (e1, o1), (a3, b3) = g
    e0, o0 = z0 + z4, z0 - z4
    t1, u = a1 + a3, a1 - a3
    v, t3 = b1 + b3, b1 - b3
    t5, t7 = SQH * (v + u), SQH * (v - u)
    t0, t2 = e0 + e1, e0 - e1
    t4, t6 = o0 + o1, o0 - o1
    return [t0 + t1, t4 + t5, t2 + t3, t6 + t7, t0 - t1, t4 - t5, t2 - t3, t6 - t7]


def _dft4(u):
    (r0, i0), (r1, i1), (r2, i2), (r3, i3) = u
    sr, si, dr, di = r0 + r2, i0 + i2, r0 - r2, i0 - i2
    tr, ti, er, ei = r1 + r3, i1 + i3, r1 - r3, i1 - i3
    return [(sr + tr, si + ti), (dr + ei, di - er), (sr - tr, si - ti), (dr - ei, di + er)]


def _dft8(x):
    a = [(x[p][0] + x[p + 4][0], x[p][1] + x[p + 4][1]) for p in range(4)]
    d = [(x[p][0] - x[p + 4][0], x[p][1] - x[p + 4][1]) for p in range(4)]
    ev = _dft4(a)
    (r0, i0), (r1, i1), (r2, i2), (r3, i3) = d
    b1r, b1i = SQH * (r1 + i1), SQH * (i1 - r1)
    b3r, n3i = SQH * (i3 - r3), SQH * (r3 + i3)
    sr, si, dr, di = r0 + i2, i0 - r2, r0 - i2, i0 + r2
    tr, ti, er, ei = b1r + b3r, b1i - n3i, b1r - b3r, b1i + n3i
    od = [(sr + tr, si + ti), (dr + ei, di - er), (sr - tr, si - ti), (dr - ei, di + er)]
    return [ev[0], od[0], ev[1], od[1], ev[2], od[2], ev[3], od[3]]


def _swap(x):
    return [(b, a) for (a, b) in x]


G = 4
NG = H // G
NEG = -1e9
N_L1, N_L2, N_L3 = 8, 16, 8


def _kernel(x_hbm, x3_hbm, mem_hbm, wq_hbm, wk_hbm, wv_hbm, wo_hbm, bx_hbm, wr_hbm, wi_hbm,
            fd_hbm, ms_hbm, tv_hbm, out_hbm,
            xo_ref, mem_ref, xcraw_ref, raw_ref, w0_ref, w1_ref, w2_ref, w3_ref, w4_ref, w5_ref,
            wo_ref, xc_ref, xs_ref, qkvc_ref, kve_ref,
            oall_ref, oc_ref, os_ref, ws_ref, fille_ref, fillo_ref, bx_ref, wt_ref, wp_ref, ub_ref, ny_ref, sa_ref, fd_ref, ms_ref, tv_ref,
            tw_ref, zero_ref, sem_in, sem_out):
    scale = DH ** -0.5
    w_hbm = (wq_hbm, wk_hbm, wv_hbm)
    w_refs = (w0_ref, w1_ref, w2_ref, w3_ref, w4_ref, w5_ref)

    def raw_copy(c, i=0, nd=DM):
        rows = pl.ds(pl.multiple_of(i * nd, nd), nd)
        return pltpu.make_async_copy(
            w_hbm[c // 2].at[rows, pl.ds((c % 2) * 16, 16), :],
            raw_ref.at[c % 4, rows], sem_in.at[8 + min(c, 3) * 8 + max(c - 3, 0) * 2 + i])

    def xc_copy(k):
        return pltpu.make_async_copy(
            x3_hbm.at[:, pl.ds(8, 8), pl.ds(pl.multiple_of(k * 128, 128), 128)], xcraw_ref.at[k], sem_in.at[40 + k])

    def wo_copies(half):
        return [pltpu.make_async_copy(wo_hbm.at[:, :, pl.ds(pl.multiple_of(half * 512 + j * 128, 128), 128)],
                                      raw_ref.at[2 + half, j * 256:(j + 1) * 256], sem_in.at[76 + half * 4 + j])
                for j in range(4)]

    def bx_copy(p):
        rows = pl.ds(pl.multiple_of(p * 64, 64), 64)
        return pltpu.make_async_copy(bx_hbm.at[:, rows, :], bx_ref.at[0:4, rows, :], sem_in.at[64 + p])

    n_head = N_L1 * 2 * SEG
    cp_x = [pltpu.make_async_copy(x_hbm.at[lo:hi, half * 512:(half + 1) * 512], xo_ref.at[half, lo:hi],
                                  sem_in.at[72 + (lo > 0) * 2 + half])
            for lo, hi in ((0, n_head), (n_head, S)) for half in range(2)]
    cp_mem = pltpu.make_async_copy(mem_hbm, mem_ref, sem_in.at[1])
    cp_fd = pltpu.make_async_copy(fd_hbm, fd_ref, sem_in.at[4])
    cp_ms = pltpu.make_async_copy(ms_hbm, ms_ref, sem_in.at[5])
    cp_tv = pltpu.make_async_copy(tv_hbm, tv_ref, sem_in.at[6])
    cp_wt = [pltpu.make_async_copy(src.at[:, pl.ds(lg * 256, 256)], wt_ref.at[a * 8 + lg], sem_in.at[48 + a * 8 + lg])
             for a, src in enumerate((wr_hbm, wi_hbm)) for lg in range(8)]

    for i in range(8):
        raw_copy(0, i, 128).start()
        if i < 4:
            xc_copy(i).start()
        if 3 <= i < 7:
            xc_copy(i + 1).start()
        if i >= 3:
            raw_copy(2, i - 3, 128).start()
        if i == 7:
            raw_copy(2, 5, 128).start()
        raw_copy(1, i, 128).start()
    for i in range(6, 8):
        raw_copy(2, i, 128).start()
    for i in range(2):
        raw_copy(3, i, 512).start()
    for cp in cp_x[0:2] + [cp_mem, cp_fd, cp_tv] + [bx_copy(p) for p in range(8)] + cp_x[2:4] + [cp_ms]:
        cp.start(priority=1)

    zero_ref[0] = 0

    def pin_slot(n):
        return n - jnp.clip(zero_ref[0], 0, 1) * 4

    def pin_rows(r):
        return pl.ds(pl.multiple_of(r + jnp.clip(zero_ref[0], 0, 1) * 32, 8), 8)

    for p in range(8):
        for jq in range(4):
            tw_ref[(p * 4 + jq) * 2] = jnp.float32(math.cos(2 * math.pi * p * jq / 32))
            tw_ref[(p * 4 + jq) * 2 + 1] = jnp.float32(math.sin(2 * math.pi * p * jq / 32))

    ub_ref[128:136] = jnp.zeros((8, 128, 128), f32)
    wp_ref[12800:12872] = jnp.zeros((72, 128), u32)

    qi = jax.lax.broadcasted_iota(jnp.int32, (48, 128), 0)
    ki = jax.lax.broadcasted_iota(jnp.int32, (48, 128), 1)

    def between(v, lo, hi):
        return (v >= lo) & (v < hi)

    def table(keep, other):
        return jnp.where(other, -jnp.inf, jnp.where(keep, 0.0, NEG)).astype(f32)

    keep = between(qi, 8, 16) | between(ki, 8, 16) | (qi >= jnp.where(ki < 32, ki, ki - 24))
    fille_ref[...] = table(keep, ki >= 40)[:32]
    q_even = between(qi, 32, 40)
    k_even = between(ki, 32, 40) | (ki >= 48)
    qpos = jnp.where(qi < 32, qi, jnp.where(qi < 40, qi - 24, qi - 32))
    kpos = jnp.where(ki < 32, ki, jnp.where(ki < 40, ki - 24, jnp.where(ki < 48, ki - 32, ki - 48)))
    keep = between(qi, 8, 16) | between(ki, 8, 16) | (ki >= 56) | (qpos >= kpos)
    fillo_ref[...] = table(keep, (q_even != k_even) | (ki >= 64))

    def relayout16(c, blk):
        w0 = pl.multiple_of(blk * 8, 8)
        v = _tou(raw_ref[c % 4, pl.ds(blk * 16, 16)]).reshape(8, 2, 8, 128)
        a, b = v[:, 0], v[:, 1]
        w_refs[c][0:8, pl.ds(w0, 8), :] = jnp.swapaxes((a & jnp.uint32(0xFFFF)) | (b << 16), 0, 1)
        w_refs[c][8:16, pl.ds(w0, 8), :] = jnp.swapaxes((a >> 16) | (b & jnp.uint32(0xFFFF0000)), 0, 1)

    def slot_of(h):
        return (h // 16) * 16 + (h % 2) * 8 + (h % 16) // 2

    def repack_wo(i, blk):
        v = _tou(raw_ref[2 + i, blk * 32:(blk + 1) * 32]).reshape(256, 128)
        wo_ref[i, blk // 8, (blk % 8) * 256:(blk % 8 + 1) * 256] = v

    sub4 = jax.lax.broadcasted_iota(jnp.int32, (128, 128), 0) & 3

    def wp_store(t, kb, tile):
        v = tile.T.reshape(4, 32, 128)
        v = jnp.concatenate([v, v[:, 0:8]], axis=1).reshape(160, 128)
        wp_ref[pl.ds(pl.multiple_of(t * 2560 + kb * 160, 32), 160), :] = v

    def b_prep(lg, hb, par):
        cols = slice(hb * 128, (hb + 1) * 128)
        a = _tou(wt_ref[lg, 0:512, cols])
        b = _tou(wt_ref[8 + lg, 0:512, cols])
        if par == 0:
            w = (a << 16) | (b & jnp.uint32(0xFFFF))
            m = (sub4 == 0) | (sub4 == 2)
        else:
            w = (a & jnp.uint32(0xFFFF0000)) | (b >> 16)
            m = (sub4 == 0) | (sub4 == 3)
        top = w[:128]
        bot = pltpu.roll(w[128:].reshape(16, 8, 128), 1 + par, 1).reshape(128, 128)
        wp_store(par, lg * 2 + hb, jnp.where(m, top, bot))
        wp_store(par + 2, lg * 2 + hb, jnp.where(m, bot, top))
        if par == 0:
            na = jnp.broadcast_to(wt_ref[lg, 512:513, cols].astype(f32), (128, 128))
            nb = jnp.broadcast_to(wt_ref[8 + lg, 512:513, cols].astype(f32), (128, 128))
            wp_store(4, lg * 2 + hb, pltpu.bitcast(na, u32) | (pltpu.bitcast(nb, u32) >> 16))

    def gather_c(k):
        xc_ref[k] = _tou(xcraw_ref[k].astype(f32).reshape(512, 128).astype(bf16))

    def store_qkvc(n, y):
        qkvc_ref[:, n] = y.reshape(NSEG // 2, 8, 128)

    def q_unit(i, groups, first, last, fillers):
        xk = _tobf(xc_ref[i])
        w0 = pl.multiple_of(i * 64, 64)
        for g in groups:
            rhs = jnp.concatenate(
                [_tobf(w_refs[h // 16][h % 16, pl.ds(w0, 64), :]) for h in range(4 * g, 4 * g + 4)], axis=1)
            y = _dot(xk, rhs)
            for h in range(4 * g, 4 * g + 4):
                yh = y[:, (h % 4) * 128:(h % 4 + 1) * 128]
                if not first:
                    yh = yh + ub_ref[h * 4:(h + 1) * 4].reshape(512, 128)
                if last:
                    store_qkvc(h, _tou(yh.astype(bf16)))
                else:
                    ub_ref[h * 4:(h + 1) * 4] = yh.reshape(4, 128, 128)
            mine = fillers.get(g, [])
            for fi, item in enumerate(mine):
                r = (fi * 512 // len(mine)) // 8 * 8
                item(pltpu.bitcast(y[r:r + 8, 0:128], u32))

    def rl_item(c, blk):
        def item(pin):
            w_refs[c][pin_slot(15), 512:520] = pin
            relayout16(c, blk)
        return item

    def spread(fillers, items, groups):
        for k, item in enumerate(items):
            fillers.setdefault(groups[k * len(groups) // len(items)], []).append(item)
        return fillers

    def half_items(f, c, i, groups):
        return spread(f, [rl_item(c, i * 8 + blk) for blk in range(8)], groups)

    def piece_items(i):
        f = half_items(half_items({}, 1, i, (0, 1, 2)), 0, i + 1, (4, 5, 6))
        return spread(f, [lambda pin: gather_c(i + 1)], (7,))

    def chunk2_items(f, lo, hi, groups):
        return spread(f, [rl_item(2, blk) for blk in range(lo, hi)], groups)

    def wait_piece(i):
        raw_copy(1, i, 128).wait()
        raw_copy(0, i + 1, 128).wait()

    raw_copy(0, 0, 128).wait()
    for blk in range(8):
        relayout16(0, blk)
    xc_copy(0).wait()
    gather_c(0)
    q_unit(0, range(0, 2), True, False, {})
    raw_copy(1, 0, 128).wait()
    q_unit(0, range(2, 4), True, False, half_items({}, 1, 0, (2, 2, 3)))
    q_unit(0, range(4, 6), True, False, {})
    xc_copy(1).wait()
    raw_copy(0, 1, 128).wait()
    q_unit(0, range(6, 8), True, False,
           spread(half_items({}, 0, 1, (6, 6, 7)), [lambda pin: gather_c(1)], (6,)))
    raw_copy(1, 1, 128).wait()
    q_unit(1, range(0, 4), False, False, half_items({}, 1, 1, (0, 1, 2)))
    xc_copy(2).wait()
    raw_copy(0, 2, 128).wait()
    q_unit(1, range(4, 8), False, False,
           spread(half_items({}, 0, 2, (4, 5, 6)), [lambda pin: gather_c(2)], (6,)))

    def xsum_item(j, rq):
        def item(pin):
            xs_ref[pin_slot(4), 0, 128:136] = pin
            a11, a21, a12, a22 = [
                xcraw_ref[j + 4 * kh, rh * 32 + rq * 8:rh * 32 + (rq + 1) * 8].astype(f32).reshape(64, 128)
                for kh in range(2) for rh in range(2)]
            for k, v in enumerate((a11 + a22, a21 + a22, a11 + a12, a21 - a11, a12 - a22)):
                xs_ref[k, j, rq * 32:(rq + 1) * 32] = _tou(v.astype(bf16))
        return item

    def q_c(i, carry):
        wait_piece(i)
        xc_copy(i + 2).wait()
        raw_copy(2, i - 2, 128).wait()
        f = half_items(piece_items(i), 2, i - 2, (3, 3, 3, 3, 4, 5, 6, 7))
        q_unit(i, range(8), False, False, spread(f, [xsum_item(i - 2, rq) for rq in range(4)], (3, 4, 5, 6)))
        return carry
    xc_copy(3).wait()
    jax.lax.fori_loop(2, 6, q_c, 0)

    wait_piece(6)
    raw_copy(2, 4, 128).wait()
    raw_copy(2, 5, 128).wait()
    q_unit(6, range(8), False, False, chunk2_items(piece_items(6), 32, 48, (0, 1, 2, 3, 3, 4, 5, 6)))
    raw_copy(1, 7, 128).wait()
    raw_copy(2, 6, 128).wait()
    raw_copy(2, 7, 128).wait()
    q_unit(7, range(8), False, True, chunk2_items(half_items({}, 1, 7, (0, 1, 2)), 48, 64, (3, 4, 5, 6)))
    raw_copy(4).start()
    raw_copy(5).start()
    for cp in cp_wt + wo_copies(0):
        cp.start()

    def bulk_iter(c, i):
        def xs(k):
            return jnp.concatenate([_tobf(xs_ref[k, j, 0:128]) for j in range(4)], axis=1)

        def xc(rh, kh):
            return jnp.concatenate(
                [_tobf(xc_ref[4 * kh + j, rh * 128:(rh + 1) * 128]) for j in range(4)], axis=1)

        for pr in range(4):
            n1 = i * 8 + pr * 2
            n2 = n1 + 1

            def w(n, kh):
                return _tobf(w_refs[c][n, kh * 256:(kh + 1) * 256])

            def wsum(a, b, sign):
                a, b = a.astype(f32), b.astype(f32)
                return (a + b if sign > 0 else a - b).astype(bf16)

            def out(rh, n, v):
                qkvc_ref[rh * 16:(rh + 1) * 16, c * 16 + n] = _tou(v.astype(bf16)).reshape(16, 8, 128)

            def side(k, m):
                for blk, r in ((k, 0), (7, 128)) if k == 0 else ((k, 0),):
                    pin = pltpu.bitcast(m[r:r + 8], u32)
                    if c + 1 < 6:
                        w_refs[c + 1][pin_slot(15), 512:520] = pin
                        relayout16(c + 1, i * 32 + (pr * 8 + blk))
                    else:
                        wo_ref[pin_slot(4) >> 2, 3, 2048:2056] = pin
                        repack_wo(i, pr * 8 + blk)
                if c >= 4 and k in (1, 4):
                    wp_ref[pin_rows(12832), :] = pltpu.bitcast(m[128:136], u32)
                    b_prep((c - 4) * 4 + i * 2 + pr // 2, pr % 2, k // 4)

            m2 = _dot(xs(1), w(n1, 0))
            side(0, m2)
            m4 = _dot(xc(1, 1), wsum(w(n1, 1), w(n1, 0), -1))
            side(1, m4)
            out(1, n1, m4 + m2)
            m1 = _dot(xs(0), wsum(w(n1, 0), w(n2, 1), 1))
            side(2, m1)
            m5 = _dot(xs(2), w(n2, 1))
            side(3, m5)
            m3 = _dot(xc(0, 0), wsum(w(n2, 0), w(n2, 1), -1))
            side(4, m3)
            out(0, n2, m3 + m5)
            c22 = _dot(xs(3), wsum(w(n1, 0), w(n2, 0), 1)) + ((m1 - m2) + m3)
            side(5, c22)
            out(1, n2, c22)
            c11 = _dot(xs(4), wsum(w(n1, 1), w(n2, 1), 1)) + ((m1 + m4) - m5)
            side(6, c11)
            out(0, n1, c11)

    for c in range(2, 6):
        if c == 4:
            for cp in cp_wt:
                cp.wait()
        if c == 3:
            for cp in wo_copies(1):
                cp.start()
        if 2 < c < 5:
            raw_copy(c + 1).wait()

        def bulk(i, carry, c=c):
            if c == 2:
                raw_copy(3, i, 512).wait()
            if c == 5:
                for cp in wo_copies(i):
                    cp.wait()
            bulk_iter(c, i)
            return carry
        jax.lax.fori_loop(0, 2, bulk, 0)

    cp_x[0].wait()
    cp_x[1].wait()
    cp_mem.wait()
    cp_fd.wait()
    cp_tv.wait()

    lane = jax.lax.broadcasted_iota(jnp.int32, (1, 128), 1)
    lane0 = lane == 0
    sgn0 = jnp.where(lane0, 1.0, -1.0)

    def first_lanes(t):
        la, lb = [k for k in range(4) if _FIRST[t][k]]
        return ((lane & 3) == la) | ((lane & 3) == lb)

    def d_products(st_ref, d, t, rows):
        return [_dot(st_ref[n, rows].astype(bf16), _tobf(fd_ref[d * 12 + n])) if n else None
                for n in range(3 * t, 3 * t + 3)]

    def twiddles(p):
        return [(tw_ref[p * 8 + jq * 2], tw_ref[p * 8 + jq * 2 + 1]) if jq else None for jq in range(4)]

    def p1_pre(p, rs, q):
        def item(y):
            sa_ref[0, pin_rows(0), :] = y
            xq = bx_ref[q, pl.ds(pl.multiple_of(p * 64 + rs * 16, 16), 16), :].astype(f32)
            zz = _r8_real([xq[:, a * 128:(a + 1) * 128] for a in range(8)])
            r = (rs * 4 + q) * 16
            sa_ref[1:12, r:r + 16] = jnp.stack([v for (a, b) in zz for v in (a + b, b, a)][1:])
        return item

    def p1_mm(p, t):
        def item(y):
            cs = twiddles(p)

            def put(ref, n, rs, re, im):
                v = jnp.stack([re.reshape(2, 8, 128), im.reshape(2, 8, 128)], axis=1)
                ref[n * 8 + p, rs * 32:(rs + 1) * 32] = v.reshape(32, 128)

            first = first_lanes(t)
            for rs in range(4):
                k1, k2, k3 = d_products(sa_ref, 0, t, slice(rs * 64, (rs + 1) * 64))
                if t == 0:
                    up = jnp.where(first, k2, k3)
                    re, im = jnp.where(first, k3, k2), pltpu.roll(up, 126, 1)
                    ny = jnp.where(lane0, im, up)
                    u = [ny[q * 16:(q + 1) * 16] for q in range(4)]
                    odd_lane = (lane & 1) == 1
                    nr = jnp.where(odd_lane, pltpu.roll(u[0] - u[2], 1, 1), u[0] + u[2] + (u[1] + u[3]) * sgn0)
                    ni = jnp.where(odd_lane, pltpu.roll((u[3] - u[1]) * sgn0, 1, 1), 0.0)
                    rows = pl.ds(pl.multiple_of(p * 64 + rs * 16, 16), 16)
                    c, sn = tv_ref[0, rows], tv_ref[1, rows]
                    put(ny_ref, 0, rs, nr * c + ni * sn, ni * c - nr * sn)
                    im = jnp.where(lane0, 0.0, im)
                else:
                    re, im = k1 + k2, (k3 - k1) * jnp.where(first, 1.0, -1.0)
                a = _dft4([(re[q * 16:(q + 1) * 16], im[q * 16:(q + 1) * 16]) for q in range(4)])
                for jq in range(4):
                    re, im = a[jq]
                    if jq > 0:
                        c, sn = cs[jq]
                        re, im = re * c + im * sn, im * c - re * sn
                    put(ub_ref, t * 4 + jq, rs, re, im)
        return item

    def p2_bfly(u, g, inverse, ref=ub_ref):
        def item(y):
            if y is not None:
                ub_ref[136, pin_rows(0), :] = y
            v = ref[pl.ds(u * 8, 8), g * 16:(g + 1) * 16]
            x = [(v[p, 0:8], v[p, 8:16]) for p in range(8)]
            x = _swap(_dft8(_swap(x))) if inverse else _dft8(x)
            ref[pl.ds(u * 8, 8), g * 16:(g + 1) * 16] = jnp.stack([w for c in x for w in c]).reshape(8, 16, 128)
        return item

    def filtered(xx, w):
        wr = pltpu.bitcast(w & jnp.uint32(0xFFFF0000), f32).reshape(8, 8, 128)
        wi = pltpu.bitcast(w << 16, f32).reshape(8, 8, 128)
        xx = xx.reshape(8, 2, 8, 128)
        xr, xi = xx[:, 0], xx[:, 1]
        return jnp.stack([xr * wr - xi * wi, xr * wi + xi * wr], axis=1).reshape(128, 128)

    def p2_fwd(u, jps):
        def item(y):
            t = u >> 2
            jq = u & 3
            xs = [_dot(_tobf(ms_ref[jq + 4 * jp]), ub_ref[u * 8 + jp].astype(bf16)) for jp in jps]
            for jp, xx in zip(jps, xs):
                ub_ref[u * 8 + jp] = filtered(xx, wp_ref[pl.ds(t * 2560 + jq + 4 * jp, 64, stride=40), :])
        return item

    def p2_nyq(u):
        def item(y):
            jp = u & 7
            rhs = ny_ref[jp].astype(bf16)
            xx = jnp.concatenate([_dot(_tobf(ms_ref[u * 4, m * 16:(m + 1) * 16]), rhs) for m in range(4)], axis=0)
            w = wp_ref[pl.ds(4 * 2560 + 4 * jp, 64, stride=40), :]
            for jq in range(1, 4):
                w = jnp.where(lane == jq, wp_ref[pl.ds(4 * 2560 + 4 * jp + jq, 64, stride=40), :], w)
            w = jnp.where(u < 8, w, jnp.uint32(0x3F800000))
            ny_ref[jp] = filtered(xx, w)
        return item

    def p2_inv(u, jps):
        def item(y):
            jq = u & 3
            zs = [_dot(_tobf(ms_ref[32 + jq + 4 * jp]), ub_ref[u * 8 + jp].astype(bf16)) for jp in jps]
            for jp, zz in zip(jps, zs):
                ub_ref[u * 8 + jp] = zz
        return item

    def p3_pre(p, g, t):
        def item(y):
            sa_ref[0, pin_rows(0), :] = y
            cs = twiddles(p)

            def fetch(t):
                a = []
                for jq in range(4):
                    v = ub_ref[(t * 4 + jq) * 8 + p, g * 16:(g + 1) * 16]
                    re, im = v[0:8], v[8:16]
                    if jq > 0:
                        c, sn = cs[jq]
                        re, im = re * c - im * sn, im * c + re * sn
                    a.append((re, im))
                return _swap(_dft4(_swap(a)))

            u = fetch(t)
            if t == 0:
                v = ny_ref[p, g * 16:(g + 1) * 16]
                rows = pl.ds(pl.multiple_of(p * 64 + g * 8, 8), 8)
                c, sn = tv_ref[0, rows], tv_ref[1, rows]
                nr, ni = v[0:8] * c - v[8:16] * sn, v[8:16] * c + v[0:8] * sn
                zr, zi = pltpu.roll(nr, 127, 1), pltpu.roll(ni, 127, 1)
                ny = (nr + zr, (nr - zi) * sgn0, nr - zr, (nr + zi) * sgn0)
            first = first_lanes(t)
            for q in range(4):
                re, im = u[q]
                rows = slice(q * 64 + g * 8, q * 64 + (g + 1) * 8)
                if t == 0:
                    im = pltpu.roll(jnp.where(lane0, ny[q], im), 2, 1) + jnp.where(lane == 2, ny[q], 0.0)
                    sa_ref[1:3, rows] = jnp.stack((jnp.where(first, im, re), jnp.where(first, re, im)))
                else:
                    im = im * jnp.where(first, 1.0, -1.0)
                    sa_ref[3 * t:3 * t + 3, rows] = jnp.stack((re + im, im, re))
        return item

    def p3_mm(p, q):
        def item(y):
            g = []
            for t in range(4):
                k1, k2, k3 = d_products(sa_ref, 1, t, slice(q * 64, (q + 1) * 64))
                g.append((k3, k2) if t == 0 else (k2 + k1, k3 - k1))
            yy = _r8_real_t(g)
            bx_ref[q, pl.ds(pl.multiple_of(p * 64, 64), 64), :] = jnp.concatenate(yy, axis=1).astype(bf16)
        return item

    def b_out(p):
        def item(y):
            rows = pl.ds(pl.multiple_of(p * 64, 64), 64)
            pltpu.make_async_copy(bx_ref.at[0:4, rows, :], out_hbm.at[:, rows, pl.ds(DM, DM)],
                                  sem_out.at[1]).start()
            bx_ref[4, pin_rows(0), 0:128] = y.astype(bf16)
        return item

    def a_out(blk, half):
        pltpu.make_async_copy(
            xo_ref.at[half, pl.ds(pl.multiple_of(blk * 64, 64), 64), :],
            out_hbm.at[blk >> 3, pl.ds(pl.multiple_of((blk & 7) * 64, 64), 64),
                       pl.ds(pl.multiple_of(half * 512, 512), 512)],
            sem_out.at[0]).start()

    def step(pp, odd, mem, hooks, fast=False):
        r0 = pl.multiple_of(pp * 64 + 32 * odd, SEG)
        xs = jnp.concatenate([xo_ref[0, pl.ds(r0, SEG), :], xo_ref[1, pl.ds(r0, SEG), :]], axis=1)
        x_lo = xs[0:8].astype(f32)
        hm = jnp.concatenate(
            [jnp.concatenate([x_lo, jnp.concatenate(mem, axis=1)], axis=0).astype(bf16), xs[16:32]], axis=0)
        fill = fillo_ref[:, 0:64] if odd else fille_ref[:, 0:48]
        nrow = 48 if odd else 32
        qkv, ps = {}, {}

        def head_of(v):
            return (v // 16) * 16 + (v % 2) * 8 + (v % 16) // 2 if fast else v

        def do_qkv(v0, v1):
            for v in range(v0, v1):
                h = head_of(v)
                for t in range(3):
                    n = t * H + slot_of(h)
                    y32 = _dot(hm, _tobf(w_refs[n // 16][n % 16, 0:512]))
                    y = y32.astype(bf16)
                    parts = [y]
                    if odd or t > 0:
                        parts.append(_tobf(qkvc_ref[pp, n]))
                    if t > 0:
                        if odd:
                            parts.append(_tobf(kve_ref[(t - 1) * H + h]))
                        else:
                            kve_ref[(t - 1) * H + h] = _tou(y[0:16])
                    qkv[(t, v)] = jnp.concatenate(parts, axis=0) if len(parts) > 1 else y
                for item in hooks.get(v, ()):
                    item(y32[0:8])

        def do_s(g):
            for v in range(g * G, (g + 1) * G):
                sc = jax.lax.dot_general(qkv[(0, v)], qkv[(1, v)], (((1,), (1,)), ((), ())),
                                         preferred_element_type=f32)
                sc = jnp.where(fill == 0.0, sc * scale, fill)
                e = jnp.exp(sc - jnp.max(sc, axis=1, keepdims=True))
                den = jnp.sum(e, axis=1, keepdims=True)
                r = pl.reciprocal(den, approx=True)
                r = r * (2.0 - den * r)
                ps[v] = (e * r).astype(bf16)

        def do_pv(g):
            o = {v: _dot(ps[v], qkv[(2, v)]) for v in range(g * G, (g + 1) * G)}
            for v in o:
                h = head_of(v)
                oall_ref[0:nrow // 2, h * DH:(h + 1) * DH] = _tou(o[v].astype(bf16))
            if fast:
                for v in range(g * G, (g + 1) * G, 2):
                    a11, a12 = o[v][0:32], o[v + 1][0:32]
                    a21 = jnp.concatenate([oc_ref[head_of(v)], o[v][32:48]], axis=0)
                    a22 = jnp.concatenate([oc_ref[head_of(v + 1)], o[v + 1][32:48]], axis=0)
                    for k, a in enumerate((a11 + a22, a21 + a22, a22, a11 + a12, a21 - a11, a12 - a22)):
                        os_ref[k, :, (v // 2) * DH:(v // 2 + 1) * DH] = _tou(a.astype(bf16))
            if odd:
                for v in o:
                    oc_ref[head_of(v)] = o[v][32:48]

        def plain(half, j, rows, h0, h1):
            return _dot(_tobf(oall_ref[0:rows // 2, h0 * DH:h1 * DH]), _tobf(wo_ref[half, j, h0 * 64:h1 * 64, :]))

        hb = pp & 1
        if fast:
            def product(jp, k):
                def fn(part):
                    h0 = part * 16
                    if k == 2:
                        lhs = oall_ref[0:16, h0 * DH:(h0 + 8) * DH]
                    else:
                        lhs = os_ref[k - (k > 2), :, part * 1024:(part + 1) * 1024]
                    if k == 1:
                        rhs = wo_ref[hb, jp * 2, h0 * 64:(h0 + 8) * 64, :]
                    elif k == 4:
                        rhs = wo_ref[hb, jp * 2 + 1, (h0 + 8) * 64:(h0 + 16) * 64, :]
                    else:
                        rhs = ws_ref[hb, jp * 5 + (0, 0, 1, 2, 0, 3, 4)[k], part * 512:(part + 1) * 512, :]
                    return _dot(_tobf(lhs), _tobf(rhs))
                return fn
            jobs = [product(jp, k) for jp in range(2) for k in range(7)]
            jobs += [(lambda part, j=j: plain(1 - hb, j, 32, part * 16, part * 16 + 16)) for j in range(4)]
            marks = (3, 12)
        else:
            jobs = [(lambda part, j=j: plain(j // 4, j % 4, nrow, part * 24, 24 + part * 8)) for j in range(8)]
            marks = (2, 5)

        for g in range(NG):
            do_qkv(g * G, g * G + G // 2)
            if g >= 1:
                do_s(g - 1)
            do_qkv(g * G + G // 2, (g + 1) * G)
            if g >= 2:
                do_pv(g - 2)
        part = []
        for k, job in enumerate(jobs):
            items = hooks.get(('o', k), ())
            if len(items) == 2:
                half = plain(k // 4, k % 4, nrow, 0, 12)
                items[0](half[0:8])
                part.append(plain(k // 4, k % 4, nrow, 12, 24) + half)
                items[1](part[k][0:8])
            else:
                part.append(job(0))
                for item in items:
                    item(part[k][0:8])
            if k == marks[0]:
                do_s(NG - 1)
                do_pv(NG - 2)
            if k == marks[1]:
                do_pv(NG - 1)

        def put(half, j, r, v):
            xo_ref[half, pl.ds(r0 + r, v.shape[0]), j * 128:(j + 1) * 128] = v.astype(bf16)

        if fast:
            own = []
            for jp in range(2):
                m1, m2, m3, m4, m5, m6, m7 = [jobs[jp * 7 + k](1) + part[jp * 7 + k] for k in range(7)]
                for jj, top, bot in ((0, ((m1 + m4) - m5) + m7, m2 + m4), (1, m3 + m5, ((m1 - m2) + m3) + m6)):
                    j = jp * 2 + jj
                    own.append(top[8:16])
                    put(hb, j, 0, jnp.concatenate([top[0:8], bot[24:32], top[16:32]], axis=0))
                    put(hb, j, -24, bot[16:24])
                    put(hb, j, -56, bot[8:16])
                    put(hb, j, -88, bot[0:8])
            for j in range(4):
                res = jobs[14 + j](1) + part[14 + j]
                own.append(res[8:16])
                put(1 - hb, j, 0, res)
            new_mem = [jnp.where(hb == 0, own[j], own[(j + 4) % 8]) for j in range(8)]
        else:
            new_mem = []
            for j in range(8):
                res = jobs[j](1) + part[j]
                new_mem.append(res[8:16])
                if odd:
                    put(j // 4, j % 4, 0, jnp.concatenate([res[0:8], res[40:48], res[16:32]], axis=0))
                    put(j // 4, j % 4, -24, res[32:40])
                else:
                    put(j // 4, j % 4, 0, res)
        for item in hooks.get(H, ()):
            item(None)
        if odd:
            a_out(pp, hb)
            if fast:
                a_out(pp - 1, hb)
            else:
                pl.when(pp > 0)(lambda: a_out(pp - 1, hb))
        return new_mem

    def wsum_item(i, k):
        def item(y):
            ws_ref[pin_slot(4) >> 2, 9, 1024:1032] = pltpu.bitcast(y, u32)
            jp = k & 1
            r = (i & 1) * 256 + (k >> 1) * 16
            b11, b21, b12, b22 = [
                _tobf(wo_ref[i >> 2, jp * 2 + jj, pl.ds(pl.multiple_of((i & 2) * 512 + r + kh * 512, 16), 16), :]
                      ).astype(f32) for jj in range(2) for kh in range(2)]
            rows = pl.ds(pl.multiple_of((i & 2) * 256 + r, 16), 16)
            for n, v in enumerate((b11 + b22, b12 - b22, b21 - b11, b11 + b12, b21 + b22)):
                ws_ref[i >> 2, jp * 5 + n, rows, :] = _tou(v.astype(bf16))
        return item

    def l1(i, mem):
        bx_copy(i).wait()
        he = {2 * k: [p1_pre(i, k // 4, k % 4)] for k in range(16)}
        he[H] = [p1_mm(i, 1)]
        ho = {('o', 0): [p1_mm(i, 2)], ('o', 3): [p1_mm(i, 3)], ('o', 5): [p1_mm(i, 0)]}
        ho.update({k: [wsum_item(i, k)] for k in range(32)})
        mem = step(i, 0, mem, he)
        mem = step(i, 1, mem, ho)
        return mem

    def l2(i, mem):
        u = i - N_L1
        he = {3: [p2_fwd(u, range(0, 4))], 7: [p2_fwd(u, range(4, 8))], 17: [p2_nyq(u)],
              H: [p2_inv(u, range(0, 8))]}
        ho = {('o', k): [p2_bfly(u + k % 2, k // 2, k % 2 == 0)] for k in range(16)}
        mem = step(i, 0, mem, he)
        mem = step(i, 1, mem, ho, fast=True)
        return mem

    def l3(i, mem):
        p = i - N_L1 - N_L2
        he = {h: [p3_pre(p, h // 3, 1 + h % 3)] for h in range(24)}
        for j in range(4):
            he[('o', 3 + j)] = [p3_pre(p, 2 * j, 0), p3_pre(p, 2 * j + 1, 0)]
        he[H] = [p3_mm(p, q) for q in range(4)]
        ho = {12: [b_out(p)]}
        mem = step(i, 0, mem, he)
        mem = step(i, 1, mem, ho, fast=True)
        return mem

    m0 = mem_ref[...].astype(f32)
    mem = [m0[:, j * 128:(j + 1) * 128] for j in range(8)]
    mem = jax.lax.fori_loop(0, N_L1, l1, mem)
    cp_x[2].wait()
    cp_x[3].wait()
    cp_ms.wait()
    for g in range(8):
        p2_bfly(0, g, False)(None)
        p2_bfly(0, g, False, ny_ref)(None)
    mem = jax.lax.fori_loop(N_L1, N_L1 + N_L2, l2, mem)
    for g in range(8):
        p2_bfly(0, g, True, ny_ref)(None)
    mem = jax.lax.fori_loop(N_L1 + N_L2, NSEG // 2, l3, mem)

    for j in range(4):
        res = _dot(_tobf(oall_ref[16:24, :]), _tobf(wo_ref[0, j, 0:2048, :])).astype(bf16)
        xo_ref[0, S - 56:S - 48, j * 128:(j + 1) * 128] = res[0:8]
        xo_ref[0, S - 24:S - 16, j * 128:(j + 1) * 128] = res[8:16]
    a_out(NSEG // 2 - 1, 0)

    pltpu.make_async_copy(bx_ref.at[0:4], out_hbm.at[:, :, pl.ds(DM, DM)], sem_out.at[1]).wait()
    pltpu.make_async_copy(xo_ref, xo_ref, sem_out.at[0]).wait()


@jax.jit
def _run(x, mem0, wq, wk, wv, wo, bx, w_r, w_i):
    fd, ms, tv = _tables()
    hbm = pl.BlockSpec(memory_space=pl.ANY)
    out = pl.pallas_call(
        _kernel,
        out_shape=jax.ShapeDtypeStruct((4, S // 4, 2 * DM), bf16),
        in_specs=[hbm] * 13,
        out_specs=hbm,
        scratch_shapes=[
            pltpu.VMEM((2, S, DM // 2), bf16),
            pltpu.VMEM((MEM, DM), bf16),
            pltpu.VMEM((8, NSEG, 8, 128), bf16),
            pltpu.VMEM((4, DM, 16, DH), bf16),
        ] + [pltpu.VMEM((16, DM // 2 + 8, DH), u32)] * 6 + [
            pltpu.VMEM((2, 4, H * DH // 2 + 8, 128), u32),
            pltpu.VMEM((8, 256, 128), u32),
            pltpu.VMEM((5, 4, 136, 128), u32),
            pltpu.VMEM((NSEG // 2, 3 * H, 8, 128), u32),
            pltpu.VMEM((2 * H, 8, 128), u32),
            pltpu.VMEM((24, H * DH), u32),
            pltpu.VMEM((H, 16, DH), f32),
            pltpu.VMEM((6, 16, 16 * DH), u32),
            pltpu.VMEM((2, 10, 1040, 128), u32),
            pltpu.VMEM((32, 128), f32),
            pltpu.VMEM((48, 128), f32),
            pltpu.VMEM((5, S // 4, DM), bf16),
            pltpu.VMEM((16, DM // 2 + 1, 256), bf16),
            pltpu.VMEM((12872, 128), u32),
            pltpu.VMEM((137, 128, 128), f32),
            pltpu.VMEM((8, 128, 128), f32),
            pltpu.VMEM((12, 264, 128), f32),
            pltpu.VMEM((24, 64, 128), u32),
            pltpu.VMEM((64, 64, 128), u32),
            pltpu.VMEM((2, 512, 128), f32),
            pltpu.SMEM((64,), f32),
            pltpu.SMEM((1,), jnp.int32),
            pltpu.SemaphoreType.DMA((84,)),
            pltpu.SemaphoreType.DMA((2,)),
        ],
        compiler_params=pltpu.CompilerParams(vmem_limit_bytes=120 * 1024 * 1024,
                                             disable_semaphore_checks=True,
                                             disable_bounds_checks=True),
    )(x.reshape(S, DM), x.reshape(NSEG, SEG, DM), mem0.reshape(MEM, DM), wq, wk, wv,
      wo.reshape(H * DH // 16, 16, DM), bx.reshape(4, S // 4, DM), w_r.T, w_i.T, jnp.asarray(fd), jnp.asarray(ms), jnp.asarray(tv))
    return out.reshape(1, S, 2 * DM)


def pallas_concat_heads__memory_aug_recurrent_mem_tr__spectral_gfnet__prompt_kernel(
    A_x: jax.Array,
    A_mem0: jax.Array,
    A_Wq: jax.Array,
    A_Wk: jax.Array,
    A_Wv: jax.Array,
    A_Wo: jax.Array,
    A_seg_len,
    B_x: jax.Array,
    B_w_r: jax.Array,
    B_w_i: jax.Array,
):
    if isinstance(A_seg_len, int):
        assert A_seg_len == SEG
    assert A_x.shape == (1, S, DM) and A_mem0.shape == (1, MEM, DM) and A_Wq.shape == (DM, H, DH)
    assert B_x.shape == (1, S, DM) and B_w_r.shape == (S, DM // 2 + 1)
    return _run(A_x, A_mem0, A_Wq, A_Wk, A_Wv, A_Wo, B_x, B_w_r, B_w_i)
```

```python
import math

import numpy as np
import jax
import jax.numpy as jnp
import jax.experimental.pallas as pl
import jax.experimental.pallas.tpu as pltpu

bf16 = jnp.bfloat16
f32 = jnp.float32
u32 = jnp.uint32

S, DM = 2048, 1024
H, DH = 32, 128
MEM, SEG = 8, 32
NSEG = S // SEG
SQH = math.sqrt(0.5)

_PAIRS = ((0, 4), (1, 7), (2, 6), (3, 5))
_FIRST = np.array([[1, 1, 0, 0], [1, 0, 1, 0], [0, 1, 1, 0], [0, 1, 0, 1]], bool)


def _pack_rows(a):
    u = np.ascontiguousarray(a, dtype=np.float32).view(np.uint32).astype(np.uint64)
    b = ((u + 0x7FFF + ((u >> 16) & 1)) >> 16).astype(np.uint32)
    return (b[..., 0::2, :] | (b[..., 1::2, :] << 16)).astype(np.uint32)


def _tables():
    k2 = np.zeros((4, 128), np.int64)
    for t in range(4):
        odd = t % 2
        for lam in range(128):
            k = 2 * lam + odd
            if k % 8 not in _PAIRS[t]:
                k = 2 * (128 + 8 * (lam // 8) + (lam % 8 - 1 - odd) % 8) + odd
            assert k % 8 in _PAIRS[t]
            k2[t, lam] = k
    b = np.arange(128)[:, None]
    F = np.zeros((12, 128, 128))
    G = np.zeros((12, 128, 128))
    for t in range(4):
        th = 2 * np.pi * ((b * k2[t][None, :]) % DM) / DM
        C, Sn = np.cos(th), np.sin(th)
        first = ((k2[t] % 8) == _PAIRS[t][0])[None, :]
        assert np.array_equal(first[0], _FIRST[t][np.arange(128) % 4])
        if t == 0:
            im = -Sn
            im[:, 0] = (-1.0) ** np.arange(128)
            im = np.roll(im, 2, axis=1)
            F[1:3] = np.where(first, im, C), np.where(first, C, im)
            G[1:3] = F[1:3]
            G[2, :, 0] *= 0.5
            G[2, :, 2] *= 0.5
        else:
            Sg = np.where(first, Sn, -Sn)
            F[3 * t:3 * t + 3] = C, -(C + Sg), C - Sg
            G[3 * t:3 * t + 3] = F[3 * t:3 * t + 3]
    Finv = np.transpose(G, (0, 2, 1)) * (2.0 / DM)
    fd = _pack_rows(np.concatenate([F, Finv]))
    M = np.zeros((32, 128, 128))
    r = np.arange(64)[None, :]
    l = np.arange(64)[:, None]
    for j in range(32):
        th = 2 * np.pi * ((r * (j + 32 * l)) % S) / S
        C, Sn = np.cos(th), np.sin(th)
        M[j, :64, :64] = C
        M[j, :64, 64:] = Sn
        M[j, 64:, :64] = -Sn
        M[j, 64:, 64:] = C
    perm = np.arange(128).reshape(2, 8, 8).transpose(1, 0, 2).reshape(128)
    M = M[:, perm][:, :, perm]
    Minv = np.transpose(M, (0, 2, 1)) / S
    ms = _pack_rows(np.concatenate([M, Minv]))
    th = 2 * np.pi * np.outer(np.arange(512), np.arange(128) % 4) / S
    tv = np.stack([np.cos(th), np.sin(th)]).astype(np.float32)
    return fd, ms, tv


def _tobf(w):
    return pltpu.bitcast(w, bf16)


def _tou(w):
    return pltpu.bitcast(w, u32)


def _dot(a, b):
    return jnp.dot(a, b, preferred_element_type=f32)


def _r8_real(x):
    t0, t1 = x[0] + x[4], x[0] - x[4]
    t2, t3 = x[2] + x[6], x[2] - x[6]
    t4, t5 = x[1] + x[5], x[1] - x[5]
    t6, t7 = x[3] + x[7], x[3] - x[7]
    e0, e1 = t0 + t2, t0 - t2
    o0, o1 = t4 + t6, t4 - t6
    u, v = SQH * (t5 - t7), SQH * (t5 + t7)
    return [(e0 + o0, e0 - o0), (t1 + u, v + t3), (e1, o1), (t1 - u, v - t3)]


def _r8_real_t(g):
    (z0, z4), (a1, b1), (e1, o1), (a3, b3) = g
    e0, o0 = z0 + z4, z0 - z4
    t1, u = a1 + a3, a1 - a3
    v, t3 = b1 + b3, b1 - b3
    t5, t7 = SQH * (v + u), SQH * (v - u)
    t0, t2 = e0 + e1, e0 - e1
    t4, t6 = o0 + o1, o0 - o1
    return [t0 + t1, t4 + t5, t2 + t3, t6 + t7, t0 - t1, t4 - t5, t2 - t3, t6 - t7]


def _dft4(u):
    (r0, i0), (r1, i1), (r2, i2), (r3, i3) = u
    sr, si, dr, di = r0 + r2, i0 + i2, r0 - r2, i0 - i2
    tr, ti, er, ei = r1 + r3, i1 + i3, r1 - r3, i1 - i3
    return [(sr + tr, si + ti), (dr + ei, di - er), (sr - tr, si - ti), (dr - ei, di + er)]


def _dft8(x):
    a = [(x[p][0] + x[p + 4][0], x[p][1] + x[p + 4][1]) for p in range(4)]
    d = [(x[p][0] - x[p + 4][0], x[p][1] - x[p + 4][1]) for p in range(4)]
    ev = _dft4(a)
    (r0, i0), (r1, i1), (r2, i2), (r3, i3) = d
    b1r, b1i = SQH * (r1 + i1), SQH * (i1 - r1)
    b3r, n3i = SQH * (i3 - r3), SQH * (r3 + i3)
    sr, si, dr, di = r0 + i2, i0 - r2, r0 - i2, i0 + r2
    tr, ti, er, ei = b1r + b3r, b1i - n3i, b1r - b3r, b1i + n3i
    od = [(sr + tr, si + ti), (dr + ei, di - er), (sr - tr, si - ti), (dr - ei, di + er)]
    return [ev[0], od[0], ev[1], od[1], ev[2], od[2], ev[3], od[3]]


def _swap(x):
    return [(b, a) for (a, b) in x]


G = 4
NG = H // G
NEG = -1e9
N_L1, N_L2, N_L3 = 8, 16, 8


def _kernel(x_hbm, x3_hbm, mem_hbm, wq_hbm, wk_hbm, wv_hbm, wo_hbm, bx_hbm, wr_hbm, wi_hbm,
            fd_hbm, ms_hbm, tv_hbm, out_hbm,
            xo_ref, mem_ref, xcraw_ref, raw_ref, w0_ref, w1_ref, w2_ref, w3_ref, w4_ref, w5_ref,
            wo_ref, xc_ref, xs_ref, qkvc_ref, kve_ref,
            oall_ref, oc_ref, os_ref, ws_ref, fille_ref, fillo_ref, bx_ref, wt_ref, wp_ref, ub_ref, ny_ref, sa_ref, fd_ref, ms_ref, tv_ref,
            tw_ref, zero_ref, sem_in, sem_out):
    scale = DH ** -0.5
    w_hbm = (wq_hbm, wk_hbm, wv_hbm)
    w_refs = (w0_ref, w1_ref, w2_ref, w3_ref, w4_ref, w5_ref)

    def raw_copy(c, i=0, nd=DM):
        rows = pl.ds(pl.multiple_of(i * nd, nd), nd)
        return pltpu.make_async_copy(
            w_hbm[c // 2].at[rows, pl.ds((c % 2) * 16, 16), :],
            raw_ref.at[c % 4, rows], sem_in.at[8 + min(c, 3) * 8 + max(c - 3, 0) * 2 + i])

    def xc_copy(k):
        return pltpu.make_async_copy(
            x3_hbm.at[:, pl.ds(8, 8), pl.ds(pl.multiple_of(k * 128, 128), 128)], xcraw_ref.at[k], sem_in.at[40 + k])

    def wo_copies(half):
        return [pltpu.make_async_copy(wo_hbm.at[:, :, pl.ds(pl.multiple_of(half * 512 + j * 128, 128), 128)],
                                      raw_ref.at[2 + half, j * 256:(j + 1) * 256], sem_in.at[76 + half * 4 + j])
                for j in range(4)]

    def bx_copy(p):
        rows = pl.ds(pl.multiple_of(p * 64, 64), 64)
        return pltpu.make_async_copy(bx_hbm.at[:, rows, :], bx_ref.at[0:4, rows, :], sem_in.at[64 + p])

    n_head = N_L1 * 2 * SEG
    cp_x = [pltpu.make_async_copy(x_hbm.at[lo:hi, half * 512:(half + 1) * 512], xo_ref.at[half, lo:hi],
                                  sem_in.at[72 + (lo > 0) * 2 + half])
            for lo, hi in ((0, n_head), (n_head, S)) for half in range(2)]
    cp_mem = pltpu.make_async_copy(mem_hbm, mem_ref, sem_in.at[1])
    cp_fd = pltpu.make_async_copy(fd_hbm, fd_ref, sem_in.at[4])
    cp_ms = pltpu.make_async_copy(ms_hbm, ms_ref, sem_in.at[5])
    cp_tv = pltpu.make_async_copy(tv_hbm, tv_ref, sem_in.at[6])
    cp_wt = [pltpu.make_async_copy(src.at[:, pl.ds(lg * 256, 256)], wt_ref.at[a * 8 + lg], sem_in.at[48 + a * 8 + lg])
             for a, src in enumerate((wr_hbm, wi_hbm)) for lg in range(8)]

    for i in range(8):
        raw_copy(0, i, 128).start()
        if i < 4:
            xc_copy(i).start()
        if 3 <= i < 7:
            xc_copy(i + 1).start()
        if i >= 3:
            raw_copy(2, i - 3, 128).start()
        if i == 7:
            raw_copy(2, 5, 128).start()
        raw_copy(1, i, 128).start()
    for i in range(6, 8):
        raw_copy(2, i, 128).start()
    for i in range(2):
        raw_copy(3, i, 512).start()
    for cp in cp_x[0:2] + [cp_mem, cp_fd, cp_tv] + [bx_copy(p) for p in range(8)] + cp_x[2:4] + [cp_ms]:
        cp.start(priority=1)

    zero_ref[0] = 0

    def pin_slot(n):
        return n - jnp.clip(zero_ref[0], 0, 1) * 4

    def pin_rows(r):
        return pl.ds(pl.multiple_of(r + jnp.clip(zero_ref[0], 0, 1) * 32, 8), 8)

    for p in range(8):
        for jq in range(4):
            tw_ref[(p * 4 + jq) * 2] = jnp.float32(math.cos(2 * math.pi * p * jq / 32))
            tw_ref[(p * 4 + jq) * 2 + 1] = jnp.float32(math.sin(2 * math.pi * p * jq / 32))

    ub_ref[128:136] = jnp.zeros((8, 128, 128), f32)
    wp_ref[12800:12872] = jnp.zeros((72, 128), u32)

    qi = jax.lax.broadcasted_iota(jnp.int32, (48, 128), 0)
    ki = jax.lax.broadcasted_iota(jnp.int32, (48, 128), 1)

    def between(v, lo, hi):
        return (v >= lo) & (v < hi)

    def table(keep, other):
        return jnp.where(other, -jnp.inf, jnp.where(keep, 0.0, NEG)).astype(f32)

    keep = between(qi, 8, 16) | between(ki, 8, 16) | (qi >= jnp.where(ki < 32, ki, ki - 24))
    fille_ref[...] = table(keep, ki >= 40)[:32]
    q_even = between(qi, 32, 40)
    k_even = between(ki, 32, 40) | (ki >= 48)
    qpos = jnp.where(qi < 32, qi, jnp.where(qi < 40, qi - 24, qi - 32))
    kpos = jnp.where(ki < 32, ki, jnp.where(ki < 40, ki - 24, jnp.where(ki < 48, ki - 32, ki - 48)))
    keep = between(qi, 8, 16) | between(ki, 8, 16) | (ki >= 56) | (qpos >= kpos)
    fillo_ref[...] = table(keep, (q_even != k_even) | (ki >= 64))

    def relayout16(c, blk):
        w0 = pl.multiple_of(blk * 8, 8)
        v = _tou(raw_ref[c % 4, pl.ds(blk * 16, 16)]).reshape(8, 2, 8, 128)
        a, b = v[:, 0], v[:, 1]
        w_refs[c][0:8, pl.ds(w0, 8), :] = jnp.swapaxes((a & jnp.uint32(0xFFFF)) | (b << 16), 0, 1)
        w_refs[c][8:16, pl.ds(w0, 8), :] = jnp.swapaxes((a >> 16) | (b & jnp.uint32(0xFFFF0000)), 0, 1)

    def slot_of(h):
        return (h // 16) * 16 + (h % 2) * 8 + (h % 16) // 2

    def repack_wo(i, blk):
        v = _tou(raw_ref[2 + i, blk * 32:(blk + 1) * 32]).reshape(256, 128)
        wo_ref[i, blk // 8, (blk % 8) * 256:(blk % 8 + 1) * 256] = v

    sub4 = jax.lax.broadcasted_iota(jnp.int32, (128, 128), 0) & 3

    def wp_store(t, kb, tile):
        v = tile.T.reshape(4, 32, 128)
        v = jnp.concatenate([v, v[:, 0:8]], axis=1).reshape(160, 128)
        wp_ref[pl.ds(pl.multiple_of(t * 2560 + kb * 160, 32), 160), :] = v

    def b_prep(lg, hb, par):
        cols = slice(hb * 128, (hb + 1) * 128)
        a = _tou(wt_ref[lg, 0:512, cols])
        b = _tou(wt_ref[8 + lg, 0:512, cols])
        if par == 0:
            w = (a << 16) | (b & jnp.uint32(0xFFFF))
            m = (sub4 == 0) | (sub4 == 2)
        else:
            w = (a & jnp.uint32(0xFFFF0000)) | (b >> 16)
            m = (sub4 == 0) | (sub4 == 3)
        top = w[:128]
        bot = pltpu.roll(w[128:].reshape(16, 8, 128), 1 + par, 1).reshape(128, 128)
        wp_store(par, lg * 2 + hb, jnp.where(m, top, bot))
        wp_store(par + 2, lg * 2 + hb, jnp.where(m, bot, top))
        if par == 0:
            na = jnp.broadcast_to(wt_ref[lg, 512:513, cols].astype(f32), (128, 128))
            nb = jnp.broadcast_to(wt_ref[8 + lg, 512:513, cols].astype(f32), (128, 128))
            wp_store(4, lg * 2 + hb, pltpu.bitcast(na, u32) | (pltpu.bitcast(nb, u32) >> 16))

    def gather_c(k):
        xc_ref[k] = _tou(xcraw_ref[k].astype(f32).reshape(512, 128).astype(bf16))

    def store_qkvc(n, y):
        qkvc_ref[:, n] = y.reshape(NSEG // 2, 8, 128)

    def q_unit(i, groups, first, last, fillers):
        xk = _tobf(xc_ref[i])
        w0 = pl.multiple_of(i * 64, 64)
        for g in groups:
            rhs = jnp.concatenate(
                [_tobf(w_refs[h // 16][h % 16, pl.ds(w0, 64), :]) for h in range(4 * g, 4 * g + 4)], axis=1)
            y = _dot(xk, rhs)
            for h in range(4 * g, 4 * g + 4):
                yh = y[:, (h % 4) * 128:(h % 4 + 1) * 128]
                if not first:
                    yh = yh + ub_ref[h * 4:(h + 1) * 4].reshape(512, 128)
                if last:
                    store_qkvc(h, _tou(yh.astype(bf16)))
                else:
                    ub_ref[h * 4:(h + 1) * 4] = yh.reshape(4, 128, 128)
            mine = fillers.get(g, [])
            for fi, item in enumerate(mine):
                r = (fi * 512 // len(mine)) // 8 * 8
                item(pltpu.bitcast(y[r:r + 8, 0:128], u32))

    def rl_item(c, blk):
        def item(pin):
            w_refs[c][pin_slot(15), 512:520] = pin
            relayout16(c, blk)
        return item

    def spread(fillers, items, groups):
        for k, item in enumerate(items):
            fillers.setdefault(groups[k * len(groups) // len(items)], []).append(item)
        return fillers

    def half_items(f, c, i, groups):
        return spread(f, [rl_item(c, i * 8 + blk) for blk in range(8)], groups)

    def piece_items(i):
        f = half_items(half_items({}, 1, i, (0, 1, 2)), 0, i + 1, (4, 5, 6))
        return spread(f, [lambda pin: gather_c(i + 1)], (7,))

    def chunk2_items(f, lo, hi, groups):
        return spread(f, [rl_item(2, blk) for blk in range(lo, hi)], groups)

    def wait_piece(i):
        raw_copy(1, i, 128).wait()
        raw_copy(0, i + 1, 128).wait()

    raw_copy(0, 0, 128).wait()
    for blk in range(8):
        relayout16(0, blk)
    xc_copy(0).wait()
    gather_c(0)
    q_unit(0, range(0, 2), True, False, {})
    raw_copy(1, 0, 128).wait()
    q_unit(0, range(2, 4), True, False, half_items({}, 1, 0, (2, 2, 3)))
    q_unit(0, range(4, 6), True, False, {})
    xc_copy(1).wait()
    raw_copy(0, 1, 128).wait()
    q_unit(0, range(6, 8), True, False,
           spread(half_items({}, 0, 1, (6, 6, 7)), [lambda pin: gather_c(1)], (6,)))
    raw_copy(1, 1, 128).wait()
    q_unit(1, range(0, 4), False, False, half_items({}, 1, 1, (0, 1, 2)))
    xc_copy(2).wait()
    raw_copy(0, 2, 128).wait()
    q_unit(1, range(4, 8), False, False,
           spread(half_items({}, 0, 2, (4, 5, 6)), [lambda pin: gather_c(2)], (6,)))

    def xsum_item(j, rq):
        def item(pin):
            xs_ref[pin_slot(4), 0, 128:136] = pin
            a11, a21, a12, a22 = [
                xcraw_ref[j + 4 * kh, rh * 32 + rq * 8:rh * 32 + (rq + 1) * 8].astype(f32).reshape(64, 128)
                for kh in range(2) for rh in range(2)]
            for k, v in enumerate((a11 + a22, a21 + a22, a11 + a12, a21 - a11, a12 - a22)):
                xs_ref[k, j, rq * 32:(rq + 1) * 32] = _tou(v.astype(bf16))
        return item

    def q_c(i, carry):
        wait_piece(i)
        xc_copy(i + 2).wait()
        raw_copy(2, i - 2, 128).wait()
        f = half_items(piece_items(i), 2, i - 2, (3, 3, 3, 3, 4, 5, 6, 7))
        q_unit(i, range(8), False, False, spread(f, [xsum_item(i - 2, rq) for rq in range(4)], (3, 4, 5, 6)))
        return carry
    xc_copy(3).wait()
    jax.lax.fori_loop(2, 6, q_c, 0)

    wait_piece(6)
    raw_copy(2, 4, 128).wait()
    raw_copy(2, 5, 128).wait()
    q_unit(6, range(8), False, False, chunk2_items(piece_items(6), 32, 48, (0, 1, 2, 3, 3, 4, 5, 6)))
    raw_copy(1, 7, 128).wait()
    raw_copy(2, 6, 128).wait()
    raw_copy(2, 7, 128).wait()
    q_unit(7, range(8), False, True, chunk2_items(half_items({}, 1, 7, (0, 1, 2)), 48, 64, (3, 4, 5, 6)))
    raw_copy(4).start()
    raw_copy(5).start()
    for cp in cp_wt + wo_copies(0):
        cp.start()

    def bulk_iter(c, i):
        def xs(k):
            return jnp.concatenate([_tobf(xs_ref[k, j, 0:128]) for j in range(4)], axis=1)

        def xc(rh, kh):
            return jnp.concatenate(
                [_tobf(xc_ref[4 * kh + j, rh * 128:(rh + 1) * 128]) for j in range(4)], axis=1)

        for pr in range(4):
            n1 = i * 8 + pr * 2
            n2 = n1 + 1

            def w(n, kh):
                return _tobf(w_refs[c][n, kh * 256:(kh + 1) * 256])

            def wsum(a, b, sign):
                a, b = a.astype(f32), b.astype(f32)
                return (a + b if sign > 0 else a - b).astype(bf16)

            def out(rh, n, v):
                qkvc_ref[rh * 16:(rh + 1) * 16, c * 16 + n] = _tou(v.astype(bf16)).reshape(16, 8, 128)

            def side(k, m):
                for blk, r in ((k, 0), (7, 128)) if k == 0 else ((k, 0),):
                    pin = pltpu.bitcast(m[r:r + 8], u32)
                    if c + 1 < 6:
                        w_refs[c + 1][pin_slot(15), 512:520] = pin
                        relayout16(c + 1, i * 32 + (pr * 8 + blk))
                    else:
                        wo_ref[pin_slot(4) >> 2, 3, 2048:2056] = pin
                        repack_wo(i, pr * 8 + blk)
                if c >= 4 and k in (1, 4):
                    wp_ref[pin_rows(12832), :] = pltpu.bitcast(m[128:136], u32)
                    b_prep((c - 4) * 4 + i * 2 + pr // 2, pr % 2, k // 4)

            m2 = _dot(xs(1), w(n1, 0))
            side(0, m2)
            m4 = _dot(xc(1, 1), wsum(w(n1, 1), w(n1, 0), -1))
            side(1, m4)
            out(1, n1, m4 + m2)
            m1 = _dot(xs(0), wsum(w(n1, 0), w(n2, 1), 1))
            side(2, m1)
            m5 = _dot(xs(2), w(n2, 1))
            side(3, m5)
            m3 = _dot(xc(0, 0), wsum(w(n2, 0), w(n2, 1), -1))
            side(4, m3)
            out(0, n2, m3 + m5)
            c22 = _dot(xs(3), wsum(w(n1, 0), w(n2, 0), 1)) + ((m1 - m2) + m3)
            side(5, c22)
            out(1, n2, c22)
            c11 = _dot(xs(4), wsum(w(n1, 1), w(n2, 1), 1)) + ((m1 + m4) - m5)
            side(6, c11)
            out(0, n1, c11)

    for c in range(2, 6):
        if c == 4:
            for cp in cp_wt:
                cp.wait()
        if c == 3:
            for cp in wo_copies(1):
                cp.start()
        if 2 < c < 5:
            raw_copy(c + 1).wait()

        def bulk(i, carry, c=c):
            if c == 2:
                raw_copy(3, i, 512).wait()
            if c == 5:
                for cp in wo_copies(i):
                    cp.wait()
            bulk_iter(c, i)
            return carry
        jax.lax.fori_loop(0, 2, bulk, 0)

    cp_x[0].wait()
    cp_x[1].wait()
    cp_mem.wait()
    cp_fd.wait()
    cp_tv.wait()

    lane = jax.lax.broadcasted_iota(jnp.int32, (1, 128), 1)
    lane0 = lane == 0
    sgn0 = jnp.where(lane0, 1.0, -1.0)

    def first_lanes(t):
        la, lb = [k for k in range(4) if _FIRST[t][k]]
        return ((lane & 3) == la) | ((lane & 3) == lb)

    def d_products(st_ref, d, t, rows):
        return [_dot(st_ref[n, rows].astype(bf16), _tobf(fd_ref[d * 12 + n])) if n else None
                for n in range(3 * t, 3 * t + 3)]

    def twiddles(p):
        return [(tw_ref[p * 8 + jq * 2], tw_ref[p * 8 + jq * 2 + 1]) if jq else None for jq in range(4)]

    def p1_pre(p, rs, q):
        def item(y):
            sa_ref[0, pin_rows(0), :] = y
            xq = bx_ref[q, pl.ds(pl.multiple_of(p * 64 + rs * 16, 16), 16), :].astype(f32)
            zz = _r8_real([xq[:, a * 128:(a + 1) * 128] for a in range(8)])
            r = (rs * 4 + q) * 16
            sa_ref[1:12, r:r + 16] = jnp.stack([v for (a, b) in zz for v in (a + b, b, a)][1:])
        return item

    def p1_mm(p, t):
        def item(y):
            cs = twiddles(p)

            def put(ref, n, rs, re, im):
                v = jnp.stack([re.reshape(2, 8, 128), im.reshape(2, 8, 128)], axis=1)
                ref[n * 8 + p, rs * 32:(rs + 1) * 32] = v.reshape(32, 128)

            first = first_lanes(t)
            for rs in range(4):
                k1, k2, k3 = d_products(sa_ref, 0, t, slice(rs * 64, (rs + 1) * 64))
                if t == 0:
                    up = jnp.where(first, k2, k3)
                    re, im = jnp.where(first, k3, k2), pltpu.roll(up, 126, 1)
                    ny = jnp.where(lane0, im, up)
                    u = [ny[q * 16:(q + 1) * 16] for q in range(4)]
                    odd_lane = (lane & 1) == 1
                    nr = jnp.where(odd_lane, pltpu.roll(u[0] - u[2], 1, 1), u[0] + u[2] + (u[1] + u[3]) * sgn0)
                    ni = jnp.where(odd_lane, pltpu.roll((u[3] - u[1]) * sgn0, 1, 1), 0.0)
                    rows = pl.ds(pl.multiple_of(p * 64 + rs * 16, 16), 16)
                    c, sn = tv_ref[0, rows], tv_ref[1, rows]
                    put(ny_ref, 0, rs, nr * c + ni * sn, ni * c - nr * sn)
                    im = jnp.where(lane0, 0.0, im)
                else:
                    re, im = k1 + k2, (k3 - k1) * jnp.where(first, 1.0, -1.0)
                a = _dft4([(re[q * 16:(q + 1) * 16], im[q * 16:(q + 1) * 16]) for q in range(4)])
                for jq in range(4):
                    re, im = a[jq]
                    if jq > 0:
                        c, sn = cs[jq]
                        re, im = re * c + im * sn, im * c - re * sn
                    put(ub_ref, t * 4 + jq, rs, re, im)
        return item

    def p2_bfly(u, g, inverse, ref=ub_ref):
        def item(y):
            if y is not None:
                ub_ref[136, pin_rows(0), :] = y
            v = ref[pl.ds(u * 8, 8), g * 16:(g + 1) * 16]
            x = [(v[p, 0:8], v[p, 8:16]) for p in range(8)]
            x = _swap(_dft8(_swap(x))) if inverse else _dft8(x)
            ref[pl.ds(u * 8, 8), g * 16:(g + 1) * 16] = jnp.stack([w for c in x for w in c]).reshape(8, 16, 128)
        return item

    def filtered(xx, w):
        wr = pltpu.bitcast(w & jnp.uint32(0xFFFF0000), f32).reshape(8, 8, 128)
        wi = pltpu.bitcast(w << 16, f32).reshape(8, 8, 128)
        xx = xx.reshape(8, 2, 8, 128)
        xr, xi = xx[:, 0], xx[:, 1]
        return jnp.stack([xr * wr - xi * wi, xr * wi + xi * wr], axis=1).reshape(128, 128)

    def p2_fwd(u, jps):
        def item(y):
            t = u >> 2
            jq = u & 3
            xs = [_dot(_tobf(ms_ref[jq + 4 * jp]), ub_ref[u * 8 + jp].astype(bf16)) for jp in jps]
            for jp, xx in zip(jps, xs):
                ub_ref[u * 8 + jp] = filtered(xx, wp_ref[pl.ds(t * 2560 + jq + 4 * jp, 64, stride=40), :])
        return item

    def p2_nyq(u):
        def item(y):
            jp = u & 7
            rhs = ny_ref[jp].astype(bf16)
            xx = jnp.concatenate([_dot(_tobf(ms_ref[u * 4, m * 16:(m + 1) * 16]), rhs) for m in range(4)], axis=0)
            w = wp_ref[pl.ds(4 * 2560 + 4 * jp, 64, stride=40), :]
            for jq in range(1, 4):
                w = jnp.where(lane == jq, wp_ref[pl.ds(4 * 2560 + 4 * jp + jq, 64, stride=40), :], w)
            w = jnp.where(u < 8, w, jnp.uint32(0x3F800000))
            ny_ref[jp] = filtered(xx, w)
        return item

    def p2_inv(u, jps):
        def item(y):
            jq = u & 3
            zs = [_dot(_tobf(ms_ref[32 + jq + 4 * jp]), ub_ref[u * 8 + jp].astype(bf16)) for jp in jps]
            for jp, zz in zip(jps, zs):
                ub_ref[u * 8 + jp] = zz
        return item

    def p3_pre(p, g, t):
        def item(y):
            sa_ref[0, pin_rows(0), :] = y
            cs = twiddles(p)

            def fetch(t):
                a = []
                for jq in range(4):
                    v = ub_ref[(t * 4 + jq) * 8 + p, g * 16:(g + 1) * 16]
                    re, im = v[0:8], v[8:16]
                    if jq > 0:
                        c, sn = cs[jq]
                        re, im = re * c - im * sn, im * c + re * sn
                    a.append((re, im))
                return _swap(_dft4(_swap(a)))

            u = fetch(t)
            if t == 0:
                v = ny_ref[p, g * 16:(g + 1) * 16]
                rows = pl.ds(pl.multiple_of(p * 64 + g * 8, 8), 8)
                c, sn = tv_ref[0, rows], tv_ref[1, rows]
                nr, ni = v[0:8] * c - v[8:16] * sn, v[8:16] * c + v[0:8] * sn
                zr, zi = pltpu.roll(nr, 127, 1), pltpu.roll(ni, 127, 1)
                ny = (nr + zr, (nr - zi) * sgn0, nr - zr, (nr + zi) * sgn0)
            first = first_lanes(t)
            for q in range(4):
                re, im = u[q]
                rows = slice(q * 64 + g * 8, q * 64 + (g + 1) * 8)
                if t == 0:
                    im = pltpu.roll(jnp.where(lane0, ny[q], im), 2, 1) + jnp.where(lane == 2, ny[q], 0.0)
                    sa_ref[1:3, rows] = jnp.stack((jnp.where(first, im, re), jnp.where(first, re, im)))
                else:
                    im = im * jnp.where(first, 1.0, -1.0)
                    sa_ref[3 * t:3 * t + 3, rows] = jnp.stack((re + im, im, re))
        return item

    def p3_mm(p, q):
        def item(y):
            g = []
            for t in range(4):
                k1, k2, k3 = d_products(sa_ref, 1, t, slice(q * 64, (q + 1) * 64))
                g.append((k3, k2) if t == 0 else (k2 + k1, k3 - k1))
            yy = _r8_real_t(g)
            bx_ref[q, pl.ds(pl.multiple_of(p * 64, 64), 64), :] = jnp.concatenate(yy, axis=1).astype(bf16)
        return item

    def b_out(p):
        def item(y):
            rows = pl.ds(pl.multiple_of(p * 64, 64), 64)
            pltpu.make_async_copy(bx_ref.at[0:4, rows, :], out_hbm.at[:, rows, pl.ds(DM, DM)],
                                  sem_out.at[1]).start()
            bx_ref[4, pin_rows(0), 0:128] = y.astype(bf16)
        return item

    def a_out(blk, half):
        pltpu.make_async_copy(
            xo_ref.at[half, pl.ds(pl.multiple_of(blk * 64, 64), 64), :],
            out_hbm.at[blk >> 3, pl.ds(pl.multiple_of((blk & 7) * 64, 64), 64),
                       pl.ds(pl.multiple_of(half * 512, 512), 512)],
            sem_out.at[0]).start()

    def step(pp, odd, mem, hooks, fast=False):
        r0 = pl.multiple_of(pp * 64 + 32 * odd, SEG)
        xs = jnp.concatenate([xo_ref[0, pl.ds(r0, SEG), :], xo_ref[1, pl.ds(r0, SEG), :]], axis=1)
        x_lo = xs[0:8].astype(f32)
        hm = jnp.concatenate(
            [jnp.concatenate([x_lo, jnp.concatenate(mem, axis=1)], axis=0).astype(bf16), xs[16:32]], axis=0)
        fill = fillo_ref[:, 0:64] if odd else fille_ref[:, 0:48]
        nrow = 48 if odd else 32
        qkv, ps = {}, {}

        def head_of(v):
            return (v // 16) * 16 + (v % 2) * 8 + (v % 16) // 2 if fast else v

        def do_qkv(v0, v1):
            for v in range(v0, v1):
                h = head_of(v)
                for t in range(3):
                    n = t * H + slot_of(h)
                    y32 = _dot(hm, _tobf(w_refs[n // 16][n % 16, 0:512]))
                    y = y32.astype(bf16)
                    parts = [y]
                    if odd or t > 0:
                        parts.append(_tobf(qkvc_ref[pp, n]))
                    if t > 0:
                        if odd:
                            parts.append(_tobf(kve_ref[(t - 1) * H + h]))
                        else:
                            kve_ref[(t - 1) * H + h] = _tou(y[0:16])
                    qkv[(t, v)] = jnp.concatenate(parts, axis=0) if len(parts) > 1 else y
                for item in hooks.get(v, ()):
                    item(y32[0:8])

        def do_s(g):
            for v in range(g * G, (g + 1) * G):
                sc = jax.lax.dot_general(qkv[(0, v)], qkv[(1, v)], (((1,), (1,)), ((), ())),
                                         preferred_element_type=f32)
                sc = jnp.where(fill == 0.0, sc * scale, fill)
                e = jnp.exp(sc - jnp.max(sc, axis=1, keepdims=True))
                den = jnp.sum(e, axis=1, keepdims=True)
                r = pl.reciprocal(den, approx=True)
                r = r * (2.0 - den * r)
                ps[v] = (e * r).astype(bf16)

        def do_pv(g):
            o = {v: _dot(ps[v], qkv[(2, v)]) for v in range(g * G, (g + 1) * G)}
            for v in o:
                h = head_of(v)
                nr = 32 if fast else nrow
                oall_ref[0:nr // 2, h * DH:(h + 1) * DH] = _tou(o[v][0:nr].astype(bf16))
            if fast:
                for v in range(g * G, (g + 1) * G, 2):
                    a11, a12 = o[v][0:32], o[v + 1][0:32]
                    a21 = jnp.concatenate([oc_ref[head_of(v)], o[v][32:48]], axis=0)
                    a22 = jnp.concatenate([oc_ref[head_of(v + 1)], o[v + 1][32:48]], axis=0)
                    for k, a in enumerate((a11 + a22, a21 + a22, a22, a11 + a12, a21 - a11, a12 - a22)):
                        os_ref[k, :, (v // 2) * DH:(v // 2 + 1) * DH] = a
            if odd:
                for v in o:
                    oc_ref[head_of(v)] = o[v][32:48]

        def plain(half, j, rows, h0, h1):
            return _dot(_tobf(oall_ref[0:rows // 2, h0 * DH:h1 * DH]), _tobf(wo_ref[half, j, h0 * 64:h1 * 64, :]))

        hb = pp & 1
        if fast:
            def product(jp, k):
                def fn(part):
                    h0 = part * 16
                    if k == 2:
                        lhs = _tobf(oall_ref[0:16, h0 * DH:(h0 + 8) * DH])
                    else:
                        lhs = os_ref[k - (k > 2), :, part * 1024:(part + 1) * 1024].astype(bf16)
                    if k == 1:
                        rhs = wo_ref[hb, jp * 2, h0 * 64:(h0 + 8) * 64, :]
                    elif k == 4:
                        rhs = wo_ref[hb, jp * 2 + 1, (h0 + 8) * 64:(h0 + 16) * 64, :]
                    else:
                        rhs = ws_ref[hb, jp * 5 + (0, 0, 1, 2, 0, 3, 4)[k], part * 512:(part + 1) * 512, :]
                    return _dot(lhs, _tobf(rhs))
                return fn
            jobs = [product(jp, k) for jp in range(2) for k in range(7)]
            jobs += [(lambda part, j=j: plain(1 - hb, j, 32, part * 16, part * 16 + 16)) for j in range(4)]
            marks = (2, 10)
        else:
            jobs = [(lambda part, j=j: plain(j // 4, j % 4, nrow, part * 24, 24 + part * 8)) for j in range(8)]
            marks = (2, 5)

        for g in range(NG):
            do_qkv(g * G, g * G + G // 2)
            if g >= 1:
                do_s(g - 1)
            do_qkv(g * G + G // 2, (g + 1) * G)
            if g >= 2:
                do_pv(g - 2)
        part = []
        for k, job in enumerate(jobs):
            items = hooks.get(('o', k), ())
            if len(items) == 2:
                half = plain(k // 4, k % 4, nrow, 0, 12)
                items[0](half[0:8])
                part.append(plain(k // 4, k % 4, nrow, 12, 24) + half)
                items[1](part[k][0:8])
            else:
                part.append(job(0))
                for item in items:
                    item(part[k][0:8])
            if k == marks[0]:
                do_s(NG - 1)
                do_pv(NG - 2)
            if k == marks[1]:
                do_pv(NG - 1)

        def finish(k):
            res = jobs[k](1) + part[k]
            for item in hooks.get(('p', k), ()):
                item(res[0:8])
            return res

        def put(half, j, r, v):
            xo_ref[half, pl.ds(r0 + r, v.shape[0]), j * 128:(j + 1) * 128] = v.astype(bf16)

        if fast:
            own = []
            for jp in range(2):
                m1, m2, m3, m4, m5, m6, m7 = [finish(jp * 7 + k) for k in range(7)]
                for jj, top, bot in ((0, ((m1 + m4) - m5) + m7, m2 + m4), (1, m3 + m5, ((m1 - m2) + m3) + m6)):
                    j = jp * 2 + jj
                    own.append(top[8:16])
                    put(hb, j, 0, jnp.concatenate([top[0:8], bot[24:32], top[16:32]], axis=0))
                    put(hb, j, -24, bot[16:24])
                    put(hb, j, -56, bot[8:16])
                    put(hb, j, -88, bot[0:8])
            for j in range(4):
                res = finish(14 + j)
                own.append(res[8:16])
                put(1 - hb, j, 0, res)
            new_mem = [jnp.where(hb == 0, own[j], own[(j + 4) % 8]) for j in range(8)]
        else:
            new_mem = []
            for j in range(8):
                res = finish(j)
                new_mem.append(res[8:16])
                if odd:
                    put(j // 4, j % 4, 0, jnp.concatenate([res[0:8], res[40:48], res[16:32]], axis=0))
                    put(j // 4, j % 4, -24, res[32:40])
                else:
                    put(j // 4, j % 4, 0, res)
        for item in hooks.get(H, ()):
            item(None)
        if odd:
            a_out(pp, hb)
            if fast:
                a_out(pp - 1, hb)
            else:
                pl.when(pp > 0)(lambda: a_out(pp - 1, hb))
        return new_mem

    def wsum_item(i, k):
        def item(y):
            ws_ref[pin_slot(4) >> 2, 9, 1024:1032] = pltpu.bitcast(y, u32)
            jp = k & 1
            r = (i & 1) * 256 + (k >> 1) * 16
            b11, b21, b12, b22 = [
                _tobf(wo_ref[i >> 2, jp * 2 + jj, pl.ds(pl.multiple_of((i & 2) * 512 + r + kh * 512, 16), 16), :]
                      ).astype(f32) for jj in range(2) for kh in range(2)]
            rows = pl.ds(pl.multiple_of((i & 2) * 256 + r, 16), 16)
            for n, v in enumerate((b11 + b22, b12 - b22, b21 - b11, b11 + b12, b21 + b22)):
                ws_ref[i >> 2, jp * 5 + n, rows, :] = _tou(v.astype(bf16))
        return item

    def l1(i, mem):
        bx_copy(i).wait()
        he = {2 * k: [p1_pre(i, k // 4, k % 4)] for k in range(16)}
        he[H] = [p1_mm(i, 1)]
        ho = {('o', 0): [p1_mm(i, 2)], ('o', 3): [p1_mm(i, 3)], ('o', 5): [p1_mm(i, 0)]}
        ho.update({k: [wsum_item(i, k)] for k in range(32)})
        mem = step(i, 0, mem, he)
        mem = step(i, 1, mem, ho)
        return mem

    def l2(i, mem):
        u = i - N_L1
        he = {3: [p2_fwd(u, range(0, 4))], 7: [p2_fwd(u, range(4, 8))], 17: [p2_nyq(u)],
              H: [p2_inv(u, range(0, 8))]}
        ho = {('p', k): [p2_bfly(u + k % 2, k // 2, k % 2 == 0)] for k in range(16)}
        mem = step(i, 0, mem, he)
        mem = step(i, 1, mem, ho, fast=True)
        return mem

    def l3(i, mem):
        p = i - N_L1 - N_L2
        he = {h: [p3_pre(p, h // 3, 1 + h % 3)] for h in range(24)}
        for j in range(4):
            he[('o', 3 + j)] = [p3_pre(p, 2 * j, 0), p3_pre(p, 2 * j + 1, 0)]
        he[H] = [p3_mm(p, q) for q in range(4)]
        ho = {12: [b_out(p)]}
        mem = step(i, 0, mem, he)
        mem = step(i, 1, mem, ho, fast=True)
        return mem

    m0 = mem_ref[...].astype(f32)
    mem = [m0[:, j * 128:(j + 1) * 128] for j in range(8)]
    mem = jax.lax.fori_loop(0, N_L1, l1, mem)
    cp_x[2].wait()
    cp_x[3].wait()
    cp_ms.wait()
    for g in range(8):
        p2_bfly(0, g, False)(None)
        p2_bfly(0, g, False, ny_ref)(None)
    mem = jax.lax.fori_loop(N_L1, N_L1 + N_L2, l2, mem)
    for g in range(8):
        p2_bfly(0, g, True, ny_ref)(None)
    mem = jax.lax.fori_loop(N_L1 + N_L2, NSEG // 2, l3, mem)

    oc_last = jnp.concatenate([oc_ref[h] for h in range(H)], axis=1).astype(bf16)
    for j in range(4):
        res = _dot(oc_last, _tobf(wo_ref[0, j, 0:2048, :])).astype(bf16)
        xo_ref[0, S - 56:S - 48, j * 128:(j + 1) * 128] = res[0:8]
        xo_ref[0, S - 24:S - 16, j * 128:(j + 1) * 128] = res[8:16]
    a_out(NSEG // 2 - 1, 0)

    pltpu.make_async_copy(bx_ref.at[0:4], out_hbm.at[:, :, pl.ds(DM, DM)], sem_out.at[1]).wait()
    pltpu.make_async_copy(xo_ref, xo_ref, sem_out.at[0]).wait()


@jax.jit
def _run(x, mem0, wq, wk, wv, wo, bx, w_r, w_i):
    fd, ms, tv = _tables()
    hbm = pl.BlockSpec(memory_space=pl.ANY)
    out = pl.pallas_call(
        _kernel,
        out_shape=jax.ShapeDtypeStruct((4, S // 4, 2 * DM), bf16),
        in_specs=[hbm] * 13,
        out_specs=hbm,
        scratch_shapes=[
            pltpu.VMEM((2, S, DM // 2), bf16),
            pltpu.VMEM((MEM, DM), bf16),
            pltpu.VMEM((8, NSEG, 8, 128), bf16),
            pltpu.VMEM((4, DM, 16, DH), bf16),
        ] + [pltpu.VMEM((16, DM // 2 + 8, DH), u32)] * 6 + [
            pltpu.VMEM((2, 4, H * DH // 2 + 8, 128), u32),
            pltpu.VMEM((8, 256, 128), u32),
            pltpu.VMEM((5, 4, 136, 128), u32),
            pltpu.VMEM((NSEG // 2, 3 * H, 8, 128), u32),
            pltpu.VMEM((2 * H, 8, 128), u32),
            pltpu.VMEM((24, H * DH), u32),
            pltpu.VMEM((H, 16, DH), f32),
            pltpu.VMEM((6, 32, 16 * DH), f32),
            pltpu.VMEM((2, 10, 1040, 128), u32),
            pltpu.VMEM((32, 128), f32),
            pltpu.VMEM((48, 128), f32),
            pltpu.VMEM((5, S // 4, DM), bf16),
            pltpu.VMEM((16, DM // 2 + 1, 256), bf16),
            pltpu.VMEM((12872, 128), u32),
            pltpu.VMEM((137, 128, 128), f32),
            pltpu.VMEM((8, 128, 128), f32),
            pltpu.VMEM((12, 264, 128), f32),
            pltpu.VMEM((24, 64, 128), u32),
            pltpu.VMEM((64, 64, 128), u32),
            pltpu.VMEM((2, 512, 128), f32),
            pltpu.SMEM((64,), f32),
            pltpu.SMEM((1,), jnp.int32),
            pltpu.SemaphoreType.DMA((84,)),
            pltpu.SemaphoreType.DMA((2,)),
        ],
        compiler_params=pltpu.CompilerParams(vmem_limit_bytes=120 * 1024 * 1024,
                                             disable_semaphore_checks=True,
                                             disable_bounds_checks=True),
    )(x.reshape(S, DM), x.reshape(NSEG, SEG, DM), mem0.reshape(MEM, DM), wq, wk, wv,
      wo.reshape(H * DH // 16, 16, DM), bx.reshape(4, S // 4, DM), w_r.T, w_i.T, jnp.asarray(fd), jnp.asarray(ms), jnp.asarray(tv))
    return out.reshape(1, S, 2 * DM)


def pallas_concat_heads__memory_aug_recurrent_mem_tr__spectral_gfnet__prompt_kernel(
    A_x: jax.Array,
    A_mem0: jax.Array,
    A_Wq: jax.Array,
    A_Wk: jax.Array,
    A_Wv: jax.Array,
    A_Wo: jax.Array,
    A_seg_len,
    B_x: jax.Array,
    B_w_r: jax.Array,
    B_w_i: jax.Array,
):
    if isinstance(A_seg_len, int):
        assert A_seg_len == SEG
    assert A_x.shape == (1, S, DM) and A_mem0.shape == (1, MEM, DM) and A_Wq.shape == (DM, H, DH)
    assert B_x.shape == (1, S, DM) and B_w_r.shape == (S, DM // 2 + 1)
    return _run(A_x, A_mem0, A_Wq, A_Wk, A_Wv, A_Wo, B_x, B_w_r, B_w_i)
```

```python
import math

import numpy as np
import jax
import jax.numpy as jnp
import jax.experimental.pallas as pl
import jax.experimental.pallas.tpu as pltpu

bf16 = jnp.bfloat16
f32 = jnp.float32
u32 = jnp.uint32

S, DM = 2048, 1024
H, DH = 32, 128
MEM, SEG = 8, 32
NSEG = S // SEG
SQH = math.sqrt(0.5)

_PAIRS = ((0, 4), (1, 7), (2, 6), (3, 5))
_FIRST = np.array([[1, 1, 0, 0], [1, 0, 1, 0], [0, 1, 1, 0], [0, 1, 0, 1]], bool)


def _pack_rows(a):
    u = np.ascontiguousarray(a, dtype=np.float32).view(np.uint32).astype(np.uint64)
    b = ((u + 0x7FFF + ((u >> 16) & 1)) >> 16).astype(np.uint32)
    return (b[..., 0::2, :] | (b[..., 1::2, :] << 16)).astype(np.uint32)


def _tables():
    k2 = np.zeros((4, 128), np.int64)
    for t in range(4):
        odd = t % 2
        for lam in range(128):
            k = 2 * lam + odd
            if k % 8 not in _PAIRS[t]:
                k = 2 * (128 + 8 * (lam // 8) + (lam % 8 - 1 - odd) % 8) + odd
            assert k % 8 in _PAIRS[t]
            k2[t, lam] = k
    b = np.arange(128)[:, None]
    F = np.zeros((12, 128, 128))
    G = np.zeros((12, 128, 128))
    for t in range(4):
        th = 2 * np.pi * ((b * k2[t][None, :]) % DM) / DM
        C, Sn = np.cos(th), np.sin(th)
        first = ((k2[t] % 8) == _PAIRS[t][0])[None, :]
        assert np.array_equal(first[0], _FIRST[t][np.arange(128) % 4])
        if t == 0:
            im = -Sn
            im[:, 0] = (-1.0) ** np.arange(128)
            im = np.roll(im, 2, axis=1)
            F[1:3] = np.where(first, im, C), np.where(first, C, im)
            G[1:3] = F[1:3]
            G[2, :, 0] *= 0.5
            G[2, :, 2] *= 0.5
        else:
            Sg = np.where(first, Sn, -Sn)
            F[3 * t:3 * t + 3] = C, -(C + Sg), C - Sg
            G[3 * t:3 * t + 3] = F[3 * t:3 * t + 3]
    Finv = np.transpose(G, (0, 2, 1)) * (2.0 / DM)
    fd = _pack_rows(np.concatenate([F, Finv]))
    M = np.zeros((32, 128, 128))
    r = np.arange(64)[None, :]
    l = np.arange(64)[:, None]
    for j in range(32):
        th = 2 * np.pi * ((r * (j + 32 * l)) % S) / S
        C, Sn = np.cos(th), np.sin(th)
        M[j, :64, :64] = C
        M[j, :64, 64:] = Sn
        M[j, 64:, :64] = -Sn
        M[j, 64:, 64:] = C
    perm = np.arange(128).reshape(2, 8, 8).transpose(1, 0, 2).reshape(128)
    M = M[:, perm][:, :, perm]
    Minv = np.transpose(M, (0, 2, 1)) / S
    ms = _pack_rows(np.concatenate([M, Minv]))
    th = 2 * np.pi * np.outer(np.arange(512), np.arange(128) % 4) / S
    tv = np.stack([np.cos(th), np.sin(th)]).astype(np.float32)
    return fd, ms, tv


def _tobf(w):
    return pltpu.bitcast(w, bf16)


def _tou(w):
    return pltpu.bitcast(w, u32)


def _dot(a, b):
    return jnp.dot(a, b, preferred_element_type=f32)


def _r8_real(x):
    t0, t1 = x[0] + x[4], x[0] - x[4]
    t2, t3 = x[2] + x[6], x[2] - x[6]
    t4, t5 = x[1] + x[5], x[1] - x[5]
    t6, t7 = x[3] + x[7], x[3] - x[7]
    e0, e1 = t0 + t2, t0 - t2
    o0, o1 = t4 + t6, t4 - t6
    u, v = SQH * (t5 - t7), SQH * (t5 + t7)
    return [(e0 + o0, e0 - o0), (t1 + u, v + t3), (e1, o1), (t1 - u, v - t3)]


def _r8_real_t(g):
    (z0, z4), (a1, b1), (e1, o1), (a3, b3) = g
    e0, o0 = z0 + z4, z0 - z4
    t1, u = a1 + a3, a1 - a3
    v, t3 = b1 + b3, b1 - b3
    t5, t7 = SQH * (v + u), SQH * (v - u)
    t0, t2 = e0 + e1, e0 - e1
    t4, t6 = o0 + o1, o0 - o1
    return [t0 + t1, t4 + t5, t2 + t3, t6 + t7, t0 - t1, t4 - t5, t2 - t3, t6 - t7]


def _dft4(u):
    (r0, i0), (r1, i1), (r2, i2), (r3, i3) = u
    sr, si, dr, di = r0 + r2, i0 + i2, r0 - r2, i0 - i2
    tr, ti, er, ei = r1 + r3, i1 + i3, r1 - r3, i1 - i3
    return [(sr + tr, si + ti), (dr + ei, di - er), (sr - tr, si - ti), (dr - ei, di + er)]


def _dft8(x):
    a = [(x[p][0] + x[p + 4][0], x[p][1] + x[p + 4][1]) for p in range(4)]
    d = [(x[p][0] - x[p + 4][0], x[p][1] - x[p + 4][1]) for p in range(4)]
    ev = _dft4(a)
    (r0, i0), (r1, i1), (r2, i2), (r3, i3) = d
    b1r, b1i = SQH * (r1 + i1), SQH * (i1 - r1)
    b3r, n3i = SQH * (i3 - r3), SQH * (r3 + i3)
    sr, si, dr, di = r0 + i2, i0 - r2, r0 - i2, i0 + r2
    tr, ti, er, ei = b1r + b3r, b1i - n3i, b1r - b3r, b1i + n3i
    od = [(sr + tr, si + ti), (dr + ei, di - er), (sr - tr, si - ti), (dr - ei, di + er)]
    return [ev[0], od[0], ev[1], od[1], ev[2], od[2], ev[3], od[3]]


def _swap(x):
    return [(b, a) for (a, b) in x]


G = 4
NG = H // G
NEG = -1e9
N_L1, N_L2, N_L3 = 8, 16, 8


def _kernel(x_hbm, x3_hbm, mem_hbm, wq_hbm, wk_hbm, wv_hbm, wo_hbm, bx_hbm, wr_hbm, wi_hbm,
            fd_hbm, ms_hbm, tv_hbm, out_hbm,
            xo_ref, mem_ref, xcraw_ref, raw_ref, w0_ref, w1_ref, w2_ref, w3_ref, w4_ref, w5_ref,
            wo_ref, xc_ref, xs_ref, qkvc_ref, kve_ref,
            oall_ref, oc_ref, os_ref, ws_ref, fille_ref, fillo_ref, bx_ref, wt_ref, wp_ref, ub_ref, ny_ref, sa_ref, fd_ref, ms_ref, tv_ref,
            tw_ref, zero_ref, sem_in, sem_out):
    scale = DH ** -0.5
    w_hbm = (wq_hbm, wk_hbm, wv_hbm)
    w_refs = (w0_ref, w1_ref, w2_ref, w3_ref, w4_ref, w5_ref)

    def raw_copy(c, i=0, nd=DM):
        rows = pl.ds(pl.multiple_of(i * nd, nd), nd)
        return pltpu.make_async_copy(
            w_hbm[c // 2].at[rows, pl.ds((c % 2) * 16, 16), :],
            raw_ref.at[c % 4, rows], sem_in.at[8 + min(c, 3) * 8 + max(c - 3, 0) * 2 + i])

    def xc_copy(k):
        return pltpu.make_async_copy(
            x3_hbm.at[:, pl.ds(8, 8), pl.ds(pl.multiple_of(k * 128, 128), 128)], xcraw_ref.at[k], sem_in.at[40 + k])

    def wo_copies(half):
        return [pltpu.make_async_copy(wo_hbm.at[:, :, pl.ds(pl.multiple_of(half * 512 + j * 128, 128), 128)],
                                      raw_ref.at[2 + half, j * 256:(j + 1) * 256], sem_in.at[76 + half * 4 + j])
                for j in range(4)]

    def wt_copies(i):
        return [pltpu.make_async_copy(src.at[:, pl.ds(pl.multiple_of(i * 1024 + k * 256, 256), 256)],
                                      wt_ref.at[i * 4 + (a * 8 + k)], sem_in.at[i * 4 + (48 + a * 8 + k)])
                for k in range(4) for a, src in enumerate((wr_hbm, wi_hbm))]

    def bx_copy(p):
        rows = pl.ds(pl.multiple_of(p * 64, 64), 64)
        return pltpu.make_async_copy(bx_hbm.at[:, rows, :], bx_ref.at[0:4, rows, :], sem_in.at[64 + p])

    n_head = N_L1 * 2 * SEG
    cp_x = [pltpu.make_async_copy(x_hbm.at[lo:hi, half * 512:(half + 1) * 512], xo_ref.at[half, 64 + lo:64 + hi],
                                  sem_in.at[72 + (lo > 0) * 2 + half])
            for lo, hi in ((0, n_head), (n_head, S)) for half in range(2)]
    cp_mem = pltpu.make_async_copy(mem_hbm, mem_ref, sem_in.at[1])
    cp_fd = pltpu.make_async_copy(fd_hbm, fd_ref, sem_in.at[4])
    cp_ms = pltpu.make_async_copy(ms_hbm, ms_ref, sem_in.at[5])
    cp_tv = pltpu.make_async_copy(tv_hbm, tv_ref, sem_in.at[6])

    for i in range(8):
        raw_copy(0, i, 128).start()
        if i < 4:
            xc_copy(i).start()
        if 3 <= i < 7:
            xc_copy(i + 1).start()
        if i >= 3:
            raw_copy(2, i - 3, 128).start()
        if i == 7:
            raw_copy(2, 5, 128).start()
        raw_copy(1, i, 128).start()
    for i in range(6, 8):
        raw_copy(2, i, 128).start()
    for i in range(2):
        raw_copy(3, i, 512).start()
    for cp in cp_x[0:2] + [cp_mem, cp_fd, cp_tv] + [bx_copy(p) for p in range(8)] + cp_x[2:4] + [cp_ms]:
        cp.start(priority=1)

    zero_ref[0] = 0

    def pin_slot(n):
        return n - jnp.clip(zero_ref[0], 0, 1) * 4

    def pin_rows(r):
        return pl.ds(pl.multiple_of(r + jnp.clip(zero_ref[0], 0, 1) * 32, 8), 8)

    for p in range(8):
        for jq in range(4):
            tw_ref[(p * 4 + jq) * 2] = jnp.float32(math.cos(2 * math.pi * p * jq / 32))
            tw_ref[(p * 4 + jq) * 2 + 1] = jnp.float32(math.sin(2 * math.pi * p * jq / 32))

    ub_ref[128:136] = jnp.zeros((8, 128, 128), f32)
    wp_ref[12800:12872] = jnp.zeros((72, 128), u32)
    oc_ref[...] = jnp.zeros((H, 16, DH), f32)

    qi = jax.lax.broadcasted_iota(jnp.int32, (48, 128), 0)
    ki = jax.lax.broadcasted_iota(jnp.int32, (48, 128), 1)

    def between(v, lo, hi):
        return (v >= lo) & (v < hi)

    def table(keep, other):
        return jnp.where(other, -jnp.inf, jnp.where(keep, 0.0, NEG)).astype(f32)

    keep = between(qi, 8, 16) | between(ki, 8, 16) | (qi >= jnp.where(ki < 32, ki, ki - 24))
    fille_ref[...] = table(keep, ki >= 40)[:32]
    q_even = between(qi, 32, 40)
    k_even = between(ki, 32, 40) | (ki >= 48)
    qpos = jnp.where(qi < 32, qi, jnp.where(qi < 40, qi - 24, qi - 32))
    kpos = jnp.where(ki < 32, ki, jnp.where(ki < 40, ki - 24, jnp.where(ki < 48, ki - 32, ki - 48)))
    keep = between(qi, 8, 16) | between(ki, 8, 16) | (ki >= 56) | (qpos >= kpos)
    fillo_ref[...] = table(keep, (q_even != k_even) | (ki >= 64))

    def relayout16(c, blk):
        w0 = pl.multiple_of(blk * 8, 8)
        v = _tou(raw_ref[c % 4, pl.ds(blk * 16, 16)]).reshape(8, 2, 8, 128)
        a, b = v[:, 0], v[:, 1]
        w_refs[c][0:8, pl.ds(w0, 8), :] = jnp.swapaxes((a & jnp.uint32(0xFFFF)) | (b << 16), 0, 1)
        w_refs[c][8:16, pl.ds(w0, 8), :] = jnp.swapaxes((a >> 16) | (b & jnp.uint32(0xFFFF0000)), 0, 1)

    def slot_of(h):
        return (h // 16) * 16 + (h % 2) * 8 + (h % 16) // 2

    def repack_wo(half, part, k):
        jp, g0 = k & 1, part * 128 + (k >> 1) * 2
        quad = []
        for jj in range(2):
            for kh in range(2):
                v = _tou(raw_ref[2 + half, pl.ds((jp * 2 + jj) * 256 + kh * 64 + g0, 2)]).reshape(16, 128)
                wo_ref[half, jp * 2 + jj, pl.ds(pl.multiple_of(g0 * 8 + kh * 512, 16), 16), :] = v
                quad.append(_tobf(v).astype(f32))
        b11, b21, b12, b22 = quad
        rows = pl.ds(pl.multiple_of(part * 512 + (k >> 1) * 16, 16), 16)
        for n, v in enumerate((b11 + b22, b12 - b22, b21 - b11, b11 + b12, b21 + b22)):
            ws_ref[half, jp * 5 + n, rows, :] = _tou(v.astype(bf16))

    sub4 = jax.lax.broadcasted_iota(jnp.int32, (128, 128), 0) & 3

    def wp_store(t, kb, tile):
        v = tile.T.reshape(4, 32, 128)
        v = jnp.concatenate([v, v[:, 0:8]], axis=1).reshape(160, 128)
        wp_ref[pl.ds(pl.multiple_of(t * 2560 + kb * 160, 32), 160), :] = v

    def b_prep(lg, hb, par):
        cols = slice(hb * 128, (hb + 1) * 128)
        a = _tou(wt_ref[lg, 0:512, cols])
        b = _tou(wt_ref[8 + lg, 0:512, cols])
        if par == 0:
            w = (a << 16) | (b & jnp.uint32(0xFFFF))
            m = (sub4 == 0) | (sub4 == 2)
        else:
            w = (a & jnp.uint32(0xFFFF0000)) | (b >> 16)
            m = (sub4 == 0) | (sub4 == 3)
        top = w[:128]
        bot = pltpu.roll(w[128:].reshape(16, 8, 128), 1 + par, 1).reshape(128, 128)
        wp_store(par, lg * 2 + hb, jnp.where(m, top, bot))
        wp_store(par + 2, lg * 2 + hb, jnp.where(m, bot, top))
        if par == 0:
            na = jnp.broadcast_to(wt_ref[lg, 512:513, cols].astype(f32), (128, 128))
            nb = jnp.broadcast_to(wt_ref[8 + lg, 512:513, cols].astype(f32), (128, 128))
            wp_store(4, lg * 2 + hb, pltpu.bitcast(na, u32) | (pltpu.bitcast(nb, u32) >> 16))

    def gather_c(k):
        xc_ref[k] = _tou(xcraw_ref[k].astype(f32).reshape(512, 128).astype(bf16))

    def store_qkvc(n, y):
        qkvc_ref[:, n] = y.reshape(NSEG // 2, 8, 128)

    def q_unit(i, groups, first, last, fillers):
        xk = _tobf(xc_ref[i])
        w0 = pl.multiple_of(i * 64, 64)
        for g in groups:
            rhs = jnp.concatenate(
                [_tobf(w_refs[h // 16][h % 16, pl.ds(w0, 64), :]) for h in range(4 * g, 4 * g + 4)], axis=1)
            y = _dot(xk, rhs)
            for h in range(4 * g, 4 * g + 4):
                yh = y[:, (h % 4) * 128:(h % 4 + 1) * 128]
                if not first:
                    yh = yh + ub_ref[h * 4:(h + 1) * 4].reshape(512, 128)
                if last:
                    store_qkvc(h, _tou(yh.astype(bf16)))
                else:
                    ub_ref[h * 4:(h + 1) * 4] = yh.reshape(4, 128, 128)
            mine = fillers.get(g, [])
            for fi, item in enumerate(mine):
                r = (fi * 512 // len(mine)) // 8 * 8
                item(pltpu.bitcast(y[r:r + 8, 0:128], u32))

    def rl_item(c, blk):
        def item(pin):
            w_refs[c][pin_slot(15), 512:520] = pin
            relayout16(c, blk)
        return item

    def spread(fillers, items, groups):
        for k, item in enumerate(items):
            fillers.setdefault(groups[k * len(groups) // len(items)], []).append(item)
        return fillers

    def half_items(f, c, i, groups):
        return spread(f, [rl_item(c, i * 8 + blk) for blk in range(8)], groups)

    def piece_items(i):
        f = half_items(half_items({}, 1, i, (0, 1, 2)), 0, i + 1, (4, 5, 6))
        return spread(f, [lambda pin: gather_c(i + 1)], (7,))

    def chunk2_items(f, lo, hi, groups):
        return spread(f, [rl_item(2, blk) for blk in range(lo, hi)], groups)

    def wait_piece(i):
        raw_copy(1, i, 128).wait()
        raw_copy(0, i + 1, 128).wait()

    raw_copy(0, 0, 128).wait()
    for blk in range(8):
        relayout16(0, blk)
    xc_copy(0).wait()
    gather_c(0)
    q_unit(0, range(0, 2), True, False, {})
    raw_copy(1, 0, 128).wait()
    q_unit(0, range(2, 4), True, False, half_items({}, 1, 0, (2, 2, 3)))
    q_unit(0, range(4, 6), True, False, {})
    xc_copy(1).wait()
    raw_copy(0, 1, 128).wait()
    q_unit(0, range(6, 8), True, False,
           spread(half_items({}, 0, 1, (6, 6, 7)), [lambda pin: gather_c(1)], (6,)))
    raw_copy(1, 1, 128).wait()
    q_unit(1, range(0, 4), False, False, half_items({}, 1, 1, (0, 1, 2)))
    xc_copy(2).wait()
    raw_copy(0, 2, 128).wait()
    q_unit(1, range(4, 8), False, False,
           spread(half_items({}, 0, 2, (4, 5, 6)), [lambda pin: gather_c(2)], (6,)))

    def xsum_item(j, rq):
        def item(pin):
            xs_ref[pin_slot(4), 0, 128:136] = pin
            a11, a21, a12, a22 = [
                xcraw_ref[j + 4 * kh, rh * 32 + rq * 8:rh * 32 + (rq + 1) * 8].astype(f32).reshape(64, 128)
                for kh in range(2) for rh in range(2)]
            for k, v in enumerate((a11 + a22, a21 + a22, a11 + a12, a21 - a11, a12 - a22)):
                xs_ref[k, j, rq * 32:(rq + 1) * 32] = _tou(v.astype(bf16))
        return item

    def q_c(i, carry):
        wait_piece(i)
        xc_copy(i + 2).wait()
        raw_copy(2, i - 2, 128).wait()
        f = half_items(piece_items(i), 2, i - 2, (3, 3, 3, 3, 4, 5, 6, 7))
        q_unit(i, range(8), False, False, spread(f, [xsum_item(i - 2, rq) for rq in range(4)], (3, 4, 5, 6)))
        return carry
    xc_copy(3).wait()
    jax.lax.fori_loop(2, 6, q_c, 0)

    wait_piece(6)
    raw_copy(2, 4, 128).wait()
    raw_copy(2, 5, 128).wait()
    q_unit(6, range(8), False, False, chunk2_items(piece_items(6), 32, 48, (0, 1, 2, 3, 3, 4, 5, 6)))
    raw_copy(1, 7, 128).wait()
    raw_copy(2, 6, 128).wait()
    raw_copy(2, 7, 128).wait()
    q_unit(7, range(8), False, True, chunk2_items(half_items({}, 1, 7, (0, 1, 2)), 48, 64, (3, 4, 5, 6)))
    raw_copy(4).start()
    for cp in wo_copies(0):
        cp.start()
    raw_copy(5).start()

    def bulk_iter(c, i):
        def xs(k):
            return jnp.concatenate([_tobf(xs_ref[k, j, 0:128]) for j in range(4)], axis=1)

        def xc(rh, kh):
            return jnp.concatenate(
                [_tobf(xc_ref[4 * kh + j, rh * 128:(rh + 1) * 128]) for j in range(4)], axis=1)

        for pr in range(4):
            n1 = i * 8 + pr * 2
            n2 = n1 + 1

            def w(n, kh):
                return _tobf(w_refs[c][n, kh * 256:(kh + 1) * 256])

            def wsum(a, b, sign):
                a, b = a.astype(f32), b.astype(f32)
                return (a + b if sign > 0 else a - b).astype(bf16)

            def out(rh, n, v):
                qkvc_ref[rh * 16:(rh + 1) * 16, c * 16 + n] = _tou(v.astype(bf16)).reshape(16, 8, 128)

            def side(k, m):
                blks = (k, 7) if k == 0 else (k,)
                items = []
                if c < 5:
                    items += [('w', blk) for blk in blks]
                if c >= 4:
                    items += [('o', blk) for blk in range(k * 16 // 7, (k + 1) * 16 // 7)]
                if c == 5 and k in (1, 2, 4, 5):
                    items.append(('f', (1, 2, 4, 5).index(k)))
                for n, (kind, blk) in enumerate(items):
                    r = n * 256 // len(items) // 8 * 8
                    pin = pltpu.bitcast(m[r:r + 8], u32)
                    if kind == 'w':
                        w_refs[c + 1][pin_slot(15), 512:520] = pin
                        relayout16(c + 1, i * 32 + (pr * 8 + blk))
                    elif kind == 'o':
                        ws_ref[pin_slot(4) >> 2, 9, 1024:1032] = pin
                        wo_ref[pin_slot(4) >> 2, 3, 2048:2056] = pin
                        repack_wo(c - 4, i, pr * 16 + blk)
                    else:
                        wp_ref[pin_rows(12832), :] = pin
                        b_prep(i * 4 + pr, blk // 2, blk % 2)

            m2 = _dot(xs(1), w(n1, 0))
            side(0, m2)
            m4 = _dot(xc(1, 1), wsum(w(n1, 1), w(n1, 0), -1))
            side(1, m4)
            out(1, n1, m4 + m2)
            m1 = _dot(xs(0), wsum(w(n1, 0), w(n2, 1), 1))
            side(2, m1)
            m5 = _dot(xs(2), w(n2, 1))
            side(3, m5)
            m3 = _dot(xc(0, 0), wsum(w(n2, 0), w(n2, 1), -1))
            side(4, m3)
            out(0, n2, m3 + m5)
            c22 = _dot(xs(3), wsum(w(n1, 0), w(n2, 0), 1)) + ((m1 - m2) + m3)
            side(5, c22)
            out(1, n2, c22)
            c11 = _dot(xs(4), wsum(w(n1, 1), w(n2, 1), 1)) + ((m1 + m4) - m5)
            side(6, c11)
            out(0, n1, c11)

    for c in range(2, 6):
        if c == 3:
            for cp in wo_copies(1) + wt_copies(0) + wt_copies(1):
                cp.start()
        if c >= 4:
            for cp in wo_copies(c - 4):
                cp.wait()
        if 2 < c < 5:
            raw_copy(c + 1).wait()

        def bulk(i, carry, c=c):
            if c == 2:
                raw_copy(3, i, 512).wait()
            if c == 5:
                for cp in wt_copies(i):
                    cp.wait()
            bulk_iter(c, i)
            return carry
        jax.lax.fori_loop(0, 2, bulk, 0)

    cp_x[0].wait()
    cp_x[1].wait()
    cp_mem.wait()
    cp_fd.wait()
    cp_tv.wait()

    lane = jax.lax.broadcasted_iota(jnp.int32, (1, 128), 1)
    lane0 = lane == 0
    sgn0 = jnp.where(lane0, 1.0, -1.0)

    def first_lanes(t):
        la, lb = [k for k in range(4) if _FIRST[t][k]]
        return ((lane & 3) == la) | ((lane & 3) == lb)

    def d_products(st_ref, d, t, rows):
        return [_dot(st_ref[n, rows].astype(bf16), _tobf(fd_ref[d * 12 + n])) if n else None
                for n in range(3 * t, 3 * t + 3)]

    def twiddles(p):
        return [(tw_ref[p * 8 + jq * 2], tw_ref[p * 8 + jq * 2 + 1]) if jq else None for jq in range(4)]

    def p1_pre(p, rs, q):
        def item(y):
            sa_ref[0, pin_rows(0), :] = y
            xq = bx_ref[q, pl.ds(pl.multiple_of(p * 64 + rs * 16, 16), 16), :].astype(f32)
            zz = _r8_real([xq[:, a * 128:(a + 1) * 128] for a in range(8)])
            r = (rs * 4 + q) * 16
            sa_ref[1:12, r:r + 16] = jnp.stack([v for (a, b) in zz for v in (a + b, b, a)][1:])
        return item

    def p1_mm(p, t):
        def item(y):
            cs = twiddles(p)

            def put(ref, n, rs, re, im):
                v = jnp.stack([re.reshape(2, 8, 128), im.reshape(2, 8, 128)], axis=1)
                ref[n * 8 + p, rs * 32:(rs + 1) * 32] = v.reshape(32, 128)

            first = first_lanes(t)
            for rs in range(4):
                k1, k2, k3 = d_products(sa_ref, 0, t, slice(rs * 64, (rs + 1) * 64))
                if t == 0:
                    up = jnp.where(first, k2, k3)
                    re, im = jnp.where(first, k3, k2), pltpu.roll(up, 126, 1)
                    ny = jnp.where(lane0, im, up)
                    u = [ny[q * 16:(q + 1) * 16] for q in range(4)]
                    odd_lane = (lane & 1) == 1
                    nr = jnp.where(odd_lane, pltpu.roll(u[0] - u[2], 1, 1), u[0] + u[2] + (u[1] + u[3]) * sgn0)
                    ni = jnp.where(odd_lane, pltpu.roll((u[3] - u[1]) * sgn0, 1, 1), 0.0)
                    rows = pl.ds(pl.multiple_of(p * 64 + rs * 16, 16), 16)
                    c, sn = tv_ref[0, rows], tv_ref[1, rows]
                    put(ny_ref, 0, rs, nr * c + ni * sn, ni * c - nr * sn)
                    im = jnp.where(lane0, 0.0, im)
                else:
                    re, im = k1 + k2, (k3 - k1) * jnp.where(first, 1.0, -1.0)
                a = _dft4([(re[q * 16:(q + 1) * 16], im[q * 16:(q + 1) * 16]) for q in range(4)])
                for jq in range(4):
                    re, im = a[jq]
                    if jq > 0:
                        c, sn = cs[jq]
                        re, im = re * c + im * sn, im * c - re * sn
                    put(ub_ref, t * 4 + jq, rs, re, im)
        return item

    def p2_bfly(u, g, inverse, ref=ub_ref):
        def item(y):
            if y is not None:
                ub_ref[136, pin_rows(0), :] = y
            v = ref[pl.ds(u * 8, 8), g * 16:(g + 1) * 16]
            x = [(v[p, 0:8], v[p, 8:16]) for p in range(8)]
            x = _swap(_dft8(_swap(x))) if inverse else _dft8(x)
            ref[pl.ds(u * 8, 8), g * 16:(g + 1) * 16] = jnp.stack([w for c in x for w in c]).reshape(8, 16, 128)
        return item

    def filtered(xx, w):
        wr = pltpu.bitcast(w & jnp.uint32(0xFFFF0000), f32).reshape(8, 8, 128)
        wi = pltpu.bitcast(w << 16, f32).reshape(8, 8, 128)
        xx = xx.reshape(8, 2, 8, 128)
        xr, xi = xx[:, 0], xx[:, 1]
        return jnp.stack([xr * wr - xi * wi, xr * wi + xi * wr], axis=1).reshape(128, 128)

    def p2_fwd(u, jps):
        def item(y):
            t = u >> 2
            jq = u & 3
            xs = [_dot(_tobf(ms_ref[jq + 4 * jp]), ub_ref[u * 8 + jp].astype(bf16)) for jp in jps]
            for jp, xx in zip(jps, xs):
                ub_ref[u * 8 + jp] = filtered(xx, wp_ref[pl.ds(t * 2560 + jq + 4 * jp, 64, stride=40), :])
        return item

    def p2_nyq(u):
        def item(y):
            jp = u & 7
            rhs = ny_ref[jp].astype(bf16)
            xx = jnp.concatenate([_dot(_tobf(ms_ref[u * 4, m * 16:(m + 1) * 16]), rhs) for m in range(4)], axis=0)
            w = wp_ref[pl.ds(4 * 2560 + 4 * jp, 64, stride=40), :]
            for jq in range(1, 4):
                w = jnp.where(lane == jq, wp_ref[pl.ds(4 * 2560 + 4 * jp + jq, 64, stride=40), :], w)
            w = jnp.where(u < 8, w, jnp.uint32(0x3F800000))
            ny_ref[jp] = filtered(xx, w)
        return item

    def p2_inv(u, jps):
        def item(y):
            jq = u & 3
            zs = [_dot(_tobf(ms_ref[32 + jq + 4 * jp]), ub_ref[u * 8 + jp].astype(bf16)) for jp in jps]
            for jp, zz in zip(jps, zs):
                ub_ref[u * 8 + jp] = zz
        return item

    def p3_pre(p, g, t):
        def item(y):
            sa_ref[0, pin_rows(0), :] = y
            cs = twiddles(p)

            def fetch(t):
                a = []
                for jq in range(4):
                    v = ub_ref[(t * 4 + jq) * 8 + p, g * 16:(g + 1) * 16]
                    re, im = v[0:8], v[8:16]
                    if jq > 0:
                        c, sn = cs[jq]
                        re, im = re * c - im * sn, im * c + re * sn
                    a.append((re, im))
                return _swap(_dft4(_swap(a)))

            u = fetch(t)
            if t == 0:
                v = ny_ref[p, g * 16:(g + 1) * 16]
                rows = pl.ds(pl.multiple_of(p * 64 + g * 8, 8), 8)
                c, sn = tv_ref[0, rows], tv_ref[1, rows]
                nr, ni = v[0:8] * c - v[8:16] * sn, v[8:16] * c + v[0:8] * sn
                zr, zi = pltpu.roll(nr, 127, 1), pltpu.roll(ni, 127, 1)
                ny = (nr + zr, (nr - zi) * sgn0, nr - zr, (nr + zi) * sgn0)
            first = first_lanes(t)
            for q in range(4):
                re, im = u[q]
                rows = slice(q * 64 + g * 8, q * 64 + (g + 1) * 8)
                if t == 0:
                    im = pltpu.roll(jnp.where(lane0, ny[q], im), 2, 1) + jnp.where(lane == 2, ny[q], 0.0)
                    sa_ref[1:3, rows] = jnp.stack((jnp.where(first, im, re), jnp.where(first, re, im)))
                else:
                    im = im * jnp.where(first, 1.0, -1.0)
                    sa_ref[3 * t:3 * t + 3, rows] = jnp.stack((re + im, im, re))
        return item

    def p3_mm(p, q):
        def item(y):
            g = []
            for t in range(4):
                k1, k2, k3 = d_products(sa_ref, 1, t, slice(q * 64, (q + 1) * 64))
                g.append((k3, k2) if t == 0 else (k2 + k1, k3 - k1))
            yy = _r8_real_t(g)
            bx_ref[q, pl.ds(pl.multiple_of(p * 64, 64), 64), :] = jnp.concatenate(yy, axis=1).astype(bf16)
        return item

    def b_out(p):
        def item(y):
            rows = pl.ds(pl.multiple_of(p * 64, 64), 64)
            pltpu.make_async_copy(bx_ref.at[0:4, rows, :], out_hbm.at[:, rows, pl.ds(DM, DM)],
                                  sem_out.at[1]).start()
            bx_ref[4, pin_rows(0), 0:128] = y.astype(bf16)
        return item

    def a_out(blk, half):
        pltpu.make_async_copy(
            xo_ref.at[half, pl.ds(pl.multiple_of(blk * 64 + 64, 64), 64), :],
            out_hbm.at[blk >> 3, pl.ds(pl.multiple_of((blk & 7) * 64, 64), 64),
                       pl.ds(pl.multiple_of(half * 512, 512), 512)],
            sem_out.at[0]).start()

    def step(pp, odd, mem, hooks, first=False):
        r0 = pl.multiple_of(pp * 64 + (64 + 32 * odd), SEG)
        xs = jnp.concatenate([xo_ref[0, pl.ds(r0, SEG), :], xo_ref[1, pl.ds(r0, SEG), :]], axis=1)
        x_lo = xs[0:8].astype(f32)
        hm = jnp.concatenate(
            [jnp.concatenate([x_lo, jnp.concatenate(mem, axis=1)], axis=0).astype(bf16), xs[16:32]], axis=0)
        fill = fillo_ref[:, 0:64] if odd else fille_ref[:, 0:48]
        qkv, ps = {}, {}

        def head_of(v):
            return (v // 16) * 16 + (v % 2) * 8 + (v % 16) // 2 if odd else v

        def do_qkv(v0, v1):
            for v in range(v0, v1):
                h = head_of(v)
                for t in range(3):
                    n = t * H + slot_of(h)
                    y32 = _dot(hm, _tobf(w_refs[n // 16][n % 16, 0:512]))
                    y = y32.astype(bf16)
                    parts = [y]
                    if odd or t > 0:
                        parts.append(_tobf(qkvc_ref[pp, n]))
                    if t > 0:
                        if odd:
                            parts.append(_tobf(kve_ref[(t - 1) * H + h]))
                        else:
                            kve_ref[(t - 1) * H + h] = _tou(y[0:16])
                    qkv[(t, v)] = jnp.concatenate(parts, axis=0) if len(parts) > 1 else y
                for item in hooks.get(v, ()):
                    item(y32[0:8])

        def do_s(g):
            for v in range(g * G, (g + 1) * G):
                sc = jax.lax.dot_general(qkv[(0, v)], qkv[(1, v)], (((1,), (1,)), ((), ())),
                                         preferred_element_type=f32)
                sc = jnp.where(fill == 0.0, sc * scale, fill)
                e = jnp.exp(sc - jnp.max(sc, axis=1, keepdims=True))
                den = jnp.sum(e, axis=1, keepdims=True)
                r = pl.reciprocal(den, approx=True)
                r = r * (2.0 - den * r)
                ps[v] = (e * r).astype(bf16)

        def do_pv(g):
            o = {v: _dot(ps[v], qkv[(2, v)]) for v in range(g * G, (g + 1) * G)}
            for v in o:
                h = head_of(v)
                oall_ref[:, h * DH:(h + 1) * DH] = _tou(o[v][0:32].astype(bf16))
            if odd:
                for v in range(g * G, (g + 1) * G, 2):
                    a11, a12 = o[v][0:32], o[v + 1][0:32]
                    a21 = jnp.concatenate([oc_ref[head_of(v)], o[v][32:48]], axis=0)
                    a22 = jnp.concatenate([oc_ref[head_of(v + 1)], o[v + 1][32:48]], axis=0)
                    for k, a in enumerate((a11 + a22, a21 + a22, a22, a11 + a12, a21 - a11, a12 - a22)):
                        os_ref[k, :, (v // 2) * DH:(v // 2 + 1) * DH] = a
                for v in o:
                    oc_ref[head_of(v)] = o[v][32:48]

        def plain(half, j, h0, h1):
            return _dot(_tobf(oall_ref[:, h0 * DH:h1 * DH]), _tobf(wo_ref[half, j, h0 * 64:h1 * 64, :]))

        hb = pp & 1
        if odd:
            def product(jp, k):
                def fn(part):
                    h0 = part * 16
                    if k == 2:
                        lhs = _tobf(oall_ref[:, h0 * DH:(h0 + 8) * DH])
                    else:
                        lhs = os_ref[k - (k > 2), :, part * 1024:(part + 1) * 1024].astype(bf16)
                    if k == 1:
                        rhs = wo_ref[hb, jp * 2, h0 * 64:(h0 + 8) * 64, :]
                    elif k == 4:
                        rhs = wo_ref[hb, jp * 2 + 1, (h0 + 8) * 64:(h0 + 16) * 64, :]
                    else:
                        rhs = ws_ref[hb, jp * 5 + (0, 0, 1, 2, 0, 3, 4)[k], part * 512:(part + 1) * 512, :]
                    return _dot(lhs, _tobf(rhs))
                return fn
            jobs = [product(jp, k) for jp in range(2) for k in range(7)]
            jobs += [(lambda part, j=j: plain(1 - hb, j, part * 16, part * 16 + 16)) for j in range(4)]
            marks = (2, 10)
        else:
            jobs = [(lambda part, j=j: plain(j // 4, j % 4, part * 24, 24 + part * 8)) for j in range(8)]
            marks = (2, 5)

        for g in range(NG):
            do_qkv(g * G, g * G + G // 2)
            if g >= 1:
                do_s(g - 1)
            do_qkv(g * G + G // 2, (g + 1) * G)
            if g >= 2:
                do_pv(g - 2)
        part = []
        for k, job in enumerate(jobs):
            items = hooks.get(('o', k), ())
            if len(items) == 2:
                half = plain(k // 4, k % 4, 0, 12)
                items[0](half[0:8])
                part.append(plain(k // 4, k % 4, 12, 24) + half)
                items[1](part[k][0:8])
            else:
                part.append(job(0))
                for item in items:
                    item(part[k][0:8])
            if k == marks[0]:
                do_s(NG - 1)
                do_pv(NG - 2)
            if k == marks[1]:
                do_pv(NG - 1)

        def finish(k):
            res = jobs[k](1) + part[k]
            for item in hooks.get(('p', k), ()):
                item(res[0:8])
            return res

        def put(half, j, r, v):
            xo_ref[half, pl.ds(r0 + r, v.shape[0]), j * 128:(j + 1) * 128] = v.astype(bf16)

        if odd:
            own = []
            for jp in range(2):
                m1, m2, m3, m4, m5, m6, m7 = [finish(jp * 7 + k) for k in range(7)]
                for jj, top, bot in ((0, ((m1 + m4) - m5) + m7, m2 + m4), (1, m3 + m5, ((m1 - m2) + m3) + m6)):
                    j = jp * 2 + jj
                    own.append(top[8:16])
                    put(hb, j, 0, jnp.concatenate([top[0:8], bot[24:32], top[16:32]], axis=0))
                    put(hb, j, -24, bot[16:24])
                    put(hb, j, -56, bot[8:16])
                    put(hb, j, -88, bot[0:8])
            for j in range(4):
                res = finish(14 + j)
                own.append(res[8:16])
                put(1 - hb, j, 0, res)
            new_mem = [jnp.where(hb == 0, own[j], own[(j + 4) % 8]) for j in range(8)]
        else:
            new_mem = []
            for j in range(8):
                res = finish(j)
                new_mem.append(res[8:16])
                put(j // 4, j % 4, 0, res)
        for item in hooks.get(H, ()):
            item(None)
        if odd:
            a_out(pp, hb)
            if first:
                pl.when(pp > 0)(lambda: a_out(pp - 1, hb))
            else:
                a_out(pp - 1, hb)
        return new_mem

    def l1(i, mem):
        bx_copy(i).wait()
        he = {2 * k: [p1_pre(i, k // 4, k % 4)] for k in range(16)}
        he[H] = [p1_mm(i, 1), p1_mm(i, 2), p1_mm(i, 3)]
        ho = {('p', 2): [p1_mm(i, 0)]}
        mem = step(i, 0, mem, he)
        mem = step(i, 1, mem, ho, first=True)
        return mem

    def l2(i, mem):
        u = i - N_L1
        he = {3: [p2_fwd(u, range(0, 4))], 7: [p2_fwd(u, range(4, 8))], 17: [p2_nyq(u)],
              H: [p2_inv(u, range(0, 8))]}
        ho = {('p', k): [p2_bfly(u + k % 2, k // 2, k % 2 == 0)] for k in range(16)}
        mem = step(i, 0, mem, he)
        mem = step(i, 1, mem, ho)
        return mem

    def l3(i, mem):
        p = i - N_L1 - N_L2
        he = {h: [p3_pre(p, h // 3, 1 + h % 3)] for h in range(24)}
        for j in range(4):
            he[('o', 3 + j)] = [p3_pre(p, 2 * j, 0), p3_pre(p, 2 * j + 1, 0)]
        he[H] = [p3_mm(p, q) for q in range(4)]
        ho = {12: [b_out(p)]}
        mem = step(i, 0, mem, he)
        mem = step(i, 1, mem, ho)
        return mem

    m0 = mem_ref[...].astype(f32)
    mem = [m0[:, j * 128:(j + 1) * 128] for j in range(8)]
    mem = jax.lax.fori_loop(0, N_L1, l1, mem)
    cp_x[2].wait()
    cp_x[3].wait()
    cp_ms.wait()
    for g in range(8):
        p2_bfly(0, g, False)(None)
        p2_bfly(0, g, False, ny_ref)(None)
    mem = jax.lax.fori_loop(N_L1, N_L1 + N_L2, l2, mem)
    for g in range(8):
        p2_bfly(0, g, True, ny_ref)(None)
    mem = jax.lax.fori_loop(N_L1 + N_L2, NSEG // 2, l3, mem)

    oc_last = jnp.concatenate([oc_ref[h] for h in range(H)], axis=1).astype(bf16)
    for j in range(4):
        res = _dot(oc_last, _tobf(wo_ref[0, j, 0:2048, :])).astype(bf16)
        xo_ref[0, S + 8:S + 16, j * 128:(j + 1) * 128] = res[0:8]
        xo_ref[0, S + 40:S + 48, j * 128:(j + 1) * 128] = res[8:16]
    a_out(NSEG // 2 - 1, 0)

    pltpu.make_async_copy(bx_ref.at[0:4], out_hbm.at[:, :, pl.ds(DM, DM)], sem_out.at[1]).wait()
    pltpu.make_async_copy(xo_ref.at[:, 64:64 + S], xo_ref.at[:, 64:64 + S], sem_out.at[0]).wait()


@jax.jit
def _run(x, mem0, wq, wk, wv, wo, bx, w_r, w_i):
    fd, ms, tv = _tables()
    hbm = pl.BlockSpec(memory_space=pl.ANY)
    out = pl.pallas_call(
        _kernel,
        out_shape=jax.ShapeDtypeStruct((4, S // 4, 2 * DM), bf16),
        in_specs=[hbm] * 13,
        out_specs=hbm,
        scratch_shapes=[
            pltpu.VMEM((2, 64 + S, DM // 2), bf16),
            pltpu.VMEM((MEM, DM), bf16),
            pltpu.VMEM((8, NSEG, 8, 128), bf16),
            pltpu.VMEM((4, DM, 16, DH), bf16),
        ] + [pltpu.VMEM((16, DM // 2 + 8, DH), u32)] * 6 + [
            pltpu.VMEM((2, 4, H * DH // 2 + 8, 128), u32),
            pltpu.VMEM((8, 256, 128), u32),
            pltpu.VMEM((5, 4, 136, 128), u32),
            pltpu.VMEM((NSEG // 2, 3 * H, 8, 128), u32),
            pltpu.VMEM((2 * H, 8, 128), u32),
            pltpu.VMEM((16, H * DH), u32),
            pltpu.VMEM((H, 16, DH), f32),
            pltpu.VMEM((6, 32, 16 * DH), f32),
            pltpu.VMEM((2, 10, 1040, 128), u32),
            pltpu.VMEM((32, 128), f32),
            pltpu.VMEM((48, 128), f32),
            pltpu.VMEM((5, S // 4, DM), bf16),
            pltpu.VMEM((16, DM // 2 + 1, 256), bf16),
            pltpu.VMEM((12872, 128), u32),
            pltpu.VMEM((137, 128, 128), f32),
            pltpu.VMEM((8, 128, 128), f32),
            pltpu.VMEM((12, 264, 128), f32),
            pltpu.VMEM((24, 64, 128), u32),
            pltpu.VMEM((64, 64, 128), u32),
            pltpu.VMEM((2, 512, 128), f32),
            pltpu.SMEM((64,), f32),
            pltpu.SMEM((1,), jnp.int32),
            pltpu.SemaphoreType.DMA((84,)),
            pltpu.SemaphoreType.DMA((2,)),
        ],
        compiler_params=pltpu.CompilerParams(vmem_limit_bytes=120 * 1024 * 1024,
                                             disable_semaphore_checks=True,
                                             disable_bounds_checks=True),
    )(x.reshape(S, DM), x.reshape(NSEG, SEG, DM), mem0.reshape(MEM, DM), wq, wk, wv,
      wo.reshape(H * DH // 16, 16, DM), bx.reshape(4, S // 4, DM), w_r.T, w_i.T, jnp.asarray(fd), jnp.asarray(ms), jnp.asarray(tv))
    return out.reshape(1, S, 2 * DM)


def pallas_concat_heads__memory_aug_recurrent_mem_tr__spectral_gfnet__prompt_kernel(
    A_x: jax.Array,
    A_mem0: jax.Array,
    A_Wq: jax.Array,
    A_Wk: jax.Array,
    A_Wv: jax.Array,
    A_Wo: jax.Array,
    A_seg_len,
    B_x: jax.Array,
    B_w_r: jax.Array,
    B_w_i: jax.Array,
):
    if isinstance(A_seg_len, int):
        assert A_seg_len == SEG
    assert A_x.shape == (1, S, DM) and A_mem0.shape == (1, MEM, DM) and A_Wq.shape == (DM, H, DH)
    assert B_x.shape == (1, S, DM) and B_w_r.shape == (S, DM // 2 + 1)
    return _run(A_x, A_mem0, A_Wq, A_Wk, A_Wv, A_Wo, B_x, B_w_r, B_w_i)
```

```python
import math

import numpy as np
import jax
import jax.numpy as jnp
import jax.experimental.pallas as pl
import jax.experimental.pallas.tpu as pltpu

bf16 = jnp.bfloat16
f32 = jnp.float32
u32 = jnp.uint32

S, DM = 2048, 1024
H, DH = 32, 128
MEM, SEG = 8, 32
NSEG = S // SEG
SQH = math.sqrt(0.5)

_PAIRS = ((0, 4), (1, 7), (2, 6), (3, 5))
_FIRST = np.array([[1, 1, 0, 0], [1, 0, 1, 0], [0, 1, 1, 0], [0, 1, 0, 1]], bool)


def _pack_rows(a):
    u = np.ascontiguousarray(a, dtype=np.float32).view(np.uint32).astype(np.uint64)
    b = ((u + 0x7FFF + ((u >> 16) & 1)) >> 16).astype(np.uint32)
    return (b[..., 0::2, :] | (b[..., 1::2, :] << 16)).astype(np.uint32)


def _tables():
    k2 = np.zeros((4, 128), np.int64)
    for t in range(4):
        odd = t % 2
        for lam in range(128):
            k = 2 * lam + odd
            if k % 8 not in _PAIRS[t]:
                k = 2 * (128 + 8 * (lam // 8) + (lam % 8 - 1 - odd) % 8) + odd
            assert k % 8 in _PAIRS[t]
            k2[t, lam] = k
    b = np.arange(128)[:, None]
    F = np.zeros((12, 128, 128))
    G = np.zeros((12, 128, 128))
    for t in range(4):
        th = 2 * np.pi * ((b * k2[t][None, :]) % DM) / DM
        C, Sn = np.cos(th), np.sin(th)
        first = ((k2[t] % 8) == _PAIRS[t][0])[None, :]
        assert np.array_equal(first[0], _FIRST[t][np.arange(128) % 4])
        if t == 0:
            im = -Sn
            im[:, 0] = (-1.0) ** np.arange(128)
            im = np.roll(im, 2, axis=1)
            F[1:3] = np.where(first, im, C), np.where(first, C, im)
            G[1:3] = F[1:3]
            G[2, :, 0] *= 0.5
            G[2, :, 2] *= 0.5
        else:
            Sg = np.where(first, Sn, -Sn)
            F[3 * t:3 * t + 3] = C, -(C + Sg), C - Sg
            G[3 * t:3 * t + 3] = F[3 * t:3 * t + 3]
    Finv = np.transpose(G, (0, 2, 1)) * (2.0 / DM)
    fd = _pack_rows(np.concatenate([F, Finv]))
    M = np.zeros((32, 128, 128))
    r = np.arange(64)[None, :]
    l = np.arange(64)[:, None]
    for j in range(32):
        th = 2 * np.pi * ((r * (j + 32 * l)) % S) / S
        C, Sn = np.cos(th), np.sin(th)
        M[j, :64, :64] = C
        M[j, :64, 64:] = Sn
        M[j, 64:, :64] = -Sn
        M[j, 64:, 64:] = C
    perm = np.arange(128).reshape(2, 8, 8).transpose(1, 0, 2).reshape(128)
    M = M[:, perm][:, :, perm]
    Minv = np.transpose(M, (0, 2, 1)) / S
    ms = _pack_rows(np.concatenate([M, Minv]))
    th = 2 * np.pi * np.outer(np.arange(512), np.arange(128) % 4) / S
    tv = np.stack([np.cos(th), np.sin(th)]).astype(np.float32)
    return fd, ms, tv


def _tobf(w):
    return pltpu.bitcast(w, bf16)


def _tou(w):
    return pltpu.bitcast(w, u32)


def _dot(a, b):
    return jnp.dot(a, b, preferred_element_type=f32)


def _r8_real(x):
    t0, t1 = x[0] + x[4], x[0] - x[4]
    t2, t3 = x[2] + x[6], x[2] - x[6]
    t4, t5 = x[1] + x[5], x[1] - x[5]
    t6, t7 = x[3] + x[7], x[3] - x[7]
    e0, e1 = t0 + t2, t0 - t2
    o0, o1 = t4 + t6, t4 - t6
    u, v = SQH * (t5 - t7), SQH * (t5 + t7)
    return [(e0 + o0, e0 - o0), (t1 + u, v + t3), (e1, o1), (t1 - u, v - t3)]


def _r8_real_t(g):
    (z0, z4), (a1, b1), (e1, o1), (a3, b3) = g
    e0, o0 = z0 + z4, z0 - z4
    t1, u = a1 + a3, a1 - a3
    v, t3 = b1 + b3, b1 - b3
    t5, t7 = SQH * (v + u), SQH * (v - u)
    t0, t2 = e0 + e1, e0 - e1
    t4, t6 = o0 + o1, o0 - o1
    return [t0 + t1, t4 + t5, t2 + t3, t6 + t7, t0 - t1, t4 - t5, t2 - t3, t6 - t7]


def _dft4(u):
    (r0, i0), (r1, i1), (r2, i2), (r3, i3) = u
    sr, si, dr, di = r0 + r2, i0 + i2, r0 - r2, i0 - i2
    tr, ti, er, ei = r1 + r3, i1 + i3, r1 - r3, i1 - i3
    return [(sr + tr, si + ti), (dr + ei, di - er), (sr - tr, si - ti), (dr - ei, di + er)]


def _dft8(x):
    a = [(x[p][0] + x[p + 4][0], x[p][1] + x[p + 4][1]) for p in range(4)]
    d = [(x[p][0] - x[p + 4][0], x[p][1] - x[p + 4][1]) for p in range(4)]
    ev = _dft4(a)
    (r0, i0), (r1, i1), (r2, i2), (r3, i3) = d
    b1r, b1i = SQH * (r1 + i1), SQH * (i1 - r1)
    b3r, n3i = SQH * (i3 - r3), SQH * (r3 + i3)
    sr, si, dr, di = r0 + i2, i0 - r2, r0 - i2, i0 + r2
    tr, ti, er, ei = b1r + b3r, b1i - n3i, b1r - b3r, b1i + n3i
    od = [(sr + tr, si + ti), (dr + ei, di - er), (sr - tr, si - ti), (dr - ei, di + er)]
    return [ev[0], od[0], ev[1], od[1], ev[2], od[2], ev[3], od[3]]


def _swap(x):
    return [(b, a) for (a, b) in x]


G = 4
NG = H // G
NEG = -1e9
N_L1, N_L2, N_L3 = 8, 16, 8


def _kernel(x_hbm, x3_hbm, mem_hbm, wq_hbm, wk_hbm, wv_hbm, wo_hbm, bx_hbm, wr_hbm, wi_hbm,
            fd_hbm, ms_hbm, tv_hbm, out_hbm,
            xo_ref, mem_ref, xcraw_ref, raw_ref, w0_ref, w1_ref, w2_ref, w3_ref, w4_ref, w5_ref,
            wo_ref, xc_ref, xs_ref, qkvc_ref, kve_ref,
            oall_ref, oc_ref, os_ref, ws_ref, fille_ref, fillo_ref, bx_ref, wt_ref, wp_ref, ub_ref, ny_ref, sa_ref, fd_ref, ms_ref, tv_ref,
            tw_ref, zero_ref, sem_in, sem_out):
    scale = DH ** -0.5
    w_hbm = (wq_hbm, wk_hbm, wv_hbm)
    w_refs = (w0_ref, w1_ref, w2_ref, w3_ref, w4_ref, w5_ref)

    def raw_copy(c, i=0, nd=DM):
        rows = pl.ds(pl.multiple_of(i * nd, nd), nd)
        return pltpu.make_async_copy(
            w_hbm[c // 2].at[rows, pl.ds((c % 2) * 16, 16), :],
            raw_ref.at[c % 4, rows], sem_in.at[8 + min(c, 3) * 8 + max(c - 3, 0) * 2 + i])

    def xc_copy(k):
        return pltpu.make_async_copy(
            x3_hbm.at[:, pl.ds(8, 8), pl.ds(pl.multiple_of(k * 128, 128), 128)], xcraw_ref.at[k], sem_in.at[40 + k])

    def wo_copies(half):
        return [pltpu.make_async_copy(wo_hbm.at[:, :, pl.ds(pl.multiple_of(half * 512 + j * 128, 128), 128)],
                                      raw_ref.at[2 + half, j * 256:(j + 1) * 256], sem_in.at[76 + half * 4 + j])
                for j in range(4)]

    def wt_copies(i):
        return [pltpu.make_async_copy(src.at[:, pl.ds(pl.multiple_of(i * 1024 + k * 256, 256), 256)],
                                      wt_ref.at[i, a * 4 + k], sem_in.at[i * 4 + (48 + a * 8 + k)])
                for k in range(4) for a, src in enumerate((wr_hbm, wi_hbm))]

    def bx_copy(p):
        rows = pl.ds(pl.multiple_of(p * 64, 64), 64)
        return pltpu.make_async_copy(bx_hbm.at[:, rows, :], bx_ref.at[0:4, rows, :], sem_in.at[64 + p])

    n_head = N_L1 * 2 * SEG
    cp_x = [pltpu.make_async_copy(x_hbm.at[lo:hi, half * 512:(half + 1) * 512], xo_ref.at[half, 64 + lo:64 + hi],
                                  sem_in.at[72 + (lo > 0) * 2 + half])
            for lo, hi in ((0, n_head), (n_head, S)) for half in range(2)]
    cp_mem = pltpu.make_async_copy(mem_hbm, mem_ref, sem_in.at[1])
    cp_fd = pltpu.make_async_copy(fd_hbm, fd_ref, sem_in.at[4])
    cp_ms = pltpu.make_async_copy(ms_hbm, ms_ref, sem_in.at[5])
    cp_tv = pltpu.make_async_copy(tv_hbm, tv_ref, sem_in.at[6])

    for i in range(8):
        raw_copy(0, i, 128).start()
        if i < 4:
            xc_copy(i).start()
        if 3 <= i < 7:
            xc_copy(i + 1).start()
        if i >= 3:
            raw_copy(2, i - 3, 128).start()
        if i == 7:
            raw_copy(2, 5, 128).start()
        raw_copy(1, i, 128).start()
    for i in range(6, 8):
        raw_copy(2, i, 128).start()
    for i in range(2):
        raw_copy(3, i, 512).start()

    zero_ref[0] = 0

    def pin_bit():
        return jnp.clip(zero_ref[0], 0, 1)

    def pin_rows(r):
        return pl.ds(pl.multiple_of(r + pin_bit() * 32, 8), 8)

    for p in range(8):
        for jq in range(4):
            tw_ref[(p * 4 + jq) * 2] = jnp.float32(math.cos(2 * math.pi * p * jq / 32))
            tw_ref[(p * 4 + jq) * 2 + 1] = jnp.float32(math.sin(2 * math.pi * p * jq / 32))

    ub_ref[128:136] = jnp.zeros((8, 128, 128), f32)
    wp_ref[12800:12872] = jnp.zeros((72, 128), u32)
    oc_ref[...] = jnp.zeros((H, 16, DH), f32)

    qi = jax.lax.broadcasted_iota(jnp.int32, (48, 128), 0)
    ki = jax.lax.broadcasted_iota(jnp.int32, (48, 128), 1)

    def between(v, lo, hi):
        return (v >= lo) & (v < hi)

    def table(keep, other):
        return jnp.where(other, -jnp.inf, jnp.where(keep, 0.0, NEG)).astype(f32)

    keep = between(qi, 8, 16) | between(ki, 8, 16) | (qi >= jnp.where(ki < 32, ki, ki - 24))
    fille_ref[...] = table(keep, ki >= 40)[:32]
    q_even = between(qi, 32, 40)
    k_even = between(ki, 32, 40) | (ki >= 48)
    qpos = jnp.where(qi < 32, qi, jnp.where(qi < 40, qi - 24, qi - 32))
    kpos = jnp.where(ki < 32, ki, jnp.where(ki < 40, ki - 24, jnp.where(ki < 48, ki - 32, ki - 48)))
    keep = between(qi, 8, 16) | between(ki, 8, 16) | (ki >= 56) | (qpos >= kpos)
    fillo_ref[...] = table(keep, (q_even != k_even) | (ki >= 64))

    def relayout16(c, blk):
        w0 = pl.multiple_of(blk * 8, 8)
        v = _tou(raw_ref[c % 4, pl.ds(blk * 16, 16)]).reshape(8, 2, 8, 128)
        a, b = v[:, 0], v[:, 1]
        w_refs[c][0, :, pl.ds(w0, 8), :] = jnp.swapaxes((a & jnp.uint32(0xFFFF)) | (b << 16), 0, 1)
        w_refs[c][1, :, pl.ds(w0, 8), :] = jnp.swapaxes((a >> 16) | (b & jnp.uint32(0xFFFF0000)), 0, 1)

    def slot_of(h):
        return (h // 16) * 16 + (h % 2) * 8 + (h % 16) // 2

    def repack_wo(half, part, k):
        jp, g0 = k & 1, part * 128 + (k >> 1) * 2
        quad = []
        for jj in range(2):
            for kh in range(2):
                v = _tou(raw_ref[2 + half, pl.ds((jp * 2 + jj) * 256 + kh * 64 + g0, 2)]).reshape(16, 128)
                wo_ref[half, jp * 2 + jj, pl.ds(pl.multiple_of(g0 * 8 + kh * 512, 16), 16), :] = v
                quad.append(_tobf(v).astype(f32))
        b11, b21, b12, b22 = quad
        rows = pl.ds(pl.multiple_of(part * 512 + (k >> 1) * 16, 16), 16)
        for n, v in enumerate((b11 + b22, b12 - b22, b21 - b11, b11 + b12, b21 + b22)):
            ws_ref[half, jp * 5 + n, rows, :] = _tou(v.astype(bf16))

    sub4 = jax.lax.broadcasted_iota(jnp.int32, (128, 128), 0) & 3

    def wp_store(t, kb, tile):
        v = tile.T.reshape(4, 32, 128)
        v = jnp.concatenate([v, v[:, 0:8]], axis=1).reshape(160, 128)
        wp_ref[pl.ds(pl.multiple_of(t * 2560 + kb * 160, 32), 160), :] = v

    def b_prep(i, k, hb, par):
        cols = slice(hb * 128, (hb + 1) * 128)
        a = _tou(wt_ref[i, k, 0:512, cols])
        b = _tou(wt_ref[i, 4 + k, 0:512, cols])
        if par == 0:
            w = (a << 16) | (b & jnp.uint32(0xFFFF))
            m = (sub4 == 0) | (sub4 == 2)
        else:
            w = (a & jnp.uint32(0xFFFF0000)) | (b >> 16)
            m = (sub4 == 0) | (sub4 == 3)
        top = w[:128]
        bot = pltpu.roll(w[128:].reshape(16, 8, 128), 1 + par, 1).reshape(128, 128)
        wp_store(par, i * 8 + (k * 2 + hb), jnp.where(m, top, bot))
        wp_store(par + 2, i * 8 + (k * 2 + hb), jnp.where(m, bot, top))
        if par == 0:
            na = jnp.broadcast_to(wt_ref[i, k, 512:513, cols].astype(f32), (128, 128))
            nb = jnp.broadcast_to(wt_ref[i, 4 + k, 512:513, cols].astype(f32), (128, 128))
            wp_store(4, i * 8 + (k * 2 + hb), pltpu.bitcast(na, u32) | (pltpu.bitcast(nb, u32) >> 16))

    def gather_c(k):
        xc_ref[k] = _tou(xcraw_ref[k].astype(f32).reshape(512, 128).astype(bf16))

    def store_qkvc(n, y):
        qkvc_ref[:, n // 8, n % 8] = y.reshape(NSEG // 2, 8, 128)

    def q_unit(i, groups, first, last, fillers):
        xk = _tobf(xc_ref[i])
        w0 = pl.multiple_of(i * 64, 64)
        for g in groups:
            rhs = jnp.concatenate(
                [_tobf(w_refs[h // 16][h // 8 % 2, h % 8, pl.ds(w0, 64), :]) for h in range(4 * g, 4 * g + 4)], axis=1)
            y = _dot(xk, rhs)
            for h in range(4 * g, 4 * g + 4):
                yh = y[:, (h % 4) * 128:(h % 4 + 1) * 128]
                if not first:
                    yh = yh + ub_ref[h * 4:(h + 1) * 4].reshape(512, 128)
                if last:
                    store_qkvc(h, _tou(yh.astype(bf16)))
                else:
                    ub_ref[h * 4:(h + 1) * 4] = yh.reshape(4, 128, 128)
            mine = fillers.get(g, [])
            for fi, item in enumerate(mine):
                r = (fi * 512 // len(mine)) // 8 * 8
                item(pltpu.bitcast(y[r:r + 8, 0:128], u32))

    def rl_item(c, blk):
        def item(pin):
            w_refs[c][pin_bit(), 7, 512:520] = pin
            relayout16(c, blk)
        return item

    def spread(fillers, items, groups):
        for k, item in enumerate(items):
            fillers.setdefault(groups[k * len(groups) // len(items)], []).append(item)
        return fillers

    def half_items(f, c, i, groups):
        return spread(f, [rl_item(c, i * 8 + blk) for blk in range(8)], groups)

    def piece_items(i):
        f = half_items(half_items({}, 1, i, (0, 1, 2)), 0, i + 1, (4, 5, 6))
        return spread(f, [lambda pin: gather_c(i + 1)], (7,))

    def chunk2_items(f, lo, hi, groups):
        return spread(f, [rl_item(2, blk) for blk in range(lo, hi)], groups)

    def wait_piece(i):
        raw_copy(1, i, 128).wait()
        raw_copy(0, i + 1, 128).wait()

    raw_copy(0, 0, 128).wait()
    for blk in range(8):
        relayout16(0, blk)
    xc_copy(0).wait()
    gather_c(0)
    q_unit(0, range(0, 2), True, False, {})
    raw_copy(1, 0, 128).wait()
    q_unit(0, range(2, 4), True, False, half_items({}, 1, 0, (2, 2, 3)))
    q_unit(0, range(4, 6), True, False, {})
    xc_copy(1).wait()
    raw_copy(0, 1, 128).wait()
    q_unit(0, range(6, 8), True, False,
           spread(half_items({}, 0, 1, (6, 6, 7)), [lambda pin: gather_c(1)], (6,)))
    raw_copy(1, 1, 128).wait()
    q_unit(1, range(0, 4), False, False, half_items({}, 1, 1, (0, 1, 2)))
    xc_copy(2).wait()
    raw_copy(0, 2, 128).wait()
    q_unit(1, range(4, 8), False, False,
           spread(half_items({}, 0, 2, (4, 5, 6)), [lambda pin: gather_c(2)], (6,)))

    def xsum_item(j, rq):
        def item(pin):
            xs_ref[pin_bit(), 0, 128:136] = pin
            a11, a21, a12, a22 = [
                xcraw_ref[j + 4 * kh, rh * 32 + rq * 8:rh * 32 + (rq + 1) * 8].astype(f32).reshape(64, 128)
                for kh in range(2) for rh in range(2)]
            for k, v in enumerate((a11 + a22, a21 + a22, a11 + a12, a21 - a11, a12 - a22)):
                xs_ref[k, j, rq * 32:(rq + 1) * 32] = _tou(v.astype(bf16))
        return item

    def q_c(i, carry):
        wait_piece(i)
        xc_copy(i + 2).wait()
        raw_copy(2, i - 2, 128).wait()
        f = half_items(piece_items(i), 2, i - 2, (3, 3, 3, 3, 4, 5, 6, 7))
        q_unit(i, range(8), False, False, spread(f, [xsum_item(i - 2, rq) for rq in range(4)], (3, 4, 5, 6)))
        return carry
    xc_copy(3).wait()
    jax.lax.fori_loop(2, 6, q_c, 0)

    wait_piece(6)
    raw_copy(2, 4, 128).wait()
    raw_copy(2, 5, 128).wait()
    q_unit(6, range(8), False, False, chunk2_items(piece_items(6), 32, 48, (0, 1, 2, 3, 3, 4, 5, 6)))
    raw_copy(1, 7, 128).wait()
    raw_copy(2, 6, 128).wait()
    raw_copy(2, 7, 128).wait()
    q_unit(7, range(8), False, True, chunk2_items(half_items({}, 1, 7, (0, 1, 2)), 48, 64, (3, 4, 5, 6)))
    raw_copy(4).start()
    for cp in wo_copies(0):
        cp.start()
    raw_copy(5).start()

    def bulk_iter(c, i):
        def xs(k):
            return jnp.concatenate([_tobf(xs_ref[k, j, 0:128]) for j in range(4)], axis=1)

        def xc(rh, kh):
            return jnp.concatenate(
                [_tobf(xc_ref[4 * kh + j, rh * 128:(rh + 1) * 128]) for j in range(4)], axis=1)

        for pr in range(4):
            n1, n2 = pr * 2, pr * 2 + 1

            def w(n, kh):
                return _tobf(w_refs[c][i, n, kh * 256:(kh + 1) * 256])

            def wsum(a, b, sign):
                a, b = a.astype(f32), b.astype(f32)
                return (a + b if sign > 0 else a - b).astype(bf16)

            def out(rh, n, v):
                qkvc_ref[rh * 16:(rh + 1) * 16, c * 2 + i, n] = _tou(v.astype(bf16)).reshape(16, 8, 128)

            def side(k, m):
                blks = (k, 7) if k == 0 else (k,)
                items = []
                if c < 5:
                    items += [('w', blk) for blk in blks]
                if c >= 4:
                    items += [('o', blk) for blk in range(k * 16 // 7, (k + 1) * 16 // 7)]
                if c == 5 and k in (1, 2, 4, 5):
                    items.append(('f', (1, 2, 4, 5).index(k)))
                for n, (kind, blk) in enumerate(items):
                    r = n * 256 // len(items) // 8 * 8
                    pin = pltpu.bitcast(m[r:r + 8], u32)
                    if kind == 'w':
                        w_refs[c + 1][pin_bit(), 7, 512:520] = pin
                        relayout16(c + 1, i * 32 + (pr * 8 + blk))
                    elif kind == 'o':
                        ws_ref[pin_bit(), 9, 1024:1032] = pin
                        wo_ref[pin_bit(), 3, 2048:2056] = pin
                        repack_wo(c - 4, i, pr * 16 + blk)
                    else:
                        wp_ref[pin_rows(12832), :] = pin
                        b_prep(i, pr, blk // 2, blk % 2)

            m2 = _dot(xs(1), w(n1, 0))
            side(0, m2)
            m4 = _dot(xc(1, 1), wsum(w(n1, 1), w(n1, 0), -1))
            side(1, m4)
            out(1, n1, m4 + m2)
            m1 = _dot(xs(0), wsum(w(n1, 0), w(n2, 1), 1))
            side(2, m1)
            m5 = _dot(xs(2), w(n2, 1))
            side(3, m5)
            m3 = _dot(xc(0, 0), wsum(w(n2, 0), w(n2, 1), -1))
            side(4, m3)
            out(0, n2, m3 + m5)
            c22 = _dot(xs(3), wsum(w(n1, 0), w(n2, 0), 1)) + ((m1 - m2) + m3)
            side(5, c22)
            out(1, n2, c22)
            c11 = _dot(xs(4), wsum(w(n1, 1), w(n2, 1), 1)) + ((m1 + m4) - m5)
            side(6, c11)
            out(0, n1, c11)

    for c in range(2, 6):
        if c == 3:
            for cp in wo_copies(1) + wt_copies(0) + wt_copies(1):
                cp.start()
        if c == 4:
            for cp in cp_x[0:2] + [cp_mem, cp_fd, cp_tv] + [bx_copy(p) for p in range(8)] + cp_x[2:4] + [cp_ms]:
                cp.start()
        if c >= 4:
            for cp in wo_copies(c - 4):
                cp.wait()
        if 2 < c < 5:
            raw_copy(c + 1).wait()

        def bulk(i, carry, c=c):
            if c == 2:
                raw_copy(3, i, 512).wait()
            if c == 5:
                for cp in wt_copies(i):
                    cp.wait()
            bulk_iter(c, i)
            return carry
        jax.lax.fori_loop(0, 2, bulk, 0)

    cp_x[0].wait()
    cp_x[1].wait()
    cp_mem.wait()
    cp_fd.wait()
    cp_tv.wait()

    lane = jax.lax.broadcasted_iota(jnp.int32, (1, 128), 1)
    lane0 = lane == 0
    sgn0 = jnp.where(lane0, 1.0, -1.0)

    def first_lanes(t):
        la, lb = [k for k in range(4) if _FIRST[t][k]]
        return ((lane & 3) == la) | ((lane & 3) == lb)

    def d_products(st_ref, d, t, rows):
        return [_dot(st_ref[n, rows].astype(bf16), _tobf(fd_ref[d * 12 + n])) if n else None
                for n in range(3 * t, 3 * t + 3)]

    def twiddles(p):
        return [(tw_ref[p * 8 + jq * 2], tw_ref[p * 8 + jq * 2 + 1]) if jq else None for jq in range(4)]

    def p1_pre(p, rs, q):
        def item(y):
            sa_ref[0, pin_rows(0), :] = y
            xq = bx_ref[q, pl.ds(pl.multiple_of(p * 64 + rs * 16, 16), 16), :].astype(f32)
            zz = _r8_real([xq[:, a * 128:(a + 1) * 128] for a in range(8)])
            r = (rs * 4 + q) * 16
            sa_ref[1:12, r:r + 16] = jnp.stack([v for (a, b) in zz for v in (a + b, b, a)][1:])
        return item

    def p1_mm(p, t):
        def item(y):
            cs = twiddles(p)

            def put(ref, n, rs, re, im):
                v = jnp.stack([re.reshape(2, 8, 128), im.reshape(2, 8, 128)], axis=1)
                ref[n * 8 + p, rs * 32:(rs + 1) * 32] = v.reshape(32, 128)

            first = first_lanes(t)
            for rs in range(4):
                k1, k2, k3 = d_products(sa_ref, 0, t, slice(rs * 64, (rs + 1) * 64))
                if t == 0:
                    up = jnp.where(first, k2, k3)
                    re, im = jnp.where(first, k3, k2), pltpu.roll(up, 126, 1)
                    ny = jnp.where(lane0, im, up)
                    u = [ny[q * 16:(q + 1) * 16] for q in range(4)]
                    odd_lane = (lane & 1) == 1
                    nr = jnp.where(odd_lane, pltpu.roll(u[0] - u[2], 1, 1), u[0] + u[2] + (u[1] + u[3]) * sgn0)
                    ni = jnp.where(odd_lane, pltpu.roll((u[3] - u[1]) * sgn0, 1, 1), 0.0)
                    rows = pl.ds(pl.multiple_of(p * 64 + rs * 16, 16), 16)
                    c, sn = tv_ref[0, rows], tv_ref[1, rows]
                    put(ny_ref, 0, rs, nr * c + ni * sn, ni * c - nr * sn)
                    im = jnp.where(lane0, 0.0, im)
                else:
                    re, im = k1 + k2, (k3 - k1) * jnp.where(first, 1.0, -1.0)
                a = _dft4([(re[q * 16:(q + 1) * 16], im[q * 16:(q + 1) * 16]) for q in range(4)])
                for jq in range(4):
                    re, im = a[jq]
                    if jq > 0:
                        c, sn = cs[jq]
                        re, im = re * c + im * sn, im * c - re * sn
                    put(ub_ref, t * 4 + jq, rs, re, im)
        return item

    def p2_bfly(u, g, inverse, ref=ub_ref):
        def item(y):
            if y is not None:
                ub_ref[136, pin_rows(0), :] = y
            v = ref[pl.ds(u * 8, 8), g * 16:(g + 1) * 16]
            x = [(v[p, 0:8], v[p, 8:16]) for p in range(8)]
            x = _swap(_dft8(_swap(x))) if inverse else _dft8(x)
            ref[pl.ds(u * 8, 8), g * 16:(g + 1) * 16] = jnp.stack([w for c in x for w in c]).reshape(8, 16, 128)
        return item

    def filtered(xx, w):
        wr = pltpu.bitcast(w & jnp.uint32(0xFFFF0000), f32).reshape(8, 8, 128)
        wi = pltpu.bitcast(w << 16, f32).reshape(8, 8, 128)
        xx = xx.reshape(8, 2, 8, 128)
        xr, xi = xx[:, 0], xx[:, 1]
        return jnp.stack([xr * wr - xi * wi, xr * wi + xi * wr], axis=1).reshape(128, 128)

    def p2_fwd(u, jps):
        def item(y):
            t = u >> 2
            jq = u & 3
            xs = [_dot(_tobf(ms_ref[jq + 4 * jp]), ub_ref[u * 8 + jp].astype(bf16)) for jp in jps]
            for jp, xx in zip(jps, xs):
                ub_ref[u * 8 + jp] = filtered(xx, wp_ref[pl.ds(t * 2560 + jq + 4 * jp, 64, stride=40), :])
        return item

    def p2_nyq(u):
        def item(y):
            jp = u & 7
            rhs = ny_ref[jp].astype(bf16)
            xx = jnp.concatenate([_dot(_tobf(ms_ref[u * 4, m * 16:(m + 1) * 16]), rhs) for m in range(4)], axis=0)
            w = wp_ref[pl.ds(4 * 2560 + 4 * jp, 64, stride=40), :]
            for jq in range(1, 4):
                w = jnp.where(lane == jq, wp_ref[pl.ds(4 * 2560 + 4 * jp + jq, 64, stride=40), :], w)
            w = jnp.where(u < 8, w, jnp.uint32(0x3F800000))
            ny_ref[jp] = filtered(xx, w)
        return item

    def p2_inv(u, jps):
        def item(y):
            jq = u & 3
            zs = [_dot(_tobf(ms_ref[32 + jq + 4 * jp]), ub_ref[u * 8 + jp].astype(bf16)) for jp in jps]
            for jp, zz in zip(jps, zs):
                ub_ref[u * 8 + jp] = zz
        return item

    def p3_pre(p, g, t):
        def item(y):
            sa_ref[0, pin_rows(0), :] = y
            cs = twiddles(p)

            def fetch(t):
                a = []
                for jq in range(4):
                    v = ub_ref[(t * 4 + jq) * 8 + p, g * 16:(g + 1) * 16]
                    re, im = v[0:8], v[8:16]
                    if jq > 0:
                        c, sn = cs[jq]
                        re, im = re * c - im * sn, im * c + re * sn
                    a.append((re, im))
                return _swap(_dft4(_swap(a)))

            u = fetch(t)
            if t == 0:
                v = ny_ref[p, g * 16:(g + 1) * 16]
                rows = pl.ds(pl.multiple_of(p * 64 + g * 8, 8), 8)
                c, sn = tv_ref[0, rows], tv_ref[1, rows]
                nr, ni = v[0:8] * c - v[8:16] * sn, v[8:16] * c + v[0:8] * sn
                zr, zi = pltpu.roll(nr, 127, 1), pltpu.roll(ni, 127, 1)
                ny = (nr + zr, (nr - zi) * sgn0, nr - zr, (nr + zi) * sgn0)
            first = first_lanes(t)
            for q in range(4):
                re, im = u[q]
                rows = slice(q * 64 + g * 8, q * 64 + (g + 1) * 8)
                if t == 0:
                    im = pltpu.roll(jnp.where(lane0, ny[q], im), 2, 1) + jnp.where(lane == 2, ny[q], 0.0)
                    sa_ref[1:3, rows] = jnp.stack((jnp.where(first, im, re), jnp.where(first, re, im)))
                else:
                    im = im * jnp.where(first, 1.0, -1.0)
                    sa_ref[3 * t:3 * t + 3, rows] = jnp.stack((re + im, im, re))
        return item

    def p3_mm(p, q):
        def item(y):
            g = []
            for t in range(4):
                k1, k2, k3 = d_products(sa_ref, 1, t, slice(q * 64, (q + 1) * 64))
                g.append((k3, k2) if t == 0 else (k2 + k1, k3 - k1))
            yy = _r8_real_t(g)
            bx_ref[q, pl.ds(pl.multiple_of(p * 64, 64), 64), :] = jnp.concatenate(yy, axis=1).astype(bf16)
        return item

    def b_out(p):
        def item(y):
            rows = pl.ds(pl.multiple_of(p * 64, 64), 64)
            pltpu.make_async_copy(bx_ref.at[0:4, rows, :], out_hbm.at[:, rows, pl.ds(DM, DM)],
                                  sem_out.at[1]).start()
            bx_ref[4, pin_rows(0), 0:128] = y.astype(bf16)
        return item

    def a_out(blk, half):
        pltpu.make_async_copy(
            xo_ref.at[half, pl.ds(pl.multiple_of(blk * 64 + 64, 64), 64), :],
            out_hbm.at[blk >> 3, pl.ds(pl.multiple_of((blk & 7) * 64, 64), 64),
                       pl.ds(pl.multiple_of(half * 512, 512), 512)],
            sem_out.at[0]).start()

    def step(pp, odd, mem, hooks, first=False):
        r0 = pl.multiple_of(pp * 64 + (64 + 32 * odd), SEG)
        xs = jnp.concatenate([xo_ref[0, pl.ds(r0, SEG), :], xo_ref[1, pl.ds(r0, SEG), :]], axis=1)
        x_lo = xs[0:8].astype(f32)
        hm = jnp.concatenate(
            [jnp.concatenate([x_lo, jnp.concatenate(mem, axis=1)], axis=0).astype(bf16), xs[16:32]], axis=0)
        fill = fillo_ref[:, 0:64] if odd else fille_ref[:, 0:48]
        qkv, ps = {}, {}

        def head_of(v):
            return (v // 16) * 16 + (v % 2) * 8 + (v % 16) // 2 if odd else v

        def do_qkv(v0, v1):
            for v in range(v0, v1):
                h = head_of(v)
                for t in range(3):
                    n = t * H + slot_of(h)
                    y32 = _dot(hm, _tobf(w_refs[n // 16][n // 8 % 2, n % 8, 0:512]))
                    y = y32.astype(bf16)
                    parts = [y]
                    if odd or t > 0:
                        parts.append(_tobf(qkvc_ref[pp, n // 8, n % 8]))
                    if t > 0:
                        if odd:
                            parts.append(_tobf(kve_ref[(t - 1) * H + h]))
                        else:
                            kve_ref[(t - 1) * H + h] = _tou(y[0:16])
                    qkv[(t, v)] = jnp.concatenate(parts, axis=0) if len(parts) > 1 else y
                for item in hooks.get(v, ()):
                    item(y32[0:8])

        def do_s(g):
            for v in range(g * G, (g + 1) * G):
                sc = jax.lax.dot_general(qkv[(0, v)], qkv[(1, v)], (((1,), (1,)), ((), ())),
                                         preferred_element_type=f32)
                sc = jnp.where(fill == 0.0, sc * scale, fill)
                e = jnp.exp(sc - jnp.max(sc, axis=1, keepdims=True))
                den = jnp.sum(e, axis=1, keepdims=True)
                r = pl.reciprocal(den, approx=True)
                r = r * (2.0 - den * r)
                ps[v] = (e * r).astype(bf16)

        def do_pv(g):
            o = {v: _dot(ps[v], qkv[(2, v)]) for v in range(g * G, (g + 1) * G)}
            for v in o:
                h = head_of(v)
                oall_ref[:, h * DH:(h + 1) * DH] = _tou(o[v][0:32].astype(bf16))
            if odd:
                for v in range(g * G, (g + 1) * G, 2):
                    a11, a12 = o[v][0:32], o[v + 1][0:32]
                    a21 = jnp.concatenate([oc_ref[head_of(v)], o[v][32:48]], axis=0)
                    a22 = jnp.concatenate([oc_ref[head_of(v + 1)], o[v + 1][32:48]], axis=0)
                    for k, a in enumerate((a11 + a22, a21 + a22, a22, a11 + a12, a21 - a11, a12 - a22)):
                        os_ref[k, :, (v // 2) * DH:(v // 2 + 1) * DH] = a
                for v in o:
                    oc_ref[head_of(v)] = o[v][32:48]

        def plain(half, j, h0, h1):
            return _dot(_tobf(oall_ref[:, h0 * DH:h1 * DH]), _tobf(wo_ref[half, j, h0 * 64:h1 * 64, :]))

        hb = pp & 1
        if odd:
            def product(jp, k):
                def fn(part):
                    h0 = part * 16
                    if k == 2:
                        lhs = _tobf(oall_ref[:, h0 * DH:(h0 + 8) * DH])
                    else:
                        lhs = os_ref[k - (k > 2), :, part * 1024:(part + 1) * 1024].astype(bf16)
                    if k == 1:
                        rhs = wo_ref[hb, jp * 2, h0 * 64:(h0 + 8) * 64, :]
                    elif k == 4:
                        rhs = wo_ref[hb, jp * 2 + 1, (h0 + 8) * 64:(h0 + 16) * 64, :]
                    else:
                        rhs = ws_ref[hb, jp * 5 + (0, 0, 1, 2, 0, 3, 4)[k], part * 512:(part + 1) * 512, :]
                    return _dot(lhs, _tobf(rhs))
                return fn
            jobs = [product(jp, k) for jp in range(2) for k in range(7)]
            jobs += [(lambda part, j=j: plain(1 - hb, j, part * 16, part * 16 + 16)) for j in range(4)]
            marks = (2, 10)
        else:
            jobs = [(lambda part, j=j: plain(j // 4, j % 4, part * 24, 24 + part * 8)) for j in range(8)]
            marks = (2, 5)

        for g in range(NG):
            do_qkv(g * G, g * G + G // 2)
            if g >= 1:
                do_s(g - 1)
            do_qkv(g * G + G // 2, (g + 1) * G)
            if g >= 2:
                do_pv(g - 2)
        part = []
        for k, job in enumerate(jobs):
            items = hooks.get(('o', k), ())
            if len(items) == 2:
                half = plain(k // 4, k % 4, 0, 12)
                items[0](half[0:8])
                part.append(plain(k // 4, k % 4, 12, 24) + half)
                items[1](part[k][0:8])
            else:
                part.append(job(0))
                for item in items:
                    item(part[k][0:8])
            if k == marks[0]:
                do_s(NG - 1)
                do_pv(NG - 2)
            if k == marks[1]:
                do_pv(NG - 1)

        def finish(k):
            res = jobs[k](1) + part[k]
            for item in hooks.get(('p', k), ()):
                item(res[0:8])
            return res

        def put(half, j, r, v):
            xo_ref[half, pl.ds(r0 + r, v.shape[0]), j * 128:(j + 1) * 128] = v.astype(bf16)

        if odd:
            own = []
            for jp in range(2):
                m1, m2, m3, m4, m5, m6, m7 = [finish(jp * 7 + k) for k in range(7)]
                for jj, top, bot in ((0, ((m1 + m4) - m5) + m7, m2 + m4), (1, m3 + m5, ((m1 - m2) + m3) + m6)):
                    j = jp * 2 + jj
                    own.append(top[8:16])
                    put(hb, j, 0, jnp.concatenate([top[0:8], bot[24:32], top[16:32]], axis=0))
                    put(hb, j, -24, bot[16:24])
                    put(hb, j, -56, bot[8:16])
                    put(hb, j, -88, bot[0:8])
            for j in range(4):
                res = finish(14 + j)
                own.append(res[8:16])
                put(1 - hb, j, 0, res)
            new_mem = [jnp.where(hb == 0, own[j], own[(j + 4) % 8]) for j in range(8)]
        else:
            new_mem = []
            for j in range(8):
                res = finish(j)
                new_mem.append(res[8:16])
                put(j // 4, j % 4, 0, res)
        for item in hooks.get(H, ()):
            item(None)
        if odd:
            a_out(pp, hb)
            if first:
                pl.when(pp > 0)(lambda: a_out(pp - 1, hb))
            else:
                a_out(pp - 1, hb)
        return new_mem

    def l1(i, mem):
        bx_copy(i).wait()
        he = {2 * k: [p1_pre(i, k // 4, k % 4)] for k in range(16)}
        he[H] = [p1_mm(i, 1), p1_mm(i, 2), p1_mm(i, 3)]
        ho = {('p', 2): [p1_mm(i, 0)]}
        mem = step(i, 0, mem, he)
        mem = step(i, 1, mem, ho, first=True)
        return mem

    def l2(i, mem):
        u = i - N_L1
        he = {3: [p2_fwd(u, range(0, 4))], 7: [p2_fwd(u, range(4, 8))], 17: [p2_nyq(u)],
              H: [p2_inv(u, range(0, 8))]}
        ho = {('p', k): [p2_bfly(u + k % 2, k // 2, k % 2 == 0)] for k in range(16)}
        mem = step(i, 0, mem, he)
        mem = step(i, 1, mem, ho)
        return mem

    def l3(i, mem):
        p = i - N_L1 - N_L2
        he = {h: [p3_pre(p, h // 3, 1 + h % 3)] for h in range(24)}
        for j in range(4):
            he[('o', 3 + j)] = [p3_pre(p, 2 * j, 0), p3_pre(p, 2 * j + 1, 0)]
        he[H] = [p3_mm(p, q) for q in range(4)]
        ho = {12: [b_out(p)]}
        mem = step(i, 0, mem, he)
        mem = step(i, 1, mem, ho)
        return mem

    m0 = mem_ref[...].astype(f32)
    mem = [m0[:, j * 128:(j + 1) * 128] for j in range(8)]
    mem = jax.lax.fori_loop(0, N_L1, l1, mem)
    cp_x[2].wait()
    cp_x[3].wait()
    cp_ms.wait()
    for g in range(8):
        p2_bfly(0, g, False)(None)
        p2_bfly(0, g, False, ny_ref)(None)
    mem = jax.lax.fori_loop(N_L1, N_L1 + N_L2, l2, mem)
    for g in range(8):
        p2_bfly(0, g, True, ny_ref)(None)
    mem = jax.lax.fori_loop(N_L1 + N_L2, NSEG // 2, l3, mem)

    oc_last = jnp.concatenate([oc_ref[h] for h in range(H)], axis=1).astype(bf16)
    for j in range(4):
        res = _dot(oc_last, _tobf(wo_ref[0, j, 0:2048, :])).astype(bf16)
        xo_ref[0, S + 8:S + 16, j * 128:(j + 1) * 128] = res[0:8]
        xo_ref[0, S + 40:S + 48, j * 128:(j + 1) * 128] = res[8:16]
    a_out(NSEG // 2 - 1, 0)

    pltpu.make_async_copy(bx_ref.at[0:4], out_hbm.at[:, :, pl.ds(DM, DM)], sem_out.at[1]).wait()
    pltpu.make_async_copy(xo_ref.at[:, 64:64 + S], xo_ref.at[:, 64:64 + S], sem_out.at[0]).wait()


@jax.jit
def _run(x, mem0, wq, wk, wv, wo, bx, w_r, w_i):
    fd, ms, tv = _tables()
    hbm = pl.BlockSpec(memory_space=pl.ANY)
    out = pl.pallas_call(
        _kernel,
        out_shape=jax.ShapeDtypeStruct((4, S // 4, 2 * DM), bf16),
        in_specs=[hbm] * 13,
        out_specs=hbm,
        scratch_shapes=[
            pltpu.VMEM((2, 64 + S, DM // 2), bf16),
            pltpu.VMEM((MEM, DM), bf16),
            pltpu.VMEM((8, NSEG, 8, 128), bf16),
            pltpu.VMEM((4, DM, 16, DH), bf16),
        ] + [pltpu.VMEM((2, 8, DM // 2 + 8, DH), u32)] * 6 + [
            pltpu.VMEM((2, 4, H * DH // 2 + 8, 128), u32),
            pltpu.VMEM((8, 256, 128), u32),
            pltpu.VMEM((5, 4, 136, 128), u32),
            pltpu.VMEM((NSEG // 2, 12, 8, 8, 128), u32),
            pltpu.VMEM((2 * H, 8, 128), u32),
            pltpu.VMEM((16, H * DH), u32),
            pltpu.VMEM((H, 16, DH), f32),
            pltpu.VMEM((6, 32, 16 * DH), f32),
            pltpu.VMEM((2, 10, 1040, 128), u32),
            pltpu.VMEM((32, 128), f32),
            pltpu.VMEM((48, 128), f32),
            pltpu.VMEM((5, S // 4, DM), bf16),
            pltpu.VMEM((2, 8, DM // 2 + 1, 256), bf16),
            pltpu.VMEM((12872, 128), u32),
            pltpu.VMEM((137, 128, 128), f32),
            pltpu.VMEM((8, 128, 128), f32),
            pltpu.VMEM((12, 264, 128), f32),
            pltpu.VMEM((24, 64, 128), u32),
            pltpu.VMEM((64, 64, 128), u32),
            pltpu.VMEM((2, 512, 128), f32),
            pltpu.SMEM((64,), f32),
            pltpu.SMEM((1,), jnp.int32),
            pltpu.SemaphoreType.DMA((84,)),
            pltpu.SemaphoreType.DMA((2,)),
        ],
        compiler_params=pltpu.CompilerParams(vmem_limit_bytes=120 * 1024 * 1024,
                                             disable_semaphore_checks=True,
                                             disable_bounds_checks=True),
    )(x.reshape(S, DM), x.reshape(NSEG, SEG, DM), mem0.reshape(MEM, DM), wq, wk, wv,
      wo.reshape(H * DH // 16, 16, DM), bx.reshape(4, S // 4, DM), w_r.T, w_i.T, jnp.asarray(fd), jnp.asarray(ms), jnp.asarray(tv))
    return out.reshape(1, S, 2 * DM)


def pallas_concat_heads__memory_aug_recurrent_mem_tr__spectral_gfnet__prompt_kernel(
    A_x: jax.Array,
    A_mem0: jax.Array,
    A_Wq: jax.Array,
    A_Wk: jax.Array,
    A_Wv: jax.Array,
    A_Wo: jax.Array,
    A_seg_len,
    B_x: jax.Array,
    B_w_r: jax.Array,
    B_w_i: jax.Array,
):
    if isinstance(A_seg_len, int):
        assert A_seg_len == SEG
    assert A_x.shape == (1, S, DM) and A_mem0.shape == (1, MEM, DM) and A_Wq.shape == (DM, H, DH)
    assert B_x.shape == (1, S, DM) and B_w_r.shape == (S, DM // 2 + 1)
    return _run(A_x, A_mem0, A_Wq, A_Wk, A_Wv, A_Wo, B_x, B_w_r, B_w_i)
```

```python
import math

import numpy as np
import jax
import jax.numpy as jnp
import jax.experimental.pallas as pl
import jax.experimental.pallas.tpu as pltpu

bf16 = jnp.bfloat16
f32 = jnp.float32
u32 = jnp.uint32

S, DM = 2048, 1024
H, DH = 32, 128
MEM, SEG = 8, 32
NSEG = S // SEG
SQH = math.sqrt(0.5)

_PAIRS = ((0, 4), (1, 7), (2, 6), (3, 5))
_FIRST = np.array([[1, 1, 0, 0], [1, 0, 1, 0], [0, 1, 1, 0], [0, 1, 0, 1]], bool)


def _pack_rows(a):
    u = np.ascontiguousarray(a, dtype=np.float32).view(np.uint32).astype(np.uint64)
    b = ((u + 0x7FFF + ((u >> 16) & 1)) >> 16).astype(np.uint32)
    return (b[..., 0::2, :] | (b[..., 1::2, :] << 16)).astype(np.uint32)


def _tables():
    k2 = np.zeros((4, 128), np.int64)
    for t in range(4):
        odd = t % 2
        for lam in range(128):
            k = 2 * lam + odd
            if k % 8 not in _PAIRS[t]:
                k = 2 * (128 + 8 * (lam // 8) + (lam % 8 - 1 - odd) % 8) + odd
            assert k % 8 in _PAIRS[t]
            k2[t, lam] = k
    b = np.arange(128)[:, None]
    F = np.zeros((12, 128, 128))
    G = np.zeros((12, 128, 128))
    for t in range(4):
        th = 2 * np.pi * ((b * k2[t][None, :]) % DM) / DM
        C, Sn = np.cos(th), np.sin(th)
        first = ((k2[t] % 8) == _PAIRS[t][0])[None, :]
        assert np.array_equal(first[0], _FIRST[t][np.arange(128) % 4])
        if t == 0:
            im = -Sn
            im[:, 0] = (-1.0) ** np.arange(128)
            im = np.roll(im, 2, axis=1)
            F[1:3] = np.where(first, im, C), np.where(first, C, im)
            G[1:3] = F[1:3]
            G[2, :, 0] *= 0.5
            G[2, :, 2] *= 0.5
        else:
            Sg = np.where(first, Sn, -Sn)
            F[3 * t:3 * t + 3] = C, -(C + Sg), C - Sg
            G[3 * t:3 * t + 3] = F[3 * t:3 * t + 3]
    Finv = np.transpose(G, (0, 2, 1)) * (2.0 / DM)
    fd = _pack_rows(np.concatenate([F, Finv]))
    M = np.zeros((32, 128, 128))
    r = np.arange(64)[None, :]
    l = np.arange(64)[:, None]
    for j in range(32):
        th = 2 * np.pi * ((r * (j + 32 * l)) % S) / S
        C, Sn = np.cos(th), np.sin(th)
        M[j, :64, :64] = C
        M[j, :64, 64:] = Sn
        M[j, 64:, :64] = -Sn
        M[j, 64:, 64:] = C
    perm = np.arange(128).reshape(2, 8, 8).transpose(1, 0, 2).reshape(128)
    M = M[:, perm][:, :, perm]
    Minv = np.transpose(M, (0, 2, 1)) / S
    ms = _pack_rows(np.concatenate([M, Minv]))
    th = 2 * np.pi * np.outer(np.arange(512), np.arange(128) % 4) / S
    tv = np.stack([np.cos(th), np.sin(th)]).astype(np.float32)
    return fd, ms, tv


def _tobf(w):
    return pltpu.bitcast(w, bf16)


def _tou(w):
    return pltpu.bitcast(w, u32)


def _dot(a, b):
    return jnp.dot(a, b, preferred_element_type=f32)


def _r8_real(x):
    t0, t1 = x[0] + x[4], x[0] - x[4]
    t2, t3 = x[2] + x[6], x[2] - x[6]
    t4, t5 = x[1] + x[5], x[1] - x[5]
    t6, t7 = x[3] + x[7], x[3] - x[7]
    e0, e1 = t0 + t2, t0 - t2
    o0, o1 = t4 + t6, t4 - t6
    u, v = SQH * (t5 - t7), SQH * (t5 + t7)
    return [(e0 + o0, e0 - o0), (t1 + u, v + t3), (e1, o1), (t1 - u, v - t3)]


def _r8_real_t(g):
    (z0, z4), (a1, b1), (e1, o1), (a3, b3) = g
    e0, o0 = z0 + z4, z0 - z4
    t1, u = a1 + a3, a1 - a3
    v, t3 = b1 + b3, b1 - b3
    t5, t7 = SQH * (v + u), SQH * (v - u)
    t0, t2 = e0 + e1, e0 - e1
    t4, t6 = o0 + o1, o0 - o1
    return [t0 + t1, t4 + t5, t2 + t3, t6 + t7, t0 - t1, t4 - t5, t2 - t3, t6 - t7]


def _dft4(u):
    (r0, i0), (r1, i1), (r2, i2), (r3, i3) = u
    sr, si, dr, di = r0 + r2, i0 + i2, r0 - r2, i0 - i2
    tr, ti, er, ei = r1 + r3, i1 + i3, r1 - r3, i1 - i3
    return [(sr + tr, si + ti), (dr + ei, di - er), (sr - tr, si - ti), (dr - ei, di + er)]


def _dft8(x):
    a = [(x[p][0] + x[p + 4][0], x[p][1] + x[p + 4][1]) for p in range(4)]
    d = [(x[p][0] - x[p + 4][0], x[p][1] - x[p + 4][1]) for p in range(4)]
    ev = _dft4(a)
    (r0, i0), (r1, i1), (r2, i2), (r3, i3) = d
    b1r, b1i = SQH * (r1 + i1), SQH * (i1 - r1)
    b3r, n3i = SQH * (i3 - r3), SQH * (r3 + i3)
    sr, si, dr, di = r0 + i2, i0 - r2, r0 - i2, i0 + r2
    tr, ti, er, ei = b1r + b3r, b1i - n3i, b1r - b3r, b1i + n3i
    od = [(sr + tr, si + ti), (dr + ei, di - er), (sr - tr, si - ti), (dr - ei, di + er)]
    return [ev[0], od[0], ev[1], od[1], ev[2], od[2], ev[3], od[3]]


def _swap(x):
    return [(b, a) for (a, b) in x]


G = 4
NG = H // G
NEG = -1e9
N_L1, N_L2, N_L3 = 8, 16, 8


def _kernel(x_hbm, x3_hbm, mem_hbm, wq_hbm, wk_hbm, wv_hbm, wo_hbm, bx_hbm, wr_hbm, wi_hbm,
            fd_hbm, ms_hbm, tv_hbm, out_hbm,
            xo_ref, mem_ref, xcraw_ref, raw_ref, w0_ref, w1_ref, w2_ref, w3_ref, w4_ref, w5_ref,
            wo_ref, xc_ref, xs_ref, qkvc_ref, kve_ref,
            oall_ref, oc_ref, os_ref, ws_ref, fille_ref, fillo_ref, bx_ref, wt_ref, wp_ref, ub_ref, ny_ref, sa_ref, fd_ref, ms_ref, tv_ref,
            tw_ref, zero_ref, sem_in, sem_out):
    scale = DH ** -0.5
    w_hbm = (wq_hbm, wk_hbm, wv_hbm)
    w_refs = (w0_ref, w1_ref, w2_ref, w3_ref, w4_ref, w5_ref)

    def raw_copy(c, i=0, nd=DM):
        rows = pl.ds(pl.multiple_of(i * nd, nd), nd)
        return pltpu.make_async_copy(
            w_hbm[c // 2].at[rows, pl.ds((c % 2) * 16, 16), :],
            raw_ref.at[c % 4, rows], sem_in.at[8 + min(c, 3) * 8 + max(c - 3, 0) * 2 + i])

    def xc_copy(k):
        return pltpu.make_async_copy(
            x3_hbm.at[:, pl.ds(8, 8), pl.ds(pl.multiple_of(k * 128, 128), 128)], xcraw_ref.at[k], sem_in.at[40 + k])

    def wo_copies(half):
        return [pltpu.make_async_copy(wo_hbm.at[:, :, pl.ds(pl.multiple_of(half * 512 + j * 128, 128), 128)],
                                      raw_ref.at[2 + half, j * 256:(j + 1) * 256], sem_in.at[76 + half * 4 + j])
                for j in range(4)]

    def wt_copies(i):
        return [pltpu.make_async_copy(src.at[:, pl.ds(pl.multiple_of(i * 1024 + k * 256, 256), 256)],
                                      wt_ref.at[i, a * 4 + k], sem_in.at[i * 4 + (48 + a * 8 + k)])
                for k in range(4) for a, src in enumerate((wr_hbm, wi_hbm))]

    def bx_copy(p):
        rows = pl.ds(pl.multiple_of(p * 64, 64), 64)
        return pltpu.make_async_copy(bx_hbm.at[:, rows, :], bx_ref.at[0:4, rows, :], sem_in.at[64 + p])

    n_head = N_L1 * 2 * SEG
    cp_x = [pltpu.make_async_copy(x_hbm.at[lo:hi, half * 512:(half + 1) * 512], xo_ref.at[half, 64 + lo:64 + hi],
                                  sem_in.at[72 + (lo > 0) * 2 + half])
            for lo, hi in ((0, n_head), (n_head, S)) for half in range(2)]
    cp_mem = pltpu.make_async_copy(mem_hbm, mem_ref, sem_in.at[1])
    cp_fd = pltpu.make_async_copy(fd_hbm, fd_ref, sem_in.at[4])
    cp_ms = pltpu.make_async_copy(ms_hbm, ms_ref, sem_in.at[5])
    cp_tv = pltpu.make_async_copy(tv_hbm, tv_ref, sem_in.at[6])

    for i in range(8):
        raw_copy(0, i, 128).start()
        xc_copy(i).start()
        if i >= 4:
            raw_copy(2, i - 4, 192).start()
        raw_copy(1, i, 128).start()
    raw_copy(2, 6, 128).start()
    raw_copy(2, 7, 128).start()
    for i in range(2):
        raw_copy(3, i, 512).start()

    zero_ref[0] = 0

    def pin_bit():
        return jnp.clip(zero_ref[0], 0, 1)

    def pin_rows(r):
        return pl.ds(pl.multiple_of(r + pin_bit() * 32, 8), 8)

    for p in range(8):
        for jq in range(4):
            tw_ref[(p * 4 + jq) * 2] = jnp.float32(math.cos(2 * math.pi * p * jq / 32))
            tw_ref[(p * 4 + jq) * 2 + 1] = jnp.float32(math.sin(2 * math.pi * p * jq / 32))

    ub_ref[128:136] = jnp.zeros((8, 128, 128), f32)
    wp_ref[12800:12872] = jnp.zeros((72, 128), u32)
    oc_ref[...] = jnp.zeros((H, 16, DH), f32)

    qi = jax.lax.broadcasted_iota(jnp.int32, (48, 128), 0)
    ki = jax.lax.broadcasted_iota(jnp.int32, (48, 128), 1)

    def between(v, lo, hi):
        return (v >= lo) & (v < hi)

    def table(keep, other):
        return jnp.where(other, -jnp.inf, jnp.where(keep, 0.0, NEG)).astype(f32)

    keep = between(qi, 8, 16) | between(ki, 8, 16) | (qi >= jnp.where(ki < 32, ki, ki - 24))
    fille_ref[...] = table(keep, ki >= 40)[:32]
    q_even = between(qi, 32, 40)
    k_even = between(ki, 32, 40) | (ki >= 48)
    qpos = jnp.where(qi < 32, qi, jnp.where(qi < 40, qi - 24, qi - 32))
    kpos = jnp.where(ki < 32, ki, jnp.where(ki < 40, ki - 24, jnp.where(ki < 48, ki - 32, ki - 48)))
    keep = between(qi, 8, 16) | between(ki, 8, 16) | (ki >= 56) | (qpos >= kpos)
    fillo_ref[...] = table(keep, (q_even != k_even) | (ki >= 64))

    def relayout16(c, blk):
        w0 = pl.multiple_of(blk * 8, 8)
        v = _tou(raw_ref[c % 4, pl.ds(blk * 16, 16)]).reshape(8, 2, 8, 128)
        a, b = v[:, 0], v[:, 1]
        w_refs[c][0, :, pl.ds(w0, 8), :] = jnp.swapaxes((a & jnp.uint32(0xFFFF)) | (b << 16), 0, 1)
        w_refs[c][1, :, pl.ds(w0, 8), :] = jnp.swapaxes((a >> 16) | (b & jnp.uint32(0xFFFF0000)), 0, 1)

    def slot_of(h):
        return (h // 16) * 16 + (h % 2) * 8 + (h % 16) // 2

    def repack_wo(half, part, k):
        jp, g0 = k & 1, part * 128 + (k >> 1) * 2
        quad = []
        for jj in range(2):
            for kh in range(2):
                v = _tou(raw_ref[2 + half, pl.ds((jp * 2 + jj) * 256 + kh * 64 + g0, 2)]).reshape(16, 128)
                wo_ref[half, jp * 2 + jj, pl.ds(pl.multiple_of(g0 * 8 + kh * 512, 16), 16), :] = v
                quad.append(_tobf(v).astype(f32))
        b11, b21, b12, b22 = quad
        rows = pl.ds(pl.multiple_of(part * 512 + (k >> 1) * 16, 16), 16)
        for n, v in enumerate((b11 + b22, b12 - b22, b21 - b11, b11 + b12, b21 + b22)):
            ws_ref[half, jp * 5 + n, rows, :] = _tou(v.astype(bf16))

    sub4 = jax.lax.broadcasted_iota(jnp.int32, (128, 128), 0) & 3

    def wp_store(t, kb, tile):
        v = tile.T.reshape(4, 32, 128)
        v = jnp.concatenate([v, v[:, 0:8]], axis=1).reshape(160, 128)
        wp_ref[pl.ds(pl.multiple_of(t * 2560 + kb * 160, 32), 160), :] = v

    def b_prep(i, k, hb, par):
        cols = slice(hb * 128, (hb + 1) * 128)
        a = _tou(wt_ref[i, k, 0:512, cols])
        b = _tou(wt_ref[i, 4 + k, 0:512, cols])
        if par == 0:
            w = (a << 16) | (b & jnp.uint32(0xFFFF))
            m = (sub4 == 0) | (sub4 == 2)
        else:
            w = (a & jnp.uint32(0xFFFF0000)) | (b >> 16)
            m = (sub4 == 0) | (sub4 == 3)
        top = w[:128]
        bot = pltpu.roll(w[128:].reshape(16, 8, 128), 1 + par, 1).reshape(128, 128)
        wp_store(par, i * 8 + (k * 2 + hb), jnp.where(m, top, bot))
        wp_store(par + 2, i * 8 + (k * 2 + hb), jnp.where(m, bot, top))
        if par == 0:
            na = jnp.broadcast_to(wt_ref[i, k, 512:513, cols].astype(f32), (128, 128))
            nb = jnp.broadcast_to(wt_ref[i, 4 + k, 512:513, cols].astype(f32), (128, 128))
            wp_store(4, i * 8 + (k * 2 + hb), pltpu.bitcast(na, u32) | (pltpu.bitcast(nb, u32) >> 16))

    def gather_c(k):
        xc_ref[k] = _tou(xcraw_ref[k].astype(f32).reshape(512, 128).astype(bf16))

    def store_qkvc(n, y):
        qkvc_ref[:, n // 8, n % 8] = y.reshape(NSEG // 2, 8, 128)

    def q_unit(i, groups, first, last, fillers):
        xk = _tobf(xc_ref[i])
        w0 = pl.multiple_of(i * 64, 64)
        for g in groups:
            rhs = jnp.concatenate(
                [_tobf(w_refs[h // 16][h // 8 % 2, h % 8, pl.ds(w0, 64), :]) for h in range(4 * g, 4 * g + 4)], axis=1)
            y = _dot(xk, rhs)
            for h in range(4 * g, 4 * g + 4):
                yh = y[:, (h % 4) * 128:(h % 4 + 1) * 128]
                if not first:
                    yh = yh + ub_ref[h * 4:(h + 1) * 4].reshape(512, 128)
                if last:
                    store_qkvc(h, _tou(yh.astype(bf16)))
                else:
                    ub_ref[h * 4:(h + 1) * 4] = yh.reshape(4, 128, 128)
            mine = fillers.get(g, [])
            for fi, item in enumerate(mine):
                r = (fi * 512 // len(mine)) // 8 * 8
                item(pltpu.bitcast(y[r:r + 8, 0:128], u32))

    def rl_item(c, blk):
        def item(pin):
            w_refs[c][pin_bit(), 7, 512:520] = pin
            relayout16(c, blk)
        return item

    def spread(fillers, items, groups):
        for k, item in enumerate(items):
            fillers.setdefault(groups[k * len(groups) // len(items)], []).append(item)
        return fillers

    def half_items(f, c, i, groups):
        return spread(f, [rl_item(c, i * 8 + blk) for blk in range(8)], groups)

    def piece_items(i):
        f = half_items(half_items({}, 1, i, (0, 1, 2)), 0, i + 1, (4, 5, 6))
        return spread(f, [lambda pin: gather_c(i + 1)], (7,))

    def chunk2_items(f, lo, hi, groups):
        return spread(f, [rl_item(2, blk) for blk in range(lo, hi)], groups)

    def wait_piece(i):
        raw_copy(1, i, 128).wait()
        raw_copy(0, i + 1, 128).wait()
        xc_copy(i + 1).wait()

    raw_copy(0, 0, 128).wait()
    for blk in range(8):
        relayout16(0, blk)
    xc_copy(0).wait()
    gather_c(0)
    q_unit(0, range(0, 2), True, False, {})
    raw_copy(1, 0, 128).wait()
    q_unit(0, range(2, 4), True, False, half_items({}, 1, 0, (2, 2, 3)))
    q_unit(0, range(4, 6), True, False, {})
    xc_copy(1).wait()
    raw_copy(0, 1, 128).wait()
    q_unit(0, range(6, 8), True, False,
           spread(half_items({}, 0, 1, (6, 6, 7)), [lambda pin: gather_c(1)], (6,)))
    raw_copy(1, 1, 128).wait()
    q_unit(1, range(0, 4), False, False, half_items({}, 1, 1, (0, 1, 2)))
    xc_copy(2).wait()
    raw_copy(0, 2, 128).wait()
    q_unit(1, range(4, 8), False, False,
           spread(half_items({}, 0, 2, (4, 5, 6)), [lambda pin: gather_c(2)], (6,)))

    def xsum_item(j, rq):
        def item(pin):
            xs_ref[pin_bit(), 0, 128:136] = pin
            a11, a21, a12, a22 = [
                xcraw_ref[j + 4 * kh, rh * 32 + rq * 8:rh * 32 + (rq + 1) * 8].astype(f32).reshape(64, 128)
                for kh in range(2) for rh in range(2)]
            for k, v in enumerate((a11 + a22, a21 + a22, a11 + a12, a21 - a11, a12 - a22)):
                xs_ref[k, j, rq * 32:(rq + 1) * 32] = _tou(v.astype(bf16))
        return item

    wait_piece(2)
    q_unit(2, range(8), False, False, piece_items(2))

    def q_c(i, carry):
        wait_piece(i)
        raw_copy(2, i - 3, 192).wait()
        f = spread(piece_items(i), [rl_item(2, (i - 3) * 12 + blk) for blk in range(12)],
                   (2, 3, 3, 3, 3, 3, 4, 4, 5, 6, 6, 7))
        q_unit(i, range(8), False, False, spread(f, [xsum_item(i - 3, rq) for rq in range(4)], (3, 4, 5, 6)))
        return carry
    jax.lax.fori_loop(3, 7, q_c, 0)

    raw_copy(1, 7, 128).wait()
    raw_copy(2, 6, 128).wait()
    raw_copy(2, 7, 128).wait()
    q_unit(7, range(8), False, True, chunk2_items(half_items({}, 1, 7, (0, 1, 2)), 48, 64, (3, 4, 5, 6)))
    raw_copy(4).start()
    for cp in wo_copies(0):
        cp.start()
    raw_copy(5).start()

    def bulk_iter(c, i):
        def xs(k):
            return jnp.concatenate([_tobf(xs_ref[k, j, 0:128]) for j in range(4)], axis=1)

        def xc(rh, kh):
            return jnp.concatenate(
                [_tobf(xc_ref[4 * kh + j, rh * 128:(rh + 1) * 128]) for j in range(4)], axis=1)

        for pr in range(4):
            n1, n2 = pr * 2, pr * 2 + 1

            def w(n, kh):
                return _tobf(w_refs[c][i, n, kh * 256:(kh + 1) * 256])

            def wsum(a, b, sign):
                a, b = a.astype(f32), b.astype(f32)
                return (a + b if sign > 0 else a - b).astype(bf16)

            def out(rh, n, v):
                qkvc_ref[rh * 16:(rh + 1) * 16, c * 2 + i, n] = _tou(v.astype(bf16)).reshape(16, 8, 128)

            def side(k, m):
                blks = (k, 7) if k == 0 else (k,)
                items = []
                if c < 5:
                    items += [('w', blk) for blk in blks]
                if c >= 4:
                    items += [('o', blk) for blk in range(k * 16 // 7, (k + 1) * 16 // 7)]
                if c == 5 and k in (1, 2, 4, 5):
                    items.append(('f', (1, 2, 4, 5).index(k)))
                for n, (kind, blk) in enumerate(items):
                    r = n * 256 // len(items) // 8 * 8
                    pin = pltpu.bitcast(m[r:r + 8], u32)
                    if kind == 'w':
                        w_refs[c + 1][pin_bit(), 7, 512:520] = pin
                        relayout16(c + 1, i * 32 + (pr * 8 + blk))
                    elif kind == 'o':
                        ws_ref[pin_bit(), 9, 1024:1032] = pin
                        wo_ref[pin_bit(), 3, 2048:2056] = pin
                        repack_wo(c - 4, i, pr * 16 + blk)
                    else:
                        wp_ref[pin_rows(12832), :] = pin
                        b_prep(i, pr, blk // 2, blk % 2)

            m2 = _dot(xs(1), w(n1, 0))
            side(0, m2)
            m4 = _dot(xc(1, 1), wsum(w(n1, 1), w(n1, 0), -1))
            side(1, m4)
            out(1, n1, m4 + m2)
            m1 = _dot(xs(0), wsum(w(n1, 0), w(n2, 1), 1))
            side(2, m1)
            m5 = _dot(xs(2), w(n2, 1))
            side(3, m5)
            m3 = _dot(xc(0, 0), wsum(w(n2, 0), w(n2, 1), -1))
            side(4, m3)
            out(0, n2, m3 + m5)
            c22 = _dot(xs(3), wsum(w(n1, 0), w(n2, 0), 1)) + ((m1 - m2) + m3)
            side(5, c22)
            out(1, n2, c22)
            c11 = _dot(xs(4), wsum(w(n1, 1), w(n2, 1), 1)) + ((m1 + m4) - m5)
            side(6, c11)
            out(0, n1, c11)

    for c in range(2, 6):
        if c == 3:
            for cp in wo_copies(1) + wt_copies(0) + wt_copies(1):
                cp.start()
        if c == 4:
            for cp in cp_x[0:2] + [cp_mem, cp_fd, cp_tv] + [bx_copy(p) for p in range(8)] + cp_x[2:4] + [cp_ms]:
                cp.start()
        if c >= 4:
            for cp in wo_copies(c - 4):
                cp.wait()
        if 2 < c < 5:
            raw_copy(c + 1).wait()

        def bulk(i, carry, c=c):
            if c == 2:
                raw_copy(3, i, 512).wait()
            if c == 5:
                for cp in wt_copies(i):
                    cp.wait()
            bulk_iter(c, i)
            return carry
        jax.lax.fori_loop(0, 2, bulk, 0)

    cp_x[0].wait()
    cp_x[1].wait()
    cp_mem.wait()
    cp_fd.wait()
    cp_tv.wait()

    lane = jax.lax.broadcasted_iota(jnp.int32, (1, 128), 1)
    lane0 = lane == 0
    sgn0 = jnp.where(lane0, 1.0, -1.0)

    def first_lanes(t):
        la, lb = [k for k in range(4) if _FIRST[t][k]]
        return ((lane & 3) == la) | ((lane & 3) == lb)

    def d_products(st_ref, d, t, rows):
        return [_dot(st_ref[n, rows].astype(bf16), _tobf(fd_ref[d * 12 + n])) if n else None
                for n in range(3 * t, 3 * t + 3)]

    def twiddles(p):
        return [(tw_ref[p * 8 + jq * 2], tw_ref[p * 8 + jq * 2 + 1]) if jq else None for jq in range(4)]

    def p1_pre(p, rs, q):
        def item(y):
            sa_ref[0, pin_rows(0), :] = y
            xq = bx_ref[q, pl.ds(pl.multiple_of(p * 64 + rs * 16, 16), 16), :].astype(f32)
            zz = _r8_real([xq[:, a * 128:(a + 1) * 128] for a in range(8)])
            r = (rs * 4 + q) * 16
            sa_ref[1:12, r:r + 16] = jnp.stack([v for (a, b) in zz for v in (a + b, b, a)][1:])
        return item

    def p1_mm(p, t):
        def item(y):
            cs = twiddles(p)

            def put(ref, n, rs, re, im):
                v = jnp.stack([re.reshape(2, 8, 128), im.reshape(2, 8, 128)], axis=1)
                ref[n * 8 + p, rs * 32:(rs + 1) * 32] = v.reshape(32, 128)

            first = first_lanes(t)
            for rs in range(4):
                k1, k2, k3 = d_products(sa_ref, 0, t, slice(rs * 64, (rs + 1) * 64))
                if t == 0:
                    up = jnp.where(first, k2, k3)
                    re, im = jnp.where(first, k3, k2), pltpu.roll(up, 126, 1)
                    ny = jnp.where(lane0, im, up)
                    u = [ny[q * 16:(q + 1) * 16] for q in range(4)]
                    odd_lane = (lane & 1) == 1
                    nr = jnp.where(odd_lane, pltpu.roll(u[0] - u[2], 1, 1), u[0] + u[2] + (u[1] + u[3]) * sgn0)
                    ni = jnp.where(odd_lane, pltpu.roll((u[3] - u[1]) * sgn0, 1, 1), 0.0)
                    rows = pl.ds(pl.multiple_of(p * 64 + rs * 16, 16), 16)
                    c, sn = tv_ref[0, rows], tv_ref[1, rows]
                    put(ny_ref, 0, rs, nr * c + ni * sn, ni * c - nr * sn)
                    im = jnp.where(lane0, 0.0, im)
                else:
                    re, im = k1 + k2, (k3 - k1) * jnp.where(first, 1.0, -1.0)
                a = _dft4([(re[q * 16:(q + 1) * 16], im[q * 16:(q + 1) * 16]) for q in range(4)])
                for jq in range(4):
                    re, im = a[jq]
                    if jq > 0:
                        c, sn = cs[jq]
                        re, im = re * c + im * sn, im * c - re * sn
                    put(ub_ref, t * 4 + jq, rs, re, im)
        return item

    def p2_bfly(u, g, inverse, ref=ub_ref):
        def item(y):
            if y is not None:
                ub_ref[136, pin_rows(0), :] = y
            v = ref[pl.ds(u * 8, 8), g * 16:(g + 1) * 16]
            x = [(v[p, 0:8], v[p, 8:16]) for p in range(8)]
            x = _swap(_dft8(_swap(x))) if inverse else _dft8(x)
            ref[pl.ds(u * 8, 8), g * 16:(g + 1) * 16] = jnp.stack([w for c in x for w in c]).reshape(8, 16, 128)
        return item

    def filtered(xx, w):
        wr = pltpu.bitcast(w & jnp.uint32(0xFFFF0000), f32).reshape(8, 8, 128)
        wi = pltpu.bitcast(w << 16, f32).reshape(8, 8, 128)
        xx = xx.reshape(8, 2, 8, 128)
        xr, xi = xx[:, 0], xx[:, 1]
        return jnp.stack([xr * wr - xi * wi, xr * wi + xi * wr], axis=1).reshape(128, 128)

    def p2_fwd(u, jps):
        def item(y):
            t = u >> 2
            jq = u & 3
            xs = [_dot(_tobf(ms_ref[jq + 4 * jp]), ub_ref[u * 8 + jp].astype(bf16)) for jp in jps]
            for jp, xx in zip(jps, xs):
                ub_ref[u * 8 + jp] = filtered(xx, wp_ref[pl.ds(t * 2560 + jq + 4 * jp, 64, stride=40), :])
        return item

    def p2_nyq(u):
        def item(y):
            jp = u & 7
            rhs = ny_ref[jp].astype(bf16)
            xx = jnp.concatenate([_dot(_tobf(ms_ref[u * 4, m * 16:(m + 1) * 16]), rhs) for m in range(4)], axis=0)
            w = wp_ref[pl.ds(4 * 2560 + 4 * jp, 64, stride=40), :]
            for jq in range(1, 4):
                w = jnp.where(lane == jq, wp_ref[pl.ds(4 * 2560 + 4 * jp + jq, 64, stride=40), :], w)
            w = jnp.where(u < 8, w, jnp.uint32(0x3F800000))
            ny_ref[jp] = filtered(xx, w)
        return item

    def p2_inv(u, jps):
        def item(y):
            jq = u & 3
            zs = [_dot(_tobf(ms_ref[32 + jq + 4 * jp]), ub_ref[u * 8 + jp].astype(bf16)) for jp in jps]
            for jp, zz in zip(jps, zs):
                ub_ref[u * 8 + jp] = zz
        return item

    def p3_pre(p, g, t):
        def item(y):
            sa_ref[0, pin_rows(0), :] = y
            cs = twiddles(p)

            def fetch(t):
                a = []
                for jq in range(4):
                    v = ub_ref[(t * 4 + jq) * 8 + p, g * 16:(g + 1) * 16]
                    re, im = v[0:8], v[8:16]
                    if jq > 0:
                        c, sn = cs[jq]
                        re, im = re * c - im * sn, im * c + re * sn
                    a.append((re, im))
                return _swap(_dft4(_swap(a)))

            u = fetch(t)
            if t == 0:
                v = ny_ref[p, g * 16:(g + 1) * 16]
                rows = pl.ds(pl.multiple_of(p * 64 + g * 8, 8), 8)
                c, sn = tv_ref[0, rows], tv_ref[1, rows]
                nr, ni = v[0:8] * c - v[8:16] * sn, v[8:16] * c + v[0:8] * sn
                zr, zi = pltpu.roll(nr, 127, 1), pltpu.roll(ni, 127, 1)
                ny = (nr + zr, (nr - zi) * sgn0, nr - zr, (nr + zi) * sgn0)
            first = first_lanes(t)
            for q in range(4):
                re, im = u[q]
                rows = slice(q * 64 + g * 8, q * 64 + (g + 1) * 8)
                if t == 0:
                    im = pltpu.roll(jnp.where(lane0, ny[q], im), 2, 1) + jnp.where(lane == 2, ny[q], 0.0)
                    sa_ref[1:3, rows] = jnp.stack((jnp.where(first, im, re), jnp.where(first, re, im)))
                else:
                    im = im * jnp.where(first, 1.0, -1.0)
                    sa_ref[3 * t:3 * t + 3, rows] = jnp.stack((re + im, im, re))
        return item

    def p3_mm(p, q):
        def item(y):
            g = []
            for t in range(4):
                k1, k2, k3 = d_products(sa_ref, 1, t, slice(q * 64, (q + 1) * 64))
                g.append((k3, k2) if t == 0 else (k2 + k1, k3 - k1))
            yy = _r8_real_t(g)
            bx_ref[q, pl.ds(pl.multiple_of(p * 64, 64), 64), :] = jnp.concatenate(yy, axis=1).astype(bf16)
        return item

    def b_out(p):
        def item(y):
            rows = pl.ds(pl.multiple_of(p * 64, 64), 64)
            pltpu.make_async_copy(bx_ref.at[0:4, rows, :], out_hbm.at[:, rows, pl.ds(DM, DM)],
                                  sem_out.at[1]).start()
            bx_ref[4, pin_rows(0), 0:128] = y.astype(bf16)
        return item

    def a_out(blk, half):
        pltpu.make_async_copy(
            xo_ref.at[half, pl.ds(pl.multiple_of(blk * 64 + 64, 64), 64), :],
            out_hbm.at[blk >> 3, pl.ds(pl.multiple_of((blk & 7) * 64, 64), 64),
                       pl.ds(pl.multiple_of(half * 512, 512), 512)],
            sem_out.at[0]).start()

    def step(pp, odd, mem, hooks, first=False):
        r0 = pl.multiple_of(pp * 64 + (64 + 32 * odd), SEG)
        xs = jnp.concatenate([xo_ref[0, pl.ds(r0, SEG), :], xo_ref[1, pl.ds(r0, SEG), :]], axis=1)
        x_lo = xs[0:8].astype(f32)
        hm = jnp.concatenate(
            [jnp.concatenate([x_lo, jnp.concatenate(mem, axis=1)], axis=0).astype(bf16), xs[16:32]], axis=0)
        fill = fillo_ref[:, 0:64] if odd else fille_ref[:, 0:48]
        qkv, ps = {}, {}

        def head_of(v):
            return (v // 16) * 16 + (v % 2) * 8 + (v % 16) // 2 if odd else v

        def do_qkv(v0, v1):
            for v in range(v0, v1):
                h = head_of(v)
                for t in range(3):
                    n = t * H + slot_of(h)
                    y32 = _dot(hm, _tobf(w_refs[n // 16][n // 8 % 2, n % 8, 0:512]))
                    y = y32.astype(bf16)
                    parts = [y]
                    if odd or t > 0:
                        parts.append(_tobf(qkvc_ref[pp, n // 8, n % 8]))
                    if t > 0:
                        if odd:
                            parts.append(_tobf(kve_ref[(t - 1) * H + h]))
                        else:
                            kve_ref[(t - 1) * H + h] = _tou(y[0:16])
                    qkv[(t, v)] = jnp.concatenate(parts, axis=0) if len(parts) > 1 else y
                for item in hooks.get(v, ()):
                    item(y32[0:8])

        def do_s(g):
            for v in range(g * G, (g + 1) * G):
                sc = jax.lax.dot_general(qkv[(0, v)], qkv[(1, v)], (((1,), (1,)), ((), ())),
                                         preferred_element_type=f32)
                sc = jnp.where(fill == 0.0, sc * scale, fill)
                e = jnp.exp(sc - jnp.max(sc, axis=1, keepdims=True))
                den = jnp.sum(e, axis=1, keepdims=True)
                r = pl.reciprocal(den, approx=True)
                r = r * (2.0 - den * r)
                ps[v] = (e * r).astype(bf16)

        def do_pv(g):
            o = {v: _dot(ps[v], qkv[(2, v)]) for v in range(g * G, (g + 1) * G)}
            for v in o:
                h = head_of(v)
                oall_ref[:, h * DH:(h + 1) * DH] = _tou(o[v][0:32].astype(bf16))
            if odd:
                for v in range(g * G, (g + 1) * G, 2):
                    a11, a12 = o[v][0:32], o[v + 1][0:32]
                    a21 = jnp.concatenate([oc_ref[head_of(v)], o[v][32:48]], axis=0)
                    a22 = jnp.concatenate([oc_ref[head_of(v + 1)], o[v + 1][32:48]], axis=0)
                    for k, a in enumerate((a11 + a22, a21 + a22, a22, a11 + a12, a21 - a11, a12 - a22)):
                        os_ref[k, :, (v // 2) * DH:(v // 2 + 1) * DH] = a
                for v in o:
                    oc_ref[head_of(v)] = o[v][32:48]

        def plain(half, j, h0, h1):
            return _dot(_tobf(oall_ref[:, h0 * DH:h1 * DH]), _tobf(wo_ref[half, j, h0 * 64:h1 * 64, :]))

        hb = pp & 1
        if odd:
            def product(jp, k):
                def fn(part):
                    h0 = part * 16
                    if k == 2:
                        lhs = _tobf(oall_ref[:, h0 * DH:(h0 + 8) * DH])
                    else:
                        lhs = os_ref[k - (k > 2), :, part * 1024:(part + 1) * 1024].astype(bf16)
                    if k == 1:
                        rhs = wo_ref[hb, jp * 2, h0 * 64:(h0 + 8) * 64, :]
                    elif k == 4:
                        rhs = wo_ref[hb, jp * 2 + 1, (h0 + 8) * 64:(h0 + 16) * 64, :]
                    else:
                        rhs = ws_ref[hb, jp * 5 + (0, 0, 1, 2, 0, 3, 4)[k], part * 512:(part + 1) * 512, :]
                    return _dot(lhs, _tobf(rhs))
                return fn
            jobs = [product(jp, k) for jp in range(2) for k in range(7)]
            jobs += [(lambda part, j=j: plain(1 - hb, j, part * 16, part * 16 + 16)) for j in range(4)]
            marks = (2, 10)
        else:
            jobs = [(lambda part, j=j: plain(j // 4, j % 4, part * 24, 24 + part * 8)) for j in range(8)]
            marks = (2, 5)

        for g in range(NG):
            do_qkv(g * G, g * G + G // 2)
            if g >= 1:
                do_s(g - 1)
            do_qkv(g * G + G // 2, (g + 1) * G)
            if g >= 2:
                do_pv(g - 2)
        part = []
        for k, job in enumerate(jobs):
            items = hooks.get(('o', k), ())
            if len(items) == 2:
                half = plain(k // 4, k % 4, 0, 12)
                items[0](half[0:8])
                part.append(plain(k // 4, k % 4, 12, 24) + half)
                items[1](part[k][0:8])
            else:
                part.append(job(0))
                for item in items:
                    item(part[k][0:8])
            if k == marks[0]:
                do_s(NG - 1)
                do_pv(NG - 2)
            if k == marks[1]:
                do_pv(NG - 1)

        def finish(k):
            res = jobs[k](1) + part[k]
            for item in hooks.get(('p', k), ()):
                item(res[0:8])
            return res

        def put(half, j, r, v):
            xo_ref[half, pl.ds(r0 + r, v.shape[0]), j * 128:(j + 1) * 128] = v.astype(bf16)

        if odd:
            own = []
            for jp in range(2):
                m1, m2, m3, m4, m5, m6, m7 = [finish(jp * 7 + k) for k in range(7)]
                for jj, top, bot in ((0, ((m1 + m4) - m5) + m7, m2 + m4), (1, m3 + m5, ((m1 - m2) + m3) + m6)):
                    j = jp * 2 + jj
                    own.append(top[8:16])
                    put(hb, j, 0, jnp.concatenate([top[0:8], bot[24:32], top[16:32]], axis=0))
                    put(hb, j, -24, bot[16:24])
                    put(hb, j, -56, bot[8:16])
                    put(hb, j, -88, bot[0:8])
            for j in range(4):
                res = finish(14 + j)
                own.append(res[8:16])
                put(1 - hb, j, 0, res)
            new_mem = [jnp.where(hb == 0, own[j], own[(j + 4) % 8]) for j in range(8)]
        else:
            new_mem = []
            for j in range(8):
                res = finish(j)
                new_mem.append(res[8:16])
                put(j // 4, j % 4, 0, res)
        for item in hooks.get(H, ()):
            item(None)
        if odd:
            a_out(pp, hb)
            if first:
                pl.when(pp > 0)(lambda: a_out(pp - 1, hb))
            else:
                a_out(pp - 1, hb)
        return new_mem

    def l1(i, mem):
        bx_copy(i).wait()
        he = {2 * k: [p1_pre(i, k // 4, k % 4)] for k in range(16)}
        he[H] = [p1_mm(i, 1), p1_mm(i, 2), p1_mm(i, 3)]
        ho = {('p', 2): [p1_mm(i, 0)]}
        mem = step(i, 0, mem, he)
        mem = step(i, 1, mem, ho, first=True)
        return mem

    def l2(i, mem):
        u = i - N_L1
        he = {3: [p2_fwd(u, range(0, 4))], 7: [p2_fwd(u, range(4, 8))], 17: [p2_nyq(u)],
              H: [p2_inv(u, range(0, 8))]}
        ho = {('p', k): [p2_bfly(u + k % 2, k // 2, k % 2 == 0)] for k in range(16)}
        mem = step(i, 0, mem, he)
        mem = step(i, 1, mem, ho)
        return mem

    def l3(i, mem):
        p = i - N_L1 - N_L2
        he = {h: [p3_pre(p, h // 3, 1 + h % 3)] for h in range(24)}
        for j in range(4):
            he[('o', 3 + j)] = [p3_pre(p, 2 * j, 0), p3_pre(p, 2 * j + 1, 0)]
        he[H] = [p3_mm(p, q) for q in range(4)]
        ho = {12: [b_out(p)]}
        mem = step(i, 0, mem, he)
        mem = step(i, 1, mem, ho)
        return mem

    m0 = mem_ref[...].astype(f32)
    mem = [m0[:, j * 128:(j + 1) * 128] for j in range(8)]
    mem = jax.lax.fori_loop(0, N_L1, l1, mem)
    cp_x[2].wait()
    cp_x[3].wait()
    cp_ms.wait()
    for g in range(8):
        p2_bfly(0, g, False)(None)
        p2_bfly(0, g, False, ny_ref)(None)
    mem = jax.lax.fori_loop(N_L1, N_L1 + N_L2, l2, mem)
    for g in range(8):
        p2_bfly(0, g, True, ny_ref)(None)
    mem = jax.lax.fori_loop(N_L1 + N_L2, NSEG // 2, l3, mem)

    oc_last = jnp.concatenate([oc_ref[h] for h in range(H)], axis=1).astype(bf16)
    for j in range(4):
        res = _dot(oc_last, _tobf(wo_ref[0, j, 0:2048, :])).astype(bf16)
        xo_ref[0, S + 8:S + 16, j * 128:(j + 1) * 128] = res[0:8]
        xo_ref[0, S + 40:S + 48, j * 128:(j + 1) * 128] = res[8:16]
    a_out(NSEG // 2 - 1, 0)

    pltpu.make_async_copy(bx_ref.at[0:4], out_hbm.at[:, :, pl.ds(DM, DM)], sem_out.at[1]).wait()
    pltpu.make_async_copy(xo_ref.at[:, 64:64 + S], xo_ref.at[:, 64:64 + S], sem_out.at[0]).wait()


@jax.jit
def _run(x, mem0, wq, wk, wv, wo, bx, w_r, w_i):
    fd, ms, tv = _tables()
    hbm = pl.BlockSpec(memory_space=pl.ANY)
    out = pl.pallas_call(
        _kernel,
        out_shape=jax.ShapeDtypeStruct((4, S // 4, 2 * DM), bf16),
        in_specs=[hbm] * 13,
        out_specs=hbm,
        scratch_shapes=[
            pltpu.VMEM((2, 64 + S, DM // 2), bf16),
            pltpu.VMEM((MEM, DM), bf16),
            pltpu.VMEM((8, NSEG, 8, 128), bf16),
            pltpu.VMEM((4, DM, 16, DH), bf16),
        ] + [pltpu.VMEM((2, 8, DM // 2 + 8, DH), u32)] * 6 + [
            pltpu.VMEM((2, 4, H * DH // 2 + 8, 128), u32),
            pltpu.VMEM((8, 256, 128), u32),
            pltpu.VMEM((5, 4, 136, 128), u32),
            pltpu.VMEM((NSEG // 2, 12, 8, 8, 128), u32),
            pltpu.VMEM((2 * H, 8, 128), u32),
            pltpu.VMEM((16, H * DH), u32),
            pltpu.VMEM((H, 16, DH), f32),
            pltpu.VMEM((6, 32, 16 * DH), f32),
            pltpu.VMEM((2, 10, 1040, 128), u32),
            pltpu.VMEM((32, 128), f32),
            pltpu.VMEM((48, 128), f32),
            pltpu.VMEM((5, S // 4, DM), bf16),
            pltpu.VMEM((2, 8, DM // 2 + 1, 256), bf16),
            pltpu.VMEM((12872, 128), u32),
            pltpu.VMEM((137, 128, 128), f32),
            pltpu.VMEM((8, 128, 128), f32),
            pltpu.VMEM((12, 264, 128), f32),
            pltpu.VMEM((24, 64, 128), u32),
            pltpu.VMEM((64, 64, 128), u32),
            pltpu.VMEM((2, 512, 128), f32),
            pltpu.SMEM((64,), f32),
            pltpu.SMEM((1,), jnp.int32),
            pltpu.SemaphoreType.DMA((84,)),
            pltpu.SemaphoreType.DMA((2,)),
        ],
        compiler_params=pltpu.CompilerParams(vmem_limit_bytes=120 * 1024 * 1024,
                                             disable_semaphore_checks=True,
                                             disable_bounds_checks=True),
    )(x.reshape(S, DM), x.reshape(NSEG, SEG, DM), mem0.reshape(MEM, DM), wq, wk, wv,
      wo.reshape(H * DH // 16, 16, DM), bx.reshape(4, S // 4, DM), w_r.T, w_i.T, jnp.asarray(fd), jnp.asarray(ms), jnp.asarray(tv))
    return out.reshape(1, S, 2 * DM)


def pallas_concat_heads__memory_aug_recurrent_mem_tr__spectral_gfnet__prompt_kernel(
    A_x: jax.Array,
    A_mem0: jax.Array,
    A_Wq: jax.Array,
    A_Wk: jax.Array,
    A_Wv: jax.Array,
    A_Wo: jax.Array,
    A_seg_len,
    B_x: jax.Array,
    B_w_r: jax.Array,
    B_w_i: jax.Array,
):
    if isinstance(A_seg_len, int):
        assert A_seg_len == SEG
    assert A_x.shape == (1, S, DM) and A_mem0.shape == (1, MEM, DM) and A_Wq.shape == (DM, H, DH)
    assert B_x.shape == (1, S, DM) and B_w_r.shape == (S, DM // 2 + 1)
    return _run(A_x, A_mem0, A_Wq, A_Wk, A_Wv, A_Wo, B_x, B_w_r, B_w_i)
```

```python
import math

import numpy as np
import jax
import jax.numpy as jnp
import jax.experimental.pallas as pl
import jax.experimental.pallas.tpu as pltpu

bf16 = jnp.bfloat16
f32 = jnp.float32
u32 = jnp.uint32

S, DM = 2048, 1024
H, DH = 32, 128
MEM, SEG = 8, 32
NSEG = S // SEG
SQH = math.sqrt(0.5)

_PAIRS = ((0, 4), (1, 7), (2, 6), (3, 5))
_FIRST = np.array([[1, 1, 0, 0], [1, 0, 1, 0], [0, 1, 1, 0], [0, 1, 0, 1]], bool)


def _pack_rows(a):
    u = np.ascontiguousarray(a, dtype=np.float32).view(np.uint32).astype(np.uint64)
    b = ((u + 0x7FFF + ((u >> 16) & 1)) >> 16).astype(np.uint32)
    return (b[..., 0::2, :] | (b[..., 1::2, :] << 16)).astype(np.uint32)


def _tables():
    k2 = np.zeros((4, 128), np.int64)
    for t in range(4):
        odd = t % 2
        for lam in range(128):
            k = 2 * lam + odd
            if k % 8 not in _PAIRS[t]:
                k = 2 * (128 + 8 * (lam // 8) + (lam % 8 - 1 - odd) % 8) + odd
            assert k % 8 in _PAIRS[t]
            k2[t, lam] = k
    b = np.arange(128)[:, None]
    F = np.zeros((12, 128, 128))
    G = np.zeros((12, 128, 128))
    for t in range(4):
        th = 2 * np.pi * ((b * k2[t][None, :]) % DM) / DM
        C, Sn = np.cos(th), np.sin(th)
        first = ((k2[t] % 8) == _PAIRS[t][0])[None, :]
        assert np.array_equal(first[0], _FIRST[t][np.arange(128) % 4])
        if t == 0:
            im = -Sn
            im[:, 0] = (-1.0) ** np.arange(128)
            im = np.roll(im, 2, axis=1)
            F[1:3] = np.where(first, im, C), np.where(first, C, im)
            G[1:3] = F[1:3]
            G[2, :, 0] *= 0.5
            G[2, :, 2] *= 0.5
        else:
            Sg = np.where(first, Sn, -Sn)
            F[3 * t:3 * t + 3] = C, -(C + Sg), C - Sg
            G[3 * t:3 * t + 3] = F[3 * t:3 * t + 3]
    Finv = np.transpose(G, (0, 2, 1)) * (2.0 / DM)
    fd = _pack_rows(np.concatenate([F, Finv]))
    M = np.zeros((32, 128, 128))
    r = np.arange(64)[None, :]
    l = np.arange(64)[:, None]
    for j in range(32):
        th = 2 * np.pi * ((r * (j + 32 * l)) % S) / S
        C, Sn = np.cos(th), np.sin(th)
        M[j, :64, :64] = C
        M[j, :64, 64:] = Sn
        M[j, 64:, :64] = -Sn
        M[j, 64:, 64:] = C
    perm = np.arange(128).reshape(2, 8, 8).transpose(1, 0, 2).reshape(128)
    M = M[:, perm][:, :, perm]
    Minv = np.transpose(M, (0, 2, 1)) / S
    ms = _pack_rows(np.concatenate([M, Minv]))
    th = 2 * np.pi * np.outer(np.arange(512), np.arange(128) % 4) / S
    tv = np.stack([np.cos(th), np.sin(th)]).astype(np.float32)
    return fd, ms, tv


def _tobf(w):
    return pltpu.bitcast(w, bf16)


def _tou(w):
    return pltpu.bitcast(w, u32)


def _dot(a, b):
    return jnp.dot(a, b, preferred_element_type=f32)


def _r8_real(x):
    t0, t1 = x[0] + x[4], x[0] - x[4]
    t2, t3 = x[2] + x[6], x[2] - x[6]
    t4, t5 = x[1] + x[5], x[1] - x[5]
    t6, t7 = x[3] + x[7], x[3] - x[7]
    e0, e1 = t0 + t2, t0 - t2
    o0, o1 = t4 + t6, t4 - t6
    u, v = SQH * (t5 - t7), SQH * (t5 + t7)
    return [(e0 + o0, e0 - o0), (t1 + u, v + t3), (e1, o1), (t1 - u, v - t3)]


def _r8_real_t(g):
    (z0, z4), (a1, b1), (e1, o1), (a3, b3) = g
    e0, o0 = z0 + z4, z0 - z4
    t1, u = a1 + a3, a1 - a3
    v, t3 = b1 + b3, b1 - b3
    t5, t7 = SQH * (v + u), SQH * (v - u)
    t0, t2 = e0 + e1, e0 - e1
    t4, t6 = o0 + o1, o0 - o1
    return [t0 + t1, t4 + t5, t2 + t3, t6 + t7, t0 - t1, t4 - t5, t2 - t3, t6 - t7]


def _dft4(u):
    (r0, i0), (r1, i1), (r2, i2), (r3, i3) = u
    sr, si, dr, di = r0 + r2, i0 + i2, r0 - r2, i0 - i2
    tr, ti, er, ei = r1 + r3, i1 + i3, r1 - r3, i1 - i3
    return [(sr + tr, si + ti), (dr + ei, di - er), (sr - tr, si - ti), (dr - ei, di + er)]


def _dft8(x):
    a = [(x[p][0] + x[p + 4][0], x[p][1] + x[p + 4][1]) for p in range(4)]
    d = [(x[p][0] - x[p + 4][0], x[p][1] - x[p + 4][1]) for p in range(4)]
    ev = _dft4(a)
    (r0, i0), (r1, i1), (r2, i2), (r3, i3) = d
    b1r, b1i = SQH * (r1 + i1), SQH * (i1 - r1)
    b3r, n3i = SQH * (i3 - r3), SQH * (r3 + i3)
    sr, si, dr, di = r0 + i2, i0 - r2, r0 - i2, i0 + r2
    tr, ti, er, ei = b1r + b3r, b1i - n3i, b1r - b3r, b1i + n3i
    od = [(sr + tr, si + ti), (dr + ei, di - er), (sr - tr, si - ti), (dr - ei, di + er)]
    return [ev[0], od[0], ev[1], od[1], ev[2], od[2], ev[3], od[3]]


def _swap(x):
    return [(b, a) for (a, b) in x]


G = 4
NG = H // G
NEG = -1e9
N_L1, N_L2 = 8, 16


def _kernel(x_hbm, x3_hbm, mem_hbm, wq_hbm, wk_hbm, wv_hbm, wo_hbm, bx_hbm, wr_hbm, wi_hbm,
            fd_hbm, ms_hbm, tv_hbm, out_hbm,
            xo_ref, mem_ref, xcraw_ref, raw_ref, w0_ref, w1_ref, w2_ref, w3_ref, w4_ref, w5_ref,
            wo_ref, xc_ref, xs_ref, qkvc_ref, kve_ref,
            oall_ref, oc_ref, os_ref, ws_ref, fille_ref, fillo_ref,
            bx_ref, wt_ref, wp_ref, ub_ref, ny_ref, sa_ref, fd_ref, ms_ref, tv_ref,
            tw_ref, zero_ref, sem_in, sem_out):
    scale = DH ** -0.5
    w_hbm = (wq_hbm, wk_hbm, wv_hbm)
    w_refs = (w0_ref, w1_ref, w2_ref, w3_ref, w4_ref, w5_ref)

    def raw_copy(c, i=0, nd=DM):
        rows = pl.ds(pl.multiple_of(i * nd, nd), nd)
        return pltpu.make_async_copy(
            w_hbm[c // 2].at[rows, pl.ds((c % 2) * 16, 16), :],
            raw_ref.at[c % 4, rows], sem_in.at[8 + min(c, 3) * 8 + max(c - 3, 0) * 2 + i])

    def xc_copy(k):
        return pltpu.make_async_copy(
            x3_hbm.at[:, pl.ds(8, 8), pl.ds(pl.multiple_of(k * 128, 128), 128)], xcraw_ref.at[k], sem_in.at[40 + k])

    def wo_copies(half):
        return [pltpu.make_async_copy(wo_hbm.at[:, :, pl.ds(pl.multiple_of(half * 512 + j * 128, 128), 128)],
                                      raw_ref.at[2 + half, j * 256:(j + 1) * 256], sem_in.at[76 + half * 4 + j])
                for j in range(4)]

    def wt_copies(i):
        return [pltpu.make_async_copy(src.at[:, pl.ds(pl.multiple_of(i * 1024 + k * 256, 256), 256)],
                                      wt_ref.at[i, a * 4 + k], sem_in.at[i * 4 + (48 + a * 8 + k)])
                for k in range(4) for a, src in enumerate((wr_hbm, wi_hbm))]

    def bx_copy(p):
        rows = pl.ds(pl.multiple_of(p * 64, 64), 64)
        return pltpu.make_async_copy(bx_hbm.at[:, rows, :], bx_ref.at[0:4, rows, :], sem_in.at[64 + p])

    n_head = N_L1 * 2 * SEG
    cp_x = [pltpu.make_async_copy(x_hbm.at[lo:hi, half * 512:(half + 1) * 512], xo_ref.at[half, 64 + lo:64 + hi],
                                  sem_in.at[72 + (lo > 0) * 2 + half])
            for lo, hi in ((0, n_head), (n_head, S)) for half in range(2)]
    cp_mem = pltpu.make_async_copy(mem_hbm, mem_ref, sem_in.at[1])
    cp_fd = pltpu.make_async_copy(fd_hbm, fd_ref, sem_in.at[4])
    cp_ms = pltpu.make_async_copy(ms_hbm, ms_ref, sem_in.at[5])
    cp_tv = pltpu.make_async_copy(tv_hbm, tv_ref, sem_in.at[6])

    for i in range(8):
        raw_copy(0, i, 128).start()
        xc_copy(i).start()
        if i >= 4:
            raw_copy(2, i - 4, 192).start()
        raw_copy(1, i, 128).start()
    raw_copy(2, 6, 128).start()
    raw_copy(2, 7, 128).start()
    for i in range(2):
        raw_copy(3, i, 512).start()

    zero_ref[0] = 0

    def pin_bit():
        return jnp.clip(zero_ref[0], 0, 1)

    def pin_rows(r):
        return pl.ds(pl.multiple_of(r + pin_bit() * 32, 8), 8)

    for p in range(8):
        for jq in range(4):
            tw_ref[(p * 4 + jq) * 2] = jnp.float32(math.cos(2 * math.pi * p * jq / 32))
            tw_ref[(p * 4 + jq) * 2 + 1] = jnp.float32(math.sin(2 * math.pi * p * jq / 32))

    ub_ref[128:136] = jnp.zeros((8, 128, 128), f32)
    wp_ref[12800:12872] = jnp.zeros((72, 128), u32)
    oc_ref[...] = jnp.zeros((H, 16, DH), f32)

    qi = jax.lax.broadcasted_iota(jnp.int32, (48, 128), 0)
    ki = jax.lax.broadcasted_iota(jnp.int32, (48, 128), 1)

    def between(v, lo, hi):
        return (v >= lo) & (v < hi)

    def table(keep, other):
        return jnp.where(other, -jnp.inf, jnp.where(keep, 0.0, NEG)).astype(f32)

    keep = between(qi, 8, 16) | between(ki, 8, 16) | (qi >= jnp.where(ki < 32, ki, ki - 24))
    fille_ref[...] = table(keep, ki >= 40)[:32]
    q_even = between(qi, 32, 40)
    k_even = between(ki, 32, 40) | (ki >= 48)
    qpos = jnp.where(qi < 32, qi, jnp.where(qi < 40, qi - 24, qi - 32))
    kpos = jnp.where(ki < 32, ki, jnp.where(ki < 40, ki - 24, jnp.where(ki < 48, ki - 32, ki - 48)))
    keep = between(qi, 8, 16) | between(ki, 8, 16) | (ki >= 56) | (qpos >= kpos)
    fillo_ref[...] = table(keep, (q_even != k_even) | (ki >= 64))

    def relayout16(c, blk):
        w0 = pl.multiple_of(blk * 8, 8)
        v = _tou(raw_ref[c % 4, pl.ds(blk * 16, 16)]).reshape(8, 2, 8, 128)
        a, b = v[:, 0], v[:, 1]
        w_refs[c][0, :, pl.ds(w0, 8), :] = jnp.swapaxes((a & jnp.uint32(0xFFFF)) | (b << 16), 0, 1)
        w_refs[c][1, :, pl.ds(w0, 8), :] = jnp.swapaxes((a >> 16) | (b & jnp.uint32(0xFFFF0000)), 0, 1)

    def slot_of(h):
        return (h // 16) * 16 + (h % 2) * 8 + (h % 16) // 2

    def repack_wo(half, part, k):
        jp, g0 = k & 1, part * 128 + (k >> 1) * 2
        quad = []
        for jj in range(2):
            for kh in range(2):
                v = _tou(raw_ref[2 + half, pl.ds((jp * 2 + jj) * 256 + kh * 64 + g0, 2)]).reshape(16, 128)
                wo_ref[half, jp * 2 + jj, pl.ds(pl.multiple_of(g0 * 8 + kh * 512, 16), 16), :] = v
                quad.append(_tobf(v).astype(f32))
        b11, b21, b12, b22 = quad
        rows = pl.ds(pl.multiple_of(part * 512 + (k >> 1) * 16, 16), 16)
        for n, v in enumerate((b11 + b22, b12 - b22, b21 - b11, b11 + b12, b21 + b22)):
            ws_ref[half, jp * 5 + n, rows, :] = _tou(v.astype(bf16))

    sub4 = jax.lax.broadcasted_iota(jnp.int32, (128, 128), 0) & 3

    def wp_store(t, kb, tile):
        v = tile.T.reshape(4, 32, 128)
        v = jnp.concatenate([v, v[:, 0:8]], axis=1).reshape(160, 128)
        wp_ref[pl.ds(pl.multiple_of(t * 2560 + kb * 160, 32), 160), :] = v

    def b_prep(i, k, hb, par):
        cols = slice(hb * 128, (hb + 1) * 128)
        a = _tou(wt_ref[i, k, 0:512, cols])
        b = _tou(wt_ref[i, 4 + k, 0:512, cols])
        if par == 0:
            w = (a << 16) | (b & jnp.uint32(0xFFFF))
            m = (sub4 == 0) | (sub4 == 2)
        else:
            w = (a & jnp.uint32(0xFFFF0000)) | (b >> 16)
            m = (sub4 == 0) | (sub4 == 3)
        top = w[:128]
        bot = pltpu.roll(w[128:].reshape(16, 8, 128), 1 + par, 1).reshape(128, 128)
        wp_store(par, i * 8 + (k * 2 + hb), jnp.where(m, top, bot))
        wp_store(par + 2, i * 8 + (k * 2 + hb), jnp.where(m, bot, top))
        if par == 0:
            na = jnp.broadcast_to(wt_ref[i, k, 512:513, cols].astype(f32), (128, 128))
            nb = jnp.broadcast_to(wt_ref[i, 4 + k, 512:513, cols].astype(f32), (128, 128))
            wp_store(4, i * 8 + (k * 2 + hb), pltpu.bitcast(na, u32) | (pltpu.bitcast(nb, u32) >> 16))

    def gather_c(k):
        xc_ref[k] = _tou(xcraw_ref[k].astype(f32).reshape(512, 128).astype(bf16))

    def store_qkvc(n, y):
        qkvc_ref[:, n // 8, n % 8] = y.reshape(NSEG // 2, 8, 128)

    def q_unit(i, groups, first, last, fillers):
        xk = _tobf(xc_ref[i])
        w0 = pl.multiple_of(i * 64, 64)
        for g in groups:
            rhs = jnp.concatenate(
                [_tobf(w_refs[h // 16][h // 8 % 2, h % 8, pl.ds(w0, 64), :]) for h in range(4 * g, 4 * g + 4)], axis=1)
            y = _dot(xk, rhs)
            for h in range(4 * g, 4 * g + 4):
                yh = y[:, (h % 4) * 128:(h % 4 + 1) * 128]
                if not first:
                    yh = yh + ub_ref[h * 4:(h + 1) * 4].reshape(512, 128)
                if last:
                    store_qkvc(h, _tou(yh.astype(bf16)))
                else:
                    ub_ref[h * 4:(h + 1) * 4] = yh.reshape(4, 128, 128)
            mine = fillers.get(g, [])
            for fi, item in enumerate(mine):
                r = (fi * 512 // len(mine)) // 8 * 8
                item(pltpu.bitcast(y[r:r + 8, 0:128], u32))

    def rl_item(c, blk):
        def item(pin):
            w_refs[c][pin_bit(), 7, 512:520] = pin
            relayout16(c, blk)
        return item

    def spread(fillers, items, groups):
        for k, item in enumerate(items):
            fillers.setdefault(groups[k * len(groups) // len(items)], []).append(item)
        return fillers

    def half_items(f, c, i, groups):
        return spread(f, [rl_item(c, i * 8 + blk) for blk in range(8)], groups)

    def piece_items(i):
        f = half_items(half_items({}, 1, i, (0, 1, 2)), 0, i + 1, (4, 5, 6))
        return spread(f, [lambda pin: gather_c(i + 1)], (7,))

    def chunk2_items(f, lo, hi, groups):
        return spread(f, [rl_item(2, blk) for blk in range(lo, hi)], groups)

    def wait_piece(i):
        raw_copy(1, i, 128).wait()
        raw_copy(0, i + 1, 128).wait()
        xc_copy(i + 1).wait()

    raw_copy(0, 0, 128).wait()
    for blk in range(8):
        relayout16(0, blk)
    xc_copy(0).wait()
    gather_c(0)
    q_unit(0, range(0, 2), True, False, {})
    raw_copy(1, 0, 128).wait()
    q_unit(0, range(2, 4), True, False, half_items({}, 1, 0, (2, 2, 3)))
    q_unit(0, range(4, 6), True, False, {})
    xc_copy(1).wait()
    raw_copy(0, 1, 128).wait()
    q_unit(0, range(6, 8), True, False,
           spread(half_items({}, 0, 1, (6, 6, 7)), [lambda pin: gather_c(1)], (6,)))
    raw_copy(1, 1, 128).wait()
    q_unit(1, range(0, 4), False, False, half_items({}, 1, 1, (0, 1, 2)))
    xc_copy(2).wait()
    raw_copy(0, 2, 128).wait()
    q_unit(1, range(4, 8), False, False,
           spread(half_items({}, 0, 2, (4, 5, 6)), [lambda pin: gather_c(2)], (6,)))

    def xsum_item(j, rq):
        def item(pin):
            xs_ref[pin_bit(), 0, 128:136] = pin
            a11, a21, a12, a22 = [
                xcraw_ref[j + 4 * kh, rh * 32 + rq * 8:rh * 32 + (rq + 1) * 8].astype(f32).reshape(64, 128)
                for kh in range(2) for rh in range(2)]
            for k, v in enumerate((a11 + a22, a21 + a22, a11 + a12, a21 - a11, a12 - a22)):
                xs_ref[k, j, rq * 32:(rq + 1) * 32] = _tou(v.astype(bf16))
        return item

    wait_piece(2)
    q_unit(2, range(8), False, False, piece_items(2))

    def q_c(i, carry):
        wait_piece(i)
        raw_copy(2, i - 3, 192).wait()
        f = spread(piece_items(i), [rl_item(2, (i - 3) * 12 + blk) for blk in range(12)],
                   (2, 3, 3, 3, 3, 3, 4, 4, 5, 6, 6, 7))
        q_unit(i, range(8), False, False, spread(f, [xsum_item(i - 3, rq) for rq in range(4)], (3, 4, 5, 6)))
        return carry
    jax.lax.fori_loop(3, 7, q_c, 0)

    raw_copy(1, 7, 128).wait()
    raw_copy(2, 6, 128).wait()
    raw_copy(2, 7, 128).wait()
    q_unit(7, range(8), False, True, chunk2_items(half_items({}, 1, 7, (0, 1, 2)), 48, 64, (3, 4, 5, 6)))
    raw_copy(4).start()
    for cp in wo_copies(0):
        cp.start()
    raw_copy(5).start()

    def bulk_iter(c, i):
        def xs(k):
            return jnp.concatenate([_tobf(xs_ref[k, j, 0:128]) for j in range(4)], axis=1)

        def xc(rh, kh):
            return jnp.concatenate(
                [_tobf(xc_ref[4 * kh + j, rh * 128:(rh + 1) * 128]) for j in range(4)], axis=1)

        for pr in range(4):
            n1, n2 = pr * 2, pr * 2 + 1

            def w(n, kh):
                return _tobf(w_refs[c][i, n, kh * 256:(kh + 1) * 256])

            def wsum(a, b, sign):
                a, b = a.astype(f32), b.astype(f32)
                return (a + b if sign > 0 else a - b).astype(bf16)

            def out(rh, n, v):
                qkvc_ref[rh * 16:(rh + 1) * 16, c * 2 + i, n] = _tou(v.astype(bf16)).reshape(16, 8, 128)

            def side(k, m):
                blks = (k, 7) if k == 0 else (k,)
                items = []
                if c < 5:
                    items += [('w', blk) for blk in blks]
                if c >= 4:
                    items += [('o', blk) for blk in range(k * 16 // 7, (k + 1) * 16 // 7)]
                if c == 5 and k in (1, 2, 4, 5):
                    items.append(('f', (1, 2, 4, 5).index(k)))
                for n, (kind, blk) in enumerate(items):
                    r = n * 256 // len(items) // 8 * 8
                    pin = pltpu.bitcast(m[r:r + 8], u32)
                    if kind == 'w':
                        w_refs[c + 1][pin_bit(), 7, 512:520] = pin
                        relayout16(c + 1, i * 32 + (pr * 8 + blk))
                    elif kind == 'o':
                        ws_ref[pin_bit(), 9, 1024:1032] = pin
                        wo_ref[pin_bit(), 3, 2048:2056] = pin
                        repack_wo(c - 4, i, pr * 16 + blk)
                    else:
                        wp_ref[pin_rows(12832), :] = pin
                        b_prep(i, pr, blk // 2, blk % 2)

            m2 = _dot(xs(1), w(n1, 0))
            side(0, m2)
            m4 = _dot(xc(1, 1), wsum(w(n1, 1), w(n1, 0), -1))
            side(1, m4)
            out(1, n1, m4 + m2)
            m1 = _dot(xs(0), wsum(w(n1, 0), w(n2, 1), 1))
            side(2, m1)
            m5 = _dot(xs(2), w(n2, 1))
            side(3, m5)
            m3 = _dot(xc(0, 0), wsum(w(n2, 0), w(n2, 1), -1))
            side(4, m3)
            out(0, n2, m3 + m5)
            c22 = _dot(xs(3), wsum(w(n1, 0), w(n2, 0), 1)) + ((m1 - m2) + m3)
            side(5, c22)
            out(1, n2, c22)
            c11 = _dot(xs(4), wsum(w(n1, 1), w(n2, 1), 1)) + ((m1 + m4) - m5)
            side(6, c11)
            out(0, n1, c11)

    for c in range(2, 6):
        if c == 3:
            for cp in wo_copies(1) + wt_copies(0) + wt_copies(1):
                cp.start()
        if c == 4:
            for cp in cp_x[0:2] + [cp_mem, cp_fd, cp_tv] + [bx_copy(p) for p in range(8)] + cp_x[2:4] + [cp_ms]:
                cp.start()
        if c >= 4:
            for cp in wo_copies(c - 4):
                cp.wait()
        if 2 < c < 5:
            raw_copy(c + 1).wait()

        def bulk(i, carry, c=c):
            if c == 2:
                raw_copy(3, i, 512).wait()
            if c == 5:
                for cp in wt_copies(i):
                    cp.wait()
            bulk_iter(c, i)
            return carry
        jax.lax.fori_loop(0, 2, bulk, 0)

    cp_x[0].wait()
    cp_x[1].wait()
    cp_mem.wait()
    cp_fd.wait()
    cp_tv.wait()

    lane = jax.lax.broadcasted_iota(jnp.int32, (1, 128), 1)
    lane0 = lane == 0
    sgn0 = jnp.where(lane0, 1.0, -1.0)

    def first_lanes(t):
        la, lb = [k for k in range(4) if _FIRST[t][k]]
        return ((lane & 3) == la) | ((lane & 3) == lb)

    def d_products(st_ref, d, t, rows):
        return [_dot(st_ref[n, rows].astype(bf16), _tobf(fd_ref[d * 12 + n])) if n else None
                for n in range(3 * t, 3 * t + 3)]

    def twiddles(p):
        return [(tw_ref[p * 8 + jq * 2], tw_ref[p * 8 + jq * 2 + 1]) if jq else None for jq in range(4)]

    def p1_pre(p, rs, q):
        def item(y):
            sa_ref[0, pin_rows(0), :] = y
            xq = bx_ref[q, pl.ds(pl.multiple_of(p * 64 + rs * 16, 16), 16), :].astype(f32)
            zz = _r8_real([xq[:, a * 128:(a + 1) * 128] for a in range(8)])
            r = (rs * 4 + q) * 16
            sa_ref[1:12, r:r + 16] = jnp.stack([v for (a, b) in zz for v in (a + b, b, a)][1:])
        return item

    def p1_mm(p, t):
        def item(y):
            cs = twiddles(p)

            def put(ref, n, rs, re, im):
                v = jnp.stack([re.reshape(2, 8, 128), im.reshape(2, 8, 128)], axis=1)
                ref[n * 8 + p, rs * 32:(rs + 1) * 32] = v.reshape(32, 128)

            first = first_lanes(t)
            for rs in range(4):
                k1, k2, k3 = d_products(sa_ref, 0, t, slice(rs * 64, (rs + 1) * 64))
                if t == 0:
                    up = jnp.where(first, k2, k3)
                    re, im = jnp.where(first, k3, k2), pltpu.roll(up, 126, 1)
                    ny = jnp.where(lane0, im, up)
                    u = [ny[q * 16:(q + 1) * 16] for q in range(4)]
                    odd_lane = (lane & 1) == 1
                    nr = jnp.where(odd_lane, pltpu.roll(u[0] - u[2], 1, 1), u[0] + u[2] + (u[1] + u[3]) * sgn0)
                    ni = jnp.where(odd_lane, pltpu.roll((u[3] - u[1]) * sgn0, 1, 1), 0.0)
                    rows = pl.ds(pl.multiple_of(p * 64 + rs * 16, 16), 16)
                    c, sn = tv_ref[0, rows], tv_ref[1, rows]
                    put(ny_ref, 0, rs, nr * c + ni * sn, ni * c - nr * sn)
                    im = jnp.where(lane0, 0.0, im)
                else:
                    re, im = k1 + k2, (k3 - k1) * jnp.where(first, 1.0, -1.0)
                a = _dft4([(re[q * 16:(q + 1) * 16], im[q * 16:(q + 1) * 16]) for q in range(4)])
                for jq in range(4):
                    re, im = a[jq]
                    if jq > 0:
                        c, sn = cs[jq]
                        re, im = re * c + im * sn, im * c - re * sn
                    put(ub_ref, t * 4 + jq, rs, re, im)
        return item

    def p2_bfly(u, g, inverse, ref=ub_ref):
        def item(y):
            if y is not None:
                ub_ref[136, pin_rows(0), :] = y
            v = ref[pl.ds(u * 8, 8), g * 16:(g + 1) * 16]
            x = [(v[p, 0:8], v[p, 8:16]) for p in range(8)]
            x = _swap(_dft8(_swap(x))) if inverse else _dft8(x)
            ref[pl.ds(u * 8, 8), g * 16:(g + 1) * 16] = jnp.stack([w for c in x for w in c]).reshape(8, 16, 128)
        return item

    def filtered(xx, w):
        wr = pltpu.bitcast(w & jnp.uint32(0xFFFF0000), f32).reshape(8, 8, 128)
        wi = pltpu.bitcast(w << 16, f32).reshape(8, 8, 128)
        xx = xx.reshape(8, 2, 8, 128)
        xr, xi = xx[:, 0], xx[:, 1]
        return jnp.stack([xr * wr - xi * wi, xr * wi + xi * wr], axis=1).reshape(128, 128)

    def p2_fwd(u, jps):
        def item(y):
            t = u >> 2
            jq = u & 3
            xs = [_dot(_tobf(ms_ref[jq + 4 * jp]), ub_ref[u * 8 + jp].astype(bf16)) for jp in jps]
            for jp, xx in zip(jps, xs):
                ub_ref[u * 8 + jp] = filtered(xx, wp_ref[pl.ds(t * 2560 + jq + 4 * jp, 64, stride=40), :])
        return item

    def p2_nyq(u):
        def item(y):
            jp = u & 7
            rhs = ny_ref[jp].astype(bf16)
            xx = jnp.concatenate([_dot(_tobf(ms_ref[u * 4, m * 16:(m + 1) * 16]), rhs) for m in range(4)], axis=0)
            w = wp_ref[pl.ds(4 * 2560 + 4 * jp, 64, stride=40), :]
            for jq in range(1, 4):
                w = jnp.where(lane == jq, wp_ref[pl.ds(4 * 2560 + 4 * jp + jq, 64, stride=40), :], w)
            w = jnp.where(u < 8, w, jnp.uint32(0x3F800000))
            ny_ref[jp] = filtered(xx, w)
        return item

    def p2_inv(u, jps):
        def item(y):
            jq = u & 3
            zs = [_dot(_tobf(ms_ref[32 + jq + 4 * jp]), ub_ref[u * 8 + jp].astype(bf16)) for jp in jps]
            for jp, zz in zip(jps, zs):
                ub_ref[u * 8 + jp] = zz
        return item

    def p3_pre(p, g, t):
        def item(y):
            sa_ref[0, pin_rows(0), :] = y
            cs = twiddles(p)

            def fetch(t):
                a = []
                for jq in range(4):
                    v = ub_ref[(t * 4 + jq) * 8 + p, g * 16:(g + 1) * 16]
                    re, im = v[0:8], v[8:16]
                    if jq > 0:
                        c, sn = cs[jq]
                        re, im = re * c - im * sn, im * c + re * sn
                    a.append((re, im))
                return _swap(_dft4(_swap(a)))

            u = fetch(t)
            if t == 0:
                v = ny_ref[p, g * 16:(g + 1) * 16]
                rows = pl.ds(pl.multiple_of(p * 64 + g * 8, 8), 8)
                c, sn = tv_ref[0, rows], tv_ref[1, rows]
                nr, ni = v[0:8] * c - v[8:16] * sn, v[8:16] * c + v[0:8] * sn
                zr, zi = pltpu.roll(nr, 127, 1), pltpu.roll(ni, 127, 1)
                ny = (nr + zr, (nr - zi) * sgn0, nr - zr, (nr + zi) * sgn0)
            first = first_lanes(t)
            for q in range(4):
                re, im = u[q]
                rows = slice(q * 64 + g * 8, q * 64 + (g + 1) * 8)
                if t == 0:
                    im = pltpu.roll(jnp.where(lane0, ny[q], im), 2, 1) + jnp.where(lane == 2, ny[q], 0.0)
                    sa_ref[1:3, rows] = jnp.stack((jnp.where(first, im, re), jnp.where(first, re, im)))
                else:
                    im = im * jnp.where(first, 1.0, -1.0)
                    sa_ref[3 * t:3 * t + 3, rows] = jnp.stack((re + im, im, re))
        return item

    def p3_mm(p, q):
        def item(y):
            g = []
            for t in range(4):
                k1, k2, k3 = d_products(sa_ref, 1, t, slice(q * 64, (q + 1) * 64))
                g.append((k3, k2) if t == 0 else (k2 + k1, k3 - k1))
            yy = _r8_real_t(g)
            bx_ref[q, pl.ds(pl.multiple_of(p * 64, 64), 64), :] = jnp.concatenate(yy, axis=1).astype(bf16)
        return item

    def b_out(p):
        def item(y):
            rows = pl.ds(pl.multiple_of(p * 64, 64), 64)
            pltpu.make_async_copy(bx_ref.at[0:4, rows, :], out_hbm.at[:, rows, pl.ds(DM, DM)],
                                  sem_out.at[1]).start()
            bx_ref[4, pin_rows(0), 0:128] = y.astype(bf16)
        return item

    def a_out(blk, half):
        pltpu.make_async_copy(
            xo_ref.at[half, pl.ds(pl.multiple_of(blk * 64 + 64, 64), 64), :],
            out_hbm.at[blk >> 3, pl.ds(pl.multiple_of((blk & 7) * 64, 64), 64),
                       pl.ds(pl.multiple_of(half * 512, 512), 512)],
            sem_out.at[0]).start()

    def step(pp, odd, mem, hooks, first=False):
        r0 = pl.multiple_of(pp * 64 + (64 + 32 * odd), SEG)
        xs = jnp.concatenate([xo_ref[0, pl.ds(r0, SEG), :], xo_ref[1, pl.ds(r0, SEG), :]], axis=1)
        x_lo = xs[0:8].astype(f32)
        hm = jnp.concatenate(
            [jnp.concatenate([x_lo, jnp.concatenate(mem, axis=1)], axis=0).astype(bf16), xs[16:32]], axis=0)
        fill = fillo_ref[:, 0:64] if odd else fille_ref[:, 0:48]
        qkv, ps = {}, {}

        def head_of(v):
            return (v // 16) * 16 + (v % 2) * 8 + (v % 16) // 2 if odd else v

        def do_qkv(v0, v1):
            for v in range(v0, v1):
                h = head_of(v)
                for t in range(3):
                    n = t * H + slot_of(h)
                    y32 = _dot(hm, _tobf(w_refs[n // 16][n // 8 % 2, n % 8, 0:512]))
                    y = y32.astype(bf16)
                    parts = [y]
                    if odd or t > 0:
                        parts.append(_tobf(qkvc_ref[pp, n // 8, n % 8]))
                    if t > 0:
                        if odd:
                            parts.append(_tobf(kve_ref[(t - 1) * H + h]))
                        else:
                            kve_ref[(t - 1) * H + h] = _tou(y[0:16])
                    qkv[(t, v)] = jnp.concatenate(parts, axis=0) if len(parts) > 1 else y
                for item in hooks.get(v, ()):
                    item(y32[0:8])

        def do_s(g):
            for v in range(g * G, (g + 1) * G):
                sc = jax.lax.dot_general(qkv[(0, v)], qkv[(1, v)], (((1,), (1,)), ((), ())),
                                         preferred_element_type=f32)
                sc = jnp.where(fill == 0.0, sc * scale, fill)
                e = jnp.exp(sc - jnp.max(sc, axis=1, keepdims=True))
                den = jnp.sum(e, axis=1, keepdims=True)
                r = pl.reciprocal(den, approx=True)
                r = r * (2.0 - den * r)
                ps[v] = (e * r).astype(bf16)

        def do_pv(g):
            o = {v: _dot(ps[v], qkv[(2, v)]) for v in range(g * G, (g + 1) * G)}
            for v in o:
                h = head_of(v)
                oall_ref[:, h * DH:(h + 1) * DH] = _tou(o[v][0:32].astype(bf16))
            if odd:
                for v in range(g * G, (g + 1) * G, 2):
                    a11, a12 = o[v][0:32], o[v + 1][0:32]
                    a21 = jnp.concatenate([oc_ref[head_of(v)], o[v][32:48]], axis=0)
                    a22 = jnp.concatenate([oc_ref[head_of(v + 1)], o[v + 1][32:48]], axis=0)
                    for k, a in enumerate((a11 + a22, a21 + a22, a22, a11 + a12, a21 - a11, a12 - a22)):
                        os_ref[k, :, (v // 2) * DH:(v // 2 + 1) * DH] = a
                for v in o:
                    oc_ref[head_of(v)] = o[v][32:48]

        def plain(half, j, h0, h1):
            return _dot(_tobf(oall_ref[:, h0 * DH:h1 * DH]), _tobf(wo_ref[half, j, h0 * 64:h1 * 64, :]))

        hb = pp & 1
        if odd:
            def product(jp, k):
                def fn(part):
                    h0 = part * 16
                    if k == 2:
                        lhs = _tobf(oall_ref[:, h0 * DH:(h0 + 8) * DH])
                    else:
                        lhs = os_ref[k - (k > 2), :, part * 1024:(part + 1) * 1024].astype(bf16)
                    if k == 1:
                        rhs = wo_ref[hb, jp * 2, h0 * 64:(h0 + 8) * 64, :]
                    elif k == 4:
                        rhs = wo_ref[hb, jp * 2 + 1, (h0 + 8) * 64:(h0 + 16) * 64, :]
                    else:
                        rhs = ws_ref[hb, jp * 5 + (0, 0, 1, 2, 0, 3, 4)[k], part * 512:(part + 1) * 512, :]
                    return _dot(lhs, _tobf(rhs))
                return fn
            jobs = [product(jp, k) for jp in range(2) for k in range(7)]
            jobs += [(lambda part, j=j: plain(1 - hb, j, part * 16, part * 16 + 16)) for j in range(4)]
            marks = (2, 10)
        else:
            jobs = [(lambda part, j=j: plain(j // 4, j % 4, part * 24, 24 + part * 8)) for j in range(8)]
            marks = (2, 5)

        for g in range(NG):
            do_qkv(g * G, g * G + G // 2)
            if g >= 1:
                do_s(g - 1)
            do_qkv(g * G + G // 2, (g + 1) * G)
            if g >= 2:
                do_pv(g - 2)
        part = []
        for k, job in enumerate(jobs):
            items = hooks.get(('o', k), ())
            if len(items) == 2:
                half = plain(k // 4, k % 4, 0, 12)
                items[0](half[0:8])
                part.append(plain(k // 4, k % 4, 12, 24) + half)
                items[1](part[k][0:8])
            else:
                part.append(job(0))
                for item in items:
                    item(part[k][0:8])
            if k == marks[0]:
                do_s(NG - 1)
                do_pv(NG - 2)
            if k == marks[1]:
                do_pv(NG - 1)

        def finish(k):
            res = jobs[k](1) + part[k]
            for item in hooks.get(('p', k), ()):
                item(res[0:8])
            return res

        def put(half, j, r, v):
            xo_ref[half, pl.ds(r0 + r, v.shape[0]), j * 128:(j + 1) * 128] = v.astype(bf16)

        if odd:
            own = []
            for jp in range(2):
                m1, m2, m3, m4, m5, m6, m7 = [finish(jp * 7 + k) for k in range(7)]
                for jj, top, bot in ((0, ((m1 + m4) - m5) + m7, m2 + m4), (1, m3 + m5, ((m1 - m2) + m3) + m6)):
                    j = jp * 2 + jj
                    own.append(top[8:16])
                    put(hb, j, 0, jnp.concatenate([top[0:8], bot[24:32], top[16:32]], axis=0))
                    put(hb, j, -24, bot[16:24])
                    put(hb, j, -56, bot[8:16])
                    put(hb, j, -88, bot[0:8])
            for j in range(4):
                res = finish(14 + j)
                own.append(res[8:16])
                put(1 - hb, j, 0, res)
            new_mem = [jnp.where(hb == 0, own[j], own[(j + 4) % 8]) for j in range(8)]
        else:
            new_mem = []
            for j in range(8):
                res = finish(j)
                new_mem.append(res[8:16])
                put(j // 4, j % 4, 0, res)
        for item in hooks.get(H, ()):
            item(None)
        if odd:
            a_out(pp, hb)
            if first:
                pl.when(pp > 0)(lambda: a_out(pp - 1, hb))
            else:
                a_out(pp - 1, hb)
        return new_mem

    def l1(i, mem):
        bx_copy(i).wait()
        he = {2 * k: [p1_pre(i, k // 4, k % 4)] for k in range(16)}
        he[H] = [p1_mm(i, 1), p1_mm(i, 2), p1_mm(i, 3)]
        ho = {('p', 2): [p1_mm(i, 0)]}
        mem = step(i, 0, mem, he)
        mem = step(i, 1, mem, ho, first=True)
        return mem

    def l2(i, mem):
        u = i - N_L1
        he = {3: [p2_fwd(u, range(0, 4))], 7: [p2_fwd(u, range(4, 8))], 17: [p2_nyq(u)],
              H: [p2_inv(u, range(0, 8))]}
        ho = {('p', k): [p2_bfly(u + k % 2, k // 2, k % 2 == 0)] for k in range(16)}
        mem = step(i, 0, mem, he)
        mem = step(i, 1, mem, ho)
        return mem

    def l3(i, mem):
        p = i - N_L1 - N_L2
        he = {h: [p3_pre(p, h // 3, 1 + h % 3)] for h in range(24)}
        for j in range(4):
            he[('o', 3 + j)] = [p3_pre(p, 2 * j, 0), p3_pre(p, 2 * j + 1, 0)]
        he[H] = [p3_mm(p, q) for q in range(4)]
        ho = {12: [b_out(p)]}
        mem = step(i, 0, mem, he)
        mem = step(i, 1, mem, ho)
        return mem

    m0 = mem_ref[...].astype(f32)
    mem = [m0[:, j * 128:(j + 1) * 128] for j in range(8)]
    mem = jax.lax.fori_loop(0, N_L1, l1, mem)
    cp_x[2].wait()
    cp_x[3].wait()
    cp_ms.wait()
    for g in range(8):
        p2_bfly(0, g, False)(None)
        p2_bfly(0, g, False, ny_ref)(None)
    mem = jax.lax.fori_loop(N_L1, N_L1 + N_L2, l2, mem)
    for g in range(8):
        p2_bfly(0, g, True, ny_ref)(None)
    mem = jax.lax.fori_loop(N_L1 + N_L2, NSEG // 2, l3, mem)

    oc_last = jnp.concatenate([oc_ref[h] for h in range(H)], axis=1).astype(bf16)
    for j in range(4):
        res = _dot(oc_last, _tobf(wo_ref[0, j, 0:2048, :])).astype(bf16)
        xo_ref[0, S + 8:S + 16, j * 128:(j + 1) * 128] = res[0:8]
        xo_ref[0, S + 40:S + 48, j * 128:(j + 1) * 128] = res[8:16]
    a_out(NSEG // 2 - 1, 0)

    for k in (1, 0):
        half = out_hbm.at[:, :, pl.ds(k * DM, DM)]
        pltpu.make_async_copy(half, half, sem_out.at[k]).wait()


@jax.jit
def _run(x, mem0, wq, wk, wv, wo, bx, w_r, w_i):
    fd, ms, tv = _tables()
    hbm = pl.BlockSpec(memory_space=pl.ANY)
    out = pl.pallas_call(
        _kernel,
        out_shape=jax.ShapeDtypeStruct((4, S // 4, 2 * DM), bf16),
        in_specs=[hbm] * 13,
        out_specs=hbm,
        scratch_shapes=[
            pltpu.VMEM((2, 64 + S, DM // 2), bf16),
            pltpu.VMEM((MEM, DM), bf16),
            pltpu.VMEM((8, NSEG, 8, 128), bf16),
            pltpu.VMEM((4, DM, 16, DH), bf16),
        ] + [pltpu.VMEM((2, 8, DM // 2 + 8, DH), u32)] * 6 + [
            pltpu.VMEM((2, 4, H * DH // 2 + 8, 128), u32),
            pltpu.VMEM((8, 256, 128), u32),
            pltpu.VMEM((5, 4, 136, 128), u32),
            pltpu.VMEM((NSEG // 2, 12, 8, 8, 128), u32),
            pltpu.VMEM((2 * H, 8, 128), u32),
            pltpu.VMEM((16, H * DH), u32),
            pltpu.VMEM((H, 16, DH), f32),
            pltpu.VMEM((6, 32, 16 * DH), f32),
            pltpu.VMEM((2, 10, 1040, 128), u32),
            pltpu.VMEM((32, 128), f32),
            pltpu.VMEM((48, 128), f32),
            pltpu.VMEM((5, S // 4, DM), bf16),
            pltpu.VMEM((2, 8, DM // 2 + 1, 256), bf16),
            pltpu.VMEM((12872, 128), u32),
            pltpu.VMEM((137, 128, 128), f32),
            pltpu.VMEM((8, 128, 128), f32),
            pltpu.VMEM((12, 264, 128), f32),
            pltpu.VMEM((24, 64, 128), u32),
            pltpu.VMEM((64, 64, 128), u32),
            pltpu.VMEM((2, 512, 128), f32),
            pltpu.SMEM((64,), f32),
            pltpu.SMEM((1,), jnp.int32),
            pltpu.SemaphoreType.DMA((84,)),
            pltpu.SemaphoreType.DMA((2,)),
        ],
        compiler_params=pltpu.CompilerParams(vmem_limit_bytes=120 * 1024 * 1024,
                                             disable_semaphore_checks=True,
                                             disable_bounds_checks=True),
    )(x.reshape(S, DM), x.reshape(NSEG, SEG, DM), mem0.reshape(MEM, DM), wq, wk, wv,
      wo.reshape(H * DH // 16, 16, DM), bx.reshape(4, S // 4, DM), w_r.T, w_i.T, jnp.asarray(fd), jnp.asarray(ms), jnp.asarray(tv))
    return out.reshape(1, S, 2 * DM)


def pallas_concat_heads__memory_aug_recurrent_mem_tr__spectral_gfnet__prompt_kernel(
    A_x: jax.Array,
    A_mem0: jax.Array,
    A_Wq: jax.Array,
    A_Wk: jax.Array,
    A_Wv: jax.Array,
    A_Wo: jax.Array,
    A_seg_len,
    B_x: jax.Array,
    B_w_r: jax.Array,
    B_w_i: jax.Array,
):
    if isinstance(A_seg_len, int):
        assert A_seg_len == SEG
    assert A_x.shape == (1, S, DM) and A_mem0.shape == (1, MEM, DM) and A_Wq.shape == (DM, H, DH)
    assert B_x.shape == (1, S, DM) and B_w_r.shape == (S, DM // 2 + 1)
    return _run(A_x, A_mem0, A_Wq, A_Wk, A_Wv, A_Wo, B_x, B_w_r, B_w_i)
```

```python
import math

import numpy as np
import jax
import jax.numpy as jnp
import jax.experimental.pallas as pl
import jax.experimental.pallas.tpu as pltpu

bf16 = jnp.bfloat16
f32 = jnp.float32
u32 = jnp.uint32

S, DM = 2048, 1024
H, DH = 32, 128
MEM, SEG = 8, 32
NSEG = S // SEG
SQH = math.sqrt(0.5)

_PAIRS = ((0, 4), (1, 7), (2, 6), (3, 5))
_FIRST = np.array([[1, 1, 0, 0], [1, 0, 1, 0], [0, 1, 1, 0], [0, 1, 0, 1]], bool)


def _pack_rows(a):
    u = np.ascontiguousarray(a, dtype=np.float32).view(np.uint32).astype(np.uint64)
    b = ((u + 0x7FFF + ((u >> 16) & 1)) >> 16).astype(np.uint32)
    return (b[..., 0::2, :] | (b[..., 1::2, :] << 16)).astype(np.uint32)


def _tables():
    k2 = np.zeros((4, 128), np.int64)
    for t in range(4):
        odd = t % 2
        for lam in range(128):
            k = 2 * lam + odd
            if k % 8 not in _PAIRS[t]:
                k = 2 * (128 + 8 * (lam // 8) + (lam % 8 - 1 - odd) % 8) + odd
            assert k % 8 in _PAIRS[t]
            k2[t, lam] = k
    b = np.arange(128)[:, None]
    F = np.zeros((12, 128, 128))
    G = np.zeros((12, 128, 128))
    for t in range(4):
        th = 2 * np.pi * ((b * k2[t][None, :]) % DM) / DM
        C, Sn = np.cos(th), np.sin(th)
        first = ((k2[t] % 8) == _PAIRS[t][0])[None, :]
        assert np.array_equal(first[0], _FIRST[t][np.arange(128) % 4])
        if t == 0:
            im = -Sn
            im[:, 0] = (-1.0) ** np.arange(128)
            im = np.roll(im, 2, axis=1)
            F[1:3] = np.where(first, im, C), np.where(first, C, im)
            G[1:3] = F[1:3]
            G[2, :, 0] *= 0.5
            G[2, :, 2] *= 0.5
        else:
            Sg = np.where(first, Sn, -Sn)
            F[3 * t:3 * t + 3] = C, -(C + Sg), C - Sg
            G[3 * t:3 * t + 3] = F[3 * t:3 * t + 3]
    Finv = np.transpose(G, (0, 2, 1)) * (2.0 / DM)
    fd = _pack_rows(np.concatenate([F, Finv]))
    M = np.zeros((32, 128, 128))
    r = np.arange(64)[None, :]
    l = np.arange(64)[:, None]
    for j in range(32):
        th = 2 * np.pi * ((r * (j + 32 * l)) % S) / S
        C, Sn = np.cos(th), np.sin(th)
        M[j, :64, :64] = C
        M[j, :64, 64:] = Sn
        M[j, 64:, :64] = -Sn
        M[j, 64:, 64:] = C
    perm = np.arange(128).reshape(2, 8, 8).transpose(1, 0, 2).reshape(128)
    M = M[:, perm][:, :, perm]
    Minv = np.transpose(M, (0, 2, 1)) / S
    ms = _pack_rows(np.concatenate([M, Minv]))
    th = 2 * np.pi * np.outer(np.arange(512), np.arange(128) % 4) / S
    tv = np.stack([np.cos(th), np.sin(th)]).astype(np.float32)
    return fd, ms, tv


def _tobf(w):
    return pltpu.bitcast(w, bf16)


def _tou(w):
    return pltpu.bitcast(w, u32)


def _dot(a, b):
    return jnp.dot(a, b, preferred_element_type=f32)


def _r8_real(x):
    t0, t1 = x[0] + x[4], x[0] - x[4]
    t2, t3 = x[2] + x[6], x[2] - x[6]
    t4, t5 = x[1] + x[5], x[1] - x[5]
    t6, t7 = x[3] + x[7], x[3] - x[7]
    e0, e1 = t0 + t2, t0 - t2
    o0, o1 = t4 + t6, t4 - t6
    u, v = SQH * (t5 - t7), SQH * (t5 + t7)
    return [(e0 + o0, e0 - o0), (t1 + u, v + t3), (e1, o1), (t1 - u, v - t3)]


def _r8_real_t(g):
    (z0, z4), (a1, b1), (e1, o1), (a3, b3) = g
    e0, o0 = z0 + z4, z0 - z4
    t1, u = a1 + a3, a1 - a3
    v, t3 = b1 + b3, b1 - b3
    t5, t7 = SQH * (v + u), SQH * (v - u)
    t0, t2 = e0 + e1, e0 - e1
    t4, t6 = o0 + o1, o0 - o1
    return [t0 + t1, t4 + t5, t2 + t3, t6 + t7, t0 - t1, t4 - t5, t2 - t3, t6 - t7]


def _dft4(u):
    (r0, i0), (r1, i1), (r2, i2), (r3, i3) = u
    sr, si, dr, di = r0 + r2, i0 + i2, r0 - r2, i0 - i2
    tr, ti, er, ei = r1 + r3, i1 + i3, r1 - r3, i1 - i3
    return [(sr + tr, si + ti), (dr + ei, di - er), (sr - tr, si - ti), (dr - ei, di + er)]


def _dft8(x):
    a = [(x[p][0] + x[p + 4][0], x[p][1] + x[p + 4][1]) for p in range(4)]
    d = [(x[p][0] - x[p + 4][0], x[p][1] - x[p + 4][1]) for p in range(4)]
    ev = _dft4(a)
    (r0, i0), (r1, i1), (r2, i2), (r3, i3) = d
    b1r, b1i = SQH * (r1 + i1), SQH * (i1 - r1)
    b3r, n3i = SQH * (i3 - r3), SQH * (r3 + i3)
    sr, si, dr, di = r0 + i2, i0 - r2, r0 - i2, i0 + r2
    tr, ti, er, ei = b1r + b3r, b1i - n3i, b1r - b3r, b1i + n3i
    od = [(sr + tr, si + ti), (dr + ei, di - er), (sr - tr, si - ti), (dr - ei, di + er)]
    return [ev[0], od[0], ev[1], od[1], ev[2], od[2], ev[3], od[3]]


def _swap(x):
    return [(b, a) for (a, b) in x]


G = 4
NG = H // G
NEG = -1e9
N_L1, N_L2 = 8, 16


def _kernel(x_hbm, x3_hbm, mem_hbm, wq_hbm, wk_hbm, wv_hbm, wo_hbm, bx_hbm, wr_hbm, wi_hbm,
            fd_hbm, ms_hbm, tv_hbm, out_hbm,
            xo_ref, mem_ref, xcraw_ref, raw_ref, w0_ref, w1_ref, w2_ref, w3_ref, w4_ref, w5_ref,
            wo_ref, xc_ref, xs_ref, qkvc_ref, kve_ref,
            oall_ref, oc_ref, os_ref, ws_ref, fille_ref, fillo_ref,
            bx_ref, wt_ref, wp_ref, ub_ref, ny_ref, sa_ref, fd_ref, ms_ref, tv_ref,
            tw_ref, zero_ref, sem_in, sem_out):
    scale = DH ** -0.5
    w_hbm = (wq_hbm, wk_hbm, wv_hbm)
    w_refs = (w0_ref, w1_ref, w2_ref, w3_ref, w4_ref, w5_ref)

    def raw_copy(c, i=0, nd=DM):
        rows = pl.ds(pl.multiple_of(i * nd, nd), nd)
        return pltpu.make_async_copy(
            w_hbm[c // 2].at[rows, pl.ds((c % 2) * 16, 16), :],
            raw_ref.at[c % 4, rows], sem_in.at[8 + min(c, 3) * 8 + max(c - 3, 0) * 2 + i])

    def xc_copy(k):
        return pltpu.make_async_copy(
            x3_hbm.at[:, pl.ds(8, 8), pl.ds(pl.multiple_of(k * 128, 128), 128)], xcraw_ref.at[k], sem_in.at[40 + k])

    def wo_copies(half):
        return [pltpu.make_async_copy(wo_hbm.at[:, :, pl.ds(pl.multiple_of(half * 512 + j * 128, 128), 128)],
                                      raw_ref.at[2 + half, j * 256:(j + 1) * 256], sem_in.at[76 + half * 4 + j])
                for j in range(4)]

    def wt_copies(i):
        return [pltpu.make_async_copy(src.at[:, pl.ds(pl.multiple_of(i * 1024 + k * 256, 256), 256)],
                                      wt_ref.at[i, a * 4 + k], sem_in.at[i * 4 + (48 + a * 8 + k)])
                for k in range(4) for a, src in enumerate((wr_hbm, wi_hbm))]

    def bx_copy(p):
        rows = pl.ds(pl.multiple_of(p * 64, 64), 64)
        return pltpu.make_async_copy(bx_hbm.at[:, rows, :], bx_ref.at[0:4, rows, :], sem_in.at[64 + p])

    n_head = N_L1 * 2 * SEG
    cp_x = [pltpu.make_async_copy(x_hbm.at[lo:hi, half * 512:(half + 1) * 512], xo_ref.at[half, 64 + lo:64 + hi],
                                  sem_in.at[72 + (lo > 0) * 2 + half])
            for lo, hi in ((0, n_head), (n_head, S)) for half in range(2)]
    cp_mem = pltpu.make_async_copy(mem_hbm, mem_ref, sem_in.at[1])
    cp_fd = pltpu.make_async_copy(fd_hbm, fd_ref, sem_in.at[4])
    cp_ms = pltpu.make_async_copy(ms_hbm, ms_ref, sem_in.at[5])
    cp_tv = pltpu.make_async_copy(tv_hbm, tv_ref, sem_in.at[6])

    for i in range(8):
        raw_copy(0, i, 128).start()
        xc_copy(i).start()
        if i >= 4:
            raw_copy(2, i - 4, 192).start()
        raw_copy(1, i, 128).start()
    raw_copy(2, 6, 128).start()
    raw_copy(2, 7, 128).start()
    for i in range(2):
        raw_copy(3, i, 512).start()

    zero_ref[0] = 0

    def pin_bit():
        return jnp.clip(zero_ref[0], 0, 1)

    def pin_rows(r):
        return pl.ds(pl.multiple_of(r + pin_bit() * 32, 8), 8)

    for p in range(8):
        for jq in range(4):
            tw_ref[(p * 4 + jq) * 2] = jnp.float32(math.cos(2 * math.pi * p * jq / 32))
            tw_ref[(p * 4 + jq) * 2 + 1] = jnp.float32(math.sin(2 * math.pi * p * jq / 32))

    ub_ref[128:136] = jnp.zeros((8, 128, 128), f32)
    wp_ref[12800:12872] = jnp.zeros((72, 128), u32)
    oc_ref[...] = jnp.zeros((H, 16, DH), f32)

    qi = jax.lax.broadcasted_iota(jnp.int32, (48, 128), 0)
    ki = jax.lax.broadcasted_iota(jnp.int32, (48, 128), 1)

    def between(v, lo, hi):
        return (v >= lo) & (v < hi)

    def table(keep, other):
        return jnp.where(other, -jnp.inf, jnp.where(keep, 0.0, NEG)).astype(f32)

    keep = between(qi, 8, 16) | between(ki, 8, 16) | (qi >= jnp.where(ki < 32, ki, ki - 24))
    fille_ref[...] = table(keep, ki >= 40)[:32]
    q_even = between(qi, 32, 40)
    k_even = between(ki, 32, 40) | (ki >= 48)
    qpos = jnp.where(qi < 32, qi, jnp.where(qi < 40, qi - 24, qi - 32))
    kpos = jnp.where(ki < 32, ki, jnp.where(ki < 40, ki - 24, jnp.where(ki < 48, ki - 32, ki - 48)))
    keep = between(qi, 8, 16) | between(ki, 8, 16) | (ki >= 56) | (qpos >= kpos)
    fillo_ref[...] = table(keep, (q_even != k_even) | (ki >= 64))

    def relayout16(c, blk):
        w0 = pl.multiple_of(blk * 8, 8)
        v = _tou(raw_ref[c % 4, pl.ds(blk * 16, 16)]).reshape(8, 2, 8, 128)
        a, b = v[:, 0], v[:, 1]
        w_refs[c][0, :, pl.ds(w0, 8), :] = jnp.swapaxes((a & jnp.uint32(0xFFFF)) | (b << 16), 0, 1)
        w_refs[c][1, :, pl.ds(w0, 8), :] = jnp.swapaxes((a >> 16) | (b & jnp.uint32(0xFFFF0000)), 0, 1)

    def slot_of(h):
        return (h // 16) * 16 + (h % 2) * 8 + (h % 16) // 2

    def repack_wo(half, part, k):
        jp, g0 = k & 1, part * 128 + (k >> 1) * 2
        quad = []
        for jj in range(2):
            for kh in range(2):
                v = _tou(raw_ref[2 + half, pl.ds((jp * 2 + jj) * 256 + kh * 64 + g0, 2)]).reshape(16, 128)
                wo_ref[half, jp * 2 + jj, pl.ds(pl.multiple_of(g0 * 8 + kh * 512, 16), 16), :] = v
                quad.append(_tobf(v).astype(f32))
        b11, b21, b12, b22 = quad
        rows = pl.ds(pl.multiple_of(part * 512 + (k >> 1) * 16, 16), 16)
        for n, v in enumerate((b11 + b22, b12 - b22, b21 - b11, b11 + b12, b21 + b22)):
            ws_ref[half, jp * 5 + n, rows, :] = _tou(v.astype(bf16))

    sub4 = jax.lax.broadcasted_iota(jnp.int32, (128, 128), 0) & 3

    def wp_store(t, kb, tile):
        v = tile.T.reshape(4, 32, 128)
        v = jnp.concatenate([v, v[:, 0:8]], axis=1).reshape(160, 128)
        wp_ref[pl.ds(pl.multiple_of(t * 2560 + kb * 160, 32), 160), :] = v

    def b_prep(i, k, hb, par):
        cols = slice(hb * 128, (hb + 1) * 128)
        a = _tou(wt_ref[i, k, 0:512, cols])
        b = _tou(wt_ref[i, 4 + k, 0:512, cols])
        if par == 0:
            w = (a << 16) | (b & jnp.uint32(0xFFFF))
            m = (sub4 == 0) | (sub4 == 2)
        else:
            w = (a & jnp.uint32(0xFFFF0000)) | (b >> 16)
            m = (sub4 == 0) | (sub4 == 3)
        top = w[:128]
        bot = pltpu.roll(w[128:].reshape(16, 8, 128), 1 + par, 1).reshape(128, 128)
        wp_store(par, i * 8 + (k * 2 + hb), jnp.where(m, top, bot))
        wp_store(par + 2, i * 8 + (k * 2 + hb), jnp.where(m, bot, top))
        if par == 0:
            na = jnp.broadcast_to(wt_ref[i, k, 512:513, cols].astype(f32), (128, 128))
            nb = jnp.broadcast_to(wt_ref[i, 4 + k, 512:513, cols].astype(f32), (128, 128))
            wp_store(4, i * 8 + (k * 2 + hb), pltpu.bitcast(na, u32) | (pltpu.bitcast(nb, u32) >> 16))

    def gather_c(k):
        xc_ref[k] = _tou(xcraw_ref[k].astype(f32).reshape(512, 128).astype(bf16))

    def store_qkvc(n, y):
        qkvc_ref[:, n // 8, n % 8] = y.reshape(NSEG // 2, 8, 128)

    def q_unit(i, groups, first, last, fillers):
        xk = _tobf(xc_ref[i])
        w0 = pl.multiple_of(i * 64, 64)
        for g in groups:
            rhs = jnp.concatenate(
                [_tobf(w_refs[h // 16][h // 8 % 2, h % 8, pl.ds(w0, 64), :]) for h in range(4 * g, 4 * g + 4)], axis=1)
            y = _dot(xk, rhs)
            for h in range(4 * g, 4 * g + 4):
                yh = y[:, (h % 4) * 128:(h % 4 + 1) * 128]
                if not first:
                    yh = yh + ub_ref[h * 4:(h + 1) * 4].reshape(512, 128)
                if last:
                    store_qkvc(h, _tou(yh.astype(bf16)))
                else:
                    ub_ref[h * 4:(h + 1) * 4] = yh.reshape(4, 128, 128)
            mine = fillers.get(g, [])
            for fi, item in enumerate(mine):
                r = (fi * 512 // len(mine)) // 8 * 8
                item(pltpu.bitcast(y[r:r + 8, 0:128], u32))

    def rl_item(c, blk):
        def item(pin):
            w_refs[c][pin_bit(), 7, 512:520] = pin
            relayout16(c, blk)
        return item

    def spread(fillers, items, groups):
        for k, item in enumerate(items):
            fillers.setdefault(groups[k * len(groups) // len(items)], []).append(item)
        return fillers

    def half_items(f, c, i, groups):
        return spread(f, [rl_item(c, i * 8 + blk) for blk in range(8)], groups)

    def piece_items(i):
        f = half_items(half_items({}, 1, i, (0, 1, 2)), 0, i + 1, (4, 5, 6))
        return spread(f, [lambda pin: gather_c(i + 1)], (7,))

    def chunk2_items(f, lo, hi, groups):
        return spread(f, [rl_item(2, blk) for blk in range(lo, hi)], groups)

    def wait_piece(i):
        raw_copy(1, i, 128).wait()
        raw_copy(0, i + 1, 128).wait()
        xc_copy(i + 1).wait()

    raw_copy(0, 0, 128).wait()
    for blk in range(8):
        relayout16(0, blk)
    xc_copy(0).wait()
    gather_c(0)
    q_unit(0, range(0, 2), True, False, {})
    raw_copy(1, 0, 128).wait()
    q_unit(0, range(2, 4), True, False, half_items({}, 1, 0, (2, 2, 3)))
    q_unit(0, range(4, 6), True, False, {})
    xc_copy(1).wait()
    raw_copy(0, 1, 128).wait()
    q_unit(0, range(6, 8), True, False,
           spread(half_items({}, 0, 1, (6, 6, 7)), [lambda pin: gather_c(1)], (6,)))
    raw_copy(1, 1, 128).wait()
    q_unit(1, range(0, 4), False, False, half_items({}, 1, 1, (0, 1, 2)))
    xc_copy(2).wait()
    raw_copy(0, 2, 128).wait()
    q_unit(1, range(4, 8), False, False,
           spread(half_items({}, 0, 2, (4, 5, 6)), [lambda pin: gather_c(2)], (6,)))

    def xsum_item(j, rq):
        def item(pin):
            xs_ref[pin_bit(), 0, 128:136] = pin
            a11, a21, a12, a22 = [
                xcraw_ref[j + 4 * kh, rh * 32 + rq * 8:rh * 32 + (rq + 1) * 8].astype(f32).reshape(64, 128)
                for kh in range(2) for rh in range(2)]
            for k, v in enumerate((a11 + a22, a21 + a22, a11 + a12, a21 - a11, a12 - a22)):
                xs_ref[k, j, rq * 32:(rq + 1) * 32] = _tou(v.astype(bf16))
        return item

    wait_piece(2)
    q_unit(2, range(8), False, False, piece_items(2))

    def q_c(i, carry):
        wait_piece(i)
        raw_copy(2, i - 3, 192).wait()
        f = spread(piece_items(i), [rl_item(2, (i - 3) * 12 + blk) for blk in range(12)],
                   (2, 3, 3, 3, 3, 3, 4, 4, 5, 6, 6, 7))
        q_unit(i, range(8), False, False, spread(f, [xsum_item(i - 3, rq) for rq in range(4)], (3, 4, 5, 6)))
        return carry
    jax.lax.fori_loop(3, 7, q_c, 0)

    raw_copy(1, 7, 128).wait()
    raw_copy(2, 6, 128).wait()
    raw_copy(2, 7, 128).wait()
    q_unit(7, range(8), False, True, chunk2_items(half_items({}, 1, 7, (0, 1, 2)), 48, 64, (3, 4, 5, 6)))
    raw_copy(4).start()
    for cp in wo_copies(0):
        cp.start()
    raw_copy(5).start()

    def bulk_iter(c, i):
        def xs(k):
            return jnp.concatenate([_tobf(xs_ref[k, j, 0:128]) for j in range(4)], axis=1)

        def xc(rh, kh):
            return jnp.concatenate(
                [_tobf(xc_ref[4 * kh + j, rh * 128:(rh + 1) * 128]) for j in range(4)], axis=1)

        for pr in range(4):
            n1, n2 = pr * 2, pr * 2 + 1

            def w(n, kh):
                return _tobf(w_refs[c][i, n, kh * 256:(kh + 1) * 256])

            def wsum(a, b, sign):
                a, b = a.astype(f32), b.astype(f32)
                return (a + b if sign > 0 else a - b).astype(bf16)

            def out(rh, n, v):
                qkvc_ref[rh * 16:(rh + 1) * 16, c * 2 + i, n] = _tou(v.astype(bf16)).reshape(16, 8, 128)

            def side(k, m):
                blks = (k, 7) if k == 0 else (k,)
                items = []
                if c < 5:
                    items += [('w', blk) for blk in blks]
                if c >= 4:
                    items += [('o', blk) for blk in range(k * 16 // 7, (k + 1) * 16 // 7)]
                if c == 5 and k in (1, 2, 4, 5):
                    items.append(('f', (1, 2, 4, 5).index(k)))
                for n, (kind, blk) in enumerate(items):
                    r = n * 256 // len(items) // 8 * 8
                    pin = pltpu.bitcast(m[r:r + 8], u32)
                    if kind == 'w':
                        w_refs[c + 1][pin_bit(), 7, 512:520] = pin
                        relayout16(c + 1, i * 32 + (pr * 8 + blk))
                    elif kind == 'o':
                        ws_ref[pin_bit(), 9, 1024:1032] = pin
                        wo_ref[pin_bit(), 3, 2048:2056] = pin
                        repack_wo(c - 4, i, pr * 16 + blk)
                    else:
                        wp_ref[pin_rows(12832), :] = pin
                        b_prep(i, pr, blk // 2, blk % 2)

            m2 = _dot(xs(1), w(n1, 0))
            side(0, m2)
            m4 = _dot(xc(1, 1), wsum(w(n1, 1), w(n1, 0), -1))
            side(1, m4)
            out(1, n1, m4 + m2)
            m1 = _dot(xs(0), wsum(w(n1, 0), w(n2, 1), 1))
            side(2, m1)
            m5 = _dot(xs(2), w(n2, 1))
            side(3, m5)
            m3 = _dot(xc(0, 0), wsum(w(n2, 0), w(n2, 1), -1))
            side(4, m3)
            out(0, n2, m3 + m5)
            c22 = _dot(xs(3), wsum(w(n1, 0), w(n2, 0), 1)) + ((m1 - m2) + m3)
            side(5, c22)
            out(1, n2, c22)
            c11 = _dot(xs(4), wsum(w(n1, 1), w(n2, 1), 1)) + ((m1 + m4) - m5)
            side(6, c11)
            out(0, n1, c11)

    for c in range(2, 6):
        if c == 3:
            for cp in wo_copies(1) + wt_copies(0) + wt_copies(1):
                cp.start()
        if c == 4:
            for cp in cp_x[0:2] + [cp_mem, cp_fd, cp_tv] + [bx_copy(p) for p in range(8)] + cp_x[2:4] + [cp_ms]:
                cp.start()
        if c >= 4:
            for cp in wo_copies(c - 4):
                cp.wait()
        if 2 < c < 5:
            raw_copy(c + 1).wait()

        def bulk(i, carry, c=c):
            if c == 2:
                raw_copy(3, i, 512).wait()
            if c == 5:
                for cp in wt_copies(i):
                    cp.wait()
            bulk_iter(c, i)
            return carry
        jax.lax.fori_loop(0, 2, bulk, 0)

    cp_x[0].wait()
    cp_x[1].wait()
    cp_mem.wait()
    cp_fd.wait()
    cp_tv.wait()

    lane = jax.lax.broadcasted_iota(jnp.int32, (1, 128), 1)
    lane0 = lane == 0
    sgn0 = jnp.where(lane0, 1.0, -1.0)

    def first_lanes(t):
        la, lb = [k for k in range(4) if _FIRST[t][k]]
        return ((lane & 3) == la) | ((lane & 3) == lb)

    def d_products(st_ref, d, t, rows):
        return [_dot(st_ref[n, rows].astype(bf16), _tobf(fd_ref[d * 12 + n])) if n else None
                for n in range(3 * t, 3 * t + 3)]

    def twiddles(p):
        return [(tw_ref[p * 8 + jq * 2], tw_ref[p * 8 + jq * 2 + 1]) if jq else None for jq in range(4)]

    def p1_pre(p, rs, q):
        def item(y):
            sa_ref[0, pin_rows(0), :] = y
            xq = bx_ref[q, pl.ds(pl.multiple_of(p * 64 + rs * 16, 16), 16), :].astype(f32)
            zz = _r8_real([xq[:, a * 128:(a + 1) * 128] for a in range(8)])
            r = (rs * 4 + q) * 16
            sa_ref[1:12, r:r + 16] = jnp.stack([v for (a, b) in zz for v in (a + b, b, a)][1:])
        return item

    def p1_mm(p, t):
        def item(y):
            cs = twiddles(p)

            def put(ref, n, rs, re, im):
                v = jnp.stack([re.reshape(2, 8, 128), im.reshape(2, 8, 128)], axis=1)
                ref[n * 8 + p, rs * 32:(rs + 1) * 32] = v.reshape(32, 128)

            first = first_lanes(t)
            for rs in range(4):
                k1, k2, k3 = d_products(sa_ref, 0, t, slice(rs * 64, (rs + 1) * 64))
                if t == 0:
                    up = jnp.where(first, k2, k3)
                    re, im = jnp.where(first, k3, k2), pltpu.roll(up, 126, 1)
                    ny = jnp.where(lane0, im, up)
                    u = [ny[q * 16:(q + 1) * 16] for q in range(4)]
                    odd_lane = (lane & 1) == 1
                    nr = jnp.where(odd_lane, pltpu.roll(u[0] - u[2], 1, 1), u[0] + u[2] + (u[1] + u[3]) * sgn0)
                    ni = jnp.where(odd_lane, pltpu.roll((u[3] - u[1]) * sgn0, 1, 1), 0.0)
                    rows = pl.ds(pl.multiple_of(p * 64 + rs * 16, 16), 16)
                    c, sn = tv_ref[0, rows], tv_ref[1, rows]
                    put(ny_ref, 0, rs, nr * c + ni * sn, ni * c - nr * sn)
                    im = jnp.where(lane0, 0.0, im)
                else:
                    re, im = k1 + k2, (k3 - k1) * jnp.where(first, 1.0, -1.0)
                a = _dft4([(re[q * 16:(q + 1) * 16], im[q * 16:(q + 1) * 16]) for q in range(4)])
                for jq in range(4):
                    re, im = a[jq]
                    if jq > 0:
                        c, sn = cs[jq]
                        re, im = re * c + im * sn, im * c - re * sn
                    put(ub_ref, t * 4 + jq, rs, re, im)
        return item

    def p2_bfly(u, g, inverse, ref=ub_ref):
        def item(y):
            if y is not None:
                ub_ref[136, pin_rows(0), :] = y
            v = ref[pl.ds(u * 8, 8), g * 16:(g + 1) * 16]
            x = [(v[p, 0:8], v[p, 8:16]) for p in range(8)]
            x = _swap(_dft8(_swap(x))) if inverse else _dft8(x)
            ref[pl.ds(u * 8, 8), g * 16:(g + 1) * 16] = jnp.stack([w for c in x for w in c]).reshape(8, 16, 128)
        return item

    def filtered(xx, w):
        wr = pltpu.bitcast(w & jnp.uint32(0xFFFF0000), f32).reshape(8, 8, 128)
        wi = pltpu.bitcast(w << 16, f32).reshape(8, 8, 128)
        xx = xx.reshape(8, 2, 8, 128)
        xr, xi = xx[:, 0], xx[:, 1]
        return jnp.stack([xr * wr - xi * wi, xr * wi + xi * wr], axis=1).reshape(128, 128)

    def p2_fwd(u, jps):
        def item(y):
            t = u >> 2
            jq = u & 3
            xs = [_dot(_tobf(ms_ref[jq + 4 * jp]), ub_ref[u * 8 + jp].astype(bf16)) for jp in jps]
            for jp, xx in zip(jps, xs):
                ub_ref[u * 8 + jp] = filtered(xx, wp_ref[pl.ds(t * 2560 + jq + 4 * jp, 64, stride=40), :])
        return item

    def p2_nyq(u):
        def item(y):
            jp = u & 7
            rhs = ny_ref[jp].astype(bf16)
            xx = jnp.concatenate([_dot(_tobf(ms_ref[u * 4, m * 16:(m + 1) * 16]), rhs) for m in range(4)], axis=0)
            w = wp_ref[pl.ds(4 * 2560 + 4 * jp, 64, stride=40), :]
            for jq in range(1, 4):
                w = jnp.where(lane == jq, wp_ref[pl.ds(4 * 2560 + 4 * jp + jq, 64, stride=40), :], w)
            w = jnp.where(u < 8, w, jnp.uint32(0x3F800000))
            ny_ref[jp] = filtered(xx, w)
        return item

    def p2_inv(u, jps):
        def item(y):
            jq = u & 3
            zs = [_dot(_tobf(ms_ref[32 + jq + 4 * jp]), ub_ref[u * 8 + jp].astype(bf16)) for jp in jps]
            for jp, zz in zip(jps, zs):
                ub_ref[u * 8 + jp] = zz
        return item

    def p3_pre(p, g, t):
        def item(y):
            sa_ref[0, pin_rows(0), :] = y
            cs = twiddles(p)

            def fetch(t):
                a = []
                for jq in range(4):
                    v = ub_ref[(t * 4 + jq) * 8 + p, g * 16:(g + 1) * 16]
                    re, im = v[0:8], v[8:16]
                    if jq > 0:
                        c, sn = cs[jq]
                        re, im = re * c - im * sn, im * c + re * sn
                    a.append((re, im))
                return _swap(_dft4(_swap(a)))

            u = fetch(t)
            if t == 0:
                v = ny_ref[p, g * 16:(g + 1) * 16]
                rows = pl.ds(pl.multiple_of(p * 64 + g * 8, 8), 8)
                c, sn = tv_ref[0, rows], tv_ref[1, rows]
                nr, ni = v[0:8] * c - v[8:16] * sn, v[8:16] * c + v[0:8] * sn
                zr, zi = pltpu.roll(nr, 127, 1), pltpu.roll(ni, 127, 1)
                ny = (nr + zr, (nr - zi) * sgn0, nr - zr, (nr + zi) * sgn0)
            first = first_lanes(t)
            for q in range(4):
                re, im = u[q]
                rows = slice(q * 64 + g * 8, q * 64 + (g + 1) * 8)
                if t == 0:
                    im = pltpu.roll(jnp.where(lane0, ny[q], im), 2, 1) + jnp.where(lane == 2, ny[q], 0.0)
                    sa_ref[1:3, rows] = jnp.stack((jnp.where(first, im, re), jnp.where(first, re, im)))
                else:
                    im = im * jnp.where(first, 1.0, -1.0)
                    sa_ref[3 * t:3 * t + 3, rows] = jnp.stack((re + im, im, re))
        return item

    def p3_mm(p, q):
        def item(y):
            g = []
            for t in range(4):
                k1, k2, k3 = d_products(sa_ref, 1, t, slice(q * 64, (q + 1) * 64))
                g.append((k3, k2) if t == 0 else (k2 + k1, k3 - k1))
            yy = _r8_real_t(g)
            bx_ref[q, pl.ds(pl.multiple_of(p * 64, 64), 64), :] = jnp.concatenate(yy, axis=1).astype(bf16)
        return item

    def b_out(p):
        def item(y):
            rows = pl.ds(pl.multiple_of(p * 64, 64), 64)
            pltpu.make_async_copy(bx_ref.at[0:4, rows, :], out_hbm.at[:, rows, pl.ds(DM, DM)],
                                  sem_out.at[1]).start()
            bx_ref[4, pin_rows(0), 0:128] = y.astype(bf16)
        return item

    def a_out(blk, half):
        pltpu.make_async_copy(
            xo_ref.at[half, pl.ds(pl.multiple_of(blk * 64 + 64, 64), 64), :],
            out_hbm.at[blk >> 3, pl.ds(pl.multiple_of((blk & 7) * 64, 64), 64),
                       pl.ds(pl.multiple_of(half * 512, 512), 512)],
            sem_out.at[0]).start()

    def step(pp, odd, mem, hooks, first=False):
        r0 = pl.multiple_of(pp * 64 + (64 + 32 * odd), SEG)
        xs = jnp.concatenate([xo_ref[0, pl.ds(r0, SEG), :], xo_ref[1, pl.ds(r0, SEG), :]], axis=1)
        x_lo = xs[0:8].astype(f32)
        hm = jnp.concatenate(
            [jnp.concatenate([x_lo, jnp.concatenate(mem, axis=1)], axis=0).astype(bf16), xs[16:32]], axis=0)
        fill = fillo_ref[:, 0:64] if odd else fille_ref[:, 0:48]
        qkv, ps = {}, {}

        def head_of(v):
            return (v // 16) * 16 + (v % 2) * 8 + (v % 16) // 2 if odd else v

        def do_qkv(v0, v1):
            for v in range(v0, v1):
                h = head_of(v)
                for t in range(3):
                    n = t * H + slot_of(h)
                    y32 = _dot(hm, _tobf(w_refs[n // 16][n // 8 % 2, n % 8, 0:512]))
                    parts = [y32]
                    if odd or t > 0:
                        parts.append(_tobf(qkvc_ref[pp, n // 8, n % 8]).astype(f32))
                    if t > 0:
                        if odd:
                            parts.append(kve_ref[(t - 1) * H + h])
                        else:
                            kve_ref[(t - 1) * H + h] = y32[0:16]
                    qkv[(t, v)] = jnp.concatenate(parts, axis=0).astype(bf16)
                for item in hooks.get(v, ()):
                    item(y32[0:8])

        def do_s(g):
            for v in range(g * G, (g + 1) * G):
                sc = jax.lax.dot_general(qkv[(0, v)], qkv[(1, v)], (((1,), (1,)), ((), ())),
                                         preferred_element_type=f32)
                sc = jnp.where(fill == 0.0, sc * scale, fill)
                e = jnp.exp(sc - jnp.max(sc, axis=1, keepdims=True))
                den = jnp.sum(e, axis=1, keepdims=True)
                r = pl.reciprocal(den, approx=True)
                r = r * (2.0 - den * r)
                ps[v] = (e * r).astype(bf16)

        def do_pv(g):
            o = {v: _dot(ps[v], qkv[(2, v)]) for v in range(g * G, (g + 1) * G)}
            for v in o:
                h = head_of(v)
                oall_ref[:, h * DH:(h + 1) * DH] = _tou(o[v][0:32].astype(bf16))
            if odd:
                for v in range(g * G, (g + 1) * G, 2):
                    a11, a12 = o[v][0:32], o[v + 1][0:32]
                    a21 = jnp.concatenate([oc_ref[head_of(v)], o[v][32:48]], axis=0)
                    a22 = jnp.concatenate([oc_ref[head_of(v + 1)], o[v + 1][32:48]], axis=0)
                    for k, a in enumerate((a11 + a22, a21 + a22, a22, a11 + a12, a21 - a11, a12 - a22)):
                        os_ref[k, :, (v // 2) * DH:(v // 2 + 1) * DH] = a
                for v in o:
                    oc_ref[head_of(v)] = o[v][32:48]

        def plain(half, j, h0, h1):
            return _dot(_tobf(oall_ref[:, h0 * DH:h1 * DH]), _tobf(wo_ref[half, j, h0 * 64:h1 * 64, :]))

        hb = pp & 1
        if odd:
            def product(jp, k):
                def fn(part):
                    h0 = part * 16
                    if k == 2:
                        lhs = _tobf(oall_ref[:, h0 * DH:(h0 + 8) * DH])
                    else:
                        lhs = os_ref[k - (k > 2), :, part * 1024:(part + 1) * 1024].astype(bf16)
                    if k == 1:
                        rhs = wo_ref[hb, jp * 2, h0 * 64:(h0 + 8) * 64, :]
                    elif k == 4:
                        rhs = wo_ref[hb, jp * 2 + 1, (h0 + 8) * 64:(h0 + 16) * 64, :]
                    else:
                        rhs = ws_ref[hb, jp * 5 + (0, 0, 1, 2, 0, 3, 4)[k], part * 512:(part + 1) * 512, :]
                    return _dot(lhs, _tobf(rhs))
                return fn
            jobs = [product(jp, k) for jp in range(2) for k in range(7)]
            jobs += [(lambda part, j=j: plain(1 - hb, j, part * 16, part * 16 + 16)) for j in range(4)]
            marks = (2, 10)
        else:
            jobs = [(lambda part, j=j: plain(j // 4, j % 4, part * 24, 24 + part * 8)) for j in range(8)]
            marks = (2, 5)

        for g in range(NG):
            do_qkv(g * G, g * G + G // 2)
            if g >= 1:
                do_s(g - 1)
            do_qkv(g * G + G // 2, (g + 1) * G)
            if g >= 2:
                do_pv(g - 2)
        part = []
        for k, job in enumerate(jobs):
            items = hooks.get(('o', k), ())
            if len(items) == 2:
                half = plain(k // 4, k % 4, 0, 12)
                items[0](half[0:8])
                part.append(plain(k // 4, k % 4, 12, 24) + half)
                items[1](part[k][0:8])
            else:
                part.append(job(0))
                for item in items:
                    item(part[k][0:8])
            if k == marks[0]:
                do_s(NG - 1)
                do_pv(NG - 2)
            if k == marks[1]:
                do_pv(NG - 1)

        def finish(k):
            res = jobs[k](1) + part[k]
            for item in hooks.get(('p', k), ()):
                item(res[0:8])
            return res

        def put(half, j, r, v):
            xo_ref[half, pl.ds(r0 + r, v.shape[0]), j * 128:(j + 1) * 128] = v.astype(bf16)

        if odd:
            own = []
            for jp in range(2):
                m1, m2, m3, m4, m5, m6, m7 = [finish(jp * 7 + k) for k in range(7)]
                for jj, top, bot in ((0, ((m1 + m4) - m5) + m7, m2 + m4), (1, m3 + m5, ((m1 - m2) + m3) + m6)):
                    j = jp * 2 + jj
                    own.append(top[8:16])
                    put(hb, j, 0, jnp.concatenate([top[0:8], bot[24:32], top[16:32]], axis=0))
                    put(hb, j, -24, bot[16:24])
                    put(hb, j, -56, bot[8:16])
                    put(hb, j, -88, bot[0:8])
            for j in range(4):
                res = finish(14 + j)
                own.append(res[8:16])
                put(1 - hb, j, 0, res)
            new_mem = [jnp.where(hb == 0, own[j], own[(j + 4) % 8]) for j in range(8)]
        else:
            new_mem = []
            for j in range(8):
                res = finish(j)
                new_mem.append(res[8:16])
                put(j // 4, j % 4, 0, res)
        for item in hooks.get(H, ()):
            item(None)
        if odd:
            a_out(pp, hb)
            if first:
                pl.when(pp > 0)(lambda: a_out(pp - 1, hb))
            else:
                a_out(pp - 1, hb)
        return new_mem

    def l1(i, mem):
        bx_copy(i).wait()
        he = {2 * k: [p1_pre(i, k // 4, k % 4)] for k in range(16)}
        he[H] = [p1_mm(i, 1), p1_mm(i, 2), p1_mm(i, 3)]
        ho = {('p', 2): [p1_mm(i, 0)]}
        mem = step(i, 0, mem, he)
        mem = step(i, 1, mem, ho, first=True)
        return mem

    def l2(i, mem):
        u = i - N_L1
        he = {3: [p2_fwd(u, range(0, 4))], 7: [p2_fwd(u, range(4, 8))], 17: [p2_nyq(u)],
              H: [p2_inv(u, range(0, 8))]}
        ho = {('p', k): [p2_bfly(u + k % 2, k // 2, k % 2 == 0)] for k in range(16)}
        mem = step(i, 0, mem, he)
        mem = step(i, 1, mem, ho)
        return mem

    def l3(i, mem):
        p = i - N_L1 - N_L2
        he = {h: [p3_pre(p, h // 3, 1 + h % 3)] for h in range(24)}
        for j in range(4):
            he[('o', 3 + j)] = [p3_pre(p, 2 * j, 0), p3_pre(p, 2 * j + 1, 0)]
        he[H] = [p3_mm(p, q) for q in range(4)]
        ho = {12: [b_out(p)]}
        mem = step(i, 0, mem, he)
        mem = step(i, 1, mem, ho)
        return mem

    m0 = mem_ref[...].astype(f32)
    mem = [m0[:, j * 128:(j + 1) * 128] for j in range(8)]
    mem = jax.lax.fori_loop(0, N_L1, l1, mem)
    for g in range(8):
        p2_bfly(0, g, False)(None)
        p2_bfly(0, g, False, ny_ref)(None)
    cp_x[2].wait()
    cp_x[3].wait()
    cp_ms.wait()
    mem = jax.lax.fori_loop(N_L1, N_L1 + N_L2, l2, mem)
    for g in range(8):
        p2_bfly(0, g, True, ny_ref)(None)
    mem = jax.lax.fori_loop(N_L1 + N_L2, NSEG // 2, l3, mem)

    oc_last = jnp.concatenate([oc_ref[h] for h in range(H)], axis=1).astype(bf16)
    for j in range(4):
        res = _dot(oc_last, _tobf(wo_ref[0, j, 0:2048, :])).astype(bf16)
        xo_ref[0, S + 8:S + 16, j * 128:(j + 1) * 128] = res[0:8]
        xo_ref[0, S + 40:S + 48, j * 128:(j + 1) * 128] = res[8:16]
    a_out(NSEG // 2 - 1, 0)

    for k in (1, 0):
        half = out_hbm.at[:, :, pl.ds(k * DM, DM)]
        pltpu.make_async_copy(half, half, sem_out.at[k]).wait()


@jax.jit
def _run(x, mem0, wq, wk, wv, wo, bx, w_r, w_i):
    fd, ms, tv = _tables()
    hbm = pl.BlockSpec(memory_space=pl.ANY)
    out = pl.pallas_call(
        _kernel,
        out_shape=jax.ShapeDtypeStruct((4, S // 4, 2 * DM), bf16),
        in_specs=[hbm] * 13,
        out_specs=hbm,
        scratch_shapes=[
            pltpu.VMEM((2, 64 + S, DM // 2), bf16),
            pltpu.VMEM((MEM, DM), bf16),
            pltpu.VMEM((8, NSEG, 8, 128), bf16),
            pltpu.VMEM((4, DM, 16, DH), bf16),
        ] + [pltpu.VMEM((2, 8, DM // 2 + 8, DH), u32)] * 6 + [
            pltpu.VMEM((2, 4, H * DH // 2 + 8, 128), u32),
            pltpu.VMEM((8, 256, 128), u32),
            pltpu.VMEM((5, 4, 136, 128), u32),
            pltpu.VMEM((NSEG // 2, 12, 8, 8, 128), u32),
            pltpu.VMEM((2 * H, 16, 128), f32),
            pltpu.VMEM((16, H * DH), u32),
            pltpu.VMEM((H, 16, DH), f32),
            pltpu.VMEM((6, 32, 16 * DH), f32),
            pltpu.VMEM((2, 10, 1040, 128), u32),
            pltpu.VMEM((32, 128), f32),
            pltpu.VMEM((48, 128), f32),
            pltpu.VMEM((5, S // 4, DM), bf16),
            pltpu.VMEM((2, 8, DM // 2 + 1, 256), bf16),
            pltpu.VMEM((12872, 128), u32),
            pltpu.VMEM((137, 128, 128), f32),
            pltpu.VMEM((8, 128, 128), f32),
            pltpu.VMEM((12, 264, 128), f32),
            pltpu.VMEM((24, 64, 128), u32),
            pltpu.VMEM((64, 64, 128), u32),
            pltpu.VMEM((2, 512, 128), f32),
            pltpu.SMEM((64,), f32),
            pltpu.SMEM((1,), jnp.int32),
            pltpu.SemaphoreType.DMA((84,)),
            pltpu.SemaphoreType.DMA((2,)),
        ],
        compiler_params=pltpu.CompilerParams(vmem_limit_bytes=120 * 1024 * 1024,
                                             disable_semaphore_checks=True,
                                             disable_bounds_checks=True),
    )(x.reshape(S, DM), x.reshape(NSEG, SEG, DM), mem0.reshape(MEM, DM), wq, wk, wv,
      wo.reshape(H * DH // 16, 16, DM), bx.reshape(4, S // 4, DM), w_r.T, w_i.T, jnp.asarray(fd), jnp.asarray(ms), jnp.asarray(tv))
    return out.reshape(1, S, 2 * DM)


def pallas_concat_heads__memory_aug_recurrent_mem_tr__spectral_gfnet__prompt_kernel(
    A_x: jax.Array,
    A_mem0: jax.Array,
    A_Wq: jax.Array,
    A_Wk: jax.Array,
    A_Wv: jax.Array,
    A_Wo: jax.Array,
    A_seg_len,
    B_x: jax.Array,
    B_w_r: jax.Array,
    B_w_i: jax.Array,
):
    if isinstance(A_seg_len, int):
        assert A_seg_len == SEG
    assert A_x.shape == (1, S, DM) and A_mem0.shape == (1, MEM, DM) and A_Wq.shape == (DM, H, DH)
    assert B_x.shape == (1, S, DM) and B_w_r.shape == (S, DM // 2 + 1)
    return _run(A_x, A_mem0, A_Wq, A_Wk, A_Wv, A_Wo, B_x, B_w_r, B_w_i)
```
